```python
import jax
import jax.numpy as jnp

def _softmax(x, axis=-1):
    return jax.nn.softmax(x, axis=axis)

def _gelu(x):
    return jax.nn.gelu(x, approximate=True)

def _silu(x):
    return jax.nn.silu(x)

def _sigmoid(x):
    return jax.nn.sigmoid(x)

def _layernorm(x, axis=-1, eps=1e-05):
    m = jnp.mean(x, axis=axis, keepdims=True)
    v = jnp.var(x, axis=axis, keepdims=True)
    return (x - m) / jnp.sqrt(v + eps)

def _scatter_add(tgt, idx, src, axis=0):
    return tgt.at[idx].add(src)

def _segment_sum(src, seg, n):
    return jax.ops.segment_sum(src, seg, n)

class _Rng:

    def __init__(self, key):
        self._k = key

    def _next(self):
        self._k, sub = jax.random.split(self._k)
        return sub

    def normal(self, shape):
        return jax.random.normal(self._next(), shape, dtype=jnp.bfloat16)

    def randint(self, lo, hi, shape):
        return jax.random.randint(self._next(), shape, lo, hi, dtype=jnp.int32)

    def uniform(self, shape, lo=0.0, hi=1.0):
        return jax.random.uniform(self._next(), shape, jnp.bfloat16, lo, hi)

    def permutation(self, n):
        return jax.random.permutation(self._next(), n)
kernel_name = 'adaLN_cond__memory_aug_recurrent_mem_tr__mixer_s_mlp__prompt'

def setup_inputs():
    _rng = _Rng(jax.random.key(int.from_bytes(__import__("os").urandom(4), "little")))
    _w = lambda a: (lambda t: t.astype(jnp.bfloat16) if jnp.issubdtype(t.dtype, jnp.floating) else t)(jnp.asarray(a))

    def _A_setup():
        B, S, Dm = (1, 2048, 1024)
        H, Dh = (32, 128)
        M, seg = (8, 32)
        seg = min(seg, S)
        S = S // seg * seg
        return {'x': _w((lambda *s: _rng.normal(s) * 0.05)(B, S, Dm)), 'mem0': _w((lambda *s: _rng.normal(s) * 0.05)(B, M, Dm)), 'Wq': _w((lambda *s: _rng.normal(s) * 0.05)(Dm, H, Dh) * Dm ** (-0.5)), 'Wk': _w((lambda *s: _rng.normal(s) * 0.05)(Dm, H, Dh) * Dm ** (-0.5)), 'Wv': _w((lambda *s: _rng.normal(s) * 0.05)(Dm, H, Dh) * Dm ** (-0.5)), 'Wo': _w((lambda *s: _rng.normal(s) * 0.05)(H, Dh, Dm) * (H * Dh) ** (-0.5)), 'seg_len': seg}
    _A_in = _A_setup()

    def _B_setup():
        B, S, D, F = (1, 2048, 1024, 3584)
        return {'x': _w((lambda *s: _rng.normal(s) * 0.05)(B, S, D)), 'w1': _w((lambda *s: _rng.normal(s) * 0.05)(D, D) * D ** (-0.5)), 'w2': _w((lambda *s: _rng.normal(s) * 0.05)(D, D) * D ** (-0.5)), 'w3': _w((lambda *s: _rng.normal(s) * 0.05)(D, F) * D ** (-0.5)), 'w4': _w((lambda *s: _rng.normal(s) * 0.05)(F, D) * F ** (-0.5))}
    _B_in = _B_setup()
    return {'A_x': _A_in['x'], 'A_mem0': _A_in['mem0'], 'A_Wq': _A_in['Wq'], 'A_Wk': _A_in['Wk'], 'A_Wv': _A_in['Wv'], 'A_Wo': _A_in['Wo'], 'A_seg_len': _A_in['seg_len'], 'B_x': _B_in['x'], 'B_w1': _B_in['w1'], 'B_w2': _B_in['w2'], 'B_w3': _B_in['w3'], 'B_w4': _B_in['w4'], 'c': _w((lambda *s: _rng.normal(s) * 0.05)(1, 1024)), 'w_mod': _w((lambda *s: _rng.normal(s) * 0.05)(1024, 6 * 1024) * 1024 ** (-0.5))}

def reference(A_x, A_mem0, A_Wq, A_Wk, A_Wv, A_Wo, A_seg_len, B_x, B_w1, B_w2, B_w3, B_w4, c, w_mod):

    def _A_ref(x, mem0, Wq, Wk, Wv, Wo, seg_len):
        B, S, Dm = x.shape
        H, Dh = (Wq.shape[1], Wq.shape[2])
        M = mem0.shape[1]
        scale = Dh ** (-0.5)
        n_seg = S // seg_len
        L = M + seg_len
        idx = jnp.arange(L)
        mask = (idx[:, None] < M) | (idx[:, None] >= idx[None, :])
        mem = mem0
        outs = []
        for s in range(n_seg):
            xs = x[:, s * seg_len:(s + 1) * seg_len, :].copy()
            h = jnp.concatenate([mem, xs], axis=1)
            q = jnp.einsum('btd,dhe->bhte', h, Wq)
            k = jnp.einsum('btd,dhe->bhte', h, Wk)
            v = jnp.einsum('btd,dhe->bhte', h, Wv)
            scores = jnp.einsum('bhqe,bhke->bhqk', q, k) * scale
            scores = jnp.where(mask[None, None], scores, -1000000000.0)
            p = _softmax(scores, axis=-1)
            o = jnp.einsum('bhqk,bhke->bhqe', p, v)
            o = jnp.einsum('bhte,hed->btd', o, Wo)
            mem = o[:, :M, :].copy()
            outs.append(o[:, M:, :])
        return jnp.concatenate(outs, axis=1)

    def _B_ref(x, w1, w2, w3, w4):
        B, S, D = x.shape
        h = _gelu(_layernorm(x, axis=-1) @ w1)
        c = D // 4
        g0 = jnp.pad(h[:, :, 0 * c:1 * c], ((0, 0), (1, 0), (0, 0)))[:, :S, :]
        g1 = jnp.pad(h[:, :, 1 * c:2 * c], ((0, 0), (0, 1), (0, 0)))[:, 1:, :]
        g2 = jnp.pad(h[:, :, 2 * c:3 * c], ((0, 0), (2, 0), (0, 0)))[:, :S, :]
        g3 = jnp.pad(h[:, :, 3 * c:], ((0, 0), (0, 2), (0, 0)))[:, 2:, :]
        hs = jnp.concatenate([g0, g1, g2, g3], axis=-1) @ w2
        x1 = x + hs
        h2 = _gelu(_layernorm(x1, axis=-1) @ w3) @ w4
        return x1 + h2
    x = A_x
    mod = (_silu(c) @ w_mod).reshape(c.shape[0], 6, 1, -1)
    sa, ca, ga, sb, cb, gb = (mod[:, 0].copy(), mod[:, 1].copy(), mod[:, 2].copy(), mod[:, 3].copy(), mod[:, 4].copy(), mod[:, 5].copy())
    h = _layernorm(x, axis=-1) * (1 + ca) + sa
    x = x + ga * _A_ref(h, A_mem0, A_Wq, A_Wk, A_Wv, A_Wo, A_seg_len)
    h = _layernorm(x, axis=-1) * (1 + cb) + sb
    x = x + gb * _B_ref(h, B_w1, B_w2, B_w3, B_w4)
    return x
```

```python
import jax
import jax.numpy as jnp
from jax import lax
import jax.experimental.pallas as pl
import jax.experimental.pallas.tpu as pltpu

bf16 = jnp.bfloat16
f32 = jnp.float32
u32 = jnp.uint32

S = 2048
D = 1024
H = 32
DH = 128
F = 3584
MEM = 8
SEG = 32
NSEG = S // SEG
L = MEM + SEG
RIDE = 24
NPRE = S - RIDE * NSEG
NR = NPRE + SEG
ROFF = (-(S - NPRE)) % NR
WP = 520
NSLOT = 8
NPIECE = 24
EPS = 1e-5
MD = 128
MB = 512
GPAD = 8


def _blk(m, h):
    g, r = divmod(h, 16)
    return m * 32 + g * 16 + (r % 2) * 8 + r // 2


def _ln(x):
    mu = jnp.mean(x, axis=-1, keepdims=True)
    xc = x - mu
    var = jnp.mean(xc * xc, axis=-1, keepdims=True)
    return xc * lax.rsqrt(var + EPS)


def _gelu(x):
    inner = x * (0.7978845608028654 + (0.7978845608028654 * 0.044715) * (x * x))
    hx = 0.5 * x
    return hx + hx * jnp.tanh(inner)


def _kernel(x_hbm, mem0_ref, wq_hbm, wk_hbm, wv_hbm, wo_hbm, w1_hbm, w2_hbm, w3_hbm, w4_hbm,
            c_ref, wmod_hbm, out_hbm,
            xbuf, wqkv, wo, w1b, w2b, w3b, w4b, wmodb, stg, ring, hpre, lhs_h, lhs_o, modv,
            h2buf, gbuf, nbuf, ubuf,
            sem_x, sem_mod, sem_stg, sem_wo, sem_mlp, sem_out):
    w_hbms = (wq_hbm, wk_hbm, wv_hbm)

    def x_copy(i):
        return pltpu.make_async_copy(x_hbm.at[pl.ds(i * 512, 512), :],
                                     xbuf.at[pl.ds(i * 512, 512), :], sem_x.at[i])

    def mod_copy(j):
        return pltpu.make_async_copy(wmod_hbm.at[:, pl.ds(j * 512, 512)], wmodb.at[j],
                                     sem_mod.at[j])

    def piece_copy(m, g, qd, slot):
        return pltpu.make_async_copy(
            w_hbms[m].at[pl.ds(qd * 256, 256), pl.ds(g * 16, 16), :], stg.at[slot],
            sem_stg.at[slot])

    def piece_start_static(p):
        piece_copy(p // 8, (p // 4) % 2, p % 4, p % NSLOT).start()

    def piece_start_dyn(p):
        g = pl.multiple_of(((p // 4) % 2) * 16, 16)
        qd = pl.multiple_of((p % 4) * 256, 256)
        slot = p % NSLOT
        for m in range(3):
            @pl.when(p // 8 == m)
            def _():
                pltpu.make_async_copy(w_hbms[m].at[pl.ds(qd, 256), pl.ds(g, 16), :],
                                      stg.at[slot], sem_stg.at[slot]).start()

    def piece_wait(slot):
        piece_copy(0, 0, 0, slot).wait()

    def wo_copy(j):
        return pltpu.make_async_copy(wo_hbm.at[:, pl.ds(j * 128, 128)], wo.at[j], sem_wo.at[j])

    def mlp_copies():
        cps = []
        for j in range(2):
            cps.append(pltpu.make_async_copy(w1_hbm.at[:, pl.ds(j * 512, 512)], w1b.at[j],
                                             sem_mlp.at[j]))
        for j in range(2):
            cps.append(pltpu.make_async_copy(w2_hbm.at[:, pl.ds(j * 512, 512)], w2b.at[j],
                                             sem_mlp.at[2 + j]))
        for j in range(7):
            cps.append(pltpu.make_async_copy(w3_hbm.at[:, pl.ds(j * 512, 512)], w3b.at[j],
                                             sem_mlp.at[4 + j]))
        for j in range(2):
            cps.append(pltpu.make_async_copy(w4_hbm.at[:, pl.ds(j * 512, 512)], w4b.at[j],
                                             sem_mlp.at[11 + j]))
        return cps

    def out_copy(row, n):
        return pltpu.make_async_copy(xbuf.at[pl.ds(row, n), :], out_hbm.at[pl.ds(row, n), :],
                                     sem_out)

    def relayout(p, lo_dp, n_dp):
        slot = p % NSLOT
        base = (p // 4) * (16 * WP) + (p % 4) * 128
        for u in range(n_dp):
            dp = lo_dp + u
            a = pltpu.bitcast(stg[slot, 2 * dp], u32)
            b = pltpu.bitcast(stg[slot, 2 * dp + 1], u32)
            lo = (a & jnp.uint32(0xFFFF)) | (b << 16)
            hi = (a >> 16) | (b & jnp.uint32(0xFFFF0000))
            wqkv[pl.ds(base + dp, 8, stride=WP), :] = lo
            wqkv[pl.ds(base + dp + 8 * WP, 8, stride=WP), :] = hi

    def mod_chunks(js):
        cv = c_ref[...].astype(f32)
        sv = cv * (1.0 / (1.0 + jnp.exp(-cv)))
        sv = jnp.broadcast_to(sv, (16, D)).astype(bf16)
        for j in js:
            mod_copy(j).wait()
            y = jnp.dot(sv, wmodb[j], preferred_element_type=f32)
            modv[:, j * 512:(j + 1) * 512] = y[0:8]

    def modrow(k):
        return modv[0:1, k * D:(k + 1) * D]

    def adaln_a(xv):
        return _ln(xv) * (1.0 + modrow(1)) + modrow(0)

    def adaln_b(xv):
        return _ln(xv) * (1.0 + modrow(4)) + modrow(3)

    x_copy(0).start()
    for j in range(4):
        mod_copy(j).start()
    for p in range(NSLOT):
        piece_start_static(p)

    mod_chunks(range(4))
    x_copy(0).wait()

    def hpre_body(i, _):
        r = pl.multiple_of(i * 64, 64)
        hpre[pl.ds(r, 64), :] = adaln_a(xbuf[pl.ds(r, 64), :].astype(f32)).astype(bf16)
        return 0
    lax.fori_loop(0, NPRE // 64, hpre_body, 0)

    for p in range(4):
        piece_wait(p)

        def rl_body(t, _, p=p):
            relayout(p, t * 32, 32)
            return 0
        lax.fori_loop(0, 4, rl_body, 0)
        piece_start_static(p + NSLOT)
    for i in range(1, 4):
        x_copy(i).start()

    def pre_iter(it, with_relayout):
        if with_relayout:
            @pl.when(jnp.logical_and(it >= 1, it + 11 < NPIECE))
            def _():
                piece_start_dyn(it + 11)

            @pl.when(it < 8)
            def _():
                wo_copy(it).start()

            @pl.when(jnp.logical_and(it >= 8, it < 16))
            def _():
                mod_copy(it - 4).start()

            piece_wait((it + 4) % NSLOT)
        hv = hpre[...]
        for q in range(4):
            b = it * 4 + q
            w = pltpu.bitcast(wqkv[pl.ds(pl.multiple_of(b * WP, 8), 512), :], bf16)
            y = jnp.dot(hv, w, preferred_element_type=f32).astype(bf16)
            n0 = NR - ROFF
            ring[b, ROFF:NR, :] = y[0:n0]
            ring[b, 0:NPRE - n0, :] = y[n0:NPRE]
            if with_relayout:
                relayout(it + 4, q * 32, 32)
        return 0

    lax.fori_loop(0, NPIECE - 4, lambda it, _: pre_iter(it, True), 0)
    for cp in mlp_copies():
        cp.start()
    lax.fori_loop(NPIECE - 4, NPIECE, lambda it, _: pre_iter(it, False), 0)

    mod_chunks(range(4, 12))
    for i in range(1, 4):
        x_copy(i).wait()
    for j in range(8):
        wo_copy(j).wait()

    lhs_h[0:MEM, :] = mem0_ref[...]
    lhs_h[MEM:32, :] = adaln_a(xbuf[NPRE:NPRE + RIDE, :].astype(f32)).astype(bf16)

    row = lax.broadcasted_iota(jnp.int32, (L, L), 0)
    col = lax.broadcasted_iota(jnp.int32, (L, L), 1)
    mask = (row >= SEG) | (col >= SEG) | (row >= col)
    scale = DH ** -0.5
    DS, DP, GW = 3, 6, 4

    def step(s, _):
        seg = pl.multiple_of((SEG * s + ROFF) % NR, SEG)
        wr = [pl.multiple_of((NPRE + RIDE * s + 8 * t + ROFF) % NR, 8) for t in range(3)]
        rd = [pl.multiple_of((RIDE * s + 8 * t + ROFF) % NR, 8) for t in range(3)]
        lhs = lhs_h[...]
        QK, VM, V, P = {}, {}, {}, {}

        def qkv(h):
            ym = []
            for m in range(3):
                b = _blk(m, h)
                w = pltpu.bitcast(wqkv[b * WP:b * WP + 512, :], bf16)
                y = jnp.dot(lhs, w, preferred_element_type=f32)
                ym.append(y[0:MEM].astype(bf16))
                for t in range(3):
                    ring[b, pl.ds(wr[t], 8), :] = y[8 + 8 * t:16 + 8 * t].astype(bf16)
            q = jnp.concatenate([ring[_blk(0, h), pl.ds(seg, SEG), :], ym[0]], axis=0)
            k = jnp.concatenate([ring[_blk(1, h), pl.ds(seg, SEG), :], ym[1]], axis=0)
            QK[h] = (q, k)
            VM[h] = ym[2]

        def scores(h):
            q, k = QK.pop(h)
            sc = lax.dot_general(q, k, (((1,), (1,)), ((), ())), preferred_element_type=f32)
            sc = jnp.where(mask, sc * scale, -1e9)
            mx = jnp.max(sc, axis=-1, keepdims=True)
            e = jnp.exp(sc - mx)
            den = jnp.sum(e, axis=-1, keepdims=True)
            P[h] = (e * pl.reciprocal(den, approx=True)).astype(bf16)

        def loadv(h):
            V[h] = jnp.concatenate([ring[_blk(2, h), pl.ds(seg, SEG), :], VM.pop(h)], axis=0)

        def pv(h):
            o = jnp.dot(P.pop(h), V.pop(h), preferred_element_type=f32)
            b = _blk(0, h)
            ring[b, pl.ds(seg, SEG), :] = o[0:SEG].astype(bf16)
            lhs_o[h, 0:MEM, :] = o[SEG:L].astype(bf16)
            for t in range(3):
                lhs_o[h, 8 + 8 * t:16 + 8 * t, :] = ring[b, pl.ds(rd[t], 8), :]

        def wo_group(g, acc):
            lo = jnp.concatenate([lhs_o[h] for h in range(GW * g, GW * (g + 1))], axis=1)
            out = []
            for j in range(8):
                y = jnp.dot(lo, wo[j, DH * GW * g:DH * GW * (g + 1), :],
                            preferred_element_type=f32)
                out.append(y if acc is None else acc[j] + y)
            return out

        def side(t):
            if 0 <= t - DP + 2 < H:
                loadv(t - DP + 2)
            if 0 <= t - DS < H:
                scores(t - DS)
            if 0 <= t - DP < H:
                pv(t - DP)

        for h in range(H):
            qkv(h)
            side(h)
        acc = None
        t = H
        for g in range(H // GW):
            acc = wo_group(g, acc)
            if t < H + DP:
                side(t)
                t += 1
        a = jnp.concatenate(acc, axis=1)
        lhs_h[0:MEM, :] = a[0:MEM].astype(bf16)
        r1 = pl.multiple_of(jnp.minimum(NPRE + RIDE * (s + 1), S - RIDE), 8)
        hn = adaln_a(xbuf[pl.ds(r1, RIDE), :].astype(f32))
        r0 = pl.multiple_of(RIDE * s, 8)
        xa = xbuf[pl.ds(r0, RIDE), :].astype(f32) + modrow(2) * a[MEM:32]
        xbuf[pl.ds(r0, RIDE), :] = xa.astype(bf16)
        lhs_h[MEM:32, :] = hn.astype(bf16)
        return 0

    lax.fori_loop(0, NSEG, step, 0)

    def wo_tail(i, _):
        p0 = pl.multiple_of(i * 128, 128)
        lo = jnp.concatenate([ring[_blk(0, h), pl.ds(p0, 128), :] for h in range(H)], axis=1)
        r = pl.multiple_of(S - NPRE + i * 128, 128)
        for j in range(8):
            y = jnp.dot(lo, wo[j], preferred_element_type=f32)
            cs = slice(j * 128, (j + 1) * 128)
            xa = xbuf[pl.ds(r, 128), cs].astype(f32) + modv[0:1, 2 * D + j * 128:2 * D + (j + 1) * 128] * y
            xbuf[pl.ds(r, 128), cs] = xa.astype(bf16)
        return 0
    lax.fori_loop(0, NPRE // 128, wo_tail, 0)

    for cp in mlp_copies():
        cp.wait()

    zpad = jnp.zeros((GPAD, 128), f32)
    for cb in range(8):
        gbuf[cb, 0:GPAD, :] = zpad
        gbuf[cb, GPAD + S:GPAD + S + GPAD, :] = zpad

    HB = MB // 2

    def stage_a(r, half):
        for k in range(HB // 64):
            rr = pl.multiple_of(r + k * 64, 64)
            h2 = adaln_b(xbuf[pl.ds(rr, 64), :].astype(f32))
            h2buf[pl.ds(rr, 64), :] = h2
            nbuf[half * HB + k * 64:half * HB + (k + 1) * 64, :] = _ln(h2).astype(bf16)

    def stage_b(r, half):
        nv = nbuf[half * HB:(half + 1) * HB, :]
        for j in range(2):
            y = _gelu(jnp.dot(nv, w1b[j], preferred_element_type=f32))
            for q in range(4):
                gbuf[4 * j + q, pl.ds(pl.multiple_of(GPAD + r, 8), HB), :] = y[:, q * 128:(q + 1) * 128]

    stage_a(0, 0)

    def ab_body(i, _):
        r = pl.multiple_of(i * MB, MB)
        stage_a(r + HB, 1)
        stage_b(r, 0)
        stage_a(jnp.minimum(r + MB, S - HB), 0)
        stage_b(r + HB, 1)
        return 0
    lax.fori_loop(0, S // MB, ab_body, 0)

    shifts = (-1, -1, 1, 1, -2, -2, 2, 2)

    def stage_shift(r, half):
        for cb in range(8):
            blkv = gbuf[cb, pl.ds(pl.multiple_of(r, 8), HB + 2 * GPAD), :]
            o = GPAD + shifts[cb]
            nbuf[half * HB:(half + 1) * HB, cb * 128:(cb + 1) * 128] = blkv[o:o + HB].astype(bf16)

    def stage_c(r, half):
        nv = nbuf[half * HB:(half + 1) * HB, :]
        rr = pl.multiple_of(r, 8)
        for j in range(2):
            y = jnp.dot(nv, w2b[j], preferred_element_type=f32)
            cs = slice(j * 512, (j + 1) * 512)
            h2buf[pl.ds(rr, HB), cs] = h2buf[pl.ds(rr, HB), cs] + y

    stage_shift(0, 0)

    def c_body(i, _):
        r = pl.multiple_of(i * MB, MB)
        stage_shift(r + HB, 1)
        stage_c(r, 0)
        stage_shift(jnp.minimum(r + MB, S - HB), 0)
        stage_c(r + HB, 1)
        return 0
    lax.fori_loop(0, S // MB, c_body, 0)

    def stage_n2(r):
        for k in range(MD // 64):
            rr = pl.multiple_of(r + k * 64, 64)
            nbuf[k * 64:(k + 1) * 64, :] = _ln(h2buf[pl.ds(rr, 64), :]).astype(bf16)

    stage_n2(0)

    def d_body(i, _):
        r = pl.multiple_of(i * MD, MD)
        nv = nbuf[0:MD, :]
        for j in range(7):
            u = _gelu(jnp.dot(nv, w3b[j], preferred_element_type=f32))
            ubuf[:, j * 512:(j + 1) * 512] = u.astype(bf16)
        stage_n2(jnp.minimum(r + MD, S - MD))
        uv = ubuf[...]
        for j in range(2):
            y = jnp.dot(uv, w4b[j], preferred_element_type=f32)
            cs = slice(j * 512, (j + 1) * 512)
            bo = h2buf[pl.ds(r, MD), cs] + y
            o = xbuf[pl.ds(r, MD), cs].astype(f32) + modv[0:1, 5 * D + j * 512:5 * D + (j + 1) * 512] * bo
            xbuf[pl.ds(r, MD), cs] = o.astype(bf16)
        out_copy(r, MD).start()
        return 0
    lax.fori_loop(0, S // MD, d_body, 0)

    out_copy(0, S).wait()


def _run(x, mem0, wq, wk, wv, wo, w1, w2, w3, w4, c, wmod):
    any_spec = pl.BlockSpec(memory_space=pl.ANY)
    vmem_spec = pl.BlockSpec(memory_space=pltpu.VMEM)
    return pl.pallas_call(
        _kernel,
        out_shape=jax.ShapeDtypeStruct((S, D), bf16),
        in_specs=[any_spec, vmem_spec, any_spec, any_spec, any_spec, any_spec, any_spec,
                  any_spec, any_spec, any_spec, vmem_spec, any_spec],
        out_specs=any_spec,
        scratch_shapes=[
            pltpu.VMEM((S, D), bf16),
            pltpu.VMEM((96 * WP, 128), u32),
            pltpu.VMEM((8, H * DH, 128), bf16),
            pltpu.VMEM((2, D, 512), bf16),
            pltpu.VMEM((2, D, 512), bf16),
            pltpu.VMEM((7, D, 512), bf16),
            pltpu.VMEM((2, F, 512), bf16),
            pltpu.VMEM((12, D, 512), bf16),
            pltpu.VMEM((NSLOT, 256, 16, 128), bf16),
            pltpu.VMEM((96, NR, 128), bf16),
            pltpu.VMEM((NPRE, D), bf16),
            pltpu.VMEM((32, D), bf16),
            pltpu.VMEM((H, 32, 128), bf16),
            pltpu.VMEM((8, 6 * D), f32),
            pltpu.VMEM((S, D), f32),
            pltpu.VMEM((8, S + 2 * GPAD, 128), f32),
            pltpu.VMEM((MB, D), bf16),
            pltpu.VMEM((MD, F), bf16),
            pltpu.SemaphoreType.DMA((4,)),
            pltpu.SemaphoreType.DMA((12,)),
            pltpu.SemaphoreType.DMA((NSLOT,)),
            pltpu.SemaphoreType.DMA((8,)),
            pltpu.SemaphoreType.DMA((13,)),
            pltpu.SemaphoreType.DMA(()),
        ],
        compiler_params=pltpu.CompilerParams(vmem_limit_bytes=124 * 1024 * 1024),
    )(x, mem0, wq, wk, wv, wo, w1, w2, w3, w4, c, wmod)


def pallas_adaLN_cond__memory_aug_recurrent_mem_tr__mixer_s_mlp__prompt_kernel(
    A_x, A_mem0, A_Wq, A_Wk, A_Wv, A_Wo, A_seg_len, B_x, B_w1, B_w2, B_w3, B_w4, c, w_mod,
):
    del B_x
    assert A_x.shape == (1, S, D) and A_mem0.shape == (1, MEM, D)
    assert isinstance(A_seg_len, int) is False or A_seg_len == SEG
    out = _run(A_x.reshape(S, D), A_mem0.reshape(MEM, D), A_Wq, A_Wk, A_Wv,
               A_Wo.reshape(H * DH, D), B_w1, B_w2, B_w3, B_w4, c, w_mod)
    return out.reshape(1, S, D)
```

```python
import jax
import jax.numpy as jnp
from jax import lax
import jax.experimental.pallas as pl
import jax.experimental.pallas.tpu as pltpu

bf16 = jnp.bfloat16
f32 = jnp.float32
u32 = jnp.uint32

S = 2048
D = 1024
H = 32
DH = 128
F = 3584
MEM = 8
SEG = 32
NSEG = S // SEG
L = MEM + SEG
RIDE = 24
NPRE = S - RIDE * NSEG
NR = NPRE + 2 * SEG
ROFF = (-(S - NPRE)) % NR
WP = 520
NGRP = 12
NSLOT = 6
NMOD = 6
EPS = 1e-5
MD = 128
MB = 512
GPAD = 8
NRING = 8
NP = 1
DS, DP, GW, WT, KSPLIT = 2, 4, 4, 1, 2
W1, W2, W3, W4 = 0, 4 * 512, 8 * 512, 22 * 512
WROWS = W4 + 4 * (F // 2)
T0 = 8
WCH = WROWS // (NSEG // 2 - T0)
_ONLY = None


def _loop(name, lo, hi, body):
    if _ONLY is not None and name not in _ONLY:
        return
    with _scope(name):
        lax.fori_loop(lo, hi, body, 0)


class _NoScope:
    def __init__(self, name):
        del name

    def __enter__(self):
        return self

    def __exit__(self, *a):
        return False


_scope = _NoScope


def _blk(m, h):
    g, r = divmod(h, 8)
    return m * 32 + g * 8 + (r % 2) * 4 + r // 2


_HEAD = sorted(range(H), key=lambda h: _blk(0, h))


def _ln(x):
    mu = jnp.mean(x, axis=-1, keepdims=True)
    xc = x - mu
    var = jnp.mean(xc * xc, axis=-1, keepdims=True)
    return xc * lax.rsqrt(var + EPS)


def _gelu(x):
    inner = x * (0.7978845608028654 + (0.7978845608028654 * 0.044715) * (x * x))
    hx = 0.5 * x
    return hx + hx * jnp.tanh(inner)


def _split_rows(x):
    m, n = x.shape
    x3 = x.reshape(m // 16, 16, n)
    return x3[:, 0:8, :].reshape(m // 2, n), x3[:, 8:16, :].reshape(m // 2, n)


def _merge_rows(top, bot):
    m, n = top.shape
    return jnp.concatenate([top.reshape(m // 8, 8, n), bot.reshape(m // 8, 8, n)],
                           axis=1).reshape(2 * m, n)


def _a_operands(a11, a12, a21, a22):
    return [a11 + a22, a21 + a22, a11, a22, a11 + a12, a21 - a11, a12 - a22]


def _b_operands(b11, b12, b21, b22):
    return [b11 + b22, b11, b12 - b22, b21 - b11, b22, b11 + b12, b21 + b22]


_BSLOT = (4, 0, 1, 2, 3, 5, 6)


def _strassen(a_of, b_of):
    def prod(k):
        return jnp.dot(a_of(k), b_of(k), preferred_element_type=f32)
    p5 = prod(4)
    p3 = prod(2)
    c12 = p3 + p5
    p1 = prod(0)
    c11 = p1 - p5
    c22 = p1 + p3
    p4 = prod(3)
    c11 = c11 + p4
    c11 = prod(6) + c11
    p2 = prod(1)
    c21 = p2 + p4
    c22 = c22 - p2
    c22 = prod(5) + c22
    return c11, c12, c21, c22


def _kernel(x_hbm, mem0_ref, wq_hbm, wk_hbm, wv_hbm, wo_hbm, w1_hbm, w2_hbm, w3_hbm, w4_hbm,
            c_ref, wmod_hbm, out_hbm,
            xbuf, wo, w7, wmodb, rings, lhs_h, lhs_o, kvm, modv, h2buf, n7,
            sem_x, sem_mod, sem_stg, sem_wo, sem_mlp, sem_out):
    w_hbms = (wq_hbm, wk_hbm, wv_hbm)

    def rget(b, row, n):
        return rings[b % NRING][b // NRING, pl.ds(row, n), :]

    def rset(b, row, val):
        rings[b % NRING][b // NRING, pl.ds(row, val.shape[0]), :] = val.astype(bf16)

    def x_copy(i):
        return pltpu.make_async_copy(x_hbm.at[pl.ds(i * 512, 512), :],
                                     xbuf.at[pl.ds(i * 512, 512), :], sem_x.at[i])

    def mod_copy(j):
        return pltpu.make_async_copy(wmod_hbm.at[:, pl.ds(j * 512, 512)], wmodb.at[j % NMOD],
                                     sem_mod.at[j % NMOD])

    def wo_copy(j):
        return pltpu.make_async_copy(wo_hbm.at[:, pl.ds(j * 128, 128)], wo.at[j], sem_wo)

    def mlp_copies():
        cps = []
        for src, base, kh, npair in ((w1_hbm, W1, 512, 4), (w2_hbm, W2, 512, 4),
                                     (w3_hbm, W3, 512, 14), (w4_hbm, W4, F // 2, 4)):
            for j in range(npair):
                for quad in range(4):
                    cps.append(pltpu.make_async_copy(
                        src.at[pl.ds((quad // 2) * kh, kh),
                               pl.ds(((quad % 2) * npair + j) * 128, 128)],
                        w7.at[quad, pl.ds(base + j * kh, kh), :], sem_mlp))
        return cps

    def mlp_wait():
        done = w7.at[pl.ds(0, 4), pl.ds(0, WROWS), :]
        pltpu.make_async_copy(done, done, sem_mlp).wait()

    def out_copy(row, n):
        return pltpu.make_async_copy(xbuf.at[pl.ds(row, n), :], out_hbm.at[pl.ds(row, n), :],
                                     sem_out)

    def mod_chunks(js, wait_each):
        cv = c_ref[...].astype(f32)
        sv = cv * (1.0 / (1.0 + jnp.exp(-cv)))
        sv = jnp.broadcast_to(sv, (16, D)).astype(bf16)
        if not wait_each:
            for j in js:
                mod_copy(j).wait()
        for j in js:
            if wait_each:
                mod_copy(j).wait()
            y = jnp.dot(sv, wmodb[j % NMOD], preferred_element_type=f32)
            modv[:, j * 512:(j + 1) * 512] = y[0:8]

    def modrow(k):
        return modv[0:1, k * D:(k + 1) * D]

    def adaln_a(xv):
        return _ln(xv) * (1.0 + modrow(1)) + modrow(0)

    def adaln_b(xv):
        return _ln(xv) * (1.0 + modrow(4)) + modrow(3)

    def row_operands(v):
        top, bot = _split_rows(v)
        k = v.shape[1] // 2
        return _a_operands(top[:, :k], top[:, k:], bot[:, :k], bot[:, k:])

    def stage_a(r, n):
        for k in range(n // 16):
            rr = pl.multiple_of(r + k * 16, 16)
            h2 = adaln_b(xbuf[pl.ds(rr, 16), :].astype(f32))
            h2buf[pl.ds(rr, 16), :] = h2
            ro = pl.multiple_of(rr // 2, 8)
            for t, op in enumerate(row_operands(_ln(h2))):
                n7[t, pl.ds(ro, 8), :] = op.astype(bf16)

    def phase1(wqkv, stg, bs):
        def piece_copies(g, dh):
            slot = (2 * g + dh) % NSLOT
            return [pltpu.make_async_copy(
                w_hbms[g // 4].at[pl.ds(dh * 256, 256), par, pl.ds((g % 4) * 8, 8), :],
                stg.at[slot, :, pl.ds(par * 8, 8), :], sem_stg.at[slot]) for par in range(2)]

        def group_start(g):
            for dh in range(2):
                for cp in piece_copies(g, dh):
                    cp.start()

        def piece_wait(slot):
            pltpu.make_async_copy(stg.at[slot], stg.at[slot], sem_stg.at[slot]).wait()

        sub = lax.broadcasted_iota(jnp.int32, (8, 128), 0) < 4
        keep = jnp.where(sub, jnp.uint32(0xFFFF), jnp.uint32(0xFFFF0000))
        shl = jnp.where(sub, jnp.uint32(16), jnp.uint32(0))
        shr = jnp.where(sub, jnp.uint32(0), jnp.uint32(16))

        def relayout(g, dh, lo_dp, n_dp):
            slot = (2 * g + dh) % NSLOT
            base = g * (8 * WP) + dh * 256
            for u in range(n_dp):
                dp = lo_dp + u
                a = pltpu.bitcast(stg[slot, dp], u32)
                b = pltpu.roll(a, 4, 0)
                wqkv[pl.ds(base + dp, 8, stride=WP), :] = (a & keep) | ((b << shl) >> shr)

        def b_prep(g, q):
            for c in range(4):
                quad = []
                for dh in range(2):
                    for blk in (q, q + 4):
                        r = pl.multiple_of((g * 8 + blk) * WP + dh * 256 + c * 64, 8)
                        quad.append(pltpu.bitcast(wqkv[pl.ds(r, 64), :], bf16).astype(f32))
                for t, op in enumerate(_b_operands(*quad)):
                    bs[q % 2, t, c * 64:(c + 1) * 64, :] = pltpu.bitcast(op.astype(bf16), u32)

        x_copy(0).start()
        group_start(0)
        for j in (0, 2, 1, 3):
            mod_copy(j).start()
        x_copy(0).wait()

        def ln0_body(i, _):
            r = pl.multiple_of(i * 64, 64)
            h2buf[pl.ds(r, 64), :] = _ln(xbuf[pl.ds(r, 64), :].astype(f32))
            return 0
        lax.fori_loop(0, NPRE // 64, ln0_body, 0)

        for dh in range(2):
            piece_wait(dh)

            def rl_body(t, _, dh=dh):
                relayout(0, dh, t * 32, 32)
                return 0
            lax.fori_loop(0, 8, rl_body, 0)
        b_prep(0, 0)
        group_start(1)
        with _scope("mod0"):
            mod_chunks((0, 2, 1, 3), True)
        group_start(2)

        def hpre_body(i, _):
            r = pl.multiple_of(i * 32, 32)
            hv = h2buf[pl.ds(r, 32), :] * (1.0 + modrow(1)) + modrow(0)
            ro = pl.multiple_of(i * 16, 16)
            for t, op in enumerate(row_operands(hv)):
                n7[t, pl.ds(ro, 16), :] = op.astype(bf16)
            return 0
        lax.fori_loop(0, NPRE // 32, hpre_body, 0)

        extra = {0: [wo_copy(0)], 1: [wo_copy(1), mod_copy(4)], 2: [wo_copy(2)],
                 3: [wo_copy(3), mod_copy(5)], 4: [wo_copy(4)], 5: [wo_copy(5), mod_copy(6)],
                 6: [wo_copy(6)], 7: [wo_copy(7), mod_copy(7)], 8: [x_copy(1)],
                 9: [mod_copy(8), mod_copy(9)]}

        def pre_iter(g, last):
            if not last:
                for k in range(NGRP - 1):
                    @pl.when(g == k)
                    def _():
                        if k + 3 < NGRP:
                            group_start(k + 3)
                        for cp in extra.get(k, []):
                            cp.start()
                piece_wait((2 * g + 2) % NSLOT)
                piece_wait((2 * g + 3) % NSLOT)
            n0 = NR - ROFF
            for q in range(4):
                if q < 3:
                    b_prep(g, q + 1)
                if not last:
                    if q < 2:
                        relayout(g + 1, q, 0, 256)
                    if q == 3:
                        b_prep(g + 1, 0)
                c11, c12, c21, c22 = _strassen(
                    lambda k: n7[k, 0:NPRE // 2, :],
                    lambda k: pltpu.bitcast(bs[q % 2, k], bf16))
                for blk, y in ((q, _merge_rows(c11, c21)), (q + 4, _merge_rows(c12, c22))):
                    y = y.astype(bf16)
                    rings[blk][g, ROFF:NR, :] = y[0:n0]
                    rings[blk][g, 0:NPRE - n0, :] = y[n0:NPRE]
            return 0

        _loop("pre1", 0, NGRP - 1, lambda g, _: pre_iter(g, False))
        _loop("pre2", NGRP - 1, NGRP, lambda g, _: pre_iter(g, True))

        with _scope("mod1"):
            mod_chunks(range(4, 10), False)
        x_copy(1).wait()
        pltpu.make_async_copy(wo, wo, sem_wo).wait()
        lhs_h[0:MEM, :] = mem0_ref[...]
        lhs_h[MEM:32, :] = adaln_a(xbuf[NPRE:NPRE + RIDE, :].astype(f32)).astype(bf16)
        for t in range(4):
            w7[t, WROWS:WROWS + WCH, :] = jnp.zeros((WCH, 128), bf16)

        scale = DH ** -0.5
        ia = lax.broadcasted_iota(jnp.int32, (32, L), 0)
        ja = lax.broadcasted_iota(jnp.int32, (32, L), 1)
        mask_a = (ia >= RIDE) | (ja >= SEG) | (ia + 8 >= ja)
        ib = lax.broadcasted_iota(jnp.int32, (48, 56), 0)
        jb = lax.broadcasted_iota(jnp.int32, (48, 56), 1)
        own = (ib < 40) == (jb < 40)
        mask_b = own & (((jb >= 32) & (jb < 48)) | (jnp.where(jb < 40, jb, jb - 8) <= ib))
        masked = -1e9 / scale
        j8 = lax.broadcasted_iota(jnp.int32, (8, 56), 1)
        fill_b = jnp.concatenate([jnp.where(j8 < 40, masked, -3e38).astype(f32)] * 5
                                 + [jnp.where(j8 < 40, -3e38, masked).astype(f32)], axis=0)

        def softmax(sc, mask, fill):
            sc = jnp.where(mask, sc, fill)
            mx = jnp.max(sc, axis=-1, keepdims=True)
            e = jnp.exp2((sc - mx) * (scale * 1.4426950408889634))
            den = jnp.sum(e, axis=-1, keepdims=True)
            return (e * pl.reciprocal(den, approx=True)).astype(bf16)

        def ride_rows(s, is_b):
            first = s < 2
            if is_b:
                g = [jnp.where(first, -3, -1), 1, 2]
            else:
                g = [jnp.where(first, 1, 0), jnp.where(first, 2, 1), 3]
            return [RIDE * s + 8 * t for t in g]

        def step(s, is_b, lhs_lo, lhs_hi, soft_in):
            seg = pl.multiple_of((SEG * s + ROFF) % NR, SEG)
            sega = pl.multiple_of(seg - SEG, SEG) if is_b else seg
            wr = [pl.multiple_of((NPRE + RIDE * s + 8 * t + ROFF) % NR, 8) for t in range(3)]
            rd = [pl.multiple_of((r + ROFF) % NR, 8) for r in ride_rows(s, is_b)]
            lhs = jnp.concatenate([lhs_lo, lhs_hi], axis=1)
            QM, P, PART = {}, {}, {}
            mrow = 0 if is_b else MEM
            seg8 = pl.multiple_of(seg + 8, 8)
            seg24 = pl.multiple_of(seg + RIDE, 8)

            def wblk(b, lo, n):
                return pltpu.bitcast(wqkv[b * WP + lo:b * WP + lo + n, :], bf16)

            def qkv_lo(i):
                for m in range(3):
                    PART[(m, i)] = jnp.dot(lhs_lo, wblk(m * H + i, 0, 256), preferred_element_type=f32)

            def qkv(i):
                for m in range(3):
                    b = m * H + i
                    if (m, i) in PART:
                        y = jnp.dot(lhs_hi, wblk(b, 256, 256),
                                    preferred_element_type=f32) + PART.pop((m, i))
                    else:
                        y = jnp.dot(lhs, wblk(b, 0, 512), preferred_element_type=f32)
                    if m < 2:
                        QM[b] = y[0:MEM]
                    if m == 2 or (m == 1 and not is_b):
                        kvm[b - H, mrow:mrow + MEM, :] = y[0:MEM].astype(bf16)
                    for t in range(3):
                        rset(b, wr[t], y[8 + 8 * t:16 + 8 * t])

            def keys(b):
                if is_b:
                    if b in QM:
                        old = kvm[b - H, MEM:2 * MEM, :].astype(f32)
                        mix = jnp.concatenate([QM.pop(b), old], axis=0).astype(bf16)
                    else:
                        mix = kvm[b - H]
                    return jnp.concatenate([rget(b, seg, SEG), mix, rget(b, sega, 8)], axis=0)
                mk = QM.pop(b).astype(bf16) if b in QM else kvm[b - H, MEM:2 * MEM, :]
                return jnp.concatenate([rget(b, seg, SEG), mk], axis=0)

            def scores(i):
                if is_b:
                    mix = jnp.concatenate([QM.pop(i), rget(i, sega, 8).astype(f32)], axis=0)
                    q = jnp.concatenate([rget(i, seg, SEG), mix.astype(bf16)], axis=0)
                else:
                    mix = jnp.concatenate([rget(i, seg24, 8).astype(f32), QM.pop(i)], axis=0)
                    q = jnp.concatenate([rget(i, seg8, 16), mix.astype(bf16)], axis=0)
                sc = lax.dot_general(q, keys(H + i), (((1,), (1,)), ((), ())),
                                     preferred_element_type=f32)
                P[i] = softmax(sc, mask_b, fill_b) if is_b else softmax(sc, mask_a, masked)

            def pv(i):
                o = jnp.dot(P.pop(i), keys(2 * H + i), preferred_element_type=f32)
                if is_b:
                    rset(i, seg, o[0:SEG])
                    rset(i, sega, o[40:48])
                    lhs_o[i, 0:MEM, :] = o[SEG:L].astype(bf16)
                else:
                    rset(i, seg8, o[0:16])
                    rset(i, seg24, o[16:RIDE])
                    lhs_o[i, 0:MEM, :] = o[RIDE:32].astype(bf16)
                for t in range(3):
                    lhs_o[i, 8 + 8 * t:16 + 8 * t, :] = rget(i, rd[t], 8)

            def wo_group(i0, i1, acc):
                lo = jnp.concatenate([lhs_o[i] for i in range(i0, i1)], axis=1)
                out = []
                for j in range(8):
                    w = jnp.concatenate([wo[j, DH * _HEAD[i]:DH * (_HEAD[i] + 1), :]
                                         for i in range(i0, i1)], axis=0)
                    y = jnp.dot(lo, w, preferred_element_type=f32)
                    out.append(y if acc is None else y + acc[j])
                return out

            def side(t):
                if 0 <= t - DP < H:
                    pv(t - DP)
                if 0 <= t - DS < H:
                    scores(t - DS)

            if soft_in:
                for h in range(KSPLIT):
                    qkv_lo(h)
            for h in range(H):
                qkv(h)
                side(h)
            acc = None
            t = H
            bounds = list(range(0, H - 2 * GW + 1, GW)) + [H]
            for h0, h1 in zip(bounds[:-1], bounds[1:]):
                acc = wo_group(h0, h1, acc)
                for _ in range(WT):
                    side(t)
                    t += 1
            assert not (QM or P or PART)
            return jnp.concatenate(acc[0:4], axis=1), jnp.concatenate(acc[4:8], axis=1)

        def combine_weights(pair):
            r0 = jnp.where(pair < T0, WROWS, (pair - T0) * WCH)
            for c in range(WCH // 64):
                r = pl.multiple_of(r0 + c * 64, 64)
                ops = _b_operands(*[w7[t, pl.ds(r, 64), :].astype(f32) for t in range(4)])
                for k in (0, 2, 3, 5, 6):
                    w7[_BSLOT[k], pl.ds(r, 64), :] = ops[k].astype(bf16)

        def rec_body(it, _):
            @pl.when(it == 1)
            def _():
                for i in (2, 3):
                    x_copy(i).start()
                for cp in mlp_copies():
                    cp.start()
                for j in (10, 11):
                    mod_copy(j).start()

            @pl.when(it == T0 // NP)
            def _():
                for i in (2, 3):
                    x_copy(i).wait()
                mlp_wait()

            lhs_lo = lhs_h[:, 0:512]
            lhs_hi = lhs_h[:, 512:1024]
            stage_a(jnp.maximum(it - 1, 0) * (2 * RIDE * NP), 2 * RIDE * NP)
            for u in range(2 * NP):
                s = it * (2 * NP) + u
                if u % 2 == 0:
                    combine_weights(it * NP + u // 2)
                r1 = pl.multiple_of(jnp.minimum(NPRE + RIDE * (s + 1), S - RIDE), 8)
                hn = adaln_a(xbuf[pl.ds(r1, RIDE), :].astype(f32))
                a_lo, a_hi = step(s, u % 2 == 1, lhs_lo, lhs_hi, u > 0)
                lhs_lo = jnp.concatenate([a_lo[0:MEM], hn[:, 0:512]], axis=0).astype(bf16)
                lhs_hi = jnp.concatenate([a_hi[0:MEM], hn[:, 512:1024]], axis=0).astype(bf16)
                a = jnp.concatenate([a_lo, a_hi], axis=1)
                for t, r in enumerate(ride_rows(s, u % 2 == 1)):
                    r0 = pl.multiple_of(r, 8)
                    xa = (xbuf[pl.ds(r0, 8), :].astype(f32)
                          + modv[:, 2 * D:3 * D] * a[8 + 8 * t:16 + 8 * t])
                    xbuf[pl.ds(r0, 8), :] = xa.astype(bf16)
            lhs_h[:, 0:512] = lhs_lo
            lhs_h[:, 512:1024] = lhs_hi
            return 0

        _loop("rec", 0, NSEG // (2 * NP), rec_body)

    pl.run_scoped(phase1,
                  pltpu.VMEM((96 * WP, 128), u32),
                  pltpu.VMEM((NSLOT, 256, 16, 128), bf16),
                  pltpu.VMEM((2, 7, 256, 128), u32))

    def wo_tail(i, _):
        p0 = pl.multiple_of(i * 128, 128)
        r = pl.multiple_of(S - NPRE + i * 128, 128)
        stage_a(r - 128, 128)
        lo = jnp.concatenate([rget(_blk(0, h), p0, 128) for h in range(H)], axis=1)
        for j in range(8):
            y = jnp.dot(lo, wo[j], preferred_element_type=f32)
            cs = slice(j * 128, (j + 1) * 128)
            ga = modv[0:1, 2 * D + j * 128:2 * D + (j + 1) * 128]
            xbuf[pl.ds(r, 128), cs] = (xbuf[pl.ds(r, 128), cs].astype(f32) + ga * y).astype(bf16)
        return 0
    _loop("wotail", 0, NPRE // 128, wo_tail)
    mod_chunks((10, 11), False)
    stage_a(S - 128, 128)

    def phase2(gbuf, c7, d7, u7):
        def wop(base, kh, j):
            return lambda k: w7[_BSLOT[k], base + j * kh:base + (j + 1) * kh, :]

        zpad = jnp.zeros((GPAD, 128), f32)
        for cb in range(8):
            gbuf[cb, 0:GPAD, :] = zpad
            gbuf[cb, GPAD + S:GPAD + S + GPAD, :] = zpad

        def b_body(i, _):
            ro = pl.multiple_of(i * (MB // 2), MB // 2)
            rg = pl.multiple_of(GPAD + i * MB, 8)
            for j in range(4):
                c11, c12, c21, c22 = _strassen(lambda k: n7[k, pl.ds(ro, MB // 2), :],
                                               wop(W1, 512, j))
                gbuf[j + 4, pl.ds(rg, MB), :] = _gelu(_merge_rows(c12, c22))
                gbuf[j, pl.ds(rg, MB), :] = _gelu(_merge_rows(c11, c21))
            return 0
        _loop("b", 0, S // MB, b_body)

        shifts = (-1, -1, 1, 1, -2, -2, 2, 2)
        HB = MB // 2

        def stage_shift(r, half):
            for cb in range(4):
                for k in range(HB // 64):
                    rr = pl.multiple_of(r + k * 64, 8)
                    quad = []
                    for c in (cb, cb + 4):
                        o = GPAD + shifts[c]
                        quad.append(_split_rows(gbuf[c, pl.ds(rr, 64 + 2 * GPAD), :][o:o + 64]))
                    ops = _a_operands(quad[0][0], quad[1][0], quad[0][1], quad[1][1])
                    for t, op in enumerate(ops):
                        c7[half, t, k * 16:(k + 1) * 16, cb * 128:(cb + 1) * 128] = (
                            pltpu.bitcast(op.astype(bf16), u32))

        def stage_c(r, half):
            rr = pl.multiple_of(r, 8)
            for j in range(4):
                c11, c12, c21, c22 = _strassen(lambda k: pltpu.bitcast(c7[half, k], bf16),
                                               wop(W2, 512, j))
                for c, y in ((j + 4, _merge_rows(c12, c22)), (j, _merge_rows(c11, c21))):
                    cs = slice(c * 128, (c + 1) * 128)
                    h2buf[pl.ds(rr, HB), cs] = h2buf[pl.ds(rr, HB), cs] + y

        stage_shift(0, 0)

        def c_body(i, _):
            r = pl.multiple_of(i * MB, MB)
            stage_shift(r + HB, 1)
            stage_c(r, 0)
            stage_shift(jnp.minimum(r + MB, S - HB), 0)
            stage_c(r + HB, 1)
            return 0
        _loop("c", 0, S // MB, c_body)

        def stage_n2(r):
            for k in range(MD // 32):
                rr = pl.multiple_of(r + k * 32, 32)
                for t, op in enumerate(row_operands(_ln(h2buf[pl.ds(rr, 32), :]))):
                    d7[t, k * 8:(k + 1) * 8, :] = pltpu.bitcast(op.astype(bf16), u32)

        stage_n2(0)

        def d_body(i, _):
            r = pl.multiple_of(i * MD, MD)
            for j in range(14):
                cq = _strassen(lambda k: pltpu.bitcast(d7[k], bf16), wop(W3, 512, j))
                for t, op in enumerate(_a_operands(*[_gelu(c) for c in cq])):
                    u7[t, :, j * 128:(j + 1) * 128] = pltpu.bitcast(op.astype(bf16), u32)
            stage_n2(jnp.minimum(r + MD, S - MD))
            for j in range(4):
                c11, c12, c21, c22 = _strassen(lambda k: pltpu.bitcast(u7[k], bf16),
                                               wop(W4, F // 2, j))
                for c, y in ((j + 4, _merge_rows(c12, c22)), (j, _merge_rows(c11, c21))):
                    cs = slice(c * 128, (c + 1) * 128)
                    gb = modv[0:1, 5 * D + c * 128:5 * D + (c + 1) * 128]
                    o = xbuf[pl.ds(r, MD), cs].astype(f32) + gb * (h2buf[pl.ds(r, MD), cs] + y)
                    xbuf[pl.ds(r, MD), cs] = o.astype(bf16)
            out_copy(r, MD).start()
            return 0
        _loop("d", 0, S // MD, d_body)

    pl.run_scoped(phase2,
                  pltpu.VMEM((8, S + 2 * GPAD, 128), f32),
                  pltpu.VMEM((2, 7, MB // 8, 512), u32),
                  pltpu.VMEM((7, MD // 4, 512), u32),
                  pltpu.VMEM((7, MD // 4, F // 2), u32))

    out_copy(0, S).wait()


def _run(x, mem0, wq, wk, wv, wo, w1, w2, w3, w4, c, wmod):
    any_spec = pl.BlockSpec(memory_space=pl.ANY)
    vmem_spec = pl.BlockSpec(memory_space=pltpu.VMEM)
    return pl.pallas_call(
        _kernel,
        out_shape=jax.ShapeDtypeStruct((S, D), bf16),
        in_specs=[any_spec, vmem_spec, any_spec, any_spec, any_spec, any_spec, any_spec,
                  any_spec, any_spec, any_spec, vmem_spec, any_spec],
        out_specs=any_spec,
        scratch_shapes=[
            pltpu.VMEM((S, D), bf16),
            pltpu.VMEM((8, H * DH, 128), bf16),
            pltpu.VMEM((7, WROWS + WCH, 128), bf16),
            pltpu.VMEM((NMOD, D, 512), bf16),
            [pltpu.VMEM((96 // NRING, NR, 128), bf16)] * NRING,
            pltpu.VMEM((32, D), bf16),
            pltpu.VMEM((H, 32, 128), bf16),
            pltpu.VMEM((2 * H, 16, 128), bf16),
            pltpu.VMEM((8, 6 * D), f32),
            pltpu.VMEM((S, D), f32),
            pltpu.VMEM((7, S // 2, 512), bf16),
            pltpu.SemaphoreType.DMA((4,)),
            pltpu.SemaphoreType.DMA((NMOD,)),
            pltpu.SemaphoreType.DMA((NSLOT,)),
            pltpu.SemaphoreType.DMA(()),
            pltpu.SemaphoreType.DMA(()),
            pltpu.SemaphoreType.DMA(()),
        ],
        compiler_params=pltpu.CompilerParams(vmem_limit_bytes=124 * 1024 * 1024),
    )(x, mem0, wq, wk, wv, wo, w1, w2, w3, w4, c, wmod)


def pallas_adaLN_cond__memory_aug_recurrent_mem_tr__mixer_s_mlp__prompt_kernel(
    A_x, A_mem0, A_Wq, A_Wk, A_Wv, A_Wo, A_seg_len, B_x, B_w1, B_w2, B_w3, B_w4, c, w_mod,
):
    del B_x
    assert A_x.shape == (1, S, D) and A_mem0.shape == (1, MEM, D)
    assert isinstance(A_seg_len, int) is False or A_seg_len == SEG
    pairs = (D // 2, 2, H, DH)
    out = _run(A_x.reshape(S, D), A_mem0.reshape(MEM, D), A_Wq.reshape(pairs),
               A_Wk.reshape(pairs), A_Wv.reshape(pairs), A_Wo.reshape(H * DH, D),
               B_w1, B_w2, B_w3, B_w4, c, w_mod)
    return out.reshape(1, S, D)
```

```python
import jax
import jax.numpy as jnp
from jax import lax
import jax.experimental.pallas as pl
import jax.experimental.pallas.tpu as pltpu

bf16 = jnp.bfloat16
f32 = jnp.float32
u32 = jnp.uint32

S = 2048
D = 1024
H = 32
DH = 128
F = 3584
MEM = 8
SEG = 32
NSEG = S // SEG
L = MEM + SEG
RIDE = 24
NPRE = S - RIDE * NSEG
NR = NPRE + 2 * SEG
ROFF = (-(S - NPRE)) % NR
WP = 520
NGRP = 12
NSLOT = 6
NMOD = 6
EPS = 1e-5
MD = 128
MB = 512
GPAD = 8
NRING = 8
RLP = 19
SUBB, SUBC = 256, 128
NP = 1
DS, DP, GW, WT, KSPLIT = 2, 4, 4, 1, 2
W1, W2, W3, W4 = 0, 4 * 512, 8 * 512, 22 * 512
WROWS = W4 + 4 * (F // 2)
T0 = 8
WCH = WROWS // (NSEG // 2 - T0)
_ONLY = None


def _loop(name, lo, hi, body):
    if _ONLY is not None and name not in _ONLY:
        return
    with _scope(name):
        lax.fori_loop(lo, hi, body, 0)


class _NoScope:
    def __init__(self, name):
        del name

    def __enter__(self):
        return self

    def __exit__(self, *a):
        return False


_scope = _NoScope


def _blk(m, h):
    g, r = divmod(h, 8)
    return m * 32 + g * 8 + (r % 2) * 4 + r // 2


_HEAD = sorted(range(H), key=lambda h: _blk(0, h))


def _ln(x):
    mu = jnp.mean(x, axis=-1, keepdims=True)
    xc = x - mu
    var = jnp.mean(xc * xc, axis=-1, keepdims=True)
    return xc * lax.rsqrt(var + EPS)


def _gelu(x):
    inner = x * (0.7978845608028654 + (0.7978845608028654 * 0.044715) * (x * x))
    hx = 0.5 * x
    return hx + hx * jnp.tanh(inner)


def _split_rows(x):
    m, n = x.shape
    x3 = x.reshape(m // 16, 16, n)
    return x3[:, 0:8, :].reshape(m // 2, n), x3[:, 8:16, :].reshape(m // 2, n)


def _merge_rows(top, bot):
    m, n = top.shape
    return jnp.concatenate([top.reshape(m // 8, 8, n), bot.reshape(m // 8, 8, n)],
                           axis=1).reshape(2 * m, n)


def _a_operands(a11, a12, a21, a22):
    return [a11 + a22, a21 + a22, a11, a22, a11 + a12, a21 - a11, a12 - a22]


def _b_operands(b11, b12, b21, b22):
    return [b11 + b22, b11, b12 - b22, b21 - b11, b22, b11 + b12, b21 + b22]


_BTERMS = ((0, 3, 1), (0, None, 0), (1, 3, -1), (2, 0, -1), (3, None, 0), (0, 1, 1), (2, 3, 1))
_BSLOT = (4, 0, 1, 2, 3, 5, 6)


def _strassen(a_of, b_of):
    def prod(k):
        return jnp.dot(a_of(k), b_of(k), preferred_element_type=f32)
    p5 = prod(4)
    p3 = prod(2)
    c12 = p3 + p5
    p1 = prod(0)
    c11 = p1 - p5
    c22 = p1 + p3
    p4 = prod(3)
    c11 = c11 + p4
    c11 = prod(6) + c11
    p2 = prod(1)
    c21 = p2 + p4
    c22 = c22 - p2
    c22 = prod(5) + c22
    return c11, c12, c21, c22


def _kernel(x_hbm, mem0_ref, wq_hbm, wk_hbm, wv_hbm, wo_hbm, w1_hbm, w2_hbm, w3_hbm, w4_hbm,
            c_ref, wmod_hbm, out_hbm,
            xbuf, wo, w7, wmodb, rings, lhs_h, lhs_o, kvm, modv, h2buf, n7,
            sems):
    w_hbms = (wq_hbm, wk_hbm, wv_hbm)
    SX, SMOD, SSTG = 0, 4, 4 + NMOD
    sem_wo, sem_mlp, sem_out = (sems.at[SSTG + NSLOT + k] for k in range(3))

    def rget(b, row, n):
        return rings[b % NRING][b // NRING, pl.ds(row, n), :]

    def rset(b, row, val):
        rings[b % NRING][b // NRING, pl.ds(row, val.shape[0]), :] = val.astype(bf16)

    def x_copy(i):
        return pltpu.make_async_copy(x_hbm.at[pl.ds(i * 512, 512), :],
                                     xbuf.at[pl.ds(i * 512, 512), :], sems.at[SX + i])

    def mod_copy(j):
        return pltpu.make_async_copy(wmod_hbm.at[:, pl.ds(j * 512, 512)], wmodb.at[j % NMOD],
                                     sems.at[SMOD + j % NMOD])

    def wo_copy(j):
        return pltpu.make_async_copy(wo_hbm.at[:, pl.ds(j * 128, 128)], wo.at[j], sem_wo)

    def mlp_copies():
        cps = []
        for src, base, kh, npair in ((w1_hbm, W1, 512, 4), (w2_hbm, W2, 512, 4),
                                     (w3_hbm, W3, 512, 14), (w4_hbm, W4, F // 2, 4)):
            for j in range(npair):
                for quad in range(4):
                    cps.append(pltpu.make_async_copy(
                        src.at[pl.ds((quad // 2) * kh, kh),
                               pl.ds(((quad % 2) * npair + j) * 128, 128)],
                        w7.at[quad, pl.ds(base + j * kh, kh), :], sem_mlp))
        return cps

    def mlp_wait():
        done = w7.at[pl.ds(0, 4), pl.ds(0, WROWS), :]
        pltpu.make_async_copy(done, done, sem_mlp).wait()

    def out_copy(row, n):
        return pltpu.make_async_copy(xbuf.at[pl.ds(row, n), :], out_hbm.at[pl.ds(row, n), :],
                                     sem_out)

    def mod_chunks(js, wait_each):
        cv = c_ref[...].astype(f32)
        sv = cv * (1.0 / (1.0 + jnp.exp(-cv)))
        sv = jnp.broadcast_to(sv, (16, D)).astype(bf16)
        if not wait_each:
            for j in js:
                mod_copy(j).wait()
        for j in js:
            if wait_each:
                mod_copy(j).wait()
            y = jnp.dot(sv, wmodb[j % NMOD], preferred_element_type=f32)
            modv[:, j * 512:(j + 1) * 512] = y[0:8]

    def modrow(k):
        return modv[0:1, k * D:(k + 1) * D]

    def adaln_a(xv):
        return _ln(xv) * (1.0 + modrow(1)) + modrow(0)

    def adaln_b(xv):
        return _ln(xv) * (1.0 + modrow(4)) + modrow(3)

    def row_operands(v):
        top, bot = _split_rows(v)
        k = v.shape[1] // 2
        return _a_operands(top[:, :k], top[:, k:], bot[:, :k], bot[:, k:])

    def stage_a(r, n):
        for k in range(n // 16):
            rr = pl.multiple_of(r + k * 16, 16)
            h2 = adaln_b(xbuf[pl.ds(rr, 16), :].astype(f32))
            h2buf[pl.ds(rr, 16), :] = h2
            ro = pl.multiple_of(rr // 2, 8)
            for t, op in enumerate(row_operands(_ln(h2))):
                n7[t, pl.ds(ro, 8), :] = op.astype(bf16)

    def phase1(wqkv, stg):
        def piece_copies(g, dh):
            slot = (2 * g + dh) % NSLOT
            return [pltpu.make_async_copy(
                w_hbms[g // 4].at[pl.ds(dh * 256, 256), par, pl.ds((g % 4) * 8, 8), :],
                stg.at[slot, :, pl.ds(par * 8, 8), :], sems.at[SSTG + slot]) for par in range(2)]

        def group_start(g):
            for dh in range(2):
                for cp in piece_copies(g, dh):
                    cp.start()

        def piece_wait(slot):
            pltpu.make_async_copy(stg.at[slot], stg.at[slot], sems.at[SSTG + slot]).wait()

        sub = lax.broadcasted_iota(jnp.int32, (8, 128), 0) < 4
        keep = jnp.where(sub, jnp.uint32(0xFFFF), jnp.uint32(0xFFFF0000))
        shl = jnp.where(sub, jnp.uint32(16), jnp.uint32(0))
        shr = jnp.where(sub, jnp.uint32(0), jnp.uint32(16))

        def relayout(g, dh, lo_dp, n_dp):
            slot = (2 * g + dh) % NSLOT
            base = g * (8 * WP) + dh * 256
            for u in range(n_dp):
                dp = lo_dp + u
                a = pltpu.bitcast(stg[slot, dp], u32)
                b = pltpu.roll(a, 4, 0)
                wqkv[pl.ds(base + dp, 8, stride=WP), :] = (a & keep) | ((b << shl) >> shr)

        def b_operand(g, q, k):
            def quad(i):
                r = pl.multiple_of((g * 8 + q + 4 * (i % 2)) * WP + (i // 2) * 256, 8)
                return pltpu.bitcast(wqkv[pl.ds(r, 256), :], bf16)
            i, j, sign = _BTERMS[k]
            if j is None:
                return quad(i)
            u, v = quad(i).astype(f32), quad(j).astype(f32)
            return (u + v if sign > 0 else u - v).astype(bf16)

        x_copy(0).start()
        group_start(0)
        for j in (0, 2, 1, 3):
            mod_copy(j).start()
        x_copy(0).wait()

        def ln0_body(i, _):
            r = pl.multiple_of(i * 64, 64)
            h2buf[pl.ds(r, 64), :] = _ln(xbuf[pl.ds(r, 64), :].astype(f32))
            return 0
        lax.fori_loop(0, NPRE // 64, ln0_body, 0)

        for dh in range(2):
            piece_wait(dh)

            def rl_body(t, _, dh=dh):
                relayout(0, dh, t * 32, 32)
                return 0
            lax.fori_loop(0, 8, rl_body, 0)
        group_start(1)
        with _scope("mod0"):
            mod_chunks((0, 2, 1, 3), True)
        group_start(2)

        def hpre_body(i, _):
            r = pl.multiple_of(i * 32, 32)
            hv = h2buf[pl.ds(r, 32), :] * (1.0 + modrow(1)) + modrow(0)
            ro = pl.multiple_of(i * 16, 16)
            for t, op in enumerate(row_operands(hv)):
                n7[t, pl.ds(ro, 16), :] = op.astype(bf16)
            return 0
        lax.fori_loop(0, NPRE // 32, hpre_body, 0)

        extra = {0: [wo_copy(0)], 1: [wo_copy(1), mod_copy(4)], 2: [wo_copy(2)],
                 3: [wo_copy(3), mod_copy(5)], 4: [wo_copy(4)], 5: [wo_copy(5), mod_copy(6)],
                 6: [wo_copy(6)], 7: [wo_copy(7), mod_copy(7)], 8: [x_copy(1)],
                 9: [mod_copy(8), mod_copy(9)]}

        def pre_iter(g, _):
            gn = jnp.minimum(g + 1, NGRP - 1)

            @pl.when(g < NGRP - 1)
            def _():
                piece_wait((2 * gn) % NSLOT)
                piece_wait((2 * gn + 1) % NSLOT)
            for k in range(NGRP - 1):
                @pl.when(g == k)
                def _():
                    if k + 3 < NGRP:
                        group_start(k + 3)
                    for cp in extra.get(k, []):
                        cp.start()
            todo = [(dh, dp) for dh in range(2) for dp in range(256)]
            for q in range(4):
                def b_of(k):
                    w = b_operand(g, q, k)
                    for dh, dp in todo[:RLP]:
                        relayout(gn, dh, dp, 1)
                    del todo[:RLP]
                    return w
                c11, c12, c21, c22 = _strassen(lambda k: n7[k, 0:NPRE // 2, :], b_of)
                for blk, y in ((q + 4, _merge_rows(c12, c22)), (q, _merge_rows(c11, c21))):
                    y = y.astype(bf16)
                    n0 = NR - ROFF
                    rings[blk][g, ROFF:NR, :] = y[0:n0]
                    rings[blk][g, 0:NPRE - n0, :] = y[n0:NPRE]
            assert not todo
            return 0

        _loop("pre1", 0, NGRP, pre_iter)

        with _scope("mod1"):
            mod_chunks(range(4, 10), False)
        x_copy(1).wait()
        pltpu.make_async_copy(wo, wo, sem_wo).wait()
        lhs_h[0:MEM, :] = mem0_ref[...]
        lhs_h[MEM:32, :] = adaln_a(xbuf[NPRE:NPRE + RIDE, :].astype(f32)).astype(bf16)
        for t in range(4):
            w7[t, WROWS:WROWS + WCH, :] = jnp.zeros((WCH, 128), bf16)

        scale = DH ** -0.5
        ia = lax.broadcasted_iota(jnp.int32, (32, L), 0)
        ja = lax.broadcasted_iota(jnp.int32, (32, L), 1)
        mask_a = (ia >= RIDE) | (ja >= SEG) | (ia + 8 >= ja)
        ib = lax.broadcasted_iota(jnp.int32, (48, 56), 0)
        jb = lax.broadcasted_iota(jnp.int32, (48, 56), 1)
        own = (ib < 40) == (jb < 40)
        mask_b = own & (((jb >= 32) & (jb < 48)) | (jnp.where(jb < 40, jb, jb - 8) <= ib))
        masked = -1e9 / scale
        j8 = lax.broadcasted_iota(jnp.int32, (8, 56), 1)
        fill_b = jnp.concatenate([jnp.where(j8 < 40, masked, -3e38).astype(f32)] * 5
                                 + [jnp.where(j8 < 40, -3e38, masked).astype(f32)], axis=0)

        def softmax(sc, mask, fill):
            sc = jnp.where(mask, sc, fill)
            mx = jnp.max(sc, axis=-1, keepdims=True)
            e = jnp.exp2((sc - mx) * (scale * 1.4426950408889634))
            den = jnp.sum(e, axis=-1, keepdims=True)
            return (e * pl.reciprocal(den, approx=True)).astype(bf16)

        def ride_rows(s, is_b):
            first = s < 2
            if is_b:
                g = [jnp.where(first, -3, -1), 1, 2]
            else:
                g = [jnp.where(first, 1, 0), jnp.where(first, 2, 1), 3]
            return [RIDE * s + 8 * t for t in g]

        def step(s, is_b, lhs_lo, lhs_hi, soft_in):
            seg = pl.multiple_of((SEG * s + ROFF) % NR, SEG)
            sega = pl.multiple_of(seg - SEG, SEG) if is_b else seg
            wr = [pl.multiple_of((NPRE + RIDE * s + 8 * t + ROFF) % NR, 8) for t in range(3)]
            rd = [pl.multiple_of((r + ROFF) % NR, 8) for r in ride_rows(s, is_b)]
            lhs = jnp.concatenate([lhs_lo, lhs_hi], axis=1)
            QM, P, PART = {}, {}, {}
            mrow = 0 if is_b else MEM
            seg8 = pl.multiple_of(seg + 8, 8)
            seg24 = pl.multiple_of(seg + RIDE, 8)

            def wblk(b, lo, n):
                return pltpu.bitcast(wqkv[b * WP + lo:b * WP + lo + n, :], bf16)

            def qkv_lo(i):
                for m in range(3):
                    PART[(m, i)] = jnp.dot(lhs_lo, wblk(m * H + i, 0, 256), preferred_element_type=f32)

            def qkv(i):
                for m in range(3):
                    b = m * H + i
                    if (m, i) in PART:
                        y = jnp.dot(lhs_hi, wblk(b, 256, 256),
                                    preferred_element_type=f32) + PART.pop((m, i))
                    else:
                        y = jnp.dot(lhs, wblk(b, 0, 512), preferred_element_type=f32)
                    if m < 2:
                        QM[b] = y[0:MEM]
                    if m == 2 or (m == 1 and not is_b):
                        kvm[b - H, mrow:mrow + MEM, :] = y[0:MEM].astype(bf16)
                    for t in range(3):
                        rset(b, wr[t], y[8 + 8 * t:16 + 8 * t])

            def keys(b):
                if is_b:
                    if b in QM:
                        old = kvm[b - H, MEM:2 * MEM, :].astype(f32)
                        mix = jnp.concatenate([QM.pop(b), old], axis=0).astype(bf16)
                    else:
                        mix = kvm[b - H]
                    return jnp.concatenate([rget(b, seg, SEG), mix, rget(b, sega, 8)], axis=0)
                mk = QM.pop(b).astype(bf16) if b in QM else kvm[b - H, MEM:2 * MEM, :]
                return jnp.concatenate([rget(b, seg, SEG), mk], axis=0)

            def scores(i):
                if is_b:
                    mix = jnp.concatenate([QM.pop(i), rget(i, sega, 8).astype(f32)], axis=0)
                    q = jnp.concatenate([rget(i, seg, SEG), mix.astype(bf16)], axis=0)
                else:
                    mix = jnp.concatenate([rget(i, seg24, 8).astype(f32), QM.pop(i)], axis=0)
                    q = jnp.concatenate([rget(i, seg8, 16), mix.astype(bf16)], axis=0)
                sc = lax.dot_general(q, keys(H + i), (((1,), (1,)), ((), ())),
                                     preferred_element_type=f32)
                P[i] = softmax(sc, mask_b, fill_b) if is_b else softmax(sc, mask_a, masked)

            def pv(i):
                o = jnp.dot(P.pop(i), keys(2 * H + i), preferred_element_type=f32)
                if is_b:
                    rset(i, seg, o[0:SEG])
                    rset(i, sega, o[40:48])
                    lhs_o[i, 0:MEM, :] = o[SEG:L].astype(bf16)
                else:
                    rset(i, seg8, o[0:16])
                    rset(i, seg24, o[16:RIDE])
                    lhs_o[i, 0:MEM, :] = o[RIDE:32].astype(bf16)
                for t in range(3):
                    lhs_o[i, 8 + 8 * t:16 + 8 * t, :] = rget(i, rd[t], 8)

            def wo_group(i0, i1, acc):
                lo = jnp.concatenate([lhs_o[i] for i in range(i0, i1)], axis=1)
                out = []
                for j in range(8):
                    w = jnp.concatenate([wo[j, DH * _HEAD[i]:DH * (_HEAD[i] + 1), :]
                                         for i in range(i0, i1)], axis=0)
                    y = jnp.dot(lo, w, preferred_element_type=f32)
                    out.append(y if acc is None else y + acc[j])
                return out

            def side(t):
                if 0 <= t - DP < H:
                    pv(t - DP)
                if 0 <= t - DS < H:
                    scores(t - DS)

            if soft_in:
                for h in range(KSPLIT):
                    qkv_lo(h)
            for h in range(H):
                qkv(h)
                side(h)
            acc = None
            t = H
            bounds = list(range(0, H - 2 * GW + 1, GW)) + [H]
            for h0, h1 in zip(bounds[:-1], bounds[1:]):
                acc = wo_group(h0, h1, acc)
                for _ in range(WT):
                    side(t)
                    t += 1
            assert not (QM or P or PART)
            return jnp.concatenate(acc[0:4], axis=1), jnp.concatenate(acc[4:8], axis=1)

        def combine_weights(pair):
            r0 = jnp.where(pair < T0, WROWS, (pair - T0) * WCH)
            for c in range(WCH // 64):
                r = pl.multiple_of(r0 + c * 64, 64)
                ops = _b_operands(*[w7[t, pl.ds(r, 64), :].astype(f32) for t in range(4)])
                for k in (0, 2, 3, 5, 6):
                    w7[_BSLOT[k], pl.ds(r, 64), :] = ops[k].astype(bf16)

        def rec_body(it, _):
            @pl.when(it == T0 // NP)
            def _():
                for i in (2, 3):
                    x_copy(i).wait()
                mlp_wait()

            late = [x_copy(2), x_copy(3)] + mlp_copies() + [mod_copy(10), mod_copy(11)]
            nl = -(-len(late) // 4)
            for k in range(4):
                @pl.when(it == k)
                def _():
                    for cp in late[k * nl:(k + 1) * nl]:
                        cp.start()

            lhs_lo = lhs_h[:, 0:512]
            lhs_hi = lhs_h[:, 512:1024]
            stage_a(jnp.maximum(it - 1, 0) * (2 * RIDE * NP), 2 * RIDE * NP)
            for u in range(2 * NP):
                s = it * (2 * NP) + u
                if u % 2 == 0:
                    combine_weights(it * NP + u // 2)
                r1 = pl.multiple_of(jnp.minimum(NPRE + RIDE * (s + 1), S - RIDE), 8)
                hn = adaln_a(xbuf[pl.ds(r1, RIDE), :].astype(f32))
                a_lo, a_hi = step(s, u % 2 == 1, lhs_lo, lhs_hi, u > 0)
                lhs_lo = jnp.concatenate([a_lo[0:MEM], hn[:, 0:512]], axis=0).astype(bf16)
                lhs_hi = jnp.concatenate([a_hi[0:MEM], hn[:, 512:1024]], axis=0).astype(bf16)
                a = jnp.concatenate([a_lo, a_hi], axis=1)
                for t, r in enumerate(ride_rows(s, u % 2 == 1)):
                    r0 = pl.multiple_of(r, 8)
                    xa = (xbuf[pl.ds(r0, 8), :].astype(f32)
                          + modv[:, 2 * D:3 * D] * a[8 + 8 * t:16 + 8 * t])
                    xbuf[pl.ds(r0, 8), :] = xa.astype(bf16)
            lhs_h[:, 0:512] = lhs_lo
            lhs_h[:, 512:1024] = lhs_hi
            return 0

        _loop("rec", 0, NSEG // (2 * NP), rec_body)

    pl.run_scoped(phase1,
                  pltpu.VMEM((96 * WP, 128), u32),
                  pltpu.VMEM((NSLOT, 256, 16, 128), bf16))

    def wo_tail(i, _):
        p0 = pl.multiple_of(i * 128, 128)
        r = pl.multiple_of(S - NPRE + i * 128, 128)
        stage_a(r - 128, 128)
        lo = jnp.concatenate([rget(_blk(0, h), p0, 128) for h in range(H)], axis=1)
        for j in range(8):
            y = jnp.dot(lo, wo[j], preferred_element_type=f32)
            cs = slice(j * 128, (j + 1) * 128)
            ga = modv[0:1, 2 * D + j * 128:2 * D + (j + 1) * 128]
            xbuf[pl.ds(r, 128), cs] = (xbuf[pl.ds(r, 128), cs].astype(f32) + ga * y).astype(bf16)
        return 0
    _loop("wotail", 0, NPRE // 128, wo_tail)
    mod_chunks((10, 11), False)
    stage_a(S - 128, 128)

    def phase2(gbuf, c7, d7, u7):
        def wop(base, kh, j):
            return lambda k: w7[_BSLOT[k], base + j * kh:base + (j + 1) * kh, :]

        zpad = jnp.zeros((GPAD, 128), f32)
        for cb in range(8):
            gbuf[cb, 0:GPAD, :] = zpad
            gbuf[cb, GPAD + S:GPAD + S + GPAD, :] = zpad

        def b_body(i, _):
            for j in range(4):
                for r in range(0, MB // 2, SUBB):
                    ro = pl.multiple_of(i * (MB // 2) + r, SUBB)
                    rg = pl.multiple_of(GPAD + i * MB + 2 * r, 8)
                    c11, c12, c21, c22 = _strassen(lambda k: n7[k, pl.ds(ro, SUBB), :],
                                                   wop(W1, 512, j))
                    gbuf[j + 4, pl.ds(rg, 2 * SUBB), :] = _gelu(_merge_rows(c12, c22))
                    gbuf[j, pl.ds(rg, 2 * SUBB), :] = _gelu(_merge_rows(c11, c21))
            return 0
        _loop("b", 0, S // MB, b_body)

        shifts = (-1, -1, 1, 1, -2, -2, 2, 2)
        HB = MB // 2

        def stage_shift(r, half):
            for cb in range(4):
                for k in range(HB // 64):
                    rr = pl.multiple_of(r + k * 64, 8)
                    quad = []
                    for c in (cb, cb + 4):
                        o = GPAD + shifts[c]
                        quad.append(_split_rows(gbuf[c, pl.ds(rr, 64 + 2 * GPAD), :][o:o + 64]))
                    ops = _a_operands(quad[0][0], quad[1][0], quad[0][1], quad[1][1])
                    for t, op in enumerate(ops):
                        c7[half, t, k * 16:(k + 1) * 16, cb * 128:(cb + 1) * 128] = (
                            pltpu.bitcast(op.astype(bf16), u32))

        def stage_c(r, half):
            for t in range(0, HB // 2, SUBC):
                rr = pl.multiple_of(r + 2 * t, 8)
                for j in range(4):
                    c11, c12, c21, c22 = _strassen(
                        lambda k: pltpu.bitcast(c7[half, k, t // 2:(t + SUBC) // 2, :], bf16),
                        wop(W2, 512, j))
                    for c, y in ((j + 4, _merge_rows(c12, c22)), (j, _merge_rows(c11, c21))):
                        cs = slice(c * 128, (c + 1) * 128)
                        h2buf[pl.ds(rr, 2 * SUBC), cs] = h2buf[pl.ds(rr, 2 * SUBC), cs] + y

        stage_shift(0, 0)

        def c_body(i, _):
            r = pl.multiple_of(i * MB, MB)
            stage_shift(r + HB, 1)
            stage_c(r, 0)
            stage_shift(jnp.minimum(r + MB, S - HB), 0)
            stage_c(r + HB, 1)
            return 0
        _loop("c", 0, S // MB, c_body)

        def stage_n2(r):
            for k in range(MD // 32):
                rr = pl.multiple_of(r + k * 32, 32)
                for t, op in enumerate(row_operands(_ln(h2buf[pl.ds(rr, 32), :]))):
                    d7[t, k * 8:(k + 1) * 8, :] = pltpu.bitcast(op.astype(bf16), u32)

        stage_n2(0)

        def d_body(i, _):
            r = pl.multiple_of(i * MD, MD)
            for j in range(14):
                cq = _strassen(lambda k: pltpu.bitcast(d7[k], bf16), wop(W3, 512, j))
                for t, op in enumerate(_a_operands(*[_gelu(c) for c in cq])):
                    u7[t, :, j * 128:(j + 1) * 128] = pltpu.bitcast(op.astype(bf16), u32)
            stage_n2(jnp.minimum(r + MD, S - MD))
            for j in range(4):
                c11, c12, c21, c22 = _strassen(lambda k: pltpu.bitcast(u7[k], bf16),
                                               wop(W4, F // 2, j))
                for c, y in ((j + 4, _merge_rows(c12, c22)), (j, _merge_rows(c11, c21))):
                    cs = slice(c * 128, (c + 1) * 128)
                    gb = modv[0:1, 5 * D + c * 128:5 * D + (c + 1) * 128]
                    o = xbuf[pl.ds(r, MD), cs].astype(f32) + gb * (h2buf[pl.ds(r, MD), cs] + y)
                    xbuf[pl.ds(r, MD), cs] = o.astype(bf16)
            out_copy(r, MD).start()
            return 0
        _loop("d", 0, S // MD, d_body)

    pl.run_scoped(phase2,
                  pltpu.VMEM((8, S + 2 * GPAD, 128), f32),
                  pltpu.VMEM((2, 7, MB // 8, 512), u32),
                  pltpu.VMEM((7, MD // 4, 512), u32),
                  pltpu.VMEM((7, MD // 4, F // 2), u32))

    out_copy(0, S).wait()


def _run(x, mem0, wq, wk, wv, wo, w1, w2, w3, w4, c, wmod):
    any_spec = pl.BlockSpec(memory_space=pl.ANY)
    vmem_spec = pl.BlockSpec(memory_space=pltpu.VMEM)
    return pl.pallas_call(
        _kernel,
        out_shape=jax.ShapeDtypeStruct((S, D), bf16),
        in_specs=[any_spec, vmem_spec, any_spec, any_spec, any_spec, any_spec, any_spec,
                  any_spec, any_spec, any_spec, vmem_spec, any_spec],
        out_specs=any_spec,
        scratch_shapes=[
            pltpu.VMEM((S, D), bf16),
            pltpu.VMEM((8, H * DH, 128), bf16),
            pltpu.VMEM((7, WROWS + WCH, 128), bf16),
            pltpu.VMEM((NMOD, D, 512), bf16),
            [pltpu.VMEM((96 // NRING, NR, 128), bf16)] * NRING,
            pltpu.VMEM((32, D), bf16),
            pltpu.VMEM((H, 32, 128), bf16),
            pltpu.VMEM((2 * H, 16, 128), bf16),
            pltpu.VMEM((8, 6 * D), f32),
            pltpu.VMEM((S, D), f32),
            pltpu.VMEM((7, S // 2, 512), bf16),
            pltpu.SemaphoreType.DMA((4 + NMOD + NSLOT + 3,)),
        ],
        compiler_params=pltpu.CompilerParams(vmem_limit_bytes=124 * 1024 * 1024),
    )(x, mem0, wq, wk, wv, wo, w1, w2, w3, w4, c, wmod)


def pallas_adaLN_cond__memory_aug_recurrent_mem_tr__mixer_s_mlp__prompt_kernel(
    A_x, A_mem0, A_Wq, A_Wk, A_Wv, A_Wo, A_seg_len, B_x, B_w1, B_w2, B_w3, B_w4, c, w_mod,
):
    del B_x
    assert A_x.shape == (1, S, D) and A_mem0.shape == (1, MEM, D)
    assert isinstance(A_seg_len, int) is False or A_seg_len == SEG
    pairs = (D // 2, 2, H, DH)
    out = _run(A_x.reshape(S, D), A_mem0.reshape(MEM, D), A_Wq.reshape(pairs),
               A_Wk.reshape(pairs), A_Wv.reshape(pairs), A_Wo.reshape(H * DH, D),
               B_w1, B_w2, B_w3, B_w4, c, w_mod)
    return out.reshape(1, S, D)
```

```python
import jax
import jax.numpy as jnp
from jax import lax
import jax.experimental.pallas as pl
import jax.experimental.pallas.tpu as pltpu

bf16 = jnp.bfloat16
f32 = jnp.float32
u32 = jnp.uint32

S = 2048
D = 1024
H = 32
DH = 128
F = 3584
MEM = 8
SEG = 32
NSEG = S // SEG
L = MEM + SEG
RIDE = 24
NPRE = S - RIDE * NSEG
NR = NPRE + 2 * SEG
ROFF = (-(S - NPRE)) % NR
WP = 516
WO = 96 * WP
NGRP = 12
NSLOT = 6
NMOD = 6
EPS = 1e-5
MD = 128
MB = 512
GPAD = 8
NRING = 8
RLP, WLP = 25, 22
NWO = 3
NCH, NANC = 16, 3
NA, HS = 1, 24
SUBB = 256
NP = 1
DS, DP, GW, WT, KSPLIT = 2, 4, 4, 1, 2
W1, W2, W3, W4 = 0, 4 * 512, 8 * 512, 22 * 512
WROWS = W4 + 4 * (F // 2)
T0 = 8
WCH = WROWS // (NSEG // 2 - T0)
_ONLY = None


def _loop(name, lo, hi, body):
    if _ONLY is not None and name not in _ONLY:
        return
    with _scope(name):
        lax.fori_loop(lo, hi, body, 0)


class _NoScope:
    def __init__(self, name):
        del name

    def __enter__(self):
        return self

    def __exit__(self, *a):
        return False


_scope = _NoScope


def _zero_after(*vs):
    bits = None
    for v in vs:
        if v is not None:
            b = pltpu.bitcast(v[0:8, 0:128], u32)
            bits = b if bits is None else bits | b
    return pltpu.bitcast((bits >> 31) >> 1, f32)


def _ln(x, anchor=None):
    if anchor is not None:
        z = jnp.concatenate([anchor] * (x.shape[0] // 8), axis=0)
        x = jnp.concatenate([x[:, 0:128] + z, x[:, 128:]], axis=1)
    mu = jnp.mean(x, axis=-1, keepdims=True)
    xc = x - mu
    var = jnp.mean(xc * xc, axis=-1, keepdims=True)
    return xc * lax.rsqrt(var + EPS)


def _gelu(x):
    inner = x * (0.7978845608028654 + (0.7978845608028654 * 0.044715) * (x * x))
    hx = 0.5 * x
    return hx + hx * jnp.tanh(inner)


def _split_rows(x):
    m, n = x.shape
    x3 = x.reshape(m // 16, 16, n)
    return x3[:, 0:8, :].reshape(m // 2, n), x3[:, 8:16, :].reshape(m // 2, n)


def _merge_rows(top, bot):
    m, n = top.shape
    return jnp.concatenate([top.reshape(m // 8, 8, n), bot.reshape(m // 8, 8, n)],
                           axis=1).reshape(2 * m, n)


def _a_operands(a11, a12, a21, a22):
    return [a11 + a22, a21 + a22, a11, a22, a11 + a12, a21 - a11, a12 - a22]


def _b_operands(b11, b12, b21, b22):
    return [b11 + b22, b11, b12 - b22, b21 - b11, b22, b11 + b12, b21 + b22]


_BTERMS = ((0, 3, 1), (0, None, 0), (1, 3, -1), (2, 0, -1), (3, None, 0), (0, 1, 1), (2, 3, 1))
_BSLOT = (4, 0, 1, 2, 3, 5, 6)


def _strassen(a_of, b_of):
    def prod(k):
        return jnp.dot(a_of(k), b_of(k), preferred_element_type=f32)
    p5 = prod(4)
    p3 = prod(2)
    c12 = p3 + p5
    p1 = prod(0)
    c11 = p1 - p5
    c22 = p1 + p3
    p4 = prod(3)
    c11 = c11 + p4
    c11 = prod(6) + c11
    p2 = prod(1)
    c21 = p2 + p4
    c22 = c22 - p2
    c22 = prod(5) + c22
    return c11, c12, c21, c22


def _kernel(x_hbm, mem0_ref, wq_hbm, wk_hbm, wv_hbm, wo_hbm, w1_hbm, w2_hbm, w3_hbm, w4_hbm,
            c_ref, wmod_hbm, out_hbm,
            xbuf, w7, wmodb, rings, lhs_h, lhs_o, kvm, modv, h2buf, n7,
            sems):
    w_hbms = (wq_hbm, wk_hbm, wv_hbm)
    SX, SMOD, SSTG = 0, 4, 4 + NMOD
    sem_mlp, sem_out = (sems.at[SSTG + NGRP + 1 + k] for k in range(2))

    def rget(b, row, n):
        return rings[b % NRING][b // NRING, pl.ds(row, n), :]

    def rset(b, row, val):
        rings[b % NRING][b // NRING, pl.ds(row, val.shape[0]), :] = val.astype(bf16)

    def x_copy(i):
        return pltpu.make_async_copy(x_hbm.at[pl.ds(i * 512, 512), :],
                                     xbuf.at[pl.ds(i * 512, 512), :], sems.at[SX + i])

    def mod_copy(j):
        return pltpu.make_async_copy(wmod_hbm.at[:, pl.ds(j * 512, 512)], wmodb.at[j % NMOD],
                                     sems.at[SMOD + j % NMOD])

    def mlp_copies():
        cps = []
        for src, base, kh, npair in ((w1_hbm, W1, 512, 4), (w2_hbm, W2, 512, 4),
                                     (w3_hbm, W3, 512, 14), (w4_hbm, W4, F // 2, 4)):
            for j in range(npair):
                for quad in range(4):
                    cps.append(pltpu.make_async_copy(
                        src.at[pl.ds((quad // 2) * kh, kh),
                               pl.ds(((quad % 2) * npair + j) * 128, 128)],
                        w7.at[quad, pl.ds(base + j * kh, kh), :], sem_mlp))
        return cps

    def mlp_wait():
        done = w7.at[pl.ds(0, 4), pl.ds(0, WROWS), :]
        pltpu.make_async_copy(done, done, sem_mlp).wait()

    def out_copy(row, n):
        return pltpu.make_async_copy(xbuf.at[pl.ds(row, n), :], out_hbm.at[pl.ds(row, n), :],
                                     sem_out)

    def mod_chunks(js, wait_each):
        cv = c_ref[...].astype(f32)
        sv = cv * (1.0 / (1.0 + jnp.exp(-cv)))
        sv = jnp.broadcast_to(sv, (16, D)).astype(bf16)
        if not wait_each:
            for j in js:
                mod_copy(j).wait()
        for j in js:
            if wait_each:
                mod_copy(j).wait()
            y = jnp.dot(sv, wmodb[j % NMOD], preferred_element_type=f32)
            modv[:, j * 512:(j + 1) * 512] = y[0:8]

    def modrow(k):
        return modv[0:1, k * D:(k + 1) * D]

    def adaln_a(xv, anchor=None):
        return _ln(xv, anchor) * (1.0 + modrow(1)) + modrow(0)

    def adaln_b(xv, anchor=None):
        return _ln(xv, anchor) * (1.0 + modrow(4)) + modrow(3)

    def row_operands(v):
        top, bot = _split_rows(v)
        k = v.shape[1] // 2
        return _a_operands(top[:, :k], top[:, k:], bot[:, :k], bot[:, k:])

    def stage_a16(r, anchor=None):
        rr = pl.multiple_of(r, 16)
        h2 = adaln_b(xbuf[pl.ds(rr, 16), :].astype(f32), anchor)
        h2buf[pl.ds(rr, 16), :] = h2
        ro = pl.multiple_of(rr // 2, 8)
        ops = row_operands(_ln(h2))
        for t, op in enumerate(ops):
            n7[t, pl.ds(ro, 8), :] = op.astype(bf16)
        return ops[0]

    def stage_a(r, n):
        for k in range(n // 16):
            stage_a16(r + k * 16)

    def phase1(wqkv, stg):
        def piece_copies(g, dh):
            slot = (2 * g + dh) % NSLOT
            return [pltpu.make_async_copy(
                w_hbms[g // 4].at[pl.ds(dh * 256, 256), par, pl.ds((g % 4) * 8, 8), :],
                stg.at[slot, :, pl.ds(par * 8, 8), :],
                sems.at[SSTG + (g + 1 if g else dh)]) for par in range(2)]

        def wo_copy(j):
            slot = NSLOT + j % NWO
            return pltpu.make_async_copy(wo_hbm.at[:, :, pl.ds(j * 128, 128)], stg.at[slot],
                                         sems.at[SSTG + j + 5])

        def group_start(g):
            for dh in range(2):
                for cp in piece_copies(g, dh):
                    cp.start()

        def stg_wait(slot, n, sem):
            dst = stg.at[pl.ds(slot, n)]
            pltpu.make_async_copy(dst, dst, sems.at[SSTG + sem]).wait()

        def relayout(g, slot, dh, lo_dp, n_dp):
            base = g * (8 * WP) + dh * 256
            for u in range(n_dp):
                dp = lo_dp + u
                ev = pltpu.bitcast(stg[slot, dp, 0:8, :].astype(f32), u32)
                od = pltpu.bitcast(stg[slot, dp, 8:16, :].astype(f32), u32)
                wqkv[pl.ds(base + dp, 8, stride=WP), :] = (ev >> 16) | od

        def b_operand(g, q, k):
            def quad(i):
                r = (g * 8 + q + 4 * (i % 2)) * WP + (i // 2) * 256
                return pltpu.bitcast(wqkv[pl.ds(r, 256), :], bf16)
            i, j, sign = _BTERMS[k]
            if j is None:
                return quad(i)
            u, v = quad(i).astype(f32), quad(j).astype(f32)
            return (u + v if sign > 0 else u - v).astype(bf16)

        x_copy(0).start()
        for j in range(4):
            mod_copy(j).start()
        for g in range(3):
            group_start(g)
        x_copy(0).wait()

        def ln0_body(i, _):
            r = pl.multiple_of(i * 64, 64)
            h2buf[pl.ds(r, 64), :] = _ln(xbuf[pl.ds(r, 64), :].astype(f32))
            return 0
        lax.fori_loop(0, NPRE // 64, ln0_body, 0)

        with _scope("mod0"):
            mod_chunks(range(4), True)

        def hpre_body(i, _):
            r = pl.multiple_of(i * 32, 32)
            hv = h2buf[pl.ds(r, 32), :] * (1.0 + modrow(1)) + modrow(0)
            ro = pl.multiple_of(i * 16, 16)
            for t, op in enumerate(row_operands(hv)):
                n7[t, pl.ds(ro, 16), :] = op.astype(bf16)
            return 0
        lax.fori_loop(0, NPRE // 32, hpre_body, 0)

        for dh in range(2):
            stg_wait(dh, 1, dh)

            def rl_body(t, _, dh=dh):
                relayout(0, dh, dh, t * 32, 32)
                return 0
            lax.fori_loop(0, 8, rl_body, 0)

        extra = {0: [mod_copy(4)], 1: [wo_copy(0)], 2: [wo_copy(1), mod_copy(5)],
                 3: [wo_copy(2)], 4: [wo_copy(3), mod_copy(6)], 5: [wo_copy(4)],
                 6: [wo_copy(5), mod_copy(7)], 7: [wo_copy(6)], 8: [wo_copy(7), x_copy(1)],
                 9: [mod_copy(8), mod_copy(9)]}

        def pre_iter(g, m3):
            last = g == NGRP - 1
            m3n = jnp.where(m3 == 2, 0, m3 + 1)
            gn = jnp.minimum(g + 1, NGRP - 1)
            gslot = 2 * jnp.where(last, m3, m3n)
            wj = jnp.clip(g - 3, 0, 7)
            wslot = jnp.where(g < 3, gslot, NSLOT + jnp.where(last, 1, m3))

            @pl.when(g < NGRP - 1)
            def _():
                stg_wait(gslot, 2, g + 2)

            @pl.when(jnp.logical_and(g >= 3, g < 11))
            def _():
                stg_wait(wslot, 1, g + 2)

            for k in range(NGRP - 1):
                @pl.when(g == k)
                def _():
                    if k + 3 < NGRP:
                        group_start(k + 3)
                    for cp in extra.get(k, []):
                        cp.start()
            wtodo = list(range(0, 256, 2))
            todo = [(dh, dp) for dh in range(2) for dp in range(256)]
            for q in range(4):
                def b_of(k):
                    w = b_operand(g, q, k)
                    nw = 0 if todo else WLP
                    for dh, dp in todo[:RLP]:
                        relayout(gn, gslot + dh, dh, dp, 1)
                    del todo[:RLP]
                    for c in wtodo[:nw]:
                        wqkv[pl.ds(pl.multiple_of(WO + wj * 2048 + c * 8, 16), 16), :] = (
                            pltpu.bitcast(stg[wslot, c:c + 2].reshape(32, 128), u32))
                    del wtodo[:nw]
                    return w
                c11, c12, c21, c22 = _strassen(lambda k: n7[k, 0:NPRE // 2, :], b_of)
                for blk, y in ((q + 4, _merge_rows(c12, c22)), (q, _merge_rows(c11, c21))):
                    y = y.astype(bf16)
                    n0 = NR - ROFF
                    rings[blk][g, ROFF:NR, :] = y[0:n0]
                    rings[blk][g, 0:NPRE - n0, :] = y[n0:NPRE]
            assert not todo and not wtodo
            return m3n

        _loop("pre1", 0, NGRP, pre_iter)

        with _scope("mod1"):
            mod_chunks(range(4, 10), False)
        x_copy(1).wait()
        lhs_h[0:MEM, :] = mem0_ref[...]
        lhs_h[MEM:32, :] = adaln_a(xbuf[NPRE:NPRE + RIDE, :].astype(f32)).astype(bf16)
        for t in range(4):
            w7[t, WROWS:WROWS + WCH, :] = jnp.zeros((WCH, 128), bf16)

        scale = DH ** -0.5
        ia = lax.broadcasted_iota(jnp.int32, (32, L), 0)
        ja = lax.broadcasted_iota(jnp.int32, (32, L), 1)
        mask_a = (ia >= RIDE) | (ja >= SEG) | (ia + 8 >= ja)
        ib = lax.broadcasted_iota(jnp.int32, (48, 56), 0)
        jb = lax.broadcasted_iota(jnp.int32, (48, 56), 1)
        own = (ib < 40) == (jb < 40)
        mask_b = own & (((jb >= 32) & (jb < 48)) | (jnp.where(jb < 40, jb, jb - 8) <= ib))
        masked = -1e9 / scale
        j8 = lax.broadcasted_iota(jnp.int32, (8, 56), 1)
        fill_b = jnp.concatenate([jnp.where(j8 < 40, masked, -3e38).astype(f32)] * 5
                                 + [jnp.where(j8 < 40, -3e38, masked).astype(f32)], axis=0)

        def softmax(sc, mask, fill):
            sc = jnp.where(mask, sc, fill)
            mx = jnp.max(sc, axis=-1, keepdims=True)
            e = jnp.exp2((sc - mx) * (scale * 1.4426950408889634))
            den = jnp.sum(e, axis=-1, keepdims=True)
            return (e * pl.reciprocal(den, approx=True)).astype(bf16)

        def ride_rows(s, is_b):
            first = s < 2
            if is_b:
                g = [jnp.where(first, -3, -1), 1, 2]
            else:
                g = [jnp.where(first, 1, 0), jnp.where(first, 2, 1), 3]
            return [RIDE * s + 8 * t for t in g]

        def step(s, is_b, lhs_lo, lhs_hi, soft_in, jobs):
            seg = pl.multiple_of((SEG * s + ROFF) % NR, SEG)
            sega = pl.multiple_of(seg - SEG, SEG) if is_b else seg
            wr = [pl.multiple_of((NPRE + RIDE * s + 8 * t + ROFF) % NR, 8) for t in range(3)]
            rd = [pl.multiple_of((r + ROFF) % NR, 8) for r in ride_rows(s, is_b)]
            lhs = jnp.concatenate([lhs_lo, lhs_hi], axis=1)
            QM, P, PART = {}, {}, {}
            mrow = 0 if is_b else MEM
            seg8 = pl.multiple_of(seg + 8, 8)
            seg24 = pl.multiple_of(seg + RIDE, 8)

            def wblk(b, lo, n):
                return pltpu.bitcast(wqkv[b * WP + lo:b * WP + lo + n, :], bf16)

            def qkv_lo(i):
                for m in range(3):
                    PART[(m, i)] = jnp.dot(lhs_lo, wblk(m * H + i, 0, 256), preferred_element_type=f32)

            def qkv(i):
                for m in range(3):
                    b = m * H + i
                    if (m, i) in PART:
                        y = jnp.dot(lhs_hi, wblk(b, 256, 256),
                                    preferred_element_type=f32) + PART.pop((m, i))
                    else:
                        y = jnp.dot(lhs, wblk(b, 0, 512), preferred_element_type=f32)
                    if m < 2:
                        QM[b] = y[0:MEM]
                    if m == 2 or (m == 1 and not is_b):
                        kvm[b - H, mrow:mrow + MEM, :] = y[0:MEM].astype(bf16)
                    for t in range(3):
                        rset(b, wr[t], y[8 + 8 * t:16 + 8 * t])
                return y

            def keys(b):
                if is_b:
                    if b in QM:
                        old = kvm[b - H, MEM:2 * MEM, :].astype(f32)
                        mix = jnp.concatenate([QM.pop(b), old], axis=0).astype(bf16)
                    else:
                        mix = kvm[b - H]
                    return jnp.concatenate([rget(b, seg, SEG), mix, rget(b, sega, 8)], axis=0)
                mk = QM.pop(b).astype(bf16) if b in QM else kvm[b - H, MEM:2 * MEM, :]
                return jnp.concatenate([rget(b, seg, SEG), mk], axis=0)

            def scores(i):
                if is_b:
                    mix = jnp.concatenate([QM.pop(i), rget(i, sega, 8).astype(f32)], axis=0)
                    q = jnp.concatenate([rget(i, seg, SEG), mix.astype(bf16)], axis=0)
                else:
                    mix = jnp.concatenate([rget(i, seg24, 8).astype(f32), QM.pop(i)], axis=0)
                    q = jnp.concatenate([rget(i, seg8, 16), mix.astype(bf16)], axis=0)
                sc = lax.dot_general(q, keys(H + i), (((1,), (1,)), ((), ())),
                                     preferred_element_type=f32)
                P[i] = softmax(sc, mask_b, fill_b) if is_b else softmax(sc, mask_a, masked)

            def pv(i):
                o = jnp.dot(P.pop(i), keys(2 * H + i), preferred_element_type=f32)
                if is_b:
                    rset(i, seg, o[0:SEG])
                    rset(i, sega, o[40:48])
                    lhs_o[i, 0:MEM, :] = o[SEG:L].astype(bf16)
                else:
                    rset(i, seg8, o[0:16])
                    rset(i, seg24, o[16:RIDE])
                    lhs_o[i, 0:MEM, :] = o[RIDE:32].astype(bf16)
                for t in range(3):
                    lhs_o[i, 8 + 8 * t:16 + 8 * t, :] = rget(i, rd[t], 8)

            def wo_lhs(i0, i1):
                return jnp.concatenate([lhs_o[i] for i in range(i0, i1)], axis=1)

            def wo_dot(lo, j, i0, i1):
                r = WO + j * 2048
                w = pltpu.bitcast(wqkv[r + 64 * i0:r + 64 * i1, :], bf16)
                return jnp.dot(lo, w, preferred_element_type=f32)

            def side(t):
                if 0 <= t - DP < H:
                    pv(t - DP)
                if 0 <= t - DS < H:
                    scores(t - DS)

            if soft_in:
                for h in range(KSPLIT):
                    qkv_lo(h)
            for h in range(H):
                y = qkv(h)
                side(h)
                for job in jobs.get(h, []):
                    job(y)
            lo = wo_lhs(0, HS)
            acc = []
            for j in range(8):
                acc.append(wo_dot(lo, j, 0, HS))
                side(H + j)
            lo = wo_lhs(HS, H)
            acc = [wo_dot(lo, j, HS, H) + acc[j] for j in range(8)]
            assert not (QM or P or PART)
            return jnp.concatenate(acc[0:4], axis=1), jnp.concatenate(acc[4:8], axis=1)

        def combine_weights(r):
            r = pl.multiple_of(r, 32)
            ops = _b_operands(*[w7[t, pl.ds(r, 32), :].astype(f32) for t in range(4)])
            for k in (0, 2, 3, 5, 6):
                w7[_BSLOT[k], pl.ds(r, 32), :] = ops[k].astype(bf16)

        def rec_body(it, _):
            @pl.when(it == T0 // NP)
            def _():
                for i in (2, 3):
                    x_copy(i).wait()
                mlp_wait()

            late = [x_copy(2), x_copy(3)] + mlp_copies() + [mod_copy(10), mod_copy(11)]
            nl = -(-len(late) // 4)
            for k in range(4):
                @pl.when(it == k)
                def _():
                    for cp in late[k * nl:(k + 1) * nl]:
                        cp.start()

            lhs_lo = lhs_h[:, 0:512]
            lhs_hi = lhs_h[:, 512:1024]
            for u in range(2 * NP):
                s = it * (2 * NP) + u
                pair = it * NP + u // 2
                jobs = {h: [] for h in range(H)}
                r1 = pl.multiple_of(jnp.minimum(NPRE + RIDE * (s + 1), S - RIDE), 8)
                hn = adaln_a(xbuf[pl.ds(r1, RIDE), :].astype(f32))
                ra = jnp.maximum(pair - 1, 0) * (2 * RIDE)
                if u % 2 == 0:
                    rw = jnp.where(pair < T0, WROWS, (pair - T0) * WCH)
                    for c in range(WCH // 32):
                        jobs[4 + c].append(lambda y, c=c, rw=rw: combine_weights(rw + 32 * c))
                    if NA:
                        z = _zero_after(*[stage_a16(ra + 16 * k) for k in range(NA)])
                        hn = jnp.concatenate(
                            [hn[:, 0:896], hn[:, 896:1024] + jnp.concatenate([z] * 3, axis=0)],
                            axis=1)
                else:
                    for k in range(NA, 3):
                        jobs[0].append(lambda y, k=k, ra=ra: stage_a16(ra + 16 * k))
                a_lo, a_hi = step(s, u % 2 == 1, lhs_lo, lhs_hi, u > 0, jobs)
                lhs_lo = jnp.concatenate([a_lo[0:MEM], hn[:, 0:512]], axis=0).astype(bf16)
                lhs_hi = jnp.concatenate([a_hi[0:MEM], hn[:, 512:1024]], axis=0).astype(bf16)
                a = jnp.concatenate([a_lo, a_hi], axis=1)
                for t, r in enumerate(ride_rows(s, u % 2 == 1)):
                    r0 = pl.multiple_of(r, 8)
                    xa = (xbuf[pl.ds(r0, 8), :].astype(f32)
                          + modv[:, 2 * D:3 * D] * a[8 + 8 * t:16 + 8 * t])
                    xbuf[pl.ds(r0, 8), :] = xa.astype(bf16)
            lhs_h[:, 0:512] = lhs_lo
            lhs_h[:, 512:1024] = lhs_hi
            return 0

        _loop("rec", 0, NSEG // (2 * NP), rec_body)

        def wo_tail(i, _):
            p0 = pl.multiple_of(i * 128, 128)
            r = pl.multiple_of(S - NPRE + i * 128, 128)
            prev = None
            lo = jnp.concatenate([rget(h, p0, 128) for h in range(H)], axis=1)
            for j in range(8):
                w = pltpu.bitcast(wqkv[WO + j * 2048:WO + (j + 1) * 2048, :], bf16)
                y = jnp.dot(lo, w, preferred_element_type=f32)
                if j < 7:
                    prev = stage_a16(r - 128 + 16 * j, _zero_after(y, prev))
                if j == 0:
                    prev = stage_a16(r - 16, _zero_after(prev))
                cs = slice(j * 128, (j + 1) * 128)
                ga = modv[0:1, 2 * D + j * 128:2 * D + (j + 1) * 128]
                xbuf[pl.ds(r, 128), cs] = (xbuf[pl.ds(r, 128), cs].astype(f32) + ga * y).astype(bf16)
            return 0
        _loop("wotail", 0, NPRE // 128, wo_tail)

    pl.run_scoped(phase1,
                  pltpu.VMEM((WO + 8 * 2048, 128), u32),
                  pltpu.VMEM((NSLOT + NWO, 256, 16, 128), bf16))

    mod_chunks((10, 11), False)
    stage_a(S - 128, 128)

    def phase2(gbuf, c7, d7):
        def wop(base, kh, j):
            return lambda k: w7[_BSLOT[k], base + j * kh:base + (j + 1) * kh, :]

        zpad = jnp.zeros((GPAD, 128), f32)
        for cb in range(8):
            gbuf[cb, 0:GPAD, :] = zpad
            gbuf[cb, GPAD + S:GPAD + S + GPAD, :] = zpad

        def b_body(i, _):
            for j in range(4):
                for r in range(0, MB // 2, SUBB):
                    ro = pl.multiple_of(i * (MB // 2) + r, SUBB)
                    rg = pl.multiple_of(GPAD + i * MB + 2 * r, 8)
                    c11, c12, c21, c22 = _strassen(lambda k: n7[k, pl.ds(ro, SUBB), :],
                                                   wop(W1, 512, j))
                    gbuf[j + 4, pl.ds(rg, 2 * SUBB), :] = _gelu(_merge_rows(c12, c22))
                    gbuf[j, pl.ds(rg, 2 * SUBB), :] = _gelu(_merge_rows(c11, c21))
            return 0
        _loop("b", 0, S // MB, b_body)

        shifts = (-1, -1, 1, 1, -2, -2, 2, 2)
        HB = MB // 2

        def stage_shift(r, half):
            for k in range(HB // 32):
                gs = jnp.concatenate([gbuf[c, pl.ds(r + (k * 32 + GPAD + shifts[c]), 32), :]
                                      for c in range(8)], axis=1)
                for t, op in enumerate(row_operands(gs)):
                    c7[half, t, k * 16:(k + 1) * 16, :] = op.astype(bf16)

        def stage_c(r, half):
            rr = pl.multiple_of(r, 8)
            lhs = [c7[half, k] for k in range(7)]
            for j in range(4):
                c11, c12, c21, c22 = _strassen(lambda k: lhs[k], wop(W2, 512, j))
                for c, y in ((j + 4, _merge_rows(c12, c22)), (j, _merge_rows(c11, c21))):
                    cs = slice(c * 128, (c + 1) * 128)
                    h2buf[pl.ds(rr, HB), cs] = h2buf[pl.ds(rr, HB), cs] + y

        stage_shift(0, 0)

        def c_body(i, _):
            r = pl.multiple_of(i * MB, MB)
            stage_shift(r + HB, 1)
            stage_c(r, 0)
            stage_shift(jnp.minimum(r + MB, S - HB), 0)
            stage_c(r + HB, 1)
            return 0
        _loop("c", 0, S // MB, c_body)

        def stage_n2(r, k, anchor=None):
            rr = pl.multiple_of(r + k * NCH, NCH)
            ops = row_operands(_ln(h2buf[pl.ds(rr, NCH), :], anchor))
            for t, op in enumerate(ops):
                d7[t, k * (NCH // 2):(k + 1) * (NCH // 2), :] = op.astype(bf16)
            return ops[0][0:8] + ops[0][NCH // 2 - 8:NCH // 2]

        for k in range(MD // NCH):
            stage_n2(0, k)

        def d_body(i, _):
            r = pl.multiple_of(i * MD, MD)
            rn = jnp.minimum(r + MD, S - MD)
            lhs = [d7[k] for k in range(7)]
            uops = []
            for j in range(14):
                cq = _strassen(lambda k: lhs[k], wop(W3, 512, j))
                uops.append(_a_operands(*[_gelu(c) for c in cq]))
            ul = [jnp.concatenate([u[k] for u in uops], axis=1).astype(bf16) for k in range(7)]
            prev = None
            todo = list(range(MD // NCH))
            for j in range(4):
                c11, c12, c21, c22 = _strassen(lambda k: ul[k], wop(W4, F // 2, j))
                for anc in (c12, c11, c22)[:NANC]:
                    if todo:
                        prev = stage_n2(rn, todo.pop(0), _zero_after(anc, prev))
                for c, y in ((j + 4, _merge_rows(c12, c22)), (j, _merge_rows(c11, c21))):
                    cs = slice(c * 128, (c + 1) * 128)
                    gb = modv[0:1, 5 * D + c * 128:5 * D + (c + 1) * 128]
                    o = xbuf[pl.ds(r, MD), cs].astype(f32) + gb * (h2buf[pl.ds(r, MD), cs] + y)
                    xbuf[pl.ds(r, MD), cs] = o.astype(bf16)
            assert not todo
            out_copy(r, MD).start()
            return 0
        _loop("d", 0, S // MD, d_body)

    pl.run_scoped(phase2,
                  pltpu.VMEM((8, S + 2 * GPAD, 128), f32),
                  pltpu.VMEM((2, 7, MB // 4, 512), bf16),
                  pltpu.VMEM((7, MD // 2, 512), bf16))

    out_copy(0, S).wait()


def _run(x, mem0, wq, wk, wv, wo, w1, w2, w3, w4, c, wmod):
    any_spec = pl.BlockSpec(memory_space=pl.ANY)
    vmem_spec = pl.BlockSpec(memory_space=pltpu.VMEM)
    return pl.pallas_call(
        _kernel,
        out_shape=jax.ShapeDtypeStruct((S, D), bf16),
        in_specs=[any_spec, vmem_spec, any_spec, any_spec, any_spec, any_spec, any_spec,
                  any_spec, any_spec, any_spec, vmem_spec, any_spec],
        out_specs=any_spec,
        scratch_shapes=[
            pltpu.VMEM((S, D), bf16),
            pltpu.VMEM((7, WROWS + WCH, 128), bf16),
            pltpu.VMEM((NMOD, D, 512), bf16),
            [pltpu.VMEM((96 // NRING, NR, 128), bf16)] * NRING,
            pltpu.VMEM((32, D), bf16),
            pltpu.VMEM((H, 32, 128), bf16),
            pltpu.VMEM((2 * H, 16, 128), bf16),
            pltpu.VMEM((8, 6 * D), f32),
            pltpu.VMEM((S, D), f32),
            pltpu.VMEM((7, S // 2, 512), bf16),
            pltpu.SemaphoreType.DMA((4 + NMOD + NGRP + 3,)),
        ],
        compiler_params=pltpu.CompilerParams(vmem_limit_bytes=124 * 1024 * 1024),
    )(x, mem0, wq, wk, wv, wo, w1, w2, w3, w4, c, wmod)


def pallas_adaLN_cond__memory_aug_recurrent_mem_tr__mixer_s_mlp__prompt_kernel(
    A_x, A_mem0, A_Wq, A_Wk, A_Wv, A_Wo, A_seg_len, B_x, B_w1, B_w2, B_w3, B_w4, c, w_mod,
):
    del B_x
    assert A_x.shape == (1, S, D) and A_mem0.shape == (1, MEM, D)
    assert isinstance(A_seg_len, int) is False or A_seg_len == SEG
    pairs = (D // 2, 2, H, DH)
    out = _run(A_x.reshape(S, D), A_mem0.reshape(MEM, D), A_Wq.reshape(pairs),
               A_Wk.reshape(pairs), A_Wv.reshape(pairs), A_Wo.reshape(H * DH // 16, 16, D),
               B_w1, B_w2, B_w3, B_w4, c, w_mod)
    return out.reshape(1, S, D)
```

```python
import jax
import jax.numpy as jnp
from jax import lax
import jax.experimental.pallas as pl
import jax.experimental.pallas.tpu as pltpu

bf16 = jnp.bfloat16
f32 = jnp.float32
u32 = jnp.uint32

S = 2048
D = 1024
H = 32
DH = 128
F = 3584
MEM = 8
SEG = 32
NSEG = S // SEG
L = MEM + SEG
RIDE = 24
NPRE = S - RIDE * NSEG
NR = NPRE + 2 * SEG
ROFF = (-(S - NPRE)) % NR
WP = 516
WO = 96 * WP
NGRP = 12
NSLOT = 6
NMOD = 6
EPS = 1e-5
MD = 128
MB = 512
GPAD = 8
NRING = 8
RLP, WLP = 25, 22
NWO = 3
NCH, NANC = 16, 3
NA, HS = 1, 24
SUBB = 256
NP = 1
DS, DP, GW, WT, KSPLIT = 2, 4, 4, 1, 2
W1, W2, W3, W4 = 0, 4 * 512, 8 * 512, 22 * 512
WROWS = W4 + 4 * (F // 2)
T0 = 8
WCH = WROWS // (NSEG // 2 - T0)
_ONLY = None


def _loop(name, lo, hi, body, init=0):
    if _ONLY is not None and name not in _ONLY:
        return
    with _scope(name):
        lax.fori_loop(lo, hi, body, init)


class _NoScope:
    def __init__(self, name):
        del name

    def __enter__(self):
        return self

    def __exit__(self, *a):
        return False


_scope = _NoScope


def _zero_after(*vs):
    bits = None
    for v in vs:
        if v is not None:
            b = pltpu.bitcast(v[0:8, 0:128], u32)
            bits = b if bits is None else bits | b
    return pltpu.bitcast((bits >> 31) >> 1, f32)


def _ln(x, anchor=None):
    if anchor is not None:
        z = jnp.concatenate([anchor] * (x.shape[0] // 8), axis=0)
        x = jnp.concatenate([x[:, 0:128] + z, x[:, 128:]], axis=1)
    mu = jnp.mean(x, axis=-1, keepdims=True)
    xc = x - mu
    var = jnp.mean(xc * xc, axis=-1, keepdims=True)
    return xc * lax.rsqrt(var + EPS)


def _gelu(x):
    inner = x * (0.7978845608028654 + (0.7978845608028654 * 0.044715) * (x * x))
    hx = 0.5 * x
    return hx + hx * jnp.tanh(inner)


def _split_rows(x):
    m, n = x.shape
    x3 = x.reshape(m // 16, 16, n)
    return x3[:, 0:8, :].reshape(m // 2, n), x3[:, 8:16, :].reshape(m // 2, n)


def _merge_rows(top, bot):
    m, n = top.shape
    return jnp.concatenate([top.reshape(m // 8, 8, n), bot.reshape(m // 8, 8, n)],
                           axis=1).reshape(2 * m, n)


def _a_operands(a11, a12, a21, a22):
    return [a11 + a22, a21 + a22, a11, a22, a11 + a12, a21 - a11, a12 - a22]


def _b_operands(b11, b12, b21, b22):
    return [b11 + b22, b11, b12 - b22, b21 - b11, b22, b11 + b12, b21 + b22]


_BTERMS = ((0, 3, 1), (0, None, 0), (1, 3, -1), (2, 0, -1), (3, None, 0), (0, 1, 1), (2, 3, 1))
_BSLOT = (4, 0, 1, 2, 3, 5, 6)


def _strassen(a_of, b_of, hook=lambda v: None):
    def prod(k):
        return jnp.dot(a_of(k), b_of(k), preferred_element_type=f32)
    p5 = prod(4)
    hook(p5)
    p3 = prod(2)
    hook(p3)
    c12 = p3 + p5
    p1 = prod(0)
    hook(p1)
    c11 = p1 - p5
    c22 = p1 + p3
    p4 = prod(3)
    hook(p4)
    c11 = c11 + p4
    c11 = prod(6) + c11
    hook(c11)
    p2 = prod(1)
    hook(p2)
    c21 = p2 + p4
    c22 = c22 - p2
    c22 = prod(5) + c22
    hook(c22)
    return c11, c12, c21, c22


def _kernel(x_hbm, mem0_ref, wq_hbm, wk_hbm, wv_hbm, wo_hbm, w1_hbm, w2_hbm, w3_hbm, w4_hbm,
            c_ref, wmod_hbm, out_hbm,
            xbuf, w7, wmodb, rings, lhs_h, lhs_o, kvm, modv, scol, h2buf, n7,
            sems):
    w_hbms = (wq_hbm, wk_hbm, wv_hbm)
    SX, SMOD, SSTG = 0, 4, 4 + NMOD
    sem_mlp, sem_out = (sems.at[SSTG + NGRP + 2 + k] for k in range(2))

    def rget(b, row, n):
        return rings[b % NRING][b // NRING, pl.ds(row, n), :]

    def rset(b, row, val):
        rings[b % NRING][b // NRING, pl.ds(row, val.shape[0]), :] = val.astype(bf16)

    def x_copy(i):
        lo, hi = (0, NPRE + 32, 1024, S)[i:i + 2]
        return pltpu.make_async_copy(x_hbm.at[pl.ds(lo, hi - lo), :],
                                     xbuf.at[pl.ds(lo, hi - lo), :], sems.at[SX + i])

    def mod_copy(j):
        sem = SSTG + j + 4 if 4 <= j < 10 else SMOD + j % NMOD
        return pltpu.make_async_copy(wmod_hbm.at[:, pl.ds(j * 512, 512)], wmodb.at[j % NMOD],
                                     sems.at[sem])

    def mlp_copies():
        cps = []
        for src, base, kh, npair in ((w1_hbm, W1, 512, 4), (w2_hbm, W2, 512, 4),
                                     (w3_hbm, W3, 512, 14), (w4_hbm, W4, F // 2, 4)):
            for j in range(npair):
                for quad in range(4):
                    cps.append(pltpu.make_async_copy(
                        src.at[pl.ds((quad // 2) * kh, kh),
                               pl.ds(((quad % 2) * npair + j) * 128, 128)],
                        w7.at[quad, pl.ds(base + j * kh, kh), :], sem_mlp))
        return cps

    def mlp_wait():
        done = w7.at[pl.ds(0, 4), pl.ds(0, WROWS), :]
        pltpu.make_async_copy(done, done, sem_mlp).wait()

    def out_copy(row, n):
        return pltpu.make_async_copy(xbuf.at[pl.ds(row, n), :], out_hbm.at[pl.ds(row, n), :],
                                     sem_out)

    def mod_rows(acc, slot, r):
        w = wmodb[slot, pl.ds(r, 16), :].astype(f32)
        sc = jnp.concatenate([scol[pl.ds(r, 16), :]] * 4, axis=1)
        p = w * sc
        return acc + p[0:8] + p[8:16]

    def mod_finish(acc, j):
        is_scale = jnp.logical_or(j // 2 == 1, j // 2 == 4)
        tot = jnp.sum(acc, axis=0, keepdims=True) + jnp.where(is_scale, 1.0, 0.0)
        modv[j] = jnp.broadcast_to(tot, (8, 512))

    def modrows(k, n, lo=0, hi=D):
        m = jnp.concatenate([modv[2 * k], modv[2 * k + 1]], axis=1)[:, lo:hi]
        return jnp.concatenate([m] * (n // 8), axis=0)

    def adaln_a(xv, anchor=None):
        n = xv.shape[0]
        return _ln(xv, anchor) * modrows(1, n) + modrows(0, n)

    def adaln_b(xv, anchor=None):
        n = xv.shape[0]
        return _ln(xv, anchor) * modrows(4, n) + modrows(3, n)

    def row_operands(v):
        top, bot = _split_rows(v)
        k = v.shape[1] // 2
        return _a_operands(top[:, :k], top[:, k:], bot[:, :k], bot[:, k:])

    def stage_a16(r, anchor=None, dst=None):
        rr = pl.multiple_of(r, 16)
        h2 = adaln_b(xbuf[pl.ds(rr, 16), :].astype(f32), anchor)
        h2buf[pl.ds(rr, 16), :] = h2
        ref, ro = (n7, pl.multiple_of(rr // 2, 8)) if dst is None else dst
        ops = row_operands(_ln(h2))
        for t, op in enumerate(ops):
            ref[t, pl.ds(ro, 8), :] = op.astype(bf16)
        return ops[0]

    def phase1(wqkv, stg):
        def piece_copies(g, dh):
            slot = (2 * g + dh) % NSLOT
            return [pltpu.make_async_copy(
                w_hbms[g // 4].at[pl.ds(dh * 256, 256), par, pl.ds((g % 4) * 8, 8), :],
                stg.at[slot, :, pl.ds(par * 8, 8), :],
                sems.at[SSTG + (g + 1 if g else dh)]) for par in range(2)]

        def wo_copy(j):
            slot = NSLOT + j % NWO
            return pltpu.make_async_copy(wo_hbm.at[:, :, pl.ds(j * 128, 128)], stg.at[slot],
                                         sems.at[SSTG + j + 6])

        def group_start(g):
            for dh in range(2):
                for cp in piece_copies(g, dh):
                    cp.start()

        def stg_wait(slot, n, sem):
            dst = stg.at[pl.ds(slot, n)]
            pltpu.make_async_copy(dst, dst, sems.at[SSTG + sem]).wait()

        def relayout(g, slot, dh, lo_dp, n_dp):
            base = g * (8 * WP) + dh * 256
            for u in range(n_dp):
                dp = lo_dp + u
                ev = pltpu.bitcast(stg[slot, dp, 0:8, :].astype(f32), u32)
                od = pltpu.bitcast(stg[slot, dp, 8:16, :].astype(f32), u32)
                wqkv[pl.ds(base + dp, 8, stride=WP), :] = (ev >> 16) | od

        def b_operand(g, q, k):
            def quad(i):
                r = (g * 8 + q + 4 * (i % 2)) * WP + (i // 2) * 256
                return pltpu.bitcast(wqkv[pl.ds(r, 256), :], bf16)
            i, j, sign = _BTERMS[k]
            if j is None:
                return quad(i)
            u, v = quad(i).astype(f32), quad(j).astype(f32)
            return (u + v if sign > 0 else u - v).astype(bf16)

        x_copy(0).start()
        for j in range(4):
            mod_copy(j).start()
        for g in range(3):
            group_start(g)
        cv = c_ref[...].astype(f32)
        sv = jnp.broadcast_to(cv * (1.0 / (1.0 + jnp.exp(-cv))), (128, D))
        for k in range(8):
            scol[k * 128:(k + 1) * 128, :] = sv[:, k * 128:(k + 1) * 128].T
        for t in range(4):
            w7[t, WROWS:WROWS + WCH, :] = jnp.zeros((WCH, 128), bf16)
        x_copy(0).wait()

        def ln0_body(i, _):
            r = pl.multiple_of(i * 64, 64)
            h2buf[pl.ds(r, 64), :] = _ln(xbuf[pl.ds(r, 64), :].astype(f32))
            return 0
        lax.fori_loop(0, NPRE // 64, ln0_body, 0)

        def mod0_body(j, _):
            pltpu.make_async_copy(wmodb.at[j], wmodb.at[j], sems.at[SMOD + j]).wait()
            accs = [jnp.zeros((8, 512), f32)] * 2
            for k in range(64):
                accs[k % 2] = mod_rows(accs[k % 2], j, k * 16)
            mod_finish(accs[0] + accs[1], j)
            return 0
        _loop("mod0", 0, 4, mod0_body)

        def hpre_body(i, _):
            r = pl.multiple_of(i * 32, 32)
            hv = h2buf[pl.ds(r, 32), :] * modrows(1, 32) + modrows(0, 32)
            ro = pl.multiple_of(i * 16, 16)
            for t, op in enumerate(row_operands(hv)):
                n7[t, pl.ds(ro, 16), :] = op.astype(bf16)
            return 0
        lax.fori_loop(0, NPRE // 32, hpre_body, 0)
        lhs_h[0:MEM, :] = mem0_ref[...]
        lhs_h[MEM:32, :] = adaln_a(xbuf[NPRE:NPRE + RIDE, :].astype(f32)).astype(bf16)

        def relayout_now(g, dh):
            def rl_body(t, _):
                relayout(g, 2 * g + dh, dh, t * 32, 32)
                return 0
            lax.fori_loop(0, 8, rl_body, 0)

        for dh in range(2):
            stg_wait(dh, 1, dh)
            relayout_now(0, dh)

        grp = lambda g: piece_copies(g, 0) + piece_copies(g, 1)
        issue = {0: [wo_copy(0)], 1: grp(3) + grp(4), 2: grp(5) + [wo_copy(1), mod_copy(4)],
                 3: grp(6) + [wo_copy(2), mod_copy(5)], 4: grp(7) + [mod_copy(6)],
                 5: grp(8) + [wo_copy(3), mod_copy(7)], 6: grp(9) + [wo_copy(4)],
                 7: grp(10) + [wo_copy(5), mod_copy(8)], 8: grp(11) + [wo_copy(6)],
                 9: [wo_copy(7), mod_copy(9), x_copy(1)]}

        def pre_iter(g, m3):
            m3n = jnp.where(m3 == 2, 0, m3 + 1)
            ends = jnp.logical_or(g == 0, g == NGRP - 1)
            gn = jnp.where(ends, g, g + 1)
            gslot = 2 * jnp.where(ends, m3, m3n)
            wj = jnp.maximum(g - 4, 0)
            wslot = jnp.where(g < 4, gslot, NSLOT + jnp.where(m3 == 0, 2, m3 - 1))
            cj = jnp.maximum(g - 2, 3)
            cslot = jnp.where(cj >= NMOD, cj - NMOD, cj)

            @pl.when(g == 1)
            def _():
                stg_wait(2, 2, 2)
                relayout_now(1, 0)
                relayout_now(1, 1)

            @pl.when(jnp.logical_not(ends))
            def _():
                stg_wait(gslot, 2, g + 2)

            @pl.when(g >= 4)
            def _():
                stg_wait(wslot, 1, g + 2)

            @pl.when(g >= 6)
            def _():
                pltpu.make_async_copy(wmodb.at[cslot], wmodb.at[cslot],
                                      sems.at[SSTG + g + 2]).wait()

            for k, cps in issue.items():
                @pl.when(g == k)
                def _():
                    for cp in cps:
                        cp.start()
            wtodo = list(range(0, 256, 2))
            todo = [(dh, dp) for dh in range(2) for dp in range(256)]
            mtodo = list(range(0, D, 16))
            macc = [jnp.zeros((8, 512), f32)]

            def hook(v):
                if mtodo:
                    acc = macc[0] + jnp.concatenate([_zero_after(v)] * 4, axis=1)
                    for r in mtodo[:3]:
                        acc = mod_rows(acc, cslot, r)
                    del mtodo[:3]
                    macc[0] = acc

            for q in range(4):
                def b_of(k):
                    w = b_operand(g, q, k)
                    nw = 0 if todo else WLP
                    for dh, dp in todo[:RLP]:
                        relayout(gn, gslot + dh, dh, dp, 1)
                    del todo[:RLP]
                    for c in wtodo[:nw]:
                        wqkv[pl.ds(pl.multiple_of(WO + wj * 2048 + c * 8, 16), 16), :] = (
                            pltpu.bitcast(stg[wslot, c:c + 2].reshape(32, 128), u32))
                    del wtodo[:nw]
                    return w
                c11, c12, c21, c22 = _strassen(lambda k: n7[k, 0:NPRE // 2, :], b_of, hook)
                for blk, y in ((q + 4, _merge_rows(c12, c22)), (q, _merge_rows(c11, c21))):
                    y = y.astype(bf16)
                    n0 = NR - ROFF
                    rings[blk][g, ROFF:NR, :] = y[0:n0]
                    rings[blk][g, 0:NPRE - n0, :] = y[n0:NPRE]
            assert not todo and not wtodo and not mtodo
            mod_finish(macc[0], cj)
            return m3n

        _loop("pre1", 0, NGRP, pre_iter)
        x_copy(1).wait()

        scale = DH ** -0.5
        ia = lax.broadcasted_iota(jnp.int32, (32, L), 0)
        ja = lax.broadcasted_iota(jnp.int32, (32, L), 1)
        mask_a = (ia >= RIDE) | (ja >= SEG) | (ia + 8 >= ja)
        ib = lax.broadcasted_iota(jnp.int32, (48, 56), 0)
        jb = lax.broadcasted_iota(jnp.int32, (48, 56), 1)
        own = (ib < 40) == (jb < 40)
        mask_b = own & (((jb >= 32) & (jb < 48)) | (jnp.where(jb < 40, jb, jb - 8) <= ib))
        masked = -1e9 / scale
        j8 = lax.broadcasted_iota(jnp.int32, (8, 56), 1)
        fill_b = jnp.concatenate([jnp.where(j8 < 40, masked, -3e38).astype(f32)] * 5
                                 + [jnp.where(j8 < 40, -3e38, masked).astype(f32)], axis=0)

        def softmax(sc, mask, fill):
            sc = jnp.where(mask, sc, fill)
            mx = jnp.max(sc, axis=-1, keepdims=True)
            e = jnp.exp2((sc - mx) * (scale * 1.4426950408889634))
            den = jnp.sum(e, axis=-1, keepdims=True)
            return (e * pl.reciprocal(den, approx=True)).astype(bf16)

        def ride_rows(s, is_b):
            first = s < 2
            if is_b:
                g = [jnp.where(first, -3, -1), 1, 2]
            else:
                g = [jnp.where(first, 1, 0), jnp.where(first, 2, 1), 3]
            return [RIDE * s + 8 * t for t in g]

        def step(s, is_b, lhs_lo, lhs_hi, soft_in, jobs):
            seg = pl.multiple_of((SEG * s + ROFF) % NR, SEG)
            sega = pl.multiple_of(seg - SEG, SEG) if is_b else seg
            wr = [pl.multiple_of((NPRE + RIDE * s + 8 * t + ROFF) % NR, 8) for t in range(3)]
            rd = [pl.multiple_of((r + ROFF) % NR, 8) for r in ride_rows(s, is_b)]
            lhs = jnp.concatenate([lhs_lo, lhs_hi], axis=1)
            QM, P, PART = {}, {}, {}
            mrow = 0 if is_b else MEM
            seg8 = pl.multiple_of(seg + 8, 8)
            seg24 = pl.multiple_of(seg + RIDE, 8)

            def wblk(b, lo, n):
                return pltpu.bitcast(wqkv[b * WP + lo:b * WP + lo + n, :], bf16)

            def qkv_lo(i):
                for m in range(3):
                    PART[(m, i)] = jnp.dot(lhs_lo, wblk(m * H + i, 0, 256), preferred_element_type=f32)

            def qkv(i):
                for m in range(3):
                    b = m * H + i
                    if (m, i) in PART:
                        y = jnp.dot(lhs_hi, wblk(b, 256, 256),
                                    preferred_element_type=f32) + PART.pop((m, i))
                    else:
                        y = jnp.dot(lhs, wblk(b, 0, 512), preferred_element_type=f32)
                    if m < 2:
                        QM[b] = y[0:MEM]
                    if m == 2 or (m == 1 and not is_b):
                        kvm[b - H, mrow:mrow + MEM, :] = y[0:MEM].astype(bf16)
                    for t in range(3):
                        rset(b, wr[t], y[8 + 8 * t:16 + 8 * t])
                return y

            def keys(b):
                if is_b:
                    if b in QM:
                        old = kvm[b - H, MEM:2 * MEM, :].astype(f32)
                        mix = jnp.concatenate([QM.pop(b), old], axis=0).astype(bf16)
                    else:
                        mix = kvm[b - H]
                    return jnp.concatenate([rget(b, seg, SEG), mix, rget(b, sega, 8)], axis=0)
                mk = QM.pop(b).astype(bf16) if b in QM else kvm[b - H, MEM:2 * MEM, :]
                return jnp.concatenate([rget(b, seg, SEG), mk], axis=0)

            def scores(i):
                if is_b:
                    mix = jnp.concatenate([QM.pop(i), rget(i, sega, 8).astype(f32)], axis=0)
                    q = jnp.concatenate([rget(i, seg, SEG), mix.astype(bf16)], axis=0)
                else:
                    mix = jnp.concatenate([rget(i, seg24, 8).astype(f32), QM.pop(i)], axis=0)
                    q = jnp.concatenate([rget(i, seg8, 16), mix.astype(bf16)], axis=0)
                sc = lax.dot_general(q, keys(H + i), (((1,), (1,)), ((), ())),
                                     preferred_element_type=f32)
                P[i] = softmax(sc, mask_b, fill_b) if is_b else softmax(sc, mask_a, masked)

            def pv(i):
                o = jnp.dot(P.pop(i), keys(2 * H + i), preferred_element_type=f32)
                if is_b:
                    rset(i, seg, o[0:SEG])
                    rset(i, sega, o[40:48])
                    lhs_o[i, 0:MEM, :] = o[SEG:L].astype(bf16)
                else:
                    rset(i, seg8, o[0:16])
                    rset(i, seg24, o[16:RIDE])
                    lhs_o[i, 0:MEM, :] = o[RIDE:32].astype(bf16)
                for t in range(3):
                    lhs_o[i, 8 + 8 * t:16 + 8 * t, :] = rget(i, rd[t], 8)

            def wo_lhs(i0, i1):
                return jnp.concatenate([lhs_o[i] for i in range(i0, i1)], axis=1)

            def wo_dot(lo, j, i0, i1):
                r = WO + j * 2048
                w = pltpu.bitcast(wqkv[r + 64 * i0:r + 64 * i1, :], bf16)
                return jnp.dot(lo, w, preferred_element_type=f32)

            def side(t):
                if 0 <= t - DP < H:
                    pv(t - DP)
                if 0 <= t - DS < H:
                    scores(t - DS)

            if soft_in:
                for h in range(KSPLIT):
                    qkv_lo(h)
            for h in range(H):
                y = qkv(h)
                side(h)
                for job in jobs.get(h, []):
                    job(y)
            lo = wo_lhs(0, HS)
            acc = []
            for j in range(8):
                acc.append(wo_dot(lo, j, 0, HS))
                side(H + j)
            lo = wo_lhs(HS, H)
            acc = [wo_dot(lo, j, HS, H) + acc[j] for j in range(8)]
            assert not (QM or P or PART)
            return jnp.concatenate(acc[0:4], axis=1), jnp.concatenate(acc[4:8], axis=1)

        def combine_weights(r):
            r = pl.multiple_of(r, 32)
            ops = _b_operands(*[w7[t, pl.ds(r, 32), :].astype(f32) for t in range(4)])
            for k in (0, 2, 3, 5, 6):
                w7[_BSLOT[k], pl.ds(r, 32), :] = ops[k].astype(bf16)

        def rec_body(it, _):
            @pl.when(it == T0 // NP)
            def _():
                x_copy(2).wait()
                mlp_wait()
                mod_copy(10).wait()
                mod_copy(11).wait()

            late = [x_copy(2)] + mlp_copies() + [mod_copy(10), mod_copy(11)]
            nl = -(-len(late) // 4)
            for k in range(4):
                @pl.when(it == k)
                def _():
                    for cp in late[k * nl:(k + 1) * nl]:
                        cp.start()

            lhs_lo = lhs_h[:, 0:512]
            lhs_hi = lhs_h[:, 512:1024]
            for u in range(2 * NP):
                s = it * (2 * NP) + u
                pair = it * NP + u // 2
                jobs = {h: [] for h in range(H)}
                r1 = pl.multiple_of(jnp.minimum(NPRE + RIDE * (s + 1), S - RIDE), 8)
                hn = adaln_a(xbuf[pl.ds(r1, RIDE), :].astype(f32))
                ra = jnp.maximum(pair - 1, 0) * (2 * RIDE)
                if u % 2 == 0:
                    rw = jnp.where(pair < T0, WROWS, (pair - T0) * WCH)
                    for c in range(WCH // 32):
                        jobs[4 + c].append(lambda y, c=c, rw=rw: combine_weights(rw + 32 * c))
                    if NA:
                        z = _zero_after(*[stage_a16(ra + 16 * k) for k in range(NA)])
                        hn = jnp.concatenate(
                            [hn[:, 0:896], hn[:, 896:1024] + jnp.concatenate([z] * 3, axis=0)],
                            axis=1)
                else:
                    for k in range(NA, 3):
                        jobs[0].append(lambda y, k=k, ra=ra: stage_a16(ra + 16 * k))
                a_lo, a_hi = step(s, u % 2 == 1, lhs_lo, lhs_hi, u > 0, jobs)
                lhs_lo = jnp.concatenate([a_lo[0:MEM], hn[:, 0:512]], axis=0).astype(bf16)
                lhs_hi = jnp.concatenate([a_hi[0:MEM], hn[:, 512:1024]], axis=0).astype(bf16)
                a = jnp.concatenate([a_lo, a_hi], axis=1)
                for t, r in enumerate(ride_rows(s, u % 2 == 1)):
                    r0 = pl.multiple_of(r, 8)
                    xa = (xbuf[pl.ds(r0, 8), :].astype(f32)
                          + modrows(2, 8) * a[8 + 8 * t:16 + 8 * t])
                    xbuf[pl.ds(r0, 8), :] = xa.astype(bf16)
            lhs_h[:, 0:512] = lhs_lo
            lhs_h[:, 512:1024] = lhs_hi
            return 0

        _loop("rec", 0, NSEG // (2 * NP), rec_body)

        def wo_tail(i, gacc):
            p0 = pl.multiple_of(i * 128, 128)
            r = pl.multiple_of(S - NPRE + i * 128, 128)
            prev = None
            gacc = list(gacc)
            lo = jnp.concatenate([rget(h, p0, 128) for h in range(H)], axis=1)
            for j in range(8):
                w = pltpu.bitcast(wqkv[WO + j * 2048:WO + (j + 1) * 2048, :], bf16)
                y = jnp.dot(lo, w, preferred_element_type=f32)
                if j < 7:
                    prev = stage_a16(r - 128 + 16 * j, _zero_after(y, prev))
                if j == 0:
                    prev = stage_a16(r - 16, _zero_after(prev))
                if j < 4:
                    z = jnp.concatenate([_zero_after(y)] * 4, axis=1)
                    for c in range(2):
                        gacc[c] = gacc[c] + z
                        for k in range(4):
                            rm = pl.multiple_of(i * 256 + j * 64 + k * 16, 16)
                            gacc[c] = mod_rows(gacc[c], (10 + c) % NMOD, rm)
                cs = slice(j * 128, (j + 1) * 128)
                ga = modrows(2, 128, j * 128, (j + 1) * 128)
                xbuf[pl.ds(r, 128), cs] = (xbuf[pl.ds(r, 128), cs].astype(f32) + ga * y).astype(bf16)
            for c in range(2):
                mod_finish(gacc[c], 10 + c)
            return tuple(gacc)
        _loop("wotail", 0, NPRE // 128, wo_tail, (jnp.zeros((8, 512), f32),) * 2)

    pl.run_scoped(phase1,
                  pltpu.VMEM((WO + 8 * 2048, 128), u32),
                  pltpu.VMEM((NSLOT + NWO, 256, 16, 128), bf16))

    def phase2(gbuf, c7, d7):
        def wop(base, kh, j):
            return lambda k: w7[_BSLOT[k], base + j * kh:base + (j + 1) * kh, :]

        zpad = jnp.zeros((GPAD, 128), f32)
        for cb in range(8):
            gbuf[cb, 0:GPAD, :] = zpad
            gbuf[cb, GPAD + S:GPAD + S + GPAD, :] = zpad

        shifts = (-1, -1, 1, 1, -2, -2, 2, 2)
        HB = MB // 2

        def shift_piece(r, half, k):
            gs = jnp.concatenate([gbuf[c, pl.ds(r + (k * 16 + GPAD + shifts[c]), 16), :]
                                  for c in range(8)], axis=1)
            for t, op in enumerate(row_operands(gs)):
                c7[half, t, k * 8:(k + 1) * 8, :] = op.astype(bf16)

        def gate(v, i):
            gbuf[0, pl.ds(GPAD + S + GPAD + 8 * (i // S), 8), :] = v[0:8]

        d7[:, 0:24, :] = jnp.zeros((7, 24, 512), bf16)

        def b_body(i, _):
            ro = pl.multiple_of(i * HB, HB)
            rg = pl.multiple_of(GPAD + i * MB, 8)
            ra = jnp.minimum(S - 128 + 48 * i, S - 48)
            rp = jnp.minimum(S - 128 + 48 * jnp.maximum(i - 1, 0), S - 48)
            n7[:, pl.ds(pl.multiple_of(rp // 2, 8), 24), :] = d7[:, 0:24, :]
            st = {"n": 0, "prev": None}

            def hook(v):
                n = st["n"]
                st["n"] += 1
                if n % 7 == 4 and n // 7 < 3:
                    st["prev"] = stage_a16(ra + 16 * (n // 7), _zero_after(v, st["prev"]),
                                           (d7, 8 * (n // 7)))
                if n < 4:
                    gate(v, i)
                    for k in range(4):
                        shift_piece(0, 0, 4 * n + k)

            for j in range(4):
                c11, c12, c21, c22 = _strassen(lambda k: n7[k, pl.ds(ro, HB), :],
                                               wop(W1, 512, j), hook)
                gbuf[j + 4, pl.ds(rg, MB), :] = _gelu(_merge_rows(c12, c22))
                gbuf[j, pl.ds(rg, MB), :] = _gelu(_merge_rows(c11, c21))
            return 0
        _loop("b", 0, S // MB, b_body)

        def stage_n2(r, k, anchor=None):
            rr = pl.multiple_of(r + k * NCH, NCH)
            ops = row_operands(_ln(h2buf[pl.ds(rr, NCH), :], anchor))
            for t, op in enumerate(ops):
                d7[t, k * (NCH // 2):(k + 1) * (NCH // 2), :] = op.astype(bf16)
            return ops[0][0:8] + ops[0][NCH // 2 - 8:NCH // 2]

        def stage_c(i, r, half, rnext):
            rr = pl.multiple_of(r, 8)
            st = {"n": 0, "prev": None}

            def hook(v):
                n = st["n"]
                st["n"] += 1
                if n < HB // 16:
                    gate(v, i)
                    shift_piece(rnext, 1 - half, n)
                if half == 1 and n % 3 == 0 and n // 3 < MD // NCH:
                    st["prev"] = stage_n2(0, n // 3, _zero_after(v, st["prev"]))

            for j in range(4):
                c11, c12, c21, c22 = _strassen(lambda k: c7[half, k], wop(W2, 512, j), hook)
                for c, y in ((j + 4, _merge_rows(c12, c22)), (j, _merge_rows(c11, c21))):
                    cs = slice(c * 128, (c + 1) * 128)
                    h2buf[pl.ds(rr, HB), cs] = h2buf[pl.ds(rr, HB), cs] + y

        def c_body(i, _):
            r = pl.multiple_of(i * MB, MB)
            stage_c(i, r, 0, r + HB)
            stage_c(i, r + HB, 1, jnp.minimum(i + 1, S // MB - 1) * MB)
            return 0
        _loop("c", 0, S // MB, c_body)

        def d_body(i, _):
            r = pl.multiple_of(i * MD, MD)
            rn = jnp.minimum(r + MD, S - MD)
            lhs = [d7[k] for k in range(7)]
            uops = []
            for j in range(14):
                cq = _strassen(lambda k: lhs[k], wop(W3, 512, j))
                uops.append(_a_operands(*[_gelu(c) for c in cq]))
            ul = [jnp.concatenate([u[k] for u in uops], axis=1).astype(bf16) for k in range(7)]
            prev = None
            todo = list(range(MD // NCH))
            for j in range(4):
                c11, c12, c21, c22 = _strassen(lambda k: ul[k], wop(W4, F // 2, j))
                for anc in (c12, c11, c22)[:NANC]:
                    if todo:
                        prev = stage_n2(rn, todo.pop(0), _zero_after(anc, prev))
                for c, y in ((j + 4, _merge_rows(c12, c22)), (j, _merge_rows(c11, c21))):
                    cs = slice(c * 128, (c + 1) * 128)
                    gb = modrows(5, MD, c * 128, (c + 1) * 128)
                    o = xbuf[pl.ds(r, MD), cs].astype(f32) + gb * (h2buf[pl.ds(r, MD), cs] + y)
                    xbuf[pl.ds(r, MD), cs] = o.astype(bf16)
            assert not todo
            out_copy(r, MD).start()
            return 0
        _loop("d", 0, S // MD, d_body)

    pl.run_scoped(phase2,
                  pltpu.VMEM((8, S + 4 * GPAD, 128), f32),
                  pltpu.VMEM((2, 7, MB // 4, 512), bf16),
                  pltpu.VMEM((7, MD // 2, 512), bf16))

    out_copy(0, S).wait()


def _run(x, mem0, wq, wk, wv, wo, w1, w2, w3, w4, c, wmod):
    any_spec = pl.BlockSpec(memory_space=pl.ANY)
    vmem_spec = pl.BlockSpec(memory_space=pltpu.VMEM)
    return pl.pallas_call(
        _kernel,
        out_shape=jax.ShapeDtypeStruct((S, D), bf16),
        in_specs=[any_spec, vmem_spec, any_spec, any_spec, any_spec, any_spec, any_spec,
                  any_spec, any_spec, any_spec, vmem_spec, any_spec],
        out_specs=any_spec,
        scratch_shapes=[
            pltpu.VMEM((S, D), bf16),
            pltpu.VMEM((7, WROWS + WCH, 128), bf16),
            pltpu.VMEM((NMOD, D, 512), bf16),
            [pltpu.VMEM((96 // NRING, NR, 128), bf16)] * NRING,
            pltpu.VMEM((32, D), bf16),
            pltpu.VMEM((H, 32, 128), bf16),
            pltpu.VMEM((2 * H, 16, 128), bf16),
            pltpu.VMEM((12, 8, 512), f32),
            pltpu.VMEM((D, 128), f32),
            pltpu.VMEM((S, D), f32),
            pltpu.VMEM((7, S // 2, 512), bf16),
            pltpu.SemaphoreType.DMA((4 + NMOD + NGRP + 4,)),
        ],
        compiler_params=pltpu.CompilerParams(vmem_limit_bytes=124 * 1024 * 1024),
    )(x, mem0, wq, wk, wv, wo, w1, w2, w3, w4, c, wmod)


def pallas_adaLN_cond__memory_aug_recurrent_mem_tr__mixer_s_mlp__prompt_kernel(
    A_x, A_mem0, A_Wq, A_Wk, A_Wv, A_Wo, A_seg_len, B_x, B_w1, B_w2, B_w3, B_w4, c, w_mod,
):
    del B_x
    assert A_x.shape == (1, S, D) and A_mem0.shape == (1, MEM, D)
    assert isinstance(A_seg_len, int) is False or A_seg_len == SEG
    pairs = (D // 2, 2, H, DH)
    out = _run(A_x.reshape(S, D), A_mem0.reshape(MEM, D), A_Wq.reshape(pairs),
               A_Wk.reshape(pairs), A_Wv.reshape(pairs), A_Wo.reshape(H * DH // 16, 16, D),
               B_w1, B_w2, B_w3, B_w4, c, w_mod)
    return out.reshape(1, S, D)
```

```python
import jax
import jax.numpy as jnp
from jax import lax
import jax.experimental.pallas as pl
import jax.experimental.pallas.tpu as pltpu

bf16 = jnp.bfloat16
f32 = jnp.float32
u32 = jnp.uint32

S = 2048
D = 1024
H = 32
DH = 128
F = 3584
MEM = 8
SEG = 32
NSEG = S // SEG
L = MEM + SEG
RIDE = 24
NPRE = S - RIDE * NSEG
NR = NPRE + 2 * SEG
ROFF = (-(S - NPRE)) % NR
WP = 516
WO = 96 * WP
NGRP = 12
NSLOT = 6
NMOD = 6
EPS = 1e-5
MD = 128
MB = 512
GPAD = 8
NRING = 8
RLP, WLP = 25, 22
NWO = 3
NCH, NANC = 16, 3
HS, BH = 24, 0
SUBB = 256
NP = 1
DS, DP, GW, WT, KSPLIT = 2, 4, 4, 1, 2
W1, W2, W3, W4 = 0, 4 * 512, 8 * 512, 22 * 512
WROWS = W4 + 4 * (F // 2)
T0 = 8
WCH = WROWS // (NSEG // 2 - T0)
_ONLY = None


def _loop(name, lo, hi, body, init=0):
    if _ONLY is not None and name not in _ONLY:
        return
    with _scope(name):
        lax.fori_loop(lo, hi, body, init)


class _NoScope:
    def __init__(self, name):
        del name

    def __enter__(self):
        return self

    def __exit__(self, *a):
        return False


_scope = _NoScope


def _zero_after(*vs):
    bits = None
    for v in vs:
        if v is not None:
            b = pltpu.bitcast(v[0:8, 0:128], u32)
            bits = b if bits is None else bits | b
    return pltpu.bitcast((bits >> 31) >> 1, f32)


def _ln(x, anchor=None):
    if anchor is not None:
        z = jnp.concatenate([anchor] * (x.shape[0] // 8), axis=0)
        x = jnp.concatenate([x[:, 0:128] + z, x[:, 128:]], axis=1)
    mu = jnp.mean(x, axis=-1, keepdims=True)
    xc = x - mu
    var = jnp.mean(xc * xc, axis=-1, keepdims=True)
    return xc * lax.rsqrt(var + EPS)


def _gelu(x):
    inner = x * (0.7978845608028654 + (0.7978845608028654 * 0.044715) * (x * x))
    hx = 0.5 * x
    return hx + hx * jnp.tanh(inner)


def _split_rows(x):
    m, n = x.shape
    x3 = x.reshape(m // 16, 16, n)
    return x3[:, 0:8, :].reshape(m // 2, n), x3[:, 8:16, :].reshape(m // 2, n)


def _merge_rows(top, bot):
    m, n = top.shape
    return jnp.concatenate([top.reshape(m // 8, 8, n), bot.reshape(m // 8, 8, n)],
                           axis=1).reshape(2 * m, n)


def _a_operands(a11, a12, a21, a22):
    return [a11 + a22, a21 + a22, a11, a22, a11 + a12, a21 - a11, a12 - a22]


def _b_operands(b11, b12, b21, b22):
    return [b11 + b22, b11, b12 - b22, b21 - b11, b22, b11 + b12, b21 + b22]


_BTERMS = ((0, 3, 1), (0, None, 0), (1, 3, -1), (2, 0, -1), (3, None, 0), (0, 1, 1), (2, 3, 1))
_BSLOT = (4, 0, 1, 2, 3, 5, 6)


def _strassen(a_of, b_of, hook=lambda v: None):
    def prod(k):
        return jnp.dot(a_of(k), b_of(k), preferred_element_type=f32)
    p5 = prod(4)
    hook(p5)
    p3 = prod(2)
    hook(p3)
    c12 = p3 + p5
    p1 = prod(0)
    hook(p1)
    c11 = p1 - p5
    c22 = p1 + p3
    p4 = prod(3)
    hook(p4)
    c11 = c11 + p4
    c11 = prod(6) + c11
    hook(c11)
    p2 = prod(1)
    hook(p2)
    c21 = p2 + p4
    c22 = c22 - p2
    c22 = prod(5) + c22
    hook(c22)
    return c11, c12, c21, c22


def _kernel(x_hbm, mem0_ref, wq_hbm, wk_hbm, wv_hbm, wo_hbm, w1_hbm, w2_hbm, w3_hbm, w4_hbm,
            c_ref, wmod_hbm, out_hbm,
            xbuf, w7, wmodb, rings, lhs_h, lhs_o, kvm, modv, scol, h2buf, n7,
            sems):
    w_hbms = (wq_hbm, wk_hbm, wv_hbm)
    SX, SMOD, SSTG = 0, 4, 4 + NMOD
    sem_mlp, sem_out = (sems.at[SSTG + NGRP + 2 + k] for k in range(2))

    def rget(b, row, n):
        return rings[b % NRING][b // NRING, pl.ds(row, n), :]

    def rset(b, row, val):
        rings[b % NRING][b // NRING, pl.ds(row, val.shape[0]), :] = val.astype(bf16)

    def x_copy(i):
        lo, hi = (0, NPRE + 32, 1024, S)[i:i + 2]
        return pltpu.make_async_copy(x_hbm.at[pl.ds(lo, hi - lo), :],
                                     xbuf.at[pl.ds(lo, hi - lo), :], sems.at[SX + i])

    def mod_copy(j):
        sem = SSTG + j + 4 if 4 <= j < 10 else SMOD + j % NMOD
        return pltpu.make_async_copy(wmod_hbm.at[:, pl.ds(j * 512, 512)], wmodb.at[j % NMOD],
                                     sems.at[sem])

    def mlp_copies():
        cps = []
        for src, base, kh, npair in ((w1_hbm, W1, 512, 4), (w2_hbm, W2, 512, 4),
                                     (w3_hbm, W3, 512, 14), (w4_hbm, W4, F // 2, 4)):
            for j in range(npair):
                for quad in range(4):
                    cps.append(pltpu.make_async_copy(
                        src.at[pl.ds((quad // 2) * kh, kh),
                               pl.ds(((quad % 2) * npair + j) * 128, 128)],
                        w7.at[quad, pl.ds(base + j * kh, kh), :], sem_mlp))
        return cps

    def mlp_wait():
        done = w7.at[pl.ds(0, 4), pl.ds(0, WROWS), :]
        pltpu.make_async_copy(done, done, sem_mlp).wait()

    def out_copy(row, n):
        return pltpu.make_async_copy(xbuf.at[pl.ds(row, n), :], out_hbm.at[pl.ds(row, n), :],
                                     sem_out)

    def mod_rows(acc, slot, r):
        w = wmodb[slot, pl.ds(r, 16), :].astype(f32)
        sc = jnp.concatenate([scol[pl.ds(r, 16), :]] * 4, axis=1)
        p = w * sc
        return acc + p[0:8] + p[8:16]

    def mod_finish(acc, j):
        is_scale = jnp.logical_or(j // 2 == 1, j // 2 == 4)
        tot = jnp.sum(acc, axis=0, keepdims=True) + jnp.where(is_scale, 1.0, 0.0)
        modv[j] = jnp.broadcast_to(tot, (8, 512))

    def modrows(k, n, lo=0, hi=D):
        m = jnp.concatenate([modv[2 * k], modv[2 * k + 1]], axis=1)[:, lo:hi]
        return jnp.concatenate([m] * (n // 8), axis=0)

    def adaln_a(xv, anchor=None):
        n = xv.shape[0]
        return _ln(xv, anchor) * modrows(1, n) + modrows(0, n)

    def adaln_b(xv, anchor=None):
        n = xv.shape[0]
        return _ln(xv, anchor) * modrows(4, n) + modrows(3, n)

    def row_operands(v):
        top, bot = _split_rows(v)
        k = v.shape[1] // 2
        return _a_operands(top[:, :k], top[:, k:], bot[:, :k], bot[:, k:])

    def stage_a16(r, anchor=None, dst=None):
        rr = pl.multiple_of(r, 16)
        h2 = adaln_b(xbuf[pl.ds(rr, 16), :].astype(f32), anchor)
        h2buf[pl.ds(rr, 16), :] = h2
        ref, ro = (n7, pl.multiple_of(rr // 2, 8)) if dst is None else dst
        ops = row_operands(_ln(h2))
        for t, op in enumerate(ops):
            ref[t, pl.ds(ro, 8), :] = op.astype(bf16)
        return ops[0]

    def phase1(wqkv, stg):
        def piece_copies(g, dh):
            slot = (2 * g + dh) % NSLOT
            return [pltpu.make_async_copy(
                w_hbms[g // 4].at[pl.ds(dh * 256, 256), par, pl.ds((g % 4) * 8, 8), :],
                stg.at[slot, :, pl.ds(par * 8, 8), :],
                sems.at[SSTG + (g + 1 if g else dh)]) for par in range(2)]

        def wo_copy(j):
            slot = NSLOT + j % NWO
            return pltpu.make_async_copy(wo_hbm.at[:, :, pl.ds(j * 128, 128)], stg.at[slot],
                                         sems.at[SSTG + j + 6])

        def group_start(g):
            for dh in range(2):
                for cp in piece_copies(g, dh):
                    cp.start()

        def stg_wait(slot, n, sem):
            dst = stg.at[pl.ds(slot, n)]
            pltpu.make_async_copy(dst, dst, sems.at[SSTG + sem]).wait()

        def relayout(g, slot, dh, lo_dp, n_dp):
            base = g * (8 * WP) + dh * 256
            for u in range(n_dp):
                dp = lo_dp + u
                ev = pltpu.bitcast(stg[slot, dp, 0:8, :].astype(f32), u32)
                od = pltpu.bitcast(stg[slot, dp, 8:16, :].astype(f32), u32)
                wqkv[pl.ds(base + dp, 8, stride=WP), :] = (ev >> 16) | od

        def b_operand(g, q, k):
            def quad(i):
                r = (g * 8 + q + 4 * (i % 2)) * WP + (i // 2) * 256
                return pltpu.bitcast(wqkv[pl.ds(r, 256), :], bf16)
            i, j, sign = _BTERMS[k]
            if j is None:
                return quad(i)
            u, v = quad(i).astype(f32), quad(j).astype(f32)
            return (u + v if sign > 0 else u - v).astype(bf16)

        x_copy(0).start()
        for j in range(4):
            mod_copy(j).start()
        for g in range(3):
            group_start(g)
        cv = c_ref[...].astype(f32)
        sv = jnp.broadcast_to(cv * (1.0 / (1.0 + jnp.exp(-cv))), (128, D))
        for k in range(8):
            scol[k * 128:(k + 1) * 128, :] = sv[:, k * 128:(k + 1) * 128].T
        for t in range(4):
            w7[t, WROWS:WROWS + WCH, :] = jnp.zeros((WCH, 128), bf16)
        x_copy(0).wait()

        def ln0_body(i, _):
            r = pl.multiple_of(i * 64, 64)
            h2buf[pl.ds(r, 64), :] = _ln(xbuf[pl.ds(r, 64), :].astype(f32))
            return 0
        lax.fori_loop(0, NPRE // 64, ln0_body, 0)

        def mod0_body(j, _):
            pltpu.make_async_copy(wmodb.at[j], wmodb.at[j], sems.at[SMOD + j]).wait()
            accs = [jnp.zeros((8, 512), f32)] * 2
            for k in range(64):
                accs[k % 2] = mod_rows(accs[k % 2], j, k * 16)
            mod_finish(accs[0] + accs[1], j)
            return 0
        _loop("mod0", 0, 4, mod0_body)

        def hpre_body(i, _):
            r = pl.multiple_of(i * 32, 32)
            hv = h2buf[pl.ds(r, 32), :] * modrows(1, 32) + modrows(0, 32)
            ro = pl.multiple_of(i * 16, 16)
            for t, op in enumerate(row_operands(hv)):
                n7[t, pl.ds(ro, 16), :] = op.astype(bf16)
            return 0
        lax.fori_loop(0, NPRE // 32, hpre_body, 0)
        lhs_h[0:MEM, :] = mem0_ref[...]
        lhs_h[MEM:32, :] = adaln_a(xbuf[NPRE:NPRE + RIDE, :].astype(f32)).astype(bf16)

        def relayout_now(g, dh):
            def rl_body(t, _):
                relayout(g, 2 * g + dh, dh, t * 32, 32)
                return 0
            lax.fori_loop(0, 8, rl_body, 0)

        for dh in range(2):
            stg_wait(dh, 1, dh)
            relayout_now(0, dh)

        grp = lambda g: piece_copies(g, 0) + piece_copies(g, 1)
        issue = {0: [wo_copy(0)], 1: grp(3) + grp(4), 2: grp(5) + [wo_copy(1), mod_copy(4)],
                 3: grp(6) + [wo_copy(2), mod_copy(5)], 4: grp(7) + [mod_copy(6)],
                 5: grp(8) + [wo_copy(3), mod_copy(7)], 6: grp(9) + [wo_copy(4)],
                 7: grp(10) + [wo_copy(5), mod_copy(8)], 8: grp(11) + [wo_copy(6)],
                 9: [wo_copy(7), mod_copy(9), x_copy(1)]}

        def pre_iter(g, m3):
            m3n = jnp.where(m3 == 2, 0, m3 + 1)
            ends = jnp.logical_or(g == 0, g == NGRP - 1)
            gn = jnp.where(ends, g, g + 1)
            gslot = 2 * jnp.where(ends, m3, m3n)
            wj = jnp.maximum(g - 4, 0)
            wslot = jnp.where(g < 4, gslot, NSLOT + jnp.where(m3 == 0, 2, m3 - 1))
            cj = jnp.maximum(g - 2, 3)
            cslot = jnp.where(cj >= NMOD, cj - NMOD, cj)

            @pl.when(g == 1)
            def _():
                stg_wait(2, 2, 2)
                relayout_now(1, 0)
                relayout_now(1, 1)

            @pl.when(jnp.logical_not(ends))
            def _():
                stg_wait(gslot, 2, g + 2)

            @pl.when(g >= 4)
            def _():
                stg_wait(wslot, 1, g + 2)

            @pl.when(g >= 6)
            def _():
                pltpu.make_async_copy(wmodb.at[cslot], wmodb.at[cslot],
                                      sems.at[SSTG + g + 2]).wait()

            for k, cps in issue.items():
                @pl.when(g == k)
                def _():
                    for cp in cps:
                        cp.start()
            wtodo = list(range(0, 256, 2))
            todo = [(dh, dp) for dh in range(2) for dp in range(256)]
            mtodo = list(range(0, D, 16))
            macc = [jnp.zeros((8, 512), f32)]

            def hook(v):
                if mtodo:
                    acc = macc[0] + jnp.concatenate([_zero_after(v)] * 4, axis=1)
                    for r in mtodo[:3]:
                        acc = mod_rows(acc, cslot, r)
                    del mtodo[:3]
                    macc[0] = acc

            for q in range(4):
                def b_of(k):
                    w = b_operand(g, q, k)
                    nw = 0 if todo else WLP
                    for dh, dp in todo[:RLP]:
                        relayout(gn, gslot + dh, dh, dp, 1)
                    del todo[:RLP]
                    for c in wtodo[:nw]:
                        wqkv[pl.ds(pl.multiple_of(WO + wj * 2048 + c * 8, 16), 16), :] = (
                            pltpu.bitcast(stg[wslot, c:c + 2].reshape(32, 128), u32))
                    del wtodo[:nw]
                    return w
                c11, c12, c21, c22 = _strassen(lambda k: n7[k, 0:NPRE // 2, :], b_of, hook)
                for blk, y in ((q + 4, _merge_rows(c12, c22)), (q, _merge_rows(c11, c21))):
                    y = y.astype(bf16)
                    n0 = NR - ROFF
                    rings[blk][g, ROFF:NR, :] = y[0:n0]
                    rings[blk][g, 0:NPRE - n0, :] = y[n0:NPRE]
            assert not todo and not wtodo and not mtodo
            mod_finish(macc[0], cj)
            return m3n

        _loop("pre1", 0, NGRP, pre_iter)
        x_copy(1).wait()

        scale = DH ** -0.5
        ia = lax.broadcasted_iota(jnp.int32, (32, L), 0)
        ja = lax.broadcasted_iota(jnp.int32, (32, L), 1)
        mask_a = (ia >= RIDE) | (ja >= SEG) | (ia + 8 >= ja)
        ib = lax.broadcasted_iota(jnp.int32, (48, 56), 0)
        jb = lax.broadcasted_iota(jnp.int32, (48, 56), 1)
        own = (ib < 40) == (jb < 40)
        mask_b = own & (((jb >= 32) & (jb < 48)) | (jnp.where(jb < 40, jb, jb - 8) <= ib))
        masked = -1e9 / scale
        j8 = lax.broadcasted_iota(jnp.int32, (8, 56), 1)
        fill_b = jnp.concatenate([jnp.where(j8 < 40, masked, -3e38).astype(f32)] * 5
                                 + [jnp.where(j8 < 40, -3e38, masked).astype(f32)], axis=0)

        def softmax(sc, mask, fill):
            sc = jnp.where(mask, sc, fill)
            mx = jnp.max(sc, axis=-1, keepdims=True)
            e = jnp.exp2((sc - mx) * (scale * 1.4426950408889634))
            den = jnp.sum(e, axis=-1, keepdims=True)
            return (e * pl.reciprocal(den, approx=True)).astype(bf16)

        def ride_rows(s, is_b):
            first = s < 2
            if is_b:
                g = [jnp.where(first, -3, -1), 1, 2]
            else:
                g = [jnp.where(first, 1, 0), jnp.where(first, 2, 1), 3]
            return [RIDE * s + 8 * t for t in g]

        def step(s, is_b, lhs_lo, lhs_hi, soft_in, jobs):
            seg = pl.multiple_of((SEG * s + ROFF) % NR, SEG)
            sega = pl.multiple_of(seg - SEG, SEG) if is_b else seg
            wr = [pl.multiple_of((NPRE + RIDE * s + 8 * t + ROFF) % NR, 8) for t in range(3)]
            rd = [pl.multiple_of((r + ROFF) % NR, 8) for r in ride_rows(s, is_b)]
            lhs = jnp.concatenate([lhs_lo, lhs_hi], axis=1)
            QM, P, PART = {}, {}, {}
            mrow = 0 if is_b else MEM
            seg8 = pl.multiple_of(seg + 8, 8)
            seg24 = pl.multiple_of(seg + RIDE, 8)

            def wblk(b, lo, n):
                return pltpu.bitcast(wqkv[b * WP + lo:b * WP + lo + n, :], bf16)

            def qkv_lo(i):
                for m in range(3):
                    PART[(m, i)] = jnp.dot(lhs_lo, wblk(m * H + i, 0, 256), preferred_element_type=f32)

            def qkv(i):
                for m in range(3):
                    b = m * H + i
                    if (m, i) in PART:
                        y = jnp.dot(lhs_hi, wblk(b, 256, 256),
                                    preferred_element_type=f32) + PART.pop((m, i))
                    else:
                        y = jnp.dot(lhs, wblk(b, 0, 512), preferred_element_type=f32)
                    if m < 2:
                        QM[b] = y[0:MEM]
                    if m == 2 or (m == 1 and not is_b):
                        kvm[b - H, mrow:mrow + MEM, :] = y[0:MEM].astype(bf16)
                    for t in range(3):
                        rset(b, wr[t], y[8 + 8 * t:16 + 8 * t])
                return y

            def keys(b):
                if is_b:
                    if b in QM:
                        old = kvm[b - H, MEM:2 * MEM, :].astype(f32)
                        mix = jnp.concatenate([QM.pop(b), old], axis=0).astype(bf16)
                    else:
                        mix = kvm[b - H]
                    return jnp.concatenate([rget(b, seg, SEG), mix, rget(b, sega, 8)], axis=0)
                mk = QM.pop(b).astype(bf16) if b in QM else kvm[b - H, MEM:2 * MEM, :]
                return jnp.concatenate([rget(b, seg, SEG), mk], axis=0)

            def scores(i):
                if is_b:
                    mix = jnp.concatenate([QM.pop(i), rget(i, sega, 8).astype(f32)], axis=0)
                    q = jnp.concatenate([rget(i, seg, SEG), mix.astype(bf16)], axis=0)
                else:
                    mix = jnp.concatenate([rget(i, seg24, 8).astype(f32), QM.pop(i)], axis=0)
                    q = jnp.concatenate([rget(i, seg8, 16), mix.astype(bf16)], axis=0)
                sc = lax.dot_general(q, keys(H + i), (((1,), (1,)), ((), ())),
                                     preferred_element_type=f32)
                P[i] = softmax(sc, mask_b, fill_b) if is_b else softmax(sc, mask_a, masked)

            def pv(i):
                o = jnp.dot(P.pop(i), keys(2 * H + i), preferred_element_type=f32)
                if is_b:
                    rset(i, seg, o[0:SEG])
                    rset(i, sega, o[40:48])
                    lhs_o[i, 0:MEM, :] = o[SEG:L].astype(bf16)
                else:
                    rset(i, seg8, o[0:16])
                    rset(i, seg24, o[16:RIDE])
                    lhs_o[i, 0:MEM, :] = o[RIDE:32].astype(bf16)
                for t in range(3):
                    lhs_o[i, 8 + 8 * t:16 + 8 * t, :] = rget(i, rd[t], 8)

            def wo_lhs(i0, i1):
                return jnp.concatenate([lhs_o[i] for i in range(i0, i1)], axis=1)

            def wo_dot(lo, j, i0, i1):
                r = WO + j * 2048
                w = pltpu.bitcast(wqkv[r + 64 * i0:r + 64 * i1, :], bf16)
                return jnp.dot(lo, w, preferred_element_type=f32)

            def side(t):
                if 0 <= t - DP < H:
                    pv(t - DP)
                if 0 <= t - DS < H:
                    scores(t - DS)

            if soft_in:
                for h in range(KSPLIT):
                    qkv_lo(h)
            for h in range(H):
                y = qkv(h)
                side(h)
                for job in jobs.get(h, []):
                    job(y)
            lo = wo_lhs(0, HS)
            acc = []
            for j in range(8):
                acc.append(wo_dot(lo, j, 0, HS))
                side(H + j)
            lo = wo_lhs(HS, H)
            acc = [wo_dot(lo, j, HS, H) + acc[j] for j in range(8)]
            assert not (QM or P or PART)
            return jnp.concatenate(acc[0:4], axis=1), jnp.concatenate(acc[4:8], axis=1)

        def combine_weights(r):
            r = pl.multiple_of(r, 32)
            ops = _b_operands(*[w7[t, pl.ds(r, 32), :].astype(f32) for t in range(4)])
            for k in (0, 2, 3, 5, 6):
                w7[_BSLOT[k], pl.ds(r, 32), :] = ops[k].astype(bf16)

        def rec_body(it, _):
            @pl.when(it <= T0 // NP)
            def _():
                late = [x_copy(2)] + mlp_copies() + [mod_copy(10), mod_copy(11)]
                nl = -(-len(late) // 4)
                for k in range(4):
                    @pl.when(it == k)
                    def _():
                        for cp in late[k * nl:(k + 1) * nl]:
                            cp.start()

                @pl.when(it == T0 // NP)
                def _():
                    x_copy(2).wait()
                    mlp_wait()
                    mod_copy(10).wait()
                    mod_copy(11).wait()

            lhs_lo = lhs_h[:, 0:512]
            lhs_hi = lhs_h[:, 512:1024]
            for u in range(2 * NP):
                s = it * (2 * NP) + u
                pair = it * NP + u // 2
                jobs = {h: [] for h in range(H)}
                r1 = pl.multiple_of(jnp.minimum(NPRE + RIDE * (s + 1), S - RIDE), 8)
                xn = xbuf[pl.ds(r1, RIDE), :].astype(f32)
                ra = jnp.maximum(pair - 1, 0) * (2 * RIDE)
                if u % 2 == 0:
                    rw = jnp.where(pair < T0, WROWS, (pair - T0) * WCH)
                    for c in range(WCH // 32):
                        jobs[4 + c].append(lambda y, c=c, rw=rw: combine_weights(rw + 32 * c))
                    hn = adaln_a(xn, _zero_after(stage_a16(ra)))
                else:
                    hn = adaln_a(xn)
                    z = _zero_after(hn[0:8], hn[8:16], hn[16:24])
                    stage_a16(ra + 32, _zero_after(stage_a16(ra + 16, z)))
                a_lo, a_hi = step(s, u % 2 == 1, lhs_lo, lhs_hi, u > 0, jobs)
                lhs_lo = jnp.concatenate([a_lo[0:MEM], hn[:, 0:512]], axis=0).astype(bf16)
                lhs_hi = jnp.concatenate([a_hi[0:MEM], hn[:, 512:1024]], axis=0).astype(bf16)
                a = jnp.concatenate([a_lo, a_hi], axis=1)
                rows = [pl.multiple_of(r, 8) for r in ride_rows(s, u % 2 == 1)]
                xs = [xbuf[pl.ds(r, 8), :].astype(f32) for r in rows]
                for t, r in enumerate(rows):
                    xa = xs[t] + modrows(2, 8) * a[8 + 8 * t:16 + 8 * t]
                    xbuf[pl.ds(r, 8), :] = xa.astype(bf16)
            lhs_h[:, 0:512] = lhs_lo
            lhs_h[:, 512:1024] = lhs_hi
            return 0

        _loop("rec", 0, NSEG // (2 * NP), rec_body)

        def wo_tail(i, gacc):
            p0 = pl.multiple_of(i * 128, 128)
            r = pl.multiple_of(S - NPRE + i * 128, 128)
            prev = None
            gacc = list(gacc)
            lo = jnp.concatenate([rget(h, p0, 128) for h in range(H)], axis=1)
            for j in range(8):
                w = pltpu.bitcast(wqkv[WO + j * 2048:WO + (j + 1) * 2048, :], bf16)
                y = jnp.dot(lo, w, preferred_element_type=f32)
                if j < 7:
                    prev = stage_a16(r - 128 + 16 * j, _zero_after(y, prev))
                if j == 0:
                    prev = stage_a16(r - 16, _zero_after(prev))
                if j < 4:
                    z = jnp.concatenate([_zero_after(y)] * 4, axis=1)
                    for c in range(2):
                        gacc[c] = gacc[c] + z
                        for k in range(4):
                            rm = pl.multiple_of(i * 256 + j * 64 + k * 16, 16)
                            gacc[c] = mod_rows(gacc[c], (10 + c) % NMOD, rm)
                cs = slice(j * 128, (j + 1) * 128)
                ga = modrows(2, 128, j * 128, (j + 1) * 128)
                xbuf[pl.ds(r, 128), cs] = (xbuf[pl.ds(r, 128), cs].astype(f32) + ga * y).astype(bf16)
            for c in range(2):
                mod_finish(gacc[c], 10 + c)
            return tuple(gacc)
        _loop("wotail", 0, NPRE // 128, wo_tail, (jnp.zeros((8, 512), f32),) * 2)

    pl.run_scoped(phase1,
                  pltpu.VMEM((WO + 8 * 2048, 128), u32),
                  pltpu.VMEM((NSLOT + NWO, 256, 16, 128), bf16))

    def phase2(gbuf, c7, d7):
        def wop(base, kh, j):
            return lambda k: w7[_BSLOT[k], base + j * kh:base + (j + 1) * kh, :]

        zpad = jnp.zeros((GPAD, 128), f32)
        for cb in range(8):
            gbuf[cb, 0:GPAD, :] = zpad
            gbuf[cb, GPAD + S:GPAD + S + GPAD, :] = zpad

        shifts = (-1, -1, 1, 1, -2, -2, 2, 2)
        HB = MB // 2

        def shift_piece(r, half, k):
            gs = jnp.concatenate([gbuf[c, pl.ds(r + (k * 16 + GPAD + shifts[c]), 16), :]
                                  for c in range(8)], axis=1)
            for t, op in enumerate(row_operands(gs)):
                c7[half, t, k * 8:(k + 1) * 8, :] = op.astype(bf16)

        def gate(v, i):
            gbuf[0, pl.ds(GPAD + S + GPAD + 8 * (i // S), 8), :] = v[0:8]

        d7[:, 0:24, :] = jnp.zeros((7, 24, 512), bf16)

        def b_body(i, _):
            ro = pl.multiple_of(i * HB, HB)
            rg = pl.multiple_of(GPAD + i * MB, 8)
            ra = jnp.minimum(S - 128 + 48 * i, S - 48)
            rp = jnp.minimum(S - 128 + 48 * jnp.maximum(i - 1, 0), S - 48)
            n7[:, pl.ds(pl.multiple_of(rp // 2, 8), 24), :] = d7[:, 0:24, :]
            st = {"n": 0, "prev": None}

            def hook(v):
                n = st["n"]
                st["n"] += 1
                if n % 7 == BH and n // 7 < 3:
                    st["prev"] = stage_a16(ra + 16 * (n // 7), _zero_after(v, st["prev"]),
                                           (d7, 8 * (n // 7)))

            for j in range(4):
                c11, c12, c21, c22 = _strassen(lambda k: n7[k, pl.ds(ro, HB), :],
                                               wop(W1, 512, j), hook)
                gbuf[j + 4, pl.ds(rg, MB), :] = _gelu(_merge_rows(c12, c22))
                gbuf[j, pl.ds(rg, MB), :] = _gelu(_merge_rows(c11, c21))
            return 0
        _loop("b", 0, S // MB, b_body)
        for k in range(HB // 16):
            shift_piece(0, 0, k)

        def stage_n2(r, k, anchor=None):
            rr = pl.multiple_of(r + k * NCH, NCH)
            ops = row_operands(_ln(h2buf[pl.ds(rr, NCH), :], anchor))
            for t, op in enumerate(ops):
                d7[t, k * (NCH // 2):(k + 1) * (NCH // 2), :] = op.astype(bf16)
            return ops[0][0:8] + ops[0][NCH // 2 - 8:NCH // 2]

        def stage_c(i, r, half, rnext):
            rr = pl.multiple_of(r, 8)
            st = {"n": 0, "prev": None}

            def hook(v):
                n = st["n"]
                st["n"] += 1
                if n < HB // 16:
                    gate(v, i)
                    shift_piece(rnext, 1 - half, n)
                if half == 1 and n % 3 == 0 and n // 3 < MD // NCH:
                    st["prev"] = stage_n2(0, n // 3, _zero_after(v, st["prev"]))

            for j in range(4):
                c11, c12, c21, c22 = _strassen(lambda k: c7[half, k], wop(W2, 512, j), hook)
                for c, y in ((j + 4, _merge_rows(c12, c22)), (j, _merge_rows(c11, c21))):
                    cs = slice(c * 128, (c + 1) * 128)
                    h2buf[pl.ds(rr, HB), cs] = h2buf[pl.ds(rr, HB), cs] + y

        def c_body(i, _):
            r = pl.multiple_of(i * MB, MB)
            stage_c(i, r, 0, r + HB)
            stage_c(i, r + HB, 1, jnp.minimum(i + 1, S // MB - 1) * MB)
            return 0
        _loop("c", 0, S // MB, c_body)

        def d_body(i, _):
            r = pl.multiple_of(i * MD, MD)
            rn = jnp.minimum(r + MD, S - MD)
            lhs = [d7[k] for k in range(7)]
            uops = []
            for j in range(14):
                cq = _strassen(lambda k: lhs[k], wop(W3, 512, j))
                uops.append(_a_operands(*[_gelu(c) for c in cq]))
            ul = [jnp.concatenate([u[k] for u in uops], axis=1).astype(bf16) for k in range(7)]
            prev = None
            todo = list(range(MD // NCH))
            for j in range(4):
                c11, c12, c21, c22 = _strassen(lambda k: ul[k], wop(W4, F // 2, j))
                for anc in (c12, c11, c22)[:NANC]:
                    if todo:
                        prev = stage_n2(rn, todo.pop(0), _zero_after(anc, prev))
                for c, y in ((j + 4, _merge_rows(c12, c22)), (j, _merge_rows(c11, c21))):
                    cs = slice(c * 128, (c + 1) * 128)
                    gb = modrows(5, MD, c * 128, (c + 1) * 128)
                    o = xbuf[pl.ds(r, MD), cs].astype(f32) + gb * (h2buf[pl.ds(r, MD), cs] + y)
                    xbuf[pl.ds(r, MD), cs] = o.astype(bf16)
            assert not todo
            out_copy(r, MD).start()
            return 0
        _loop("d", 0, S // MD, d_body)

    pl.run_scoped(phase2,
                  pltpu.VMEM((8, S + 4 * GPAD, 128), f32),
                  pltpu.VMEM((2, 7, MB // 4, 512), bf16),
                  pltpu.VMEM((7, MD // 2, 512), bf16))

    out_copy(0, S).wait()


def _run(x, mem0, wq, wk, wv, wo, w1, w2, w3, w4, c, wmod):
    any_spec = pl.BlockSpec(memory_space=pl.ANY)
    vmem_spec = pl.BlockSpec(memory_space=pltpu.VMEM)
    return pl.pallas_call(
        _kernel,
        out_shape=jax.ShapeDtypeStruct((S, D), bf16),
        in_specs=[any_spec, vmem_spec, any_spec, any_spec, any_spec, any_spec, any_spec,
                  any_spec, any_spec, any_spec, vmem_spec, any_spec],
        out_specs=any_spec,
        scratch_shapes=[
            pltpu.VMEM((S, D), bf16),
            pltpu.VMEM((7, WROWS + WCH, 128), bf16),
            pltpu.VMEM((NMOD, D, 512), bf16),
            [pltpu.VMEM((96 // NRING, NR, 128), bf16)] * NRING,
            pltpu.VMEM((32, D), bf16),
            pltpu.VMEM((H, 32, 128), bf16),
            pltpu.VMEM((2 * H, 16, 128), bf16),
            pltpu.VMEM((12, 8, 512), f32),
            pltpu.VMEM((D, 128), f32),
            pltpu.VMEM((S, D), f32),
            pltpu.VMEM((7, S // 2, 512), bf16),
            pltpu.SemaphoreType.DMA((4 + NMOD + NGRP + 4,)),
        ],
        compiler_params=pltpu.CompilerParams(vmem_limit_bytes=124 * 1024 * 1024),
    )(x, mem0, wq, wk, wv, wo, w1, w2, w3, w4, c, wmod)


def pallas_adaLN_cond__memory_aug_recurrent_mem_tr__mixer_s_mlp__prompt_kernel(
    A_x, A_mem0, A_Wq, A_Wk, A_Wv, A_Wo, A_seg_len, B_x, B_w1, B_w2, B_w3, B_w4, c, w_mod,
):
    del B_x
    assert A_x.shape == (1, S, D) and A_mem0.shape == (1, MEM, D)
    assert isinstance(A_seg_len, int) is False or A_seg_len == SEG
    pairs = (D // 2, 2, H, DH)
    out = _run(A_x.reshape(S, D), A_mem0.reshape(MEM, D), A_Wq.reshape(pairs),
               A_Wk.reshape(pairs), A_Wv.reshape(pairs), A_Wo.reshape(H * DH // 16, 16, D),
               B_w1, B_w2, B_w3, B_w4, c, w_mod)
    return out.reshape(1, S, D)
```

```python
import jax
import jax.numpy as jnp
from jax import lax
import jax.experimental.pallas as pl
import jax.experimental.pallas.tpu as pltpu

bf16 = jnp.bfloat16
f32 = jnp.float32
u32 = jnp.uint32

S = 2048
D = 1024
H = 32
DH = 128
F = 3584
MEM = 8
SEG = 32
NSEG = S // SEG
L = MEM + SEG
RIDE = 24
NPRE = S - RIDE * NSEG
NR = NPRE + 2 * SEG
ROFF = (-(S - NPRE)) % NR
WP = 516
WO = 96 * WP
NGRP = 12
NSLOT = 6
NMOD = 6
EPS = 1e-5
MD = 128
MB = 512
GPAD = 8
NRING = 8
RLP, WLP = 25, 22
NWO = 3
HS, BH, PIN = 24, 0, 6
DS, DP, KSPLIT = 2, 4, 2
X0 = NPRE + 2 * RIDE
GS = S + 4 * GPAD
W4R = 7 * 128
_ONLY = None


def _loop(name, lo, hi, body, init=0):
    if _ONLY is not None and name not in _ONLY:
        return init
    with _scope(name):
        return lax.fori_loop(lo, hi, body, init)


class _NoScope:
    def __init__(self, name):
        del name

    def __enter__(self):
        return self

    def __exit__(self, *a):
        return False


_scope = _NoScope


def _zero_after(*vs):
    bits = None
    for v in vs:
        if v is not None:
            b = pltpu.bitcast(v[0:8, 0:128], u32)
            bits = b if bits is None else bits | b
    return pltpu.bitcast((bits >> 31) >> 1, f32)


def _ln(x, anchor=None):
    if anchor is not None:
        z = jnp.concatenate([anchor] * (x.shape[0] // 8), axis=0)
        x = jnp.concatenate([x[:, 0:128] + z, x[:, 128:]], axis=1)
    mu = jnp.mean(x, axis=-1, keepdims=True)
    xc = x - mu
    var = jnp.mean(xc * xc, axis=-1, keepdims=True)
    return xc * lax.rsqrt(var + EPS)


def _gelu(x):
    inner = x * (0.7978845608028654 + (0.7978845608028654 * 0.044715) * (x * x))
    hx = 0.5 * x
    return hx + hx * jnp.tanh(inner)


def _split_rows(x):
    m, n = x.shape
    x3 = x.reshape(m // 16, 16, n)
    return x3[:, 0:8, :].reshape(m // 2, n), x3[:, 8:16, :].reshape(m // 2, n)


def _merge_rows(top, bot):
    m, n = top.shape
    return jnp.concatenate([top.reshape(m // 8, 8, n), bot.reshape(m // 8, 8, n)],
                           axis=1).reshape(2 * m, n)


def _a_operands(a11, a12, a21, a22):
    return [a11 + a22, a21 + a22, a11, a22, a11 + a12, a21 - a11, a12 - a22]


def _b_operands(b11, b12, b21, b22):
    return [b11 + b22, b11, b12 - b22, b21 - b11, b22, b11 + b12, b21 + b22]


_BTERMS = ((0, 3, 1), (0, None, 0), (1, 3, -1), (2, 0, -1), (3, None, 0), (0, 1, 1), (2, 3, 1))


def _strassen(a_of, b_of, hook=lambda v: None):
    def prod(k):
        return jnp.dot(a_of(k), b_of(k), preferred_element_type=f32)
    p5 = prod(4)
    hook(p5)
    p3 = prod(2)
    hook(p3)
    c12 = p3 + p5
    p1 = prod(0)
    hook(p1)
    c11 = p1 - p5
    c22 = p1 + p3
    p4 = prod(3)
    hook(p4)
    c11 = c11 + p4
    c11 = prod(6) + c11
    hook(c11)
    p2 = prod(1)
    hook(p2)
    c21 = p2 + p4
    c22 = c22 - p2
    c22 = prod(5) + c22
    hook(c22)
    return c11, c12, c21, c22


def _blocks4(v):
    m, n = v.shape
    v3 = v.reshape(m // 32, 32, n)
    rows = [v3[:, 8 * i:8 * i + 8, :].reshape(m // 4, n) for i in range(4)]
    k = n // 4
    return [[r[:, j * k:(j + 1) * k] for j in range(4)] for r in rows]


def _a_operands2(b):
    sub = [_a_operands(b[i][j], b[i][2 + j], b[2 + i][j], b[2 + i][2 + j])
           for i in range(2) for j in range(2)]
    return [_a_operands(*[t[k] for t in sub]) for k in range(7)]


def _strassen2(a_of, b_of, hook=lambda v: None):
    def prod(k1):
        return _strassen(lambda k: a_of(k1, k), lambda k: b_of(k1, k), hook)

    def add(x, y):
        return [p + q for p, q in zip(x, y)]

    def sub(x, y):
        return [p - q for p, q in zip(x, y)]
    p5 = prod(4)
    p3 = prod(2)
    c12 = add(p3, p5)
    p1 = prod(0)
    c11 = sub(p1, p5)
    c22 = add(p1, p3)
    p4 = prod(3)
    c11 = add(add(c11, p4), prod(6))
    p2 = prod(1)
    c21 = add(p2, p4)
    c22 = add(sub(c22, p2), prod(5))
    cq = (c11, c12, c21, c22)
    return [[cq[2 * (i // 2) + j // 2][2 * (i % 2) + j % 2] for j in range(4)] for i in range(4)]


def _packed(v):
    return pltpu.bitcast(v.astype(bf16), u32)


def _kernel(x_hbm, mem0_ref, wq_hbm, wk_hbm, wv_hbm, wo_hbm, w1_hbm, w2_hbm, w3_hbm, w4_hbm,
            c_ref, wmod_hbm, out_hbm,
            xbuf, wqkv, rings, lhs_h, lhs_o, kvm, modv, scol, h2buf, n7, ws3, wsr, t7, d49,
            sems):
    w_hbms = (wq_hbm, wk_hbm, wv_hbm)
    SMOD, SSTG = 5, 9
    sem_x, sem_out, sem_w, sem_g, sem_r = (sems.at[k] for k in range(5))

    def rget(b, row, n):
        return rings[b % NRING][b // NRING, pl.ds(row, n), :]

    def rset(b, row, val):
        rings[b % NRING][b // NRING, pl.ds(row, val.shape[0]), :] = val.astype(bf16)

    x_copy = pltpu.make_async_copy(x_hbm.at[pl.ds(0, X0), :], xbuf.at[pl.ds(0, X0), :], sem_x)

    def stream_copies(c):
        al, lo = ((lambda v, m: v), min) if isinstance(c, int) else (pl.multiple_of, jnp.minimum)
        c3 = lo(c, 27)
        cps = [pltpu.make_async_copy(
            w3_hbm.at[pl.ds(al(i * 256 + (c3 % 4) * 64, 64), 64),
                      pl.ds(al(j * (F // 4) + (c3 // 4) * 128, 128), 128)],
            ws3.at[4 * i + j], sem_w) for i in range(4) for j in range(4)]
        dst = X0 + 2 * RIDE * c
        return [
            pltpu.make_async_copy(w4_hbm.at[:, pl.ds(al(c3 * 32, 32), 32), :],
                                  wsr.at[pl.ds(0, 4)], sem_g),
            pltpu.make_async_copy(w1_hbm.at[:, pl.ds(al(c * 16, 16), 16), :],
                                  wsr.at[pl.ds(4, 2), pl.ds(0, 16), :], sem_g),
            pltpu.make_async_copy(w2_hbm.at[:, pl.ds(al(c * 16, 16), 16), :],
                                  wsr.at[pl.ds(4, 2), pl.ds(16, 16), :], sem_g),
            pltpu.make_async_copy(wmod_hbm.at[pl.ds(al(c * 32, 32), 32), pl.ds(5 * D, D)],
                                  wsr.at[6], sem_g),
            pltpu.make_async_copy(x_hbm.at[pl.ds(al(lo(dst, S - 2 * RIDE), 16), 2 * RIDE), :],
                                  xbuf.at[pl.ds(al(dst, 16), 2 * RIDE), :], sem_r)] + cps

    def stream_wait(c):
        for dst, sem in ((ws3.at[pl.ds(0, 16)], sem_w), (wsr.at[pl.ds(0, 7)], sem_g),
                         (xbuf.at[pl.ds(X0 + 2 * RIDE * c, 2 * RIDE), :], sem_r)):
            pltpu.make_async_copy(dst, dst, sem).wait()

    def out_copy(row, n):
        return pltpu.make_async_copy(xbuf.at[pl.ds(row, n), :], out_hbm.at[pl.ds(row, n), :],
                                     sem_out)

    def mod_rows(acc, w, r):
        sc = jnp.concatenate([scol[pl.ds(r, 16), :]] * (w.shape[1] // 128), axis=1)
        p = w.astype(f32) * sc
        return acc + p[0:8] + p[8:16]

    def mod_finish(acc, j):
        is_scale = jnp.logical_or(j // 2 == 1, j // 2 == 4)
        tot = jnp.sum(acc, axis=0, keepdims=True) + jnp.where(is_scale, 1.0, 0.0)
        modv[j] = jnp.broadcast_to(tot, (8, 512))

    def modrows(k, n, lo=0, hi=D):
        m = jnp.concatenate([modv[2 * k], modv[2 * k + 1]], axis=1)[:, lo:hi]
        return jnp.concatenate([m] * (n // 8), axis=0)

    def adaln_a(xv, anchor=None):
        n = xv.shape[0]
        return _ln(xv, anchor) * modrows(1, n) + modrows(0, n)

    def adaln_b(xv, anchor=None):
        n = xv.shape[0]
        return _ln(xv, anchor) * modrows(4, n) + modrows(3, n)

    def row_operands(v):
        top, bot = _split_rows(v)
        k = v.shape[1] // 2
        return _a_operands(top[:, :k], top[:, k:], bot[:, :k], bot[:, k:])

    def stage_a16(r, anchor=None, dst=None):
        rr = pl.multiple_of(r, 16)
        h2 = adaln_b(xbuf[pl.ds(rr, 16), :].astype(f32), anchor)
        h2buf[pl.ds(rr, 16), :] = h2
        ref, ro = (n7, pl.multiple_of(rr // 2, 8)) if dst is None else dst
        ops = row_operands(_ln(h2))
        for t, op in enumerate(ops):
            ref[t, pl.ds(ro, 8), :] = op.astype(bf16)
        return ops[0]

    def prologue(stg, wmodb):
        def mod_copy(j):
            return pltpu.make_async_copy(wmod_hbm.at[:, pl.ds(j * 512, 512)], wmodb.at[j % NMOD],
                                         sems.at[SSTG + j + 4 if j >= 4 else SMOD + j])

        def piece_copies(g, dh):
            slot = (2 * g + dh) % NSLOT
            return [pltpu.make_async_copy(
                w_hbms[g // 4].at[pl.ds(dh * 256, 256), par, pl.ds((g % 4) * 8, 8), :],
                stg.at[slot, :, pl.ds(par * 8, 8), :],
                sems.at[SSTG + (g + 1 if g else dh)]) for par in range(2)]

        def wo_copy(j):
            slot = NSLOT + j % NWO
            return pltpu.make_async_copy(wo_hbm.at[:, :, pl.ds(j * 128, 128)], stg.at[slot],
                                         sems.at[SSTG + j + 6])

        def group_start(g):
            for dh in range(2):
                for cp in piece_copies(g, dh):
                    cp.start()

        def stg_wait(slot, n, sem):
            dst = stg.at[pl.ds(slot, n)]
            pltpu.make_async_copy(dst, dst, sems.at[SSTG + sem]).wait()

        def relayout(g, slot, dh, lo_dp, n_dp):
            base = g * (8 * WP) + dh * 256
            for u in range(n_dp):
                dp = lo_dp + u
                ev = pltpu.bitcast(stg[slot, dp, 0:8, :].astype(f32), u32)
                od = pltpu.bitcast(stg[slot, dp, 8:16, :].astype(f32), u32)
                wqkv[pl.ds(base + dp, 8, stride=WP), :] = (ev >> 16) | od

        def b_operand(g, q, k):
            def quad(i):
                r = (g * 8 + q + 4 * (i % 2)) * WP + (i // 2) * 256
                return pltpu.bitcast(wqkv[pl.ds(r, 256), :], bf16)
            i, j, sign = _BTERMS[k]
            if j is None:
                return quad(i)
            u, v = quad(i).astype(f32), quad(j).astype(f32)
            return (u + v if sign > 0 else u - v).astype(bf16)

        x_copy.start()
        for j in range(4):
            mod_copy(j).start()
        for g in range(3):
            group_start(g)
        cv = c_ref[...].astype(f32)
        sv = jnp.broadcast_to(cv * (1.0 / (1.0 + jnp.exp(-cv))), (128, D))
        for k in range(8):
            scol[k * 128:(k + 1) * 128, :] = sv[:, k * 128:(k + 1) * 128].T
        x_copy.wait()

        def ln0_body(i, _):
            r = pl.multiple_of(i * 64, 64)
            h2buf[pl.ds(r, 64), :] = _ln(xbuf[pl.ds(r, 64), :].astype(f32))
            return 0
        lax.fori_loop(0, NPRE // 64, ln0_body, 0)

        def mod0_body(j, _):
            pltpu.make_async_copy(wmodb.at[j], wmodb.at[j], sems.at[SMOD + j]).wait()
            accs = [jnp.zeros((8, 512), f32)] * 2
            for k in range(64):
                accs[k % 2] = mod_rows(accs[k % 2], wmodb[j, k * 16:(k + 1) * 16, :], k * 16)
            mod_finish(accs[0] + accs[1], j)
            return 0
        _loop("mod0", 0, 4, mod0_body)

        def hpre_body(i, _):
            r = pl.multiple_of(i * 32, 32)
            hv = h2buf[pl.ds(r, 32), :] * modrows(1, 32) + modrows(0, 32)
            ro = pl.multiple_of(i * 16, 16)
            for t, op in enumerate(row_operands(hv)):
                n7[t, pl.ds(ro, 16), :] = op.astype(bf16)
            return 0
        lax.fori_loop(0, NPRE // 32, hpre_body, 0)
        lhs_h[0:MEM, :] = mem0_ref[...]
        lhs_h[MEM:32, :] = adaln_a(xbuf[NPRE:NPRE + RIDE, :].astype(f32)).astype(bf16)

        def relayout_now(g, dh):
            def rl_body(t, _):
                relayout(g, 2 * g + dh, dh, t * 32, 32)
                return 0
            lax.fori_loop(0, 8, rl_body, 0)

        for dh in range(2):
            stg_wait(dh, 1, dh)
            relayout_now(0, dh)

        grp = lambda g: piece_copies(g, 0) + piece_copies(g, 1)
        issue = {0: [wo_copy(0)], 1: grp(3) + grp(4), 2: grp(5) + [wo_copy(1), mod_copy(4)],
                 3: grp(6) + [wo_copy(2), mod_copy(5)], 4: grp(7) + [mod_copy(6)],
                 5: grp(8) + [wo_copy(3), mod_copy(7)], 6: grp(9) + [wo_copy(4)],
                 7: grp(10) + [wo_copy(5), mod_copy(8)], 8: grp(11) + [wo_copy(6)],
                 9: [wo_copy(7), mod_copy(9)], 10: stream_copies(0)}

        def pre_iter(g, m3):
            m3n = jnp.where(m3 == 2, 0, m3 + 1)
            ends = jnp.logical_or(g == 0, g == NGRP - 1)
            gn = jnp.where(ends, g, g + 1)
            gslot = 2 * jnp.where(ends, m3, m3n)
            wj = jnp.maximum(g - 4, 0)
            wslot = jnp.where(g < 4, gslot, NSLOT + jnp.where(m3 == 0, 2, m3 - 1))
            cj = jnp.maximum(g - 2, 3)
            cslot = jnp.where(cj >= NMOD, cj - NMOD, cj)

            @pl.when(g == 1)
            def _():
                stg_wait(2, 2, 2)
                relayout_now(1, 0)
                relayout_now(1, 1)

            @pl.when(jnp.logical_not(ends))
            def _():
                stg_wait(gslot, 2, g + 2)

            @pl.when(g >= 4)
            def _():
                stg_wait(wslot, 1, g + 2)

            @pl.when(g >= 6)
            def _():
                pltpu.make_async_copy(wmodb.at[cslot], wmodb.at[cslot],
                                      sems.at[SSTG + g + 2]).wait()

            for k, cps in issue.items():
                @pl.when(g == k)
                def _():
                    for cp in cps:
                        cp.start()
            wtodo = list(range(0, 256, 2))
            todo = [(dh, dp) for dh in range(2) for dp in range(256)]
            mtodo = list(range(0, D, 16))
            macc = [jnp.zeros((8, 512), f32)]

            def hook(v):
                if mtodo:
                    acc = macc[0] + jnp.concatenate([_zero_after(v)] * 4, axis=1)
                    for r in mtodo[:3]:
                        acc = mod_rows(acc, wmodb[cslot, r:r + 16, :], r)
                    del mtodo[:3]
                    macc[0] = acc

            for q in range(4):
                def b_of(k):
                    w = b_operand(g, q, k)
                    nw = 0 if todo else WLP
                    for dh, dp in todo[:RLP]:
                        relayout(gn, gslot + dh, dh, dp, 1)
                    del todo[:RLP]
                    for c in wtodo[:nw]:
                        wqkv[pl.ds(pl.multiple_of(WO + wj * 2048 + c * 8, 16), 16), :] = (
                            pltpu.bitcast(stg[wslot, c:c + 2].reshape(32, 128), u32))
                    del wtodo[:nw]
                    return w
                c11, c12, c21, c22 = _strassen(lambda k: n7[k, 0:NPRE // 2, :], b_of, hook)
                for blk, y in ((q + 4, _merge_rows(c12, c22)), (q, _merge_rows(c11, c21))):
                    y = y.astype(bf16)
                    n0 = NR - ROFF
                    rings[blk][g, ROFF:NR, :] = y[0:n0]
                    rings[blk][g, 0:NPRE - n0, :] = y[n0:NPRE]
            assert not todo and not wtodo and not mtodo
            mod_finish(macc[0], cj)
            return m3n

        _loop("pre1", 0, NGRP, pre_iter)

    pl.run_scoped(prologue,
                  pltpu.VMEM((NSLOT + NWO, 256, 16, 128), bf16),
                  pltpu.VMEM((NMOD, D, 512), bf16))

    def main(w7, w49):
        scale = DH ** -0.5
        ia = lax.broadcasted_iota(jnp.int32, (32, L), 0)
        ja = lax.broadcasted_iota(jnp.int32, (32, L), 1)
        mask_a = (ia >= RIDE) | (ja >= SEG) | (ia + 8 >= ja)
        ib = lax.broadcasted_iota(jnp.int32, (48, 56), 0)
        jb = lax.broadcasted_iota(jnp.int32, (48, 56), 1)
        own = (ib < 40) == (jb < 40)
        mask_b = own & (((jb >= 32) & (jb < 48)) | (jnp.where(jb < 40, jb, jb - 8) <= ib))
        masked = -1e9 / scale
        j8 = lax.broadcasted_iota(jnp.int32, (8, 56), 1)
        fill_b = jnp.concatenate([jnp.where(j8 < 40, masked, -3e38).astype(f32)] * 5
                                 + [jnp.where(j8 < 40, -3e38, masked).astype(f32)], axis=0)

        def softmax(sc, mask, fill):
            sc = jnp.where(mask, sc, fill)
            mx = jnp.max(sc, axis=-1, keepdims=True)
            e = jnp.exp2((sc - mx) * (scale * 1.4426950408889634))
            den = jnp.sum(e, axis=-1, keepdims=True)
            return (e * pl.reciprocal(den, approx=True)).astype(bf16)

        def ride_rows(s, is_b):
            first = s < 2
            if is_b:
                g = [jnp.where(first, -3, -1), 1, 2]
            else:
                g = [jnp.where(first, 1, 0), jnp.where(first, 2, 1), 3]
            return [RIDE * s + 8 * t for t in g]

        def step(s, is_b, lhs_lo, lhs_hi, soft_in, jobs):
            seg = pl.multiple_of((SEG * s + ROFF) % NR, SEG)
            sega = pl.multiple_of(seg - SEG, SEG) if is_b else seg
            wr = [pl.multiple_of((NPRE + RIDE * s + 8 * t + ROFF) % NR, 8) for t in range(3)]
            rd = [pl.multiple_of((r + ROFF) % NR, 8) for r in ride_rows(s, is_b)]
            lhs = jnp.concatenate([lhs_lo, lhs_hi], axis=1)
            QM, P, PART = {}, {}, {}
            mrow = 0 if is_b else MEM
            seg8 = pl.multiple_of(seg + 8, 8)
            seg24 = pl.multiple_of(seg + RIDE, 8)

            def wblk(b, lo, n):
                return pltpu.bitcast(wqkv[b * WP + lo:b * WP + lo + n, :], bf16)

            def qkv_lo(i):
                for m in range(3):
                    PART[(m, i)] = jnp.dot(lhs_lo, wblk(m * H + i, 0, 256), preferred_element_type=f32)

            def qkv(i):
                for m in range(3):
                    b = m * H + i
                    if (m, i) in PART:
                        y = jnp.dot(lhs_hi, wblk(b, 256, 256),
                                    preferred_element_type=f32) + PART.pop((m, i))
                    else:
                        y = jnp.dot(lhs, wblk(b, 0, 512), preferred_element_type=f32)
                    if m < 2:
                        QM[b] = y[0:MEM] + jobs["pin"] if b == PIN and is_b else y[0:MEM]
                    if m == 2 or (m == 1 and not is_b):
                        kvm[b - H, mrow:mrow + MEM, :] = y[0:MEM].astype(bf16)
                    for t in range(3):
                        rset(b, wr[t], y[8 + 8 * t:16 + 8 * t])
                    if (i, m) in jobs:
                        jobs[(i, m)](y)

            def keys(b):
                if is_b:
                    if b in QM:
                        old = kvm[b - H, MEM:2 * MEM, :].astype(f32)
                        mix = jnp.concatenate([QM.pop(b), old], axis=0).astype(bf16)
                    else:
                        mix = kvm[b - H]
                    return jnp.concatenate([rget(b, seg, SEG), mix, rget(b, sega, 8)], axis=0)
                mk = QM.pop(b).astype(bf16) if b in QM else kvm[b - H, MEM:2 * MEM, :]
                return jnp.concatenate([rget(b, seg, SEG), mk], axis=0)

            def scores(i):
                if is_b:
                    mix = jnp.concatenate([QM.pop(i), rget(i, sega, 8).astype(f32)], axis=0)
                    q = jnp.concatenate([rget(i, seg, SEG), mix.astype(bf16)], axis=0)
                else:
                    mix = jnp.concatenate([rget(i, seg24, 8).astype(f32), QM.pop(i)], axis=0)
                    q = jnp.concatenate([rget(i, seg8, 16), mix.astype(bf16)], axis=0)
                sc = lax.dot_general(q, keys(H + i), (((1,), (1,)), ((), ())),
                                     preferred_element_type=f32)
                P[i] = softmax(sc, mask_b, fill_b) if is_b else softmax(sc, mask_a, masked)

            def pv(i):
                o = jnp.dot(P.pop(i), keys(2 * H + i), preferred_element_type=f32)
                if is_b:
                    rset(i, seg, o[0:SEG])
                    rset(i, sega, o[40:48])
                    lhs_o[i, 0:MEM, :] = o[SEG:L].astype(bf16)
                else:
                    rset(i, seg8, o[0:16])
                    rset(i, seg24, o[16:RIDE])
                    lhs_o[i, 0:MEM, :] = o[RIDE:32].astype(bf16)
                for t in range(3):
                    lhs_o[i, 8 + 8 * t:16 + 8 * t, :] = rget(i, rd[t], 8)

            def wo_lhs(i0, i1):
                return jnp.concatenate([lhs_o[i] for i in range(i0, i1)], axis=1)

            def wo_dot(lo, j, i0, i1):
                r = WO + j * 2048
                w = pltpu.bitcast(wqkv[r + 64 * i0:r + 64 * i1, :], bf16)
                return jnp.dot(lo, w, preferred_element_type=f32)

            def side(t):
                if 0 <= t - DP < H:
                    pv(t - DP)
                if 0 <= t - DS < H:
                    scores(t - DS)

            if soft_in:
                for h in range(KSPLIT):
                    qkv_lo(h)
            for h in range(H):
                qkv(h)
                side(h)
            lo = wo_lhs(0, HS)
            acc = []
            for j in range(8):
                acc.append(wo_dot(lo, j, 0, HS))
                side(H + j)
            lo = wo_lhs(HS, H)
            acc = [wo_dot(lo, j, HS, H) + acc[j] for j in range(8)]
            assert not (QM or P or PART)
            return jnp.concatenate(acc[0:4], axis=1), jnp.concatenate(acc[4:8], axis=1)

        def combine12(c, m, t):
            blk = [wsr[4 + i, m * 16:(m + 1) * 16, j * 512 + t * 128:j * 512 + (t + 1) * 128]
                   .astype(f32) for i in range(2) for j in range(2)]
            r = pl.multiple_of((4 * m + t) * 256 + c * 8, 8)
            for k, op in enumerate(_b_operands(*blk)):
                w7[k, pl.ds(r, 8), :] = _packed(op)

        def combine34(c, m, p, k1):
            c3 = jnp.minimum(c, 27)
            if m == 0:
                get = lambda i, j: ws3[4 * i + j, p * 16:(p + 1) * 16, :]
                r = c3 * 32 + p * 8
            else:
                t, g = divmod(p, 2)
                get = lambda i, j: wsr[i, g * 16:(g + 1) * 16,
                                       j * 256 + t * 128:j * 256 + (t + 1) * 128]
                r = W4R + t * 448 + c3 * 16 + g * 8

            def quad(q):
                return [get(2 * (q // 2) + i, 2 * (q % 2) + j).astype(f32)
                        for i in range(2) for j in range(2)]
            qi, qj, sign = _BTERMS[k1]
            blk = quad(qi)
            if qj is not None:
                blk = [u + v if sign > 0 else u - v for u, v in zip(blk, quad(qj))]
            for k, op in enumerate(_b_operands(*blk)):
                w49[7 * k1 + k, pl.ds(pl.multiple_of(r, 8), 8), :] = _packed(op)

        def combine(c, n, y):
            mp, k1 = divmod(n, 8)
            m, p = divmod(mp, 4)
            spare = pl.ds(pl.multiple_of(8 * (c // 64), 8), 8)
            if m == 0 and k1 < 7:
                ws3[16, spare, :] = y[0:8].astype(bf16)
            else:
                wsr[7, spare, 0:128] = y[0:8].astype(bf16)
            if k1 == 7:
                combine12(c, m, p)
            else:
                combine34(c, m, p, k1)

        def rec_body(it, gacc):
            stream_wait(it)
            lhs_lo = lhs_h[:, 0:512]
            lhs_hi = lhs_h[:, 512:1024]
            ra = jnp.maximum(it - 1, 0) * (2 * RIDE)
            for u in range(2):
                s = 2 * it + u
                jobs = {}
                r1 = pl.multiple_of(jnp.minimum(NPRE + RIDE * (s + 1), S - RIDE), 8)
                xn = xbuf[pl.ds(r1, RIDE), :].astype(f32)
                if u == 0:
                    for k in range(2):
                        rm = pl.multiple_of(it * 32 + k * 16, 16)
                        gacc = mod_rows(gacc, wsr[6, k * 16:(k + 1) * 16, :], rm)
                    for n in range(64):
                        jobs[(n // 2, 2 * (n % 2))] = lambda y, n=n: combine(it, n, y)
                    hn = adaln_a(xn, _zero_after(stage_a16(ra)))
                else:
                    for cp in stream_copies(jnp.minimum(it + 1, NSEG // 2 - 1)):
                        cp.start()
                    spare = pl.ds(pl.multiple_of(8 * (it // 64), 8), 8)
                    jobs["pin"] = _zero_after(ws3[16, spare, :].astype(f32))
                    hn = adaln_a(xn)
                    z = _zero_after(hn[0:8], hn[8:16], hn[16:24])
                    stage_a16(ra + 32, _zero_after(stage_a16(ra + 16, z)))
                a_lo, a_hi = step(s, u == 1, lhs_lo, lhs_hi, u > 0, jobs)
                lhs_lo = jnp.concatenate([a_lo[0:MEM], hn[:, 0:512]], axis=0).astype(bf16)
                lhs_hi = jnp.concatenate([a_hi[0:MEM], hn[:, 512:1024]], axis=0).astype(bf16)
                a = jnp.concatenate([a_lo, a_hi], axis=1)
                rows = [pl.multiple_of(r, 8) for r in ride_rows(s, u == 1)]
                xs = [xbuf[pl.ds(r, 8), :].astype(f32) for r in rows]
                for t, r in enumerate(rows):
                    xa = xs[t] + modrows(2, 8) * a[8 + 8 * t:16 + 8 * t]
                    xbuf[pl.ds(r, 8), :] = xa.astype(bf16)
            lhs_h[:, 0:512] = lhs_lo
            lhs_h[:, 512:1024] = lhs_hi
            return gacc

        gacc = _loop("rec", 0, NSEG // 2, rec_body, jnp.zeros((8, D), f32))
        for c in range(2):
            mod_finish(gacc[:, c * 512:(c + 1) * 512], 10 + c)
        stream_wait(NSEG // 2 - 1)

        def wo_tail(i, _):
            p0 = pl.multiple_of(i * 128, 128)
            r = pl.multiple_of(S - NPRE + i * 128, 128)
            prev = None
            lo = jnp.concatenate([rget(h, p0, 128) for h in range(H)], axis=1)
            for j in range(8):
                w = pltpu.bitcast(wqkv[WO + j * 2048:WO + (j + 1) * 2048, :], bf16)
                y = jnp.dot(lo, w, preferred_element_type=f32)
                if j < 7:
                    prev = stage_a16(r - 128 + 16 * j, _zero_after(y, prev))
                if j == 0:
                    prev = stage_a16(r - 16, _zero_after(prev))
                cs = slice(j * 128, (j + 1) * 128)
                ga = modrows(2, 128, j * 128, (j + 1) * 128)
                xbuf[pl.ds(r, 128), cs] = (xbuf[pl.ds(r, 128), cs].astype(f32) + ga * y).astype(bf16)
            return 0
        _loop("wotail", 0, NPRE // 128, wo_tail)

        def gget(c, row, n):
            return pltpu.bitcast(wqkv[pl.ds(c * GS + row, n), :], f32)

        def gset(c, row, val):
            wqkv[pl.ds(c * GS + row, val.shape[0]), :] = pltpu.bitcast(val, u32)

        def wop(j):
            return lambda k: pltpu.bitcast(w7[k, j * 256:(j + 1) * 256, :], bf16)

        zpad = jnp.zeros((GPAD, 128), f32)
        for cb in range(8):
            gset(cb, 0, zpad)
            gset(cb, GPAD + S, zpad)

        shifts = (-1, -1, 1, 1, -2, -2, 2, 2)
        HB = MB // 2

        def shift_piece(r, half, k):
            gs = jnp.concatenate([gget(c, r + (k * 16 + GPAD + shifts[c]), 16)
                                  for c in range(8)], axis=1)
            ro = half * (HB // 2) + k * 8
            for t, op in enumerate(row_operands(gs)):
                n7[t, ro:ro + 8, :] = op.astype(bf16)

        def gate(v, i):
            gset(0, GPAD + S + GPAD + 8 * (i // S), v[0:8])

        t7[...] = jnp.zeros(t7.shape, bf16)

        def b_body(i, _):
            ro = pl.multiple_of(i * HB, HB)
            rg = pl.multiple_of(GPAD + i * MB, 8)
            ra = jnp.minimum(S - 128 + 48 * i, S - 48)
            rp = jnp.minimum(S - 128 + 48 * jnp.maximum(i - 1, 0), S - 48)
            n7[:, pl.ds(pl.multiple_of(rp // 2, 8), 24), :] = t7[...]
            st = {"n": 0, "prev": None}

            def hook(v):
                n = st["n"]
                st["n"] += 1
                if n % 7 == BH and n // 7 < 3:
                    st["prev"] = stage_a16(ra + 16 * (n // 7), _zero_after(v, st["prev"]),
                                           (t7, 8 * (n // 7)))

            for j in range(4):
                c11, c12, c21, c22 = _strassen(lambda k: n7[k, pl.ds(ro, HB), :], wop(j), hook)
                gset(j + 4, rg, _gelu(_merge_rows(c12, c22)))
                gset(j, rg, _gelu(_merge_rows(c11, c21)))
            return 0
        _loop("b", 0, S // MB, b_body)
        for k in range(HB // 16):
            shift_piece(0, 0, k)

        def stage_n2(r, k, anchor=None):
            rr = pl.multiple_of(r + k * 32, 32)
            ops = _a_operands2(_blocks4(_ln(h2buf[pl.ds(rr, 32), :], anchor)))
            for k1 in range(7):
                for k2 in range(7):
                    d49[7 * k1 + k2, k * 8:(k + 1) * 8, :] = ops[k1][k2].astype(bf16)
            return ops[0][0]

        def stage_c(i, r, half, rnext):
            rr = pl.multiple_of(r, 8)
            ro = half * (HB // 2)
            st = {"n": 0, "prev": None}

            def hook(v):
                n = st["n"]
                st["n"] += 1
                if n < HB // 16:
                    gate(v, i)
                    shift_piece(rnext, 1 - half, n)
                if half == 1 and n % 6 == 0 and n // 6 < MD // 32:
                    st["prev"] = stage_n2(0, n // 6, _zero_after(v, st["prev"]))

            for j in range(4):
                c11, c12, c21, c22 = _strassen(lambda k: n7[k, ro:ro + HB // 2, :], wop(4 + j),
                                               hook)
                for c, y in ((j + 4, _merge_rows(c12, c22)), (j, _merge_rows(c11, c21))):
                    cs = slice(c * 128, (c + 1) * 128)
                    h2buf[pl.ds(rr, HB), cs] = h2buf[pl.ds(rr, HB), cs] + y

        def c_body(i, _):
            r = pl.multiple_of(i * MB, MB)
            stage_c(i, r, 0, r + HB)
            stage_c(i, r + HB, 1, jnp.minimum(i + 1, S // MB - 1) * MB)
            return 0
        _loop("c", 0, S // MB, c_body)

        def wop2(lo, n):
            return lambda k1, k: pltpu.bitcast(w49[7 * k1 + k, lo:lo + n, :], bf16)

        def d_body(i, _):
            r = pl.multiple_of(i * MD, MD)
            rn = jnp.minimum(r + MD, S - MD)
            lhs = [d49[k] for k in range(49)]
            uops = []
            for t in range(7):
                cb = _strassen2(lambda k1, k: lhs[7 * k1 + k], wop2(t * 128, 128))
                uops.append(_a_operands2([[_gelu(c) for c in row] for row in cb]))
            ul = [[jnp.concatenate([u[k1][k] for u in uops], axis=1).astype(bf16)
                   for k in range(7)] for k1 in range(7)]
            st = {"n": 0, "prev": None}

            def hook(v):
                n = st["n"]
                st["n"] += 1
                if n % 21 == 6 and n // 21 < MD // 32:
                    st["prev"] = stage_n2(rn, n // 21, _zero_after(v, st["prev"]))

            for t in range(2):
                cb = _strassen2(lambda k1, k: ul[k1][k], wop2(W4R + t * 448, 448), hook)
                for j in range(4):
                    y = jnp.concatenate([cb[q][j].reshape(MD // 32, 8, 128) for q in range(4)],
                                        axis=1).reshape(MD, 128)
                    c = 2 * j + t
                    cs = slice(c * 128, (c + 1) * 128)
                    gb = modrows(5, MD, c * 128, (c + 1) * 128)
                    o = xbuf[pl.ds(r, MD), cs].astype(f32) + gb * (h2buf[pl.ds(r, MD), cs] + y)
                    xbuf[pl.ds(r, MD), cs] = o.astype(bf16)
            out_copy(r, MD).start()
            return 0
        _loop("d", 0, S // MD, d_body)

    pl.run_scoped(main,
                  pltpu.VMEM((7, 8 * 256, 128), u32),
                  pltpu.VMEM((49, 2 * W4R, 128), u32))

    out_copy(0, S).wait()


def _run(x, mem0, wq, wk, wv, wo, w1, w2, w3, w4, c, wmod):
    any_spec = pl.BlockSpec(memory_space=pl.ANY)
    vmem_spec = pl.BlockSpec(memory_space=pltpu.VMEM)
    return pl.pallas_call(
        _kernel,
        out_shape=jax.ShapeDtypeStruct((S, D), bf16),
        in_specs=[any_spec, vmem_spec, any_spec, any_spec, any_spec, any_spec, any_spec,
                  any_spec, any_spec, any_spec, vmem_spec, any_spec],
        out_specs=any_spec,
        scratch_shapes=[
            pltpu.VMEM((S + 2 * RIDE, D), bf16),
            pltpu.VMEM((WO + 8 * 2048, 128), u32),
            [pltpu.VMEM((96 // NRING, NR, 128), bf16)] * NRING,
            pltpu.VMEM((32, D), bf16),
            pltpu.VMEM((H, 32, 128), bf16),
            pltpu.VMEM((2 * H, 16, 128), bf16),
            pltpu.VMEM((12, 8, 512), f32),
            pltpu.VMEM((D, 128), f32),
            pltpu.VMEM((S, D), f32),
            pltpu.VMEM((7, S // 2, 512), bf16),
            pltpu.VMEM((17, 64, 128), bf16),
            pltpu.VMEM((8, 32, D), bf16),
            pltpu.VMEM((7, 24, 512), bf16),
            pltpu.VMEM((49, MD // 4, 256), bf16),
            pltpu.SemaphoreType.DMA((9 + NGRP + 2,)),
        ],
        compiler_params=pltpu.CompilerParams(vmem_limit_bytes=124 * 1024 * 1024,
                                             disable_bounds_checks=True),
    )(x, mem0, wq, wk, wv, wo, w1, w2, w3, w4, c, wmod)


def pallas_adaLN_cond__memory_aug_recurrent_mem_tr__mixer_s_mlp__prompt_kernel(
    A_x, A_mem0, A_Wq, A_Wk, A_Wv, A_Wo, A_seg_len, B_x, B_w1, B_w2, B_w3, B_w4, c, w_mod,
):
    del B_x
    assert A_x.shape == (1, S, D) and A_mem0.shape == (1, MEM, D)
    assert isinstance(A_seg_len, int) is False or A_seg_len == SEG
    pairs = (D // 2, 2, H, DH)
    out = _run(A_x.reshape(S, D), A_mem0.reshape(MEM, D), A_Wq.reshape(pairs),
               A_Wk.reshape(pairs), A_Wv.reshape(pairs), A_Wo.reshape(H * DH // 16, 16, D),
               B_w1.reshape(2, D // 2, D), B_w2.reshape(2, D // 2, D),
               B_w3, B_w4.reshape(4, F // 4, D), c, w_mod)
    return out.reshape(1, S, D)
```

```python
import jax
import jax.numpy as jnp
from jax import lax
import jax.experimental.pallas as pl
import jax.experimental.pallas.tpu as pltpu

bf16 = jnp.bfloat16
f32 = jnp.float32
u32 = jnp.uint32

S = 2048
D = 1024
H = 32
DH = 128
F = 3584
MEM = 8
SEG = 32
NSEG = S // SEG
L = MEM + SEG
RIDE = 24
NPRE = S - RIDE * NSEG
NR = NPRE + 2 * SEG
ROFF = (-(S - NPRE)) % NR
WP = 516
WO = 96 * WP
NGRP = 12
NSLOT = 6
NMOD = 6
EPS = 1e-5
MD = 128
MB = 512
GPAD = 8
NRING = 8
RLP, WLP = 25, 22
NWO = 3
BH, PIN = 0, 6
DF, DG, DL = 8, 9, 9
SLOTS = ([(0, n // 2, 3 * (n % 2)) for n in range(16)] + [(0, 96 + n, 0) for n in range(16)]
         + [(0, 112 + n // 2, 3 * (n % 2)) for n in range(32)])
DSA, DPA, DSB, DPB, KSPLIT = 2, 4, 2, 4, 2
X0 = NPRE + 2 * RIDE
GS = S + 4 * GPAD
W4R = 7 * 128
_ONLY = None


def _loop(name, lo, hi, body, init=0):
    if _ONLY is not None and name not in _ONLY:
        return init
    with _scope(name):
        return lax.fori_loop(lo, hi, body, init)


class _NoScope:
    def __init__(self, name):
        del name

    def __enter__(self):
        return self

    def __exit__(self, *a):
        return False


_scope = _NoScope


def _zero_after(*vs):
    bits = None
    for v in vs:
        if v is not None:
            b = pltpu.bitcast(v[0:8, 0:128], u32)
            bits = b if bits is None else bits | b
    return pltpu.bitcast((bits >> 31) >> 1, f32)


def _ln(x, anchor=None):
    if anchor is not None:
        z = jnp.concatenate([anchor] * (x.shape[0] // 8), axis=0)
        x = jnp.concatenate([x[:, 0:128] + z, x[:, 128:]], axis=1)
    mu = jnp.mean(x, axis=-1, keepdims=True)
    xc = x - mu
    var = jnp.mean(xc * xc, axis=-1, keepdims=True)
    return xc * lax.rsqrt(var + EPS)


def _gelu(x):
    inner = x * (0.7978845608028654 + (0.7978845608028654 * 0.044715) * (x * x))
    hx = 0.5 * x
    return hx + hx * jnp.tanh(inner)


def _split_rows(x):
    m, n = x.shape
    x3 = x.reshape(m // 16, 16, n)
    return x3[:, 0:8, :].reshape(m // 2, n), x3[:, 8:16, :].reshape(m // 2, n)


def _merge_rows(top, bot):
    m, n = top.shape
    return jnp.concatenate([top.reshape(m // 8, 8, n), bot.reshape(m // 8, 8, n)],
                           axis=1).reshape(2 * m, n)


def _a_operands(a11, a12, a21, a22):
    return [a11 + a22, a21 + a22, a11, a22, a11 + a12, a21 - a11, a12 - a22]


def _b_operands(b11, b12, b21, b22):
    return [b11 + b22, b11, b12 - b22, b21 - b11, b22, b11 + b12, b21 + b22]


_ATERMS = ((0, 3, 1), (2, 3, 1), (0, None, 0), (3, None, 0), (0, 1, 1), (2, 0, -1), (1, 3, -1))
_BTERMS = ((0, 3, 1), (0, None, 0), (1, 3, -1), (2, 0, -1), (3, None, 0), (0, 1, 1), (2, 3, 1))


def _strassen(a_of, b_of, hook=lambda v: None):
    def prod(k):
        return jnp.dot(a_of(k), b_of(k), preferred_element_type=f32)
    p5 = prod(4)
    hook(p5)
    p3 = prod(2)
    hook(p3)
    c12 = p3 + p5
    p4 = prod(3)
    hook(p4)
    c11 = p4 - p5
    p2 = prod(1)
    hook(p2)
    c21 = p2 + p4
    c22 = p3 - p2
    p1 = prod(0)
    hook(p1)
    c11 = prod(6) + (c11 + p1)
    hook(c11)
    c22 = prod(5) + (c22 + p1)
    hook(c22)
    return c11, c12, c21, c22


def _a_operands2(b):
    sub = [_a_operands(b[i][j], b[i][2 + j], b[2 + i][j], b[2 + i][2 + j])
           for i in range(2) for j in range(2)]
    return [_a_operands(*[t[k] for t in sub]) for k in range(7)]


def _strassen2(a_of, b_of, hook=lambda v: None):
    def prod(k1):
        return _strassen(lambda k: a_of(k1, k), lambda k: b_of(k1, k), hook)

    def add(x, y):
        return [p + q for p, q in zip(x, y)]

    def sub(x, y):
        return [p - q for p, q in zip(x, y)]
    p5 = prod(4)
    p3 = prod(2)
    c12 = add(p3, p5)
    p4 = prod(3)
    c11 = sub(p4, p5)
    p2 = prod(1)
    c21 = add(p2, p4)
    c22 = sub(p3, p2)
    p1 = prod(0)
    c11 = add(add(c11, p1), prod(6))
    c22 = add(add(c22, p1), prod(5))
    cq = (c11, c12, c21, c22)
    return [[cq[2 * (i // 2) + j // 2][2 * (i % 2) + j % 2] for j in range(4)] for i in range(4)]


def _kernel(x_hbm, mem0_ref, wq_hbm, wk_hbm, wv_hbm, wo_hbm, w1_hbm, w2_hbm, w3_hbm, w4_hbm,
            c_ref, wmod_hbm, out_hbm,
            xbuf, wqkv, rings, lhs_h, lhs_o, kvm, modv, scol, h2buf, n7, ws3, wsr, tpk, t7, d49, nrms,
            sems):
    w_hbms = (wq_hbm, wk_hbm, wv_hbm)
    SMOD, SSTG = 5, 9
    sem_x, sem_out, sem_w, sem_g, sem_r = (sems.at[k] for k in range(5))

    def rget(b, row, n):
        return rings[b % NRING][b // NRING, pl.ds(row, n), :]

    def rset(b, row, val):
        rings[b % NRING][b // NRING, pl.ds(row, val.shape[0]), :] = val.astype(bf16)

    x_copy = pltpu.make_async_copy(x_hbm.at[pl.ds(0, X0), :], xbuf.at[pl.ds(0, X0), :], sem_x)

    def stream_copies(c):
        al, lo = ((lambda v, m: v), min) if isinstance(c, int) else (pl.multiple_of, jnp.minimum)
        c3 = lo(c, 27)
        cps = [pltpu.make_async_copy(
            w3_hbm.at[pl.ds(al(i * 256 + (c3 % 4) * 64, 64), 64),
                      pl.ds(al(j * (F // 4) + (c3 // 4) * 128, 128), 128)],
            ws3.at[4 * i + j], sem_w) for i in range(4) for j in range(4)]
        dst = X0 + 2 * RIDE * c
        return [
            pltpu.make_async_copy(w4_hbm.at[:, pl.ds(al(c3 * 32, 32), 32), :],
                                  wsr.at[pl.ds(0, 4)], sem_g),
            pltpu.make_async_copy(w1_hbm.at[:, pl.ds(al(c * 16, 16), 16), :],
                                  wsr.at[pl.ds(4, 2), pl.ds(0, 16), :], sem_g),
            pltpu.make_async_copy(w2_hbm.at[:, pl.ds(al(c * 16, 16), 16), :],
                                  wsr.at[pl.ds(4, 2), pl.ds(16, 16), :], sem_g),
            pltpu.make_async_copy(wmod_hbm.at[pl.ds(al(c * 32, 32), 32), pl.ds(5 * D, D)],
                                  wsr.at[6], sem_g),
            pltpu.make_async_copy(x_hbm.at[pl.ds(al(lo(dst, S - 2 * RIDE), 16), 2 * RIDE), :],
                                  xbuf.at[pl.ds(al(dst, 16), 2 * RIDE), :], sem_r)] + cps

    def stream_wait(c):
        for dst, sem in ((ws3.at[pl.ds(0, 16)], sem_w), (wsr.at[pl.ds(0, 7)], sem_g),
                         (xbuf.at[pl.ds(X0 + 2 * RIDE * c, 2 * RIDE), :], sem_r)):
            pltpu.make_async_copy(dst, dst, sem).wait()

    def out_copy(row, n):
        return pltpu.make_async_copy(xbuf.at[pl.ds(row, n), :], out_hbm.at[pl.ds(row, n), :],
                                     sem_out)

    def mod_rows(acc, w, r):
        sc = jnp.concatenate([scol[pl.ds(r, 16), :]] * (w.shape[1] // 128), axis=1)
        p = w.astype(f32) * sc
        return acc + p[0:8] + p[8:16]

    def mod_finish(acc, j):
        is_scale = jnp.logical_or(j // 2 == 1, j // 2 == 4)
        tot = jnp.sum(acc, axis=0, keepdims=True) + jnp.where(is_scale, 1.0, 0.0)
        modv[j] = jnp.broadcast_to(tot, (8, 512))

    def modrows(k, n, lo=0, hi=D):
        m = jnp.concatenate([modv[2 * k], modv[2 * k + 1]], axis=1)[:, lo:hi]
        return jnp.concatenate([m] * (n // 8), axis=0)

    def adaln_a(xv, anchor=None):
        n = xv.shape[0]
        return _ln(xv, anchor) * modrows(1, n) + modrows(0, n)

    def adaln_b(xv, anchor=None):
        n = xv.shape[0]
        return _ln(xv, anchor) * modrows(4, n) + modrows(3, n)

    def row_operands(v):
        top, bot = _split_rows(v)
        k = v.shape[1] // 2
        return _a_operands(top[:, :k], top[:, k:], bot[:, :k], bot[:, k:])

    def stage_a16(r, anchor=None, dst=None):
        rr = pl.multiple_of(r, 16)
        h2 = adaln_b(xbuf[pl.ds(rr, 16), :].astype(f32), anchor)
        h2buf[pl.ds(rr, 16), :] = h2
        ref, ro = (n7, pl.multiple_of(rr // 2, 8)) if dst is None else dst
        ops = row_operands(_ln(h2))
        for t, op in enumerate(ops):
            ref[t, pl.ds(ro, 8), :] = op.astype(bf16)
        return ops[0]

    def prologue(stg, wmodb):
        def mod_copy(j):
            return pltpu.make_async_copy(wmod_hbm.at[:, pl.ds(j * 512, 512)], wmodb.at[j % NMOD],
                                         sems.at[SSTG + j + 4 if j >= 4 else SMOD + j])

        def piece_copies(g, dh):
            slot = (2 * g + dh) % NSLOT
            return [pltpu.make_async_copy(
                w_hbms[g // 4].at[pl.ds(dh * 256, 256), par, pl.ds((g % 4) * 8, 8), :],
                stg.at[slot, :, pl.ds(par * 8, 8), :],
                sems.at[SSTG + (g + 1 if g else dh)]) for par in range(2)]

        def wo_copy(j):
            slot = NSLOT + j % NWO
            return pltpu.make_async_copy(wo_hbm.at[:, :, pl.ds(j * 128, 128)], stg.at[slot],
                                         sems.at[SSTG + j + 6])

        def group_start(g):
            for dh in range(2):
                for cp in piece_copies(g, dh):
                    cp.start()

        def stg_wait(slot, n, sem):
            dst = stg.at[pl.ds(slot, n)]
            pltpu.make_async_copy(dst, dst, sems.at[SSTG + sem]).wait()

        def relayout(g, slot, dh, lo_dp, n_dp):
            base = g * (8 * WP) + dh * 256
            for u in range(n_dp):
                dp = lo_dp + u
                ev = pltpu.bitcast(stg[slot, dp, 0:8, :].astype(f32), u32)
                od = pltpu.bitcast(stg[slot, dp, 8:16, :].astype(f32), u32)
                wqkv[pl.ds(base + dp, 8, stride=WP), :] = (ev >> 16) | od

        def b_operand(g, q, k):
            def quad(i):
                r = (g * 8 + q + 4 * (i % 2)) * WP + (i // 2) * 256
                return pltpu.bitcast(wqkv[pl.ds(r, 256), :], bf16)
            i, j, sign = _BTERMS[k]
            if j is None:
                return quad(i)
            u, v = quad(i).astype(f32), quad(j).astype(f32)
            return (u + v if sign > 0 else u - v).astype(bf16)

        x_copy.start()
        for j in range(4):
            mod_copy(j).start()
        for g in range(3):
            group_start(g)
        cv = c_ref[...].astype(f32)
        sv = jnp.broadcast_to(cv * (1.0 / (1.0 + jnp.exp(-cv))), (128, D))
        for k in range(8):
            scol[k * 128:(k + 1) * 128, :] = sv[:, k * 128:(k + 1) * 128].T
        x_copy.wait()

        def ln0_body(i, _):
            r = pl.multiple_of(i * 64, 64)
            h2buf[pl.ds(r, 64), :] = _ln(xbuf[pl.ds(r, 64), :].astype(f32))
            return 0
        lax.fori_loop(0, NPRE // 64, ln0_body, 0)

        def mod0_body(j, _):
            pltpu.make_async_copy(wmodb.at[j], wmodb.at[j], sems.at[SMOD + j]).wait()
            accs = [jnp.zeros((8, 512), f32)] * 2
            for k in range(64):
                accs[k % 2] = mod_rows(accs[k % 2], wmodb[j, k * 16:(k + 1) * 16, :], k * 16)
            mod_finish(accs[0] + accs[1], j)
            return 0
        _loop("mod0", 0, 4, mod0_body)

        def hpre_body(i, _):
            r = pl.multiple_of(i * 32, 32)
            hv = h2buf[pl.ds(r, 32), :] * modrows(1, 32) + modrows(0, 32)
            ro = pl.multiple_of(i * 16, 16)
            for t, op in enumerate(row_operands(hv)):
                n7[t, pl.ds(ro, 16), :] = op.astype(bf16)
            return 0
        lax.fori_loop(0, NPRE // 32, hpre_body, 0)
        lhs_h[0:MEM, :] = mem0_ref[...]
        lhs_h[MEM:32, :] = adaln_a(xbuf[NPRE:NPRE + RIDE, :].astype(f32)).astype(bf16)

        def relayout_now(g, dh):
            def rl_body(t, _):
                relayout(g, 2 * g + dh, dh, t * 32, 32)
                return 0
            lax.fori_loop(0, 8, rl_body, 0)

        for dh in range(2):
            stg_wait(dh, 1, dh)
            relayout_now(0, dh)

        grp = lambda g: piece_copies(g, 0) + piece_copies(g, 1)
        issue = {0: [wo_copy(0)], 1: grp(3) + grp(4), 2: grp(5) + [wo_copy(1), mod_copy(4)],
                 3: grp(6) + [wo_copy(2), mod_copy(5)], 4: grp(7) + [mod_copy(6)],
                 5: grp(8) + [wo_copy(3), mod_copy(7)], 6: grp(9) + [wo_copy(4)],
                 7: grp(10) + [wo_copy(5), mod_copy(8)], 8: grp(11) + [wo_copy(6)],
                 9: [wo_copy(7), mod_copy(9)], 10: stream_copies(0)}

        def pre_iter(g, m3):
            m3n = jnp.where(m3 == 2, 0, m3 + 1)
            ends = jnp.logical_or(g == 0, g == NGRP - 1)
            gn = jnp.where(ends, g, g + 1)
            gslot = 2 * jnp.where(ends, m3, m3n)
            wj = jnp.maximum(g - 4, 0)
            wslot = jnp.where(g < 4, gslot, NSLOT + jnp.where(m3 == 0, 2, m3 - 1))
            cj = jnp.maximum(g - 2, 3)
            cslot = jnp.where(cj >= NMOD, cj - NMOD, cj)

            @pl.when(g == 1)
            def _():
                stg_wait(2, 2, 2)
                relayout_now(1, 0)
                relayout_now(1, 1)

            @pl.when(jnp.logical_not(ends))
            def _():
                stg_wait(gslot, 2, g + 2)

            @pl.when(g >= 4)
            def _():
                stg_wait(wslot, 1, g + 2)

            @pl.when(g >= 6)
            def _():
                pltpu.make_async_copy(wmodb.at[cslot], wmodb.at[cslot],
                                      sems.at[SSTG + g + 2]).wait()

            for k, cps in issue.items():
                @pl.when(g == k)
                def _():
                    for cp in cps:
                        cp.start()
            wtodo = list(range(0, 256, 2))
            todo = [(dh, dp) for dh in range(2) for dp in range(256)]
            mtodo = list(range(0, D, 16))
            macc = [jnp.zeros((8, 512), f32)]

            def hook(v):
                if mtodo:
                    acc = macc[0] + jnp.concatenate([_zero_after(v)] * 4, axis=1)
                    for r in mtodo[:3]:
                        acc = mod_rows(acc, wmodb[cslot, r:r + 16, :], r)
                    del mtodo[:3]
                    macc[0] = acc

            for q in range(4):
                def b_of(k):
                    w = b_operand(g, q, k)
                    nw = 0 if todo else WLP
                    for dh, dp in todo[:RLP]:
                        relayout(gn, gslot + dh, dh, dp, 1)
                    del todo[:RLP]
                    for c in wtodo[:nw]:
                        wqkv[pl.ds(pl.multiple_of(WO + wj * 2048 + c * 8, 16), 16), :] = (
                            pltpu.bitcast(stg[wslot, c:c + 2].reshape(32, 128), u32))
                    del wtodo[:nw]
                    return w
                c11, c12, c21, c22 = _strassen(lambda k: n7[k, 0:NPRE // 2, :], b_of, hook)
                for blk, y in ((q + 4, _merge_rows(c12, c22)), (q, _merge_rows(c11, c21))):
                    y = y.astype(bf16)
                    n0 = NR - ROFF
                    rings[blk][g, ROFF:NR, :] = y[0:n0]
                    rings[blk][g, 0:NPRE - n0, :] = y[n0:NPRE]
            assert not todo and not wtodo and not mtodo
            mod_finish(macc[0], cj)
            return m3n

        _loop("pre1", 0, NGRP, pre_iter)

    pl.run_scoped(prologue,
                  pltpu.VMEM((NSLOT + NWO, 256, 16, 128), bf16),
                  pltpu.VMEM((NMOD, D, 512), bf16))

    def main(w7, w49):
        scale = DH ** -0.5
        ia = lax.broadcasted_iota(jnp.int32, (32, L), 0)
        ja = lax.broadcasted_iota(jnp.int32, (32, L), 1)
        mask_a = (ia >= RIDE) | (ja >= SEG) | (ia + 8 >= ja)
        ib = lax.broadcasted_iota(jnp.int32, (48, 56), 0)
        jb = lax.broadcasted_iota(jnp.int32, (48, 56), 1)
        own = (ib < 40) == (jb < 40)
        mask_b = own & (((jb >= 32) & (jb < 48)) | (jnp.where(jb < 40, jb, jb - 8) <= ib))
        masked = -1e9 / scale
        j8 = lax.broadcasted_iota(jnp.int32, (8, 56), 1)
        fill_b = jnp.concatenate([jnp.where(j8 < 40, masked, -3e38).astype(f32)] * 5
                                 + [jnp.where(j8 < 40, -3e38, masked).astype(f32)], axis=0)

        def softmax(sc, mask, fill):
            sc = jnp.where(mask, sc, fill)
            mx = jnp.max(sc, axis=-1, keepdims=True)
            e = jnp.exp2((sc - mx) * (scale * 1.4426950408889634))
            den = jnp.sum(e, axis=-1, keepdims=True)
            return (e * pl.reciprocal(den, approx=True)).astype(bf16)

        def ride_rows(s, is_b):
            first = s < 2
            if is_b:
                g = [jnp.where(first, -3, -1), 1, 2]
            else:
                g = [jnp.where(first, 1, 0), jnp.where(first, 2, 1), 3]
            return [RIDE * s + 8 * t for t in g]

        def step(s, is_b, lhs_lo, lhs_hi, soft_in, jobs):
            seg = pl.multiple_of((SEG * s + ROFF) % NR, SEG)
            sega = pl.multiple_of(seg - SEG, SEG) if is_b else seg
            wr = [pl.multiple_of((NPRE + RIDE * s + 8 * t + ROFF) % NR, 8) for t in range(3)]
            rd = [pl.multiple_of((r + ROFF) % NR, 8) for r in ride_rows(s, is_b)]
            lhs = jnp.concatenate([lhs_lo, lhs_hi], axis=1)
            QM, P, PART = {}, {}, {}
            mrow = 0 if is_b else MEM
            seg8 = pl.multiple_of(seg + 8, 8)
            seg24 = pl.multiple_of(seg + RIDE, 8)

            def wblk(b, lo, n):
                return pltpu.bitcast(wqkv[b * WP + lo:b * WP + lo + n, :], bf16)

            def qkv_lo(i):
                for m in range(3):
                    PART[(m, i)] = jnp.dot(lhs_lo, wblk(m * H + i, 0, 256), preferred_element_type=f32)

            def qkv(i):
                for m in range(3):
                    b = m * H + i
                    if (m, i) in PART:
                        y = jnp.dot(lhs_hi, wblk(b, 256, 256),
                                    preferred_element_type=f32) + PART.pop((m, i))
                    else:
                        y = jnp.dot(lhs, wblk(b, 0, 512), preferred_element_type=f32)
                    if m < 2:
                        QM[b] = y[0:MEM] + jobs["pin"] if b == PIN and is_b else y[0:MEM]
                    if m == 2 or (m == 1 and not is_b):
                        kvm[b - H, mrow:mrow + MEM, :] = y[0:MEM].astype(bf16)
                    for t in range(3):
                        rset(b, wr[t], y[8 + 8 * t:16 + 8 * t])
                    for job in jobs.get(3 * i + m, []):
                        job(y)

            def keys(b):
                if is_b:
                    if b in QM:
                        old = kvm[b - H, MEM:2 * MEM, :].astype(f32)
                        mix = jnp.concatenate([QM.pop(b), old], axis=0).astype(bf16)
                    else:
                        mix = kvm[b - H]
                    return jnp.concatenate([rget(b, seg, SEG), mix, rget(b, sega, 8)], axis=0)
                mk = QM.pop(b).astype(bf16) if b in QM else kvm[b - H, MEM:2 * MEM, :]
                return jnp.concatenate([rget(b, seg, SEG), mk], axis=0)

            def scores(i):
                if is_b:
                    mix = jnp.concatenate([QM.pop(i), rget(i, sega, 8).astype(f32)], axis=0)
                    q = jnp.concatenate([rget(i, seg, SEG), mix.astype(bf16)], axis=0)
                else:
                    mix = jnp.concatenate([rget(i, seg24, 8).astype(f32), QM.pop(i)], axis=0)
                    q = jnp.concatenate([rget(i, seg8, 16), mix.astype(bf16)], axis=0)
                sc = lax.dot_general(q, keys(H + i), (((1,), (1,)), ((), ())),
                                     preferred_element_type=f32)
                P[i] = softmax(sc, mask_b, fill_b) if is_b else softmax(sc, mask_a, masked)

            def pv(i):
                o = jnp.dot(P.pop(i), keys(2 * H + i), preferred_element_type=f32)
                if is_b:
                    rset(i, seg, o[0:SEG])
                    rset(i, sega, o[40:48])
                    lhs_o[i, 0:MEM, :] = o[SEG:L].astype(bf16)
                else:
                    rset(i, seg8, o[0:16])
                    rset(i, seg24, o[16:RIDE])
                    lhs_o[i, 0:MEM, :] = o[RIDE:32].astype(bf16)
                for t in range(3):
                    lhs_o[i, 8 + 8 * t:16 + 8 * t, :] = rget(i, rd[t], 8)

            def wo_lhs(i0, i1):
                return jnp.concatenate([lhs_o[i] for i in range(i0, i1)], axis=1)

            def wo_dot(lo, j, i0, i1):
                r = WO + j * 2048
                w = pltpu.bitcast(wqkv[r + 64 * i0:r + 64 * i1, :], bf16)
                return jnp.dot(lo, w, preferred_element_type=f32)

            def side(t):
                ds, dp = (DSB, DPB) if is_b else (DSA, DPA)
                if 0 <= t - dp < H:
                    pv(t - dp)
                if 0 <= t - ds < H:
                    scores(t - ds)

            if soft_in:
                for h in range(KSPLIT):
                    qkv_lo(h)
            for h in range(H):
                qkv(h)
                side(h)
            lo = [wo_lhs(8 * k, 8 * k + 8) for k in range(3)]
            acc = []
            for j in range(8):
                y = None
                for k in range(3):
                    z = wo_dot(lo[k], j, 8 * k, 8 * k + 8)
                    y = z if y is None else z + y
                    for job in jobs.get(96 + 3 * j + k, []):
                        job(y)
                acc.append(y)
                side(H + j)
            lo = wo_lhs(24, H)
            for j in range(8):
                acc[j] = wo_dot(lo, j, 24, H) + acc[j]
                for job in jobs.get(120 + j, []):
                    job(acc[j])
            assert not (QM or P or PART)
            return jnp.concatenate(acc[0:4], axis=1), jnp.concatenate(acc[4:8], axis=1)

        def combine(c, n, y):
            mp, k1 = divmod(n, 8)
            m, p = divmod(mp, 4)
            c3 = jnp.minimum(c, 27)
            spare = pl.ds(pl.multiple_of(8 * (c // 64), 8), 8)
            if m == 0 and k1 < 7:
                ws3[16, spare, :] = y.astype(bf16)
            else:
                wsr[7, spare, 0:128] = y.astype(bf16)
            if k1 == 7:
                dst, base, r = w7, 0, (4 * m + p) * 256 + c * 8
                blk = [wsr[4 + i, m * 16:(m + 1) * 16, j * 512 + p * 128:j * 512 + (p + 1) * 128]
                       .astype(f32) for i in range(2) for j in range(2)]
            else:
                dst, base = w49, 7 * k1
                if m == 0:
                    r = c3 * 32 + p * 8
                    get = lambda i, j: ws3[4 * i + j, p * 16:(p + 1) * 16, :]
                else:
                    r = W4R + (p // 2) * 448 + c3 * 16 + (p % 2) * 8
                    r0, c0 = (p % 2) * 16, (p // 2) * 128
                    get = lambda i, j: wsr[i, r0:r0 + 16, j * 256 + c0:j * 256 + c0 + 128]

                def quad(q):
                    return [get(2 * (q // 2) + i, 2 * (q % 2) + j).astype(f32)
                            for i in range(2) for j in range(2)]
                qi, qj, sign = _BTERMS[k1]
                blk = quad(qi)
                if qj is not None:
                    blk = [u + v if sign > 0 else u - v for u, v in zip(blk, quad(qj))]
            for k, op in enumerate(_b_operands(*blk)):
                tpk[n % 2, k * 16:(k + 1) * 16, :] = op.astype(bf16)
                dst[base + k, pl.ds(pl.multiple_of(r, 8), 8), :] = pltpu.bitcast(
                    tpk[n % 2, k * 16:(k + 1) * 16, :], u32)

        def rec_body(it, gacc):
            stream_wait(it)
            lhs_lo = lhs_h[:, 0:512]
            lhs_hi = lhs_h[:, 512:1024]
            ra = jnp.maximum(it - 1, 0) * (2 * RIDE)
            for u in range(2):
                s = 2 * it + u
                jobs = {}
                for n, (su, d, g) in enumerate(SLOTS):
                    if su == u:
                        jobs.setdefault(d, []).append(
                            lambda y, n=n, g=g: combine(it, n, y[8 * g:8 * g + 8]))
                r1 = pl.multiple_of(jnp.minimum(NPRE + RIDE * (s + 1), S - RIDE), 8)
                xn = xbuf[pl.ds(r1, RIDE), :].astype(f32)
                if u == 0:
                    for k in range(2):
                        rm = pl.multiple_of(it * 32 + k * 16, 16)
                        gacc = mod_rows(gacc, wsr[6, k * 16:(k + 1) * 16, :], rm)
                    hn = adaln_a(xn, _zero_after(stage_a16(ra)))
                else:
                    def refill(y):
                        for cp in stream_copies(jnp.minimum(it + 1, NSEG // 2 - 1)):
                            cp.start()
                        spare = pl.ds(pl.multiple_of(8 * (it // 64), 8), 8)
                        jobs["pin"] = _zero_after(ws3[16, spare, :].astype(f32))
                    jobs.setdefault(3 * (PIN - 4) + 2, []).append(refill)
                    hn = adaln_a(xn)
                    z = _zero_after(hn[0:8], hn[8:16], hn[16:24])
                    stage_a16(ra + 32, _zero_after(stage_a16(ra + 16, z)))
                a_lo, a_hi = step(s, u == 1, lhs_lo, lhs_hi, u > 0, jobs)
                lhs_lo = jnp.concatenate([a_lo[0:MEM], hn[:, 0:512]], axis=0).astype(bf16)
                lhs_hi = jnp.concatenate([a_hi[0:MEM], hn[:, 512:1024]], axis=0).astype(bf16)
                a = jnp.concatenate([a_lo, a_hi], axis=1)
                rows = [pl.multiple_of(r, 8) for r in ride_rows(s, u == 1)]
                xs = [xbuf[pl.ds(r, 8), :].astype(f32) for r in rows]
                for t, r in enumerate(rows):
                    xa = xs[t] + modrows(2, 8) * a[8 + 8 * t:16 + 8 * t]
                    xbuf[pl.ds(r, 8), :] = xa.astype(bf16)
            lhs_h[:, 0:512] = lhs_lo
            lhs_h[:, 512:1024] = lhs_hi
            return gacc

        gacc = _loop("rec", 0, NSEG // 2, rec_body, jnp.zeros((8, D), f32))
        for c in range(2):
            mod_finish(gacc[:, c * 512:(c + 1) * 512], 10 + c)
        stream_wait(NSEG // 2 - 1)

        def wo_tail(i, _):
            p0 = pl.multiple_of(i * 128, 128)
            r = pl.multiple_of(S - NPRE + i * 128, 128)
            prev = None
            lo = jnp.concatenate([rget(h, p0, 128) for h in range(H)], axis=1)
            for j in range(8):
                w = pltpu.bitcast(wqkv[WO + j * 2048:WO + (j + 1) * 2048, :], bf16)
                y = jnp.dot(lo, w, preferred_element_type=f32)
                if j < 7:
                    prev = stage_a16(r - 128 + 16 * j, _zero_after(y, prev))
                if j == 0:
                    prev = stage_a16(r - 16, _zero_after(prev))
                cs = slice(j * 128, (j + 1) * 128)
                ga = modrows(2, 128, j * 128, (j + 1) * 128)
                xbuf[pl.ds(r, 128), cs] = (xbuf[pl.ds(r, 128), cs].astype(f32) + ga * y).astype(bf16)
            return 0
        _loop("wotail", 0, NPRE // 128, wo_tail)

        def gget(c, row, n):
            return pltpu.bitcast(wqkv[pl.ds(c * GS + row, n), :], f32)

        def gset(c, row, val):
            wqkv[pl.ds(c * GS + row, val.shape[0]), :] = pltpu.bitcast(val, u32)

        def wop(j):
            return lambda k: pltpu.bitcast(w7[k, j * 256:(j + 1) * 256, :], bf16)

        zpad = jnp.zeros((GPAD, 128), f32)
        for cb in range(8):
            gset(cb, 0, zpad)
            gset(cb, GPAD + S, zpad)

        shifts = (-1, -1, 1, 1, -2, -2, 2, 2)
        HB = MB // 2

        def shift_piece(r, half, k):
            gs = jnp.concatenate([gget(c, r + (k * 16 + GPAD + shifts[c]), 16)
                                  for c in range(8)], axis=1)
            ro = half * (HB // 2) + k * 8
            for t, op in enumerate(row_operands(gs)):
                n7[t, ro:ro + 8, :] = op.astype(bf16)

        def gate(v, i):
            gset(0, GPAD + S + GPAD + 8 * (i // S), v[0:8])

        t7[...] = jnp.zeros(t7.shape, bf16)

        def b_body(i, _):
            ro = pl.multiple_of(i * HB, HB)
            rg = pl.multiple_of(GPAD + i * MB, 8)
            ra = jnp.minimum(S - 128 + 48 * i, S - 48)
            rp = jnp.minimum(S - 128 + 48 * jnp.maximum(i - 1, 0), S - 48)
            n7[:, pl.ds(pl.multiple_of(rp // 2, 8), 24), :] = t7[...]
            st = {"n": 0, "prev": None}

            def hook(v):
                n = st["n"]
                st["n"] += 1
                if n % 7 == BH and n // 7 < 3:
                    st["prev"] = stage_a16(ra + 16 * (n // 7), _zero_after(v, st["prev"]),
                                           (t7, 8 * (n // 7)))

            for j in range(4):
                c11, c12, c21, c22 = _strassen(lambda k: n7[k, pl.ds(ro, HB), :], wop(j), hook)
                gset(j + 4, rg, _gelu(_merge_rows(c12, c22)))
                gset(j, rg, _gelu(_merge_rows(c11, c21)))
            return 0
        _loop("b", 0, S // MB, b_body)
        for k in range(HB // 16):
            shift_piece(0, 0, k)

        def n2_norm(r, k, anchor):
            v = _ln(h2buf[pl.ds(pl.multiple_of(r + k * 16, 16), 16), :], anchor)
            nrms[k // 2][(k % 2) * 16:(k % 2) * 16 + 16, :] = v
            return v[0:8] + v[8:16]

        def n2_ops(k, k1, v, i):
            nrm = nrms[k]
            nrm[pl.ds(pl.multiple_of(32 + 8 * (i // S), 8), 8), 0:128] = v[0:8]

            def quad(q):
                r0, c0 = (q // 2) * 16, (q % 2) * 512
                return [nrm[r0 + 8 * a:r0 + 8 * a + 8, c0 + 256 * b:c0 + 256 * b + 256]
                        for a in range(2) for b in range(2)]
            qi, qj, sign = _ATERMS[k1]
            blk = quad(qi)
            if qj is not None:
                blk = [u + w if sign > 0 else u - w for u, w in zip(blk, quad(qj))]
            for k2, op in enumerate(_a_operands(*blk)):
                d49[7 * k1 + k2, k * 8:(k + 1) * 8, :] = op.astype(bf16)

        def n2_hook(r, i, first, gap, lag, st):
            def hook(v):
                n = st["n"] - first
                st["n"] += 1
                if n >= 0 and n % gap == 0 and n // gap < MD // 16:
                    st["prev"] = n2_norm(r, n // gap, _zero_after(v, st["prev"]))
                for _ in range(st["per"]):
                    k, k1 = divmod(st["ops"], 7)
                    if k < MD // 32 and n >= (2 * k + 1) * gap + lag:
                        n2_ops(k, k1, v, i)
                        st["ops"] += 1
            return hook

        def stage_c(i, r, half, rnext, extra):
            rr = pl.multiple_of(r, 8)
            ro = half * (HB // 2)
            cnt = [0]

            def hook(v):
                n = cnt[0]
                cnt[0] += 1
                if n < HB // 16:
                    gate(v, i)
                    shift_piece(rnext, 1 - half, n)
                extra(v)

            for j in range(4):
                c11, c12, c21, c22 = _strassen(lambda k: n7[k, ro:ro + HB // 2, :], wop(4 + j),
                                               hook)
                for c, y in ((j + 4, _merge_rows(c12, c22)), (j, _merge_rows(c11, c21))):
                    cs = slice(c * 128, (c + 1) * 128)
                    h2buf[pl.ds(rr, HB), cs] = h2buf[pl.ds(rr, HB), cs] + y

        def c_body(i, _):
            r = pl.multiple_of(i * MB, MB)
            st = {"n": 0, "prev": None, "ops": 0, "per": 1}
            extra = n2_hook(0, i, 0, 4, 4, st)
            stage_c(i, r, 0, r + HB, extra)
            stage_c(i, r + HB, 1, jnp.minimum(i + 1, S // MB - 1) * MB, extra)
            assert st["ops"] == 28
            return 0
        _loop("c", 0, S // MB, c_body)

        def wop2(lo, n):
            return lambda k1, k: pltpu.bitcast(w49[7 * k1 + k, lo:lo + n, :], bf16)

        def d_body(i, _):
            r = pl.multiple_of(i * MD, MD)
            rn = jnp.minimum(r + MD, S - MD)
            lhs = [d49[k] for k in range(49)]
            uops = []
            for t in range(7):
                cb = _strassen2(lambda k1, k: lhs[7 * k1 + k], wop2(t * 128, 128))
                uops.append(_a_operands2([[_gelu(c) for c in row] for row in cb]))
            ul = [[jnp.concatenate([u[k1][k] for u in uops], axis=1).astype(bf16)
                   for k in range(7)] for k1 in range(7)]
            st = {"n": 0, "prev": None, "ops": 0, "per": 1}
            hook = n2_hook(rn, i, DF, DG, DL, st)
            for t in range(2):
                cb = _strassen2(lambda k1, k: ul[k1][k], wop2(W4R + t * 448, 448), hook)
                for j in range(4):
                    y = jnp.concatenate([cb[q][j].reshape(MD // 32, 8, 128) for q in range(4)],
                                        axis=1).reshape(MD, 128)
                    c = 2 * j + t
                    cs = slice(c * 128, (c + 1) * 128)
                    gb = modrows(5, MD, c * 128, (c + 1) * 128)
                    o = xbuf[pl.ds(r, MD), cs].astype(f32) + gb * (h2buf[pl.ds(r, MD), cs] + y)
                    xbuf[pl.ds(r, MD), cs] = o.astype(bf16)
            assert st["ops"] == 28
            out_copy(r, MD).start()
            return 0
        _loop("d", 0, S // MD, d_body)

    pl.run_scoped(main,
                  pltpu.VMEM((7, 8 * 256, 128), u32),
                  pltpu.VMEM((49, 2 * W4R, 128), u32))

    out_copy(0, S).wait()


def _run(x, mem0, wq, wk, wv, wo, w1, w2, w3, w4, c, wmod):
    any_spec = pl.BlockSpec(memory_space=pl.ANY)
    vmem_spec = pl.BlockSpec(memory_space=pltpu.VMEM)
    return pl.pallas_call(
        _kernel,
        out_shape=jax.ShapeDtypeStruct((S, D), bf16),
        in_specs=[any_spec, vmem_spec, any_spec, any_spec, any_spec, any_spec, any_spec,
                  any_spec, any_spec, any_spec, vmem_spec, any_spec],
        out_specs=any_spec,
        scratch_shapes=[
            pltpu.VMEM((S + 2 * RIDE, D), bf16),
            pltpu.VMEM((WO + 8 * 2048, 128), u32),
            [pltpu.VMEM((96 // NRING, NR, 128), bf16)] * NRING,
            pltpu.VMEM((32, D), bf16),
            pltpu.VMEM((H, 32, 128), bf16),
            pltpu.VMEM((2 * H, 16, 128), bf16),
            pltpu.VMEM((12, 8, 512), f32),
            pltpu.VMEM((D, 128), f32),
            pltpu.VMEM((S, D), f32),
            pltpu.VMEM((7, S // 2, 512), bf16),
            pltpu.VMEM((17, 64, 128), bf16),
            pltpu.VMEM((8, 32, D), bf16),
            pltpu.VMEM((2, 112, 128), bf16),
            pltpu.VMEM((7, 24, 512), bf16),
            pltpu.VMEM((49, MD // 4, 256), bf16),
            [pltpu.VMEM((40, D), f32)] * (MD // 32),
            pltpu.SemaphoreType.DMA((9 + NGRP + 2,)),
        ],
        compiler_params=pltpu.CompilerParams(vmem_limit_bytes=124 * 1024 * 1024,
                                             disable_bounds_checks=True),
    )(x, mem0, wq, wk, wv, wo, w1, w2, w3, w4, c, wmod)


def pallas_adaLN_cond__memory_aug_recurrent_mem_tr__mixer_s_mlp__prompt_kernel(
    A_x, A_mem0, A_Wq, A_Wk, A_Wv, A_Wo, A_seg_len, B_x, B_w1, B_w2, B_w3, B_w4, c, w_mod,
):
    del B_x
    assert A_x.shape == (1, S, D) and A_mem0.shape == (1, MEM, D)
    assert isinstance(A_seg_len, int) is False or A_seg_len == SEG
    pairs = (D // 2, 2, H, DH)
    out = _run(A_x.reshape(S, D), A_mem0.reshape(MEM, D), A_Wq.reshape(pairs),
               A_Wk.reshape(pairs), A_Wv.reshape(pairs), A_Wo.reshape(H * DH // 16, 16, D),
               B_w1.reshape(2, D // 2, D), B_w2.reshape(2, D // 2, D),
               B_w3, B_w4.reshape(4, F // 4, D), c, w_mod)
    return out.reshape(1, S, D)
```

```python
import jax
import jax.numpy as jnp
from jax import lax
import jax.experimental.pallas as pl
import jax.experimental.pallas.tpu as pltpu

bf16 = jnp.bfloat16
f32 = jnp.float32
u32 = jnp.uint32

S = 2048
D = 1024
H = 32
DH = 128
F = 3584
MEM = 8
SEG = 32
NSEG = S // SEG
L = MEM + SEG
RIDE = 24
NPRE = S - RIDE * NSEG
NR = NPRE + 2 * SEG
ROFF = (-(S - NPRE)) % NR
WP = 516
WO = 96 * WP
NGRP = 12
NSLOT = 6
NMOD = 6
EPS = 1e-5
MD = 128
MB = 512
GPAD = 8
NRING = 8
RLP, WLP = 25, 22
NWO = 3
BH, PIN = 0, 6
DF, DG, DL = 8, 9, 9
SLOTS = ([(0, n // 2, 3 * (n % 2)) for n in range(16)] + [(0, 96 + n, 0) for n in range(16)]
         + [(0, 112 + n // 2, 3 * (n % 2)) for n in range(32)])
DSA, DPA, DSB, DPB, KSPLIT = 2, 4, 2, 4, 2
X0 = NPRE + 2 * RIDE
GS = S + 4 * GPAD
W4R = 7 * 128
_ONLY = None


def _loop(name, lo, hi, body, init=0):
    if _ONLY is not None and name not in _ONLY:
        return init
    with _scope(name):
        return lax.fori_loop(lo, hi, body, init)


class _NoScope:
    def __init__(self, name):
        del name

    def __enter__(self):
        return self

    def __exit__(self, *a):
        return False


_scope = _NoScope


def _zero_after(*vs):
    bits = None
    for v in vs:
        if v is not None:
            b = pltpu.bitcast(v[0:8, 0:128], u32)
            bits = b if bits is None else bits | b
    return pltpu.bitcast((bits >> 31) >> 1, f32)


def _ln(x, anchor=None):
    if anchor is not None:
        z = jnp.concatenate([anchor] * (x.shape[0] // 8), axis=0)
        x = jnp.concatenate([x[:, 0:128] + z, x[:, 128:]], axis=1)
    mu = jnp.mean(x, axis=-1, keepdims=True)
    xc = x - mu
    var = jnp.mean(xc * xc, axis=-1, keepdims=True)
    return xc * lax.rsqrt(var + EPS)


def _gelu(x):
    inner = x * (0.7978845608028654 + (0.7978845608028654 * 0.044715) * (x * x))
    hx = 0.5 * x
    return hx + hx * jnp.tanh(inner)


def _split_rows(x):
    m, n = x.shape
    x3 = x.reshape(m // 16, 16, n)
    return x3[:, 0:8, :].reshape(m // 2, n), x3[:, 8:16, :].reshape(m // 2, n)


def _merge_rows(top, bot):
    m, n = top.shape
    return jnp.concatenate([top.reshape(m // 8, 8, n), bot.reshape(m // 8, 8, n)],
                           axis=1).reshape(2 * m, n)


def _a_operands(a11, a12, a21, a22):
    return [a11 + a22, a21 + a22, a11, a22, a11 + a12, a21 - a11, a12 - a22]


def _b_operands(b11, b12, b21, b22):
    return [b11 + b22, b11, b12 - b22, b21 - b11, b22, b11 + b12, b21 + b22]


_ATERMS = ((0, 3, 1), (2, 3, 1), (0, None, 0), (3, None, 0), (0, 1, 1), (2, 0, -1), (1, 3, -1))
_BTERMS = ((0, 3, 1), (0, None, 0), (1, 3, -1), (2, 0, -1), (3, None, 0), (0, 1, 1), (2, 3, 1))


def _strassen(a_of, b_of, hook=lambda v: None):
    def prod(k):
        return jnp.dot(a_of(k), b_of(k), preferred_element_type=f32)
    p5 = prod(4)
    hook(p5)
    p3 = prod(2)
    hook(p3)
    c12 = p3 + p5
    p4 = prod(3)
    hook(p4)
    c11 = p4 - p5
    p2 = prod(1)
    hook(p2)
    c21 = p2 + p4
    c22 = p3 - p2
    p1 = prod(0)
    hook(p1)
    c11 = prod(6) + (c11 + p1)
    hook(c11)
    c22 = prod(5) + (c22 + p1)
    hook(c22)
    return c11, c12, c21, c22


def _a_operands2(b):
    sub = [_a_operands(b[i][j], b[i][2 + j], b[2 + i][j], b[2 + i][2 + j])
           for i in range(2) for j in range(2)]
    return [_a_operands(*[t[k] for t in sub]) for k in range(7)]


def _strassen2(a_of, b_of, hook=lambda v: None):
    def prod(k1):
        return _strassen(lambda k: a_of(k1, k), lambda k: b_of(k1, k), hook)

    def add(x, y):
        return [p + q for p, q in zip(x, y)]

    def sub(x, y):
        return [p - q for p, q in zip(x, y)]
    p5 = prod(4)
    p3 = prod(2)
    c12 = add(p3, p5)
    p4 = prod(3)
    c11 = sub(p4, p5)
    p2 = prod(1)
    c21 = add(p2, p4)
    c22 = sub(p3, p2)
    p1 = prod(0)
    c11 = add(add(c11, p1), prod(6))
    c22 = add(add(c22, p1), prod(5))
    cq = (c11, c12, c21, c22)
    return [[cq[2 * (i // 2) + j // 2][2 * (i % 2) + j % 2] for j in range(4)] for i in range(4)]


def _kernel(x_hbm, mem0_ref, wq_hbm, wk_hbm, wv_hbm, wo_hbm, w1_hbm, w2_hbm, w3_hbm, w4_hbm,
            c_ref, wmod_hbm, out_hbm,
            xbuf, wqkv, rings, lhs_h, lhs_o, kvm, modv, scol, h2buf, n7, ws3, wsr, t7, d49, nrms,
            sems):
    w_hbms = (wq_hbm, wk_hbm, wv_hbm)
    SMOD, SSTG = 5, 9
    sem_x, sem_out, sem_w, sem_g, sem_r = (sems.at[k] for k in range(5))

    def rget(b, row, n):
        return rings[b % NRING][b // NRING, pl.ds(row, n), :]

    def rset(b, row, val):
        rings[b % NRING][b // NRING, pl.ds(row, val.shape[0]), :] = val.astype(bf16)

    x_copy = pltpu.make_async_copy(x_hbm.at[pl.ds(0, X0), :], xbuf.at[pl.ds(0, X0), :], sem_x)

    def stream_copies(c):
        al, lo = ((lambda v, m: v), min) if isinstance(c, int) else (pl.multiple_of, jnp.minimum)
        c3 = lo(c, 27)
        cps = [pltpu.make_async_copy(
            w3_hbm.at[pl.ds(al(i * 256 + (c3 % 4) * 64, 64), 64),
                      pl.ds(al(j * (F // 4) + (c3 // 4) * 128, 128), 128)],
            ws3.at[4 * i + j], sem_w) for i in range(4) for j in range(4)]
        dst = X0 + 2 * RIDE * c
        return [
            pltpu.make_async_copy(w4_hbm.at[:, pl.ds(al(c3 * 32, 32), 32), :],
                                  wsr.at[pl.ds(0, 4)], sem_g),
            pltpu.make_async_copy(w1_hbm.at[:, pl.ds(al(c * 16, 16), 16), :],
                                  wsr.at[pl.ds(4, 2), pl.ds(0, 16), :], sem_g),
            pltpu.make_async_copy(w2_hbm.at[:, pl.ds(al(c * 16, 16), 16), :],
                                  wsr.at[pl.ds(4, 2), pl.ds(16, 16), :], sem_g),
            pltpu.make_async_copy(wmod_hbm.at[pl.ds(al(c * 32, 32), 32), pl.ds(5 * D, D)],
                                  wsr.at[6], sem_g),
            pltpu.make_async_copy(x_hbm.at[pl.ds(al(lo(dst, S - 2 * RIDE), 16), 2 * RIDE), :],
                                  xbuf.at[pl.ds(al(dst, 16), 2 * RIDE), :], sem_r)] + cps

    def stream_wait(c):
        for dst, sem in ((ws3.at[pl.ds(0, 16)], sem_w), (wsr.at[pl.ds(0, 7)], sem_g),
                         (xbuf.at[pl.ds(X0 + 2 * RIDE * c, 2 * RIDE), :], sem_r)):
            pltpu.make_async_copy(dst, dst, sem).wait()

    def out_copy(row, n):
        return pltpu.make_async_copy(xbuf.at[pl.ds(row, n), :], out_hbm.at[pl.ds(row, n), :],
                                     sem_out)

    def mod_rows(acc, w, r):
        sc = jnp.concatenate([scol[pl.ds(r, 16), :]] * (w.shape[1] // 128), axis=1)
        p = w.astype(f32) * sc
        return acc + p[0:8] + p[8:16]

    def mod_finish(acc, j):
        is_scale = jnp.logical_or(j // 2 == 1, j // 2 == 4)
        tot = jnp.sum(acc, axis=0, keepdims=True) + jnp.where(is_scale, 1.0, 0.0)
        modv[j] = jnp.broadcast_to(tot, (8, 512))

    def modrows(k, n, lo=0, hi=D):
        m = jnp.concatenate([modv[2 * k], modv[2 * k + 1]], axis=1)[:, lo:hi]
        return jnp.concatenate([m] * (n // 8), axis=0)

    def adaln_a(xv, anchor=None):
        n = xv.shape[0]
        return _ln(xv, anchor) * modrows(1, n) + modrows(0, n)

    def adaln_b(xv, anchor=None):
        n = xv.shape[0]
        return _ln(xv, anchor) * modrows(4, n) + modrows(3, n)

    def row_operands(v):
        top, bot = _split_rows(v)
        k = v.shape[1] // 2
        return _a_operands(top[:, :k], top[:, k:], bot[:, :k], bot[:, k:])

    def stage_a16(r, anchor=None, dst=None):
        rr = pl.multiple_of(r, 16)
        h2 = adaln_b(xbuf[pl.ds(rr, 16), :].astype(f32), anchor)
        h2buf[pl.ds(rr, 16), :] = h2
        ref, ro = (n7, pl.multiple_of(rr // 2, 8)) if dst is None else dst
        ops = row_operands(_ln(h2))
        for t, op in enumerate(ops):
            ref[t, pl.ds(ro, 8), :] = op.astype(bf16)
        return ops[0]

    def prologue(stg, wmodb):
        def mod_copy(j):
            return pltpu.make_async_copy(wmod_hbm.at[:, pl.ds(j * 512, 512)], wmodb.at[j % NMOD],
                                         sems.at[SSTG + j + 4 if j >= 4 else SMOD + j])

        def piece_copies(g, dh):
            slot = (2 * g + dh) % NSLOT
            return [pltpu.make_async_copy(
                w_hbms[g // 4].at[pl.ds(dh * 256, 256), par, pl.ds((g % 4) * 8, 8), :],
                stg.at[slot, :, pl.ds(par * 8, 8), :],
                sems.at[SSTG + (g + 1 if g else dh)]) for par in range(2)]

        def wo_copy(j):
            slot = NSLOT + j % NWO
            return pltpu.make_async_copy(wo_hbm.at[:, :, pl.ds(j * 128, 128)], stg.at[slot],
                                         sems.at[SSTG + j + 6])

        def group_start(g):
            for dh in range(2):
                for cp in piece_copies(g, dh):
                    cp.start()

        def stg_wait(slot, n, sem):
            dst = stg.at[pl.ds(slot, n)]
            pltpu.make_async_copy(dst, dst, sems.at[SSTG + sem]).wait()

        def relayout(g, slot, dh, lo_dp, n_dp):
            base = g * (8 * WP) + dh * 256
            for u in range(n_dp):
                dp = lo_dp + u
                ev = pltpu.bitcast(stg[slot, dp, 0:8, :].astype(f32), u32)
                od = pltpu.bitcast(stg[slot, dp, 8:16, :].astype(f32), u32)
                wqkv[pl.ds(base + dp, 8, stride=WP), :] = (ev >> 16) | od

        def b_operand(g, q, k):
            def quad(i):
                r = (g * 8 + q + 4 * (i % 2)) * WP + (i // 2) * 256
                return pltpu.bitcast(wqkv[pl.ds(r, 256), :], bf16)
            i, j, sign = _BTERMS[k]
            if j is None:
                return quad(i)
            u, v = quad(i).astype(f32), quad(j).astype(f32)
            return (u + v if sign > 0 else u - v).astype(bf16)

        x_copy.start()
        for j in range(4):
            mod_copy(j).start()
        for g in range(3):
            group_start(g)
        cv = c_ref[...].astype(f32)
        sv = jnp.broadcast_to(cv * (1.0 / (1.0 + jnp.exp(-cv))), (128, D))
        for k in range(8):
            scol[k * 128:(k + 1) * 128, :] = sv[:, k * 128:(k + 1) * 128].T
        x_copy.wait()

        def ln0_body(i, _):
            r = pl.multiple_of(i * 64, 64)
            h2buf[pl.ds(r, 64), :] = _ln(xbuf[pl.ds(r, 64), :].astype(f32))
            return 0
        lax.fori_loop(0, NPRE // 64, ln0_body, 0)

        def mod0_body(j, _):
            pltpu.make_async_copy(wmodb.at[j], wmodb.at[j], sems.at[SMOD + j]).wait()
            accs = [jnp.zeros((8, 512), f32)] * 2
            for k in range(64):
                accs[k % 2] = mod_rows(accs[k % 2], wmodb[j, k * 16:(k + 1) * 16, :], k * 16)
            mod_finish(accs[0] + accs[1], j)
            return 0
        _loop("mod0", 0, 4, mod0_body)

        def hpre_body(i, _):
            r = pl.multiple_of(i * 32, 32)
            hv = h2buf[pl.ds(r, 32), :] * modrows(1, 32) + modrows(0, 32)
            ro = pl.multiple_of(i * 16, 16)
            for t, op in enumerate(row_operands(hv)):
                n7[t, pl.ds(ro, 16), :] = op.astype(bf16)
            return 0
        lax.fori_loop(0, NPRE // 32, hpre_body, 0)
        lhs_h[0:MEM, :] = mem0_ref[...]
        lhs_h[MEM:32, :] = adaln_a(xbuf[NPRE:NPRE + RIDE, :].astype(f32)).astype(bf16)

        def relayout_now(g, dh):
            def rl_body(t, _):
                relayout(g, 2 * g + dh, dh, t * 32, 32)
                return 0
            lax.fori_loop(0, 8, rl_body, 0)

        for dh in range(2):
            stg_wait(dh, 1, dh)
            relayout_now(0, dh)

        grp = lambda g: piece_copies(g, 0) + piece_copies(g, 1)
        issue = {0: [wo_copy(0)], 1: grp(3) + grp(4), 2: grp(5) + [wo_copy(1), mod_copy(4)],
                 3: grp(6) + [wo_copy(2), mod_copy(5)], 4: grp(7) + [mod_copy(6)],
                 5: grp(8) + [wo_copy(3), mod_copy(7)], 6: grp(9) + [wo_copy(4)],
                 7: grp(10) + [wo_copy(5), mod_copy(8)], 8: grp(11) + [wo_copy(6)],
                 9: [wo_copy(7), mod_copy(9)], 10: stream_copies(0)}

        def pre_iter(g, m3):
            m3n = jnp.where(m3 == 2, 0, m3 + 1)
            ends = jnp.logical_or(g == 0, g == NGRP - 1)
            gn = jnp.where(ends, g, g + 1)
            gslot = 2 * jnp.where(ends, m3, m3n)
            wj = jnp.maximum(g - 4, 0)
            wslot = jnp.where(g < 4, gslot, NSLOT + jnp.where(m3 == 0, 2, m3 - 1))
            cj = jnp.maximum(g - 2, 3)
            cslot = jnp.where(cj >= NMOD, cj - NMOD, cj)

            @pl.when(g == 1)
            def _():
                stg_wait(2, 2, 2)
                relayout_now(1, 0)
                relayout_now(1, 1)

            @pl.when(jnp.logical_not(ends))
            def _():
                stg_wait(gslot, 2, g + 2)

            @pl.when(g >= 4)
            def _():
                stg_wait(wslot, 1, g + 2)

            @pl.when(g >= 6)
            def _():
                pltpu.make_async_copy(wmodb.at[cslot], wmodb.at[cslot],
                                      sems.at[SSTG + g + 2]).wait()

            for k, cps in issue.items():
                @pl.when(g == k)
                def _():
                    for cp in cps:
                        cp.start()
            wtodo = list(range(0, 256, 2))
            todo = [(dh, dp) for dh in range(2) for dp in range(256)]
            mtodo = list(range(0, D, 16))
            macc = [jnp.zeros((8, 512), f32)]

            def hook(v):
                if mtodo:
                    acc = macc[0] + jnp.concatenate([_zero_after(v)] * 4, axis=1)
                    for r in mtodo[:3]:
                        acc = mod_rows(acc, wmodb[cslot, r:r + 16, :], r)
                    del mtodo[:3]
                    macc[0] = acc

            for q in range(4):
                def b_of(k):
                    w = b_operand(g, q, k)
                    nw = 0 if todo else WLP
                    for dh, dp in todo[:RLP]:
                        relayout(gn, gslot + dh, dh, dp, 1)
                    del todo[:RLP]
                    for c in wtodo[:nw]:
                        wqkv[pl.ds(pl.multiple_of(WO + wj * 2048 + c * 8, 16), 16), :] = (
                            pltpu.bitcast(stg[wslot, c:c + 2].reshape(32, 128), u32))
                    del wtodo[:nw]
                    return w
                c11, c12, c21, c22 = _strassen(lambda k: n7[k, 0:NPRE // 2, :], b_of, hook)
                for blk, y in ((q + 4, _merge_rows(c12, c22)), (q, _merge_rows(c11, c21))):
                    y = y.astype(bf16)
                    n0 = NR - ROFF
                    rings[blk][g, ROFF:NR, :] = y[0:n0]
                    rings[blk][g, 0:NPRE - n0, :] = y[n0:NPRE]
            assert not todo and not wtodo and not mtodo
            mod_finish(macc[0], cj)
            return m3n

        _loop("pre1", 0, NGRP, pre_iter)

    pl.run_scoped(prologue,
                  pltpu.VMEM((NSLOT + NWO, 256, 16, 128), bf16),
                  pltpu.VMEM((NMOD, D, 512), bf16))

    def main(w7, w49):
        scale = DH ** -0.5
        ia = lax.broadcasted_iota(jnp.int32, (32, L), 0)
        ja = lax.broadcasted_iota(jnp.int32, (32, L), 1)
        mask_a = (ia >= RIDE) | (ja >= SEG) | (ia + 8 >= ja)
        ib = lax.broadcasted_iota(jnp.int32, (48, 56), 0)
        jb = lax.broadcasted_iota(jnp.int32, (48, 56), 1)
        own = (ib < 40) == (jb < 40)
        mask_b = own & (((jb >= 32) & (jb < 48)) | (jnp.where(jb < 40, jb, jb - 8) <= ib))
        masked = -1e9 / scale
        j8 = lax.broadcasted_iota(jnp.int32, (8, 56), 1)
        fill_b = jnp.concatenate([jnp.where(j8 < 40, masked, -3e38).astype(f32)] * 5
                                 + [jnp.where(j8 < 40, -3e38, masked).astype(f32)], axis=0)

        def softmax(sc, mask, fill):
            sc = jnp.where(mask, sc, fill)
            mx = jnp.max(sc, axis=-1, keepdims=True)
            e = jnp.exp2((sc - mx) * (scale * 1.4426950408889634))
            den = jnp.sum(e, axis=-1, keepdims=True)
            return (e * pl.reciprocal(den, approx=True)).astype(bf16)

        def ride_rows(s, is_b):
            first = s < 2
            if is_b:
                g = [jnp.where(first, -3, -1), 1, 2]
            else:
                g = [jnp.where(first, 1, 0), jnp.where(first, 2, 1), 3]
            return [RIDE * s + 8 * t for t in g]

        def step(s, is_b, lhs_lo, lhs_hi, soft_in, jobs):
            seg = pl.multiple_of((SEG * s + ROFF) % NR, SEG)
            sega = pl.multiple_of(seg - SEG, SEG) if is_b else seg
            wr = [pl.multiple_of((NPRE + RIDE * s + 8 * t + ROFF) % NR, 8) for t in range(3)]
            rd = [pl.multiple_of((r + ROFF) % NR, 8) for r in ride_rows(s, is_b)]
            lhs = jnp.concatenate([lhs_lo, lhs_hi], axis=1)
            QM, P, PART = {}, {}, {}
            mrow = 0 if is_b else MEM
            seg8 = pl.multiple_of(seg + 8, 8)
            seg24 = pl.multiple_of(seg + RIDE, 8)

            def wblk(b, lo, n):
                return pltpu.bitcast(wqkv[b * WP + lo:b * WP + lo + n, :], bf16)

            def qkv_lo(i):
                for m in range(3):
                    PART[(m, i)] = jnp.dot(lhs_lo, wblk(m * H + i, 0, 256), preferred_element_type=f32)

            def qkv(i):
                for m in range(3):
                    b = m * H + i
                    if (m, i) in PART:
                        y = jnp.dot(lhs_hi, wblk(b, 256, 256),
                                    preferred_element_type=f32) + PART.pop((m, i))
                    else:
                        y = jnp.dot(lhs, wblk(b, 0, 512), preferred_element_type=f32)
                    if m < 2:
                        QM[b] = y[0:MEM] + jobs["pin"] if b == PIN and is_b else y[0:MEM]
                    if m == 2 or (m == 1 and not is_b):
                        kvm[b - H, mrow:mrow + MEM, :] = y[0:MEM].astype(bf16)
                    for t in range(3):
                        rset(b, wr[t], y[8 + 8 * t:16 + 8 * t])
                    for job in jobs.get(3 * i + m, []):
                        job(y)

            def keys(b):
                if is_b:
                    if b in QM:
                        old = kvm[b - H, MEM:2 * MEM, :].astype(f32)
                        mix = jnp.concatenate([QM.pop(b), old], axis=0).astype(bf16)
                    else:
                        mix = kvm[b - H]
                    return jnp.concatenate([rget(b, seg, SEG), mix, rget(b, sega, 8)], axis=0)
                mk = QM.pop(b).astype(bf16) if b in QM else kvm[b - H, MEM:2 * MEM, :]
                return jnp.concatenate([rget(b, seg, SEG), mk], axis=0)

            def scores(i):
                if is_b:
                    mix = jnp.concatenate([QM.pop(i), rget(i, sega, 8).astype(f32)], axis=0)
                    q = jnp.concatenate([rget(i, seg, SEG), mix.astype(bf16)], axis=0)
                else:
                    mix = jnp.concatenate([rget(i, seg24, 8).astype(f32), QM.pop(i)], axis=0)
                    q = jnp.concatenate([rget(i, seg8, 16), mix.astype(bf16)], axis=0)
                sc = lax.dot_general(q, keys(H + i), (((1,), (1,)), ((), ())),
                                     preferred_element_type=f32)
                P[i] = softmax(sc, mask_b, fill_b) if is_b else softmax(sc, mask_a, masked)

            def pv(i):
                o = jnp.dot(P.pop(i), keys(2 * H + i), preferred_element_type=f32)
                if is_b:
                    rset(i, seg, o[0:SEG])
                    rset(i, sega, o[40:48])
                    lhs_o[i, 0:MEM, :] = o[SEG:L].astype(bf16)
                else:
                    rset(i, seg8, o[0:16])
                    rset(i, seg24, o[16:RIDE])
                    lhs_o[i, 0:MEM, :] = o[RIDE:32].astype(bf16)
                for t in range(3):
                    lhs_o[i, 8 + 8 * t:16 + 8 * t, :] = rget(i, rd[t], 8)

            def wo_lhs(i0, i1):
                return jnp.concatenate([lhs_o[i] for i in range(i0, i1)], axis=1)

            def wo_dot(lo, j, i0, i1):
                r = WO + j * 2048
                w = pltpu.bitcast(wqkv[r + 64 * i0:r + 64 * i1, :], bf16)
                return jnp.dot(lo, w, preferred_element_type=f32)

            def side(t):
                ds, dp = (DSB, DPB) if is_b else (DSA, DPA)
                if 0 <= t - dp < H:
                    pv(t - dp)
                if 0 <= t - ds < H:
                    scores(t - ds)

            if soft_in:
                for h in range(KSPLIT):
                    qkv_lo(h)
            for h in range(H):
                qkv(h)
                side(h)
            lo = [wo_lhs(8 * k, 8 * k + 8) for k in range(3)]
            acc = []
            for j in range(8):
                y = None
                for k in range(3):
                    z = wo_dot(lo[k], j, 8 * k, 8 * k + 8)
                    y = z if y is None else z + y
                    for job in jobs.get(96 + 3 * j + k, []):
                        job(y)
                acc.append(y)
                side(H + j)
            lo = wo_lhs(24, H)
            for j in range(8):
                acc[j] = wo_dot(lo, j, 24, H) + acc[j]
                for job in jobs.get(120 + j, []):
                    job(acc[j])
            assert not (QM or P or PART)
            return jnp.concatenate(acc[0:4], axis=1), jnp.concatenate(acc[4:8], axis=1)

        def combine(c, n, y):
            mp, k1 = divmod(n, 8)
            m, p = divmod(mp, 4)
            c3 = jnp.minimum(c, 27)
            spare = pl.ds(pl.multiple_of(8 * (c // 64), 8), 8)
            if m == 0 and k1 < 7:
                ws3[16, spare, :] = y.astype(bf16)
            else:
                wsr[7, spare, 0:128] = y.astype(bf16)
            if k1 == 7:
                dst, base, r = w7, 0, (4 * m + p) * 256 + c * 8
                blk = [wsr[4 + i, m * 16:(m + 1) * 16, j * 512 + p * 128:j * 512 + (p + 1) * 128]
                       .astype(f32) for i in range(2) for j in range(2)]
            else:
                dst, base = w49, 7 * k1
                if m == 0:
                    r = c3 * 32 + p * 8
                    get = lambda i, j: ws3[4 * i + j, p * 16:(p + 1) * 16, :]
                else:
                    r = W4R + (p // 2) * 448 + c3 * 16 + (p % 2) * 8
                    r0, c0 = (p % 2) * 16, (p // 2) * 128
                    get = lambda i, j: wsr[i, r0:r0 + 16, j * 256 + c0:j * 256 + c0 + 128]

                def quad(q):
                    return [get(2 * (q // 2) + i, 2 * (q % 2) + j).astype(f32)
                            for i in range(2) for j in range(2)]
                qi, qj, sign = _BTERMS[k1]
                blk = quad(qi)
                if qj is not None:
                    blk = [u + v if sign > 0 else u - v for u, v in zip(blk, quad(qj))]
            for k, op in enumerate(_b_operands(*blk)):
                dst[base + k, pl.ds(pl.multiple_of(r, 8), 8), :] = pltpu.bitcast(
                    op.astype(bf16), u32)

        def rec_body(it, gacc):
            stream_wait(it)
            lhs_lo = lhs_h[:, 0:512]
            lhs_hi = lhs_h[:, 512:1024]
            ra = jnp.maximum(it - 1, 0) * (2 * RIDE)
            for u in range(2):
                s = 2 * it + u
                jobs = {}
                for n, (su, d, g) in enumerate(SLOTS):
                    if su == u:
                        jobs.setdefault(d, []).append(
                            lambda y, n=n, g=g: combine(it, n, y[8 * g:8 * g + 8]))
                r1 = pl.multiple_of(jnp.minimum(NPRE + RIDE * (s + 1), S - RIDE), 8)
                xn = xbuf[pl.ds(r1, RIDE), :].astype(f32)
                if u == 0:
                    for k in range(2):
                        rm = pl.multiple_of(it * 32 + k * 16, 16)
                        gacc = mod_rows(gacc, wsr[6, k * 16:(k + 1) * 16, :], rm)
                    hn = adaln_a(xn, _zero_after(stage_a16(ra)))
                else:
                    def refill(y):
                        for cp in stream_copies(jnp.minimum(it + 1, NSEG // 2 - 1)):
                            cp.start()
                        spare = pl.ds(pl.multiple_of(8 * (it // 64), 8), 8)
                        jobs["pin"] = _zero_after(ws3[16, spare, :].astype(f32))
                    jobs.setdefault(3 * (PIN - 4) + 2, []).append(refill)
                    hn = adaln_a(xn)
                    z = _zero_after(hn[0:8], hn[8:16], hn[16:24])
                    stage_a16(ra + 32, _zero_after(stage_a16(ra + 16, z)))
                a_lo, a_hi = step(s, u == 1, lhs_lo, lhs_hi, u > 0, jobs)
                lhs_lo = jnp.concatenate([a_lo[0:MEM], hn[:, 0:512]], axis=0).astype(bf16)
                lhs_hi = jnp.concatenate([a_hi[0:MEM], hn[:, 512:1024]], axis=0).astype(bf16)
                a = jnp.concatenate([a_lo, a_hi], axis=1)
                rows = [pl.multiple_of(r, 8) for r in ride_rows(s, u == 1)]
                xs = [xbuf[pl.ds(r, 8), :].astype(f32) for r in rows]
                for t, r in enumerate(rows):
                    xa = xs[t] + modrows(2, 8) * a[8 + 8 * t:16 + 8 * t]
                    xbuf[pl.ds(r, 8), :] = xa.astype(bf16)
            lhs_h[:, 0:512] = lhs_lo
            lhs_h[:, 512:1024] = lhs_hi
            return gacc

        gacc = _loop("rec", 0, NSEG // 2, rec_body, jnp.zeros((8, D), f32))
        for c in range(2):
            mod_finish(gacc[:, c * 512:(c + 1) * 512], 10 + c)
        stream_wait(NSEG // 2 - 1)

        def wo_tail(i, _):
            p0 = pl.multiple_of(i * 128, 128)
            r = pl.multiple_of(S - NPRE + i * 128, 128)
            prev = None
            lo = jnp.concatenate([rget(h, p0, 128) for h in range(H)], axis=1)
            for j in range(8):
                w = pltpu.bitcast(wqkv[WO + j * 2048:WO + (j + 1) * 2048, :], bf16)
                y = jnp.dot(lo, w, preferred_element_type=f32)
                if j < 7:
                    prev = stage_a16(r - 128 + 16 * j, _zero_after(y, prev))
                if j == 0:
                    prev = stage_a16(r - 16, _zero_after(prev))
                cs = slice(j * 128, (j + 1) * 128)
                ga = modrows(2, 128, j * 128, (j + 1) * 128)
                xbuf[pl.ds(r, 128), cs] = (xbuf[pl.ds(r, 128), cs].astype(f32) + ga * y).astype(bf16)
            return 0
        _loop("wotail", 0, NPRE // 128, wo_tail)

        def gget(c, row, n):
            return pltpu.bitcast(wqkv[pl.ds(c * GS + row, n), :], f32)

        def gset(c, row, val):
            wqkv[pl.ds(c * GS + row, val.shape[0]), :] = pltpu.bitcast(val, u32)

        def wop(j):
            return lambda k: pltpu.bitcast(w7[k, j * 256:(j + 1) * 256, :], bf16)

        zpad = jnp.zeros((GPAD, 128), f32)
        for cb in range(8):
            gset(cb, 0, zpad)
            gset(cb, GPAD + S, zpad)

        shifts = (-1, -1, 1, 1, -2, -2, 2, 2)
        HB = MB // 2

        def shift_piece(r, half, k):
            gs = jnp.concatenate([gget(c, r + (k * 16 + GPAD + shifts[c]), 16)
                                  for c in range(8)], axis=1)
            ro = half * (HB // 2) + k * 8
            for t, op in enumerate(row_operands(gs)):
                n7[t, ro:ro + 8, :] = op.astype(bf16)

        def gate(v, i):
            gset(0, GPAD + S + GPAD + 8 * (i // S), v[0:8])

        t7[...] = jnp.zeros(t7.shape, bf16)

        def b_body(i, _):
            ro = pl.multiple_of(i * HB, HB)
            rg = pl.multiple_of(GPAD + i * MB, 8)
            ra = jnp.minimum(S - 128 + 48 * i, S - 48)
            rp = jnp.minimum(S - 128 + 48 * jnp.maximum(i - 1, 0), S - 48)
            n7[:, pl.ds(pl.multiple_of(rp // 2, 8), 24), :] = t7[...]
            st = {"n": 0, "prev": None}

            def hook(v):
                n = st["n"]
                st["n"] += 1
                if n % 7 == BH and n // 7 < 3:
                    st["prev"] = stage_a16(ra + 16 * (n // 7), _zero_after(v, st["prev"]),
                                           (t7, 8 * (n // 7)))

            for j in range(4):
                c11, c12, c21, c22 = _strassen(lambda k: n7[k, pl.ds(ro, HB), :], wop(j), hook)
                gset(j + 4, rg, _gelu(_merge_rows(c12, c22)))
                gset(j, rg, _gelu(_merge_rows(c11, c21)))
            return 0
        _loop("b", 0, S // MB, b_body)
        for k in range(HB // 16):
            shift_piece(0, 0, k)

        def n2_norm(r, k, anchor):
            v = _ln(h2buf[pl.ds(pl.multiple_of(r + k * 16, 16), 16), :], anchor)
            nrms[k // 2][(k % 2) * 16:(k % 2) * 16 + 16, :] = v
            return v[0:8] + v[8:16]

        def n2_ops(k, k1, v, i):
            nrm = nrms[k]
            nrm[pl.ds(pl.multiple_of(32 + 8 * (i // S), 8), 8), 0:128] = v[0:8]

            def quad(q):
                r0, c0 = (q // 2) * 16, (q % 2) * 512
                return [nrm[r0 + 8 * a:r0 + 8 * a + 8, c0 + 256 * b:c0 + 256 * b + 256]
                        for a in range(2) for b in range(2)]
            qi, qj, sign = _ATERMS[k1]
            blk = quad(qi)
            if qj is not None:
                blk = [u + w if sign > 0 else u - w for u, w in zip(blk, quad(qj))]
            for k2, op in enumerate(_a_operands(*blk)):
                d49[7 * k1 + k2, k * 8:(k + 1) * 8, :] = op.astype(bf16)

        def n2_hook(r, i, first, gap, lag, st):
            def hook(v):
                n = st["n"] - first
                st["n"] += 1
                if n >= 0 and n % gap == 0 and n // gap < MD // 16:
                    st["prev"] = n2_norm(r, n // gap, _zero_after(v, st["prev"]))
                for _ in range(st["per"]):
                    k, k1 = divmod(st["ops"], 7)
                    if k < MD // 32 and n >= (2 * k + 1) * gap + lag:
                        n2_ops(k, k1, v, i)
                        st["ops"] += 1
            return hook

        def stage_c(i, r, half, rnext, extra):
            rr = pl.multiple_of(r, 8)
            ro = half * (HB // 2)
            cnt = [0]

            def hook(v):
                n = cnt[0]
                cnt[0] += 1
                if n < HB // 16:
                    gate(v, i)
                    shift_piece(rnext, 1 - half, n)
                extra(v)

            for j in range(4):
                c11, c12, c21, c22 = _strassen(lambda k: n7[k, ro:ro + HB // 2, :], wop(4 + j),
                                               hook)
                for c, y in ((j + 4, _merge_rows(c12, c22)), (j, _merge_rows(c11, c21))):
                    cs = slice(c * 128, (c + 1) * 128)
                    h2buf[pl.ds(rr, HB), cs] = h2buf[pl.ds(rr, HB), cs] + y

        def c_body(i, _):
            r = pl.multiple_of(i * MB, MB)
            st = {"n": 0, "prev": None, "ops": 0, "per": 1}
            extra = n2_hook(0, i, 0, 4, 4, st)
            stage_c(i, r, 0, r + HB, extra)
            stage_c(i, r + HB, 1, jnp.minimum(i + 1, S // MB - 1) * MB, extra)
            assert st["ops"] == 28
            return 0
        _loop("c", 0, S // MB, c_body)

        def wop2(lo, n):
            return lambda k1, k: pltpu.bitcast(w49[7 * k1 + k, lo:lo + n, :], bf16)

        def d_body(i, _):
            r = pl.multiple_of(i * MD, MD)
            rn = jnp.minimum(r + MD, S - MD)
            lhs = [d49[k] for k in range(49)]
            uops = []
            for t in range(7):
                cb = _strassen2(lambda k1, k: lhs[7 * k1 + k], wop2(t * 128, 128))
                uops.append(_a_operands2([[_gelu(c) for c in row] for row in cb]))
            ul = [[jnp.concatenate([u[k1][k] for u in uops], axis=1).astype(bf16)
                   for k in range(7)] for k1 in range(7)]
            st = {"n": 0, "prev": None, "ops": 0, "per": 1}
            hook = n2_hook(rn, i, DF, DG, DL, st)
            for t in range(2):
                cb = _strassen2(lambda k1, k: ul[k1][k], wop2(W4R + t * 448, 448), hook)
                for j in range(4):
                    y = jnp.concatenate([cb[q][j].reshape(MD // 32, 8, 128) for q in range(4)],
                                        axis=1).reshape(MD, 128)
                    c = 2 * j + t
                    cs = slice(c * 128, (c + 1) * 128)
                    gb = modrows(5, MD, c * 128, (c + 1) * 128)
                    o = xbuf[pl.ds(r, MD), cs].astype(f32) + gb * (h2buf[pl.ds(r, MD), cs] + y)
                    xbuf[pl.ds(r, MD), cs] = o.astype(bf16)
            assert st["ops"] == 28
            out_copy(r, MD).start()
            return 0
        _loop("d", 0, S // MD, d_body)

    pl.run_scoped(main,
                  pltpu.VMEM((7, 8 * 256, 128), u32),
                  pltpu.VMEM((49, 2 * W4R, 128), u32))

    out_copy(0, S).wait()


def _run(x, mem0, wq, wk, wv, wo, w1, w2, w3, w4, c, wmod):
    any_spec = pl.BlockSpec(memory_space=pl.ANY)
    vmem_spec = pl.BlockSpec(memory_space=pltpu.VMEM)
    return pl.pallas_call(
        _kernel,
        out_shape=jax.ShapeDtypeStruct((S, D), bf16),
        in_specs=[any_spec, vmem_spec, any_spec, any_spec, any_spec, any_spec, any_spec,
                  any_spec, any_spec, any_spec, vmem_spec, any_spec],
        out_specs=any_spec,
        scratch_shapes=[
            pltpu.VMEM((S + 2 * RIDE, D), bf16),
            pltpu.VMEM((WO + 8 * 2048, 128), u32),
            [pltpu.VMEM((96 // NRING, NR, 128), bf16)] * NRING,
            pltpu.VMEM((32, D), bf16),
            pltpu.VMEM((H, 32, 128), bf16),
            pltpu.VMEM((2 * H, 16, 128), bf16),
            pltpu.VMEM((12, 8, 512), f32),
            pltpu.VMEM((D, 128), f32),
            pltpu.VMEM((S, D), f32),
            pltpu.VMEM((7, S // 2, 512), bf16),
            pltpu.VMEM((17, 64, 128), bf16),
            pltpu.VMEM((8, 32, D), bf16),
            pltpu.VMEM((7, 24, 512), bf16),
            pltpu.VMEM((49, MD // 4, 256), bf16),
            [pltpu.VMEM((40, D), f32)] * (MD // 32),
            pltpu.SemaphoreType.DMA((9 + NGRP + 2,)),
        ],
        compiler_params=pltpu.CompilerParams(vmem_limit_bytes=124 * 1024 * 1024,
                                             disable_bounds_checks=True),
    )(x, mem0, wq, wk, wv, wo, w1, w2, w3, w4, c, wmod)


def pallas_adaLN_cond__memory_aug_recurrent_mem_tr__mixer_s_mlp__prompt_kernel(
    A_x, A_mem0, A_Wq, A_Wk, A_Wv, A_Wo, A_seg_len, B_x, B_w1, B_w2, B_w3, B_w4, c, w_mod,
):
    del B_x
    assert A_x.shape == (1, S, D) and A_mem0.shape == (1, MEM, D)
    assert isinstance(A_seg_len, int) is False or A_seg_len == SEG
    pairs = (D // 2, 2, H, DH)
    out = _run(A_x.reshape(S, D), A_mem0.reshape(MEM, D), A_Wq.reshape(pairs),
               A_Wk.reshape(pairs), A_Wv.reshape(pairs), A_Wo.reshape(H * DH // 16, 16, D),
               B_w1.reshape(2, D // 2, D), B_w2.reshape(2, D // 2, D),
               B_w3, B_w4.reshape(4, F // 4, D), c, w_mod)
    return out.reshape(1, S, D)
```

```python
import jax
import jax.numpy as jnp
from jax import lax
import jax.experimental.pallas as pl
import jax.experimental.pallas.tpu as pltpu

bf16 = jnp.bfloat16
f32 = jnp.float32
u32 = jnp.uint32

S = 2048
D = 1024
H = 32
DH = 128
F = 3584
MEM = 8
SEG = 32
NSEG = S // SEG
L = MEM + SEG
RIDE = 24
NPRE = S - RIDE * NSEG
NR = NPRE + 2 * SEG
ROFF = (-(S - NPRE)) % NR
WP = 516
WO = 96 * WP
NGRP = 12
NSLOT = 6
NMOD = 6
EPS = 1e-5
MD = 128
MB = 512
GPAD = 8
NRING = 8
RLP, WLP = 25, 22
NWO = 3
BG, WPP, PIN, BCH = 2, 5, 6, 2
DF, DG, DL = 8, 9, 9
SLOTS = ([(0, n // 2, 3 * (n % 2)) for n in range(16)] + [(0, 96 + n, 0) for n in range(16)]
         + [(0, 112 + n // 2, 3 * (n % 2)) for n in range(32)])
DSA, DPA, DSB, DPB, KSPLIT = 2, 4, 2, 4, 2
X0 = NPRE + 2 * RIDE
GS = S + 4 * GPAD
W4R = 7 * 128
_ONLY = None


def _loop(name, lo, hi, body, init=0):
    if _ONLY is not None and name not in _ONLY:
        return init
    with _scope(name):
        return lax.fori_loop(lo, hi, body, init)


class _NoScope:
    def __init__(self, name):
        del name

    def __enter__(self):
        return self

    def __exit__(self, *a):
        return False


_scope = _NoScope


def _zero_after(*vs):
    bits = None
    for v in vs:
        if v is not None:
            b = pltpu.bitcast(v[0:8, 0:128], u32)
            bits = b if bits is None else bits | b
    return pltpu.bitcast((bits >> 31) >> 1, f32)


def _ln(x, anchor=None):
    if anchor is not None:
        z = jnp.concatenate([anchor] * (x.shape[0] // 8), axis=0)
        x = jnp.concatenate([x[:, 0:128] + z, x[:, 128:]], axis=1)
    mu = jnp.mean(x, axis=-1, keepdims=True)
    xc = x - mu
    var = jnp.mean(xc * xc, axis=-1, keepdims=True)
    return xc * lax.rsqrt(var + EPS)


def _gelu(x):
    inner = x * (0.7978845608028654 + (0.7978845608028654 * 0.044715) * (x * x))
    hx = 0.5 * x
    return hx + hx * jnp.tanh(inner)


def _split_rows(x):
    m, n = x.shape
    x3 = x.reshape(m // 16, 16, n)
    return x3[:, 0:8, :].reshape(m // 2, n), x3[:, 8:16, :].reshape(m // 2, n)


def _merge_rows(top, bot):
    m, n = top.shape
    return jnp.concatenate([top.reshape(m // 8, 8, n), bot.reshape(m // 8, 8, n)],
                           axis=1).reshape(2 * m, n)


def _a_operands(a11, a12, a21, a22):
    return [a11 + a22, a21 + a22, a11, a22, a11 + a12, a21 - a11, a12 - a22]


def _b_operands(b11, b12, b21, b22):
    return [b11 + b22, b11, b12 - b22, b21 - b11, b22, b11 + b12, b21 + b22]


_ATERMS = ((0, 3, 1), (2, 3, 1), (0, None, 0), (3, None, 0), (0, 1, 1), (2, 0, -1), (1, 3, -1))
_BTERMS = ((0, 3, 1), (0, None, 0), (1, 3, -1), (2, 0, -1), (3, None, 0), (0, 1, 1), (2, 3, 1))


def _strassen(a_of, b_of, hook=lambda v: None):
    def prod(k):
        return jnp.dot(a_of(k), b_of(k), preferred_element_type=f32)
    p5 = prod(4)
    hook(p5)
    p3 = prod(2)
    hook(p3)
    c12 = p3 + p5
    p4 = prod(3)
    hook(p4)
    c11 = p4 - p5
    p2 = prod(1)
    hook(p2)
    c21 = p2 + p4
    c22 = p3 - p2
    p1 = prod(0)
    hook(p1)
    c11 = prod(6) + (c11 + p1)
    hook(c11)
    c22 = prod(5) + (c22 + p1)
    hook(c22)
    return c11, c12, c21, c22


def _a_operands2(b):
    sub = [_a_operands(b[i][j], b[i][2 + j], b[2 + i][j], b[2 + i][2 + j])
           for i in range(2) for j in range(2)]
    return [_a_operands(*[t[k] for t in sub]) for k in range(7)]


def _strassen2(a_of, b_of, hook=lambda v: None):
    def prod(k1):
        return _strassen(lambda k: a_of(k1, k), lambda k: b_of(k1, k), hook)

    def add(x, y):
        return [p + q for p, q in zip(x, y)]

    def sub(x, y):
        return [p - q for p, q in zip(x, y)]
    p5 = prod(4)
    p3 = prod(2)
    c12 = add(p3, p5)
    p4 = prod(3)
    c11 = sub(p4, p5)
    p2 = prod(1)
    c21 = add(p2, p4)
    c22 = sub(p3, p2)
    p1 = prod(0)
    c11 = add(add(c11, p1), prod(6))
    c22 = add(add(c22, p1), prod(5))
    cq = (c11, c12, c21, c22)
    return [[cq[2 * (i // 2) + j // 2][2 * (i % 2) + j % 2] for j in range(4)] for i in range(4)]


def _kernel(x_hbm, mem0_hbm, wq_hbm, wk_hbm, wv_hbm, wo_hbm, w1_hbm, w2_hbm, w3_hbm, w4_hbm,
            c_hbm, wmod_hbm, out_hbm,
            xbuf, wqkv, rings, lhs_h, lhs_o, kvm, modv, scol, h2buf, n7, ws3, wsr, t7, a7, d49, nrms, c_ref,
            sems):
    w_hbms = (wq_hbm, wk_hbm, wv_hbm)
    SMOD, SSTG = 5, 9
    sem_x, sem_out, sem_w, sem_g, sem_r = (sems.at[k] for k in range(5))

    def rget(b, row, n):
        return rings[b % NRING][b // NRING, pl.ds(row, n), :]

    def rset(b, row, val):
        rings[b % NRING][b // NRING, pl.ds(row, val.shape[0]), :] = val.astype(bf16)

    x_copy = pltpu.make_async_copy(x_hbm.at[pl.ds(0, X0), :], xbuf.at[pl.ds(0, X0), :], sem_x)

    def stream_copies(c):
        al, lo = ((lambda v, m: v), min) if isinstance(c, int) else (pl.multiple_of, jnp.minimum)
        c3 = lo(c, 27)
        cps = [pltpu.make_async_copy(
            w3_hbm.at[pl.ds(al(i * 256 + (c3 % 4) * 64, 64), 64),
                      pl.ds(al(j * (F // 4) + (c3 // 4) * 128, 128), 128)],
            ws3.at[4 * i + j], sem_w) for i in range(4) for j in range(4)]
        dst = X0 + 2 * RIDE * c
        return [
            pltpu.make_async_copy(w4_hbm.at[:, pl.ds(al(c3 * 32, 32), 32), :],
                                  wsr.at[pl.ds(0, 4)], sem_g),
            pltpu.make_async_copy(w1_hbm.at[:, pl.ds(al(c * 16, 16), 16), :],
                                  wsr.at[pl.ds(4, 2), pl.ds(0, 16), :], sem_g),
            pltpu.make_async_copy(w2_hbm.at[:, pl.ds(al(c * 16, 16), 16), :],
                                  wsr.at[pl.ds(4, 2), pl.ds(16, 16), :], sem_g),
            pltpu.make_async_copy(wmod_hbm.at[pl.ds(al(c * 32, 32), 32), pl.ds(5 * D, D)],
                                  wsr.at[6], sem_g),
            pltpu.make_async_copy(x_hbm.at[pl.ds(al(lo(dst, S - 2 * RIDE), 16), 2 * RIDE), :],
                                  xbuf.at[pl.ds(al(dst, 16), 2 * RIDE), :], sem_r)] + cps

    def stream_wait(c):
        for dst, sem in ((ws3.at[pl.ds(0, 16)], sem_w), (wsr.at[pl.ds(0, 7)], sem_g),
                         (xbuf.at[pl.ds(X0 + 2 * RIDE * c, 2 * RIDE), :], sem_r)):
            pltpu.make_async_copy(dst, dst, sem).wait()

    def out_copy(row, n):
        return pltpu.make_async_copy(xbuf.at[pl.ds(row, n), :], out_hbm.at[pl.ds(row, n), :],
                                     sem_out)

    def mod_rows(acc, w, r):
        sc = jnp.concatenate([scol[pl.ds(r, 16), :]] * (w.shape[1] // 128), axis=1)
        p = w.astype(f32) * sc
        return acc + p[0:8] + p[8:16]

    def mod_finish(acc, j):
        is_scale = jnp.logical_or(j // 2 == 1, j // 2 == 4)
        tot = jnp.sum(acc, axis=0, keepdims=True) + jnp.where(is_scale, 1.0, 0.0)
        modv[j] = jnp.broadcast_to(tot, (8, 512))

    def modrows(k, n, lo=0, hi=D):
        m = jnp.concatenate([modv[2 * k], modv[2 * k + 1]], axis=1)[:, lo:hi]
        return jnp.concatenate([m] * (n // 8), axis=0)

    def adaln_a(xv, anchor=None):
        n = xv.shape[0]
        return _ln(xv, anchor) * modrows(1, n) + modrows(0, n)

    def adaln_b(xv, anchor=None):
        n = xv.shape[0]
        return _ln(xv, anchor) * modrows(4, n) + modrows(3, n)

    def row_operands(v):
        top, bot = _split_rows(v)
        k = v.shape[1] // 2
        return _a_operands(top[:, :k], top[:, k:], bot[:, :k], bot[:, k:])

    def stage_a16(r, anchor=None, dst=None):
        rr = pl.multiple_of(r, 16)
        xv = xbuf[pl.ds(rr, 16), :]
        if dst is not None:
            xv = (xv.astype(f32) + modrows(2, 16) * h2buf[pl.ds(rr, 16), :]).astype(bf16)
            xbuf[pl.ds(rr, 16), :] = xv
        h2 = adaln_b(xv.astype(f32), anchor)
        h2buf[pl.ds(rr, 16), :] = h2
        ref, ro = (n7, pl.multiple_of(rr // 2, 8)) if dst is None else dst
        ops = row_operands(_ln(h2))
        for t, op in enumerate(ops):
            ref[t, pl.ds(ro, 8), :] = op.astype(bf16)
        return ops[0]

    def prologue(stg, wmodb):
        def mod_copy(j):
            return pltpu.make_async_copy(wmod_hbm.at[:, pl.ds(j * 512, 512)], wmodb.at[j % NMOD],
                                         sems.at[SSTG + j + 4 if j >= 4 else SMOD + j])

        def piece_copies(g, dh):
            slot = (2 * g + dh) % NSLOT
            return [pltpu.make_async_copy(
                w_hbms[g // 4].at[pl.ds(dh * 256, 256), par, pl.ds((g % 4) * 8, 8), :],
                stg.at[slot, :, pl.ds(par * 8, 8), :],
                sems.at[SSTG + (g + 1 if g else dh)]) for par in range(2)]

        def wo_copy(j):
            slot = NSLOT + j % NWO
            return pltpu.make_async_copy(wo_hbm.at[:, :, pl.ds(j * 128, 128)], stg.at[slot],
                                         sems.at[SSTG + j + 6])

        def group_start(g):
            for dh in range(2):
                for cp in piece_copies(g, dh):
                    cp.start()

        def stg_wait(slot, n, sem):
            dst = stg.at[pl.ds(slot, n)]
            pltpu.make_async_copy(dst, dst, sems.at[SSTG + sem]).wait()

        def relayout(g, slot, dh, lo_dp, n_dp):
            base = g * (8 * WP) + dh * 256
            for u in range(n_dp):
                dp = lo_dp + u
                ev = pltpu.bitcast(stg[slot, dp, 0:8, :].astype(f32), u32)
                od = pltpu.bitcast(stg[slot, dp, 8:16, :].astype(f32), u32)
                wqkv[pl.ds(base + dp, 8, stride=WP), :] = (ev >> 16) | od

        def b_operand(g, q, k):
            def quad(i):
                r = (g * 8 + q + 4 * (i % 2)) * WP + (i // 2) * 256
                return pltpu.bitcast(wqkv[pl.ds(r, 256), :], bf16)
            i, j, sign = _BTERMS[k]
            if j is None:
                return quad(i)
            u, v = quad(i).astype(f32), quad(j).astype(f32)
            return (u + v if sign > 0 else u - v).astype(bf16)

        c_copy = pltpu.make_async_copy(c_hbm, c_ref, sem_g)
        m_copy = pltpu.make_async_copy(mem0_hbm, lhs_h.at[pl.ds(0, MEM), :], sem_r)
        c_copy.start()
        m_copy.start()
        x_copy.start()
        for j in range(4):
            mod_copy(j).start()
        for g in range(3):
            group_start(g)
        h2buf[S - NPRE:S, :] = jnp.zeros((NPRE, D), f32)
        c_copy.wait()
        m_copy.wait()
        cv = c_ref[...].astype(f32)
        sv = jnp.broadcast_to(cv * (1.0 / (1.0 + jnp.exp(-cv))), (128, D))
        for k in range(8):
            scol[k * 128:(k + 1) * 128, :] = sv[:, k * 128:(k + 1) * 128].T
        x_copy.wait()

        def ln0_body(i, _):
            r = pl.multiple_of(i * 64, 64)
            h2buf[pl.ds(r, 64), :] = _ln(xbuf[pl.ds(r, 64), :].astype(f32))
            return 0
        lax.fori_loop(0, NPRE // 64, ln0_body, 0)

        def mod0_body(j, _):
            pltpu.make_async_copy(wmodb.at[j], wmodb.at[j], sems.at[SMOD + j]).wait()
            accs = [jnp.zeros((8, 512), f32)] * 2
            for k in range(64):
                accs[k % 2] = mod_rows(accs[k % 2], wmodb[j, k * 16:(k + 1) * 16, :], k * 16)
            mod_finish(accs[0] + accs[1], j)
            return 0
        _loop("mod0", 0, 4, mod0_body)

        def hpre_body(i, _):
            r = pl.multiple_of(i * 32, 32)
            hv = h2buf[pl.ds(r, 32), :] * modrows(1, 32) + modrows(0, 32)
            ro = pl.multiple_of(i * 16, 16)
            for t, op in enumerate(row_operands(hv)):
                n7[t, pl.ds(ro, 16), :] = op.astype(bf16)
            return 0
        lax.fori_loop(0, NPRE // 32, hpre_body, 0)
        lhs_h[MEM:32, :] = adaln_a(xbuf[NPRE:NPRE + RIDE, :].astype(f32)).astype(bf16)

        def relayout_now(g, dh):
            def rl_body(t, _):
                relayout(g, 2 * g + dh, dh, t * 32, 32)
                return 0
            lax.fori_loop(0, 8, rl_body, 0)

        for dh in range(2):
            stg_wait(dh, 1, dh)
            relayout_now(0, dh)

        grp = lambda g: piece_copies(g, 0) + piece_copies(g, 1)
        issue = {0: [wo_copy(0)], 1: grp(3) + grp(4), 2: grp(5) + [wo_copy(1), mod_copy(4)],
                 3: grp(6) + [wo_copy(2), mod_copy(5)], 4: grp(7) + [mod_copy(6)],
                 5: grp(8) + [wo_copy(3), mod_copy(7)], 6: grp(9) + [wo_copy(4)],
                 7: grp(10) + [wo_copy(5), mod_copy(8)], 8: grp(11) + [wo_copy(6)],
                 9: [wo_copy(7), mod_copy(9)], 10: stream_copies(0)}

        def pre_iter(g, m3):
            m3n = jnp.where(m3 == 2, 0, m3 + 1)
            ends = jnp.logical_or(g == 0, g == NGRP - 1)
            gn = jnp.where(ends, g, g + 1)
            gslot = 2 * jnp.where(ends, m3, m3n)
            wj = jnp.maximum(g - 4, 0)
            wslot = jnp.where(g < 4, gslot, NSLOT + jnp.where(m3 == 0, 2, m3 - 1))
            cj = jnp.maximum(g - 2, 3)
            cslot = jnp.where(cj >= NMOD, cj - NMOD, cj)

            @pl.when(g == 1)
            def _():
                stg_wait(2, 2, 2)
                relayout_now(1, 0)
                relayout_now(1, 1)

            @pl.when(jnp.logical_not(ends))
            def _():
                stg_wait(gslot, 2, g + 2)

            @pl.when(g >= 4)
            def _():
                stg_wait(wslot, 1, g + 2)

            @pl.when(g >= 6)
            def _():
                pltpu.make_async_copy(wmodb.at[cslot], wmodb.at[cslot],
                                      sems.at[SSTG + g + 2]).wait()

            for k, cps in issue.items():
                @pl.when(g == k)
                def _():
                    for cp in cps:
                        cp.start()
            wtodo = list(range(0, 256, 2))
            todo = [(dh, dp) for dh in range(2) for dp in range(256)]
            mtodo = list(range(0, D, 16))
            macc = [jnp.zeros((8, 512), f32)]

            def hook(v):
                if mtodo:
                    acc = macc[0] + jnp.concatenate([_zero_after(v)] * 4, axis=1)
                    for r in mtodo[:3]:
                        acc = mod_rows(acc, wmodb[cslot, r:r + 16, :], r)
                    del mtodo[:3]
                    macc[0] = acc

            for q in range(4):
                def b_of(k):
                    w = b_operand(g, q, k)
                    nw = 0 if todo else WLP
                    for dh, dp in todo[:RLP]:
                        relayout(gn, gslot + dh, dh, dp, 1)
                    del todo[:RLP]
                    for c in wtodo[:nw]:
                        wqkv[pl.ds(pl.multiple_of(WO + wj * 2048 + c * 8, 16), 16), :] = (
                            pltpu.bitcast(stg[wslot, c:c + 2].reshape(32, 128), u32))
                    del wtodo[:nw]
                    return w
                c11, c12, c21, c22 = _strassen(lambda k: n7[k, 0:NPRE // 2, :], b_of, hook)
                for blk, y in ((q + 4, _merge_rows(c12, c22)), (q, _merge_rows(c11, c21))):
                    y = y.astype(bf16)
                    n0 = NR - ROFF
                    rings[blk][g, ROFF:NR, :] = y[0:n0]
                    rings[blk][g, 0:NPRE - n0, :] = y[n0:NPRE]
            assert not todo and not wtodo and not mtodo
            mod_finish(macc[0], cj)
            return m3n

        _loop("pre1", 0, NGRP, pre_iter)

    pl.run_scoped(prologue,
                  pltpu.VMEM((NSLOT + NWO, 256, 16, 128), bf16),
                  pltpu.VMEM((NMOD, D, 512), bf16))

    def main(w7, w49):
        scale = DH ** -0.5
        ia = lax.broadcasted_iota(jnp.int32, (32, L), 0)
        ja = lax.broadcasted_iota(jnp.int32, (32, L), 1)
        mask_a = (ia >= RIDE) | (ja >= SEG) | (ia + 8 >= ja)
        ib = lax.broadcasted_iota(jnp.int32, (48, 56), 0)
        jb = lax.broadcasted_iota(jnp.int32, (48, 56), 1)
        own = (ib < 40) == (jb < 40)
        mask_b = own & (((jb >= 32) & (jb < 48)) | (jnp.where(jb < 40, jb, jb - 8) <= ib))
        masked = -1e9 / scale
        j8 = lax.broadcasted_iota(jnp.int32, (8, 56), 1)
        fill_b = jnp.concatenate([jnp.where(j8 < 40, masked, -3e38).astype(f32)] * 5
                                 + [jnp.where(j8 < 40, -3e38, masked).astype(f32)], axis=0)

        def softmax(sc, mask, fill):
            sc = jnp.where(mask, sc, fill)
            mx = jnp.max(sc, axis=-1, keepdims=True)
            e = jnp.exp2((sc - mx) * (scale * 1.4426950408889634))
            den = jnp.sum(e, axis=-1, keepdims=True)
            return (e * pl.reciprocal(den, approx=True)).astype(bf16)

        def ride_rows(s, is_b):
            first = s < 2
            if is_b:
                g = [jnp.where(first, -3, -1), 1, 2]
            else:
                g = [jnp.where(first, 1, 0), jnp.where(first, 2, 1), 3]
            return [RIDE * s + 8 * t for t in g]

        def step(s, is_b, lhs_lo, lhs_hi, soft_in, jobs):
            seg = pl.multiple_of((SEG * s + ROFF) % NR, SEG)
            sega = pl.multiple_of(seg - SEG, SEG) if is_b else seg
            wr = [pl.multiple_of((NPRE + RIDE * s + 8 * t + ROFF) % NR, 8) for t in range(3)]
            rd = [pl.multiple_of((r + ROFF) % NR, 8) for r in ride_rows(s, is_b)]
            lhs = jnp.concatenate([lhs_lo, lhs_hi], axis=1)
            QM, P, PART = {}, {}, {}
            mrow = 0 if is_b else MEM
            seg8 = pl.multiple_of(seg + 8, 8)
            seg24 = pl.multiple_of(seg + RIDE, 8)

            def wblk(b, lo, n):
                return pltpu.bitcast(wqkv[b * WP + lo:b * WP + lo + n, :], bf16)

            def qkv_lo(i):
                for m in range(3):
                    PART[(m, i)] = jnp.dot(lhs_lo, wblk(m * H + i, 0, 256), preferred_element_type=f32)

            def qkv(i):
                for m in range(3):
                    b = m * H + i
                    if (m, i) in PART:
                        y = jnp.dot(lhs_hi, wblk(b, 256, 256),
                                    preferred_element_type=f32) + PART.pop((m, i))
                    else:
                        y = jnp.dot(lhs, wblk(b, 0, 512), preferred_element_type=f32)
                    if m < 2:
                        QM[b] = y[0:MEM] + jobs["pin"] if b == PIN and is_b else y[0:MEM]
                    if m == 2 or (m == 1 and not is_b):
                        kvm[b - H, mrow:mrow + MEM, :] = y[0:MEM].astype(bf16)
                    for t in range(3):
                        rset(b, wr[t], y[8 + 8 * t:16 + 8 * t])
                    for job in jobs.get(3 * i + m, []):
                        job(y)

            def keys(b):
                if is_b:
                    if b in QM:
                        old = kvm[b - H, MEM:2 * MEM, :].astype(f32)
                        mix = jnp.concatenate([QM.pop(b), old], axis=0).astype(bf16)
                    else:
                        mix = kvm[b - H]
                    return jnp.concatenate([rget(b, seg, SEG), mix, rget(b, sega, 8)], axis=0)
                mk = QM.pop(b).astype(bf16) if b in QM else kvm[b - H, MEM:2 * MEM, :]
                return jnp.concatenate([rget(b, seg, SEG), mk], axis=0)

            def scores(i):
                if is_b:
                    mix = jnp.concatenate([QM.pop(i), rget(i, sega, 8).astype(f32)], axis=0)
                    q = jnp.concatenate([rget(i, seg, SEG), mix.astype(bf16)], axis=0)
                else:
                    mix = jnp.concatenate([rget(i, seg24, 8).astype(f32), QM.pop(i)], axis=0)
                    q = jnp.concatenate([rget(i, seg8, 16), mix.astype(bf16)], axis=0)
                sc = lax.dot_general(q, keys(H + i), (((1,), (1,)), ((), ())),
                                     preferred_element_type=f32)
                P[i] = softmax(sc, mask_b, fill_b) if is_b else softmax(sc, mask_a, masked)

            def pv(i):
                o = jnp.dot(P.pop(i), keys(2 * H + i), preferred_element_type=f32)
                if is_b:
                    rset(i, seg, o[0:SEG])
                    rset(i, sega, o[40:48])
                    lhs_o[i, 0:MEM, :] = o[SEG:L].astype(bf16)
                else:
                    rset(i, seg8, o[0:16])
                    rset(i, seg24, o[16:RIDE])
                    lhs_o[i, 0:MEM, :] = o[RIDE:32].astype(bf16)
                for t in range(3):
                    lhs_o[i, 8 + 8 * t:16 + 8 * t, :] = rget(i, rd[t], 8)

            def wo_lhs(i0, i1):
                return jnp.concatenate([lhs_o[i] for i in range(i0, i1)], axis=1)

            def wo_dot(lo, j, i0, i1):
                r = WO + j * 2048
                w = pltpu.bitcast(wqkv[r + 64 * i0:r + 64 * i1, :], bf16)
                return jnp.dot(lo, w, preferred_element_type=f32)

            def side(t):
                ds, dp = (DSB, DPB) if is_b else (DSA, DPA)
                if 0 <= t - dp < H:
                    pv(t - dp)
                if 0 <= t - ds < H:
                    scores(t - ds)

            if soft_in:
                for h in range(KSPLIT):
                    qkv_lo(h)
            for h in range(H):
                qkv(h)
                side(h)
            lo = [wo_lhs(8 * k, 8 * k + 8) for k in range(3)]
            acc = []
            for j in range(8):
                y = None
                for k in range(3):
                    z = wo_dot(lo[k], j, 8 * k, 8 * k + 8)
                    y = z if y is None else z + y
                    for job in jobs.get(96 + 3 * j + k, []):
                        job(y)
                acc.append(y)
                side(H + j)
            lo = wo_lhs(24, H)
            for j in range(8):
                acc[j] = wo_dot(lo, j, 24, H) + acc[j]
                for job in jobs.get(120 + j, []):
                    job(acc[j])
            assert not (QM or P or PART)
            return jnp.concatenate(acc[0:4], axis=1), jnp.concatenate(acc[4:8], axis=1)

        def combine(c, n, y):
            mp, k1 = divmod(n, 8)
            m, p = divmod(mp, 4)
            c3 = jnp.minimum(c, 27)
            spare = pl.ds(pl.multiple_of(8 * (c // 64), 8), 8)
            if m == 0 and k1 < 7:
                ws3[16, spare, :] = y.astype(bf16)
            else:
                wsr[7, spare, 0:128] = y.astype(bf16)
            if k1 == 7:
                dst, base, r = w7, 0, (4 * m + p) * 256 + c * 8
                blk = [wsr[4 + i, m * 16:(m + 1) * 16, j * 512 + p * 128:j * 512 + (p + 1) * 128]
                       .astype(f32) for i in range(2) for j in range(2)]
            else:
                dst, base = w49, 7 * k1
                if m == 0:
                    r = c3 * 32 + p * 8
                    get = lambda i, j: ws3[4 * i + j, p * 16:(p + 1) * 16, :]
                else:
                    r = W4R + (p // 2) * 448 + c3 * 16 + (p % 2) * 8
                    r0, c0 = (p % 2) * 16, (p // 2) * 128
                    get = lambda i, j: wsr[i, r0:r0 + 16, j * 256 + c0:j * 256 + c0 + 128]

                def quad(q):
                    return [get(2 * (q // 2) + i, 2 * (q % 2) + j).astype(f32)
                            for i in range(2) for j in range(2)]
                qi, qj, sign = _BTERMS[k1]
                blk = quad(qi)
                if qj is not None:
                    blk = [u + v if sign > 0 else u - v for u, v in zip(blk, quad(qj))]
            for k, op in enumerate(_b_operands(*blk)):
                dst[base + k, pl.ds(pl.multiple_of(r, 8), 8), :] = pltpu.bitcast(
                    op.astype(bf16), u32)

        def rec_body(it, gacc):
            stream_wait(it)
            lhs_lo = lhs_h[:, 0:512]
            lhs_hi = lhs_h[:, 512:1024]
            ra = jnp.maximum(it - 1, 0) * (2 * RIDE)
            for u in range(2):
                s = 2 * it + u
                jobs = {}
                for n, (su, d, g) in enumerate(SLOTS):
                    if su == u:
                        jobs.setdefault(d, []).append(
                            lambda y, n=n, g=g: combine(it, n, y[8 * g:8 * g + 8]))
                r1 = pl.multiple_of(jnp.minimum(NPRE + RIDE * (s + 1), S - RIDE), 8)
                xn = xbuf[pl.ds(r1, RIDE), :].astype(f32)
                if u == 0:
                    for k in range(2):
                        rm = pl.multiple_of(it * 32 + k * 16, 16)
                        gacc = mod_rows(gacc, wsr[6, k * 16:(k + 1) * 16, :], rm)
                    hn = adaln_a(xn, _zero_after(stage_a16(ra)))
                else:
                    def refill(y):
                        for cp in stream_copies(jnp.minimum(it + 1, NSEG // 2 - 1)):
                            cp.start()
                        spare = pl.ds(pl.multiple_of(8 * (it // 64), 8), 8)
                        jobs["pin"] = _zero_after(ws3[16, spare, :].astype(f32))
                    jobs.setdefault(3 * (PIN - 4) + 2, []).append(refill)
                    hn = adaln_a(xn)
                    z = _zero_after(hn[0:8], hn[8:16], hn[16:24])
                    stage_a16(ra + 32, _zero_after(stage_a16(ra + 16, z)))
                a_lo, a_hi = step(s, u == 1, lhs_lo, lhs_hi, u > 0, jobs)
                lhs_lo = jnp.concatenate([a_lo[0:MEM], hn[:, 0:512]], axis=0).astype(bf16)
                lhs_hi = jnp.concatenate([a_hi[0:MEM], hn[:, 512:1024]], axis=0).astype(bf16)
                a = jnp.concatenate([a_lo, a_hi], axis=1)
                rows = [pl.multiple_of(r, 8) for r in ride_rows(s, u == 1)]
                xs = [xbuf[pl.ds(r, 8), :].astype(f32) for r in rows]
                for t, r in enumerate(rows):
                    xa = xs[t] + modrows(2, 8) * a[8 + 8 * t:16 + 8 * t]
                    xbuf[pl.ds(r, 8), :] = xa.astype(bf16)
            lhs_h[:, 0:512] = lhs_lo
            lhs_h[:, 512:1024] = lhs_hi
            return gacc

        gacc = _loop("rec", 0, NSEG // 2, rec_body, jnp.zeros((8, D), f32))
        for c in range(2):
            mod_finish(gacc[:, c * 512:(c + 1) * 512], 10 + c)
        stream_wait(NSEG // 2 - 1)

        def wo_prep(i, half, k):
            o = jnp.concatenate([rings[4 * half + h][i, k * 16:(k + 1) * 16, :].astype(f32)
                                 for h in range(4)], axis=1)
            for t, op in enumerate(row_operands(o)):
                a7[half, t, k * 8:(k + 1) * 8, :] = op.astype(bf16)

        def wo_chunk(i, half, inext, extra):
            row = pl.multiple_of(i * 512 + half * 256, 256)
            todo = list(range(NPRE // 16))
            spare = pl.ds(pl.multiple_of(8 * (i // 64), 8), 8)

            def hook(v):
                if todo:
                    for h in range(4):
                        rings[4 * (1 - half) + h][4, spare, :] = v[0:8].astype(bf16)
                    n = 2 if len(todo) % WPP == 0 else 1
                    for k in todo[:n]:
                        wo_prep(inext, 1 - half, k)
                    del todo[:n]
                extra(v)

            for j in range(4):
                def b_of(k):
                    def quad(q):
                        r = WO + (j + 4 * (q % 2)) * 2048 + (q // 2) * 128 + row
                        return pltpu.bitcast(wqkv[pl.ds(r, 128), :], bf16)
                    qi, qj, sign = _BTERMS[k]
                    if qj is None:
                        return quad(qi)
                    u, v = quad(qi).astype(f32), quad(qj).astype(f32)
                    return (u + v if sign > 0 else u - v).astype(bf16)
                c11, c12, c21, c22 = _strassen(lambda k: a7[half, k], b_of, hook)
                for c, y in ((j + 4, _merge_rows(c12, c22)), (j, _merge_rows(c11, c21))):
                    cs = slice(c * 128, (c + 1) * 128)
                    h2buf[S - NPRE:S, cs] = h2buf[S - NPRE:S, cs] + y

        for k in range(NPRE // 16):
            wo_prep(0, 0, k)

        def wo_tail(i, _):
            st = {"n": 0, "prev": None}

            def extra(v):
                n = st["n"]
                st["n"] += 1
                if n % 16 == 2 and n // 16 < 3:
                    st["prev"] = stage_a16(S - NPRE - 48 + 16 * (n // 16),
                                           _zero_after(v, st["prev"]))
            wo_chunk(i, 0, i, extra)
            wo_chunk(i, 1, jnp.minimum(i + 1, 3), extra)
            return 0
        _loop("wotail", 0, 4, wo_tail)

        def gget(c, row, n):
            return pltpu.bitcast(wqkv[pl.ds(c * GS + row, n), :], f32)

        def gset(c, row, val):
            wqkv[pl.ds(c * GS + row, val.shape[0]), :] = pltpu.bitcast(val, u32)

        def wop(j):
            return lambda k: pltpu.bitcast(w7[k, j * 256:(j + 1) * 256, :], bf16)

        zpad = jnp.zeros((GPAD, 128), f32)
        for cb in range(8):
            gset(cb, 0, zpad)
            gset(cb, GPAD + S, zpad)

        shifts = (-1, -1, 1, 1, -2, -2, 2, 2)
        HB = MB // 2

        def shift_piece(r, half, k):
            gs = jnp.concatenate([gget(c, r + (k * 16 + GPAD + shifts[c]), 16)
                                  for c in range(8)], axis=1)
            ro = half * (HB // 2) + k * 8
            for t, op in enumerate(row_operands(gs)):
                n7[t, ro:ro + 8, :] = op.astype(bf16)

        def gate(v, i):
            gset(0, GPAD + S + GPAD + 8 * (i // S), v[0:8])

        def b_body(i, _):
            rl = S - NPRE + i * 128
            st = {"n": 0, "prev": [None, None]}

            def hook(v):
                n = st["n"]
                st["n"] += 1
                if n % BG == 0 and n // BG < 8:
                    k = n // BG
                    st["prev"][k % BCH] = stage_a16(rl + 16 * k,
                                                    _zero_after(v, st["prev"][k % BCH]),
                                                    (t7, 8 * k))

            ro = pl.multiple_of(i * 192, 64)
            for lhs, row in ((lambda k: n7[k, pl.ds(ro, 192), :], i * 384), (lambda k: t7[k], rl)):
                rg = pl.multiple_of(GPAD + row, 8)
                for j in range(4):
                    c11, c12, c21, c22 = _strassen(lhs, wop(j), hook)
                    gset(j + 4, rg, _gelu(_merge_rows(c12, c22)))
                    gset(j, rg, _gelu(_merge_rows(c11, c21)))
            return 0
        _loop("b", 0, S // MB, b_body)
        for k in range(HB // 16):
            shift_piece(0, 0, k)

        def n2_norm(r, k, anchor):
            v = _ln(h2buf[pl.ds(pl.multiple_of(r + k * 16, 16), 16), :], anchor)
            nrms[k // 2][(k % 2) * 16:(k % 2) * 16 + 16, :] = v
            return v[0:8] + v[8:16]

        def n2_ops(k, k1, v, i):
            nrm = nrms[k]
            nrm[pl.ds(pl.multiple_of(32 + 8 * (i // S), 8), 8), 0:128] = v[0:8]

            def quad(q):
                r0, c0 = (q // 2) * 16, (q % 2) * 512
                return [nrm[r0 + 8 * a:r0 + 8 * a + 8, c0 + 256 * b:c0 + 256 * b + 256]
                        for a in range(2) for b in range(2)]
            qi, qj, sign = _ATERMS[k1]
            blk = quad(qi)
            if qj is not None:
                blk = [u + w if sign > 0 else u - w for u, w in zip(blk, quad(qj))]
            for k2, op in enumerate(_a_operands(*blk)):
                d49[7 * k1 + k2, k * 8:(k + 1) * 8, :] = op.astype(bf16)

        def n2_hook(r, i, first, gap, lag, st):
            def hook(v):
                n = st["n"] - first
                st["n"] += 1
                if n >= 0 and n % gap == 0 and n // gap < MD // 16:
                    st["prev"] = n2_norm(r, n // gap, _zero_after(v, st["prev"]))
                for _ in range(st["per"]):
                    k, k1 = divmod(st["ops"], 7)
                    if k < MD // 32 and n >= (2 * k + 1) * gap + lag:
                        n2_ops(k, k1, v, i)
                        st["ops"] += 1
            return hook

        def stage_c(i, r, half, rnext, extra):
            rr = pl.multiple_of(r, 8)
            ro = half * (HB // 2)
            cnt = [0]

            def hook(v):
                n = cnt[0]
                cnt[0] += 1
                if n < HB // 16:
                    gate(v, i)
                    shift_piece(rnext, 1 - half, n)
                extra(v)

            for j in range(4):
                c11, c12, c21, c22 = _strassen(lambda k: n7[k, ro:ro + HB // 2, :], wop(4 + j),
                                               hook)
                for c, y in ((j + 4, _merge_rows(c12, c22)), (j, _merge_rows(c11, c21))):
                    cs = slice(c * 128, (c + 1) * 128)
                    h2buf[pl.ds(rr, HB), cs] = h2buf[pl.ds(rr, HB), cs] + y

        def c_body(i, _):
            r = pl.multiple_of(i * MB, MB)
            st = {"n": 0, "prev": None, "ops": 0, "per": 1}
            extra = n2_hook(0, i, 0, 4, 4, st)
            stage_c(i, r, 0, r + HB, extra)
            stage_c(i, r + HB, 1, jnp.minimum(i + 1, S // MB - 1) * MB, extra)
            assert st["ops"] == 28
            return 0
        _loop("c", 0, S // MB, c_body)

        def wop2(lo, n):
            return lambda k1, k: pltpu.bitcast(w49[7 * k1 + k, lo:lo + n, :], bf16)

        def d_body(i, _):
            r = pl.multiple_of(i * MD, MD)
            rn = jnp.minimum(r + MD, S - MD)
            lhs = [d49[k] for k in range(49)]
            uops = []
            for t in range(7):
                cb = _strassen2(lambda k1, k: lhs[7 * k1 + k], wop2(t * 128, 128))
                uops.append(_a_operands2([[_gelu(c) for c in row] for row in cb]))
            ul = [[jnp.concatenate([u[k1][k] for u in uops], axis=1).astype(bf16)
                   for k in range(7)] for k1 in range(7)]
            st = {"n": 0, "prev": None, "ops": 0, "per": 1}
            hook = n2_hook(rn, i, DF, DG, DL, st)
            for t in range(2):
                cb = _strassen2(lambda k1, k: ul[k1][k], wop2(W4R + t * 448, 448), hook)
                for j in range(4):
                    y = jnp.concatenate([cb[q][j].reshape(MD // 32, 8, 128) for q in range(4)],
                                        axis=1).reshape(MD, 128)
                    c = 2 * j + t
                    cs = slice(c * 128, (c + 1) * 128)
                    gb = modrows(5, MD, c * 128, (c + 1) * 128)
                    o = xbuf[pl.ds(r, MD), cs].astype(f32) + gb * (h2buf[pl.ds(r, MD), cs] + y)
                    xbuf[pl.ds(r, MD), cs] = o.astype(bf16)
            assert st["ops"] == 28
            out_copy(r, MD).start()
            return 0
        _loop("d", 0, S // MD, d_body)

    pl.run_scoped(main,
                  pltpu.VMEM((7, 8 * 256, 128), u32),
                  pltpu.VMEM((49, 2 * W4R, 128), u32))

    out_copy(0, S).wait()


def _run(x, mem0, wq, wk, wv, wo, w1, w2, w3, w4, c, wmod):
    any_spec = pl.BlockSpec(memory_space=pl.ANY)
    return pl.pallas_call(
        _kernel,
        out_shape=jax.ShapeDtypeStruct((S, D), bf16),
        in_specs=[any_spec] * 12,
        out_specs=any_spec,
        scratch_shapes=[
            pltpu.VMEM((S + 2 * RIDE, D), bf16),
            pltpu.VMEM((WO + 8 * 2048, 128), u32),
            [pltpu.VMEM((96 // NRING, NR, 128), bf16)] * NRING,
            pltpu.VMEM((32, D), bf16),
            pltpu.VMEM((H, 32, 128), bf16),
            pltpu.VMEM((2 * H, 16, 128), bf16),
            pltpu.VMEM((12, 8, 512), f32),
            pltpu.VMEM((D, 128), f32),
            pltpu.VMEM((S, D), f32),
            pltpu.VMEM((7, (S - NPRE) // 2, 512), bf16),
            pltpu.VMEM((17, 64, 128), bf16),
            pltpu.VMEM((8, 32, D), bf16),
            pltpu.VMEM((7, 64, 512), bf16),
            pltpu.VMEM((2, 7, NPRE // 2, 256), bf16),
            pltpu.VMEM((49, MD // 4, 256), bf16),
            [pltpu.VMEM((40, D), f32)] * (MD // 32),
            pltpu.VMEM((1, D), bf16),
            pltpu.SemaphoreType.DMA((9 + NGRP + 2,)),
        ],
        compiler_params=pltpu.CompilerParams(vmem_limit_bytes=124 * 1024 * 1024,
                                             disable_bounds_checks=True),
    )(x, mem0, wq, wk, wv, wo, w1, w2, w3, w4, c, wmod)


def pallas_adaLN_cond__memory_aug_recurrent_mem_tr__mixer_s_mlp__prompt_kernel(
    A_x, A_mem0, A_Wq, A_Wk, A_Wv, A_Wo, A_seg_len, B_x, B_w1, B_w2, B_w3, B_w4, c, w_mod,
):
    del B_x
    assert A_x.shape == (1, S, D) and A_mem0.shape == (1, MEM, D)
    assert isinstance(A_seg_len, int) is False or A_seg_len == SEG
    pairs = (D // 2, 2, H, DH)
    out = _run(A_x.reshape(S, D), A_mem0.reshape(MEM, D), A_Wq.reshape(pairs),
               A_Wk.reshape(pairs), A_Wv.reshape(pairs), A_Wo.reshape(H * DH // 16, 16, D),
               B_w1.reshape(2, D // 2, D), B_w2.reshape(2, D // 2, D),
               B_w3, B_w4.reshape(4, F // 4, D), c, w_mod)
    return out.reshape(1, S, D)
```

```python
import jax
import jax.numpy as jnp
from jax import lax
import jax.experimental.pallas as pl
import jax.experimental.pallas.tpu as pltpu

bf16 = jnp.bfloat16
f32 = jnp.float32
u32 = jnp.uint32

S = 2048
D = 1024
H = 32
DH = 128
F = 3584
MEM = 8
SEG = 32
NSEG = S // SEG
L = MEM + SEG
RIDE = 24
NPRE = S - RIDE * NSEG
NR = NPRE + 2 * SEG
ROFF = (-(S - NPRE)) % NR
WP = 516
WO = 96 * WP
NGRP = 12
NSLOT = 6
NMOD = 6
EPS = 1e-5
MD = 128
MB = 512
GPAD = 8
NRING = 8
RLP, WLP = 25, 22
NWO = 3
BG, WPP, PIN, BCH = 2, 5, 6, 2
DF, DG, DL = 8, 9, 9
SLOTS = ([(0, n // 2, 3 * (n % 2)) for n in range(16)] + [(0, 96 + n, 0) for n in range(16)]
         + [(0, 112 + n // 2, 3 * (n % 2)) for n in range(32)])
DSA, DPA, DSB, DPB, KSPLIT = 2, 4, 2, 4, 2
X0 = NPRE + 2 * RIDE
GS = S + 4 * GPAD
W4R = 7 * 128
_ONLY = None


def _loop(name, lo, hi, body, init=0):
    if _ONLY is not None and name not in _ONLY:
        return init
    with _scope(name):
        return lax.fori_loop(lo, hi, body, init)


class _NoScope:
    def __init__(self, name):
        del name

    def __enter__(self):
        return self

    def __exit__(self, *a):
        return False


_scope = _NoScope


def _zero_after(*vs):
    bits = None
    for v in vs:
        if v is not None:
            b = pltpu.bitcast(v[0:8, 0:128], u32)
            bits = b if bits is None else bits | b
    return pltpu.bitcast((bits >> 31) >> 1, f32)


def _ln(x, anchor=None):
    if anchor is not None:
        z = jnp.concatenate([anchor] * (x.shape[0] // 8), axis=0)
        x = jnp.concatenate([x[:, 0:128] + z, x[:, 128:]], axis=1)
    mu = jnp.mean(x, axis=-1, keepdims=True)
    xc = x - mu
    var = jnp.mean(xc * xc, axis=-1, keepdims=True)
    return xc * lax.rsqrt(var + EPS)


def _gelu(x):
    inner = x * (0.7978845608028654 + (0.7978845608028654 * 0.044715) * (x * x))
    hx = 0.5 * x
    return hx + hx * jnp.tanh(inner)


def _split_rows(x):
    m, n = x.shape
    x3 = x.reshape(m // 16, 16, n)
    return x3[:, 0:8, :].reshape(m // 2, n), x3[:, 8:16, :].reshape(m // 2, n)


def _merge_rows(top, bot):
    m, n = top.shape
    return jnp.concatenate([top.reshape(m // 8, 8, n), bot.reshape(m // 8, 8, n)],
                           axis=1).reshape(2 * m, n)


def _a_operands(a11, a12, a21, a22):
    return [a11 + a22, a21 + a22, a11, a22, a11 + a12, a21 - a11, a12 - a22]


def _b_operands(b11, b12, b21, b22):
    return [b11 + b22, b11, b12 - b22, b21 - b11, b22, b11 + b12, b21 + b22]


_ATERMS = ((0, 3, 1), (2, 3, 1), (0, None, 0), (3, None, 0), (0, 1, 1), (2, 0, -1), (1, 3, -1))
_BTERMS = ((0, 3, 1), (0, None, 0), (1, 3, -1), (2, 0, -1), (3, None, 0), (0, 1, 1), (2, 3, 1))


def _strassen(a_of, b_of, hook=lambda v: None):
    def prod(k):
        return jnp.dot(a_of(k), b_of(k), preferred_element_type=f32)
    p5 = prod(4)
    hook(p5)
    p3 = prod(2)
    hook(p3)
    c12 = p3 + p5
    p4 = prod(3)
    hook(p4)
    c11 = p4 - p5
    p2 = prod(1)
    hook(p2)
    c21 = p2 + p4
    c22 = p3 - p2
    p1 = prod(0)
    hook(p1)
    c11 = prod(6) + (c11 + p1)
    hook(c11)
    c22 = prod(5) + (c22 + p1)
    hook(c22)
    return c11, c12, c21, c22


def _a_operands2(b):
    sub = [_a_operands(b[i][j], b[i][2 + j], b[2 + i][j], b[2 + i][2 + j])
           for i in range(2) for j in range(2)]
    return [_a_operands(*[t[k] for t in sub]) for k in range(7)]


def _strassen2(a_of, b_of, hook=lambda v: None):
    def prod(k1):
        return _strassen(lambda k: a_of(k1, k), lambda k: b_of(k1, k), hook)

    def add(x, y):
        return [p + q for p, q in zip(x, y)]

    def sub(x, y):
        return [p - q for p, q in zip(x, y)]
    p5 = prod(4)
    p3 = prod(2)
    c12 = add(p3, p5)
    p4 = prod(3)
    c11 = sub(p4, p5)
    p2 = prod(1)
    c21 = add(p2, p4)
    c22 = sub(p3, p2)
    p1 = prod(0)
    c11 = add(add(c11, p1), prod(6))
    c22 = add(add(c22, p1), prod(5))
    cq = (c11, c12, c21, c22)
    return [[cq[2 * (i // 2) + j // 2][2 * (i % 2) + j % 2] for j in range(4)] for i in range(4)]


def _kernel(x_hbm, mem0_hbm, wq_hbm, wk_hbm, wv_hbm, wo_hbm, w1_hbm, w2_hbm, w3_hbm, w4_hbm,
            c_hbm, wmod_hbm, out_hbm,
            xbuf, wqkv, rings, lhs_h, lhs_o, kvm, modv, scol, h2buf, n7, ws3, wsr, t7, a7, d49, nrms, c_ref,
            sems):
    w_hbms = (wq_hbm, wk_hbm, wv_hbm)
    SMOD, SSTG = 5, 9
    sem_x, sem_out, sem_w, sem_g, sem_r = (sems.at[k] for k in range(5))

    def rget(b, row, n):
        return rings[b % NRING][b // NRING, pl.ds(row, n), :]

    def rset(b, row, val):
        rings[b % NRING][b // NRING, pl.ds(row, val.shape[0]), :] = val.astype(bf16)

    x_copy = pltpu.make_async_copy(x_hbm.at[pl.ds(0, X0), :], xbuf.at[pl.ds(0, X0), :], sem_x)

    def stream_copies(c):
        al, lo = ((lambda v, m: v), min) if isinstance(c, int) else (pl.multiple_of, jnp.minimum)
        c3 = lo(c, 27)
        cps = [pltpu.make_async_copy(
            w3_hbm.at[pl.ds(al(i * 256 + (c3 % 4) * 64, 64), 64),
                      pl.ds(al(j * (F // 4) + (c3 // 4) * 128, 128), 128)],
            ws3.at[4 * i + j], sem_w) for i in range(4) for j in range(4)]
        dst = X0 + 2 * RIDE * c
        return [
            pltpu.make_async_copy(w4_hbm.at[:, pl.ds(al(c3 * 32, 32), 32), :],
                                  wsr.at[pl.ds(0, 4)], sem_g),
            pltpu.make_async_copy(w1_hbm.at[:, pl.ds(al(c * 16, 16), 16), :],
                                  wsr.at[pl.ds(4, 2), pl.ds(0, 16), :], sem_g),
            pltpu.make_async_copy(w2_hbm.at[:, pl.ds(al(c * 16, 16), 16), :],
                                  wsr.at[pl.ds(4, 2), pl.ds(16, 16), :], sem_g),
            pltpu.make_async_copy(wmod_hbm.at[pl.ds(al(c * 32, 32), 32), pl.ds(5 * D, D)],
                                  wsr.at[6], sem_g),
            pltpu.make_async_copy(x_hbm.at[pl.ds(al(lo(dst, S - 2 * RIDE), 16), 2 * RIDE), :],
                                  xbuf.at[pl.ds(al(dst, 16), 2 * RIDE), :], sem_r)] + cps

    def stream_wait(c):
        for dst, sem in ((ws3.at[pl.ds(0, 16)], sem_w), (wsr.at[pl.ds(0, 7)], sem_g),
                         (xbuf.at[pl.ds(X0 + 2 * RIDE * c, 2 * RIDE), :], sem_r)):
            pltpu.make_async_copy(dst, dst, sem).wait()

    def out_copy(row, n):
        return pltpu.make_async_copy(xbuf.at[pl.ds(row, n), :], out_hbm.at[pl.ds(row, n), :],
                                     sem_out)

    def mod_rows(acc, w, r):
        sc = jnp.concatenate([scol[pl.ds(r, 16), :]] * (w.shape[1] // 128), axis=1)
        p = w.astype(f32) * sc
        return acc + p[0:8] + p[8:16]

    def mod_finish(acc, j):
        is_scale = jnp.logical_or(j // 2 == 1, j // 2 == 4)
        tot = jnp.sum(acc, axis=0, keepdims=True) + jnp.where(is_scale, 1.0, 0.0)
        modv[j] = jnp.broadcast_to(tot, (8, 512))

    def modrows(k, n, lo=0, hi=D):
        m = jnp.concatenate([modv[2 * k], modv[2 * k + 1]], axis=1)[:, lo:hi]
        return jnp.concatenate([m] * (n // 8), axis=0)

    def adaln_a(xv, anchor=None):
        n = xv.shape[0]
        return _ln(xv, anchor) * modrows(1, n) + modrows(0, n)

    def adaln_b(xv, anchor=None):
        n = xv.shape[0]
        return _ln(xv, anchor) * modrows(4, n) + modrows(3, n)

    def row_operands(v):
        top, bot = _split_rows(v)
        k = v.shape[1] // 2
        return _a_operands(top[:, :k], top[:, k:], bot[:, :k], bot[:, k:])

    def stage_a16(r, anchor=None, dst=None):
        rr = pl.multiple_of(r, 16)
        xv = xbuf[pl.ds(rr, 16), :]
        if dst is not None:
            xv = (xv.astype(f32) + modrows(2, 16) * h2buf[pl.ds(rr, 16), :]).astype(bf16)
            xbuf[pl.ds(rr, 16), :] = xv
        h2 = adaln_b(xv.astype(f32), anchor)
        h2buf[pl.ds(rr, 16), :] = h2
        ref, ro = (n7, pl.multiple_of(rr // 2, 8)) if dst is None else dst
        ops = row_operands(_ln(h2))
        for t, op in enumerate(ops):
            ref[t, pl.ds(ro, 8), :] = op.astype(bf16)
        return ops[0]

    def prologue(stg, wos, wmodb):
        def mod_copy(j):
            return pltpu.make_async_copy(wmod_hbm.at[:, pl.ds(j * 512, 512)], wmodb.at[j % NMOD],
                                         sems.at[SSTG + j + 4 if j >= 4 else SMOD + j])

        def piece_copies(g, dh):
            slot = (2 * g + dh) % NSLOT
            return [pltpu.make_async_copy(
                w_hbms[g // 4].at[pl.ds(dh * 256, 256), par, pl.ds((g % 4) * 8, 8), :],
                stg.at[slot, :, pl.ds(par * 8, 8), :],
                sems.at[SSTG + (g + 1 if g else dh)]) for par in range(2)]

        def wo_copy(j):
            return pltpu.make_async_copy(wo_hbm.at[pl.ds(j * 512, 512), :], wos.at[j % NWO],
                                         sems.at[SSTG + j + 6])

        def group_start(g):
            for dh in range(2):
                for cp in piece_copies(g, dh):
                    cp.start()

        def stg_wait(slot, n, sem):
            dst = stg.at[pl.ds(slot, n)]
            pltpu.make_async_copy(dst, dst, sems.at[SSTG + sem]).wait()

        def relayout(g, slot, dh, lo_dp, n_dp):
            base = g * (8 * WP) + dh * 256
            for u in range(n_dp):
                dp = lo_dp + u
                ev = pltpu.bitcast(stg[slot, dp, 0:8, :].astype(f32), u32)
                od = pltpu.bitcast(stg[slot, dp, 8:16, :].astype(f32), u32)
                wqkv[pl.ds(base + dp, 8, stride=WP), :] = (ev >> 16) | od

        def b_operand(g, q, k):
            def quad(i):
                r = (g * 8 + q + 4 * (i % 2)) * WP + (i // 2) * 256
                return pltpu.bitcast(wqkv[pl.ds(r, 256), :], bf16)
            i, j, sign = _BTERMS[k]
            if j is None:
                return quad(i)
            u, v = quad(i).astype(f32), quad(j).astype(f32)
            return (u + v if sign > 0 else u - v).astype(bf16)

        c_copy = pltpu.make_async_copy(c_hbm, c_ref, sem_g)
        m_copy = pltpu.make_async_copy(mem0_hbm, lhs_h.at[pl.ds(0, MEM), :], sem_r)
        c_copy.start()
        m_copy.start()
        x_copy.start()
        for j in range(4):
            mod_copy(j).start()
        for g in range(3):
            group_start(g)
        h2buf[S - NPRE:S, :] = jnp.zeros((NPRE, D), f32)
        wos[2] = jnp.zeros((512, D), bf16)
        c_copy.wait()
        m_copy.wait()
        cv = c_ref[...].astype(f32)
        sv = jnp.broadcast_to(cv * (1.0 / (1.0 + jnp.exp(-cv))), (128, D))
        for k in range(8):
            scol[k * 128:(k + 1) * 128, :] = sv[:, k * 128:(k + 1) * 128].T
        x_copy.wait()

        def ln0_body(i, _):
            r = pl.multiple_of(i * 64, 64)
            h2buf[pl.ds(r, 64), :] = _ln(xbuf[pl.ds(r, 64), :].astype(f32))
            return 0
        lax.fori_loop(0, NPRE // 64, ln0_body, 0)

        def mod0_body(j, _):
            pltpu.make_async_copy(wmodb.at[j], wmodb.at[j], sems.at[SMOD + j]).wait()
            accs = [jnp.zeros((8, 512), f32)] * 2
            for k in range(64):
                accs[k % 2] = mod_rows(accs[k % 2], wmodb[j, k * 16:(k + 1) * 16, :], k * 16)
            mod_finish(accs[0] + accs[1], j)
            return 0
        _loop("mod0", 0, 4, mod0_body)

        def hpre_body(i, _):
            r = pl.multiple_of(i * 32, 32)
            hv = h2buf[pl.ds(r, 32), :] * modrows(1, 32) + modrows(0, 32)
            ro = pl.multiple_of(i * 16, 16)
            for t, op in enumerate(row_operands(hv)):
                n7[t, pl.ds(ro, 16), :] = op.astype(bf16)
            return 0
        lax.fori_loop(0, NPRE // 32, hpre_body, 0)
        lhs_h[MEM:32, :] = adaln_a(xbuf[NPRE:NPRE + RIDE, :].astype(f32)).astype(bf16)

        def relayout_now(g, dh):
            def rl_body(t, _):
                relayout(g, 2 * g + dh, dh, t * 32, 32)
                return 0
            lax.fori_loop(0, 8, rl_body, 0)

        for dh in range(2):
            stg_wait(dh, 1, dh)
            relayout_now(0, dh)

        grp = lambda g: piece_copies(g, 0) + piece_copies(g, 1)
        issue = {0: [wo_copy(0)], 1: grp(3) + grp(4), 2: grp(5) + [wo_copy(1), mod_copy(4)],
                 3: grp(6) + [mod_copy(5), mod_copy(6)], 4: grp(7) + [wo_copy(2)],
                 5: grp(8) + [wo_copy(3), mod_copy(7)], 6: grp(9) + [wo_copy(4)],
                 7: grp(10) + [wo_copy(5), mod_copy(8)], 8: grp(11) + [wo_copy(6)],
                 9: [wo_copy(7), mod_copy(9)], 10: stream_copies(0)}

        def pre_iter(g, m3):
            m3n = jnp.where(m3 == 2, 0, m3 + 1)
            ends = jnp.logical_or(g == 0, g == NGRP - 1)
            gn = jnp.where(ends, g, g + 1)
            gslot = 2 * jnp.where(ends, m3, m3n)
            wrow = WO + jnp.maximum(g - 4, 0) * 256
            wslot = jnp.where(jnp.logical_or(g < 4, m3 == 0), 2, m3 - 1)
            cj = jnp.maximum(g - 2, 3)
            cslot = jnp.where(cj >= NMOD, cj - NMOD, cj)

            @pl.when(g == 1)
            def _():
                stg_wait(2, 2, 2)
                relayout_now(1, 0)
                relayout_now(1, 1)

            @pl.when(jnp.logical_not(ends))
            def _():
                stg_wait(gslot, 2, g + 2)

            @pl.when(g >= 4)
            def _():
                pltpu.make_async_copy(wos.at[wslot], wos.at[wslot], sems.at[SSTG + g + 2]).wait()

            @pl.when(g >= 6)
            def _():
                pltpu.make_async_copy(wmodb.at[cslot], wmodb.at[cslot],
                                      sems.at[SSTG + g + 2]).wait()

            for k, cps in issue.items():
                @pl.when(g == k)
                def _():
                    for cp in cps:
                        cp.start()
            wtodo = [(r, c) for r in range(16) for c in range(8)]
            todo = [(dh, dp) for dh in range(2) for dp in range(256)]
            mtodo = list(range(0, D, 16))
            macc = [jnp.zeros((8, 512), f32)]

            def hook(v):
                if mtodo:
                    acc = macc[0] + jnp.concatenate([_zero_after(v)] * 4, axis=1)
                    for r in mtodo[:3]:
                        acc = mod_rows(acc, wmodb[cslot, r:r + 16, :], r)
                    del mtodo[:3]
                    macc[0] = acc

            for q in range(4):
                def b_of(k):
                    w = b_operand(g, q, k)
                    nw = 0 if todo else WLP
                    for dh, dp in todo[:RLP]:
                        relayout(gn, gslot + dh, dh, dp, 1)
                    del todo[:RLP]
                    for r, c in wtodo[:nw]:
                        wqkv[pl.ds(wrow + (c * 2048 + r * 16), 16), :] = pltpu.bitcast(
                            wos[wslot, r * 32:(r + 1) * 32, c * 128:(c + 1) * 128], u32)
                    del wtodo[:nw]
                    return w
                c11, c12, c21, c22 = _strassen(lambda k: n7[k, 0:NPRE // 2, :], b_of, hook)
                for blk, y in ((q + 4, _merge_rows(c12, c22)), (q, _merge_rows(c11, c21))):
                    y = y.astype(bf16)
                    n0 = NR - ROFF
                    rings[blk][g, ROFF:NR, :] = y[0:n0]
                    rings[blk][g, 0:NPRE - n0, :] = y[n0:NPRE]
            assert not todo and not wtodo and not mtodo
            mod_finish(macc[0], cj)
            return m3n

        _loop("pre1", 0, NGRP, pre_iter)

    pl.run_scoped(prologue,
                  pltpu.VMEM((NSLOT, 256, 16, 128), bf16),
                  pltpu.VMEM((NWO, 512, D), bf16),
                  pltpu.VMEM((NMOD, D, 512), bf16))

    def main(w7, w49):
        scale = DH ** -0.5
        ia = lax.broadcasted_iota(jnp.int32, (32, L), 0)
        ja = lax.broadcasted_iota(jnp.int32, (32, L), 1)
        mask_a = (ia >= RIDE) | (ja >= SEG) | (ia + 8 >= ja)
        ib = lax.broadcasted_iota(jnp.int32, (48, 56), 0)
        jb = lax.broadcasted_iota(jnp.int32, (48, 56), 1)
        own = (ib < 40) == (jb < 40)
        mask_b = own & (((jb >= 32) & (jb < 48)) | (jnp.where(jb < 40, jb, jb - 8) <= ib))
        masked = -1e9 / scale
        j8 = lax.broadcasted_iota(jnp.int32, (8, 56), 1)
        fill_b = jnp.concatenate([jnp.where(j8 < 40, masked, -3e38).astype(f32)] * 5
                                 + [jnp.where(j8 < 40, -3e38, masked).astype(f32)], axis=0)

        def softmax(sc, mask, fill):
            sc = jnp.where(mask, sc, fill)
            mx = jnp.max(sc, axis=-1, keepdims=True)
            e = jnp.exp2((sc - mx) * (scale * 1.4426950408889634))
            den = jnp.sum(e, axis=-1, keepdims=True)
            return (e * pl.reciprocal(den, approx=True)).astype(bf16)

        def ride_rows(s, is_b):
            first = s < 2
            if is_b:
                g = [jnp.where(first, -3, -1), 1, 2]
            else:
                g = [jnp.where(first, 1, 0), jnp.where(first, 2, 1), 3]
            return [RIDE * s + 8 * t for t in g]

        def step(s, is_b, lhs_lo, lhs_hi, soft_in, jobs):
            seg = pl.multiple_of((SEG * s + ROFF) % NR, SEG)
            sega = pl.multiple_of(seg - SEG, SEG) if is_b else seg
            wr = [pl.multiple_of((NPRE + RIDE * s + 8 * t + ROFF) % NR, 8) for t in range(3)]
            rd = [pl.multiple_of((r + ROFF) % NR, 8) for r in ride_rows(s, is_b)]
            lhs = jnp.concatenate([lhs_lo, lhs_hi], axis=1)
            QM, P, PART = {}, {}, {}
            mrow = 0 if is_b else MEM
            seg8 = pl.multiple_of(seg + 8, 8)
            seg24 = pl.multiple_of(seg + RIDE, 8)

            def wblk(b, lo, n):
                return pltpu.bitcast(wqkv[b * WP + lo:b * WP + lo + n, :], bf16)

            def qkv_lo(i):
                for m in range(3):
                    PART[(m, i)] = jnp.dot(lhs_lo, wblk(m * H + i, 0, 256), preferred_element_type=f32)

            def qkv(i):
                for m in range(3):
                    b = m * H + i
                    if (m, i) in PART:
                        y = jnp.dot(lhs_hi, wblk(b, 256, 256),
                                    preferred_element_type=f32) + PART.pop((m, i))
                    else:
                        y = jnp.dot(lhs, wblk(b, 0, 512), preferred_element_type=f32)
                    if m < 2:
                        QM[b] = y[0:MEM] + jobs["pin"] if b == PIN and is_b else y[0:MEM]
                    if m == 2 or (m == 1 and not is_b):
                        kvm[b - H, mrow:mrow + MEM, :] = y[0:MEM].astype(bf16)
                    for t in range(3):
                        rset(b, wr[t], y[8 + 8 * t:16 + 8 * t])
                    for job in jobs.get(3 * i + m, []):
                        job(y)

            def keys(b):
                if is_b:
                    if b in QM:
                        old = kvm[b - H, MEM:2 * MEM, :].astype(f32)
                        mix = jnp.concatenate([QM.pop(b), old], axis=0).astype(bf16)
                    else:
                        mix = kvm[b - H]
                    return jnp.concatenate([rget(b, seg, SEG), mix, rget(b, sega, 8)], axis=0)
                mk = QM.pop(b).astype(bf16) if b in QM else kvm[b - H, MEM:2 * MEM, :]
                return jnp.concatenate([rget(b, seg, SEG), mk], axis=0)

            def scores(i):
                if is_b:
                    mix = jnp.concatenate([QM.pop(i), rget(i, sega, 8).astype(f32)], axis=0)
                    q = jnp.concatenate([rget(i, seg, SEG), mix.astype(bf16)], axis=0)
                else:
                    mix = jnp.concatenate([rget(i, seg24, 8).astype(f32), QM.pop(i)], axis=0)
                    q = jnp.concatenate([rget(i, seg8, 16), mix.astype(bf16)], axis=0)
                sc = lax.dot_general(q, keys(H + i), (((1,), (1,)), ((), ())),
                                     preferred_element_type=f32)
                P[i] = softmax(sc, mask_b, fill_b) if is_b else softmax(sc, mask_a, masked)

            def pv(i):
                o = jnp.dot(P.pop(i), keys(2 * H + i), preferred_element_type=f32)
                if is_b:
                    rset(i, seg, o[0:SEG])
                    rset(i, sega, o[40:48])
                    lhs_o[i, 0:MEM, :] = o[SEG:L].astype(bf16)
                else:
                    rset(i, seg8, o[0:16])
                    rset(i, seg24, o[16:RIDE])
                    lhs_o[i, 0:MEM, :] = o[RIDE:32].astype(bf16)
                for t in range(3):
                    lhs_o[i, 8 + 8 * t:16 + 8 * t, :] = rget(i, rd[t], 8)

            def wo_lhs(i0, i1):
                return jnp.concatenate([lhs_o[i] for i in range(i0, i1)], axis=1)

            def wo_dot(lo, j, i0, i1):
                r = WO + j * 2048
                w = pltpu.bitcast(wqkv[r + 64 * i0:r + 64 * i1, :], bf16)
                return jnp.dot(lo, w, preferred_element_type=f32)

            def side(t):
                ds, dp = (DSB, DPB) if is_b else (DSA, DPA)
                if 0 <= t - dp < H:
                    pv(t - dp)
                if 0 <= t - ds < H:
                    scores(t - ds)

            if soft_in:
                for h in range(KSPLIT):
                    qkv_lo(h)
            for h in range(H):
                qkv(h)
                side(h)
            lo = [wo_lhs(8 * k, 8 * k + 8) for k in range(3)]
            acc = []
            for j in range(8):
                y = None
                for k in range(3):
                    z = wo_dot(lo[k], j, 8 * k, 8 * k + 8)
                    y = z if y is None else z + y
                    for job in jobs.get(96 + 3 * j + k, []):
                        job(y)
                acc.append(y)
                side(H + j)
            lo = wo_lhs(24, H)
            for j in range(8):
                acc[j] = wo_dot(lo, j, 24, H) + acc[j]
                for job in jobs.get(120 + j, []):
                    job(acc[j])
            assert not (QM or P or PART)
            return jnp.concatenate(acc[0:4], axis=1), jnp.concatenate(acc[4:8], axis=1)

        def combine(c, n, y):
            mp, k1 = divmod(n, 8)
            m, p = divmod(mp, 4)
            c3 = jnp.minimum(c, 27)
            spare = pl.ds(pl.multiple_of(8 * (c // 64), 8), 8)
            if m == 0 and k1 < 7:
                ws3[16, spare, :] = y.astype(bf16)
            else:
                wsr[7, spare, 0:128] = y.astype(bf16)
            if k1 == 7:
                dst, base, r = w7, 0, (4 * m + p) * 256 + c * 8
                blk = [wsr[4 + i, m * 16:(m + 1) * 16, j * 512 + p * 128:j * 512 + (p + 1) * 128]
                       .astype(f32) for i in range(2) for j in range(2)]
            else:
                dst, base = w49, 7 * k1
                if m == 0:
                    r = c3 * 32 + p * 8
                    get = lambda i, j: ws3[4 * i + j, p * 16:(p + 1) * 16, :]
                else:
                    r = W4R + (p // 2) * 448 + c3 * 16 + (p % 2) * 8
                    r0, c0 = (p % 2) * 16, (p // 2) * 128
                    get = lambda i, j: wsr[i, r0:r0 + 16, j * 256 + c0:j * 256 + c0 + 128]

                def quad(q):
                    return [get(2 * (q // 2) + i, 2 * (q % 2) + j).astype(f32)
                            for i in range(2) for j in range(2)]
                qi, qj, sign = _BTERMS[k1]
                blk = quad(qi)
                if qj is not None:
                    blk = [u + v if sign > 0 else u - v for u, v in zip(blk, quad(qj))]
            for k, op in enumerate(_b_operands(*blk)):
                dst[base + k, pl.ds(pl.multiple_of(r, 8), 8), :] = pltpu.bitcast(
                    op.astype(bf16), u32)

        def rec_body(it, gacc):
            stream_wait(it)
            lhs_lo = lhs_h[:, 0:512]
            lhs_hi = lhs_h[:, 512:1024]
            ra = jnp.maximum(it - 1, 0) * (2 * RIDE)
            for u in range(2):
                s = 2 * it + u
                jobs = {}
                for n, (su, d, g) in enumerate(SLOTS):
                    if su == u:
                        jobs.setdefault(d, []).append(
                            lambda y, n=n, g=g: combine(it, n, y[8 * g:8 * g + 8]))
                r1 = pl.multiple_of(jnp.minimum(NPRE + RIDE * (s + 1), S - RIDE), 8)
                xn = xbuf[pl.ds(r1, RIDE), :].astype(f32)
                if u == 0:
                    for k in range(2):
                        rm = pl.multiple_of(it * 32 + k * 16, 16)
                        gacc = mod_rows(gacc, wsr[6, k * 16:(k + 1) * 16, :], rm)
                    hn = adaln_a(xn, _zero_after(stage_a16(ra)))
                else:
                    def refill(y):
                        for cp in stream_copies(jnp.minimum(it + 1, NSEG // 2 - 1)):
                            cp.start()
                        spare = pl.ds(pl.multiple_of(8 * (it // 64), 8), 8)
                        jobs["pin"] = _zero_after(ws3[16, spare, :].astype(f32))
                    jobs.setdefault(3 * (PIN - 4) + 2, []).append(refill)
                    hn = adaln_a(xn)
                    z = _zero_after(hn[0:8], hn[8:16], hn[16:24])
                    stage_a16(ra + 32, _zero_after(stage_a16(ra + 16, z)))
                a_lo, a_hi = step(s, u == 1, lhs_lo, lhs_hi, u > 0, jobs)
                lhs_lo = jnp.concatenate([a_lo[0:MEM], hn[:, 0:512]], axis=0).astype(bf16)
                lhs_hi = jnp.concatenate([a_hi[0:MEM], hn[:, 512:1024]], axis=0).astype(bf16)
                a = jnp.concatenate([a_lo, a_hi], axis=1)
                rows = [pl.multiple_of(r, 8) for r in ride_rows(s, u == 1)]
                xs = [xbuf[pl.ds(r, 8), :].astype(f32) for r in rows]
                for t, r in enumerate(rows):
                    xa = xs[t] + modrows(2, 8) * a[8 + 8 * t:16 + 8 * t]
                    xbuf[pl.ds(r, 8), :] = xa.astype(bf16)
            lhs_h[:, 0:512] = lhs_lo
            lhs_h[:, 512:1024] = lhs_hi
            return gacc

        gacc = _loop("rec", 0, NSEG // 2, rec_body, jnp.zeros((8, D), f32))
        for c in range(2):
            mod_finish(gacc[:, c * 512:(c + 1) * 512], 10 + c)
        stream_wait(NSEG // 2 - 1)

        def wo_prep(i, half, k):
            o = jnp.concatenate([rings[4 * half + h][i, k * 16:(k + 1) * 16, :].astype(f32)
                                 for h in range(4)], axis=1)
            for t, op in enumerate(row_operands(o)):
                a7[half, t, k * 8:(k + 1) * 8, :] = op.astype(bf16)

        def wo_chunk(i, half, inext, extra):
            row = pl.multiple_of(i * 512 + half * 256, 256)
            todo = list(range(NPRE // 16))
            spare = pl.ds(pl.multiple_of(8 * (i // 64), 8), 8)

            def hook(v):
                if todo:
                    for h in range(4):
                        rings[4 * (1 - half) + h][4, spare, :] = v[0:8].astype(bf16)
                    n = 2 if len(todo) % WPP == 0 else 1
                    for k in todo[:n]:
                        wo_prep(inext, 1 - half, k)
                    del todo[:n]
                extra(v)

            for j in range(4):
                def b_of(k):
                    def quad(q):
                        r = WO + (j + 4 * (q % 2)) * 2048 + (q // 2) * 128 + row
                        return pltpu.bitcast(wqkv[pl.ds(r, 128), :], bf16)
                    qi, qj, sign = _BTERMS[k]
                    if qj is None:
                        return quad(qi)
                    u, v = quad(qi).astype(f32), quad(qj).astype(f32)
                    return (u + v if sign > 0 else u - v).astype(bf16)
                c11, c12, c21, c22 = _strassen(lambda k: a7[half, k], b_of, hook)
                for c, y in ((j + 4, _merge_rows(c12, c22)), (j, _merge_rows(c11, c21))):
                    cs = slice(c * 128, (c + 1) * 128)
                    h2buf[S - NPRE:S, cs] = h2buf[S - NPRE:S, cs] + y

        for k in range(NPRE // 16):
            wo_prep(0, 0, k)

        def wo_tail(i, _):
            st = {"n": 0, "prev": None}

            def extra(v):
                n = st["n"]
                st["n"] += 1
                if n % 16 == 2 and n // 16 < 3:
                    st["prev"] = stage_a16(S - NPRE - 48 + 16 * (n // 16),
                                           _zero_after(v, st["prev"]))
            wo_chunk(i, 0, i, extra)
            wo_chunk(i, 1, jnp.minimum(i + 1, 3), extra)
            return 0
        _loop("wotail", 0, 4, wo_tail)

        def gget(c, row, n):
            return pltpu.bitcast(wqkv[pl.ds(c * GS + row, n), :], f32)

        def gset(c, row, val):
            wqkv[pl.ds(c * GS + row, val.shape[0]), :] = pltpu.bitcast(val, u32)

        def wop(j):
            return lambda k: pltpu.bitcast(w7[k, j * 256:(j + 1) * 256, :], bf16)

        zpad = jnp.zeros((GPAD, 128), f32)
        for cb in range(8):
            gset(cb, 0, zpad)
            gset(cb, GPAD + S, zpad)

        shifts = (-1, -1, 1, 1, -2, -2, 2, 2)
        HB = MB // 2

        def shift_piece(r, half, k):
            gs = jnp.concatenate([gget(c, r + (k * 16 + GPAD + shifts[c]), 16)
                                  for c in range(8)], axis=1)
            ro = half * (HB // 2) + k * 8
            for t, op in enumerate(row_operands(gs)):
                n7[t, ro:ro + 8, :] = op.astype(bf16)

        def gate(v, i):
            gset(0, GPAD + S + GPAD + 8 * (i // S), v[0:8])

        def b_body(i, _):
            rl = S - NPRE + i * 128
            st = {"n": 0, "prev": [None, None]}

            def hook(v):
                n = st["n"]
                st["n"] += 1
                if n % BG == 0 and n // BG < 8:
                    k = n // BG
                    st["prev"][k % BCH] = stage_a16(rl + 16 * k,
                                                    _zero_after(v, st["prev"][k % BCH]),
                                                    (t7, 8 * k))

            ro = pl.multiple_of(i * 192, 64)
            for lhs, row in ((lambda k: n7[k, pl.ds(ro, 192), :], i * 384), (lambda k: t7[k], rl)):
                rg = pl.multiple_of(GPAD + row, 8)
                for j in range(4):
                    c11, c12, c21, c22 = _strassen(lhs, wop(j), hook)
                    gset(j + 4, rg, _gelu(_merge_rows(c12, c22)))
                    gset(j, rg, _gelu(_merge_rows(c11, c21)))
            return 0
        _loop("b", 0, S // MB, b_body)
        for k in range(HB // 16):
            shift_piece(0, 0, k)

        def n2_norm(r, k, anchor):
            v = _ln(h2buf[pl.ds(pl.multiple_of(r + k * 16, 16), 16), :], anchor)
            nrms[k // 2][(k % 2) * 16:(k % 2) * 16 + 16, :] = v
            return v[0:8] + v[8:16]

        def n2_ops(k, k1, v, i):
            nrm = nrms[k]
            nrm[pl.ds(pl.multiple_of(32 + 8 * (i // S), 8), 8), 0:128] = v[0:8]

            def quad(q):
                r0, c0 = (q // 2) * 16, (q % 2) * 512
                return [nrm[r0 + 8 * a:r0 + 8 * a + 8, c0 + 256 * b:c0 + 256 * b + 256]
                        for a in range(2) for b in range(2)]
            qi, qj, sign = _ATERMS[k1]
            blk = quad(qi)
            if qj is not None:
                blk = [u + w if sign > 0 else u - w for u, w in zip(blk, quad(qj))]
            for k2, op in enumerate(_a_operands(*blk)):
                d49[7 * k1 + k2, k * 8:(k + 1) * 8, :] = op.astype(bf16)

        def n2_hook(r, i, first, gap, lag, st):
            def hook(v):
                n = st["n"] - first
                st["n"] += 1
                if n >= 0 and n % gap == 0 and n // gap < MD // 16:
                    st["prev"] = n2_norm(r, n // gap, _zero_after(v, st["prev"]))
                for _ in range(st["per"]):
                    k, k1 = divmod(st["ops"], 7)
                    if k < MD // 32 and n >= (2 * k + 1) * gap + lag:
                        n2_ops(k, k1, v, i)
                        st["ops"] += 1
            return hook

        def stage_c(i, r, half, rnext, extra):
            rr = pl.multiple_of(r, 8)
            ro = half * (HB // 2)
            cnt = [0]

            def hook(v):
                n = cnt[0]
                cnt[0] += 1
                if n < HB // 16:
                    gate(v, i)
                    shift_piece(rnext, 1 - half, n)
                extra(v)

            for j in range(4):
                c11, c12, c21, c22 = _strassen(lambda k: n7[k, ro:ro + HB // 2, :], wop(4 + j),
                                               hook)
                for c, y in ((j + 4, _merge_rows(c12, c22)), (j, _merge_rows(c11, c21))):
                    cs = slice(c * 128, (c + 1) * 128)
                    h2buf[pl.ds(rr, HB), cs] = h2buf[pl.ds(rr, HB), cs] + y

        def c_body(i, _):
            r = pl.multiple_of(i * MB, MB)
            st = {"n": 0, "prev": None, "ops": 0, "per": 1}
            extra = n2_hook(0, i, 0, 4, 4, st)
            stage_c(i, r, 0, r + HB, extra)
            stage_c(i, r + HB, 1, jnp.minimum(i + 1, S // MB - 1) * MB, extra)
            assert st["ops"] == 28
            return 0
        _loop("c", 0, S // MB, c_body)

        def wop2(lo, n):
            return lambda k1, k: pltpu.bitcast(w49[7 * k1 + k, lo:lo + n, :], bf16)

        def d_body(i, _):
            r = pl.multiple_of(i * MD, MD)
            rn = jnp.minimum(r + MD, S - MD)
            lhs = [d49[k] for k in range(49)]
            uops = []
            for t in range(7):
                cb = _strassen2(lambda k1, k: lhs[7 * k1 + k], wop2(t * 128, 128))
                uops.append(_a_operands2([[_gelu(c) for c in row] for row in cb]))
            ul = [[jnp.concatenate([u[k1][k] for u in uops], axis=1).astype(bf16)
                   for k in range(7)] for k1 in range(7)]
            st = {"n": 0, "prev": None, "ops": 0, "per": 1}
            hook = n2_hook(rn, i, DF, DG, DL, st)
            for t in range(2):
                cb = _strassen2(lambda k1, k: ul[k1][k], wop2(W4R + t * 448, 448), hook)
                for j in range(4):
                    y = jnp.concatenate([cb[q][j].reshape(MD // 32, 8, 128) for q in range(4)],
                                        axis=1).reshape(MD, 128)
                    c = 2 * j + t
                    cs = slice(c * 128, (c + 1) * 128)
                    gb = modrows(5, MD, c * 128, (c + 1) * 128)
                    o = xbuf[pl.ds(r, MD), cs].astype(f32) + gb * (h2buf[pl.ds(r, MD), cs] + y)
                    xbuf[pl.ds(r, MD), cs] = o.astype(bf16)
            assert st["ops"] == 28
            out_copy(r, MD).start()
            return 0
        _loop("d", 0, S // MD, d_body)

    pl.run_scoped(main,
                  pltpu.VMEM((7, 8 * 256, 128), u32),
                  pltpu.VMEM((49, 2 * W4R, 128), u32))

    out_copy(0, S).wait()


def _run(x, mem0, wq, wk, wv, wo, w1, w2, w3, w4, c, wmod):
    any_spec = pl.BlockSpec(memory_space=pl.ANY)
    return pl.pallas_call(
        _kernel,
        out_shape=jax.ShapeDtypeStruct((S, D), bf16),
        in_specs=[any_spec] * 12,
        out_specs=any_spec,
        scratch_shapes=[
            pltpu.VMEM((S + 2 * RIDE, D), bf16),
            pltpu.VMEM((WO + 8 * 2048, 128), u32),
            [pltpu.VMEM((96 // NRING, NR, 128), bf16)] * NRING,
            pltpu.VMEM((32, D), bf16),
            pltpu.VMEM((H, 32, 128), bf16),
            pltpu.VMEM((2 * H, 16, 128), bf16),
            pltpu.VMEM((12, 8, 512), f32),
            pltpu.VMEM((D, 128), f32),
            pltpu.VMEM((S, D), f32),
            pltpu.VMEM((7, (S - NPRE) // 2, 512), bf16),
            pltpu.VMEM((17, 64, 128), bf16),
            pltpu.VMEM((8, 32, D), bf16),
            pltpu.VMEM((7, 64, 512), bf16),
            pltpu.VMEM((2, 7, NPRE // 2, 256), bf16),
            pltpu.VMEM((49, MD // 4, 256), bf16),
            [pltpu.VMEM((40, D), f32)] * (MD // 32),
            pltpu.VMEM((1, D), bf16),
            pltpu.SemaphoreType.DMA((9 + NGRP + 2,)),
        ],
        compiler_params=pltpu.CompilerParams(vmem_limit_bytes=124 * 1024 * 1024,
                                             disable_bounds_checks=True),
    )(x, mem0, wq, wk, wv, wo, w1, w2, w3, w4, c, wmod)


def pallas_adaLN_cond__memory_aug_recurrent_mem_tr__mixer_s_mlp__prompt_kernel(
    A_x, A_mem0, A_Wq, A_Wk, A_Wv, A_Wo, A_seg_len, B_x, B_w1, B_w2, B_w3, B_w4, c, w_mod,
):
    del B_x
    assert A_x.shape == (1, S, D) and A_mem0.shape == (1, MEM, D)
    assert isinstance(A_seg_len, int) is False or A_seg_len == SEG
    pairs = (D // 2, 2, H, DH)
    out = _run(A_x.reshape(S, D), A_mem0.reshape(MEM, D), A_Wq.reshape(pairs),
               A_Wk.reshape(pairs), A_Wv.reshape(pairs), A_Wo.reshape(H * DH, D),
               B_w1.reshape(2, D // 2, D), B_w2.reshape(2, D // 2, D),
               B_w3, B_w4.reshape(4, F // 4, D), c, w_mod)
    return out.reshape(1, S, D)
```

```python
import jax
import jax.numpy as jnp
from jax import lax
import jax.experimental.pallas as pl
import jax.experimental.pallas.tpu as pltpu

bf16 = jnp.bfloat16
f32 = jnp.float32
u32 = jnp.uint32

S = 2048
D = 1024
H = 32
DH = 128
F = 3584
MEM = 8
SEG = 32
NSEG = S // SEG
L = MEM + SEG
RIDE = 24
NPRE = S - RIDE * NSEG
NR = NPRE + 2 * SEG
ROFF = (-(S - NPRE)) % NR
WP = 516
WO = 96 * WP
NGRP = 12
NSLOT = 6
NMOD = 6
EPS = 1e-5
MD = 128
MB = 512
GPAD = 8
NRING = 8
RLP, WLP, RSK = 27, 22, 2
NWO = 3
BG, WPP, PIN, BCH = 2, 5, 6, 2
DF, DG, DL = 2, 10, 9
SLOTS = ([(0, n // 2, 3 * (n % 2)) for n in range(16)] + [(0, 96 + n, 0) for n in range(16)]
         + [(0, 112 + n // 2, 3 * (n % 2)) for n in range(32)])
DSA, DPA, DSB, DPB, KSPLIT = 2, 4, 2, 4, 2
X0 = NPRE + 2 * RIDE
GS = S + 4 * GPAD
W4R = 7 * 128
_ONLY = None


def _loop(name, lo, hi, body, init=0):
    if _ONLY is not None and name not in _ONLY:
        return init
    with _scope(name):
        return lax.fori_loop(lo, hi, body, init)


class _NoScope:
    def __init__(self, name):
        del name

    def __enter__(self):
        return self

    def __exit__(self, *a):
        return False


_scope = _NoScope


def _zero_after(*vs):
    bits = None
    for v in vs:
        if v is not None:
            b = pltpu.bitcast(v[0:8, 0:128], u32)
            bits = b if bits is None else bits | b
    return pltpu.bitcast((bits >> 31) >> 1, f32)


def _ln(x, anchor=None):
    if anchor is not None:
        z = jnp.concatenate([anchor] * (x.shape[0] // 8), axis=0)
        x = jnp.concatenate([x[:, 0:128] + z, x[:, 128:]], axis=1)
    mu = jnp.mean(x, axis=-1, keepdims=True)
    xc = x - mu
    var = jnp.mean(xc * xc, axis=-1, keepdims=True)
    return xc * lax.rsqrt(var + EPS)


def _gelu(x):
    inner = x * (0.7978845608028654 + (0.7978845608028654 * 0.044715) * (x * x))
    hx = 0.5 * x
    return hx + hx * jnp.tanh(inner)


def _split_rows(x):
    m, n = x.shape
    x3 = x.reshape(m // 16, 16, n)
    return x3[:, 0:8, :].reshape(m // 2, n), x3[:, 8:16, :].reshape(m // 2, n)


def _merge_rows(top, bot):
    m, n = top.shape
    return jnp.concatenate([top.reshape(m // 8, 8, n), bot.reshape(m // 8, 8, n)],
                           axis=1).reshape(2 * m, n)


def _a_operands(a11, a12, a21, a22):
    return [a11 + a22, a21 + a22, a11, a22, a11 + a12, a21 - a11, a12 - a22]


def _b_operands(b11, b12, b21, b22):
    return [b11 + b22, b11, b12 - b22, b21 - b11, b22, b11 + b12, b21 + b22]


_ATERMS = ((0, 3, 1), (2, 3, 1), (0, None, 0), (3, None, 0), (0, 1, 1), (2, 0, -1), (1, 3, -1))
_BTERMS = ((0, 3, 1), (0, None, 0), (1, 3, -1), (2, 0, -1), (3, None, 0), (0, 1, 1), (2, 3, 1))


def _strassen(a_of, b_of, hook=lambda v: None):
    def prod(k):
        return jnp.dot(a_of(k), b_of(k), preferred_element_type=f32)
    p5 = prod(4)
    hook(p5)
    p3 = prod(2)
    hook(p3)
    c12 = p3 + p5
    p4 = prod(3)
    hook(p4)
    c11 = p4 - p5
    p2 = prod(1)
    hook(p2)
    c21 = p2 + p4
    c22 = p3 - p2
    p1 = prod(0)
    hook(p1)
    c11 = prod(6) + (c11 + p1)
    hook(c11)
    c22 = prod(5) + (c22 + p1)
    hook(c22)
    return c11, c12, c21, c22


def _a_operands2(b):
    sub = [_a_operands(b[i][j], b[i][2 + j], b[2 + i][j], b[2 + i][2 + j])
           for i in range(2) for j in range(2)]
    return [_a_operands(*[t[k] for t in sub]) for k in range(7)]


def _strassen2(a_of, b_of, hook=lambda v: None):
    def prod(k1):
        return _strassen(lambda k: a_of(k1, k), lambda k: b_of(k1, k), hook)

    def add(x, y):
        return [p + q for p, q in zip(x, y)]

    def sub(x, y):
        return [p - q for p, q in zip(x, y)]
    p5 = prod(4)
    p3 = prod(2)
    c12 = add(p3, p5)
    p4 = prod(3)
    c11 = sub(p4, p5)
    p2 = prod(1)
    c21 = add(p2, p4)
    c22 = sub(p3, p2)
    p1 = prod(0)
    c11 = add(add(c11, p1), prod(6))
    c22 = add(add(c22, p1), prod(5))
    cq = (c11, c12, c21, c22)
    return [[cq[2 * (i // 2) + j // 2][2 * (i % 2) + j % 2] for j in range(4)] for i in range(4)]


def _kernel(x_hbm, mem0_hbm, wq_hbm, wk_hbm, wv_hbm, wo_hbm, w1_hbm, w2_hbm, w3_hbm, w4_hbm,
            c_hbm, wmod_hbm, out_hbm,
            xbuf, wqkv, rings, lhs_h, lhs_o, kvm, modv, scol, h2buf, n7, ws3, wsr, t7, a7, d49, nrms, c_ref,
            sems):
    w_hbms = (wq_hbm, wk_hbm, wv_hbm)
    SMOD, SSTG = 5, 9
    sem_x, sem_out, sem_w, sem_g, sem_r = (sems.at[k] for k in range(5))

    def rget(b, row, n):
        return rings[b % NRING][b // NRING, pl.ds(row, n), :]

    def rset(b, row, val):
        rings[b % NRING][b // NRING, pl.ds(row, val.shape[0]), :] = val.astype(bf16)

    x_copy = pltpu.make_async_copy(x_hbm.at[pl.ds(0, X0), :], xbuf.at[pl.ds(0, X0), :], sem_x)

    def stream_copies(c):
        al, lo = ((lambda v, m: v), min) if isinstance(c, int) else (pl.multiple_of, jnp.minimum)
        c3 = lo(c, 27)
        cps = [pltpu.make_async_copy(
            w3_hbm.at[pl.ds(al(i * 256 + (c3 % 4) * 64, 64), 64),
                      pl.ds(al(j * (F // 4) + (c3 // 4) * 128, 128), 128)],
            ws3.at[4 * i + j], sem_w) for i in range(4) for j in range(4)]
        dst = X0 + 2 * RIDE * c
        return [
            pltpu.make_async_copy(w4_hbm.at[:, pl.ds(al(c3 * 32, 32), 32), :],
                                  wsr.at[pl.ds(0, 4)], sem_g),
            pltpu.make_async_copy(w1_hbm.at[:, pl.ds(al(c * 16, 16), 16), :],
                                  wsr.at[pl.ds(4, 2), pl.ds(0, 16), :], sem_g),
            pltpu.make_async_copy(w2_hbm.at[:, pl.ds(al(c * 16, 16), 16), :],
                                  wsr.at[pl.ds(4, 2), pl.ds(16, 16), :], sem_g),
            pltpu.make_async_copy(wmod_hbm.at[pl.ds(al(c * 32, 32), 32), pl.ds(5 * D, D)],
                                  wsr.at[6], sem_g),
            pltpu.make_async_copy(x_hbm.at[pl.ds(al(lo(dst, S - 2 * RIDE), 16), 2 * RIDE), :],
                                  xbuf.at[pl.ds(al(dst, 16), 2 * RIDE), :], sem_r)] + cps

    def stream_wait(c):
        for dst, sem in ((ws3.at[pl.ds(0, 16)], sem_w), (wsr.at[pl.ds(0, 7)], sem_g),
                         (xbuf.at[pl.ds(X0 + 2 * RIDE * c, 2 * RIDE), :], sem_r)):
            pltpu.make_async_copy(dst, dst, sem).wait()

    def out_copy(row, n):
        return pltpu.make_async_copy(xbuf.at[pl.ds(row, n), :], out_hbm.at[pl.ds(row, n), :],
                                     sem_out)

    def mod_rows(acc, w, r):
        sc = jnp.concatenate([scol[pl.ds(r, 16), :]] * (w.shape[1] // 128), axis=1)
        p = w.astype(f32) * sc
        return acc + p[0:8] + p[8:16]

    def mod_finish(acc, j):
        is_scale = jnp.logical_or(j // 2 == 1, j // 2 == 4)
        tot = jnp.sum(acc, axis=0, keepdims=True) + jnp.where(is_scale, 1.0, 0.0)
        modv[j] = jnp.broadcast_to(tot, (8, 512))

    def modrows(k, n, lo=0, hi=D):
        m = jnp.concatenate([modv[2 * k], modv[2 * k + 1]], axis=1)[:, lo:hi]
        return jnp.concatenate([m] * (n // 8), axis=0)

    def adaln_a(xv, anchor=None):
        n = xv.shape[0]
        return _ln(xv, anchor) * modrows(1, n) + modrows(0, n)

    def adaln_b(xv, anchor=None):
        n = xv.shape[0]
        return _ln(xv, anchor) * modrows(4, n) + modrows(3, n)

    def row_operands(v):
        top, bot = _split_rows(v)
        k = v.shape[1] // 2
        return _a_operands(top[:, :k], top[:, k:], bot[:, :k], bot[:, k:])

    def stage_a16(r, anchor=None, dst=None):
        rr = pl.multiple_of(r, 16)
        xv = xbuf[pl.ds(rr, 16), :]
        if dst is not None:
            xv = (xv.astype(f32) + modrows(2, 16) * h2buf[pl.ds(rr, 16), :]).astype(bf16)
            xbuf[pl.ds(rr, 16), :] = xv
        h2 = adaln_b(xv.astype(f32), anchor)
        h2buf[pl.ds(rr, 16), :] = h2
        ref, ro = (n7, pl.multiple_of(rr // 2, 8)) if dst is None else dst
        ops = row_operands(_ln(h2))
        for t, op in enumerate(ops):
            ref[t, pl.ds(ro, 8), :] = op.astype(bf16)
        return ops[0]

    def prologue(stg, wos, wmodb, h7):
        def mod_copy(j):
            return pltpu.make_async_copy(wmod_hbm.at[:, pl.ds(j * 512, 512)], wmodb.at[j % NMOD],
                                         sems.at[SSTG + j + 4 if j >= 4 else SMOD + j])

        def piece_copy(g, dh):
            return pltpu.make_async_copy(
                w_hbms[g // 4].at[pl.ds(dh * 512, 512), pl.ds((g % 4) * 8, 8), :],
                stg.at[(2 * g + dh) % NSLOT], sems.at[SSTG + (g + 1 if g else dh)])

        def wo_copy(j):
            return pltpu.make_async_copy(wo_hbm.at[pl.ds(j * 512, 512), :], wos.at[j % NWO],
                                         sems.at[SSTG + j + 6])

        def group_start(g):
            for dh in range(2):
                piece_copy(g, dh).start()

        def stg_wait(slot, n, sem):
            dst = stg.at[pl.ds(slot, n)]
            pltpu.make_async_copy(dst, dst, sems.at[SSTG + sem]).wait()

        def relayout(g, slot, dh, lo_dp, n_dp):
            base = g * (8 * WP) + dh * 256
            for u in range(n_dp):
                dp = lo_dp + u
                ev = pltpu.bitcast(stg[slot, 2 * dp].astype(f32), u32)
                od = pltpu.bitcast(stg[slot, 2 * dp + 1].astype(f32), u32)
                wqkv[pl.ds(base + dp, 8, stride=WP), :] = (ev >> 16) | od

        def b_operand(gbase, q, k):
            def quad(i):
                r = gbase + ((q + 4 * (i % 2)) * WP + (i // 2) * 256)
                return pltpu.bitcast(wqkv[pl.ds(r, 256), :], bf16)
            i, j, sign = _BTERMS[k]
            if j is None:
                return quad(i)
            u, v = quad(i).astype(f32), quad(j).astype(f32)
            return (u + v if sign > 0 else u - v).astype(bf16)

        c_copy = pltpu.make_async_copy(c_hbm, c_ref, sem_g)
        m_copy = pltpu.make_async_copy(mem0_hbm, lhs_h.at[pl.ds(0, MEM), :], sem_r)
        c_copy.start()
        m_copy.start()
        x_copy.start()
        for j in range(4):
            mod_copy(j).start()
        for g in range(3):
            group_start(g)
        h2buf[S - NPRE:S, :] = jnp.zeros((NPRE, D), f32)
        wos[2] = jnp.zeros((512, D), bf16)
        c_copy.wait()
        m_copy.wait()
        cv = c_ref[...].astype(f32)
        sv = jnp.broadcast_to(cv * (1.0 / (1.0 + jnp.exp(-cv))), (128, D))
        for k in range(8):
            scol[k * 128:(k + 1) * 128, :] = sv[:, k * 128:(k + 1) * 128].T
        x_copy.wait()

        def ln0_body(i, _):
            r = pl.multiple_of(i * 64, 64)
            h2buf[pl.ds(r, 64), :] = _ln(xbuf[pl.ds(r, 64), :].astype(f32))
            return 0
        lax.fori_loop(0, NPRE // 64, ln0_body, 0)

        def mod0_body(j, _):
            pltpu.make_async_copy(wmodb.at[j], wmodb.at[j], sems.at[SMOD + j]).wait()
            accs = [jnp.zeros((8, 512), f32)] * 2
            for k in range(64):
                accs[k % 2] = mod_rows(accs[k % 2], wmodb[j, k * 16:(k + 1) * 16, :], k * 16)
            mod_finish(accs[0] + accs[1], j)
            return 0
        _loop("mod0", 0, 4, mod0_body)

        def hpre_body(i, _):
            r = pl.multiple_of(i * 32, 32)
            hv = h2buf[pl.ds(r, 32), :] * modrows(1, 32) + modrows(0, 32)
            ro = pl.multiple_of(i * 8, 8)
            for t, op in enumerate(row_operands(hv)):
                h7[t, pl.ds(ro, 8), :] = pltpu.bitcast(op.astype(bf16), u32)
            return 0
        lax.fori_loop(0, NPRE // 32, hpre_body, 0)
        lhs_h[MEM:32, :] = adaln_a(xbuf[NPRE:NPRE + RIDE, :].astype(f32)).astype(bf16)

        def relayout_now(g, dh):
            def rl_body(t, _):
                relayout(g, 2 * g + dh, dh, t * 32, 32)
                return 0
            lax.fori_loop(0, 8, rl_body, 0)

        for dh in range(2):
            stg_wait(dh, 1, dh)
            relayout_now(0, dh)

        grp = lambda g: [piece_copy(g, 0), piece_copy(g, 1)]
        issue = {0: [wo_copy(0)], 1: grp(3) + grp(4), 2: grp(5) + [wo_copy(1), mod_copy(4)],
                 3: grp(6) + [mod_copy(5), mod_copy(6)], 4: grp(7) + [wo_copy(2)],
                 5: grp(8) + [wo_copy(3), mod_copy(7)], 6: grp(9) + [wo_copy(4)],
                 7: grp(10) + [wo_copy(5), mod_copy(8)], 8: grp(11) + [wo_copy(6)],
                 9: [wo_copy(7), mod_copy(9)], 10: stream_copies(0)}

        def pre_iter(g, carry):
            m3, gbase = carry

            @pl.when(g == 1)
            def _():
                stg_wait(2, 2, 2)
                relayout_now(1, 0)
                relayout_now(1, 1)

            def slots():
                m3n = jnp.where(m3 == 2, 0, m3 + 1)
                cj = jnp.maximum(g - 2, 3)
                return (m3n, 2 * jnp.where(ends, m3, m3n),
                        jnp.where(jnp.logical_or(g < 4, m3 == 0), 2, m3 - 1),
                        cj, jnp.where(cj >= NMOD, cj - NMOD, cj))

            ends = jnp.logical_or(g == 0, g == NGRP - 1)

            @pl.when(jnp.logical_not(ends))
            def _():
                stg_wait(slots()[1], 2, g + 2)

            @pl.when(g >= 4)
            def _():
                buf = wos.at[slots()[2]]
                pltpu.make_async_copy(buf, buf, sems.at[SSTG + g + 2]).wait()

            @pl.when(g >= 6)
            def _():
                buf = wmodb.at[slots()[4]]
                pltpu.make_async_copy(buf, buf, sems.at[SSTG + g + 2]).wait()

            m3n, gslot, wslot, cj, cslot = slots()
            gn = jnp.where(ends, g, g + 1)
            wrow = WO + jnp.maximum(g - 4, 0) * 256
            for k, cps in issue.items():
                @pl.when(g == k)
                def _():
                    for cp in cps:
                        cp.start()
            wtodo = [(r, c) for r in range(16) for c in range(8)]
            todo = [(dh, dp) for dh in range(2) for dp in range(256)]
            skip = [0] * RSK
            mtodo = list(range(0, D, 16))
            macc = [jnp.zeros((8, 512), f32)]

            def hook(v):
                if mtodo:
                    acc = macc[0] + jnp.concatenate([_zero_after(v)] * 4, axis=1)
                    for r in mtodo[:3]:
                        acc = mod_rows(acc, wmodb[cslot, r:r + 16, :], r)
                    del mtodo[:3]
                    macc[0] = acc

            for q in range(4):
                def b_of(k):
                    w = b_operand(gbase, q, k)
                    if skip:
                        skip.pop()
                        return w
                    nw = 0 if todo else WLP
                    for dh, dp in todo[:RLP]:
                        relayout(gn, gslot + dh, dh, dp, 1)
                    del todo[:RLP]
                    for r, c in wtodo[:nw]:
                        wqkv[pl.ds(wrow + (c * 2048 + r * 16), 16), :] = pltpu.bitcast(
                            wos[wslot, r * 32:(r + 1) * 32, c * 128:(c + 1) * 128], u32)
                    del wtodo[:nw]
                    return w
                c11, c12, c21, c22 = _strassen(lambda k: pltpu.bitcast(h7[k], bf16), b_of, hook)
                for blk, y in ((q + 4, _merge_rows(c12, c22)), (q, _merge_rows(c11, c21))):
                    y = y.astype(bf16)
                    n0 = NR - ROFF
                    rings[blk][g, ROFF:NR, :] = y[0:n0]
                    rings[blk][g, 0:NPRE - n0, :] = y[n0:NPRE]
            assert not todo and not wtodo and not mtodo
            mod_finish(macc[0], cj)
            return m3n, gbase + 8 * WP

        _loop("pre1", 0, NGRP, pre_iter, (0, 0))

    pl.run_scoped(prologue,
                  pltpu.VMEM((NSLOT, 512, 8, 128), bf16),
                  pltpu.VMEM((NWO, 512, D), bf16),
                  pltpu.VMEM((NMOD, D, 512), bf16),
                  pltpu.VMEM((7, NPRE // 4, 512), u32))

    def main(w7, w49):
        scale = DH ** -0.5
        ia = lax.broadcasted_iota(jnp.int32, (32, L), 0)
        ja = lax.broadcasted_iota(jnp.int32, (32, L), 1)
        mask_a = (ia >= RIDE) | (ja >= SEG) | (ia + 8 >= ja)
        ib = lax.broadcasted_iota(jnp.int32, (48, 56), 0)
        jb = lax.broadcasted_iota(jnp.int32, (48, 56), 1)
        own = (ib < 40) == (jb < 40)
        mask_b = own & (((jb >= 32) & (jb < 48)) | (jnp.where(jb < 40, jb, jb - 8) <= ib))
        masked = -1e9 / scale
        j8 = lax.broadcasted_iota(jnp.int32, (8, 56), 1)
        fill_b = jnp.concatenate([jnp.where(j8 < 40, masked, -3e38).astype(f32)] * 5
                                 + [jnp.where(j8 < 40, -3e38, masked).astype(f32)], axis=0)

        def softmax(sc, mask, fill):
            sc = jnp.where(mask, sc, fill)
            mx = jnp.max(sc, axis=-1, keepdims=True)
            e = jnp.exp2((sc - mx) * (scale * 1.4426950408889634))
            den = jnp.sum(e, axis=-1, keepdims=True)
            return (e * pl.reciprocal(den, approx=True)).astype(bf16)

        def ride_rows(s, is_b):
            first = s < 2
            if is_b:
                g = [jnp.where(first, -3, -1), 1, 2]
            else:
                g = [jnp.where(first, 1, 0), jnp.where(first, 2, 1), 3]
            return [RIDE * s + 8 * t for t in g]

        def step(s, is_b, lhs_lo, lhs_hi, soft_in, jobs):
            seg = pl.multiple_of((SEG * s + ROFF) % NR, SEG)
            sega = pl.multiple_of(seg - SEG, SEG) if is_b else seg
            wr = [pl.multiple_of((NPRE + RIDE * s + 8 * t + ROFF) % NR, 8) for t in range(3)]
            rd = [pl.multiple_of((r + ROFF) % NR, 8) for r in ride_rows(s, is_b)]
            lhs = jnp.concatenate([lhs_lo, lhs_hi], axis=1)
            QM, P, PART = {}, {}, {}
            mrow = 0 if is_b else MEM
            seg8 = pl.multiple_of(seg + 8, 8)
            seg24 = pl.multiple_of(seg + RIDE, 8)

            def wblk(b, lo, n):
                return pltpu.bitcast(wqkv[b * WP + lo:b * WP + lo + n, :], bf16)

            def qkv_lo(i):
                for m in range(3):
                    PART[(m, i)] = jnp.dot(lhs_lo, wblk(m * H + i, 0, 256), preferred_element_type=f32)

            def qkv(i):
                for m in range(3):
                    b = m * H + i
                    if (m, i) in PART:
                        y = jnp.dot(lhs_hi, wblk(b, 256, 256),
                                    preferred_element_type=f32) + PART.pop((m, i))
                    else:
                        y = jnp.dot(lhs, wblk(b, 0, 512), preferred_element_type=f32)
                    if m < 2:
                        QM[b] = y[0:MEM] + jobs["pin"] if b == PIN and is_b else y[0:MEM]
                    if m == 2 or (m == 1 and not is_b):
                        kvm[b - H, mrow:mrow + MEM, :] = y[0:MEM].astype(bf16)
                    for t in range(3):
                        rset(b, wr[t], y[8 + 8 * t:16 + 8 * t])
                    for job in jobs.get(3 * i + m, []):
                        job(y)

            def keys(b):
                if is_b:
                    if b in QM:
                        old = kvm[b - H, MEM:2 * MEM, :].astype(f32)
                        mix = jnp.concatenate([QM.pop(b), old], axis=0).astype(bf16)
                    else:
                        mix = kvm[b - H]
                    return jnp.concatenate([rget(b, seg, SEG), mix, rget(b, sega, 8)], axis=0)
                mk = QM.pop(b).astype(bf16) if b in QM else kvm[b - H, MEM:2 * MEM, :]
                return jnp.concatenate([rget(b, seg, SEG), mk], axis=0)

            def scores(i):
                if is_b:
                    mix = jnp.concatenate([QM.pop(i), rget(i, sega, 8).astype(f32)], axis=0)
                    q = jnp.concatenate([rget(i, seg, SEG), mix.astype(bf16)], axis=0)
                else:
                    mix = jnp.concatenate([rget(i, seg24, 8).astype(f32), QM.pop(i)], axis=0)
                    q = jnp.concatenate([rget(i, seg8, 16), mix.astype(bf16)], axis=0)
                sc = lax.dot_general(q, keys(H + i), (((1,), (1,)), ((), ())),
                                     preferred_element_type=f32)
                P[i] = softmax(sc, mask_b, fill_b) if is_b else softmax(sc, mask_a, masked)

            def pv(i):
                o = jnp.dot(P.pop(i), keys(2 * H + i), preferred_element_type=f32)
                if is_b:
                    rset(i, seg, o[0:SEG])
                    rset(i, sega, o[40:48])
                    lhs_o[i, 0:MEM, :] = o[SEG:L].astype(bf16)
                else:
                    rset(i, seg8, o[0:16])
                    rset(i, seg24, o[16:RIDE])
                    lhs_o[i, 0:MEM, :] = o[RIDE:32].astype(bf16)
                for t in range(3):
                    lhs_o[i, 8 + 8 * t:16 + 8 * t, :] = rget(i, rd[t], 8)

            def wo_lhs(i0, i1):
                return jnp.concatenate([lhs_o[i] for i in range(i0, i1)], axis=1)

            def wo_dot(lo, j, i0, i1):
                r = WO + j * 2048
                w = pltpu.bitcast(wqkv[r + 64 * i0:r + 64 * i1, :], bf16)
                return jnp.dot(lo, w, preferred_element_type=f32)

            def side(t):
                ds, dp = (DSB, DPB) if is_b else (DSA, DPA)
                if 0 <= t - dp < H:
                    pv(t - dp)
                if 0 <= t - ds < H:
                    scores(t - ds)

            if soft_in:
                for h in range(KSPLIT):
                    qkv_lo(h)
            for h in range(H):
                qkv(h)
                side(h)
            lo = [wo_lhs(8 * k, 8 * k + 8) for k in range(3)]
            acc = []
            for j in range(8):
                y = None
                for k in range(3):
                    z = wo_dot(lo[k], j, 8 * k, 8 * k + 8)
                    y = z if y is None else z + y
                    for job in jobs.get(96 + 3 * j + k, []):
                        job(y)
                acc.append(y)
                side(H + j)
            lo = wo_lhs(24, H)
            for j in range(8):
                acc[j] = wo_dot(lo, j, 24, H) + acc[j]
                for job in jobs.get(120 + j, []):
                    job(acc[j])
            assert not (QM or P or PART)
            return jnp.concatenate(acc[0:4], axis=1), jnp.concatenate(acc[4:8], axis=1)

        def combine(c, n, y):
            mp, k1 = divmod(n, 8)
            m, p = divmod(mp, 4)
            c3 = jnp.minimum(c, 27)
            spare = pl.ds(pl.multiple_of(8 * (c // 64), 8), 8)
            if m == 0 and k1 < 7:
                ws3[16, spare, :] = y.astype(bf16)
            else:
                wsr[7, spare, 0:128] = y.astype(bf16)
            if k1 == 7:
                dst, base, r = w7, 0, (4 * m + p) * 256 + c * 8
                blk = [wsr[4 + i, m * 16:(m + 1) * 16, j * 512 + p * 128:j * 512 + (p + 1) * 128]
                       .astype(f32) for i in range(2) for j in range(2)]
            else:
                dst, base = w49, 7 * k1
                if m == 0:
                    r = c3 * 32 + p * 8
                    get = lambda i, j: ws3[4 * i + j, p * 16:(p + 1) * 16, :]
                else:
                    r = W4R + (p // 2) * 448 + c3 * 16 + (p % 2) * 8
                    r0, c0 = (p % 2) * 16, (p // 2) * 128
                    get = lambda i, j: wsr[i, r0:r0 + 16, j * 256 + c0:j * 256 + c0 + 128]

                def quad(q):
                    return [get(2 * (q // 2) + i, 2 * (q % 2) + j).astype(f32)
                            for i in range(2) for j in range(2)]
                qi, qj, sign = _BTERMS[k1]
                blk = quad(qi)
                if qj is not None:
                    blk = [u + v if sign > 0 else u - v for u, v in zip(blk, quad(qj))]
            for k, op in enumerate(_b_operands(*blk)):
                dst[base + k, pl.ds(pl.multiple_of(r, 8), 8), :] = pltpu.bitcast(
                    op.astype(bf16), u32)

        def rec_body(it, gacc):
            stream_wait(it)
            lhs_lo = lhs_h[:, 0:512]
            lhs_hi = lhs_h[:, 512:1024]
            ra = jnp.maximum(it - 1, 0) * (2 * RIDE)
            for u in range(2):
                s = 2 * it + u
                jobs = {}
                for n, (su, d, g) in enumerate(SLOTS):
                    if su == u:
                        jobs.setdefault(d, []).append(
                            lambda y, n=n, g=g: combine(it, n, y[8 * g:8 * g + 8]))
                r1 = pl.multiple_of(jnp.minimum(NPRE + RIDE * (s + 1), S - RIDE), 8)
                xn = xbuf[pl.ds(r1, RIDE), :].astype(f32)
                if u == 0:
                    for k in range(2):
                        rm = pl.multiple_of(it * 32 + k * 16, 16)
                        gacc = mod_rows(gacc, wsr[6, k * 16:(k + 1) * 16, :], rm)
                    hn = adaln_a(xn, _zero_after(stage_a16(ra)))
                else:
                    def refill(y):
                        for cp in stream_copies(jnp.minimum(it + 1, NSEG // 2 - 1)):
                            cp.start()
                        spare = pl.ds(pl.multiple_of(8 * (it // 64), 8), 8)
                        jobs["pin"] = _zero_after(ws3[16, spare, :].astype(f32))
                    jobs.setdefault(3 * (PIN - 4) + 2, []).append(refill)
                    hn = adaln_a(xn)
                    z = _zero_after(hn[0:8], hn[8:16], hn[16:24])
                    stage_a16(ra + 32, _zero_after(stage_a16(ra + 16, z)))
                a_lo, a_hi = step(s, u == 1, lhs_lo, lhs_hi, u > 0, jobs)
                lhs_lo = jnp.concatenate([a_lo[0:MEM], hn[:, 0:512]], axis=0).astype(bf16)
                lhs_hi = jnp.concatenate([a_hi[0:MEM], hn[:, 512:1024]], axis=0).astype(bf16)
                a = jnp.concatenate([a_lo, a_hi], axis=1)
                rows = [pl.multiple_of(r, 8) for r in ride_rows(s, u == 1)]
                xs = [xbuf[pl.ds(r, 8), :].astype(f32) for r in rows]
                for t, r in enumerate(rows):
                    xa = xs[t] + modrows(2, 8) * a[8 + 8 * t:16 + 8 * t]
                    xbuf[pl.ds(r, 8), :] = xa.astype(bf16)
            lhs_h[:, 0:512] = lhs_lo
            lhs_h[:, 512:1024] = lhs_hi
            return gacc

        gacc = _loop("rec", 0, NSEG // 2, rec_body, jnp.zeros((8, D), f32))
        for c in range(2):
            mod_finish(gacc[:, c * 512:(c + 1) * 512], 10 + c)
        stream_wait(NSEG // 2 - 1)

        def wo_prep(i, half, k):
            o = jnp.concatenate([rings[4 * half + h][i, k * 16:(k + 1) * 16, :].astype(f32)
                                 for h in range(4)], axis=1)
            for t, op in enumerate(row_operands(o)):
                a7[half, t, k * 8:(k + 1) * 8, :] = op.astype(bf16)

        def wo_chunk(i, half, inext, extra):
            row = pl.multiple_of(i * 512 + half * 256, 256)
            todo = list(range(NPRE // 16))
            spare = pl.ds(pl.multiple_of(8 * (i // 64), 8), 8)

            def hook(v):
                if todo:
                    for h in range(4):
                        rings[4 * (1 - half) + h][4, spare, :] = v[0:8].astype(bf16)
                    n = 2 if len(todo) % WPP == 0 else 1
                    for k in todo[:n]:
                        wo_prep(inext, 1 - half, k)
                    del todo[:n]
                extra(v)

            for j in range(4):
                def b_of(k):
                    def quad(q):
                        r = WO + (j + 4 * (q % 2)) * 2048 + (q // 2) * 128 + row
                        return pltpu.bitcast(wqkv[pl.ds(r, 128), :], bf16)
                    qi, qj, sign = _BTERMS[k]
                    if qj is None:
                        return quad(qi)
                    u, v = quad(qi).astype(f32), quad(qj).astype(f32)
                    return (u + v if sign > 0 else u - v).astype(bf16)
                c11, c12, c21, c22 = _strassen(lambda k: a7[half, k], b_of, hook)
                for c, y in ((j + 4, _merge_rows(c12, c22)), (j, _merge_rows(c11, c21))):
                    cs = slice(c * 128, (c + 1) * 128)
                    h2buf[S - NPRE:S, cs] = h2buf[S - NPRE:S, cs] + y

        for k in range(NPRE // 16):
            wo_prep(0, 0, k)

        def wo_tail(i, _):
            st = {"n": 0, "prev": None}

            def extra(v):
                n = st["n"]
                st["n"] += 1
                if n % 16 == 2 and n // 16 < 3:
                    st["prev"] = stage_a16(S - NPRE - 48 + 16 * (n // 16),
                                           _zero_after(v, st["prev"]))
            wo_chunk(i, 0, i, extra)
            wo_chunk(i, 1, jnp.minimum(i + 1, 3), extra)
            return 0
        _loop("wotail", 0, 4, wo_tail)

        def gget(c, row, n):
            return pltpu.bitcast(wqkv[pl.ds(c * GS + row, n), :], f32)

        def gset(c, row, val):
            wqkv[pl.ds(c * GS + row, val.shape[0]), :] = pltpu.bitcast(val, u32)

        def wop(j):
            return lambda k: pltpu.bitcast(w7[k, j * 256:(j + 1) * 256, :], bf16)

        zpad = jnp.zeros((GPAD, 128), f32)
        for cb in range(8):
            gset(cb, 0, zpad)
            gset(cb, GPAD + S, zpad)

        shifts = (-1, -1, 1, 1, -2, -2, 2, 2)
        HB = MB // 2

        def shift_piece(r, half, k):
            gs = jnp.concatenate([gget(c, r + (k * 16 + GPAD + shifts[c]), 16)
                                  for c in range(8)], axis=1)
            ro = half * (HB // 2) + k * 8
            for t, op in enumerate(row_operands(gs)):
                n7[t, ro:ro + 8, :] = op.astype(bf16)

        def gate(v, i):
            gset(0, GPAD + S + GPAD + 8 * (i // S), v[0:8])

        def b_body(i, _):
            rl = S - NPRE + i * 128
            st = {"n": 0, "prev": [None, None]}

            def hook(v):
                n = st["n"]
                st["n"] += 1
                if n % BG == 0 and n // BG < 8:
                    k = n // BG
                    st["prev"][k % BCH] = stage_a16(rl + 16 * k,
                                                    _zero_after(v, st["prev"][k % BCH]),
                                                    (t7, 8 * k))

            ro = pl.multiple_of(i * 192, 64)
            for lhs, row in ((lambda k: n7[k, pl.ds(ro, 192), :], i * 384), (lambda k: t7[k], rl)):
                rg = pl.multiple_of(GPAD + row, 8)
                for j in range(4):
                    c11, c12, c21, c22 = _strassen(lhs, wop(j), hook)
                    gset(j + 4, rg, _gelu(_merge_rows(c12, c22)))
                    gset(j, rg, _gelu(_merge_rows(c11, c21)))
            return 0
        _loop("b", 0, S // MB, b_body)
        for k in range(HB // 16):
            shift_piece(0, 0, k)

        def n2_norm(r, k, anchor):
            v = _ln(h2buf[pl.ds(pl.multiple_of(r + k * 16, 16), 16), :], anchor)
            nrms[k // 2][(k % 2) * 16:(k % 2) * 16 + 16, :] = v
            return v[0:8] + v[8:16]

        def n2_ops(k, k1, v, i):
            nrm = nrms[k]
            nrm[pl.ds(pl.multiple_of(32 + 8 * (i // S), 8), 8), 0:128] = v[0:8]

            def quad(q):
                r0, c0 = (q // 2) * 16, (q % 2) * 512
                return [nrm[r0 + 8 * a:r0 + 8 * a + 8, c0 + 256 * b:c0 + 256 * b + 256]
                        for a in range(2) for b in range(2)]
            qi, qj, sign = _ATERMS[k1]
            blk = quad(qi)
            if qj is not None:
                blk = [u + w if sign > 0 else u - w for u, w in zip(blk, quad(qj))]
            for k2, op in enumerate(_a_operands(*blk)):
                d49[7 * k1 + k2, k * 8:(k + 1) * 8, :] = op.astype(bf16)

        def n2_hook(r, i, first, gap, lag, st):
            def hook(v):
                n = st["n"] - first
                st["n"] += 1
                if n >= 0 and n % gap == 0 and n // gap < MD // 16:
                    st["prev"] = n2_norm(r, n // gap, _zero_after(v, st["prev"]))
                for _ in range(st["per"]):
                    k, k1 = divmod(st["ops"], 7)
                    if k < MD // 32 and n >= (2 * k + 1) * gap + lag:
                        n2_ops(k, k1, v, i)
                        st["ops"] += 1
            return hook

        def stage_c(i, r, half, rnext, extra):
            rr = pl.multiple_of(r, 8)
            ro = half * (HB // 2)
            cnt = [0]

            def hook(v):
                n = cnt[0]
                cnt[0] += 1
                if n < HB // 16:
                    gate(v, i)
                    shift_piece(rnext, 1 - half, n)
                extra(v)

            for j in range(4):
                c11, c12, c21, c22 = _strassen(lambda k: n7[k, ro:ro + HB // 2, :], wop(4 + j),
                                               hook)
                for c, y in ((j + 4, _merge_rows(c12, c22)), (j, _merge_rows(c11, c21))):
                    cs = slice(c * 128, (c + 1) * 128)
                    h2buf[pl.ds(rr, HB), cs] = h2buf[pl.ds(rr, HB), cs] + y

        def c_body(i, _):
            r = pl.multiple_of(i * MB, MB)
            st = {"n": 0, "prev": None, "ops": 0, "per": 1}
            extra = n2_hook(0, i, 0, 4, 4, st)
            stage_c(i, r, 0, r + HB, extra)
            stage_c(i, r + HB, 1, jnp.minimum(i + 1, S // MB - 1) * MB, extra)
            assert st["ops"] == 28
            return 0
        _loop("c", 0, S // MB, c_body)

        def wop2(lo, n):
            return lambda k1, k: pltpu.bitcast(w49[7 * k1 + k, lo:lo + n, :], bf16)

        def d_body(i, _):
            r = pl.multiple_of(i * MD, MD)
            rn = jnp.minimum(r + MD, S - MD)
            lhs = [d49[k] for k in range(49)]
            uops = []
            for t in range(7):
                cb = _strassen2(lambda k1, k: lhs[7 * k1 + k], wop2(t * 128, 128))
                uops.append(_a_operands2([[_gelu(c) for c in row] for row in cb]))
            ul = [[jnp.concatenate([u[k1][k] for u in uops], axis=1).astype(bf16)
                   for k in range(7)] for k1 in range(7)]
            st = {"n": 0, "prev": None, "ops": 0, "per": 1}
            hook = n2_hook(rn, i, DF, DG, DL, st)
            for t in range(2):
                cb = _strassen2(lambda k1, k: ul[k1][k], wop2(W4R + t * 448, 448), hook)
                for j in range(4):
                    y = jnp.concatenate([cb[q][j].reshape(MD // 32, 8, 128) for q in range(4)],
                                        axis=1).reshape(MD, 128)
                    c = 2 * j + t
                    cs = slice(c * 128, (c + 1) * 128)
                    gb = modrows(5, MD, c * 128, (c + 1) * 128)
                    o = xbuf[pl.ds(r, MD), cs].astype(f32) + gb * (h2buf[pl.ds(r, MD), cs] + y)
                    xbuf[pl.ds(r, MD), cs] = o.astype(bf16)
            assert st["ops"] == 28
            out_copy(r, MD).start()
            return 0
        _loop("d", 0, S // MD, d_body)

    pl.run_scoped(main,
                  pltpu.VMEM((7, 8 * 256, 128), u32),
                  pltpu.VMEM((49, 2 * W4R, 128), u32))

    out_copy(0, S).wait()


def _run(x, mem0, wq, wk, wv, wo, w1, w2, w3, w4, c, wmod):
    any_spec = pl.BlockSpec(memory_space=pl.ANY)
    return pl.pallas_call(
        _kernel,
        out_shape=jax.ShapeDtypeStruct((S, D), bf16),
        in_specs=[any_spec] * 12,
        out_specs=any_spec,
        scratch_shapes=[
            pltpu.VMEM((S + 2 * RIDE, D), bf16),
            pltpu.VMEM((WO + 8 * 2048, 128), u32),
            [pltpu.VMEM((96 // NRING, NR, 128), bf16)] * NRING,
            pltpu.VMEM((32, D), bf16),
            pltpu.VMEM((H, 32, 128), bf16),
            pltpu.VMEM((2 * H, 16, 128), bf16),
            pltpu.VMEM((12, 8, 512), f32),
            pltpu.VMEM((D, 128), f32),
            pltpu.VMEM((S, D), f32),
            pltpu.VMEM((7, (S - NPRE) // 2, 512), bf16),
            pltpu.VMEM((17, 64, 128), bf16),
            pltpu.VMEM((8, 32, D), bf16),
            pltpu.VMEM((7, 64, 512), bf16),
            pltpu.VMEM((2, 7, NPRE // 2, 256), bf16),
            pltpu.VMEM((49, MD // 4, 256), bf16),
            [pltpu.VMEM((40, D), f32)] * (MD // 32),
            pltpu.VMEM((1, D), bf16),
            pltpu.SemaphoreType.DMA((9 + NGRP + 2,)),
        ],
        compiler_params=pltpu.CompilerParams(vmem_limit_bytes=124 * 1024 * 1024,
                                             disable_bounds_checks=True,
                                             disable_semaphore_checks=True),
    )(x, mem0, wq, wk, wv, wo, w1, w2, w3, w4, c, wmod)


def pallas_adaLN_cond__memory_aug_recurrent_mem_tr__mixer_s_mlp__prompt_kernel(
    A_x, A_mem0, A_Wq, A_Wk, A_Wv, A_Wo, A_seg_len, B_x, B_w1, B_w2, B_w3, B_w4, c, w_mod,
):
    del B_x
    assert A_x.shape == (1, S, D) and A_mem0.shape == (1, MEM, D)
    assert isinstance(A_seg_len, int) is False or A_seg_len == SEG
    out = _run(A_x.reshape(S, D), A_mem0.reshape(MEM, D), A_Wq, A_Wk, A_Wv,
               A_Wo.reshape(H * DH, D),
               B_w1.reshape(2, D // 2, D), B_w2.reshape(2, D // 2, D),
               B_w3, B_w4.reshape(4, F // 4, D), c, w_mod)
    return out.reshape(1, S, D)
```

```python
import jax
import jax.numpy as jnp
from jax import lax
import jax.experimental.pallas as pl
import jax.experimental.pallas.tpu as pltpu

bf16 = jnp.bfloat16
f32 = jnp.float32
u32 = jnp.uint32

S = 2048
D = 1024
H = 32
DH = 128
F = 3584
MEM = 8
SEG = 32
NSEG = S // SEG
L = MEM + SEG
RIDE = 24
NPRE = S - RIDE * NSEG
NR = NPRE + 2 * SEG
ROFF = (-(S - NPRE)) % NR
WP = 516
WO = 96 * WP
NGRP = 12
NSLOT = 6
NMOD = 6
EPS = 1e-5
MD = 128
MB = 512
GPAD = 8
NRING = 8
RLP, WLP, RSK = 27, 22, 2
NWO = 3
BG, WPP, PIN, BCH = 2, 5, 6, 2
DF, DG, DL = 2, 10, 9
SLOTS = ([(0, n // 2, 3 * (n % 2)) for n in range(16)] + [(0, 96 + n, 0) for n in range(16)]
         + [(0, 112 + n // 2, 3 * (n % 2)) for n in range(32)])
DSA, DPA, DSB, DPB, KSPLIT = 6, 12, 6, 12, 2
X0 = NPRE + 2 * RIDE
GS = S + 4 * GPAD
W4R = 7 * 128
_ONLY = None


def _loop(name, lo, hi, body, init=0):
    if _ONLY is not None and name not in _ONLY:
        return init
    with _scope(name):
        return lax.fori_loop(lo, hi, body, init)


class _NoScope:
    def __init__(self, name):
        del name

    def __enter__(self):
        return self

    def __exit__(self, *a):
        return False


_scope = _NoScope


def _zero_after(*vs):
    bits = None
    for v in vs:
        if v is not None:
            b = pltpu.bitcast(v[0:8, 0:128], u32)
            bits = b if bits is None else bits | b
    return pltpu.bitcast((bits >> 31) >> 1, f32)


def _ln(x, anchor=None):
    if anchor is not None:
        z = jnp.concatenate([anchor] * (x.shape[0] // 8), axis=0)
        x = jnp.concatenate([x[:, 0:128] + z, x[:, 128:]], axis=1)
    mu = jnp.mean(x, axis=-1, keepdims=True)
    xc = x - mu
    var = jnp.mean(xc * xc, axis=-1, keepdims=True)
    return xc * lax.rsqrt(var + EPS)


def _gelu(x):
    inner = x * (0.7978845608028654 + (0.7978845608028654 * 0.044715) * (x * x))
    hx = 0.5 * x
    return hx + hx * jnp.tanh(inner)


def _split_rows(x):
    m, n = x.shape
    x3 = x.reshape(m // 16, 16, n)
    return x3[:, 0:8, :].reshape(m // 2, n), x3[:, 8:16, :].reshape(m // 2, n)


def _merge_rows(top, bot):
    m, n = top.shape
    return jnp.concatenate([top.reshape(m // 8, 8, n), bot.reshape(m // 8, 8, n)],
                           axis=1).reshape(2 * m, n)


def _a_operands(a11, a12, a21, a22):
    return [a11 + a22, a21 + a22, a11, a22, a11 + a12, a21 - a11, a12 - a22]


def _b_operands(b11, b12, b21, b22):
    return [b11 + b22, b11, b12 - b22, b21 - b11, b22, b11 + b12, b21 + b22]


_ATERMS = ((0, 3, 1), (2, 3, 1), (0, None, 0), (3, None, 0), (0, 1, 1), (2, 0, -1), (1, 3, -1))
_BTERMS = ((0, 3, 1), (0, None, 0), (1, 3, -1), (2, 0, -1), (3, None, 0), (0, 1, 1), (2, 3, 1))


def _strassen(a_of, b_of, hook=lambda v: None):
    def prod(k):
        return jnp.dot(a_of(k), b_of(k), preferred_element_type=f32)
    p5 = prod(4)
    hook(p5)
    p3 = prod(2)
    hook(p3)
    c12 = p3 + p5
    p4 = prod(3)
    hook(p4)
    c11 = p4 - p5
    p2 = prod(1)
    hook(p2)
    c21 = p2 + p4
    c22 = p3 - p2
    p1 = prod(0)
    hook(p1)
    c11 = prod(6) + (c11 + p1)
    hook(c11)
    c22 = prod(5) + (c22 + p1)
    hook(c22)
    return c11, c12, c21, c22


def _a_operands2(b):
    sub = [_a_operands(b[i][j], b[i][2 + j], b[2 + i][j], b[2 + i][2 + j])
           for i in range(2) for j in range(2)]
    return [_a_operands(*[t[k] for t in sub]) for k in range(7)]


def _strassen2(a_of, b_of, hook=lambda v: None):
    def prod(k1):
        return _strassen(lambda k: a_of(k1, k), lambda k: b_of(k1, k), hook)

    def add(x, y):
        return [p + q for p, q in zip(x, y)]

    def sub(x, y):
        return [p - q for p, q in zip(x, y)]
    p5 = prod(4)
    p3 = prod(2)
    c12 = add(p3, p5)
    p4 = prod(3)
    c11 = sub(p4, p5)
    p2 = prod(1)
    c21 = add(p2, p4)
    c22 = sub(p3, p2)
    p1 = prod(0)
    c11 = add(add(c11, p1), prod(6))
    c22 = add(add(c22, p1), prod(5))
    cq = (c11, c12, c21, c22)
    return [[cq[2 * (i // 2) + j // 2][2 * (i % 2) + j % 2] for j in range(4)] for i in range(4)]


def _kernel(x_hbm, mem0_hbm, wq_hbm, wk_hbm, wv_hbm, wo_hbm, w1_hbm, w2_hbm, w3_hbm, w4_hbm,
            c_hbm, wmod_hbm, out_hbm,
            xbuf, wqkv, rings, lhs_h, lhs_o, kvm, modv, scol, h2buf, n7, ws3, wsr, t7, a7, d49, nrms, c_ref,
            sems):
    w_hbms = (wq_hbm, wk_hbm, wv_hbm)
    SMOD, SSTG = 5, 9
    sem_x, sem_out, sem_w, sem_g, sem_r = (sems.at[k] for k in range(5))

    def rget(b, row, n):
        return rings[b % NRING][b // NRING, pl.ds(row, n), :]

    def rset(b, row, val):
        rings[b % NRING][b // NRING, pl.ds(row, val.shape[0]), :] = val.astype(bf16)

    x_copy = pltpu.make_async_copy(x_hbm.at[pl.ds(0, X0), :], xbuf.at[pl.ds(0, X0), :], sem_x)

    def stream_copies(c):
        al, lo = ((lambda v, m: v), min) if isinstance(c, int) else (pl.multiple_of, jnp.minimum)
        c3 = lo(c, 27)
        cps = [pltpu.make_async_copy(
            w3_hbm.at[pl.ds(al(i * 256 + (c3 % 4) * 64, 64), 64),
                      pl.ds(al(j * (F // 4) + (c3 // 4) * 128, 128), 128)],
            ws3.at[4 * i + j], sem_w) for i in range(4) for j in range(4)]
        dst = X0 + 2 * RIDE * c
        return [
            pltpu.make_async_copy(w4_hbm.at[:, pl.ds(al(c3 * 32, 32), 32), :],
                                  wsr.at[pl.ds(0, 4)], sem_g),
            pltpu.make_async_copy(w1_hbm.at[:, pl.ds(al(c * 16, 16), 16), :],
                                  wsr.at[pl.ds(4, 2), pl.ds(0, 16), :], sem_g),
            pltpu.make_async_copy(w2_hbm.at[:, pl.ds(al(c * 16, 16), 16), :],
                                  wsr.at[pl.ds(4, 2), pl.ds(16, 16), :], sem_g),
            pltpu.make_async_copy(wmod_hbm.at[pl.ds(al(c * 32, 32), 32), pl.ds(5 * D, D)],
                                  wsr.at[6], sem_g),
            pltpu.make_async_copy(x_hbm.at[pl.ds(al(lo(dst, S - 2 * RIDE), 16), 2 * RIDE), :],
                                  xbuf.at[pl.ds(al(dst, 16), 2 * RIDE), :], sem_r)] + cps

    def stream_wait(c):
        for dst, sem in ((ws3.at[pl.ds(0, 16)], sem_w), (wsr.at[pl.ds(0, 7)], sem_g),
                         (xbuf.at[pl.ds(X0 + 2 * RIDE * c, 2 * RIDE), :], sem_r)):
            pltpu.make_async_copy(dst, dst, sem).wait()

    def out_copy(row, n):
        return pltpu.make_async_copy(xbuf.at[pl.ds(row, n), :], out_hbm.at[pl.ds(row, n), :],
                                     sem_out)

    def mod_rows(acc, w, r):
        sc = jnp.concatenate([scol[pl.ds(r, 16), :]] * (w.shape[1] // 128), axis=1)
        p = w.astype(f32) * sc
        return acc + p[0:8] + p[8:16]

    def mod_finish(acc, j):
        is_scale = jnp.logical_or(j // 2 == 1, j // 2 == 4)
        tot = jnp.sum(acc, axis=0, keepdims=True) + jnp.where(is_scale, 1.0, 0.0)
        modv[j] = jnp.broadcast_to(tot, (8, 512))

    def modrows(k, n, lo=0, hi=D):
        m = jnp.concatenate([modv[2 * k], modv[2 * k + 1]], axis=1)[:, lo:hi]
        return jnp.concatenate([m] * (n // 8), axis=0)

    def adaln_a(xv, anchor=None):
        n = xv.shape[0]
        return _ln(xv, anchor) * modrows(1, n) + modrows(0, n)

    def adaln_b(xv, anchor=None):
        n = xv.shape[0]
        return _ln(xv, anchor) * modrows(4, n) + modrows(3, n)

    def row_operands(v):
        top, bot = _split_rows(v)
        k = v.shape[1] // 2
        return _a_operands(top[:, :k], top[:, k:], bot[:, :k], bot[:, k:])

    def stage_a16(r, anchor=None, dst=None):
        rr = pl.multiple_of(r, 16)
        xv = xbuf[pl.ds(rr, 16), :]
        if dst is not None:
            xv = (xv.astype(f32) + modrows(2, 16) * h2buf[pl.ds(rr, 16), :]).astype(bf16)
            xbuf[pl.ds(rr, 16), :] = xv
        h2 = adaln_b(xv.astype(f32), anchor)
        h2buf[pl.ds(rr, 16), :] = h2
        ref, ro = (n7, pl.multiple_of(rr // 2, 8)) if dst is None else dst
        ops = row_operands(_ln(h2))
        for t, op in enumerate(ops):
            ref[t, pl.ds(ro, 8), :] = op.astype(bf16)
        return ops[0]

    def prologue(stg, wos, wmodb, h7):
        def mod_copy(j):
            return pltpu.make_async_copy(wmod_hbm.at[:, pl.ds(j * 512, 512)], wmodb.at[j % NMOD],
                                         sems.at[SSTG + j + 4 if j >= 4 else SMOD + j])

        def piece_copy(g, dh):
            return pltpu.make_async_copy(
                w_hbms[g // 4].at[pl.ds(dh * 512, 512), pl.ds((g % 4) * 8, 8), :],
                stg.at[(2 * g + dh) % NSLOT], sems.at[SSTG + (g + 1 if g else dh)])

        def wo_copy(j):
            return pltpu.make_async_copy(wo_hbm.at[pl.ds(j * 512, 512), :], wos.at[j % NWO],
                                         sems.at[SSTG + j + 6])

        def group_start(g):
            for dh in range(2):
                piece_copy(g, dh).start()

        def stg_wait(slot, n, sem):
            dst = stg.at[pl.ds(slot, n)]
            pltpu.make_async_copy(dst, dst, sems.at[SSTG + sem]).wait()

        def relayout(g, slot, dh, lo_dp, n_dp):
            base = g * (8 * WP) + dh * 256
            for u in range(n_dp):
                dp = lo_dp + u
                ev = pltpu.bitcast(stg[slot, 2 * dp].astype(f32), u32)
                od = pltpu.bitcast(stg[slot, 2 * dp + 1].astype(f32), u32)
                wqkv[pl.ds(base + dp, 8, stride=WP), :] = (ev >> 16) | od

        def b_operand(gbase, q, k):
            def quad(i):
                r = gbase + ((q + 4 * (i % 2)) * WP + (i // 2) * 256)
                return pltpu.bitcast(wqkv[pl.ds(r, 256), :], bf16)
            i, j, sign = _BTERMS[k]
            if j is None:
                return quad(i)
            u, v = quad(i).astype(f32), quad(j).astype(f32)
            return (u + v if sign > 0 else u - v).astype(bf16)

        c_copy = pltpu.make_async_copy(c_hbm, c_ref, sem_g)
        m_copy = pltpu.make_async_copy(mem0_hbm, lhs_h.at[pl.ds(0, MEM), :], sem_r)
        c_copy.start()
        m_copy.start()
        x_copy.start()
        for j in range(4):
            mod_copy(j).start()
        for g in range(3):
            group_start(g)
        h2buf[S - NPRE:S, :] = jnp.zeros((NPRE, D), f32)
        wos[2] = jnp.zeros((512, D), bf16)
        c_copy.wait()
        m_copy.wait()
        cv = c_ref[...].astype(f32)
        sv = jnp.broadcast_to(cv * (1.0 / (1.0 + jnp.exp(-cv))), (128, D))
        for k in range(8):
            scol[k * 128:(k + 1) * 128, :] = sv[:, k * 128:(k + 1) * 128].T
        x_copy.wait()

        def ln0_body(i, _):
            r = pl.multiple_of(i * 64, 64)
            h2buf[pl.ds(r, 64), :] = _ln(xbuf[pl.ds(r, 64), :].astype(f32))
            return 0
        lax.fori_loop(0, NPRE // 64, ln0_body, 0)

        def mod0_body(j, _):
            pltpu.make_async_copy(wmodb.at[j], wmodb.at[j], sems.at[SMOD + j]).wait()
            accs = [jnp.zeros((8, 512), f32)] * 2
            for k in range(64):
                accs[k % 2] = mod_rows(accs[k % 2], wmodb[j, k * 16:(k + 1) * 16, :], k * 16)
            mod_finish(accs[0] + accs[1], j)
            return 0
        _loop("mod0", 0, 4, mod0_body)

        def hpre_body(i, _):
            r = pl.multiple_of(i * 32, 32)
            hv = h2buf[pl.ds(r, 32), :] * modrows(1, 32) + modrows(0, 32)
            ro = pl.multiple_of(i * 8, 8)
            for t, op in enumerate(row_operands(hv)):
                h7[t, pl.ds(ro, 8), :] = pltpu.bitcast(op.astype(bf16), u32)
            return 0
        lax.fori_loop(0, NPRE // 32, hpre_body, 0)
        lhs_h[MEM:32, :] = adaln_a(xbuf[NPRE:NPRE + RIDE, :].astype(f32)).astype(bf16)

        def relayout_now(g, dh):
            def rl_body(t, _):
                relayout(g, 2 * g + dh, dh, t * 32, 32)
                return 0
            lax.fori_loop(0, 8, rl_body, 0)

        for dh in range(2):
            stg_wait(dh, 1, dh)
            relayout_now(0, dh)

        grp = lambda g: [piece_copy(g, 0), piece_copy(g, 1)]
        issue = {0: [wo_copy(0)], 1: grp(3) + grp(4), 2: grp(5) + [wo_copy(1), mod_copy(4)],
                 3: grp(6) + [mod_copy(5), mod_copy(6)], 4: grp(7) + [wo_copy(2)],
                 5: grp(8) + [wo_copy(3), mod_copy(7)], 6: grp(9) + [wo_copy(4)],
                 7: grp(10) + [wo_copy(5), mod_copy(8)], 8: grp(11) + [wo_copy(6)],
                 9: [wo_copy(7), mod_copy(9)], 10: stream_copies(0)}

        def pre_iter(g, carry):
            m3, gbase = carry

            @pl.when(g == 1)
            def _():
                stg_wait(2, 2, 2)
                relayout_now(1, 0)
                relayout_now(1, 1)

            def slots():
                m3n = jnp.where(m3 == 2, 0, m3 + 1)
                cj = jnp.maximum(g - 2, 3)
                return (m3n, 2 * jnp.where(ends, m3, m3n),
                        jnp.where(jnp.logical_or(g < 4, m3 == 0), 2, m3 - 1),
                        cj, jnp.where(cj >= NMOD, cj - NMOD, cj))

            ends = jnp.logical_or(g == 0, g == NGRP - 1)

            @pl.when(jnp.logical_not(ends))
            def _():
                stg_wait(slots()[1], 2, g + 2)

            @pl.when(g >= 4)
            def _():
                buf = wos.at[slots()[2]]
                pltpu.make_async_copy(buf, buf, sems.at[SSTG + g + 2]).wait()

            @pl.when(g >= 6)
            def _():
                buf = wmodb.at[slots()[4]]
                pltpu.make_async_copy(buf, buf, sems.at[SSTG + g + 2]).wait()

            m3n, gslot, wslot, cj, cslot = slots()
            gn = jnp.where(ends, g, g + 1)
            wrow = WO + jnp.maximum(g - 4, 0) * 256
            for k, cps in issue.items():
                @pl.when(g == k)
                def _():
                    for cp in cps:
                        cp.start()
            wtodo = [(r, c) for r in range(16) for c in range(8)]
            todo = [(dh, dp) for dh in range(2) for dp in range(256)]
            skip = [0] * RSK
            mtodo = list(range(0, D, 16))
            macc = [jnp.zeros((8, 512), f32)]

            def hook(v):
                if mtodo:
                    acc = macc[0] + jnp.concatenate([_zero_after(v)] * 4, axis=1)
                    for r in mtodo[:3]:
                        acc = mod_rows(acc, wmodb[cslot, r:r + 16, :], r)
                    del mtodo[:3]
                    macc[0] = acc

            for q in range(4):
                def b_of(k):
                    w = b_operand(gbase, q, k)
                    if skip:
                        skip.pop()
                        return w
                    nw = 0 if todo else WLP
                    for dh, dp in todo[:RLP]:
                        relayout(gn, gslot + dh, dh, dp, 1)
                    del todo[:RLP]
                    for r, c in wtodo[:nw]:
                        wqkv[pl.ds(wrow + (c * 2048 + r * 16), 16), :] = pltpu.bitcast(
                            wos[wslot, r * 32:(r + 1) * 32, c * 128:(c + 1) * 128], u32)
                    del wtodo[:nw]
                    return w
                c11, c12, c21, c22 = _strassen(lambda k: pltpu.bitcast(h7[k], bf16), b_of, hook)
                for blk, y in ((q + 4, _merge_rows(c12, c22)), (q, _merge_rows(c11, c21))):
                    y = y.astype(bf16)
                    n0 = NR - ROFF
                    rings[blk][g, ROFF:NR, :] = y[0:n0]
                    rings[blk][g, 0:NPRE - n0, :] = y[n0:NPRE]
            assert not todo and not wtodo and not mtodo
            mod_finish(macc[0], cj)
            return m3n, gbase + 8 * WP

        _loop("pre1", 0, NGRP, pre_iter, (0, 0))

    pl.run_scoped(prologue,
                  pltpu.VMEM((NSLOT, 512, 8, 128), bf16),
                  pltpu.VMEM((NWO, 512, D), bf16),
                  pltpu.VMEM((NMOD, D, 512), bf16),
                  pltpu.VMEM((7, NPRE // 4, 512), u32))

    def main(w7, w49):
        scale = DH ** -0.5
        ia = lax.broadcasted_iota(jnp.int32, (32, L), 0)
        ja = lax.broadcasted_iota(jnp.int32, (32, L), 1)
        mask_a = (ia >= RIDE) | (ja >= SEG) | (ia + 8 >= ja)
        ib = lax.broadcasted_iota(jnp.int32, (48, 56), 0)
        jb = lax.broadcasted_iota(jnp.int32, (48, 56), 1)
        own = (ib < 40) == (jb < 40)
        mask_b = own & (((jb >= 32) & (jb < 48)) | (jnp.where(jb < 40, jb, jb - 8) <= ib))
        masked = -1e9 / scale
        j8 = lax.broadcasted_iota(jnp.int32, (8, 56), 1)
        fill_b = jnp.concatenate([jnp.where(j8 < 40, masked, -3e38).astype(f32)] * 5
                                 + [jnp.where(j8 < 40, -3e38, masked).astype(f32)], axis=0)

        def softmax(sc, mask, fill):
            sc = jnp.where(mask, sc, fill)
            mx = jnp.max(sc, axis=-1, keepdims=True)
            e = jnp.exp2((sc - mx) * (scale * 1.4426950408889634))
            den = jnp.sum(e, axis=-1, keepdims=True)
            return (e * pl.reciprocal(den, approx=True)).astype(bf16)

        def ride_rows(s, is_b):
            first = s < 2
            if is_b:
                g = [jnp.where(first, -3, -1), 1, 2]
            else:
                g = [jnp.where(first, 1, 0), jnp.where(first, 2, 1), 3]
            return [RIDE * s + 8 * t for t in g]

        def step(s, is_b, lhs_lo, lhs_hi, soft_in, jobs):
            seg = pl.multiple_of((SEG * s + ROFF) % NR, SEG)
            sega = pl.multiple_of(seg - SEG, SEG) if is_b else seg
            wr = [pl.multiple_of((NPRE + RIDE * s + 8 * t + ROFF) % NR, 8) for t in range(3)]
            rd = [pl.multiple_of((r + ROFF) % NR, 8) for r in ride_rows(s, is_b)]
            lhs = jnp.concatenate([lhs_lo, lhs_hi], axis=1)
            QM, P, PART = {}, {}, {}
            mrow = 0 if is_b else MEM
            seg8 = pl.multiple_of(seg + 8, 8)
            seg24 = pl.multiple_of(seg + RIDE, 8)

            def wblk(b, lo, n):
                return pltpu.bitcast(wqkv[b * WP + lo:b * WP + lo + n, :], bf16)

            def qkv_lo(i):
                for m in range(3):
                    PART[(m, i)] = jnp.dot(lhs_lo, wblk(m * H + i, 0, 256), preferred_element_type=f32)

            def qkv(i):
                for m in range(3):
                    b = m * H + i
                    if (m, i) in PART:
                        y = jnp.dot(lhs_hi, wblk(b, 256, 256),
                                    preferred_element_type=f32) + PART.pop((m, i))
                    else:
                        y = jnp.dot(lhs, wblk(b, 0, 512), preferred_element_type=f32)
                    if m < 2:
                        QM[b] = y[0:MEM] + jobs["pin"] if b == PIN and is_b else y[0:MEM]
                    if m == 2 or (m == 1 and not is_b):
                        kvm[b - H, mrow:mrow + MEM, :] = y[0:MEM].astype(bf16)
                    for t in range(3):
                        rset(b, wr[t], y[8 + 8 * t:16 + 8 * t])
                    for job in jobs.get(3 * i + m, []):
                        job(y)
                    side(3 * i + m)

            def keys(b):
                if is_b:
                    if b in QM:
                        old = kvm[b - H, MEM:2 * MEM, :].astype(f32)
                        mix = jnp.concatenate([QM.pop(b), old], axis=0).astype(bf16)
                    else:
                        mix = kvm[b - H]
                    return jnp.concatenate([rget(b, seg, SEG), mix, rget(b, sega, 8)], axis=0)
                mk = QM.pop(b).astype(bf16) if b in QM else kvm[b - H, MEM:2 * MEM, :]
                return jnp.concatenate([rget(b, seg, SEG), mk], axis=0)

            def scores(i):
                if is_b:
                    mix = jnp.concatenate([QM.pop(i), rget(i, sega, 8).astype(f32)], axis=0)
                    q = jnp.concatenate([rget(i, seg, SEG), mix.astype(bf16)], axis=0)
                else:
                    mix = jnp.concatenate([rget(i, seg24, 8).astype(f32), QM.pop(i)], axis=0)
                    q = jnp.concatenate([rget(i, seg8, 16), mix.astype(bf16)], axis=0)
                sc = lax.dot_general(q, keys(H + i), (((1,), (1,)), ((), ())),
                                     preferred_element_type=f32)
                P[i] = softmax(sc, mask_b, fill_b) if is_b else softmax(sc, mask_a, masked)

            def pv(i):
                o = jnp.dot(P.pop(i), keys(2 * H + i), preferred_element_type=f32)
                if is_b:
                    rset(i, seg, o[0:SEG])
                    rset(i, sega, o[40:48])
                    lhs_o[i, 0:MEM, :] = o[SEG:L].astype(bf16)
                else:
                    rset(i, seg8, o[0:16])
                    rset(i, seg24, o[16:RIDE])
                    lhs_o[i, 0:MEM, :] = o[RIDE:32].astype(bf16)
                for t in range(3):
                    lhs_o[i, 8 + 8 * t:16 + 8 * t, :] = rget(i, rd[t], 8)

            def wo_lhs(i0, i1):
                return jnp.concatenate([lhs_o[i] for i in range(i0, i1)], axis=1)

            def wo_dot(lo, j, i0, i1):
                r = WO + j * 2048
                w = pltpu.bitcast(wqkv[r + 64 * i0:r + 64 * i1, :], bf16)
                return jnp.dot(lo, w, preferred_element_type=f32)

            def side(d):
                ds, dp = (DSB, DPB) if is_b else (DSA, DPA)
                if (d - dp) % 3 == 2 and 0 <= (d - dp) // 3 < H:
                    pv((d - dp) // 3)
                if (d - ds) % 3 == 2 and 0 <= (d - ds) // 3 < H:
                    scores((d - ds) // 3)

            if soft_in:
                for h in range(KSPLIT):
                    qkv_lo(h)
            for h in range(H):
                qkv(h)
            lo = [wo_lhs(8 * k, 8 * k + 8) for k in range(3)]
            acc = []
            for j in range(8):
                y = None
                for k in range(3):
                    z = wo_dot(lo[k], j, 8 * k, 8 * k + 8)
                    y = z if y is None else z + y
                    for job in jobs.get(96 + 3 * j + k, []):
                        job(y)
                    side(96 + 3 * j + k)
                acc.append(y)
            lo = wo_lhs(24, H)
            for j in range(8):
                acc[j] = wo_dot(lo, j, 24, H) + acc[j]
                for job in jobs.get(120 + j, []):
                    job(acc[j])
            assert not (QM or P or PART)
            return jnp.concatenate(acc[0:4], axis=1), jnp.concatenate(acc[4:8], axis=1)

        def combine(c, n, y):
            mp, k1 = divmod(n, 8)
            m, p = divmod(mp, 4)
            c3 = jnp.minimum(c, 27)
            spare = pl.ds(pl.multiple_of(8 * (c // 64), 8), 8)
            if m == 0 and k1 < 7:
                ws3[16, spare, :] = y.astype(bf16)
            else:
                wsr[7, spare, 0:128] = y.astype(bf16)
            if k1 == 7:
                dst, base, r = w7, 0, (4 * m + p) * 256 + c * 8
                blk = [wsr[4 + i, m * 16:(m + 1) * 16, j * 512 + p * 128:j * 512 + (p + 1) * 128]
                       .astype(f32) for i in range(2) for j in range(2)]
            else:
                dst, base = w49, 7 * k1
                if m == 0:
                    r = c3 * 32 + p * 8
                    get = lambda i, j: ws3[4 * i + j, p * 16:(p + 1) * 16, :]
                else:
                    r = W4R + (p // 2) * 448 + c3 * 16 + (p % 2) * 8
                    r0, c0 = (p % 2) * 16, (p // 2) * 128
                    get = lambda i, j: wsr[i, r0:r0 + 16, j * 256 + c0:j * 256 + c0 + 128]

                def quad(q):
                    return [get(2 * (q // 2) + i, 2 * (q % 2) + j).astype(f32)
                            for i in range(2) for j in range(2)]
                qi, qj, sign = _BTERMS[k1]
                blk = quad(qi)
                if qj is not None:
                    blk = [u + v if sign > 0 else u - v for u, v in zip(blk, quad(qj))]
            for k, op in enumerate(_b_operands(*blk)):
                for e in range(2):
                    dst[base + k, pl.ds(r + 4 * e, 4), :] = pltpu.bitcast(
                        op[8 * e:8 * e + 8].astype(bf16), u32)

        def rec_body(it, gacc):
            stream_wait(it)
            lhs_lo = lhs_h[:, 0:512]
            lhs_hi = lhs_h[:, 512:1024]
            ra = jnp.maximum(it - 1, 0) * (2 * RIDE)
            for u in range(2):
                s = 2 * it + u
                jobs = {}
                for n, (su, d, g) in enumerate(SLOTS):
                    if su == u:
                        jobs.setdefault(d, []).append(
                            lambda y, n=n, g=g: combine(it, n, y[8 * g:8 * g + 8]))
                r1 = pl.multiple_of(jnp.minimum(NPRE + RIDE * (s + 1), S - RIDE), 8)
                xn = xbuf[pl.ds(r1, RIDE), :].astype(f32)
                if u == 0:
                    for k in range(2):
                        rm = pl.multiple_of(it * 32 + k * 16, 16)
                        gacc = mod_rows(gacc, wsr[6, k * 16:(k + 1) * 16, :], rm)
                    hn = adaln_a(xn, _zero_after(stage_a16(ra)))
                else:
                    def refill(y):
                        for cp in stream_copies(jnp.minimum(it + 1, NSEG // 2 - 1)):
                            cp.start()
                        spare = pl.ds(pl.multiple_of(8 * (it // 64), 8), 8)
                        jobs["pin"] = _zero_after(ws3[16, spare, :].astype(f32))
                    jobs.setdefault(3 * (PIN - 4) + 2, []).append(refill)
                    hn = adaln_a(xn)
                    z = _zero_after(hn[0:8], hn[8:16], hn[16:24])
                    stage_a16(ra + 32, _zero_after(stage_a16(ra + 16, z)))
                a_lo, a_hi = step(s, u == 1, lhs_lo, lhs_hi, u > 0, jobs)
                lhs_lo = jnp.concatenate([a_lo[0:MEM], hn[:, 0:512]], axis=0).astype(bf16)
                lhs_hi = jnp.concatenate([a_hi[0:MEM], hn[:, 512:1024]], axis=0).astype(bf16)
                a = jnp.concatenate([a_lo, a_hi], axis=1)
                rows = [pl.multiple_of(r, 8) for r in ride_rows(s, u == 1)]
                xs = [xbuf[pl.ds(r, 8), :].astype(f32) for r in rows]
                for t, r in enumerate(rows):
                    xa = xs[t] + modrows(2, 8) * a[8 + 8 * t:16 + 8 * t]
                    xbuf[pl.ds(r, 8), :] = xa.astype(bf16)
            lhs_h[:, 0:512] = lhs_lo
            lhs_h[:, 512:1024] = lhs_hi
            return gacc

        gacc = _loop("rec", 0, NSEG // 2, rec_body, jnp.zeros((8, D), f32))
        for c in range(2):
            mod_finish(gacc[:, c * 512:(c + 1) * 512], 10 + c)
        stream_wait(NSEG // 2 - 1)

        def wo_prep(i, half, k):
            o = jnp.concatenate([rings[4 * half + h][i, k * 16:(k + 1) * 16, :].astype(f32)
                                 for h in range(4)], axis=1)
            for t, op in enumerate(row_operands(o)):
                a7[half, t, k * 8:(k + 1) * 8, :] = op.astype(bf16)

        def wo_chunk(i, half, inext, extra):
            row = pl.multiple_of(i * 512 + half * 256, 256)
            todo = list(range(NPRE // 16))
            spare = pl.ds(pl.multiple_of(8 * (i // 64), 8), 8)

            def hook(v):
                if todo:
                    for h in range(4):
                        rings[4 * (1 - half) + h][4, spare, :] = v[0:8].astype(bf16)
                    n = 2 if len(todo) % WPP == 0 else 1
                    for k in todo[:n]:
                        wo_prep(inext, 1 - half, k)
                    del todo[:n]
                extra(v)

            for j in range(4):
                def b_of(k):
                    def quad(q):
                        r = WO + (j + 4 * (q % 2)) * 2048 + (q // 2) * 128 + row
                        return pltpu.bitcast(wqkv[pl.ds(r, 128), :], bf16)
                    qi, qj, sign = _BTERMS[k]
                    if qj is None:
                        return quad(qi)
                    u, v = quad(qi).astype(f32), quad(qj).astype(f32)
                    return (u + v if sign > 0 else u - v).astype(bf16)
                c11, c12, c21, c22 = _strassen(lambda k: a7[half, k], b_of, hook)
                for c, y in ((j + 4, _merge_rows(c12, c22)), (j, _merge_rows(c11, c21))):
                    cs = slice(c * 128, (c + 1) * 128)
                    h2buf[S - NPRE:S, cs] = h2buf[S - NPRE:S, cs] + y

        for k in range(NPRE // 16):
            wo_prep(0, 0, k)

        def wo_tail(i, _):
            st = {"n": 0, "prev": None}

            def extra(v):
                n = st["n"]
                st["n"] += 1
                if n % 16 == 2 and n // 16 < 3:
                    st["prev"] = stage_a16(S - NPRE - 48 + 16 * (n // 16),
                                           _zero_after(v, st["prev"]))
            wo_chunk(i, 0, i, extra)
            wo_chunk(i, 1, jnp.minimum(i + 1, 3), extra)
            return 0
        _loop("wotail", 0, 4, wo_tail)

        def gget(c, row, n):
            return pltpu.bitcast(wqkv[pl.ds(c * GS + row, n), :], f32)

        def gset(c, row, val):
            wqkv[pl.ds(c * GS + row, val.shape[0]), :] = pltpu.bitcast(val, u32)

        def wop(j):
            return lambda k: pltpu.bitcast(w7[k, j * 256:(j + 1) * 256, :], bf16)

        zpad = jnp.zeros((GPAD, 128), f32)
        for cb in range(8):
            gset(cb, 0, zpad)
            gset(cb, GPAD + S, zpad)

        shifts = (-1, -1, 1, 1, -2, -2, 2, 2)
        HB = MB // 2

        def shift_piece(r, half, k):
            gs = jnp.concatenate([gget(c, r + (k * 16 + GPAD + shifts[c]), 16)
                                  for c in range(8)], axis=1)
            ro = half * (HB // 2) + k * 8
            for t, op in enumerate(row_operands(gs)):
                n7[t, ro:ro + 8, :] = op.astype(bf16)

        def gate(v, i):
            gset(0, GPAD + S + GPAD + 8 * (i // S), v[0:8])

        def b_body(i, _):
            rl = S - NPRE + i * 128
            st = {"n": 0, "prev": [None, None]}

            def hook(v):
                n = st["n"]
                st["n"] += 1
                if n % BG == 0 and n // BG < 8:
                    k = n // BG
                    st["prev"][k % BCH] = stage_a16(rl + 16 * k,
                                                    _zero_after(v, st["prev"][k % BCH]),
                                                    (t7, 8 * k))

            ro = pl.multiple_of(i * 192, 64)
            for lhs, row in ((lambda k: n7[k, pl.ds(ro, 192), :], i * 384), (lambda k: t7[k], rl)):
                rg = pl.multiple_of(GPAD + row, 8)
                for j in range(4):
                    c11, c12, c21, c22 = _strassen(lhs, wop(j), hook)
                    gset(j + 4, rg, _gelu(_merge_rows(c12, c22)))
                    gset(j, rg, _gelu(_merge_rows(c11, c21)))
            return 0
        _loop("b", 0, S // MB, b_body)
        for k in range(HB // 16):
            shift_piece(0, 0, k)

        def n2_norm(r, k, anchor):
            v = _ln(h2buf[pl.ds(pl.multiple_of(r + k * 16, 16), 16), :], anchor)
            nrms[k // 2][(k % 2) * 16:(k % 2) * 16 + 16, :] = v
            return v[0:8] + v[8:16]

        def n2_ops(k, k1, v, i):
            nrm = nrms[k]
            nrm[pl.ds(pl.multiple_of(32 + 8 * (i // S), 8), 8), 0:128] = v[0:8]

            def quad(q):
                r0, c0 = (q // 2) * 16, (q % 2) * 512
                return [nrm[r0 + 8 * a:r0 + 8 * a + 8, c0 + 256 * b:c0 + 256 * b + 256]
                        for a in range(2) for b in range(2)]
            qi, qj, sign = _ATERMS[k1]
            blk = quad(qi)
            if qj is not None:
                blk = [u + w if sign > 0 else u - w for u, w in zip(blk, quad(qj))]
            for k2, op in enumerate(_a_operands(*blk)):
                d49[7 * k1 + k2, k * 8:(k + 1) * 8, :] = op.astype(bf16)

        def n2_hook(r, i, first, gap, lag, st):
            def hook(v):
                n = st["n"] - first
                st["n"] += 1
                if n >= 0 and n % gap == 0 and n // gap < MD // 16:
                    st["prev"] = n2_norm(r, n // gap, _zero_after(v, st["prev"]))
                for _ in range(st["per"]):
                    k, k1 = divmod(st["ops"], 7)
                    if k < MD // 32 and n >= (2 * k + 1) * gap + lag:
                        n2_ops(k, k1, v, i)
                        st["ops"] += 1
            return hook

        def stage_c(i, r, half, rnext, extra):
            rr = pl.multiple_of(r, 8)
            ro = half * (HB // 2)
            cnt = [0]

            def hook(v):
                n = cnt[0]
                cnt[0] += 1
                if n < HB // 16:
                    gate(v, i)
                    shift_piece(rnext, 1 - half, n)
                extra(v)

            for j in range(4):
                c11, c12, c21, c22 = _strassen(lambda k: n7[k, ro:ro + HB // 2, :], wop(4 + j),
                                               hook)
                for c, y in ((j + 4, _merge_rows(c12, c22)), (j, _merge_rows(c11, c21))):
                    cs = slice(c * 128, (c + 1) * 128)
                    h2buf[pl.ds(rr, HB), cs] = h2buf[pl.ds(rr, HB), cs] + y

        def c_body(i, _):
            r = pl.multiple_of(i * MB, MB)
            st = {"n": 0, "prev": None, "ops": 0, "per": 1}
            extra = n2_hook(0, i, 0, 4, 4, st)
            stage_c(i, r, 0, r + HB, extra)
            stage_c(i, r + HB, 1, jnp.minimum(i + 1, S // MB - 1) * MB, extra)
            assert st["ops"] == 28
            return 0
        _loop("c", 0, S // MB, c_body)

        def wop2(lo, n):
            return lambda k1, k: pltpu.bitcast(w49[7 * k1 + k, lo:lo + n, :], bf16)

        def d_body(i, _):
            r = pl.multiple_of(i * MD, MD)
            rn = jnp.minimum(r + MD, S - MD)
            lhs = [d49[k] for k in range(49)]
            uops = []
            for t in range(7):
                cb = _strassen2(lambda k1, k: lhs[7 * k1 + k], wop2(t * 128, 128))
                uops.append(_a_operands2([[_gelu(c) for c in row] for row in cb]))
            ul = [[jnp.concatenate([u[k1][k] for u in uops], axis=1).astype(bf16)
                   for k in range(7)] for k1 in range(7)]
            st = {"n": 0, "prev": None, "ops": 0, "per": 1}
            hook = n2_hook(rn, i, DF, DG, DL, st)
            for t in range(2):
                cb = _strassen2(lambda k1, k: ul[k1][k], wop2(W4R + t * 448, 448), hook)
                for j in range(4):
                    y = jnp.concatenate([cb[q][j].reshape(MD // 32, 8, 128) for q in range(4)],
                                        axis=1).reshape(MD, 128)
                    c = 2 * j + t
                    cs = slice(c * 128, (c + 1) * 128)
                    gb = modrows(5, MD, c * 128, (c + 1) * 128)
                    o = xbuf[pl.ds(r, MD), cs].astype(f32) + gb * (h2buf[pl.ds(r, MD), cs] + y)
                    xbuf[pl.ds(r, MD), cs] = o.astype(bf16)
            assert st["ops"] == 28
            out_copy(r, MD).start()
            return 0
        _loop("d", 0, S // MD, d_body)

    pl.run_scoped(main,
                  pltpu.VMEM((7, 8 * 256, 128), u32),
                  pltpu.VMEM((49, 2 * W4R, 128), u32))

    out_copy(0, S).wait()


def _run(x, mem0, wq, wk, wv, wo, w1, w2, w3, w4, c, wmod):
    any_spec = pl.BlockSpec(memory_space=pl.ANY)
    return pl.pallas_call(
        _kernel,
        out_shape=jax.ShapeDtypeStruct((S, D), bf16),
        in_specs=[any_spec] * 12,
        out_specs=any_spec,
        scratch_shapes=[
            pltpu.VMEM((S + 2 * RIDE, D), bf16),
            pltpu.VMEM((WO + 8 * 2048, 128), u32),
            [pltpu.VMEM((96 // NRING, NR, 128), bf16)] * NRING,
            pltpu.VMEM((32, D), bf16),
            pltpu.VMEM((H, 32, 128), bf16),
            pltpu.VMEM((2 * H, 16, 128), bf16),
            pltpu.VMEM((12, 8, 512), f32),
            pltpu.VMEM((D, 128), f32),
            pltpu.VMEM((S, D), f32),
            pltpu.VMEM((7, (S - NPRE) // 2, 512), bf16),
            pltpu.VMEM((17, 64, 128), bf16),
            pltpu.VMEM((8, 32, D), bf16),
            pltpu.VMEM((7, 64, 512), bf16),
            pltpu.VMEM((2, 7, NPRE // 2, 256), bf16),
            pltpu.VMEM((49, MD // 4, 256), bf16),
            [pltpu.VMEM((40, D), f32)] * (MD // 32),
            pltpu.VMEM((1, D), bf16),
            pltpu.SemaphoreType.DMA((9 + NGRP + 2,)),
        ],
        compiler_params=pltpu.CompilerParams(vmem_limit_bytes=124 * 1024 * 1024,
                                             disable_bounds_checks=True,
                                             disable_semaphore_checks=True),
    )(x, mem0, wq, wk, wv, wo, w1, w2, w3, w4, c, wmod)


def pallas_adaLN_cond__memory_aug_recurrent_mem_tr__mixer_s_mlp__prompt_kernel(
    A_x, A_mem0, A_Wq, A_Wk, A_Wv, A_Wo, A_seg_len, B_x, B_w1, B_w2, B_w3, B_w4, c, w_mod,
):
    del B_x
    assert A_x.shape == (1, S, D) and A_mem0.shape == (1, MEM, D)
    assert isinstance(A_seg_len, int) is False or A_seg_len == SEG
    out = _run(A_x.reshape(S, D), A_mem0.reshape(MEM, D), A_Wq, A_Wk, A_Wv,
               A_Wo.reshape(H * DH, D),
               B_w1.reshape(2, D // 2, D), B_w2.reshape(2, D // 2, D),
               B_w3, B_w4.reshape(4, F // 4, D), c, w_mod)
    return out.reshape(1, S, D)
```

```python
import jax
import jax.numpy as jnp
from jax import lax
import jax.experimental.pallas as pl
import jax.experimental.pallas.tpu as pltpu

bf16 = jnp.bfloat16
f32 = jnp.float32
u32 = jnp.uint32

S = 2048
D = 1024
H = 32
DH = 128
F = 3584
MEM = 8
SEG = 32
NSEG = S // SEG
L = MEM + SEG
RIDE = 24
NPRE = S - RIDE * NSEG
NR = NPRE + 2 * SEG
ROFF = (-(S - NPRE)) % NR
WP = 516
WO = 96 * WP
NGRP = 12
NSLOT = 6
NMOD = 6
EPS = 1e-5
MD = 128
MB = 512
GPAD = 8
NRING = 8
RLP, WLP, RSK = 27, 22, 2
NWO = 3
BG, WPP, PIN, BCH = 2, 5, 6, 2
DF, DG, DL = 2, 10, 9
SLOTS = ([(0, n // 2, 3 * (n % 2)) for n in range(16)] + [(0, 96 + n, 0) for n in range(16)]
         + [(0, 112 + n // 2, 3 * (n % 2)) for n in range(32)])
DSA, DPA, DSB, DPB, KSPLIT = 6, 12, 6, 12, 2
X0 = NPRE + 2 * RIDE
GS = S + 4 * GPAD
W4R = 7 * 128
_ONLY = None


def _loop(name, lo, hi, body, init=0):
    if _ONLY is not None and name not in _ONLY:
        return init
    with _scope(name):
        return lax.fori_loop(lo, hi, body, init)


class _NoScope:
    def __init__(self, name):
        del name

    def __enter__(self):
        return self

    def __exit__(self, *a):
        return False


_scope = _NoScope


def _zero_after(*vs):
    bits = None
    for v in vs:
        if v is not None:
            b = pltpu.bitcast(v[0:8, 0:128], u32)
            bits = b if bits is None else bits | b
    return pltpu.bitcast((bits >> 31) >> 1, f32)


def _ln(x, anchor=None):
    if anchor is not None:
        z = jnp.concatenate([anchor] * (x.shape[0] // 8), axis=0)
        x = jnp.concatenate([x[:, 0:128] + z, x[:, 128:]], axis=1)
    mu = jnp.mean(x, axis=-1, keepdims=True)
    xc = x - mu
    var = jnp.mean(xc * xc, axis=-1, keepdims=True)
    return xc * lax.rsqrt(var + EPS)


def _gelu(x):
    inner = x * (0.7978845608028654 + (0.7978845608028654 * 0.044715) * (x * x))
    hx = 0.5 * x
    return hx + hx * jnp.tanh(inner)


def _split_rows(x):
    m, n = x.shape
    x3 = x.reshape(m // 16, 16, n)
    return x3[:, 0:8, :].reshape(m // 2, n), x3[:, 8:16, :].reshape(m // 2, n)


def _merge_rows(top, bot):
    m, n = top.shape
    return jnp.concatenate([top.reshape(m // 8, 8, n), bot.reshape(m // 8, 8, n)],
                           axis=1).reshape(2 * m, n)


def _a_operands(a11, a12, a21, a22):
    return [a11 + a22, a21 + a22, a11, a22, a11 + a12, a21 - a11, a12 - a22]


def _b_operands(b11, b12, b21, b22):
    return [b11 + b22, b11, b12 - b22, b21 - b11, b22, b11 + b12, b21 + b22]


_ATERMS = ((0, 3, 1), (2, 3, 1), (0, None, 0), (3, None, 0), (0, 1, 1), (2, 0, -1), (1, 3, -1))
_BTERMS = ((0, 3, 1), (0, None, 0), (1, 3, -1), (2, 0, -1), (3, None, 0), (0, 1, 1), (2, 3, 1))


def _strassen(a_of, b_of, hook=lambda v: None):
    def prod(k):
        return jnp.dot(a_of(k), b_of(k), preferred_element_type=f32)
    p5 = prod(4)
    hook(p5)
    p3 = prod(2)
    hook(p3)
    c12 = p3 + p5
    p4 = prod(3)
    hook(p4)
    c11 = p4 - p5
    p2 = prod(1)
    hook(p2)
    c21 = p2 + p4
    c22 = p3 - p2
    p1 = prod(0)
    hook(p1)
    c11 = prod(6) + (c11 + p1)
    hook(c11)
    c22 = prod(5) + (c22 + p1)
    hook(c22)
    return c11, c12, c21, c22


def _a_operands2(b):
    sub = [_a_operands(b[i][j], b[i][2 + j], b[2 + i][j], b[2 + i][2 + j])
           for i in range(2) for j in range(2)]
    return [_a_operands(*[t[k] for t in sub]) for k in range(7)]


def _strassen2(a_of, b_of, hook=lambda v: None):
    def prod(k1):
        return _strassen(lambda k: a_of(k1, k), lambda k: b_of(k1, k), hook)

    def add(x, y):
        return [p + q for p, q in zip(x, y)]

    def sub(x, y):
        return [p - q for p, q in zip(x, y)]
    p5 = prod(4)
    p3 = prod(2)
    c12 = add(p3, p5)
    p4 = prod(3)
    c11 = sub(p4, p5)
    p2 = prod(1)
    c21 = add(p2, p4)
    c22 = sub(p3, p2)
    p1 = prod(0)
    c11 = add(add(c11, p1), prod(6))
    c22 = add(add(c22, p1), prod(5))
    cq = (c11, c12, c21, c22)
    return [[cq[2 * (i // 2) + j // 2][2 * (i % 2) + j % 2] for j in range(4)] for i in range(4)]


def _pack8(v):
    return pltpu.bitcast(v.astype(bf16), u32)


def _unpack(w):
    return pltpu.bitcast(w, bf16)


def _kernel(x_hbm, mem0_hbm, wq_hbm, wk_hbm, wv_hbm, wo_hbm, w1_hbm, w2_hbm, w3_hbm, w4_hbm,
            c_hbm, wmod_hbm, out_hbm,
            xbuf, wqkv, rings, lhs_h, lhs_o, kvm, modv, scol, h2buf, n7, ws3, wsr, t7, a7, d49, nrms, c_ref,
            sems):
    w_hbms = (wq_hbm, wk_hbm, wv_hbm)
    SMOD, SSTG = 5, 9
    sem_x, sem_out, sem_w, sem_g, sem_r = (sems.at[k] for k in range(5))

    def rget(b, pos, n):
        return rings[b % NRING][b // NRING, pl.ds(pos, n), :]

    def rset(b, pos, val):
        for e in range(val.shape[0] // 8):
            rings[b % NRING][b // NRING, pl.ds(pos + 4 * e, 4), :] = _pack8(val[8 * e:8 * e + 8])

    x_copy = pltpu.make_async_copy(x_hbm.at[pl.ds(0, X0), :], xbuf.at[pl.ds(0, X0), :], sem_x)

    def stream_copies(c):
        al, lo = ((lambda v, m: v), min) if isinstance(c, int) else (pl.multiple_of, jnp.minimum)
        c3 = lo(c, 27)
        cps = [pltpu.make_async_copy(
            w3_hbm.at[pl.ds(al(i * 256 + (c3 % 4) * 64, 64), 64),
                      pl.ds(al(j * (F // 4) + (c3 // 4) * 128, 128), 128)],
            ws3.at[4 * i + j], sem_w) for i in range(4) for j in range(4)]
        dst = X0 + 2 * RIDE * c
        return [
            pltpu.make_async_copy(w4_hbm.at[:, pl.ds(al(c3 * 32, 32), 32), :],
                                  wsr.at[pl.ds(0, 4)], sem_g),
            pltpu.make_async_copy(w1_hbm.at[:, pl.ds(al(c * 16, 16), 16), :],
                                  wsr.at[pl.ds(4, 2), pl.ds(0, 16), :], sem_g),
            pltpu.make_async_copy(w2_hbm.at[:, pl.ds(al(c * 16, 16), 16), :],
                                  wsr.at[pl.ds(4, 2), pl.ds(16, 16), :], sem_g),
            pltpu.make_async_copy(wmod_hbm.at[pl.ds(al(c * 32, 32), 32), pl.ds(5 * D, D)],
                                  wsr.at[6], sem_g),
            pltpu.make_async_copy(x_hbm.at[pl.ds(al(lo(dst, S - 2 * RIDE), 16), 2 * RIDE), :],
                                  xbuf.at[pl.ds(al(dst, 16), 2 * RIDE), :], sem_r)] + cps

    def stream_wait(c):
        for dst, sem in ((ws3.at[pl.ds(0, 16)], sem_w), (wsr.at[pl.ds(0, 7)], sem_g),
                         (xbuf.at[pl.ds(X0 + 2 * RIDE * c, 2 * RIDE), :], sem_r)):
            pltpu.make_async_copy(dst, dst, sem).wait()

    def out_copy(row, n):
        return pltpu.make_async_copy(xbuf.at[pl.ds(row, n), :], out_hbm.at[pl.ds(row, n), :],
                                     sem_out)

    def mod_rows(acc, w, r):
        sc = jnp.concatenate([scol[pl.ds(r, 16), :]] * (w.shape[1] // 128), axis=1)
        p = w.astype(f32) * sc
        return acc + p[0:8] + p[8:16]

    def mod_finish(acc, j):
        is_scale = jnp.logical_or(j // 2 == 1, j // 2 == 4)
        tot = jnp.sum(acc, axis=0, keepdims=True) + jnp.where(is_scale, 1.0, 0.0)
        modv[j] = jnp.broadcast_to(tot, (8, 512))

    def modrows(k, n, lo=0, hi=D):
        m = jnp.concatenate([modv[2 * k], modv[2 * k + 1]], axis=1)[:, lo:hi]
        return jnp.concatenate([m] * (n // 8), axis=0)

    def adaln_a(xv, anchor=None):
        n = xv.shape[0]
        return _ln(xv, anchor) * modrows(1, n) + modrows(0, n)

    def adaln_b(xv, anchor=None):
        n = xv.shape[0]
        return _ln(xv, anchor) * modrows(4, n) + modrows(3, n)

    def row_operands(v):
        top, bot = _split_rows(v)
        k = v.shape[1] // 2
        return _a_operands(top[:, :k], top[:, k:], bot[:, :k], bot[:, k:])

    def stage_a16(r, anchor=None, dst=None):
        rr = pl.multiple_of(r, 16)
        xv = xbuf[pl.ds(rr, 16), :]
        if dst is not None:
            xv = (xv.astype(f32) + modrows(2, 16) * h2buf[pl.ds(rr, 16), :]).astype(bf16)
            xbuf[pl.ds(rr, 16), :] = xv
        h2 = adaln_b(xv.astype(f32), anchor)
        h2buf[pl.ds(rr, 16), :] = h2
        ref, ro = (n7, pl.multiple_of(rr // 2, 8)) if dst is None else dst
        ops = row_operands(_ln(h2))
        for t, op in enumerate(ops):
            ref[t, pl.ds(ro, 8), :] = op.astype(bf16)
        return ops[0]

    def prologue(stg, wos, wmodb, h7):
        def mod_copy(j):
            return pltpu.make_async_copy(wmod_hbm.at[:, pl.ds(j * 512, 512)], wmodb.at[j % NMOD],
                                         sems.at[SSTG + j + 4 if j >= 4 else SMOD + j])

        def piece_copy(g, dh):
            return pltpu.make_async_copy(
                w_hbms[g // 4].at[pl.ds(dh * 512, 512), pl.ds((g % 4) * 8, 8), :],
                stg.at[(2 * g + dh) % NSLOT], sems.at[SSTG + (g + 1 if g else dh)])

        def wo_copy(j):
            return pltpu.make_async_copy(wo_hbm.at[pl.ds(j * 512, 512), :], wos.at[j % NWO],
                                         sems.at[SSTG + j + 6])

        def group_start(g):
            for dh in range(2):
                piece_copy(g, dh).start()

        def stg_wait(slot, n, sem):
            dst = stg.at[pl.ds(slot, n)]
            pltpu.make_async_copy(dst, dst, sems.at[SSTG + sem]).wait()

        def relayout(g, slot, dh, lo_dp, n_dp):
            base = g * (8 * WP) + dh * 256
            for u in range(n_dp):
                dp = lo_dp + u
                ev = pltpu.bitcast(stg[slot, 2 * dp].astype(f32), u32)
                od = pltpu.bitcast(stg[slot, 2 * dp + 1].astype(f32), u32)
                wqkv[pl.ds(base + dp, 8, stride=WP), :] = (ev >> 16) | od

        def b_operand(gbase, q, k):
            def quad(i):
                r = gbase + ((q + 4 * (i % 2)) * WP + (i // 2) * 256)
                return pltpu.bitcast(wqkv[pl.ds(r, 256), :], bf16)
            i, j, sign = _BTERMS[k]
            if j is None:
                return quad(i)
            u, v = quad(i).astype(f32), quad(j).astype(f32)
            return (u + v if sign > 0 else u - v).astype(bf16)

        c_copy = pltpu.make_async_copy(c_hbm, c_ref, sem_g)
        m_copy = pltpu.make_async_copy(mem0_hbm, lhs_h.at[pl.ds(0, MEM), :], sem_r)
        c_copy.start()
        m_copy.start()
        x_copy.start()
        for j in range(4):
            mod_copy(j).start()
        for g in range(3):
            group_start(g)
        h2buf[S - NPRE:S, :] = jnp.zeros((NPRE, D), f32)
        wos[2] = jnp.zeros((512, D), bf16)
        c_copy.wait()
        m_copy.wait()
        cv = c_ref[...].astype(f32)
        sv = jnp.broadcast_to(cv * (1.0 / (1.0 + jnp.exp(-cv))), (128, D))
        for k in range(8):
            scol[k * 128:(k + 1) * 128, :] = sv[:, k * 128:(k + 1) * 128].T
        x_copy.wait()

        def ln0_body(i, _):
            r = pl.multiple_of(i * 64, 64)
            h2buf[pl.ds(r, 64), :] = _ln(xbuf[pl.ds(r, 64), :].astype(f32))
            return 0
        lax.fori_loop(0, NPRE // 64, ln0_body, 0)

        def mod0_body(j, _):
            pltpu.make_async_copy(wmodb.at[j], wmodb.at[j], sems.at[SMOD + j]).wait()
            accs = [jnp.zeros((8, 512), f32)] * 2
            for k in range(64):
                accs[k % 2] = mod_rows(accs[k % 2], wmodb[j, k * 16:(k + 1) * 16, :], k * 16)
            mod_finish(accs[0] + accs[1], j)
            return 0
        _loop("mod0", 0, 4, mod0_body)

        def hpre_body(i, _):
            r = pl.multiple_of(i * 32, 32)
            hv = h2buf[pl.ds(r, 32), :] * modrows(1, 32) + modrows(0, 32)
            ro = pl.multiple_of(i * 8, 8)
            for t, op in enumerate(row_operands(hv)):
                h7[t, pl.ds(ro, 8), :] = pltpu.bitcast(op.astype(bf16), u32)
            return 0
        lax.fori_loop(0, NPRE // 32, hpre_body, 0)
        lhs_h[MEM:32, :] = adaln_a(xbuf[NPRE:NPRE + RIDE, :].astype(f32)).astype(bf16)

        def relayout_now(g, dh):
            def rl_body(t, _):
                relayout(g, 2 * g + dh, dh, t * 32, 32)
                return 0
            lax.fori_loop(0, 8, rl_body, 0)

        for dh in range(2):
            stg_wait(dh, 1, dh)
            relayout_now(0, dh)

        grp = lambda g: [piece_copy(g, 0), piece_copy(g, 1)]
        issue = {0: [wo_copy(0)], 1: grp(3) + grp(4), 2: grp(5) + [wo_copy(1), mod_copy(4)],
                 3: grp(6) + [mod_copy(5), mod_copy(6)], 4: grp(7) + [wo_copy(2)],
                 5: grp(8) + [wo_copy(3), mod_copy(7)], 6: grp(9) + [wo_copy(4)],
                 7: grp(10) + [wo_copy(5), mod_copy(8)], 8: grp(11) + [wo_copy(6)],
                 9: [wo_copy(7), mod_copy(9)], 10: stream_copies(0)}

        def pre_iter(g, carry):
            m3, gbase = carry

            @pl.when(g == 1)
            def _():
                stg_wait(2, 2, 2)
                relayout_now(1, 0)
                relayout_now(1, 1)

            def slots():
                m3n = jnp.where(m3 == 2, 0, m3 + 1)
                cj = jnp.maximum(g - 2, 3)
                return (m3n, 2 * jnp.where(ends, m3, m3n),
                        jnp.where(jnp.logical_or(g < 4, m3 == 0), 2, m3 - 1),
                        cj, jnp.where(cj >= NMOD, cj - NMOD, cj))

            ends = jnp.logical_or(g == 0, g == NGRP - 1)

            @pl.when(jnp.logical_not(ends))
            def _():
                stg_wait(slots()[1], 2, g + 2)

            @pl.when(g >= 4)
            def _():
                buf = wos.at[slots()[2]]
                pltpu.make_async_copy(buf, buf, sems.at[SSTG + g + 2]).wait()

            @pl.when(g >= 6)
            def _():
                buf = wmodb.at[slots()[4]]
                pltpu.make_async_copy(buf, buf, sems.at[SSTG + g + 2]).wait()

            m3n, gslot, wslot, cj, cslot = slots()
            gn = jnp.where(ends, g, g + 1)
            wrow = WO + jnp.maximum(g - 4, 0) * 256
            for k, cps in issue.items():
                @pl.when(g == k)
                def _():
                    for cp in cps:
                        cp.start()
            wtodo = [(r, c) for r in range(16) for c in range(8)]
            todo = [(dh, dp) for dh in range(2) for dp in range(256)]
            skip = [0] * RSK
            mtodo = list(range(0, D, 16))
            macc = [jnp.zeros((8, 512), f32)]

            def hook(v):
                if mtodo:
                    acc = macc[0] + jnp.concatenate([_zero_after(v)] * 4, axis=1)
                    for r in mtodo[:3]:
                        acc = mod_rows(acc, wmodb[cslot, r:r + 16, :], r)
                    del mtodo[:3]
                    macc[0] = acc

            for q in range(4):
                def b_of(k):
                    w = b_operand(gbase, q, k)
                    if skip:
                        skip.pop()
                        return w
                    nw = 0 if todo else WLP
                    for dh, dp in todo[:RLP]:
                        relayout(gn, gslot + dh, dh, dp, 1)
                    del todo[:RLP]
                    for r, c in wtodo[:nw]:
                        wqkv[pl.ds(wrow + (c * 2048 + r * 16), 16), :] = pltpu.bitcast(
                            wos[wslot, r * 32:(r + 1) * 32, c * 128:(c + 1) * 128], u32)
                    del wtodo[:nw]
                    return w
                c11, c12, c21, c22 = _strassen(lambda k: pltpu.bitcast(h7[k], bf16), b_of, hook)
                for blk, y in ((q + 4, _merge_rows(c12, c22)), (q, _merge_rows(c11, c21))):
                    for e in range(NPRE // 8):
                        pos = ((8 * e + ROFF) % NR) // 2
                        rings[blk][g, pos:pos + 4, :] = _pack8(y[8 * e:8 * e + 8])
            assert not todo and not wtodo and not mtodo
            mod_finish(macc[0], cj)
            return m3n, gbase + 8 * WP

        _loop("pre1", 0, NGRP, pre_iter, (0, 0))

    pl.run_scoped(prologue,
                  pltpu.VMEM((NSLOT, 512, 8, 128), bf16),
                  pltpu.VMEM((NWO, 512, D), bf16),
                  pltpu.VMEM((NMOD, D, 512), bf16),
                  pltpu.VMEM((7, NPRE // 4, 512), u32))

    def main(w7, w49):
        scale = DH ** -0.5
        ia = lax.broadcasted_iota(jnp.int32, (32, L), 0)
        ja = lax.broadcasted_iota(jnp.int32, (32, L), 1)
        mask_a = ((ia >= 16) & (ia < 24)) | (ja >= SEG) | (jnp.where(ia < 16, ia + 8, ia) >= ja)
        ib = lax.broadcasted_iota(jnp.int32, (48, 56), 0)
        jb = lax.broadcasted_iota(jnp.int32, (48, 56), 1)
        own = (ib < 40) == (jb < 40)
        mask_b = own & (((jb >= 32) & (jb < 48)) | (jnp.where(jb < 40, jb, jb - 8) <= ib))
        masked = -1e9 / scale
        j8 = lax.broadcasted_iota(jnp.int32, (8, 56), 1)
        fill_b = jnp.concatenate([jnp.where(j8 < 40, masked, -3e38).astype(f32)] * 5
                                 + [jnp.where(j8 < 40, -3e38, masked).astype(f32)], axis=0)

        def softmax(sc, mask, fill):
            sc = jnp.where(mask, sc, fill)
            mx = jnp.max(sc, axis=-1, keepdims=True)
            e = jnp.exp2((sc - mx) * (scale * 1.4426950408889634))
            den = jnp.sum(e, axis=-1, keepdims=True)
            return (e * pl.reciprocal(den, approx=True)).astype(bf16)

        def ride_rows(s, is_b):
            first = s < 2
            if is_b:
                g = [jnp.where(first, -3, -1), 1, 2]
            else:
                g = [jnp.where(first, 1, 0), jnp.where(first, 2, 1), 3]
            return [RIDE * s + 8 * t for t in g]

        def step(s, is_b, lhs_lo, lhs_hi, soft_in, jobs):
            seg = ((SEG * s + ROFF) // 2) % (NR // 2)
            sega = seg - SEG // 2
            wr = [((NPRE + RIDE * s + 8 * t + ROFF) // 2) % (NR // 2) for t in range(3)]
            rd = [((r + ROFF) // 2) % (NR // 2) for r in ride_rows(s, is_b)]
            lhs = jnp.concatenate([lhs_lo, lhs_hi], axis=1)
            QM, P, PART = {}, {}, {}
            mrow = 0 if is_b else 4

            def wblk(b, lo, n):
                return pltpu.bitcast(wqkv[b * WP + lo:b * WP + lo + n, :], bf16)

            def qkv_lo(i):
                for m in range(3):
                    PART[(m, i)] = jnp.dot(lhs_lo, wblk(m * H + i, 0, 256), preferred_element_type=f32)

            def qkv(i):
                for m in range(3):
                    b = m * H + i
                    if (m, i) in PART:
                        y = jnp.dot(lhs_hi, wblk(b, 256, 256),
                                    preferred_element_type=f32) + PART.pop((m, i))
                    else:
                        y = jnp.dot(lhs, wblk(b, 0, 512), preferred_element_type=f32)
                    if m < 2:
                        QM[b] = y[0:MEM] + jobs["pin"] if b == PIN and is_b else y[0:MEM]
                    if m == 2 or (m == 1 and not is_b):
                        kvm[b - H, mrow:mrow + 4, :] = _pack8(y[0:MEM])
                    for t in range(3):
                        rset(b, wr[t], y[8 + 8 * t:16 + 8 * t])
                    for job in jobs.get(3 * i + m, []):
                        job(y)
                    side(3 * i + m)

            def keys(b):
                if is_b:
                    if b in QM:
                        mix = jnp.concatenate([_pack8(QM.pop(b)), kvm[b - H, 4:8, :]], axis=0)
                    else:
                        mix = kvm[b - H]
                    return _unpack(jnp.concatenate([rget(b, seg, 16), mix, rget(b, sega, 4)], axis=0))
                mk = _pack8(QM.pop(b)) if b in QM else kvm[b - H, 4:8, :]
                return _unpack(jnp.concatenate([rget(b, seg, 16), mk], axis=0))

            def scores(i):
                if is_b:
                    q = [rget(i, seg, 16), _pack8(QM.pop(i)), rget(i, sega, 4)]
                else:
                    q = [rget(i, seg + 4, 8), _pack8(QM.pop(i)), rget(i, seg + 12, 4)]
                sc = lax.dot_general(_unpack(jnp.concatenate(q, axis=0)), keys(H + i),
                                     (((1,), (1,)), ((), ())), preferred_element_type=f32)
                P[i] = softmax(sc, mask_b, fill_b) if is_b else softmax(sc, mask_a, masked)

            def pv(i):
                o = jnp.dot(P.pop(i), keys(2 * H + i), preferred_element_type=f32)
                if is_b:
                    rset(i, seg, o[0:SEG])
                    rset(i, sega, o[40:48])
                    lhs_o[i, 0:4, :] = _pack8(o[SEG:L])
                    lhs_o[i, 4:8, :] = rget(i, rd[0], 4)
                    lhs_o[i, 8:16, :] = rget(i, rd[1], 8)
                else:
                    rset(i, seg + 4, o[0:16])
                    rset(i, seg + 12, o[24:32])
                    lhs_o[i, 0:4, :] = _pack8(o[16:24])
                    lhs_o[i, 4:12, :] = rget(i, rd[0], 8)
                    lhs_o[i, 12:16, :] = rget(i, rd[2], 4)

            def wo_lhs(i0, i1):
                return _unpack(jnp.concatenate([lhs_o[i] for i in range(i0, i1)], axis=1))

            def wo_dot(lo, j, i0, i1):
                r = WO + j * 2048
                w = pltpu.bitcast(wqkv[r + 64 * i0:r + 64 * i1, :], bf16)
                return jnp.dot(lo, w, preferred_element_type=f32)

            def side(d):
                ds, dp = (DSB, DPB) if is_b else (DSA, DPA)
                if (d - dp) % 3 == 2 and 0 <= (d - dp) // 3 < H:
                    pv((d - dp) // 3)
                if (d - ds) % 3 == 2 and 0 <= (d - ds) // 3 < H:
                    scores((d - ds) // 3)

            if soft_in:
                for h in range(KSPLIT):
                    qkv_lo(h)
            for h in range(H):
                qkv(h)
            lo = [wo_lhs(8 * k, 8 * k + 8) for k in range(3)]
            acc = []
            for j in range(8):
                y = None
                for k in range(3):
                    z = wo_dot(lo[k], j, 8 * k, 8 * k + 8)
                    y = z if y is None else z + y
                    for job in jobs.get(96 + 3 * j + k, []):
                        job(y)
                    side(96 + 3 * j + k)
                acc.append(y)
            lo = wo_lhs(24, H)
            for j in range(8):
                acc[j] = wo_dot(lo, j, 24, H) + acc[j]
                for job in jobs.get(120 + j, []):
                    job(acc[j])
            assert not (QM or P or PART)
            return jnp.concatenate(acc[0:4], axis=1), jnp.concatenate(acc[4:8], axis=1)

        def combine(c, n, y):
            mp, k1 = divmod(n, 8)
            m, p = divmod(mp, 4)
            c3 = jnp.minimum(c, 27)
            spare = pl.ds(pl.multiple_of(8 * (c // 64), 8), 8)
            if m == 0 and k1 < 7:
                ws3[16, spare, :] = y.astype(bf16)
            else:
                wsr[7, spare, 0:128] = y.astype(bf16)
            if k1 == 7:
                dst, base, r = w7, 0, (4 * m + p) * 256 + c * 8
                blk = [wsr[4 + i, m * 16:(m + 1) * 16, j * 512 + p * 128:j * 512 + (p + 1) * 128]
                       .astype(f32) for i in range(2) for j in range(2)]
            else:
                dst, base = w49, 7 * k1
                if m == 0:
                    r = c3 * 32 + p * 8
                    get = lambda i, j: ws3[4 * i + j, p * 16:(p + 1) * 16, :]
                else:
                    r = W4R + (p // 2) * 448 + c3 * 16 + (p % 2) * 8
                    r0, c0 = (p % 2) * 16, (p // 2) * 128
                    get = lambda i, j: wsr[i, r0:r0 + 16, j * 256 + c0:j * 256 + c0 + 128]

                def quad(q):
                    return [get(2 * (q // 2) + i, 2 * (q % 2) + j).astype(f32)
                            for i in range(2) for j in range(2)]
                qi, qj, sign = _BTERMS[k1]
                blk = quad(qi)
                if qj is not None:
                    blk = [u + v if sign > 0 else u - v for u, v in zip(blk, quad(qj))]
            for k, op in enumerate(_b_operands(*blk)):
                for e in range(2):
                    dst[base + k, pl.ds(r + 4 * e, 4), :] = _pack8(op[8 * e:8 * e + 8])

        def rec_body(it, gacc):
            stream_wait(it)
            lhs_lo = lhs_h[:, 0:512]
            lhs_hi = lhs_h[:, 512:1024]
            ra = jnp.maximum(it - 1, 0) * (2 * RIDE)
            for u in range(2):
                s = 2 * it + u
                jobs = {}
                for n, (su, d, g) in enumerate(SLOTS):
                    if su == u:
                        jobs.setdefault(d, []).append(
                            lambda y, n=n, g=g: combine(it, n, y[8 * g:8 * g + 8]))
                r1 = pl.multiple_of(jnp.minimum(NPRE + RIDE * (s + 1), S - RIDE), 8)
                xn = xbuf[pl.ds(r1, RIDE), :].astype(f32)
                if u == 0:
                    for k in range(2):
                        rm = pl.multiple_of(it * 32 + k * 16, 16)
                        gacc = mod_rows(gacc, wsr[6, k * 16:(k + 1) * 16, :], rm)
                    hn = adaln_a(xn, _zero_after(stage_a16(ra)))
                else:
                    def refill(y):
                        for cp in stream_copies(jnp.minimum(it + 1, NSEG // 2 - 1)):
                            cp.start()
                        spare = pl.ds(pl.multiple_of(8 * (it // 64), 8), 8)
                        jobs["pin"] = _zero_after(ws3[16, spare, :].astype(f32))
                    jobs.setdefault(3 * (PIN - 4) + 2, []).append(refill)
                    hn = adaln_a(xn)
                    z = _zero_after(hn[0:8], hn[8:16], hn[16:24])
                    stage_a16(ra + 32, _zero_after(stage_a16(ra + 16, z)))
                a_lo, a_hi = step(s, u == 1, lhs_lo, lhs_hi, u > 0, jobs)
                lhs_lo = jnp.concatenate([a_lo[0:MEM], hn[:, 0:512]], axis=0).astype(bf16)
                lhs_hi = jnp.concatenate([a_hi[0:MEM], hn[:, 512:1024]], axis=0).astype(bf16)
                a = jnp.concatenate([a_lo, a_hi], axis=1)
                rows = [pl.multiple_of(r, 8) for r in ride_rows(s, u == 1)]
                xs = [xbuf[pl.ds(r, 8), :].astype(f32) for r in rows]
                for t, r in enumerate(rows):
                    xa = xs[t] + modrows(2, 8) * a[8 + 8 * t:16 + 8 * t]
                    xbuf[pl.ds(r, 8), :] = xa.astype(bf16)
            lhs_h[:, 0:512] = lhs_lo
            lhs_h[:, 512:1024] = lhs_hi
            return gacc

        gacc = _loop("rec", 0, NSEG // 2, rec_body, jnp.zeros((8, D), f32))
        for c in range(2):
            mod_finish(gacc[:, c * 512:(c + 1) * 512], 10 + c)
        stream_wait(NSEG // 2 - 1)

        def wo_prep(i, half, k):
            o = jnp.concatenate([_unpack(rings[4 * half + h][i, k * 8:(k + 1) * 8, :]).astype(f32)
                                 for h in range(4)], axis=1)
            for t, op in enumerate(row_operands(o)):
                a7[half, t, k * 8:(k + 1) * 8, :] = op.astype(bf16)

        def wo_chunk(i, half, inext, extra):
            row = pl.multiple_of(i * 512 + half * 256, 256)
            todo = list(range(NPRE // 16))
            spare = pl.ds(pl.multiple_of(8 * (i // 64), 8), 8)

            def hook(v):
                if todo:
                    for h in range(4):
                        rings[4 * (1 - half) + h][4, spare, :] = pltpu.bitcast(v[0:8], u32)
                    n = 2 if len(todo) % WPP == 0 else 1
                    for k in todo[:n]:
                        wo_prep(inext, 1 - half, k)
                    del todo[:n]
                extra(v)

            for j in range(4):
                def b_of(k):
                    def quad(q):
                        r = WO + (j + 4 * (q % 2)) * 2048 + (q // 2) * 128 + row
                        return pltpu.bitcast(wqkv[pl.ds(r, 128), :], bf16)
                    qi, qj, sign = _BTERMS[k]
                    if qj is None:
                        return quad(qi)
                    u, v = quad(qi).astype(f32), quad(qj).astype(f32)
                    return (u + v if sign > 0 else u - v).astype(bf16)
                c11, c12, c21, c22 = _strassen(lambda k: a7[half, k], b_of, hook)
                for c, y in ((j + 4, _merge_rows(c12, c22)), (j, _merge_rows(c11, c21))):
                    cs = slice(c * 128, (c + 1) * 128)
                    h2buf[S - NPRE:S, cs] = h2buf[S - NPRE:S, cs] + y

        for k in range(NPRE // 16):
            wo_prep(0, 0, k)

        def wo_tail(i, _):
            st = {"n": 0, "prev": None}

            def extra(v):
                n = st["n"]
                st["n"] += 1
                if n % 16 == 2 and n // 16 < 3:
                    st["prev"] = stage_a16(S - NPRE - 48 + 16 * (n // 16),
                                           _zero_after(v, st["prev"]))
            wo_chunk(i, 0, i, extra)
            wo_chunk(i, 1, jnp.minimum(i + 1, 3), extra)
            return 0
        _loop("wotail", 0, 4, wo_tail)

        def gget(c, row, n):
            return pltpu.bitcast(wqkv[pl.ds(c * GS + row, n), :], f32)

        def gset(c, row, val):
            wqkv[pl.ds(c * GS + row, val.shape[0]), :] = pltpu.bitcast(val, u32)

        def wop(j):
            return lambda k: pltpu.bitcast(w7[k, j * 256:(j + 1) * 256, :], bf16)

        zpad = jnp.zeros((GPAD, 128), f32)
        for cb in range(8):
            gset(cb, 0, zpad)
            gset(cb, GPAD + S, zpad)

        shifts = (-1, -1, 1, 1, -2, -2, 2, 2)
        HB = MB // 2

        def shift_piece(r, half, k):
            gs = jnp.concatenate([gget(c, r + (k * 16 + GPAD + shifts[c]), 16)
                                  for c in range(8)], axis=1)
            ro = half * (HB // 2) + k * 8
            for t, op in enumerate(row_operands(gs)):
                n7[t, ro:ro + 8, :] = op.astype(bf16)

        def gate(v, i):
            gset(0, GPAD + S + GPAD + 8 * (i // S), v[0:8])

        def b_body(i, _):
            rl = S - NPRE + i * 128
            st = {"n": 0, "prev": [None, None]}

            def hook(v):
                n = st["n"]
                st["n"] += 1
                if n % BG == 0 and n // BG < 8:
                    k = n // BG
                    st["prev"][k % BCH] = stage_a16(rl + 16 * k,
                                                    _zero_after(v, st["prev"][k % BCH]),
                                                    (t7, 8 * k))

            ro = pl.multiple_of(i * 192, 64)
            for lhs, row in ((lambda k: n7[k, pl.ds(ro, 192), :], i * 384), (lambda k: t7[k], rl)):
                rg = pl.multiple_of(GPAD + row, 8)
                for j in range(4):
                    c11, c12, c21, c22 = _strassen(lhs, wop(j), hook)
                    gset(j + 4, rg, _gelu(_merge_rows(c12, c22)))
                    gset(j, rg, _gelu(_merge_rows(c11, c21)))
            return 0
        _loop("b", 0, S // MB, b_body)
        for k in range(HB // 16):
            shift_piece(0, 0, k)

        def n2_norm(r, k, anchor):
            v = _ln(h2buf[pl.ds(pl.multiple_of(r + k * 16, 16), 16), :], anchor)
            nrms[k // 2][(k % 2) * 16:(k % 2) * 16 + 16, :] = v
            return v[0:8] + v[8:16]

        def n2_ops(k, k1, v, i):
            nrm = nrms[k]
            nrm[pl.ds(pl.multiple_of(32 + 8 * (i // S), 8), 8), 0:128] = v[0:8]

            def quad(q):
                r0, c0 = (q // 2) * 16, (q % 2) * 512
                return [nrm[r0 + 8 * a:r0 + 8 * a + 8, c0 + 256 * b:c0 + 256 * b + 256]
                        for a in range(2) for b in range(2)]
            qi, qj, sign = _ATERMS[k1]
            blk = quad(qi)
            if qj is not None:
                blk = [u + w if sign > 0 else u - w for u, w in zip(blk, quad(qj))]
            for k2, op in enumerate(_a_operands(*blk)):
                d49[7 * k1 + k2, k * 8:(k + 1) * 8, :] = op.astype(bf16)

        def n2_hook(r, i, first, gap, lag, st):
            def hook(v):
                n = st["n"] - first
                st["n"] += 1
                if n >= 0 and n % gap == 0 and n // gap < MD // 16:
                    st["prev"] = n2_norm(r, n // gap, _zero_after(v, st["prev"]))
                for _ in range(st["per"]):
                    k, k1 = divmod(st["ops"], 7)
                    if k < MD // 32 and n >= (2 * k + 1) * gap + lag:
                        n2_ops(k, k1, v, i)
                        st["ops"] += 1
            return hook

        def stage_c(i, r, half, rnext, extra):
            rr = pl.multiple_of(r, 8)
            ro = half * (HB // 2)
            cnt = [0]

            def hook(v):
                n = cnt[0]
                cnt[0] += 1
                if n < HB // 16:
                    gate(v, i)
                    shift_piece(rnext, 1 - half, n)
                extra(v)

            for j in range(4):
                c11, c12, c21, c22 = _strassen(lambda k: n7[k, ro:ro + HB // 2, :], wop(4 + j),
                                               hook)
                for c, y in ((j + 4, _merge_rows(c12, c22)), (j, _merge_rows(c11, c21))):
                    cs = slice(c * 128, (c + 1) * 128)
                    h2buf[pl.ds(rr, HB), cs] = h2buf[pl.ds(rr, HB), cs] + y

        def c_body(i, _):
            r = pl.multiple_of(i * MB, MB)
            st = {"n": 0, "prev": None, "ops": 0, "per": 1}
            extra = n2_hook(0, i, 0, 4, 4, st)
            stage_c(i, r, 0, r + HB, extra)
            stage_c(i, r + HB, 1, jnp.minimum(i + 1, S // MB - 1) * MB, extra)
            assert st["ops"] == 28
            return 0
        _loop("c", 0, S // MB, c_body)

        def wop2(lo, n):
            return lambda k1, k: pltpu.bitcast(w49[7 * k1 + k, lo:lo + n, :], bf16)

        def d_body(i, _):
            r = pl.multiple_of(i * MD, MD)
            rn = jnp.minimum(r + MD, S - MD)
            lhs = [d49[k] for k in range(49)]
            uops = []
            for t in range(7):
                cb = _strassen2(lambda k1, k: lhs[7 * k1 + k], wop2(t * 128, 128))
                uops.append(_a_operands2([[_gelu(c) for c in row] for row in cb]))
            ul = [[jnp.concatenate([u[k1][k] for u in uops], axis=1).astype(bf16)
                   for k in range(7)] for k1 in range(7)]
            st = {"n": 0, "prev": None, "ops": 0, "per": 1}
            hook = n2_hook(rn, i, DF, DG, DL, st)
            for t in range(2):
                cb = _strassen2(lambda k1, k: ul[k1][k], wop2(W4R + t * 448, 448), hook)
                for j in range(4):
                    y = jnp.concatenate([cb[q][j].reshape(MD // 32, 8, 128) for q in range(4)],
                                        axis=1).reshape(MD, 128)
                    c = 2 * j + t
                    cs = slice(c * 128, (c + 1) * 128)
                    gb = modrows(5, MD, c * 128, (c + 1) * 128)
                    o = xbuf[pl.ds(r, MD), cs].astype(f32) + gb * (h2buf[pl.ds(r, MD), cs] + y)
                    xbuf[pl.ds(r, MD), cs] = o.astype(bf16)
            assert st["ops"] == 28
            out_copy(r, MD).start()
            return 0
        _loop("d", 0, S // MD, d_body)

    pl.run_scoped(main,
                  pltpu.VMEM((7, 8 * 256, 128), u32),
                  pltpu.VMEM((49, 2 * W4R, 128), u32))

    out_copy(0, S).wait()


def _run(x, mem0, wq, wk, wv, wo, w1, w2, w3, w4, c, wmod):
    any_spec = pl.BlockSpec(memory_space=pl.ANY)
    return pl.pallas_call(
        _kernel,
        out_shape=jax.ShapeDtypeStruct((S, D), bf16),
        in_specs=[any_spec] * 12,
        out_specs=any_spec,
        scratch_shapes=[
            pltpu.VMEM((S + 2 * RIDE, D), bf16),
            pltpu.VMEM((WO + 8 * 2048, 128), u32),
            [pltpu.VMEM((96 // NRING, NR // 2, 128), u32)] * NRING,
            pltpu.VMEM((32, D), bf16),
            pltpu.VMEM((H, 16, 128), u32),
            pltpu.VMEM((2 * H, 8, 128), u32),
            pltpu.VMEM((12, 8, 512), f32),
            pltpu.VMEM((D, 128), f32),
            pltpu.VMEM((S, D), f32),
            pltpu.VMEM((7, (S - NPRE) // 2, 512), bf16),
            pltpu.VMEM((17, 64, 128), bf16),
            pltpu.VMEM((8, 32, D), bf16),
            pltpu.VMEM((7, 64, 512), bf16),
            pltpu.VMEM((2, 7, NPRE // 2, 256), bf16),
            pltpu.VMEM((49, MD // 4, 256), bf16),
            [pltpu.VMEM((40, D), f32)] * (MD // 32),
            pltpu.VMEM((1, D), bf16),
            pltpu.SemaphoreType.DMA((9 + NGRP + 2,)),
        ],
        compiler_params=pltpu.CompilerParams(vmem_limit_bytes=124 * 1024 * 1024,
                                             disable_bounds_checks=True,
                                             disable_semaphore_checks=True),
    )(x, mem0, wq, wk, wv, wo, w1, w2, w3, w4, c, wmod)


def pallas_adaLN_cond__memory_aug_recurrent_mem_tr__mixer_s_mlp__prompt_kernel(
    A_x, A_mem0, A_Wq, A_Wk, A_Wv, A_Wo, A_seg_len, B_x, B_w1, B_w2, B_w3, B_w4, c, w_mod,
):
    del B_x
    assert A_x.shape == (1, S, D) and A_mem0.shape == (1, MEM, D)
    assert isinstance(A_seg_len, int) is False or A_seg_len == SEG
    out = _run(A_x.reshape(S, D), A_mem0.reshape(MEM, D), A_Wq, A_Wk, A_Wv,
               A_Wo.reshape(H * DH, D),
               B_w1.reshape(2, D // 2, D), B_w2.reshape(2, D // 2, D),
               B_w3, B_w4.reshape(4, F // 4, D), c, w_mod)
    return out.reshape(1, S, D)
```

```python
import jax
import jax.numpy as jnp
from jax import lax
import jax.experimental.pallas as pl
import jax.experimental.pallas.tpu as pltpu

bf16 = jnp.bfloat16
f32 = jnp.float32
u32 = jnp.uint32

S = 2048
D = 1024
H = 32
DH = 128
F = 3584
MEM = 8
SEG = 32
NSEG = S // SEG
L = MEM + SEG
RIDE = 24
NPRE = S - RIDE * NSEG
NR = NPRE + 2 * SEG
ROFF = (-(S - NPRE)) % NR
WP = 516
WO = 96 * WP
NGRP = 12
NSLOT = 6
NMOD = 6
EPS = 1e-5
MD = 128
MB = 512
GPAD = 8
NRING = 8
RLP, WLP, RSK = 27, 22, 2
NWO = 3
BG, WPP, PIN, BCH = 2, 5, 6, 2
DF, DG, DL = 2, 10, 9
SLOTS = ([(0, n // 2, 3 * (n % 2)) for n in range(16)] + [(0, 96 + n, 0) for n in range(16)]
         + [(0, 112 + n // 2, 3 * (n % 2)) for n in range(32)])
DSA, DPA, DSB, DPB, KSPLIT = 6, 12, 6, 12, 2
X0 = NPRE + 2 * RIDE
GS = S + 4 * GPAD
W4T = 7 * 16
_ONLY = None


def _loop(name, lo, hi, body, init=0):
    if _ONLY is not None and name not in _ONLY:
        return init
    with _scope(name):
        return lax.fori_loop(lo, hi, body, init)


class _NoScope:
    def __init__(self, name):
        del name

    def __enter__(self):
        return self

    def __exit__(self, *a):
        return False


_scope = _NoScope


def _zero_after(*vs):
    bits = None
    for v in vs:
        if v is not None:
            b = pltpu.bitcast(v[0:8, 0:128], u32)
            bits = b if bits is None else bits | b
    return pltpu.bitcast((bits >> 31) >> 1, f32)


def _ln(x, anchor=None):
    if anchor is not None:
        z = jnp.concatenate([anchor] * (x.shape[0] // 8), axis=0)
        x = jnp.concatenate([x[:, 0:128] + z, x[:, 128:]], axis=1)
    mu = jnp.mean(x, axis=-1, keepdims=True)
    xc = x - mu
    var = jnp.mean(xc * xc, axis=-1, keepdims=True)
    return xc * lax.rsqrt(var + EPS)


def _gelu(x):
    inner = x * (0.7978845608028654 + (0.7978845608028654 * 0.044715) * (x * x))
    hx = 0.5 * x
    return hx + hx * jnp.tanh(inner)


def _split_rows(x):
    m, n = x.shape
    x3 = x.reshape(m // 16, 16, n)
    return x3[:, 0:8, :].reshape(m // 2, n), x3[:, 8:16, :].reshape(m // 2, n)


def _merge_rows(top, bot):
    m, n = top.shape
    return jnp.concatenate([top.reshape(m // 8, 8, n), bot.reshape(m // 8, 8, n)],
                           axis=1).reshape(2 * m, n)


def _a_operands(a11, a12, a21, a22):
    return [a11 + a22, a21 + a22, a11, a22, a11 + a12, a21 - a11, a12 - a22]


def _b_operands(b11, b12, b21, b22):
    return [b11 + b22, b11, b12 - b22, b21 - b11, b22, b11 + b12, b21 + b22]


_ATERMS = ((0, 3, 1), (2, 3, 1), (0, None, 0), (3, None, 0), (0, 1, 1), (2, 0, -1), (1, 3, -1))
_BTERMS = ((0, 3, 1), (0, None, 0), (1, 3, -1), (2, 0, -1), (3, None, 0), (0, 1, 1), (2, 3, 1))


def _strassen(a_of, b_of, hook=lambda v: None):
    def prod(k):
        return jnp.dot(a_of(k), b_of(k), preferred_element_type=f32)
    p5 = prod(4)
    hook(p5)
    p3 = prod(2)
    hook(p3)
    c12 = p3 + p5
    p4 = prod(3)
    hook(p4)
    c11 = p4 - p5
    p2 = prod(1)
    hook(p2)
    c21 = p2 + p4
    c22 = p3 - p2
    p1 = prod(0)
    hook(p1)
    c11 = prod(6) + (c11 + p1)
    hook(c11)
    c22 = prod(5) + (c22 + p1)
    hook(c22)
    return c11, c12, c21, c22


def _a_operands2(b):
    sub = [_a_operands(b[i][j], b[i][2 + j], b[2 + i][j], b[2 + i][2 + j])
           for i in range(2) for j in range(2)]
    return [_a_operands(*[t[k] for t in sub]) for k in range(7)]


def _strassen2(a_of, b_of, hook=lambda v: None):
    def prod(k1):
        return _strassen(lambda k: a_of(k1, k), lambda k: b_of(k1, k), hook)

    def add(x, y):
        return [p + q for p, q in zip(x, y)]

    def sub(x, y):
        return [p - q for p, q in zip(x, y)]
    p5 = prod(4)
    p3 = prod(2)
    c12 = add(p3, p5)
    p4 = prod(3)
    c11 = sub(p4, p5)
    p2 = prod(1)
    c21 = add(p2, p4)
    c22 = sub(p3, p2)
    p1 = prod(0)
    c11 = add(add(c11, p1), prod(6))
    c22 = add(add(c22, p1), prod(5))
    cq = (c11, c12, c21, c22)
    return [[cq[2 * (i // 2) + j // 2][2 * (i % 2) + j % 2] for j in range(4)] for i in range(4)]


def _pack8(v):
    return pltpu.bitcast(v.astype(bf16), u32)


def _unpack(w):
    return pltpu.bitcast(w, bf16)


def _kernel(x_hbm, mem0_hbm, wq_hbm, wk_hbm, wv_hbm, wo_hbm, w1_hbm, w2_hbm, w3_hbm, w4_hbm,
            c_hbm, wmod_hbm, out_hbm,
            xbuf, wqkv, rings, lhs_h, lhs_o, kvm, modv, scol, h2buf, n7, ws3, wsr, t7, a7, d49, nrms, c_ref,
            sems):
    w_hbms = (wq_hbm, wk_hbm, wv_hbm)
    SMOD, SSTG = 5, 9
    sem_x, sem_out, sem_w, sem_g, sem_r = (sems.at[k] for k in range(5))

    def rget(b, tile, n):
        return rings[b % NRING][b // NRING, pl.ds(tile, n)].reshape(8 * n, 128)

    def rhalf(b, tile, half):
        return rings[b % NRING][b // NRING, tile, 4 * half:4 * half + 4, :]

    def rset(b, tile, half, val):
        rings[b % NRING][b // NRING, tile, 4 * half:4 * half + 4, :] = _pack8(val)

    x_copy = pltpu.make_async_copy(x_hbm.at[pl.ds(0, X0), :], xbuf.at[pl.ds(0, X0), :], sem_x)

    def stream_copies(c):
        al, lo = ((lambda v, m: v), min) if isinstance(c, int) else (pl.multiple_of, jnp.minimum)
        c3 = lo(c, 27)
        cps = [pltpu.make_async_copy(
            w3_hbm.at[pl.ds(al(i * 256 + (c3 % 4) * 64, 64), 64),
                      pl.ds(al(j * (F // 4) + (c3 // 4) * 128, 128), 128)],
            ws3.at[4 * i + j], sem_w) for i in range(4) for j in range(4)]
        dst = X0 + 2 * RIDE * c
        return [
            pltpu.make_async_copy(w4_hbm.at[:, pl.ds(al(c3 * 32, 32), 32), :],
                                  wsr.at[pl.ds(0, 4)], sem_g),
            pltpu.make_async_copy(w1_hbm.at[:, pl.ds(al(c * 16, 16), 16), :],
                                  wsr.at[pl.ds(4, 2), pl.ds(0, 16), :], sem_g),
            pltpu.make_async_copy(w2_hbm.at[:, pl.ds(al(c * 16, 16), 16), :],
                                  wsr.at[pl.ds(4, 2), pl.ds(16, 16), :], sem_g),
            pltpu.make_async_copy(wmod_hbm.at[pl.ds(al(c * 32, 32), 32), pl.ds(5 * D, D)],
                                  wsr.at[6], sem_g),
            pltpu.make_async_copy(x_hbm.at[pl.ds(al(lo(dst, S - 2 * RIDE), 16), 2 * RIDE), :],
                                  xbuf.at[pl.ds(al(dst, 16), 2 * RIDE), :], sem_r)] + cps

    def stream_wait(c):
        for dst, sem in ((ws3.at[pl.ds(0, 16)], sem_w), (wsr.at[pl.ds(0, 7)], sem_g),
                         (xbuf.at[pl.ds(X0 + 2 * RIDE * c, 2 * RIDE), :], sem_r)):
            pltpu.make_async_copy(dst, dst, sem).wait()

    def out_copy(row, n):
        return pltpu.make_async_copy(xbuf.at[pl.ds(row, n), :], out_hbm.at[pl.ds(row, n), :],
                                     sem_out)

    def mod_rows(acc, w, r):
        sc = jnp.concatenate([scol[pl.ds(r, 16), :]] * (w.shape[1] // 128), axis=1)
        p = w.astype(f32) * sc
        return acc + p[0:8] + p[8:16]

    def mod_finish(acc, j):
        is_scale = jnp.logical_or(j // 2 == 1, j // 2 == 4)
        tot = jnp.sum(acc, axis=0, keepdims=True) + jnp.where(is_scale, 1.0, 0.0)
        modv[j] = jnp.broadcast_to(tot, (8, 512))

    def modrows(k, n, lo=0, hi=D):
        m = jnp.concatenate([modv[2 * k], modv[2 * k + 1]], axis=1)[:, lo:hi]
        return jnp.concatenate([m] * (n // 8), axis=0)

    def adaln_a(xv, anchor=None):
        n = xv.shape[0]
        return _ln(xv, anchor) * modrows(1, n) + modrows(0, n)

    def adaln_b(xv, anchor=None):
        n = xv.shape[0]
        return _ln(xv, anchor) * modrows(4, n) + modrows(3, n)

    def row_operands(v):
        top, bot = _split_rows(v)
        k = v.shape[1] // 2
        return _a_operands(top[:, :k], top[:, k:], bot[:, :k], bot[:, k:])

    def stage_a16(r, anchor=None, dst=None):
        rr = pl.multiple_of(r, 16)
        xv = xbuf[pl.ds(rr, 16), :]
        if dst is not None:
            xv = (xv.astype(f32) + modrows(2, 16) * h2buf[pl.ds(rr, 16), :]).astype(bf16)
            xbuf[pl.ds(rr, 16), :] = xv
        h2 = adaln_b(xv.astype(f32), anchor)
        h2buf[pl.ds(rr, 16), :] = h2
        ref, ro = (n7, pl.multiple_of(rr // 2, 8)) if dst is None else dst
        ops = row_operands(_ln(h2))
        for t, op in enumerate(ops):
            ref[t, pl.ds(ro, 8), :] = op.astype(bf16)
        return ops[0]

    def prologue(stg, wos, wmodb, h7):
        def mod_copy(j):
            return pltpu.make_async_copy(wmod_hbm.at[:, pl.ds(j * 512, 512)], wmodb.at[j % NMOD],
                                         sems.at[SSTG + j + 4 if j >= 4 else SMOD + j])

        def piece_copy(g, dh):
            return pltpu.make_async_copy(
                w_hbms[g // 4].at[pl.ds(dh * 512, 512), pl.ds((g % 4) * 8, 8), :],
                stg.at[(2 * g + dh) % NSLOT], sems.at[SSTG + (g + 1 if g else dh)])

        def wo_copy(j):
            return pltpu.make_async_copy(wo_hbm.at[pl.ds(j * 512, 512), :], wos.at[j % NWO],
                                         sems.at[SSTG + j + 6])

        def group_start(g):
            for dh in range(2):
                piece_copy(g, dh).start()

        def stg_wait(slot, n, sem):
            dst = stg.at[pl.ds(slot, n)]
            pltpu.make_async_copy(dst, dst, sems.at[SSTG + sem]).wait()

        def relayout(g, slot, dh, lo_dp, n_dp):
            base = g * (8 * WP) + dh * 256
            for u in range(n_dp):
                dp = lo_dp + u
                ev = pltpu.bitcast(stg[slot, 2 * dp].astype(f32), u32)
                od = pltpu.bitcast(stg[slot, 2 * dp + 1].astype(f32), u32)
                wqkv[pl.ds(base + dp, 8, stride=WP), :] = (ev >> 16) | od

        def b_operand(gbase, q, k):
            def quad(i):
                r = gbase + ((q + 4 * (i % 2)) * WP + (i // 2) * 256)
                return pltpu.bitcast(wqkv[pl.ds(r, 256), :], bf16)
            i, j, sign = _BTERMS[k]
            if j is None:
                return quad(i)
            u, v = quad(i).astype(f32), quad(j).astype(f32)
            return (u + v if sign > 0 else u - v).astype(bf16)

        c_copy = pltpu.make_async_copy(c_hbm, c_ref, sem_g)
        m_copy = pltpu.make_async_copy(mem0_hbm, lhs_h.at[pl.ds(0, MEM), :], sem_r)
        c_copy.start()
        m_copy.start()
        x_copy.start()
        for j in range(4):
            mod_copy(j).start()
        for g in range(3):
            group_start(g)
        h2buf[S - NPRE:S, :] = jnp.zeros((NPRE, D), f32)
        wos[2] = jnp.zeros((512, D), bf16)
        c_copy.wait()
        m_copy.wait()
        cv = c_ref[...].astype(f32)
        sv = jnp.broadcast_to(cv * (1.0 / (1.0 + jnp.exp(-cv))), (128, D))
        for k in range(8):
            scol[k * 128:(k + 1) * 128, :] = sv[:, k * 128:(k + 1) * 128].T
        x_copy.wait()

        def ln0_body(i, _):
            r = pl.multiple_of(i * 64, 64)
            h2buf[pl.ds(r, 64), :] = _ln(xbuf[pl.ds(r, 64), :].astype(f32))
            return 0
        lax.fori_loop(0, NPRE // 64, ln0_body, 0)

        def mod0_body(j, _):
            pltpu.make_async_copy(wmodb.at[j], wmodb.at[j], sems.at[SMOD + j]).wait()
            accs = [jnp.zeros((8, 512), f32)] * 2
            for k in range(64):
                accs[k % 2] = mod_rows(accs[k % 2], wmodb[j, k * 16:(k + 1) * 16, :], k * 16)
            mod_finish(accs[0] + accs[1], j)
            return 0
        _loop("mod0", 0, 4, mod0_body)

        def hpre_body(i, _):
            r = pl.multiple_of(i * 32, 32)
            hv = h2buf[pl.ds(r, 32), :] * modrows(1, 32) + modrows(0, 32)
            ro = pl.multiple_of(i * 8, 8)
            for t, op in enumerate(row_operands(hv)):
                h7[t, pl.ds(ro, 8), :] = pltpu.bitcast(op.astype(bf16), u32)
            return 0
        lax.fori_loop(0, NPRE // 32, hpre_body, 0)
        lhs_h[MEM:32, :] = adaln_a(xbuf[NPRE:NPRE + RIDE, :].astype(f32)).astype(bf16)

        def relayout_now(g, dh):
            def rl_body(t, _):
                relayout(g, 2 * g + dh, dh, t * 32, 32)
                return 0
            lax.fori_loop(0, 8, rl_body, 0)

        for dh in range(2):
            stg_wait(dh, 1, dh)
            relayout_now(0, dh)

        grp = lambda g: [piece_copy(g, 0), piece_copy(g, 1)]
        issue = {0: [wo_copy(0)], 1: grp(3) + grp(4), 2: grp(5) + [wo_copy(1), mod_copy(4)],
                 3: grp(6) + [mod_copy(5), mod_copy(6)], 4: grp(7) + [wo_copy(2)],
                 5: grp(8) + [wo_copy(3), mod_copy(7)], 6: grp(9) + [wo_copy(4)],
                 7: grp(10) + [wo_copy(5), mod_copy(8)], 8: grp(11) + [wo_copy(6)],
                 9: [wo_copy(7), mod_copy(9)], 10: stream_copies(0)}

        def pre_iter(g, carry):
            m3, gbase = carry

            @pl.when(g == 1)
            def _():
                stg_wait(2, 2, 2)
                relayout_now(1, 0)
                relayout_now(1, 1)

            def slots():
                m3n = jnp.where(m3 == 2, 0, m3 + 1)
                cj = jnp.maximum(g - 2, 3)
                return (m3n, 2 * jnp.where(ends, m3, m3n),
                        jnp.where(jnp.logical_or(g < 4, m3 == 0), 2, m3 - 1),
                        cj, jnp.where(cj >= NMOD, cj - NMOD, cj))

            ends = jnp.logical_or(g == 0, g == NGRP - 1)

            @pl.when(jnp.logical_not(ends))
            def _():
                stg_wait(slots()[1], 2, g + 2)

            @pl.when(g >= 4)
            def _():
                buf = wos.at[slots()[2]]
                pltpu.make_async_copy(buf, buf, sems.at[SSTG + g + 2]).wait()

            @pl.when(g >= 6)
            def _():
                buf = wmodb.at[slots()[4]]
                pltpu.make_async_copy(buf, buf, sems.at[SSTG + g + 2]).wait()

            m3n, gslot, wslot, cj, cslot = slots()
            gn = jnp.where(ends, g, g + 1)
            wrow = WO + jnp.maximum(g - 4, 0) * 256
            for k, cps in issue.items():
                @pl.when(g == k)
                def _():
                    for cp in cps:
                        cp.start()
            wtodo = [(r, c) for r in range(16) for c in range(8)]
            todo = [(dh, dp) for dh in range(2) for dp in range(256)]
            skip = [0] * RSK
            mtodo = list(range(0, D, 16))
            macc = [jnp.zeros((8, 512), f32)]

            def hook(v):
                if mtodo:
                    acc = macc[0] + jnp.concatenate([_zero_after(v)] * 4, axis=1)
                    for r in mtodo[:3]:
                        acc = mod_rows(acc, wmodb[cslot, r:r + 16, :], r)
                    del mtodo[:3]
                    macc[0] = acc

            for q in range(4):
                def b_of(k):
                    w = b_operand(gbase, q, k)
                    if skip:
                        skip.pop()
                        return w
                    nw = 0 if todo else WLP
                    for dh, dp in todo[:RLP]:
                        relayout(gn, gslot + dh, dh, dp, 1)
                    del todo[:RLP]
                    for r, c in wtodo[:nw]:
                        wqkv[pl.ds(wrow + (c * 2048 + r * 16), 16), :] = pltpu.bitcast(
                            wos[wslot, r * 32:(r + 1) * 32, c * 128:(c + 1) * 128], u32)
                    del wtodo[:nw]
                    return w
                c11, c12, c21, c22 = _strassen(lambda k: pltpu.bitcast(h7[k], bf16), b_of, hook)
                for blk, y in ((q + 4, _merge_rows(c12, c22)), (q, _merge_rows(c11, c21))):
                    for e in range(NPRE // 8):
                        tile, half = divmod(((8 * e + ROFF) % NR) // 8, 2)
                        rings[blk][g, tile, 4 * half:4 * half + 4, :] = _pack8(y[8 * e:8 * e + 8])
            assert not todo and not wtodo and not mtodo
            mod_finish(macc[0], cj)
            return m3n, gbase + 8 * WP

        _loop("pre1", 0, NGRP, pre_iter, (0, 0))

    pl.run_scoped(prologue,
                  pltpu.VMEM((NSLOT, 512, 8, 128), bf16),
                  pltpu.VMEM((NWO, 512, D), bf16),
                  pltpu.VMEM((NMOD, D, 512), bf16),
                  pltpu.VMEM((7, NPRE // 4, 512), u32))

    def main(w7, w49):
        scale = DH ** -0.5
        ia = lax.broadcasted_iota(jnp.int32, (32, L), 0)
        ja = lax.broadcasted_iota(jnp.int32, (32, L), 1)
        mask_a = (((ia >= 16) & (ia < 24)) | (ja >= SEG)
                  | (jnp.where(ia < 16, ia + 16, ia - 16) >= ja))
        ib = lax.broadcasted_iota(jnp.int32, (48, 56), 0)
        jb = lax.broadcasted_iota(jnp.int32, (48, 56), 1)
        own = (ib < 40) == (jb < 40)
        mask_b = own & (((jb >= 32) & (jb < 48)) | (jnp.where(jb < 40, jb, jb - 8) <= ib))
        masked = -1e9 / scale
        j8 = lax.broadcasted_iota(jnp.int32, (8, 56), 1)
        fill_b = jnp.concatenate([jnp.where(j8 < 40, masked, -3e38).astype(f32)] * 5
                                 + [jnp.where(j8 < 40, -3e38, masked).astype(f32)], axis=0)

        def softmax(sc, mask, fill):
            sc = jnp.where(mask, sc, fill)
            mx = jnp.max(sc, axis=-1, keepdims=True)
            e = jnp.exp2((sc - mx) * (scale * 1.4426950408889634))
            den = jnp.sum(e, axis=-1, keepdims=True)
            return (e * pl.reciprocal(den, approx=True)).astype(bf16)

        def ride_tiles(it, is_b):
            first = (it == 0).astype(jnp.int32)
            if is_b:
                return 3 * it + 1 - first, 0, 3 * it + 2
            return 3 * it + 1 - first, 1, 3 * it + first

        def step(it, is_b, lhs_lo, lhs_hi, jobs):
            NT, TOFF = NR // 16, ROFF // 16
            sega = (4 * it + TOFF) % NT
            seg = sega + 2 if is_b else sega
            wt = [(3 * it + (NPRE // 16 + TOFF + t + is_b)) % NT for t in range(2)]
            wr = [(wt[(t + is_b) // 2], (t + is_b) % 2) for t in range(3)]
            rt, rh, rf = ride_tiles(it, is_b)
            rt, rf = (rt + TOFF) % NT, (rf + TOFF) % NT
            lhs = jnp.concatenate([lhs_lo, lhs_hi], axis=1)
            QM, P, PART = {}, {}, {}
            mrow = 0 if is_b else 4

            def wblk(b, lo, n):
                return pltpu.bitcast(wqkv[b * WP + lo:b * WP + lo + n, :], bf16)

            def qkv_lo(i):
                for m in range(3):
                    PART[(m, i)] = jnp.dot(lhs_lo, wblk(m * H + i, 0, 256), preferred_element_type=f32)

            def qkv(i):
                for m in range(3):
                    b = m * H + i
                    if (m, i) in PART:
                        y = jnp.dot(lhs_hi, wblk(b, 256, 256),
                                    preferred_element_type=f32) + PART.pop((m, i))
                    else:
                        y = jnp.dot(lhs, wblk(b, 0, 512), preferred_element_type=f32)
                    if m < 2:
                        QM[b] = y[0:MEM] + jobs["pin"] if b == PIN and is_b else y[0:MEM]
                    if m == 2 or (m == 1 and not is_b):
                        kvm[b - H, mrow:mrow + 4, :] = _pack8(y[0:MEM])
                    for t in range(3):
                        rset(b, *wr[t], y[8 + 8 * t:16 + 8 * t])
                    for job in jobs.get(3 * i + m, []):
                        job(y)
                    side(3 * i + m)

            def keys(b):
                if is_b:
                    if b in QM:
                        mix = jnp.concatenate([_pack8(QM.pop(b)), kvm[b - H, 4:8, :]], axis=0)
                    else:
                        mix = kvm[b - H]
                    return _unpack(jnp.concatenate([rget(b, seg, 2), mix, rhalf(b, sega, 0)], axis=0))
                mk = _pack8(QM.pop(b)) if b in QM else kvm[b - H, 4:8, :]
                return _unpack(jnp.concatenate([rget(b, seg, 2), mk], axis=0))

            def scores(i):
                if is_b:
                    q = [rget(i, seg, 2), _pack8(QM.pop(i)), rhalf(i, sega, 0)]
                else:
                    q = [rget(i, seg + 1, 1), _pack8(QM.pop(i)), rhalf(i, seg, 1)]
                sc = lax.dot_general(_unpack(jnp.concatenate(q, axis=0)), keys(H + i),
                                     (((1,), (1,)), ((), ())), preferred_element_type=f32)
                P[i] = softmax(sc, mask_b, fill_b) if is_b else softmax(sc, mask_a, masked)

            def pv(i):
                o = jnp.dot(P.pop(i), keys(2 * H + i), preferred_element_type=f32)
                if is_b:
                    for e in range(4):
                        rset(i, seg + e // 2, e % 2, o[8 * e:8 * e + 8])
                    rset(i, sega, 0, o[40:48])
                    lhs_o[i, 0:4, :] = _pack8(o[SEG:L])
                else:
                    for e in range(2):
                        rset(i, seg + 1, e, o[8 * e:8 * e + 8])
                    rset(i, seg, 1, o[24:32])
                    lhs_o[i, 0:4, :] = _pack8(o[16:24])
                lhs_o[i, 4:8, :] = rhalf(i, rt, rh)
                lhs_o[i, 8:16, :] = rget(i, rf, 1)

            def wo_lhs(i0, i1):
                return _unpack(jnp.concatenate([lhs_o[i] for i in range(i0, i1)], axis=1))

            def wo_dot(lo, j, i0, i1):
                r = WO + j * 2048
                w = pltpu.bitcast(wqkv[r + 64 * i0:r + 64 * i1, :], bf16)
                return jnp.dot(lo, w, preferred_element_type=f32)

            def side(d):
                ds, dp = (DSB, DPB) if is_b else (DSA, DPA)
                if (d - dp) % 3 == 2 and 0 <= (d - dp) // 3 < H:
                    pv((d - dp) // 3)
                if (d - ds) % 3 == 2 and 0 <= (d - ds) // 3 < H:
                    scores((d - ds) // 3)

            if is_b:
                for h in range(KSPLIT):
                    qkv_lo(h)
            for h in range(H):
                qkv(h)
            lo = [wo_lhs(8 * k, 8 * k + 8) for k in range(3)]
            acc = []
            for j in range(8):
                y = None
                for k in range(3):
                    z = wo_dot(lo[k], j, 8 * k, 8 * k + 8)
                    y = z if y is None else z + y
                    for job in jobs.get(96 + 3 * j + k, []):
                        job(y)
                    side(96 + 3 * j + k)
                acc.append(y)
            lo = wo_lhs(24, H)
            for j in range(8):
                acc[j] = wo_dot(lo, j, 24, H) + acc[j]
                for job in jobs.get(120 + j, []):
                    job(acc[j])
            assert not (QM or P or PART)
            return jnp.concatenate(acc[0:4], axis=1), jnp.concatenate(acc[4:8], axis=1)

        def combine(c, n, y):
            mp, k1 = divmod(n, 8)
            m, p = divmod(mp, 4)
            c3 = jnp.minimum(c, 27)
            spare = pl.ds(pl.multiple_of(8 * (c // 64), 8), 8)
            if m == 0 and k1 < 7:
                ws3[16, spare, :] = y.astype(bf16)
            else:
                wsr[7, spare, 0:128] = y.astype(bf16)
            if k1 == 7:
                dst, base, r = w7, 0, (4 * m + p) * 32 + c
                blk = [wsr[4 + i, m * 16:(m + 1) * 16, j * 512 + p * 128:j * 512 + (p + 1) * 128]
                       .astype(f32) for i in range(2) for j in range(2)]
            else:
                dst, base = w49, 7 * k1
                if m == 0:
                    r = c3 * 4 + p
                    get = lambda i, j: ws3[4 * i + j, p * 16:(p + 1) * 16, :]
                else:
                    r = W4T + (p // 2) * 56 + c3 * 2 + p % 2
                    r0, c0 = (p % 2) * 16, (p // 2) * 128
                    get = lambda i, j: wsr[i, r0:r0 + 16, j * 256 + c0:j * 256 + c0 + 128]

                def quad(q):
                    return [get(2 * (q // 2) + i, 2 * (q % 2) + j).astype(f32)
                            for i in range(2) for j in range(2)]
                qi, qj, sign = _BTERMS[k1]
                blk = quad(qi)
                if qj is not None:
                    blk = [u + v if sign > 0 else u - v for u, v in zip(blk, quad(qj))]
            for k, op in enumerate(_b_operands(*blk)):
                for e in range(2):
                    dst[base + k, r, 4 * e:4 * e + 4, :] = _pack8(op[8 * e:8 * e + 8])

        def rec_body(it, gacc):
            stream_wait(it)
            lhs_lo = lhs_h[:, 0:512]
            lhs_hi = lhs_h[:, 512:1024]
            ra = jnp.maximum(it - 1, 0) * (2 * RIDE)
            for u in range(2):
                s = 2 * it + u
                jobs = {}
                for n, (su, d, g) in enumerate(SLOTS):
                    if su == u:
                        jobs.setdefault(d, []).append(
                            lambda y, n=n, g=g: combine(it, n, y[8 * g:8 * g + 8]))
                r1 = pl.multiple_of(jnp.minimum(NPRE + RIDE * (s + 1), S - RIDE), 8)
                xn = xbuf[pl.ds(r1, RIDE), :].astype(f32)
                if u == 0:
                    for k in range(2):
                        rm = pl.multiple_of(it * 32 + k * 16, 16)
                        gacc = mod_rows(gacc, wsr[6, k * 16:(k + 1) * 16, :], rm)
                    hn = adaln_a(xn, _zero_after(stage_a16(ra)))
                else:
                    def refill(y):
                        for cp in stream_copies(jnp.minimum(it + 1, NSEG // 2 - 1)):
                            cp.start()
                        spare = pl.ds(pl.multiple_of(8 * (it // 64), 8), 8)
                        jobs["pin"] = _zero_after(ws3[16, spare, :].astype(f32))
                    jobs.setdefault(3 * (PIN - 4) + 2, []).append(refill)
                    hn = adaln_a(xn)
                    z = _zero_after(hn[0:8], hn[8:16], hn[16:24])
                    stage_a16(ra + 32, _zero_after(stage_a16(ra + 16, z)))
                a_lo, a_hi = step(it, u, lhs_lo, lhs_hi, jobs)
                lhs_lo = jnp.concatenate([a_lo[0:MEM], hn[:, 0:512]], axis=0).astype(bf16)
                lhs_hi = jnp.concatenate([a_hi[0:MEM], hn[:, 512:1024]], axis=0).astype(bf16)
                a = jnp.concatenate([a_lo, a_hi], axis=1)
                rt, rh, rf = ride_tiles(it, u)
                rows = [pl.ds(pl.multiple_of(16 * rt + 8 * rh, 8), 8),
                        pl.ds(pl.multiple_of(16 * rf, 16), 16)]
                xs = [xbuf[r, :].astype(f32) for r in rows]
                xbuf[rows[0], :] = (xs[0] + modrows(2, 8) * a[8:16]).astype(bf16)
                xbuf[rows[1], :] = (xs[1] + modrows(2, 16) * a[16:32]).astype(bf16)
            lhs_h[:, 0:512] = lhs_lo
            lhs_h[:, 512:1024] = lhs_hi
            return gacc

        gacc = _loop("rec", 0, NSEG // 2, rec_body, jnp.zeros((8, D), f32))
        for c in range(2):
            mod_finish(gacc[:, c * 512:(c + 1) * 512], 10 + c)
        stream_wait(NSEG // 2 - 1)

        def wo_prep(i, half, k):
            o = jnp.concatenate([_unpack(rings[4 * half + h][i, k]).astype(f32)
                                 for h in range(4)], axis=1)
            for t, op in enumerate(row_operands(o)):
                a7[half, t, k * 8:(k + 1) * 8, :] = op.astype(bf16)

        def wo_chunk(i, half, inext, extra):
            row = pl.multiple_of(i * 512 + half * 256, 256)
            todo = list(range(NPRE // 16))

            def hook(v):
                if todo:
                    for h in range(4):
                        rings[4 * (1 - half) + h][4, i // 64] = pltpu.bitcast(v[0:8], u32)
                    n = 2 if len(todo) % WPP == 0 else 1
                    for k in todo[:n]:
                        wo_prep(inext, 1 - half, k)
                    del todo[:n]
                extra(v)

            for j in range(4):
                def b_of(k):
                    def quad(q):
                        r = WO + (j + 4 * (q % 2)) * 2048 + (q // 2) * 128 + row
                        return pltpu.bitcast(wqkv[pl.ds(r, 128), :], bf16)
                    qi, qj, sign = _BTERMS[k]
                    if qj is None:
                        return quad(qi)
                    u, v = quad(qi).astype(f32), quad(qj).astype(f32)
                    return (u + v if sign > 0 else u - v).astype(bf16)
                c11, c12, c21, c22 = _strassen(lambda k: a7[half, k], b_of, hook)
                for c, y in ((j + 4, _merge_rows(c12, c22)), (j, _merge_rows(c11, c21))):
                    cs = slice(c * 128, (c + 1) * 128)
                    h2buf[S - NPRE:S, cs] = h2buf[S - NPRE:S, cs] + y

        for k in range(NPRE // 16):
            wo_prep(0, 0, k)

        def wo_tail(i, _):
            st = {"n": 0, "prev": None}

            def extra(v):
                n = st["n"]
                st["n"] += 1
                if n % 16 == 2 and n // 16 < 3:
                    st["prev"] = stage_a16(S - NPRE - 48 + 16 * (n // 16),
                                           _zero_after(v, st["prev"]))
            wo_chunk(i, 0, i, extra)
            wo_chunk(i, 1, jnp.minimum(i + 1, 3), extra)
            return 0
        _loop("wotail", 0, 4, wo_tail)

        def gget(c, row, n):
            return pltpu.bitcast(wqkv[pl.ds(c * GS + row, n), :], f32)

        def gset(c, row, val):
            wqkv[pl.ds(c * GS + row, val.shape[0]), :] = pltpu.bitcast(val, u32)

        def wop(j):
            return lambda k: _unpack(w7[k, j * 32:(j + 1) * 32].reshape(256, 128))

        zpad = jnp.zeros((GPAD, 128), f32)
        for cb in range(8):
            gset(cb, 0, zpad)
            gset(cb, GPAD + S, zpad)

        shifts = (-1, -1, 1, 1, -2, -2, 2, 2)
        HB = MB // 2

        def shift_piece(r, half, k):
            gs = jnp.concatenate([gget(c, r + (k * 16 + GPAD + shifts[c]), 16)
                                  for c in range(8)], axis=1)
            ro = half * (HB // 2) + k * 8
            for t, op in enumerate(row_operands(gs)):
                n7[t, ro:ro + 8, :] = op.astype(bf16)

        def gate(v, i):
            gset(0, GPAD + S + GPAD + 8 * (i // S), v[0:8])

        def b_body(i, _):
            rl = S - NPRE + i * 128
            st = {"n": 0, "prev": [None, None]}

            def hook(v):
                n = st["n"]
                st["n"] += 1
                if n % BG == 0 and n // BG < 8:
                    k = n // BG
                    st["prev"][k % BCH] = stage_a16(rl + 16 * k,
                                                    _zero_after(v, st["prev"][k % BCH]),
                                                    (t7, 8 * k))

            ro = pl.multiple_of(i * 192, 64)
            for lhs, row in ((lambda k: n7[k, pl.ds(ro, 192), :], i * 384), (lambda k: t7[k], rl)):
                rg = pl.multiple_of(GPAD + row, 8)
                for j in range(4):
                    c11, c12, c21, c22 = _strassen(lhs, wop(j), hook)
                    gset(j + 4, rg, _gelu(_merge_rows(c12, c22)))
                    gset(j, rg, _gelu(_merge_rows(c11, c21)))
            return 0
        _loop("b", 0, S // MB, b_body)
        for k in range(HB // 16):
            shift_piece(0, 0, k)

        def n2_norm(r, k, anchor):
            v = _ln(h2buf[pl.ds(pl.multiple_of(r + k * 16, 16), 16), :], anchor)
            nrms[k // 2][(k % 2) * 16:(k % 2) * 16 + 16, :] = v
            return v[0:8] + v[8:16]

        def n2_ops(k, k1, v, i):
            nrm = nrms[k]
            nrm[pl.ds(pl.multiple_of(32 + 8 * (i // S), 8), 8), 0:128] = v[0:8]

            def quad(q):
                r0, c0 = (q // 2) * 16, (q % 2) * 512
                return [nrm[r0 + 8 * a:r0 + 8 * a + 8, c0 + 256 * b:c0 + 256 * b + 256]
                        for a in range(2) for b in range(2)]
            qi, qj, sign = _ATERMS[k1]
            blk = quad(qi)
            if qj is not None:
                blk = [u + w if sign > 0 else u - w for u, w in zip(blk, quad(qj))]
            for k2, op in enumerate(_a_operands(*blk)):
                d49[7 * k1 + k2, k * 8:(k + 1) * 8, :] = op.astype(bf16)

        def n2_hook(r, i, first, gap, lag, st):
            def hook(v):
                n = st["n"] - first
                st["n"] += 1
                if n >= 0 and n % gap == 0 and n // gap < MD // 16:
                    st["prev"] = n2_norm(r, n // gap, _zero_after(v, st["prev"]))
                for _ in range(st["per"]):
                    k, k1 = divmod(st["ops"], 7)
                    if k < MD // 32 and n >= (2 * k + 1) * gap + lag:
                        n2_ops(k, k1, v, i)
                        st["ops"] += 1
            return hook

        def stage_c(i, r, half, rnext, extra):
            rr = pl.multiple_of(r, 8)
            ro = half * (HB // 2)
            cnt = [0]

            def hook(v):
                n = cnt[0]
                cnt[0] += 1
                if n < HB // 16:
                    gate(v, i)
                    shift_piece(rnext, 1 - half, n)
                extra(v)

            for j in range(4):
                c11, c12, c21, c22 = _strassen(lambda k: n7[k, ro:ro + HB // 2, :], wop(4 + j),
                                               hook)
                for c, y in ((j + 4, _merge_rows(c12, c22)), (j, _merge_rows(c11, c21))):
                    cs = slice(c * 128, (c + 1) * 128)
                    h2buf[pl.ds(rr, HB), cs] = h2buf[pl.ds(rr, HB), cs] + y

        def c_body(i, _):
            r = pl.multiple_of(i * MB, MB)
            st = {"n": 0, "prev": None, "ops": 0, "per": 1}
            extra = n2_hook(0, i, 0, 4, 4, st)
            stage_c(i, r, 0, r + HB, extra)
            stage_c(i, r + HB, 1, jnp.minimum(i + 1, S // MB - 1) * MB, extra)
            assert st["ops"] == 28
            return 0
        _loop("c", 0, S // MB, c_body)

        def wop2(lo, n):
            return lambda k1, k: _unpack(w49[7 * k1 + k, lo:lo + n].reshape(8 * n, 128))

        def d_body(i, _):
            r = pl.multiple_of(i * MD, MD)
            rn = jnp.minimum(r + MD, S - MD)
            lhs = [d49[k] for k in range(49)]
            uops = []
            for t in range(7):
                cb = _strassen2(lambda k1, k: lhs[7 * k1 + k], wop2(t * 16, 16))
                uops.append(_a_operands2([[_gelu(c) for c in row] for row in cb]))
            ul = [[jnp.concatenate([u[k1][k] for u in uops], axis=1).astype(bf16)
                   for k in range(7)] for k1 in range(7)]
            st = {"n": 0, "prev": None, "ops": 0, "per": 1}
            hook = n2_hook(rn, i, DF, DG, DL, st)
            for t in range(2):
                cb = _strassen2(lambda k1, k: ul[k1][k], wop2(W4T + t * 56, 56), hook)
                for j in range(4):
                    y = jnp.concatenate([cb[q][j].reshape(MD // 32, 8, 128) for q in range(4)],
                                        axis=1).reshape(MD, 128)
                    c = 2 * j + t
                    cs = slice(c * 128, (c + 1) * 128)
                    gb = modrows(5, MD, c * 128, (c + 1) * 128)
                    o = xbuf[pl.ds(r, MD), cs].astype(f32) + gb * (h2buf[pl.ds(r, MD), cs] + y)
                    xbuf[pl.ds(r, MD), cs] = o.astype(bf16)
            assert st["ops"] == 28
            out_copy(r, MD).start()
            return 0
        _loop("d", 0, S // MD, d_body)

    pl.run_scoped(main,
                  pltpu.VMEM((7, 8 * 32, 8, 128), u32),
                  pltpu.VMEM((49, 2 * W4T, 8, 128), u32))

    out_copy(0, S).wait()


def _run(x, mem0, wq, wk, wv, wo, w1, w2, w3, w4, c, wmod):
    any_spec = pl.BlockSpec(memory_space=pl.ANY)
    return pl.pallas_call(
        _kernel,
        out_shape=jax.ShapeDtypeStruct((S, D), bf16),
        in_specs=[any_spec] * 12,
        out_specs=any_spec,
        scratch_shapes=[
            pltpu.VMEM((S + 2 * RIDE, D), bf16),
            pltpu.VMEM((WO + 8 * 2048, 128), u32),
            [pltpu.VMEM((96 // NRING, NR // 16, 8, 128), u32)] * NRING,
            pltpu.VMEM((32, D), bf16),
            pltpu.VMEM((H, 16, 128), u32),
            pltpu.VMEM((2 * H, 8, 128), u32),
            pltpu.VMEM((12, 8, 512), f32),
            pltpu.VMEM((D, 128), f32),
            pltpu.VMEM((S, D), f32),
            pltpu.VMEM((7, (S - NPRE) // 2, 512), bf16),
            pltpu.VMEM((17, 64, 128), bf16),
            pltpu.VMEM((8, 32, D), bf16),
            pltpu.VMEM((7, 64, 512), bf16),
            pltpu.VMEM((2, 7, NPRE // 2, 256), bf16),
            pltpu.VMEM((49, MD // 4, 256), bf16),
            [pltpu.VMEM((40, D), f32)] * (MD // 32),
            pltpu.VMEM((1, D), bf16),
            pltpu.SemaphoreType.DMA((9 + NGRP + 2,)),
        ],
        compiler_params=pltpu.CompilerParams(vmem_limit_bytes=124 * 1024 * 1024,
                                             disable_bounds_checks=True,
                                             disable_semaphore_checks=True),
    )(x, mem0, wq, wk, wv, wo, w1, w2, w3, w4, c, wmod)


def pallas_adaLN_cond__memory_aug_recurrent_mem_tr__mixer_s_mlp__prompt_kernel(
    A_x, A_mem0, A_Wq, A_Wk, A_Wv, A_Wo, A_seg_len, B_x, B_w1, B_w2, B_w3, B_w4, c, w_mod,
):
    del B_x
    assert A_x.shape == (1, S, D) and A_mem0.shape == (1, MEM, D)
    assert isinstance(A_seg_len, int) is False or A_seg_len == SEG
    out = _run(A_x.reshape(S, D), A_mem0.reshape(MEM, D), A_Wq, A_Wk, A_Wv,
               A_Wo.reshape(H * DH, D),
               B_w1.reshape(2, D // 2, D), B_w2.reshape(2, D // 2, D),
               B_w3, B_w4.reshape(4, F // 4, D), c, w_mod)
    return out.reshape(1, S, D)
```

```python
import jax
import jax.numpy as jnp
from jax import lax
import jax.experimental.pallas as pl
import jax.experimental.pallas.tpu as pltpu

bf16 = jnp.bfloat16
f32 = jnp.float32
u32 = jnp.uint32

S = 2048
D = 1024
H = 32
DH = 128
F = 3584
MEM = 8
SEG = 32
NSEG = S // SEG
L = MEM + SEG
RIDE = 24
NPRE = S - RIDE * NSEG
NR = NPRE + 2 * SEG
ROFF = (-(S - NPRE)) % NR
WP = 516
WO = 96 * WP
NGRP = 12
NSLOT = 6
NMOD = 6
EPS = 1e-5
MD = 128
MB = 512
GPAD = 8
NRING = 8
RLP, WLP, RSK = 27, 22, 2
NWO = 3
BG, WPP, PIN, BCH = 2, 5, 6, 2
DF, DG, DL = 2, 10, 9
SLOTS = ([(0, n // 2, 3 * (n % 2)) for n in range(16)] + [(0, 96 + n, 0) for n in range(16)]
         + [(0, 112 + n // 2, 3 * (n % 2)) for n in range(32)])
DSA, DPA, DSB, DPB, KSPLIT = 6, 12, 6, 12, 2
X0 = NPRE + 2 * RIDE
GS = S + 4 * GPAD
W4T = 7 * 16
_ONLY = None


def _loop(name, lo, hi, body, init=0):
    if _ONLY is not None and name not in _ONLY:
        return init
    with _scope(name):
        return lax.fori_loop(lo, hi, body, init)


class _NoScope:
    def __init__(self, name):
        del name

    def __enter__(self):
        return self

    def __exit__(self, *a):
        return False


_scope = _NoScope


def _zero_after(*vs):
    bits = None
    for v in vs:
        if v is not None:
            b = pltpu.bitcast(v[0:8, 0:128], u32)
            bits = b if bits is None else bits | b
    return pltpu.bitcast((bits >> 31) >> 1, f32)


def _ln(x, anchor=None):
    if anchor is not None:
        z = jnp.concatenate([anchor] * (x.shape[0] // 8), axis=0)
        x = jnp.concatenate([x[:, 0:128] + z, x[:, 128:]], axis=1)
    mu = jnp.mean(x, axis=-1, keepdims=True)
    xc = x - mu
    var = jnp.mean(xc * xc, axis=-1, keepdims=True)
    return xc * lax.rsqrt(var + EPS)


def _gelu(x):
    inner = x * (0.7978845608028654 + (0.7978845608028654 * 0.044715) * (x * x))
    hx = 0.5 * x
    return hx + hx * jnp.tanh(inner)


def _split_rows(x):
    m, n = x.shape
    x3 = x.reshape(m // 16, 16, n)
    return x3[:, 0:8, :].reshape(m // 2, n), x3[:, 8:16, :].reshape(m // 2, n)


def _merge_rows(top, bot):
    m, n = top.shape
    return jnp.concatenate([top.reshape(m // 8, 8, n), bot.reshape(m // 8, 8, n)],
                           axis=1).reshape(2 * m, n)


def _a_operands(a11, a12, a21, a22):
    return [a11 + a22, a21 + a22, a11, a22, a11 + a12, a21 - a11, a12 - a22]


def _b_operands(b11, b12, b21, b22):
    return [b11 + b22, b11, b12 - b22, b21 - b11, b22, b11 + b12, b21 + b22]


_ATERMS = ((0, 3, 1), (2, 3, 1), (0, None, 0), (3, None, 0), (0, 1, 1), (2, 0, -1), (1, 3, -1))
_BTERMS = ((0, 3, 1), (0, None, 0), (1, 3, -1), (2, 0, -1), (3, None, 0), (0, 1, 1), (2, 3, 1))


def _strassen(a_of, b_of, hook=lambda v: None):
    def prod(k):
        return jnp.dot(a_of(k), b_of(k), preferred_element_type=f32)
    p5 = prod(4)
    hook(p5)
    p3 = prod(2)
    hook(p3)
    c12 = p3 + p5
    p4 = prod(3)
    hook(p4)
    c11 = p4 - p5
    p2 = prod(1)
    hook(p2)
    c21 = p2 + p4
    c22 = p3 - p2
    p1 = prod(0)
    hook(p1)
    c11 = prod(6) + (c11 + p1)
    hook(c11)
    c22 = prod(5) + (c22 + p1)
    hook(c22)
    return c11, c12, c21, c22


def _a_operands2(b):
    sub = [_a_operands(b[i][j], b[i][2 + j], b[2 + i][j], b[2 + i][2 + j])
           for i in range(2) for j in range(2)]
    return [_a_operands(*[t[k] for t in sub]) for k in range(7)]


def _strassen2(a_of, b_of, hook=lambda v: None):
    def prod(k1):
        return _strassen(lambda k: a_of(k1, k), lambda k: b_of(k1, k), hook)

    def add(x, y):
        return [p + q for p, q in zip(x, y)]

    def sub(x, y):
        return [p - q for p, q in zip(x, y)]
    p5 = prod(4)
    p3 = prod(2)
    c12 = add(p3, p5)
    p4 = prod(3)
    c11 = sub(p4, p5)
    p2 = prod(1)
    c21 = add(p2, p4)
    c22 = sub(p3, p2)
    p1 = prod(0)
    c11 = add(add(c11, p1), prod(6))
    c22 = add(add(c22, p1), prod(5))
    cq = (c11, c12, c21, c22)
    return [[cq[2 * (i // 2) + j // 2][2 * (i % 2) + j % 2] for j in range(4)] for i in range(4)]


def _pack8(v):
    return pltpu.bitcast(v.astype(bf16), u32)


def _unpack(w):
    return pltpu.bitcast(w, bf16)


def _kernel(x_hbm, mem0_hbm, wq_hbm, wk_hbm, wv_hbm, wo_hbm, w1_hbm, w2_hbm, w3_hbm, w4_hbm,
            c_hbm, wmod_hbm, out_hbm,
            xbuf, wqkv, rings, lhs_h, lhs_o, kvm, modv, scol, h2buf, n7, ws3, wsr, t7, a7, d49, nrms, c_ref,
            sems):
    w_hbms = (wq_hbm, wk_hbm, wv_hbm)
    SMOD, SSTG = 5, 9
    sem_x, sem_out, sem_w, sem_g, sem_r = (sems.at[k] for k in range(5))

    def rget(b, tile, n):
        return jnp.concatenate([rings[b % NRING][tile + e, b // NRING] for e in range(n)], axis=0)

    def rhalf(b, tile, half):
        return rings[b % NRING][tile, b // NRING, 4 * half:4 * half + 4, :]

    def rset(b, tile, half, val):
        rings[b % NRING][tile, b // NRING, 4 * half:4 * half + 4, :] = _pack8(val)

    x_copy = pltpu.make_async_copy(x_hbm.at[pl.ds(0, X0), :], xbuf.at[pl.ds(0, X0), :], sem_x)

    def stream_copies(c):
        al, lo = ((lambda v, m: v), min) if isinstance(c, int) else (pl.multiple_of, jnp.minimum)
        c3 = lo(c, 27)
        cps = [pltpu.make_async_copy(
            w3_hbm.at[pl.ds(al(i * 256 + (c3 % 4) * 64, 64), 64),
                      pl.ds(al(j * (F // 4) + (c3 // 4) * 128, 128), 128)],
            ws3.at[4 * i + j], sem_w) for i in range(4) for j in range(4)]
        dst = X0 + 2 * RIDE * c
        return [
            pltpu.make_async_copy(w4_hbm.at[:, pl.ds(al(c3 * 32, 32), 32), :],
                                  wsr.at[pl.ds(0, 4)], sem_g),
            pltpu.make_async_copy(w1_hbm.at[:, pl.ds(al(c * 16, 16), 16), :],
                                  wsr.at[pl.ds(4, 2), pl.ds(0, 16), :], sem_g),
            pltpu.make_async_copy(w2_hbm.at[:, pl.ds(al(c * 16, 16), 16), :],
                                  wsr.at[pl.ds(4, 2), pl.ds(16, 16), :], sem_g),
            pltpu.make_async_copy(wmod_hbm.at[pl.ds(al(c * 32, 32), 32), pl.ds(5 * D, D)],
                                  wsr.at[6], sem_g),
            pltpu.make_async_copy(x_hbm.at[pl.ds(al(lo(dst, S - 2 * RIDE), 16), 2 * RIDE), :],
                                  xbuf.at[pl.ds(al(dst, 16), 2 * RIDE), :], sem_r)] + cps

    def stream_wait(c):
        for dst, sem in ((ws3.at[pl.ds(0, 16)], sem_w), (wsr.at[pl.ds(0, 7)], sem_g),
                         (xbuf.at[pl.ds(X0 + 2 * RIDE * c, 2 * RIDE), :], sem_r)):
            pltpu.make_async_copy(dst, dst, sem).wait()

    def out_copy(row, n):
        return pltpu.make_async_copy(xbuf.at[pl.ds(row, n), :], out_hbm.at[pl.ds(row, n), :],
                                     sem_out)

    def mod_rows(acc, w, r):
        sc = jnp.concatenate([scol[pl.ds(r, 16), :]] * (w.shape[1] // 128), axis=1)
        p = w.astype(f32) * sc
        return acc + p[0:8] + p[8:16]

    def mod_finish(acc, j):
        is_scale = jnp.logical_or(j // 2 == 1, j // 2 == 4)
        tot = jnp.sum(acc, axis=0, keepdims=True) + jnp.where(is_scale, 1.0, 0.0)
        modv[j] = jnp.broadcast_to(tot, (8, 512))

    def modrows(k, n, lo=0, hi=D):
        m = jnp.concatenate([modv[2 * k], modv[2 * k + 1]], axis=1)[:, lo:hi]
        return jnp.concatenate([m] * (n // 8), axis=0)

    def adaln_a(xv, anchor=None):
        n = xv.shape[0]
        return _ln(xv, anchor) * modrows(1, n) + modrows(0, n)

    def adaln_b(xv, anchor=None):
        n = xv.shape[0]
        return _ln(xv, anchor) * modrows(4, n) + modrows(3, n)

    def row_operands(v):
        top, bot = _split_rows(v)
        k = v.shape[1] // 2
        return _a_operands(top[:, :k], top[:, k:], bot[:, :k], bot[:, k:])

    def stage_a16(r, anchor=None, dst=None):
        rr = pl.multiple_of(r, 16)
        xv = xbuf[pl.ds(rr, 16), :]
        if dst is not None:
            xv = (xv.astype(f32) + modrows(2, 16) * h2buf[pl.ds(rr, 16), :]).astype(bf16)
            xbuf[pl.ds(rr, 16), :] = xv
        h2 = adaln_b(xv.astype(f32), anchor)
        h2buf[pl.ds(rr, 16), :] = h2
        ref, ro = (n7, pl.multiple_of(rr // 2, 8)) if dst is None else dst
        ops = row_operands(_ln(h2))
        for t, op in enumerate(ops):
            ref[t, pl.ds(ro, 8), :] = op.astype(bf16)
        return ops[0]

    def prologue(stg, wos, wmodb, h7):
        def mod_copy(j):
            return pltpu.make_async_copy(wmod_hbm.at[:, pl.ds(j * 512, 512)], wmodb.at[j % NMOD],
                                         sems.at[SSTG + j + 4 if j >= 4 else SMOD + j])

        def piece_copy(g, dh):
            return pltpu.make_async_copy(
                w_hbms[g // 4].at[pl.ds(dh * 512, 512), pl.ds((g % 4) * 8, 8), :],
                stg.at[(2 * g + dh) % NSLOT], sems.at[SSTG + (g + 1 if g else dh)])

        def wo_copy(j):
            return pltpu.make_async_copy(wo_hbm.at[pl.ds(j * 512, 512), :], wos.at[j % NWO],
                                         sems.at[SSTG + j + 6])

        def group_start(g):
            for dh in range(2):
                piece_copy(g, dh).start()

        def stg_wait(slot, n, sem):
            dst = stg.at[pl.ds(slot, n)]
            pltpu.make_async_copy(dst, dst, sems.at[SSTG + sem]).wait()

        def relayout(g, slot, dh, lo_dp, n_dp):
            base = g * (8 * WP) + dh * 256
            for u in range(n_dp):
                dp = lo_dp + u
                ev = pltpu.bitcast(stg[slot, 2 * dp].astype(f32), u32)
                od = pltpu.bitcast(stg[slot, 2 * dp + 1].astype(f32), u32)
                wqkv[pl.ds(base + dp, 8, stride=WP), :] = (ev >> 16) | od

        def b_operand(gbase, q, k):
            def quad(i):
                r = gbase + ((q + 4 * (i % 2)) * WP + (i // 2) * 256)
                return pltpu.bitcast(wqkv[pl.ds(r, 256), :], bf16)
            i, j, sign = _BTERMS[k]
            if j is None:
                return quad(i)
            u, v = quad(i).astype(f32), quad(j).astype(f32)
            return (u + v if sign > 0 else u - v).astype(bf16)

        c_copy = pltpu.make_async_copy(c_hbm, c_ref, sem_g)
        m_copy = pltpu.make_async_copy(mem0_hbm, lhs_h.at[pl.ds(0, MEM), :], sem_r)
        c_copy.start()
        m_copy.start()
        x_copy.start()
        for j in range(4):
            mod_copy(j).start()
        for g in range(3):
            group_start(g)
        h2buf[S - NPRE:S, :] = jnp.zeros((NPRE, D), f32)
        wos[2] = jnp.zeros((512, D), bf16)
        c_copy.wait()
        m_copy.wait()
        cv = c_ref[...].astype(f32)
        sv = jnp.broadcast_to(cv * (1.0 / (1.0 + jnp.exp(-cv))), (128, D))
        for k in range(8):
            scol[k * 128:(k + 1) * 128, :] = sv[:, k * 128:(k + 1) * 128].T
        x_copy.wait()

        def ln0_body(i, _):
            r = pl.multiple_of(i * 64, 64)
            h2buf[pl.ds(r, 64), :] = _ln(xbuf[pl.ds(r, 64), :].astype(f32))
            return 0
        lax.fori_loop(0, NPRE // 64, ln0_body, 0)

        def mod0_body(j, _):
            pltpu.make_async_copy(wmodb.at[j], wmodb.at[j], sems.at[SMOD + j]).wait()
            accs = [jnp.zeros((8, 512), f32)] * 2
            for k in range(64):
                accs[k % 2] = mod_rows(accs[k % 2], wmodb[j, k * 16:(k + 1) * 16, :], k * 16)
            mod_finish(accs[0] + accs[1], j)
            return 0
        _loop("mod0", 0, 4, mod0_body)

        def hpre_body(i, _):
            r = pl.multiple_of(i * 32, 32)
            hv = h2buf[pl.ds(r, 32), :] * modrows(1, 32) + modrows(0, 32)
            ro = pl.multiple_of(i * 8, 8)
            for t, op in enumerate(row_operands(hv)):
                h7[t, pl.ds(ro, 8), :] = pltpu.bitcast(op.astype(bf16), u32)
            return 0
        lax.fori_loop(0, NPRE // 32, hpre_body, 0)
        lhs_h[MEM:32, :] = adaln_a(xbuf[NPRE:NPRE + RIDE, :].astype(f32)).astype(bf16)

        def relayout_now(g, dh):
            def rl_body(t, _):
                relayout(g, 2 * g + dh, dh, t * 32, 32)
                return 0
            lax.fori_loop(0, 8, rl_body, 0)

        for dh in range(2):
            stg_wait(dh, 1, dh)
            relayout_now(0, dh)

        grp = lambda g: [piece_copy(g, 0), piece_copy(g, 1)]
        issue = {0: [wo_copy(0)], 1: grp(3) + grp(4), 2: grp(5) + [wo_copy(1), mod_copy(4)],
                 3: grp(6) + [mod_copy(5), mod_copy(6)], 4: grp(7) + [wo_copy(2)],
                 5: grp(8) + [wo_copy(3), mod_copy(7)], 6: grp(9) + [wo_copy(4)],
                 7: grp(10) + [wo_copy(5), mod_copy(8)], 8: grp(11) + [wo_copy(6)],
                 9: [wo_copy(7), mod_copy(9)], 10: stream_copies(0)}

        def pre_iter(g, carry):
            m3, gbase = carry

            @pl.when(g == 1)
            def _():
                stg_wait(2, 2, 2)
                relayout_now(1, 0)
                relayout_now(1, 1)

            def slots():
                m3n = jnp.where(m3 == 2, 0, m3 + 1)
                cj = jnp.maximum(g - 2, 3)
                return (m3n, 2 * jnp.where(ends, m3, m3n),
                        jnp.where(jnp.logical_or(g < 4, m3 == 0), 2, m3 - 1),
                        cj, jnp.where(cj >= NMOD, cj - NMOD, cj))

            ends = jnp.logical_or(g == 0, g == NGRP - 1)

            @pl.when(jnp.logical_not(ends))
            def _():
                stg_wait(slots()[1], 2, g + 2)

            @pl.when(g >= 4)
            def _():
                buf = wos.at[slots()[2]]
                pltpu.make_async_copy(buf, buf, sems.at[SSTG + g + 2]).wait()

            @pl.when(g >= 6)
            def _():
                buf = wmodb.at[slots()[4]]
                pltpu.make_async_copy(buf, buf, sems.at[SSTG + g + 2]).wait()

            m3n, gslot, wslot, cj, cslot = slots()
            gn = jnp.where(ends, g, g + 1)
            wrow = WO + jnp.maximum(g - 4, 0) * 256
            for k, cps in issue.items():
                @pl.when(g == k)
                def _():
                    for cp in cps:
                        cp.start()
            wtodo = [(r, c) for r in range(16) for c in range(8)]
            todo = [(dh, dp) for dh in range(2) for dp in range(256)]
            skip = [0] * RSK
            mtodo = list(range(0, D, 16))
            macc = [jnp.zeros((8, 512), f32)]

            def hook(v):
                if mtodo:
                    acc = macc[0] + jnp.concatenate([_zero_after(v)] * 4, axis=1)
                    for r in mtodo[:3]:
                        acc = mod_rows(acc, wmodb[cslot, r:r + 16, :], r)
                    del mtodo[:3]
                    macc[0] = acc

            for q in range(4):
                def b_of(k):
                    w = b_operand(gbase, q, k)
                    if skip:
                        skip.pop()
                        return w
                    nw = 0 if todo else WLP
                    for dh, dp in todo[:RLP]:
                        relayout(gn, gslot + dh, dh, dp, 1)
                    del todo[:RLP]
                    for r, c in wtodo[:nw]:
                        wqkv[pl.ds(wrow + (c * 2048 + r * 16), 16), :] = pltpu.bitcast(
                            wos[wslot, r * 32:(r + 1) * 32, c * 128:(c + 1) * 128], u32)
                    del wtodo[:nw]
                    return w
                c11, c12, c21, c22 = _strassen(lambda k: pltpu.bitcast(h7[k], bf16), b_of, hook)
                for blk, y in ((q + 4, _merge_rows(c12, c22)), (q, _merge_rows(c11, c21))):
                    for e in range(NPRE // 8):
                        tile, half = divmod(((8 * e + ROFF) % NR) // 8, 2)
                        rings[blk][tile, g, 4 * half:4 * half + 4, :] = _pack8(y[8 * e:8 * e + 8])
            assert not todo and not wtodo and not mtodo
            mod_finish(macc[0], cj)
            return m3n, gbase + 8 * WP

        _loop("pre1", 0, NGRP, pre_iter, (0, 0))

    pl.run_scoped(prologue,
                  pltpu.VMEM((NSLOT, 512, 8, 128), bf16),
                  pltpu.VMEM((NWO, 512, D), bf16),
                  pltpu.VMEM((NMOD, D, 512), bf16),
                  pltpu.VMEM((7, NPRE // 4, 512), u32))

    def main(w7, w49):
        scale = DH ** -0.5
        ia = lax.broadcasted_iota(jnp.int32, (32, L), 0)
        ja = lax.broadcasted_iota(jnp.int32, (32, L), 1)
        mask_a = (((ia >= 16) & (ia < 24)) | (ja >= SEG)
                  | (jnp.where(ia < 16, ia + 16, ia - 16) >= ja))
        ib = lax.broadcasted_iota(jnp.int32, (48, 56), 0)
        jb = lax.broadcasted_iota(jnp.int32, (48, 56), 1)
        own = (ib < 40) == (jb < 40)
        mask_b = own & (((jb >= 32) & (jb < 48)) | (jnp.where(jb < 40, jb, jb - 8) <= ib))
        masked = -1e9 / scale
        j8 = lax.broadcasted_iota(jnp.int32, (8, 56), 1)
        fill_b = jnp.concatenate([jnp.where(j8 < 40, masked, -3e38).astype(f32)] * 5
                                 + [jnp.where(j8 < 40, -3e38, masked).astype(f32)], axis=0)

        def softmax(sc, mask, fill):
            sc = jnp.where(mask, sc, fill)
            mx = jnp.max(sc, axis=-1, keepdims=True)
            e = jnp.exp2((sc - mx) * (scale * 1.4426950408889634))
            den = jnp.sum(e, axis=-1, keepdims=True)
            return (e * pl.reciprocal(den, approx=True)).astype(bf16)

        def ride_tiles(it, is_b):
            first = (it == 0).astype(jnp.int32)
            if is_b:
                return 3 * it + 1 - first, 0, 3 * it + 2
            return 3 * it + 1 - first, 1, 3 * it + first

        def step(it, is_b, lhs_lo, lhs_hi, jobs):
            NT, TOFF = NR // 16, ROFF // 16
            sega = (4 * it + TOFF) % NT
            seg = sega + 2 if is_b else sega
            wt = [(3 * it + (NPRE // 16 + TOFF + t + is_b)) % NT for t in range(2)]
            wr = [(wt[(t + is_b) // 2], (t + is_b) % 2) for t in range(3)]
            rt, rh, rf = ride_tiles(it, is_b)
            rt, rf = (rt + TOFF) % NT, (rf + TOFF) % NT
            lhs = jnp.concatenate([lhs_lo, lhs_hi], axis=1)
            QM, P, PART = {}, {}, {}
            mrow = 0 if is_b else 4

            def wblk(b, lo, n):
                return pltpu.bitcast(wqkv[b * WP + lo:b * WP + lo + n, :], bf16)

            def qkv_lo(i):
                for m in range(3):
                    PART[(m, i)] = jnp.dot(lhs_lo, wblk(m * H + i, 0, 256), preferred_element_type=f32)

            def qkv(i):
                for m in range(3):
                    b = m * H + i
                    if (m, i) in PART:
                        y = jnp.dot(lhs_hi, wblk(b, 256, 256),
                                    preferred_element_type=f32) + PART.pop((m, i))
                    else:
                        y = jnp.dot(lhs, wblk(b, 0, 512), preferred_element_type=f32)
                    if m < 2:
                        QM[b] = y[0:MEM] + jobs["pin"] if b == PIN and is_b else y[0:MEM]
                    if m == 2 or (m == 1 and not is_b):
                        kvm[b - H, mrow:mrow + 4, :] = _pack8(y[0:MEM])
                    for t in range(3):
                        rset(b, *wr[t], y[8 + 8 * t:16 + 8 * t])
                    for job in jobs.get(3 * i + m, []):
                        job(y)
                    side(3 * i + m)

            def keys(b):
                if is_b:
                    if b in QM:
                        mix = jnp.concatenate([_pack8(QM.pop(b)), kvm[b - H, 4:8, :]], axis=0)
                    else:
                        mix = kvm[b - H]
                    return _unpack(jnp.concatenate([rget(b, seg, 2), mix, rhalf(b, sega, 0)], axis=0))
                mk = _pack8(QM.pop(b)) if b in QM else kvm[b - H, 4:8, :]
                return _unpack(jnp.concatenate([rget(b, seg, 2), mk], axis=0))

            def scores(i):
                if is_b:
                    q = [rget(i, seg, 2), _pack8(QM.pop(i)), rhalf(i, sega, 0)]
                else:
                    q = [rget(i, seg + 1, 1), _pack8(QM.pop(i)), rhalf(i, seg, 1)]
                sc = lax.dot_general(_unpack(jnp.concatenate(q, axis=0)), keys(H + i),
                                     (((1,), (1,)), ((), ())), preferred_element_type=f32)
                P[i] = softmax(sc, mask_b, fill_b) if is_b else softmax(sc, mask_a, masked)

            def pv(i):
                o = jnp.dot(P.pop(i), keys(2 * H + i), preferred_element_type=f32)
                if is_b:
                    for e in range(4):
                        rset(i, seg + e // 2, e % 2, o[8 * e:8 * e + 8])
                    rset(i, sega, 0, o[40:48])
                    lhs_o[i, 0:4, :] = _pack8(o[SEG:L])
                else:
                    for e in range(2):
                        rset(i, seg + 1, e, o[8 * e:8 * e + 8])
                    rset(i, seg, 1, o[24:32])
                    lhs_o[i, 0:4, :] = _pack8(o[16:24])
                lhs_o[i, 4:8, :] = rhalf(i, rt, rh)
                lhs_o[i, 8:16, :] = rget(i, rf, 1)

            def wo_lhs(i0, i1):
                return _unpack(jnp.concatenate([lhs_o[i] for i in range(i0, i1)], axis=1))

            def wo_dot(lo, j, i0, i1):
                r = WO + j * 2048
                w = pltpu.bitcast(wqkv[r + 64 * i0:r + 64 * i1, :], bf16)
                return jnp.dot(lo, w, preferred_element_type=f32)

            def side(d):
                ds, dp = (DSB, DPB) if is_b else (DSA, DPA)
                if (d - dp) % 3 == 2 and 0 <= (d - dp) // 3 < H:
                    pv((d - dp) // 3)
                if (d - ds) % 3 == 2 and 0 <= (d - ds) // 3 < H:
                    scores((d - ds) // 3)

            if is_b:
                for h in range(KSPLIT):
                    qkv_lo(h)
            for h in range(H):
                qkv(h)
            lo = [wo_lhs(8 * k, 8 * k + 8) for k in range(3)]
            acc = []
            for j in range(8):
                y = None
                for k in range(3):
                    z = wo_dot(lo[k], j, 8 * k, 8 * k + 8)
                    y = z if y is None else z + y
                    for job in jobs.get(96 + 3 * j + k, []):
                        job(y)
                    side(96 + 3 * j + k)
                acc.append(y)
            lo = wo_lhs(24, H)
            for j in range(8):
                acc[j] = wo_dot(lo, j, 24, H) + acc[j]
                for job in jobs.get(120 + j, []):
                    job(acc[j])
            assert not (QM or P or PART)
            return jnp.concatenate(acc[0:4], axis=1), jnp.concatenate(acc[4:8], axis=1)

        def combine(c, n, y):
            mp, k1 = divmod(n, 8)
            m, p = divmod(mp, 4)
            c3 = jnp.minimum(c, 27)
            spare = pl.ds(pl.multiple_of(8 * (c // 64), 8), 8)
            if m == 0 and k1 < 7:
                ws3[16, spare, :] = y.astype(bf16)
            else:
                wsr[7, spare, 0:128] = y.astype(bf16)
            if k1 == 7:
                dst, base, r = w7, 0, (4 * m + p) * 32 + c
                blk = [wsr[4 + i, m * 16:(m + 1) * 16, j * 512 + p * 128:j * 512 + (p + 1) * 128]
                       .astype(f32) for i in range(2) for j in range(2)]
            else:
                dst, base = w49, 7 * k1
                if m == 0:
                    r = c3 * 4 + p
                    get = lambda i, j: ws3[4 * i + j, p * 16:(p + 1) * 16, :]
                else:
                    r = W4T + (p // 2) * 56 + c3 * 2 + p % 2
                    r0, c0 = (p % 2) * 16, (p // 2) * 128
                    get = lambda i, j: wsr[i, r0:r0 + 16, j * 256 + c0:j * 256 + c0 + 128]

                def quad(q):
                    return [get(2 * (q // 2) + i, 2 * (q % 2) + j).astype(f32)
                            for i in range(2) for j in range(2)]
                qi, qj, sign = _BTERMS[k1]
                blk = quad(qi)
                if qj is not None:
                    blk = [u + v if sign > 0 else u - v for u, v in zip(blk, quad(qj))]
            for k, op in enumerate(_b_operands(*blk)):
                for e in range(2):
                    dst[base + k, r, 4 * e:4 * e + 4, :] = _pack8(op[8 * e:8 * e + 8])

        def rec_body(it, gacc):
            stream_wait(it)
            lhs_lo = lhs_h[:, 0:512]
            lhs_hi = lhs_h[:, 512:1024]
            ra = jnp.maximum(it - 1, 0) * (2 * RIDE)
            for u in range(2):
                s = 2 * it + u
                jobs = {}
                for n, (su, d, g) in enumerate(SLOTS):
                    if su == u:
                        jobs.setdefault(d, []).append(
                            lambda y, n=n, g=g: combine(it, n, y[8 * g:8 * g + 8]))
                r1 = pl.multiple_of(jnp.minimum(NPRE + RIDE * (s + 1), S - RIDE), 8)
                xn = xbuf[pl.ds(r1, RIDE), :].astype(f32)
                if u == 0:
                    for k in range(2):
                        rm = pl.multiple_of(it * 32 + k * 16, 16)
                        gacc = mod_rows(gacc, wsr[6, k * 16:(k + 1) * 16, :], rm)
                    hn = adaln_a(xn, _zero_after(stage_a16(ra)))
                else:
                    def refill(y):
                        for cp in stream_copies(jnp.minimum(it + 1, NSEG // 2 - 1)):
                            cp.start()
                        spare = pl.ds(pl.multiple_of(8 * (it // 64), 8), 8)
                        jobs["pin"] = _zero_after(ws3[16, spare, :].astype(f32))
                    jobs.setdefault(3 * (PIN - 4) + 2, []).append(refill)
                    hn = adaln_a(xn)
                    z = _zero_after(hn[0:8], hn[8:16], hn[16:24])
                    stage_a16(ra + 32, _zero_after(stage_a16(ra + 16, z)))
                a_lo, a_hi = step(it, u, lhs_lo, lhs_hi, jobs)
                lhs_lo = jnp.concatenate([a_lo[0:MEM], hn[:, 0:512]], axis=0).astype(bf16)
                lhs_hi = jnp.concatenate([a_hi[0:MEM], hn[:, 512:1024]], axis=0).astype(bf16)
                a = jnp.concatenate([a_lo, a_hi], axis=1)
                rt, rh, rf = ride_tiles(it, u)
                rows = [pl.ds(pl.multiple_of(16 * rt + 8 * rh, 8), 8),
                        pl.ds(pl.multiple_of(16 * rf, 16), 16)]
                xs = [xbuf[r, :].astype(f32) for r in rows]
                xbuf[rows[0], :] = (xs[0] + modrows(2, 8) * a[8:16]).astype(bf16)
                xbuf[rows[1], :] = (xs[1] + modrows(2, 16) * a[16:32]).astype(bf16)
            lhs_h[:, 0:512] = lhs_lo
            lhs_h[:, 512:1024] = lhs_hi
            return gacc

        gacc = _loop("rec", 0, NSEG // 2, rec_body, jnp.zeros((8, D), f32))
        for c in range(2):
            mod_finish(gacc[:, c * 512:(c + 1) * 512], 10 + c)
        stream_wait(NSEG // 2 - 1)

        def wo_prep(i, half, k):
            o = jnp.concatenate([_unpack(rings[4 * half + h][k, i]).astype(f32)
                                 for h in range(4)], axis=1)
            for t, op in enumerate(row_operands(o)):
                a7[half, t, k * 8:(k + 1) * 8, :] = op.astype(bf16)

        def wo_chunk(i, half, inext, extra):
            row = pl.multiple_of(i * 512 + half * 256, 256)
            todo = list(range(NPRE // 16))

            def hook(v):
                if todo:
                    for h in range(4):
                        rings[4 * (1 - half) + h][i // 64, 4] = pltpu.bitcast(v[0:8], u32)
                    n = 2 if len(todo) % WPP == 0 else 1
                    for k in todo[:n]:
                        wo_prep(inext, 1 - half, k)
                    del todo[:n]
                extra(v)

            for j in range(4):
                def b_of(k):
                    def quad(q):
                        r = WO + (j + 4 * (q % 2)) * 2048 + (q // 2) * 128 + row
                        return pltpu.bitcast(wqkv[pl.ds(r, 128), :], bf16)
                    qi, qj, sign = _BTERMS[k]
                    if qj is None:
                        return quad(qi)
                    u, v = quad(qi).astype(f32), quad(qj).astype(f32)
                    return (u + v if sign > 0 else u - v).astype(bf16)
                c11, c12, c21, c22 = _strassen(lambda k: a7[half, k], b_of, hook)
                for c, y in ((j + 4, _merge_rows(c12, c22)), (j, _merge_rows(c11, c21))):
                    cs = slice(c * 128, (c + 1) * 128)
                    h2buf[S - NPRE:S, cs] = h2buf[S - NPRE:S, cs] + y

        for k in range(NPRE // 16):
            wo_prep(0, 0, k)

        def wo_tail(i, _):
            st = {"n": 0, "prev": None}

            def extra(v):
                n = st["n"]
                st["n"] += 1
                if n % 16 == 2 and n // 16 < 3:
                    st["prev"] = stage_a16(S - NPRE - 48 + 16 * (n // 16),
                                           _zero_after(v, st["prev"]))
            wo_chunk(i, 0, i, extra)
            wo_chunk(i, 1, jnp.minimum(i + 1, 3), extra)
            return 0
        _loop("wotail", 0, 4, wo_tail)

        def gget(c, row, n):
            return pltpu.bitcast(wqkv[pl.ds(c * GS + row, n), :], f32)

        def gset(c, row, val):
            wqkv[pl.ds(c * GS + row, val.shape[0]), :] = pltpu.bitcast(val, u32)

        def wop(j):
            return lambda k: _unpack(w7[k, j * 32:(j + 1) * 32].reshape(256, 128))

        zpad = jnp.zeros((GPAD, 128), f32)
        for cb in range(8):
            gset(cb, 0, zpad)
            gset(cb, GPAD + S, zpad)

        shifts = (-1, -1, 1, 1, -2, -2, 2, 2)
        HB = MB // 2

        def shift_piece(r, half, k):
            gs = jnp.concatenate([gget(c, r + (k * 16 + GPAD + shifts[c]), 16)
                                  for c in range(8)], axis=1)
            ro = half * (HB // 2) + k * 8
            for t, op in enumerate(row_operands(gs)):
                n7[t, ro:ro + 8, :] = op.astype(bf16)

        def gate(v, i):
            gset(0, GPAD + S + GPAD + 8 * (i // S), v[0:8])

        def b_body(i, _):
            rl = S - NPRE + i * 128
            st = {"n": 0, "prev": [None, None]}

            def hook(v):
                n = st["n"]
                st["n"] += 1
                if n % BG == 0 and n // BG < 8:
                    k = n // BG
                    st["prev"][k % BCH] = stage_a16(rl + 16 * k,
                                                    _zero_after(v, st["prev"][k % BCH]),
                                                    (t7, 8 * k))

            ro = pl.multiple_of(i * 192, 64)
            for lhs, row in ((lambda k: n7[k, pl.ds(ro, 192), :], i * 384), (lambda k: t7[k], rl)):
                rg = pl.multiple_of(GPAD + row, 8)
                for j in range(4):
                    c11, c12, c21, c22 = _strassen(lhs, wop(j), hook)
                    gset(j + 4, rg, _gelu(_merge_rows(c12, c22)))
                    gset(j, rg, _gelu(_merge_rows(c11, c21)))
            return 0
        _loop("b", 0, S // MB, b_body)
        for k in range(HB // 16):
            shift_piece(0, 0, k)

        def n2_norm(r, k, anchor):
            v = _ln(h2buf[pl.ds(pl.multiple_of(r + k * 16, 16), 16), :], anchor)
            nrms[k // 2][(k % 2) * 16:(k % 2) * 16 + 16, :] = v
            return v[0:8] + v[8:16]

        def n2_ops(k, k1, v, i):
            nrm = nrms[k]
            nrm[pl.ds(pl.multiple_of(32 + 8 * (i // S), 8), 8), 0:128] = v[0:8]

            def quad(q):
                r0, c0 = (q // 2) * 16, (q % 2) * 512
                return [nrm[r0 + 8 * a:r0 + 8 * a + 8, c0 + 256 * b:c0 + 256 * b + 256]
                        for a in range(2) for b in range(2)]
            qi, qj, sign = _ATERMS[k1]
            blk = quad(qi)
            if qj is not None:
                blk = [u + w if sign > 0 else u - w for u, w in zip(blk, quad(qj))]
            for k2, op in enumerate(_a_operands(*blk)):
                d49[7 * k1 + k2, k * 8:(k + 1) * 8, :] = op.astype(bf16)

        def n2_hook(r, i, first, gap, lag, st):
            def hook(v):
                n = st["n"] - first
                st["n"] += 1
                if n >= 0 and n % gap == 0 and n // gap < MD // 16:
                    st["prev"] = n2_norm(r, n // gap, _zero_after(v, st["prev"]))
                for _ in range(st["per"]):
                    k, k1 = divmod(st["ops"], 7)
                    if k < MD // 32 and n >= (2 * k + 1) * gap + lag:
                        n2_ops(k, k1, v, i)
                        st["ops"] += 1
            return hook

        def stage_c(i, r, half, rnext, extra):
            rr = pl.multiple_of(r, 8)
            ro = half * (HB // 2)
            cnt = [0]

            def hook(v):
                n = cnt[0]
                cnt[0] += 1
                if n < HB // 16:
                    gate(v, i)
                    shift_piece(rnext, 1 - half, n)
                extra(v)

            for j in range(4):
                c11, c12, c21, c22 = _strassen(lambda k: n7[k, ro:ro + HB // 2, :], wop(4 + j),
                                               hook)
                for c, y in ((j + 4, _merge_rows(c12, c22)), (j, _merge_rows(c11, c21))):
                    cs = slice(c * 128, (c + 1) * 128)
                    h2buf[pl.ds(rr, HB), cs] = h2buf[pl.ds(rr, HB), cs] + y

        def c_body(i, _):
            r = pl.multiple_of(i * MB, MB)
            st = {"n": 0, "prev": None, "ops": 0, "per": 1}
            extra = n2_hook(0, i, 0, 4, 4, st)
            stage_c(i, r, 0, r + HB, extra)
            stage_c(i, r + HB, 1, jnp.minimum(i + 1, S // MB - 1) * MB, extra)
            assert st["ops"] == 28
            return 0
        _loop("c", 0, S // MB, c_body)

        def wop2(lo, n):
            return lambda k1, k: _unpack(w49[7 * k1 + k, lo:lo + n].reshape(8 * n, 128))

        def d_body(i, _):
            r = pl.multiple_of(i * MD, MD)
            rn = jnp.minimum(r + MD, S - MD)
            lhs = [d49[k] for k in range(49)]
            uops = []
            for t in range(7):
                cb = _strassen2(lambda k1, k: lhs[7 * k1 + k], wop2(t * 16, 16))
                uops.append(_a_operands2([[_gelu(c) for c in row] for row in cb]))
            ul = [[jnp.concatenate([u[k1][k] for u in uops], axis=1).astype(bf16)
                   for k in range(7)] for k1 in range(7)]
            st = {"n": 0, "prev": None, "ops": 0, "per": 1}
            hook = n2_hook(rn, i, DF, DG, DL, st)
            for t in range(2):
                cb = _strassen2(lambda k1, k: ul[k1][k], wop2(W4T + t * 56, 56), hook)
                for j in range(4):
                    y = jnp.concatenate([cb[q][j].reshape(MD // 32, 8, 128) for q in range(4)],
                                        axis=1).reshape(MD, 128)
                    c = 2 * j + t
                    cs = slice(c * 128, (c + 1) * 128)
                    gb = modrows(5, MD, c * 128, (c + 1) * 128)
                    o = xbuf[pl.ds(r, MD), cs].astype(f32) + gb * (h2buf[pl.ds(r, MD), cs] + y)
                    xbuf[pl.ds(r, MD), cs] = o.astype(bf16)
            assert st["ops"] == 28
            out_copy(r, MD).start()
            return 0
        _loop("d", 0, S // MD, d_body)

    pl.run_scoped(main,
                  pltpu.VMEM((7, 8 * 32, 8, 128), u32),
                  pltpu.VMEM((49, 2 * W4T, 8, 128), u32))

    out_copy(0, S).wait()


def _run(x, mem0, wq, wk, wv, wo, w1, w2, w3, w4, c, wmod):
    any_spec = pl.BlockSpec(memory_space=pl.ANY)
    return pl.pallas_call(
        _kernel,
        out_shape=jax.ShapeDtypeStruct((S, D), bf16),
        in_specs=[any_spec] * 12,
        out_specs=any_spec,
        scratch_shapes=[
            pltpu.VMEM((S + 2 * RIDE, D), bf16),
            pltpu.VMEM((WO + 8 * 2048, 128), u32),
            [pltpu.VMEM((NR // 16, 96 // NRING, 8, 128), u32)] * NRING,
            pltpu.VMEM((32, D), bf16),
            pltpu.VMEM((H, 16, 128), u32),
            pltpu.VMEM((2 * H, 8, 128), u32),
            pltpu.VMEM((12, 8, 512), f32),
            pltpu.VMEM((D, 128), f32),
            pltpu.VMEM((S, D), f32),
            pltpu.VMEM((7, (S - NPRE) // 2, 512), bf16),
            pltpu.VMEM((17, 64, 128), bf16),
            pltpu.VMEM((8, 32, D), bf16),
            pltpu.VMEM((7, 64, 512), bf16),
            pltpu.VMEM((2, 7, NPRE // 2, 256), bf16),
            pltpu.VMEM((49, MD // 4, 256), bf16),
            [pltpu.VMEM((40, D), f32)] * (MD // 32),
            pltpu.VMEM((1, D), bf16),
            pltpu.SemaphoreType.DMA((9 + NGRP + 2,)),
        ],
        compiler_params=pltpu.CompilerParams(vmem_limit_bytes=124 * 1024 * 1024,
                                             disable_bounds_checks=True,
                                             disable_semaphore_checks=True),
    )(x, mem0, wq, wk, wv, wo, w1, w2, w3, w4, c, wmod)


def pallas_adaLN_cond__memory_aug_recurrent_mem_tr__mixer_s_mlp__prompt_kernel(
    A_x, A_mem0, A_Wq, A_Wk, A_Wv, A_Wo, A_seg_len, B_x, B_w1, B_w2, B_w3, B_w4, c, w_mod,
):
    del B_x
    assert A_x.shape == (1, S, D) and A_mem0.shape == (1, MEM, D)
    assert isinstance(A_seg_len, int) is False or A_seg_len == SEG
    out = _run(A_x.reshape(S, D), A_mem0.reshape(MEM, D), A_Wq, A_Wk, A_Wv,
               A_Wo.reshape(H * DH, D),
               B_w1.reshape(2, D // 2, D), B_w2.reshape(2, D // 2, D),
               B_w3, B_w4.reshape(4, F // 4, D), c, w_mod)
    return out.reshape(1, S, D)
```

```python
import jax
import jax.numpy as jnp
from jax import lax
import jax.experimental.pallas as pl
import jax.experimental.pallas.tpu as pltpu

bf16 = jnp.bfloat16
f32 = jnp.float32
u32 = jnp.uint32

S = 2048
D = 1024
H = 32
DH = 128
F = 3584
MEM = 8
SEG = 32
NSEG = S // SEG
L = MEM + SEG
RIDE = 24
NPRE = S - RIDE * NSEG
NR = NPRE + 2 * SEG
ROFF = (-(S - NPRE)) % NR
WP = 516
NGRP = 12
NSLOT = 6
NMOD = 6
EPS = 1e-5
MD = 128
MB = 512
GPAD = 8
NRING = 8
RLP, WLP, RSK = 27, 22, 2
NWO = 3
BG, WPP, PIN, BCH = 2, 5, 6, 2
DF, DG, DL = 2, 10, 9
SLOTS = ([(0, n // 2, 3 * (n % 2)) for n in range(16)] + [(0, 96 + n, 0) for n in range(16)]
         + [(0, 112 + n // 2, 3 * (n % 2)) for n in range(32)])
DSA, DPA, DSB, DPB, KSPLIT = 6, 12, 6, 12, 2
X0 = NPRE + 2 * RIDE
W4T = 7 * 16
_ONLY = None


def _loop(name, lo, hi, body, init=0):
    if _ONLY is not None and name not in _ONLY:
        return init
    with _scope(name):
        return lax.fori_loop(lo, hi, body, init)


class _NoScope:
    def __init__(self, name):
        del name

    def __enter__(self):
        return self

    def __exit__(self, *a):
        return False


_scope = _NoScope


def _zero_after(*vs):
    bits = None
    for v in vs:
        if v is not None:
            b = pltpu.bitcast(v[0:8, 0:128], u32)
            bits = b if bits is None else bits | b
    return pltpu.bitcast((bits >> 31) >> 1, f32)


def _ln(x, anchor=None):
    if anchor is not None:
        z = jnp.concatenate([anchor] * (x.shape[0] // 8), axis=0)
        x = jnp.concatenate([x[:, 0:128] + z, x[:, 128:]], axis=1)
    mu = jnp.mean(x, axis=-1, keepdims=True)
    xc = x - mu
    var = jnp.mean(xc * xc, axis=-1, keepdims=True)
    return xc * lax.rsqrt(var + EPS)


def _gelu(x):
    inner = x * (0.7978845608028654 + (0.7978845608028654 * 0.044715) * (x * x))
    hx = 0.5 * x
    return hx + hx * jnp.tanh(inner)


def _split_rows(x):
    m, n = x.shape
    x3 = x.reshape(m // 16, 16, n)
    return x3[:, 0:8, :].reshape(m // 2, n), x3[:, 8:16, :].reshape(m // 2, n)


def _merge_rows(top, bot):
    m, n = top.shape
    return jnp.concatenate([top.reshape(m // 8, 8, n), bot.reshape(m // 8, 8, n)],
                           axis=1).reshape(2 * m, n)


def _a_operands(a11, a12, a21, a22):
    return [a11 + a22, a21 + a22, a11, a22, a11 + a12, a21 - a11, a12 - a22]


def _b_operands(b11, b12, b21, b22):
    return [b11 + b22, b11, b12 - b22, b21 - b11, b22, b11 + b12, b21 + b22]


_ATERMS = ((0, 3, 1), (2, 3, 1), (0, None, 0), (3, None, 0), (0, 1, 1), (2, 0, -1), (1, 3, -1))
_BTERMS = ((0, 3, 1), (0, None, 0), (1, 3, -1), (2, 0, -1), (3, None, 0), (0, 1, 1), (2, 3, 1))


def _strassen(a_of, b_of, hook=lambda v: None):
    def prod(k):
        return jnp.dot(a_of(k), b_of(k), preferred_element_type=f32)
    p5 = prod(4)
    hook(p5)
    p3 = prod(2)
    hook(p3)
    c12 = p3 + p5
    p4 = prod(3)
    hook(p4)
    c11 = p4 - p5
    p2 = prod(1)
    hook(p2)
    c21 = p2 + p4
    c22 = p3 - p2
    p1 = prod(0)
    hook(p1)
    c11 = prod(6) + (c11 + p1)
    hook(c11)
    c22 = prod(5) + (c22 + p1)
    hook(c22)
    return c11, c12, c21, c22


def _a_operands2(b):
    sub = [_a_operands(b[i][j], b[i][2 + j], b[2 + i][j], b[2 + i][2 + j])
           for i in range(2) for j in range(2)]
    return [_a_operands(*[t[k] for t in sub]) for k in range(7)]


def _strassen2(a_of, b_of, hook=lambda v: None):
    def prod(k1):
        return _strassen(lambda k: a_of(k1, k), lambda k: b_of(k1, k), hook)

    def add(x, y):
        return [p + q for p, q in zip(x, y)]

    def sub(x, y):
        return [p - q for p, q in zip(x, y)]
    p5 = prod(4)
    p3 = prod(2)
    c12 = add(p3, p5)
    p4 = prod(3)
    c11 = sub(p4, p5)
    p2 = prod(1)
    c21 = add(p2, p4)
    c22 = sub(p3, p2)
    p1 = prod(0)
    c11 = add(add(c11, p1), prod(6))
    c22 = add(add(c22, p1), prod(5))
    cq = (c11, c12, c21, c22)
    return [[cq[2 * (i // 2) + j // 2][2 * (i % 2) + j % 2] for j in range(4)] for i in range(4)]


def _pack8(v):
    return pltpu.bitcast(v.astype(bf16), u32)


def _unpack(w):
    return pltpu.bitcast(w, bf16)


def _kernel(x_hbm, mem0_hbm, wq_hbm, wk_hbm, wv_hbm, wo_hbm, w1_hbm, w2_hbm, w3_hbm, w4_hbm,
            c_hbm, wmod_hbm, out_hbm,
            xbuf, wqkv, rings, lhs_h, lhs_o, kvm, modv, scol, h2buf, n7, ws3, wsr, t7, a7, d49, nrms, c_ref,
            sems):
    w_hbms = (wq_hbm, wk_hbm, wv_hbm)
    SMOD, SSTG = 5, 9
    sem_x, sem_out, sem_w, sem_g, sem_r = (sems.at[k] for k in range(5))

    def rget(b, tile, n):
        return jnp.concatenate([rings[b % NRING][tile + e, b // NRING] for e in range(n)], axis=0)

    def rhalf(b, tile, half):
        return rings[b % NRING][tile, b // NRING, 4 * half:4 * half + 4, :]

    def rset(b, tile, half, val):
        rings[b % NRING][tile, b // NRING, 4 * half:4 * half + 4, :] = _pack8(val)

    x_copy = pltpu.make_async_copy(x_hbm.at[pl.ds(0, X0), :], xbuf.at[pl.ds(0, X0), :], sem_x)

    def stream_copies(c):
        al, lo = ((lambda v, m: v), min) if isinstance(c, int) else (pl.multiple_of, jnp.minimum)
        c3 = lo(c, 27)
        cps = [pltpu.make_async_copy(
            w3_hbm.at[pl.ds(al(i * 256 + (c3 % 4) * 64, 64), 64),
                      pl.ds(al(j * (F // 4) + (c3 // 4) * 128, 128), 128)],
            ws3.at[4 * i + j], sem_w) for i in range(4) for j in range(4)]
        dst = X0 + 2 * RIDE * c
        return [
            pltpu.make_async_copy(w4_hbm.at[:, pl.ds(al(c3 * 32, 32), 32), :],
                                  wsr.at[pl.ds(0, 4)], sem_g),
            pltpu.make_async_copy(w1_hbm.at[:, pl.ds(al(c * 16, 16), 16), :],
                                  wsr.at[pl.ds(4, 2), pl.ds(0, 16), :], sem_g),
            pltpu.make_async_copy(w2_hbm.at[:, pl.ds(al(c * 16, 16), 16), :],
                                  wsr.at[pl.ds(4, 2), pl.ds(16, 16), :], sem_g),
            pltpu.make_async_copy(wmod_hbm.at[pl.ds(al(c * 32, 32), 32), pl.ds(5 * D, D)],
                                  wsr.at[6], sem_g),
            pltpu.make_async_copy(x_hbm.at[pl.ds(al(lo(dst, S - 2 * RIDE), 16), 2 * RIDE), :],
                                  xbuf.at[pl.ds(al(dst, 16), 2 * RIDE), :], sem_r)] + cps

    def stream_wait(c):
        for dst, sem in ((ws3.at[pl.ds(0, 16)], sem_w), (wsr.at[pl.ds(0, 7)], sem_g),
                         (xbuf.at[pl.ds(X0 + 2 * RIDE * c, 2 * RIDE), :], sem_r)):
            pltpu.make_async_copy(dst, dst, sem).wait()

    def out_copy(row, n):
        return pltpu.make_async_copy(xbuf.at[pl.ds(row, n), :], out_hbm.at[pl.ds(row, n), :],
                                     sem_out)

    def mod_rows(acc, w, r):
        sc = jnp.concatenate([scol[pl.ds(r, 16), :]] * (w.shape[1] // 128), axis=1)
        p = w.astype(f32) * sc
        return acc + p[0:8] + p[8:16]

    def mod_finish(acc, j):
        is_scale = jnp.logical_or(j // 2 == 1, j // 2 == 4)
        tot = jnp.sum(acc, axis=0, keepdims=True) + jnp.where(is_scale, 1.0, 0.0)
        modv[j] = jnp.broadcast_to(tot, (8, 512))

    def modrows(k, n, lo=0, hi=D):
        m = jnp.concatenate([modv[2 * k], modv[2 * k + 1]], axis=1)[:, lo:hi]
        return jnp.concatenate([m] * (n // 8), axis=0)

    def adaln_a(xv, anchor=None):
        n = xv.shape[0]
        return _ln(xv, anchor) * modrows(1, n) + modrows(0, n)

    def adaln_b(xv, anchor=None):
        n = xv.shape[0]
        return _ln(xv, anchor) * modrows(4, n) + modrows(3, n)

    def row_operands(v):
        top, bot = _split_rows(v)
        k = v.shape[1] // 2
        return _a_operands(top[:, :k], top[:, k:], bot[:, :k], bot[:, k:])

    def stage_a16(r, anchor=None, dst=None):
        rr = pl.multiple_of(r, 16)
        xv = xbuf[pl.ds(rr, 16), :]
        if dst is not None:
            xv = (xv.astype(f32) + modrows(2, 16) * h2buf[pl.ds(rr, 16), :]).astype(bf16)
            xbuf[pl.ds(rr, 16), :] = xv
        h2 = adaln_b(xv.astype(f32), anchor)
        h2buf[pl.ds(rr, 16), :] = h2
        ref, ro = (n7, pl.multiple_of(rr // 2, 8)) if dst is None else dst
        ops = row_operands(_ln(h2))
        for t, op in enumerate(ops):
            ref[t, pl.ds(ro, 8), :] = op.astype(bf16)
        return ops[0]

    def prologue(stg, wos, wmodb, h7):
        def mod_copy(j):
            return pltpu.make_async_copy(wmod_hbm.at[:, pl.ds(j * 512, 512)], wmodb.at[j % NMOD],
                                         sems.at[SSTG + j + 4 if j >= 4 else SMOD + j])

        def piece_copy(g, dh):
            return pltpu.make_async_copy(
                w_hbms[g // 4].at[pl.ds(dh * 512, 512), pl.ds((g % 4) * 8, 8), :],
                stg.at[(2 * g + dh) % NSLOT], sems.at[SSTG + (g + 1 if g else dh)])

        def wo_copy(j):
            return pltpu.make_async_copy(wo_hbm.at[pl.ds(j * 512, 512), :], wos.at[j % NWO],
                                         sems.at[SSTG + j + 6])

        def group_start(g):
            for dh in range(2):
                piece_copy(g, dh).start()

        def stg_wait(slot, n, sem):
            dst = stg.at[pl.ds(slot, n)]
            pltpu.make_async_copy(dst, dst, sems.at[SSTG + sem]).wait()

        def relayout(g, slot, dh, lo_dp, n_dp):
            for u in range(n_dp):
                dp = lo_dp + u
                ev = pltpu.bitcast(stg[slot, 2 * dp].astype(f32), u32)
                od = pltpu.bitcast(stg[slot, 2 * dp + 1].astype(f32), u32)
                wqkv[g, pl.ds(dh * 256 + dp, 8, stride=WP), :] = (ev >> 16) | od

        def b_operand(g, q, k):
            def quad(i):
                r = (q + 4 * (i % 2)) * WP + (i // 2) * 256
                return _unpack(wqkv[g, r:r + 256, :])
            i, j, sign = _BTERMS[k]
            if j is None:
                return quad(i)
            u, v = quad(i).astype(f32), quad(j).astype(f32)
            return (u + v if sign > 0 else u - v).astype(bf16)

        c_copy = pltpu.make_async_copy(c_hbm, c_ref, sem_g)
        m_copy = pltpu.make_async_copy(mem0_hbm, lhs_h.at[pl.ds(0, MEM), :], sem_r)
        c_copy.start()
        m_copy.start()
        x_copy.start()
        for j in range(4):
            mod_copy(j).start()
        for g in range(3):
            group_start(g)
        h2buf[S - NPRE:S, :] = jnp.zeros((NPRE, D), f32)
        wos[2] = jnp.zeros((512, D), bf16)
        c_copy.wait()
        m_copy.wait()
        cv = c_ref[...].astype(f32)
        sv = jnp.broadcast_to(cv * (1.0 / (1.0 + jnp.exp(-cv))), (128, D))
        for k in range(8):
            scol[k * 128:(k + 1) * 128, :] = sv[:, k * 128:(k + 1) * 128].T
        x_copy.wait()

        def ln0_body(i, _):
            r = pl.multiple_of(i * 64, 64)
            h2buf[pl.ds(r, 64), :] = _ln(xbuf[pl.ds(r, 64), :].astype(f32))
            return 0
        lax.fori_loop(0, NPRE // 64, ln0_body, 0)

        def mod0_body(j, _):
            pltpu.make_async_copy(wmodb.at[j], wmodb.at[j], sems.at[SMOD + j]).wait()
            accs = [jnp.zeros((8, 512), f32)] * 2
            for k in range(64):
                accs[k % 2] = mod_rows(accs[k % 2], wmodb[j, k * 16:(k + 1) * 16, :], k * 16)
            mod_finish(accs[0] + accs[1], j)
            return 0
        _loop("mod0", 0, 4, mod0_body)

        def hpre_body(i, _):
            r = pl.multiple_of(i * 32, 32)
            hv = h2buf[pl.ds(r, 32), :] * modrows(1, 32) + modrows(0, 32)
            ro = pl.multiple_of(i * 8, 8)
            for t, op in enumerate(row_operands(hv)):
                h7[t, pl.ds(ro, 8), :] = pltpu.bitcast(op.astype(bf16), u32)
            return 0
        lax.fori_loop(0, NPRE // 32, hpre_body, 0)
        lhs_h[MEM:32, :] = adaln_a(xbuf[NPRE:NPRE + RIDE, :].astype(f32)).astype(bf16)

        def relayout_now(g, dh):
            def rl_body(t, _):
                relayout(g, 2 * g + dh, dh, t * 32, 32)
                return 0
            lax.fori_loop(0, 8, rl_body, 0)

        for dh in range(2):
            stg_wait(dh, 1, dh)
            relayout_now(0, dh)

        grp = lambda g: [piece_copy(g, 0), piece_copy(g, 1)]
        issue = {0: [wo_copy(0)], 1: grp(3) + grp(4), 2: grp(5) + [wo_copy(1), mod_copy(4)],
                 3: grp(6) + [mod_copy(5), mod_copy(6)], 4: grp(7) + [wo_copy(2)],
                 5: grp(8) + [wo_copy(3), mod_copy(7)], 6: grp(9) + [wo_copy(4)],
                 7: grp(10) + [wo_copy(5), mod_copy(8)], 8: grp(11) + [wo_copy(6)],
                 9: [wo_copy(7), mod_copy(9)], 10: stream_copies(0)}

        def pre_iter(g, m3):

            @pl.when(g == 1)
            def _():
                stg_wait(2, 2, 2)
                relayout_now(1, 0)
                relayout_now(1, 1)

            def slots():
                m3n = jnp.where(m3 == 2, 0, m3 + 1)
                cj = jnp.maximum(g - 2, 3)
                return (m3n, 2 * jnp.where(ends, m3, m3n),
                        jnp.where(jnp.logical_or(g < 4, m3 == 0), 2, m3 - 1),
                        cj, jnp.where(cj >= NMOD, cj - NMOD, cj))

            ends = jnp.logical_or(g == 0, g == NGRP - 1)

            @pl.when(jnp.logical_not(ends))
            def _():
                stg_wait(slots()[1], 2, g + 2)

            @pl.when(g >= 4)
            def _():
                buf = wos.at[slots()[2]]
                pltpu.make_async_copy(buf, buf, sems.at[SSTG + g + 2]).wait()

            @pl.when(g >= 6)
            def _():
                buf = wmodb.at[slots()[4]]
                pltpu.make_async_copy(buf, buf, sems.at[SSTG + g + 2]).wait()

            m3n, gslot, wslot, cj, cslot = slots()
            gn = jnp.where(ends, g, g + 1)
            wj = jnp.maximum(g - 4, 0)
            wgrp, wrow = NGRP + wj // 2, (wj % 2) * 256
            for k, cps in issue.items():
                @pl.when(g == k)
                def _():
                    for cp in cps:
                        cp.start()
            wtodo = [(r, c) for r in range(16) for c in range(8)]
            todo = [(dh, dp) for dh in range(2) for dp in range(256)]
            skip = [0] * RSK
            mtodo = list(range(0, D, 16))
            macc = [jnp.zeros((8, 512), f32)]

            def hook(v):
                if mtodo:
                    acc = macc[0] + jnp.concatenate([_zero_after(v)] * 4, axis=1)
                    for r in mtodo[:3]:
                        acc = mod_rows(acc, wmodb[cslot, r:r + 16, :], r)
                    del mtodo[:3]
                    macc[0] = acc

            for q in range(4):
                def b_of(k):
                    w = b_operand(g, q, k)
                    if skip:
                        skip.pop()
                        return w
                    nw = 0 if todo else WLP
                    for dh, dp in todo[:RLP]:
                        relayout(gn, gslot + dh, dh, dp, 1)
                    del todo[:RLP]
                    for r, c in wtodo[:nw]:
                        wqkv[wgrp, pl.ds(wrow + (c * 512 + r * 16), 16), :] = pltpu.bitcast(
                            wos[wslot, r * 32:(r + 1) * 32, c * 128:(c + 1) * 128], u32)
                    del wtodo[:nw]
                    return w
                c11, c12, c21, c22 = _strassen(lambda k: pltpu.bitcast(h7[k], bf16), b_of, hook)
                for blk, y in ((q + 4, _merge_rows(c12, c22)), (q, _merge_rows(c11, c21))):
                    for e in range(NPRE // 8):
                        tile, half = divmod(((8 * e + ROFF) % NR) // 8, 2)
                        rings[blk][tile, g, 4 * half:4 * half + 4, :] = _pack8(y[8 * e:8 * e + 8])
            assert not todo and not wtodo and not mtodo
            mod_finish(macc[0], cj)
            return m3n

        _loop("pre1", 0, NGRP, pre_iter)

    pl.run_scoped(prologue,
                  pltpu.VMEM((NSLOT, 512, 8, 128), bf16),
                  pltpu.VMEM((NWO, 512, D), bf16),
                  pltpu.VMEM((NMOD, D, 512), bf16),
                  pltpu.VMEM((7, NPRE // 4, 512), u32))

    def main(w7, w49):
        scale = DH ** -0.5
        ia = lax.broadcasted_iota(jnp.int32, (32, L), 0)
        ja = lax.broadcasted_iota(jnp.int32, (32, L), 1)
        mask_a = (((ia >= 16) & (ia < 24)) | (ja >= SEG)
                  | (jnp.where(ia < 16, ia + 16, ia - 16) >= ja))
        ib = lax.broadcasted_iota(jnp.int32, (48, 56), 0)
        jb = lax.broadcasted_iota(jnp.int32, (48, 56), 1)
        own = (ib < 40) == (jb < 40)
        mask_b = own & (((jb >= 32) & (jb < 48)) | (jnp.where(jb < 40, jb, jb - 8) <= ib))
        masked = -1e9 / scale
        j8 = lax.broadcasted_iota(jnp.int32, (8, 56), 1)
        fill_b = jnp.concatenate([jnp.where(j8 < 40, masked, -3e38).astype(f32)] * 5
                                 + [jnp.where(j8 < 40, -3e38, masked).astype(f32)], axis=0)

        def softmax(sc, mask, fill):
            sc = jnp.where(mask, sc, fill)
            mx = jnp.max(sc, axis=-1, keepdims=True)
            e = jnp.exp2((sc - mx) * (scale * 1.4426950408889634))
            den = jnp.sum(e, axis=-1, keepdims=True)
            return (e * pl.reciprocal(den, approx=True)).astype(bf16)

        def ride_tiles(it, is_b):
            first = (it == 0).astype(jnp.int32)
            if is_b:
                return 3 * it + 1 - first, 0, 3 * it + 2
            return 3 * it + 1 - first, 1, 3 * it + first

        def step(it, is_b, lhs_lo, lhs_hi, jobs):
            NT, TOFF = NR // 16, ROFF // 16
            sega = (4 * it + TOFF) % NT
            seg = sega + 2 if is_b else sega
            wt = [(3 * it + (NPRE // 16 + TOFF + t + is_b)) % NT for t in range(2)]
            wr = [(wt[(t + is_b) // 2], (t + is_b) % 2) for t in range(3)]
            rt, rh, rf = ride_tiles(it, is_b)
            rt, rf = (rt + TOFF) % NT, (rf + TOFF) % NT
            lhs = jnp.concatenate([lhs_lo, lhs_hi], axis=1)
            QM, P, PART = {}, {}, {}
            mrow = 0 if is_b else 4

            def wblk(b, lo, n):
                r = (b % 8) * WP + lo
                return _unpack(wqkv[b // 8, r:r + n, :])

            def qkv_lo(i):
                for m in range(3):
                    PART[(m, i)] = jnp.dot(lhs_lo, wblk(m * H + i, 0, 256), preferred_element_type=f32)

            def qkv(i):
                for m in range(3):
                    b = m * H + i
                    if (m, i) in PART:
                        y = jnp.dot(lhs_hi, wblk(b, 256, 256),
                                    preferred_element_type=f32) + PART.pop((m, i))
                    else:
                        y = jnp.dot(lhs, wblk(b, 0, 512), preferred_element_type=f32)
                    if m < 2:
                        QM[b] = y[0:MEM] + jobs["pin"] if b == PIN and is_b else y[0:MEM]
                    if m == 2 or (m == 1 and not is_b):
                        kvm[b - H, mrow:mrow + 4, :] = _pack8(y[0:MEM])
                    for t in range(3):
                        rset(b, *wr[t], y[8 + 8 * t:16 + 8 * t])
                    for job in jobs.get(3 * i + m, []):
                        job(y)
                    side(3 * i + m)

            def keys(b):
                if is_b:
                    if b in QM:
                        mix = jnp.concatenate([_pack8(QM.pop(b)), kvm[b - H, 4:8, :]], axis=0)
                    else:
                        mix = kvm[b - H]
                    return _unpack(jnp.concatenate([rget(b, seg, 2), mix, rhalf(b, sega, 0)], axis=0))
                mk = _pack8(QM.pop(b)) if b in QM else kvm[b - H, 4:8, :]
                return _unpack(jnp.concatenate([rget(b, seg, 2), mk], axis=0))

            def scores(i):
                if is_b:
                    q = [rget(i, seg, 2), _pack8(QM.pop(i)), rhalf(i, sega, 0)]
                else:
                    q = [rget(i, seg + 1, 1), _pack8(QM.pop(i)), rhalf(i, seg, 1)]
                sc = lax.dot_general(_unpack(jnp.concatenate(q, axis=0)), keys(H + i),
                                     (((1,), (1,)), ((), ())), preferred_element_type=f32)
                P[i] = softmax(sc, mask_b, fill_b) if is_b else softmax(sc, mask_a, masked)

            def pv(i):
                o = jnp.dot(P.pop(i), keys(2 * H + i), preferred_element_type=f32)
                if is_b:
                    for e in range(4):
                        rset(i, seg + e // 2, e % 2, o[8 * e:8 * e + 8])
                    rset(i, sega, 0, o[40:48])
                    lhs_o[i, 0:4, :] = _pack8(o[SEG:L])
                else:
                    for e in range(2):
                        rset(i, seg + 1, e, o[8 * e:8 * e + 8])
                    rset(i, seg, 1, o[24:32])
                    lhs_o[i, 0:4, :] = _pack8(o[16:24])
                lhs_o[i, 4:8, :] = rhalf(i, rt, rh)
                lhs_o[i, 8:16, :] = rget(i, rf, 1)

            def wo_lhs(i0, i1):
                return _unpack(jnp.concatenate([lhs_o[i] for i in range(i0, i1)], axis=1))

            def wo_dot(lo, j, k):
                w = _unpack(wqkv[NGRP + k, j * 512:(j + 1) * 512, :])
                return jnp.dot(lo, w, preferred_element_type=f32)

            def side(d):
                ds, dp = (DSB, DPB) if is_b else (DSA, DPA)
                if (d - dp) % 3 == 2 and 0 <= (d - dp) // 3 < H:
                    pv((d - dp) // 3)
                if (d - ds) % 3 == 2 and 0 <= (d - ds) // 3 < H:
                    scores((d - ds) // 3)

            if is_b:
                for h in range(KSPLIT):
                    qkv_lo(h)
            for h in range(H):
                qkv(h)
            lo = [wo_lhs(8 * k, 8 * k + 8) for k in range(3)]
            acc = []
            for j in range(8):
                y = None
                for k in range(3):
                    z = wo_dot(lo[k], j, k)
                    y = z if y is None else z + y
                    for job in jobs.get(96 + 3 * j + k, []):
                        job(y)
                    side(96 + 3 * j + k)
                acc.append(y)
            lo = wo_lhs(24, H)
            for j in range(8):
                acc[j] = wo_dot(lo, j, 3) + acc[j]
                for job in jobs.get(120 + j, []):
                    job(acc[j])
            assert not (QM or P or PART)
            return jnp.concatenate(acc[0:4], axis=1), jnp.concatenate(acc[4:8], axis=1)

        def combine(c, n, y):
            mp, k1 = divmod(n, 8)
            m, p = divmod(mp, 4)
            c3 = jnp.minimum(c, 27)
            spare = pl.ds(pl.multiple_of(8 * (c // 64), 8), 8)
            if m == 0 and k1 < 7:
                ws3[16, spare, :] = y.astype(bf16)
            else:
                wsr[7, spare, 0:128] = y.astype(bf16)
            if k1 == 7:
                dst, base, r = w7, 0, (4 * m + p) * 32 + c
                blk = [wsr[4 + i, m * 16:(m + 1) * 16, j * 512 + p * 128:j * 512 + (p + 1) * 128]
                       .astype(f32) for i in range(2) for j in range(2)]
            else:
                dst, base = w49, 7 * k1
                if m == 0:
                    r = c3 * 4 + p
                    get = lambda i, j: ws3[4 * i + j, p * 16:(p + 1) * 16, :]
                else:
                    r = W4T + (p // 2) * 56 + c3 * 2 + p % 2
                    r0, c0 = (p % 2) * 16, (p // 2) * 128
                    get = lambda i, j: wsr[i, r0:r0 + 16, j * 256 + c0:j * 256 + c0 + 128]

                def quad(q):
                    return [get(2 * (q // 2) + i, 2 * (q % 2) + j).astype(f32)
                            for i in range(2) for j in range(2)]
                qi, qj, sign = _BTERMS[k1]
                blk = quad(qi)
                if qj is not None:
                    blk = [u + v if sign > 0 else u - v for u, v in zip(blk, quad(qj))]
            for k, op in enumerate(_b_operands(*blk)):
                for e in range(2):
                    dst[base + k, r, 4 * e:4 * e + 4, :] = _pack8(op[8 * e:8 * e + 8])

        def rec_body(it, gacc):
            stream_wait(it)
            lhs_lo = lhs_h[:, 0:512]
            lhs_hi = lhs_h[:, 512:1024]
            ra = jnp.maximum(it - 1, 0) * (2 * RIDE)
            for u in range(2):
                s = 2 * it + u
                jobs = {}
                for n, (su, d, g) in enumerate(SLOTS):
                    if su == u:
                        jobs.setdefault(d, []).append(
                            lambda y, n=n, g=g: combine(it, n, y[8 * g:8 * g + 8]))
                r1 = pl.multiple_of(jnp.minimum(NPRE + RIDE * (s + 1), S - RIDE), 8)
                xn = xbuf[pl.ds(r1, RIDE), :].astype(f32)
                if u == 0:
                    for k in range(2):
                        rm = pl.multiple_of(it * 32 + k * 16, 16)
                        gacc = mod_rows(gacc, wsr[6, k * 16:(k + 1) * 16, :], rm)
                    hn = adaln_a(xn, _zero_after(stage_a16(ra)))
                else:
                    def refill(y):
                        for cp in stream_copies(jnp.minimum(it + 1, NSEG // 2 - 1)):
                            cp.start()
                        spare = pl.ds(pl.multiple_of(8 * (it // 64), 8), 8)
                        jobs["pin"] = _zero_after(ws3[16, spare, :].astype(f32))
                    jobs.setdefault(3 * (PIN - 4) + 2, []).append(refill)
                    hn = adaln_a(xn)
                    z = _zero_after(hn[0:8], hn[8:16], hn[16:24])
                    stage_a16(ra + 32, _zero_after(stage_a16(ra + 16, z)))
                a_lo, a_hi = step(it, u, lhs_lo, lhs_hi, jobs)
                lhs_lo = jnp.concatenate([a_lo[0:MEM], hn[:, 0:512]], axis=0).astype(bf16)
                lhs_hi = jnp.concatenate([a_hi[0:MEM], hn[:, 512:1024]], axis=0).astype(bf16)
                a = jnp.concatenate([a_lo, a_hi], axis=1)
                rt, rh, rf = ride_tiles(it, u)
                rows = [pl.ds(pl.multiple_of(16 * rt + 8 * rh, 8), 8),
                        pl.ds(pl.multiple_of(16 * rf, 16), 16)]
                xs = [xbuf[r, :].astype(f32) for r in rows]
                xbuf[rows[0], :] = (xs[0] + modrows(2, 8) * a[8:16]).astype(bf16)
                xbuf[rows[1], :] = (xs[1] + modrows(2, 16) * a[16:32]).astype(bf16)
            lhs_h[:, 0:512] = lhs_lo
            lhs_h[:, 512:1024] = lhs_hi
            return gacc

        gacc = _loop("rec", 0, NSEG // 2, rec_body, jnp.zeros((8, D), f32))
        for c in range(2):
            mod_finish(gacc[:, c * 512:(c + 1) * 512], 10 + c)
        stream_wait(NSEG // 2 - 1)

        def wo_prep(i, half, k):
            o = jnp.concatenate([_unpack(rings[4 * half + h][k, i]).astype(f32)
                                 for h in range(4)], axis=1)
            for t, op in enumerate(row_operands(o)):
                a7[half, t, k * 8:(k + 1) * 8, :] = op.astype(bf16)

        def wo_chunk(i, half, inext, extra):
            todo = list(range(NPRE // 16))

            def hook(v):
                if todo:
                    for h in range(4):
                        rings[4 * (1 - half) + h][i // 64, 4] = pltpu.bitcast(v[0:8], u32)
                    n = 2 if len(todo) % WPP == 0 else 1
                    for k in todo[:n]:
                        wo_prep(inext, 1 - half, k)
                    del todo[:n]
                extra(v)

            for j in range(4):
                def b_of(k):
                    def quad(q):
                        r = (j + 4 * (q % 2)) * 512 + half * 256 + (q // 2) * 128
                        return _unpack(wqkv[NGRP + i, r:r + 128, :])
                    qi, qj, sign = _BTERMS[k]
                    if qj is None:
                        return quad(qi)
                    u, v = quad(qi).astype(f32), quad(qj).astype(f32)
                    return (u + v if sign > 0 else u - v).astype(bf16)
                c11, c12, c21, c22 = _strassen(lambda k: a7[half, k], b_of, hook)
                for c, y in ((j + 4, _merge_rows(c12, c22)), (j, _merge_rows(c11, c21))):
                    cs = slice(c * 128, (c + 1) * 128)
                    h2buf[S - NPRE:S, cs] = h2buf[S - NPRE:S, cs] + y

        for k in range(NPRE // 16):
            wo_prep(0, 0, k)

        def wo_tail(i, _):
            st = {"n": 0, "prev": None}

            def extra(v):
                n = st["n"]
                st["n"] += 1
                if n % 16 == 2 and n // 16 < 3:
                    st["prev"] = stage_a16(S - NPRE - 48 + 16 * (n // 16),
                                           _zero_after(v, st["prev"]))
            wo_chunk(i, 0, i, extra)
            wo_chunk(i, 1, jnp.minimum(i + 1, 3), extra)
            return 0
        _loop("wotail", 0, 4, wo_tail)

        def gget(c, row, n):
            return pltpu.bitcast(wqkv[c, pl.ds(row, n), :], f32)

        def gset(c, row, val):
            wqkv[c, pl.ds(row, val.shape[0]), :] = pltpu.bitcast(val, u32)

        def wop(j):
            return lambda k: _unpack(w7[k, j * 32:(j + 1) * 32].reshape(256, 128))

        zpad = jnp.zeros((GPAD, 128), f32)
        for cb in range(8):
            gset(cb, 0, zpad)
            gset(cb, GPAD + S, zpad)

        shifts = (-1, -1, 1, 1, -2, -2, 2, 2)
        HB = MB // 2

        def shift_piece(r, half, k):
            gs = jnp.concatenate([gget(c, r + (k * 16 + GPAD + shifts[c]), 16)
                                  for c in range(8)], axis=1)
            ro = half * (HB // 2) + k * 8
            for t, op in enumerate(row_operands(gs)):
                n7[t, ro:ro + 8, :] = op.astype(bf16)

        def gate(v, i):
            gset(0, GPAD + S + GPAD + 8 * (i // S), v[0:8])

        def b_body(i, _):
            rl = S - NPRE + i * 128
            st = {"n": 0, "prev": [None, None]}

            def hook(v):
                n = st["n"]
                st["n"] += 1
                if n % BG == 0 and n // BG < 8:
                    k = n // BG
                    st["prev"][k % BCH] = stage_a16(rl + 16 * k,
                                                    _zero_after(v, st["prev"][k % BCH]),
                                                    (t7, 8 * k))

            ro = pl.multiple_of(i * 192, 64)
            for lhs, row in ((lambda k: n7[k, pl.ds(ro, 192), :], i * 384), (lambda k: t7[k], rl)):
                rg = pl.multiple_of(GPAD + row, 8)
                for j in range(4):
                    c11, c12, c21, c22 = _strassen(lhs, wop(j), hook)
                    gset(j + 4, rg, _gelu(_merge_rows(c12, c22)))
                    gset(j, rg, _gelu(_merge_rows(c11, c21)))
            return 0
        _loop("b", 0, S // MB, b_body)
        for k in range(HB // 16):
            shift_piece(0, 0, k)

        def n2_norm(r, k, anchor):
            v = _ln(h2buf[pl.ds(pl.multiple_of(r + k * 16, 16), 16), :], anchor)
            nrms[k // 2][(k % 2) * 16:(k % 2) * 16 + 16, :] = v
            return v[0:8] + v[8:16]

        def n2_ops(k, k1, v, i):
            nrm = nrms[k]
            nrm[pl.ds(pl.multiple_of(32 + 8 * (i // S), 8), 8), 0:128] = v[0:8]

            def quad(q):
                r0, c0 = (q // 2) * 16, (q % 2) * 512
                return [nrm[r0 + 8 * a:r0 + 8 * a + 8, c0 + 256 * b:c0 + 256 * b + 256]
                        for a in range(2) for b in range(2)]
            qi, qj, sign = _ATERMS[k1]
            blk = quad(qi)
            if qj is not None:
                blk = [u + w if sign > 0 else u - w for u, w in zip(blk, quad(qj))]
            for k2, op in enumerate(_a_operands(*blk)):
                d49[7 * k1 + k2, k * 8:(k + 1) * 8, :] = op.astype(bf16)

        def n2_hook(r, i, first, gap, lag, st):
            def hook(v):
                n = st["n"] - first
                st["n"] += 1
                if n >= 0 and n % gap == 0 and n // gap < MD // 16:
                    st["prev"] = n2_norm(r, n // gap, _zero_after(v, st["prev"]))
                for _ in range(st["per"]):
                    k, k1 = divmod(st["ops"], 7)
                    if k < MD // 32 and n >= (2 * k + 1) * gap + lag:
                        n2_ops(k, k1, v, i)
                        st["ops"] += 1
            return hook

        def stage_c(i, r, half, rnext, extra):
            rr = pl.multiple_of(r, 8)
            ro = half * (HB // 2)
            cnt = [0]

            def hook(v):
                n = cnt[0]
                cnt[0] += 1
                if n < HB // 16:
                    gate(v, i)
                    shift_piece(rnext, 1 - half, n)
                extra(v)

            for j in range(4):
                c11, c12, c21, c22 = _strassen(lambda k: n7[k, ro:ro + HB // 2, :], wop(4 + j),
                                               hook)
                for c, y in ((j + 4, _merge_rows(c12, c22)), (j, _merge_rows(c11, c21))):
                    cs = slice(c * 128, (c + 1) * 128)
                    h2buf[pl.ds(rr, HB), cs] = h2buf[pl.ds(rr, HB), cs] + y

        def c_body(i, _):
            r = pl.multiple_of(i * MB, MB)
            st = {"n": 0, "prev": None, "ops": 0, "per": 1}
            extra = n2_hook(0, i, 0, 4, 4, st)
            stage_c(i, r, 0, r + HB, extra)
            stage_c(i, r + HB, 1, jnp.minimum(i + 1, S // MB - 1) * MB, extra)
            assert st["ops"] == 28
            return 0
        _loop("c", 0, S // MB, c_body)

        def wop2(lo, n):
            return lambda k1, k: _unpack(w49[7 * k1 + k, lo:lo + n].reshape(8 * n, 128))

        def d_body(i, _):
            r = pl.multiple_of(i * MD, MD)
            rn = jnp.minimum(r + MD, S - MD)
            lhs = [d49[k] for k in range(49)]
            uops = []
            for t in range(7):
                cb = _strassen2(lambda k1, k: lhs[7 * k1 + k], wop2(t * 16, 16))
                uops.append(_a_operands2([[_gelu(c) for c in row] for row in cb]))
            ul = [[jnp.concatenate([u[k1][k] for u in uops], axis=1).astype(bf16)
                   for k in range(7)] for k1 in range(7)]
            st = {"n": 0, "prev": None, "ops": 0, "per": 1}
            hook = n2_hook(rn, i, DF, DG, DL, st)
            for t in range(2):
                cb = _strassen2(lambda k1, k: ul[k1][k], wop2(W4T + t * 56, 56), hook)
                for j in range(4):
                    y = jnp.concatenate([cb[q][j].reshape(MD // 32, 8, 128) for q in range(4)],
                                        axis=1).reshape(MD, 128)
                    c = 2 * j + t
                    cs = slice(c * 128, (c + 1) * 128)
                    gb = modrows(5, MD, c * 128, (c + 1) * 128)
                    o = xbuf[pl.ds(r, MD), cs].astype(f32) + gb * (h2buf[pl.ds(r, MD), cs] + y)
                    xbuf[pl.ds(r, MD), cs] = o.astype(bf16)
            assert st["ops"] == 28
            out_copy(r, MD).start()
            return 0
        _loop("d", 0, S // MD, d_body)

    pl.run_scoped(main,
                  pltpu.VMEM((7, 8 * 32, 8, 128), u32),
                  pltpu.VMEM((49, 2 * W4T, 8, 128), u32))

    out_copy(0, S).wait()


def _run(x, mem0, wq, wk, wv, wo, w1, w2, w3, w4, c, wmod):
    any_spec = pl.BlockSpec(memory_space=pl.ANY)
    return pl.pallas_call(
        _kernel,
        out_shape=jax.ShapeDtypeStruct((S, D), bf16),
        in_specs=[any_spec] * 12,
        out_specs=any_spec,
        scratch_shapes=[
            pltpu.VMEM((S + 2 * RIDE, D), bf16),
            pltpu.VMEM((NGRP + 4, 8 * WP, 128), u32),
            [pltpu.VMEM((NR // 16, 96 // NRING, 8, 128), u32)] * NRING,
            pltpu.VMEM((32, D), bf16),
            pltpu.VMEM((H, 16, 128), u32),
            pltpu.VMEM((2 * H, 8, 128), u32),
            pltpu.VMEM((12, 8, 512), f32),
            pltpu.VMEM((D, 128), f32),
            pltpu.VMEM((S, D), f32),
            pltpu.VMEM((7, (S - NPRE) // 2, 512), bf16),
            pltpu.VMEM((17, 64, 128), bf16),
            pltpu.VMEM((8, 32, D), bf16),
            pltpu.VMEM((7, 64, 512), bf16),
            pltpu.VMEM((2, 7, NPRE // 2, 256), bf16),
            pltpu.VMEM((49, MD // 4, 256), bf16),
            [pltpu.VMEM((40, D), f32)] * (MD // 32),
            pltpu.VMEM((1, D), bf16),
            pltpu.SemaphoreType.DMA((9 + NGRP + 2,)),
        ],
        compiler_params=pltpu.CompilerParams(vmem_limit_bytes=124 * 1024 * 1024,
                                             disable_bounds_checks=True,
                                             disable_semaphore_checks=True),
    )(x, mem0, wq, wk, wv, wo, w1, w2, w3, w4, c, wmod)


def pallas_adaLN_cond__memory_aug_recurrent_mem_tr__mixer_s_mlp__prompt_kernel(
    A_x, A_mem0, A_Wq, A_Wk, A_Wv, A_Wo, A_seg_len, B_x, B_w1, B_w2, B_w3, B_w4, c, w_mod,
):
    del B_x
    assert A_x.shape == (1, S, D) and A_mem0.shape == (1, MEM, D)
    assert isinstance(A_seg_len, int) is False or A_seg_len == SEG
    out = _run(A_x.reshape(S, D), A_mem0.reshape(MEM, D), A_Wq, A_Wk, A_Wv,
               A_Wo.reshape(H * DH, D),
               B_w1.reshape(2, D // 2, D), B_w2.reshape(2, D // 2, D),
               B_w3, B_w4.reshape(4, F // 4, D), c, w_mod)
    return out.reshape(1, S, D)
```

```python
import jax
import jax.numpy as jnp
from jax import lax
import jax.experimental.pallas as pl
import jax.experimental.pallas.tpu as pltpu

bf16 = jnp.bfloat16
f32 = jnp.float32
u32 = jnp.uint32

S = 2048
D = 1024
H = 32
DH = 128
F = 3584
MEM = 8
SEG = 32
NSEG = S // SEG
L = MEM + SEG
RIDE = 24
NPRE = S - RIDE * NSEG
NR = NPRE + 2 * SEG
ROFF = (-(S - NPRE)) % NR
WP = 516
NGRP = 12
NSLOT = 6
NMOD = 6
EPS = 1e-5
MD = 128
MB = 512
GPAD = 8
NRING = 8
NWO = 3
X0 = NPRE + 2 * RIDE
W4T = 7 * 16

RLP, WLP, RSK = 27, 22, 2
DSA, DPA, DSB, DPB = 6, 12, 6, 12
KSPLIT = 2
PIN = 6
SLOTS = ([(0, n // 2, 3 * (n % 2)) for n in range(16)] + [(0, 96 + n, 0) for n in range(16)]
         + [(0, 112 + n // 2, 3 * (n % 2)) for n in range(32)])
WPP, BG, BCH = 5, 2, 2
DF, DG, DL = 2, 10, 9
_ONLY = None


def _loop(name, lo, hi, body, init=0):
    if _ONLY is not None and name not in _ONLY:
        return init
    with _scope(name):
        return lax.fori_loop(lo, hi, body, init)


class _NoScope:
    def __init__(self, name):
        del name

    def __enter__(self):
        return self

    def __exit__(self, *a):
        return False


_scope = _NoScope


def _zero_after(*vs):
    bits = None
    for v in vs:
        if v is not None:
            b = pltpu.bitcast(v[0:8, 0:128], u32)
            bits = b if bits is None else bits | b
    return pltpu.bitcast((bits >> 31) >> 1, f32)


def _ln(x, anchor=None):
    if anchor is not None:
        z = jnp.concatenate([anchor] * (x.shape[0] // 8), axis=0)
        x = jnp.concatenate([x[:, 0:128] + z, x[:, 128:]], axis=1)
    mu = jnp.mean(x, axis=-1, keepdims=True)
    xc = x - mu
    var = jnp.mean(xc * xc, axis=-1, keepdims=True)
    return xc * lax.rsqrt(var + EPS)


def _gelu(x):
    inner = x * (0.7978845608028654 + (0.7978845608028654 * 0.044715) * (x * x))
    hx = 0.5 * x
    return hx + hx * jnp.tanh(inner)


def _split_rows(x):
    m, n = x.shape
    x3 = x.reshape(m // 16, 16, n)
    return x3[:, 0:8, :].reshape(m // 2, n), x3[:, 8:16, :].reshape(m // 2, n)


def _merge_rows(top, bot):
    m, n = top.shape
    return jnp.concatenate([top.reshape(m // 8, 8, n), bot.reshape(m // 8, 8, n)],
                           axis=1).reshape(2 * m, n)


def _a_operands(a11, a12, a21, a22):
    return [a11 + a22, a21 + a22, a11, a22, a11 + a12, a21 - a11, a12 - a22]


def _b_operands(b11, b12, b21, b22):
    return [b11 + b22, b11, b12 - b22, b21 - b11, b22, b11 + b12, b21 + b22]


_ATERMS = ((0, 3, 1), (2, 3, 1), (0, None, 0), (3, None, 0), (0, 1, 1), (2, 0, -1), (1, 3, -1))
_BTERMS = ((0, 3, 1), (0, None, 0), (1, 3, -1), (2, 0, -1), (3, None, 0), (0, 1, 1), (2, 3, 1))


def _strassen(a_of, b_of, hook=lambda v: None):
    def prod(k):
        return jnp.dot(a_of(k), b_of(k), preferred_element_type=f32)
    p5 = prod(4)
    hook(p5)
    p3 = prod(2)
    hook(p3)
    c12 = p3 + p5
    p4 = prod(3)
    hook(p4)
    c11 = p4 - p5
    p2 = prod(1)
    hook(p2)
    c21 = p2 + p4
    c22 = p3 - p2
    p1 = prod(0)
    hook(p1)
    c11 = prod(6) + (c11 + p1)
    hook(c11)
    c22 = prod(5) + (c22 + p1)
    hook(c22)
    return c11, c12, c21, c22


def _a_operands2(b):
    sub = [_a_operands(b[i][j], b[i][2 + j], b[2 + i][j], b[2 + i][2 + j])
           for i in range(2) for j in range(2)]
    return [_a_operands(*[t[k] for t in sub]) for k in range(7)]


def _strassen2(a_of, b_of, hook=lambda v: None):
    def prod(k1):
        return _strassen(lambda k: a_of(k1, k), lambda k: b_of(k1, k), hook)

    def add(x, y):
        return [p + q for p, q in zip(x, y)]

    def sub(x, y):
        return [p - q for p, q in zip(x, y)]
    p5 = prod(4)
    p3 = prod(2)
    c12 = add(p3, p5)
    p4 = prod(3)
    c11 = sub(p4, p5)
    p2 = prod(1)
    c21 = add(p2, p4)
    c22 = sub(p3, p2)
    p1 = prod(0)
    c11 = add(add(c11, p1), prod(6))
    c22 = add(add(c22, p1), prod(5))
    cq = (c11, c12, c21, c22)
    return [[cq[2 * (i // 2) + j // 2][2 * (i % 2) + j % 2] for j in range(4)] for i in range(4)]


def _pack8(v):
    return pltpu.bitcast(v.astype(bf16), u32)


def _unpack(w):
    return pltpu.bitcast(w, bf16)


def _kernel(x_hbm, mem0_hbm, wq_hbm, wk_hbm, wv_hbm, wo_hbm, w1_hbm, w2_hbm, w3_hbm, w4_hbm,
            c_hbm, wmod_hbm, out_hbm,
            xbuf, wqkv, rings, lhs_h, lhs_o, kvm, modv, scol, h2buf, n7, ws3, wsr, t7, a7, d49,
            nrms, c_ref, sems):
    w_hbms = (wq_hbm, wk_hbm, wv_hbm)
    SMOD, SSTG = 5, 9
    sem_x, sem_out, sem_w, sem_g, sem_r = (sems.at[k] for k in range(5))

    def rget(b, tile, n):
        return jnp.concatenate([rings[b % NRING][tile + e, b // NRING] for e in range(n)], axis=0)

    def rhalf(b, tile, half):
        return rings[b % NRING][tile, b // NRING, 4 * half:4 * half + 4, :]

    def rset(b, tile, half, val):
        rings[b % NRING][tile, b // NRING, 4 * half:4 * half + 4, :] = _pack8(val)

    x_copy = pltpu.make_async_copy(x_hbm.at[pl.ds(0, X0), :], xbuf.at[pl.ds(0, X0), :], sem_x)

    def stream_copies(c):
        al, lo = ((lambda v, m: v), min) if isinstance(c, int) else (pl.multiple_of, jnp.minimum)
        c3 = lo(c, 27)
        cps = [pltpu.make_async_copy(
            w3_hbm.at[pl.ds(al(i * 256 + (c3 % 4) * 64, 64), 64),
                      pl.ds(al(j * (F // 4) + (c3 // 4) * 128, 128), 128)],
            ws3.at[4 * i + j], sem_w) for i in range(4) for j in range(4)]
        dst = X0 + 2 * RIDE * c
        return [
            pltpu.make_async_copy(w4_hbm.at[:, pl.ds(al(c3 * 32, 32), 32), :],
                                  wsr.at[pl.ds(0, 4)], sem_g),
            pltpu.make_async_copy(w1_hbm.at[:, pl.ds(al(c * 16, 16), 16), :],
                                  wsr.at[pl.ds(4, 2), pl.ds(0, 16), :], sem_g),
            pltpu.make_async_copy(w2_hbm.at[:, pl.ds(al(c * 16, 16), 16), :],
                                  wsr.at[pl.ds(4, 2), pl.ds(16, 16), :], sem_g),
            pltpu.make_async_copy(wmod_hbm.at[pl.ds(al(c * 32, 32), 32), pl.ds(5 * D, D)],
                                  wsr.at[6], sem_g),
            pltpu.make_async_copy(x_hbm.at[pl.ds(al(lo(dst, S - 2 * RIDE), 16), 2 * RIDE), :],
                                  xbuf.at[pl.ds(al(dst, 16), 2 * RIDE), :], sem_r)] + cps

    def stream_wait(c):
        for dst, sem in ((ws3.at[pl.ds(0, 16)], sem_w), (wsr.at[pl.ds(0, 7)], sem_g),
                         (xbuf.at[pl.ds(X0 + 2 * RIDE * c, 2 * RIDE), :], sem_r)):
            pltpu.make_async_copy(dst, dst, sem).wait()

    def out_copy(row, n):
        return pltpu.make_async_copy(xbuf.at[pl.ds(row, n), :], out_hbm.at[pl.ds(row, n), :],
                                     sem_out)

    def mod_rows(acc, w, r):
        sc = jnp.concatenate([scol[pl.ds(r, 16), :]] * (w.shape[1] // 128), axis=1)
        p = w.astype(f32) * sc
        return acc + p[0:8] + p[8:16]

    def mod_finish(acc, j):
        is_scale = jnp.logical_or(j // 2 == 1, j // 2 == 4)
        tot = jnp.sum(acc, axis=0, keepdims=True) + jnp.where(is_scale, 1.0, 0.0)
        modv[j] = jnp.broadcast_to(tot, (8, 512))

    def modrows(k, n, lo=0, hi=D):
        m = jnp.concatenate([modv[2 * k], modv[2 * k + 1]], axis=1)[:, lo:hi]
        return jnp.concatenate([m] * (n // 8), axis=0)

    def adaln_a(xv, anchor=None):
        n = xv.shape[0]
        return _ln(xv, anchor) * modrows(1, n) + modrows(0, n)

    def adaln_b(xv, anchor=None):
        n = xv.shape[0]
        return _ln(xv, anchor) * modrows(4, n) + modrows(3, n)

    def row_operands(v):
        top, bot = _split_rows(v)
        k = v.shape[1] // 2
        return _a_operands(top[:, :k], top[:, k:], bot[:, :k], bot[:, k:])

    def stage_a16(r, anchor=None, dst=None):
        rr = pl.multiple_of(r, 16)
        xv = xbuf[pl.ds(rr, 16), :]
        if dst is not None:
            xv = (xv.astype(f32) + modrows(2, 16) * h2buf[pl.ds(rr, 16), :]).astype(bf16)
            xbuf[pl.ds(rr, 16), :] = xv
        h2 = adaln_b(xv.astype(f32), anchor)
        h2buf[pl.ds(rr, 16), :] = h2
        ref, ro = (n7, pl.multiple_of(rr // 2, 8)) if dst is None else dst
        ops = row_operands(_ln(h2))
        for t, op in enumerate(ops):
            ref[t, pl.ds(ro, 8), :] = op.astype(bf16)
        return ops[0]

    def prologue(stg, wos, wmodb, h7):
        def mod_copy(j):
            return pltpu.make_async_copy(wmod_hbm.at[:, pl.ds(j * 512, 512)], wmodb.at[j % NMOD],
                                         sems.at[SSTG + j + 4 if j >= 4 else SMOD + j])

        def piece_copy(g, dh):
            return pltpu.make_async_copy(
                w_hbms[g // 4].at[pl.ds(dh * 512, 512), pl.ds((g % 4) * 8, 8), :],
                stg.at[(2 * g + dh) % NSLOT], sems.at[SSTG + (g + 1 if g else dh)])

        def wo_copy(j):
            return pltpu.make_async_copy(wo_hbm.at[pl.ds(j * 512, 512), :], wos.at[j % NWO],
                                         sems.at[SSTG + j + 6])

        def group_start(g):
            for dh in range(2):
                piece_copy(g, dh).start()

        def stg_wait(slot, n, sem):
            dst = stg.at[pl.ds(slot, n)]
            pltpu.make_async_copy(dst, dst, sems.at[SSTG + sem]).wait()

        def relayout(g, slot, dh, lo_dp, n_dp):
            for u in range(n_dp):
                dp = lo_dp + u
                ev = pltpu.bitcast(stg[slot, 2 * dp].astype(f32), u32)
                od = pltpu.bitcast(stg[slot, 2 * dp + 1].astype(f32), u32)
                wqkv[g, pl.ds(dh * 256 + dp, 8, stride=WP), :] = (ev >> 16) | od

        def b_operand(g, q, k):
            def quad(i):
                r = (q + 4 * (i % 2)) * WP + (i // 2) * 256
                return _unpack(wqkv[g, r:r + 256, :])
            i, j, sign = _BTERMS[k]
            if j is None:
                return quad(i)
            u, v = quad(i).astype(f32), quad(j).astype(f32)
            return (u + v if sign > 0 else u - v).astype(bf16)

        c_copy = pltpu.make_async_copy(c_hbm, c_ref, sem_g)
        m_copy = pltpu.make_async_copy(mem0_hbm, lhs_h.at[pl.ds(0, MEM), :], sem_r)
        c_copy.start()
        m_copy.start()
        x_copy.start()
        for j in range(4):
            mod_copy(j).start()
        for g in range(3):
            group_start(g)
        h2buf[S - NPRE:S, :] = jnp.zeros((NPRE, D), f32)
        wos[2] = jnp.zeros((512, D), bf16)
        c_copy.wait()
        m_copy.wait()
        cv = c_ref[...].astype(f32)
        sv = jnp.broadcast_to(cv * (1.0 / (1.0 + jnp.exp(-cv))), (128, D))
        for k in range(8):
            scol[k * 128:(k + 1) * 128, :] = sv[:, k * 128:(k + 1) * 128].T
        x_copy.wait()

        def ln0_body(i, _):
            r = pl.multiple_of(i * 64, 64)
            h2buf[pl.ds(r, 64), :] = _ln(xbuf[pl.ds(r, 64), :].astype(f32))
            return 0
        lax.fori_loop(0, NPRE // 64, ln0_body, 0)

        def mod0_body(j, _):
            pltpu.make_async_copy(wmodb.at[j], wmodb.at[j], sems.at[SMOD + j]).wait()
            accs = [jnp.zeros((8, 512), f32)] * 2
            for k in range(64):
                accs[k % 2] = mod_rows(accs[k % 2], wmodb[j, k * 16:(k + 1) * 16, :], k * 16)
            mod_finish(accs[0] + accs[1], j)
            return 0
        _loop("mod0", 0, 4, mod0_body)

        def hpre_body(i, _):
            r = pl.multiple_of(i * 32, 32)
            hv = h2buf[pl.ds(r, 32), :] * modrows(1, 32) + modrows(0, 32)
            ro = pl.multiple_of(i * 8, 8)
            for t, op in enumerate(row_operands(hv)):
                h7[t, pl.ds(ro, 8), :] = pltpu.bitcast(op.astype(bf16), u32)
            return 0
        lax.fori_loop(0, NPRE // 32, hpre_body, 0)
        lhs_h[MEM:32, :] = adaln_a(xbuf[NPRE:NPRE + RIDE, :].astype(f32)).astype(bf16)

        def relayout_now(g, dh):
            def rl_body(t, _):
                relayout(g, 2 * g + dh, dh, t * 32, 32)
                return 0
            lax.fori_loop(0, 8, rl_body, 0)

        for dh in range(2):
            stg_wait(dh, 1, dh)
            relayout_now(0, dh)

        grp = lambda g: [piece_copy(g, 0), piece_copy(g, 1)]
        issue = {0: [wo_copy(0)], 1: grp(3) + grp(4), 2: grp(5) + [wo_copy(1), mod_copy(4)],
                 3: grp(6) + [mod_copy(5), mod_copy(6)], 4: grp(7) + [wo_copy(2)],
                 5: grp(8) + [wo_copy(3), mod_copy(7)], 6: grp(9) + [wo_copy(4)],
                 7: grp(10) + [wo_copy(5), mod_copy(8)], 8: grp(11) + [wo_copy(6)],
                 9: [wo_copy(7), mod_copy(9)], 10: stream_copies(0)}

        def pre_iter(g, m3):

            @pl.when(g == 1)
            def _():
                stg_wait(2, 2, 2)
                relayout_now(1, 0)
                relayout_now(1, 1)

            def slots():
                m3n = jnp.where(m3 == 2, 0, m3 + 1)
                cj = jnp.maximum(g - 2, 3)
                return (m3n, 2 * jnp.where(ends, m3, m3n),
                        jnp.where(jnp.logical_or(g < 4, m3 == 0), 2, m3 - 1),
                        cj, jnp.where(cj >= NMOD, cj - NMOD, cj))

            ends = jnp.logical_or(g == 0, g == NGRP - 1)

            @pl.when(jnp.logical_not(ends))
            def _():
                stg_wait(slots()[1], 2, g + 2)

            @pl.when(g >= 4)
            def _():
                buf = wos.at[slots()[2]]
                pltpu.make_async_copy(buf, buf, sems.at[SSTG + g + 2]).wait()

            @pl.when(g >= 6)
            def _():
                buf = wmodb.at[slots()[4]]
                pltpu.make_async_copy(buf, buf, sems.at[SSTG + g + 2]).wait()

            m3n, gslot, wslot, cj, cslot = slots()
            gn = jnp.where(ends, g, g + 1)
            wj = jnp.maximum(g - 4, 0)
            wgrp, wrow = NGRP + wj // 2, (wj % 2) * 256
            for k, cps in issue.items():
                @pl.when(g == k)
                def _():
                    for cp in cps:
                        cp.start()
            wtodo = [(r, c) for r in range(16) for c in range(8)]
            todo = [(dh, dp) for dh in range(2) for dp in range(256)]
            skip = [0] * RSK
            mtodo = list(range(0, D, 16))
            macc = [jnp.zeros((8, 512), f32)]

            def hook(v):
                if mtodo:
                    acc = macc[0] + jnp.concatenate([_zero_after(v)] * 4, axis=1)
                    for r in mtodo[:3]:
                        acc = mod_rows(acc, wmodb[cslot, r:r + 16, :], r)
                    del mtodo[:3]
                    macc[0] = acc

            for q in range(4):
                def b_of(k):
                    w = b_operand(g, q, k)
                    if skip:
                        skip.pop()
                        return w
                    nw = 0 if todo else WLP
                    for dh, dp in todo[:RLP]:
                        relayout(gn, gslot + dh, dh, dp, 1)
                    del todo[:RLP]
                    for r, c in wtodo[:nw]:
                        wqkv[wgrp, pl.ds(wrow + (c * 512 + r * 16), 16), :] = pltpu.bitcast(
                            wos[wslot, r * 32:(r + 1) * 32, c * 128:(c + 1) * 128], u32)
                    del wtodo[:nw]
                    return w
                c11, c12, c21, c22 = _strassen(lambda k: pltpu.bitcast(h7[k], bf16), b_of, hook)
                for blk, y in ((q + 4, _merge_rows(c12, c22)), (q, _merge_rows(c11, c21))):
                    for e in range(NPRE // 8):
                        tile, half = divmod(((8 * e + ROFF) % NR) // 8, 2)
                        rings[blk][tile, g, 4 * half:4 * half + 4, :] = _pack8(y[8 * e:8 * e + 8])
            assert not todo and not wtodo and not mtodo
            mod_finish(macc[0], cj)
            return m3n

        _loop("pre1", 0, NGRP, pre_iter)

    pl.run_scoped(prologue,
                  pltpu.VMEM((NSLOT, 512, 8, 128), bf16),
                  pltpu.VMEM((NWO, 512, D), bf16),
                  pltpu.VMEM((NMOD, D, 512), bf16),
                  pltpu.VMEM((7, NPRE // 4, 512), u32))

    def main(w7, w49):
        scale = DH ** -0.5
        ia = lax.broadcasted_iota(jnp.int32, (32, L), 0)
        ja = lax.broadcasted_iota(jnp.int32, (32, L), 1)
        mask_a = (((ia >= 16) & (ia < 24)) | (ja >= SEG)
                  | (jnp.where(ia < 16, ia + 16, ia - 16) >= ja))
        ib = lax.broadcasted_iota(jnp.int32, (48, 56), 0)
        jb = lax.broadcasted_iota(jnp.int32, (48, 56), 1)
        own = (ib < 40) == (jb < 40)
        mask_b = own & (((jb >= 32) & (jb < 48)) | (jnp.where(jb < 40, jb, jb - 8) <= ib))
        masked = -1e9 / scale
        j8 = lax.broadcasted_iota(jnp.int32, (8, 56), 1)
        fill_b = jnp.concatenate([jnp.where(j8 < 40, masked, -3e38).astype(f32)] * 5
                                 + [jnp.where(j8 < 40, -3e38, masked).astype(f32)], axis=0)

        def softmax(sc, mask, fill):
            sc = jnp.where(mask, sc, fill)
            mx = jnp.max(sc, axis=-1, keepdims=True)
            e = jnp.exp2((sc - mx) * (scale * 1.4426950408889634))
            den = jnp.sum(e, axis=-1, keepdims=True)
            return (e * pl.reciprocal(den, approx=True)).astype(bf16)

        def ride_tiles(it, is_b):
            first = (it == 0).astype(jnp.int32)
            if is_b:
                return 3 * it + 1 - first, 0, 3 * it + 2
            return 3 * it + 1 - first, 1, 3 * it + first

        def step(it, is_b, lhs_lo, lhs_hi, jobs):
            NT, TOFF = NR // 16, ROFF // 16
            sega = (4 * it + TOFF) % NT
            seg = sega + 2 if is_b else sega
            wt = [(3 * it + (NPRE // 16 + TOFF + t + is_b)) % NT for t in range(2)]
            wr = [(wt[(t + is_b) // 2], (t + is_b) % 2) for t in range(3)]
            rt, rh, rf = ride_tiles(it, is_b)
            rt, rf = (rt + TOFF) % NT, (rf + TOFF) % NT
            lhs = jnp.concatenate([lhs_lo, lhs_hi], axis=1)
            QM, P, PART = {}, {}, {}
            mrow = 0 if is_b else 4

            def wblk(b, lo, n):
                r = (b % 8) * WP + lo
                return _unpack(wqkv[b // 8, r:r + n, :])

            def qkv_lo(i):
                for m in range(3):
                    PART[(m, i)] = jnp.dot(lhs_lo, wblk(m * H + i, 0, 256), preferred_element_type=f32)

            def qkv(i):
                for m in range(3):
                    b = m * H + i
                    if (m, i) in PART:
                        y = jnp.dot(lhs_hi, wblk(b, 256, 256),
                                    preferred_element_type=f32) + PART.pop((m, i))
                    else:
                        y = jnp.dot(lhs, wblk(b, 0, 512), preferred_element_type=f32)
                    if m < 2:
                        QM[b] = y[0:MEM] + jobs["pin"] if b == PIN and is_b else y[0:MEM]
                    if m == 2 or (m == 1 and not is_b):
                        kvm[b - H, mrow:mrow + 4, :] = _pack8(y[0:MEM])
                    for t in range(3):
                        rset(b, *wr[t], y[8 + 8 * t:16 + 8 * t])
                    for job in jobs.get(3 * i + m, []):
                        job(y)
                    side(3 * i + m)

            def keys(b):
                if is_b:
                    if b in QM:
                        mix = jnp.concatenate([_pack8(QM.pop(b)), kvm[b - H, 4:8, :]], axis=0)
                    else:
                        mix = kvm[b - H]
                    return _unpack(jnp.concatenate([rget(b, seg, 2), mix, rhalf(b, sega, 0)], axis=0))
                mk = _pack8(QM.pop(b)) if b in QM else kvm[b - H, 4:8, :]
                return _unpack(jnp.concatenate([rget(b, seg, 2), mk], axis=0))

            def scores(i):
                if is_b:
                    q = [rget(i, seg, 2), _pack8(QM.pop(i)), rhalf(i, sega, 0)]
                else:
                    q = [rget(i, seg + 1, 1), _pack8(QM.pop(i)), rhalf(i, seg, 1)]
                sc = lax.dot_general(_unpack(jnp.concatenate(q, axis=0)), keys(H + i),
                                     (((1,), (1,)), ((), ())), preferred_element_type=f32)
                P[i] = softmax(sc, mask_b, fill_b) if is_b else softmax(sc, mask_a, masked)

            def pv(i):
                o = jnp.dot(P.pop(i), keys(2 * H + i), preferred_element_type=f32)
                if is_b:
                    for e in range(4):
                        rset(i, seg + e // 2, e % 2, o[8 * e:8 * e + 8])
                    rset(i, sega, 0, o[40:48])
                    lhs_o[i, 0:4, :] = _pack8(o[SEG:L])
                else:
                    for e in range(2):
                        rset(i, seg + 1, e, o[8 * e:8 * e + 8])
                    rset(i, seg, 1, o[24:32])
                    lhs_o[i, 0:4, :] = _pack8(o[16:24])
                lhs_o[i, 4:8, :] = rhalf(i, rt, rh)
                lhs_o[i, 8:16, :] = rget(i, rf, 1)

            def wo_lhs(i0, i1):
                return _unpack(jnp.concatenate([lhs_o[i] for i in range(i0, i1)], axis=1))

            def wo_dot(lo, j, k):
                w = _unpack(wqkv[NGRP + k, j * 512:(j + 1) * 512, :])
                return jnp.dot(lo, w, preferred_element_type=f32)

            def side(d):
                ds, dp = (DSB, DPB) if is_b else (DSA, DPA)
                if (d - dp) % 3 == 2 and 0 <= (d - dp) // 3 < H:
                    pv((d - dp) // 3)
                if (d - ds) % 3 == 2 and 0 <= (d - ds) // 3 < H:
                    scores((d - ds) // 3)

            if is_b:
                for h in range(KSPLIT):
                    qkv_lo(h)
            for h in range(H):
                qkv(h)
            lo = [wo_lhs(8 * k, 8 * k + 8) for k in range(3)]
            acc = []
            for j in range(8):
                y = None
                for k in range(3):
                    z = wo_dot(lo[k], j, k)
                    y = z if y is None else z + y
                    for job in jobs.get(96 + 3 * j + k, []):
                        job(y)
                    side(96 + 3 * j + k)
                acc.append(y)
            lo = wo_lhs(24, H)
            for j in range(8):
                acc[j] = wo_dot(lo, j, 3) + acc[j]
                for job in jobs.get(120 + j, []):
                    job(acc[j])
            assert not (QM or P or PART)
            return jnp.concatenate(acc[0:4], axis=1), jnp.concatenate(acc[4:8], axis=1)

        def combine(c, n, y):
            mp, k1 = divmod(n, 8)
            m, p = divmod(mp, 4)
            c3 = jnp.minimum(c, 27)
            spare = pl.ds(pl.multiple_of(8 * (c // 64), 8), 8)
            if m == 0 and k1 < 7:
                ws3[16, spare, :] = y.astype(bf16)
            else:
                wsr[7, spare, 0:128] = y.astype(bf16)
            if k1 == 7:
                dst, base, r = w7, 0, (4 * m + p) * 32 + c
                blk = [wsr[4 + i, m * 16:(m + 1) * 16, j * 512 + p * 128:j * 512 + (p + 1) * 128]
                       .astype(f32) for i in range(2) for j in range(2)]
            else:
                dst, base = w49, 7 * k1
                if m == 0:
                    r = c3 * 4 + p
                    get = lambda i, j: ws3[4 * i + j, p * 16:(p + 1) * 16, :]
                else:
                    r = W4T + (p // 2) * 56 + c3 * 2 + p % 2
                    r0, c0 = (p % 2) * 16, (p // 2) * 128
                    get = lambda i, j: wsr[i, r0:r0 + 16, j * 256 + c0:j * 256 + c0 + 128]

                def quad(q):
                    return [get(2 * (q // 2) + i, 2 * (q % 2) + j).astype(f32)
                            for i in range(2) for j in range(2)]
                qi, qj, sign = _BTERMS[k1]
                blk = quad(qi)
                if qj is not None:
                    blk = [u + v if sign > 0 else u - v for u, v in zip(blk, quad(qj))]
            for k, op in enumerate(_b_operands(*blk)):
                for e in range(2):
                    dst[base + k, r, 4 * e:4 * e + 4, :] = _pack8(op[8 * e:8 * e + 8])

        def rec_body(it, gacc):
            stream_wait(it)
            lhs_lo = lhs_h[:, 0:512]
            lhs_hi = lhs_h[:, 512:1024]
            ra = jnp.maximum(it - 1, 0) * (2 * RIDE)
            for u in range(2):
                s = 2 * it + u
                jobs = {}
                for n, (su, d, g) in enumerate(SLOTS):
                    if su == u:
                        jobs.setdefault(d, []).append(
                            lambda y, n=n, g=g: combine(it, n, y[8 * g:8 * g + 8]))
                r1 = pl.multiple_of(jnp.minimum(NPRE + RIDE * (s + 1), S - RIDE), 8)
                xn = xbuf[pl.ds(r1, RIDE), :].astype(f32)
                if u == 0:
                    for k in range(2):
                        rm = pl.multiple_of(it * 32 + k * 16, 16)
                        gacc = mod_rows(gacc, wsr[6, k * 16:(k + 1) * 16, :], rm)
                    hn = adaln_a(xn, _zero_after(stage_a16(ra)))
                else:
                    def refill(y):
                        for cp in stream_copies(jnp.minimum(it + 1, NSEG // 2 - 1)):
                            cp.start()
                        spare = pl.ds(pl.multiple_of(8 * (it // 64), 8), 8)
                        jobs["pin"] = _zero_after(ws3[16, spare, :].astype(f32))
                    jobs.setdefault(3 * (PIN - 4) + 2, []).append(refill)
                    hn = adaln_a(xn)
                    z = _zero_after(hn[0:8], hn[8:16], hn[16:24])
                    stage_a16(ra + 32, _zero_after(stage_a16(ra + 16, z)))
                a_lo, a_hi = step(it, u, lhs_lo, lhs_hi, jobs)
                lhs_lo = jnp.concatenate([a_lo[0:MEM], hn[:, 0:512]], axis=0).astype(bf16)
                lhs_hi = jnp.concatenate([a_hi[0:MEM], hn[:, 512:1024]], axis=0).astype(bf16)
                a = jnp.concatenate([a_lo, a_hi], axis=1)
                rt, rh, rf = ride_tiles(it, u)
                rows = [pl.ds(pl.multiple_of(16 * rt + 8 * rh, 8), 8),
                        pl.ds(pl.multiple_of(16 * rf, 16), 16)]
                xs = [xbuf[r, :].astype(f32) for r in rows]
                xbuf[rows[0], :] = (xs[0] + modrows(2, 8) * a[8:16]).astype(bf16)
                xbuf[rows[1], :] = (xs[1] + modrows(2, 16) * a[16:32]).astype(bf16)
            lhs_h[:, 0:512] = lhs_lo
            lhs_h[:, 512:1024] = lhs_hi
            return gacc

        gacc = _loop("rec", 0, NSEG // 2, rec_body, jnp.zeros((8, D), f32))
        for c in range(2):
            mod_finish(gacc[:, c * 512:(c + 1) * 512], 10 + c)
        stream_wait(NSEG // 2 - 1)

        def wo_prep(i, half, k):
            o = jnp.concatenate([_unpack(rings[4 * half + h][k, i]).astype(f32)
                                 for h in range(4)], axis=1)
            for t, op in enumerate(row_operands(o)):
                a7[half, t, k * 8:(k + 1) * 8, :] = op.astype(bf16)

        def wo_chunk(i, half, inext, extra):
            todo = list(range(NPRE // 16))

            def hook(v):
                if todo:
                    for h in range(4):
                        rings[4 * (1 - half) + h][i // 64, 4] = pltpu.bitcast(v[0:8], u32)
                    n = 2 if len(todo) % WPP == 0 else 1
                    for k in todo[:n]:
                        wo_prep(inext, 1 - half, k)
                    del todo[:n]
                extra(v)

            for j in range(4):
                def b_of(k):
                    def quad(q):
                        r = (j + 4 * (q % 2)) * 512 + half * 256 + (q // 2) * 128
                        return _unpack(wqkv[NGRP + i, r:r + 128, :])
                    qi, qj, sign = _BTERMS[k]
                    if qj is None:
                        return quad(qi)
                    u, v = quad(qi).astype(f32), quad(qj).astype(f32)
                    return (u + v if sign > 0 else u - v).astype(bf16)
                c11, c12, c21, c22 = _strassen(lambda k: a7[half, k], b_of, hook)
                for c, y in ((j + 4, _merge_rows(c12, c22)), (j, _merge_rows(c11, c21))):
                    cs = slice(c * 128, (c + 1) * 128)
                    h2buf[S - NPRE:S, cs] = h2buf[S - NPRE:S, cs] + y

        for k in range(NPRE // 16):
            wo_prep(0, 0, k)

        def wo_tail(i, _):
            st = {"n": 0, "prev": None}

            def extra(v):
                n = st["n"]
                st["n"] += 1
                if n % 16 == 2 and n // 16 < 3:
                    st["prev"] = stage_a16(S - NPRE - 48 + 16 * (n // 16),
                                           _zero_after(v, st["prev"]))
            wo_chunk(i, 0, i, extra)
            wo_chunk(i, 1, jnp.minimum(i + 1, 3), extra)
            return 0
        _loop("wotail", 0, 4, wo_tail)

        def gget(c, row, n):
            return pltpu.bitcast(wqkv[c, pl.ds(row, n), :], f32)

        def gset(c, row, val):
            wqkv[c, pl.ds(row, val.shape[0]), :] = pltpu.bitcast(val, u32)

        def wop(j):
            return lambda k: _unpack(w7[k, j * 32:(j + 1) * 32].reshape(256, 128))

        zpad = jnp.zeros((GPAD, 128), f32)
        for cb in range(8):
            gset(cb, 0, zpad)
            gset(cb, GPAD + S, zpad)

        shifts = (-1, -1, 1, 1, -2, -2, 2, 2)
        HB = MB // 2

        def shift_piece(r, half, k):
            gs = jnp.concatenate([gget(c, r + (k * 16 + GPAD + shifts[c]), 16)
                                  for c in range(8)], axis=1)
            ro = half * (HB // 2) + k * 8
            for t, op in enumerate(row_operands(gs)):
                n7[t, ro:ro + 8, :] = op.astype(bf16)

        def gate(v, i):
            gset(0, GPAD + S + GPAD + 8 * (i // S), v[0:8])

        def b_body(i, _):
            rl = S - NPRE + i * 128
            st = {"n": 0, "prev": [None, None]}

            def hook(v):
                n = st["n"]
                st["n"] += 1
                if n % BG == 0 and n // BG < 8:
                    k = n // BG
                    st["prev"][k % BCH] = stage_a16(rl + 16 * k,
                                                    _zero_after(v, st["prev"][k % BCH]),
                                                    (t7, 8 * k))

            ro = pl.multiple_of(i * 192, 64)
            for lhs, row in ((lambda k: n7[k, pl.ds(ro, 192), :], i * 384), (lambda k: t7[k], rl)):
                rg = pl.multiple_of(GPAD + row, 8)
                for j in range(4):
                    c11, c12, c21, c22 = _strassen(lhs, wop(j), hook)
                    gset(j + 4, rg, _gelu(_merge_rows(c12, c22)))
                    gset(j, rg, _gelu(_merge_rows(c11, c21)))
            return 0
        _loop("b", 0, S // MB, b_body)
        for k in range(HB // 16):
            shift_piece(0, 0, k)

        def n2_norm(r, k, anchor):
            v = _ln(h2buf[pl.ds(pl.multiple_of(r + k * 16, 16), 16), :], anchor)
            nrms[k // 2][(k % 2) * 16:(k % 2) * 16 + 16, :] = v
            return v[0:8] + v[8:16]

        def n2_ops(k, k1, v, i):
            nrm = nrms[k]
            nrm[pl.ds(pl.multiple_of(32 + 8 * (i // S), 8), 8), 0:128] = v[0:8]

            def quad(q):
                r0, c0 = (q // 2) * 16, (q % 2) * 512
                return [nrm[r0 + 8 * a:r0 + 8 * a + 8, c0 + 256 * b:c0 + 256 * b + 256]
                        for a in range(2) for b in range(2)]
            qi, qj, sign = _ATERMS[k1]
            blk = quad(qi)
            if qj is not None:
                blk = [u + w if sign > 0 else u - w for u, w in zip(blk, quad(qj))]
            for k2, op in enumerate(_a_operands(*blk)):
                d49[7 * k1 + k2, k * 8:(k + 1) * 8, :] = op.astype(bf16)

        def n2_hook(r, i, first, gap, lag, st):
            def hook(v):
                n = st["n"] - first
                st["n"] += 1
                if n >= 0 and n % gap == 0 and n // gap < MD // 16:
                    st["prev"] = n2_norm(r, n // gap, _zero_after(v, st["prev"]))
                for _ in range(st["per"]):
                    k, k1 = divmod(st["ops"], 7)
                    if k < MD // 32 and n >= (2 * k + 1) * gap + lag:
                        n2_ops(k, k1, v, i)
                        st["ops"] += 1
            return hook

        def stage_c(i, r, half, rnext, extra):
            rr = pl.multiple_of(r, 8)
            ro = half * (HB // 2)
            cnt = [0]

            def hook(v):
                n = cnt[0]
                cnt[0] += 1
                if n < HB // 16:
                    gate(v, i)
                    shift_piece(rnext, 1 - half, n)
                extra(v)

            for j in range(4):
                c11, c12, c21, c22 = _strassen(lambda k: n7[k, ro:ro + HB // 2, :], wop(4 + j),
                                               hook)
                for c, y in ((j + 4, _merge_rows(c12, c22)), (j, _merge_rows(c11, c21))):
                    cs = slice(c * 128, (c + 1) * 128)
                    h2buf[pl.ds(rr, HB), cs] = h2buf[pl.ds(rr, HB), cs] + y

        def c_body(i, _):
            r = pl.multiple_of(i * MB, MB)
            st = {"n": 0, "prev": None, "ops": 0, "per": 1}
            extra = n2_hook(0, i, 0, 4, 4, st)
            stage_c(i, r, 0, r + HB, extra)
            stage_c(i, r + HB, 1, jnp.minimum(i + 1, S // MB - 1) * MB, extra)
            assert st["ops"] == 28
            return 0
        _loop("c", 0, S // MB, c_body)

        def wop2(lo, n):
            return lambda k1, k: _unpack(w49[7 * k1 + k, lo:lo + n].reshape(8 * n, 128))

        def d_body(i, _):
            r = pl.multiple_of(i * MD, MD)
            rn = jnp.minimum(r + MD, S - MD)
            lhs = [d49[k] for k in range(49)]
            uops = []
            for t in range(7):
                cb = _strassen2(lambda k1, k: lhs[7 * k1 + k], wop2(t * 16, 16))
                uops.append(_a_operands2([[_gelu(c) for c in row] for row in cb]))
            ul = [[jnp.concatenate([u[k1][k] for u in uops], axis=1).astype(bf16)
                   for k in range(7)] for k1 in range(7)]
            st = {"n": 0, "prev": None, "ops": 0, "per": 1}
            hook = n2_hook(rn, i, DF, DG, DL, st)
            for t in range(2):
                cb = _strassen2(lambda k1, k: ul[k1][k], wop2(W4T + t * 56, 56), hook)
                for j in range(4):
                    y = jnp.concatenate([cb[q][j].reshape(MD // 32, 8, 128) for q in range(4)],
                                        axis=1).reshape(MD, 128)
                    c = 2 * j + t
                    cs = slice(c * 128, (c + 1) * 128)
                    gb = modrows(5, MD, c * 128, (c + 1) * 128)
                    o = xbuf[pl.ds(r, MD), cs].astype(f32) + gb * (h2buf[pl.ds(r, MD), cs] + y)
                    xbuf[pl.ds(r, MD), cs] = o.astype(bf16)
            assert st["ops"] == 28
            out_copy(r, MD).start()
            return 0
        _loop("d", 0, S // MD, d_body)

    pl.run_scoped(main,
                  pltpu.VMEM((7, 8 * 32, 8, 128), u32),
                  pltpu.VMEM((49, 2 * W4T, 8, 128), u32))

    out_copy(0, S).wait()


def _run(x, mem0, wq, wk, wv, wo, w1, w2, w3, w4, c, wmod):
    any_spec = pl.BlockSpec(memory_space=pl.ANY)
    return pl.pallas_call(
        _kernel,
        out_shape=jax.ShapeDtypeStruct((S, D), bf16),
        in_specs=[any_spec] * 12,
        out_specs=any_spec,
        scratch_shapes=[
            pltpu.VMEM((S + 2 * RIDE, D), bf16),
            pltpu.VMEM((NGRP + 4, 8 * WP, 128), u32),
            [pltpu.VMEM((NR // 16, 96 // NRING, 8, 128), u32)] * NRING,
            pltpu.VMEM((32, D), bf16),
            pltpu.VMEM((H, 16, 128), u32),
            pltpu.VMEM((2 * H, 8, 128), u32),
            pltpu.VMEM((12, 8, 512), f32),
            pltpu.VMEM((D, 128), f32),
            pltpu.VMEM((S, D), f32),
            pltpu.VMEM((7, (S - NPRE) // 2, 512), bf16),
            pltpu.VMEM((17, 64, 128), bf16),
            pltpu.VMEM((8, 32, D), bf16),
            pltpu.VMEM((7, 64, 512), bf16),
            pltpu.VMEM((2, 7, NPRE // 2, 256), bf16),
            pltpu.VMEM((49, MD // 4, 256), bf16),
            [pltpu.VMEM((40, D), f32)] * (MD // 32),
            pltpu.VMEM((1, D), bf16),
            pltpu.SemaphoreType.DMA((9 + NGRP + 2,)),
        ],
        compiler_params=pltpu.CompilerParams(vmem_limit_bytes=124 * 1024 * 1024,
                                             disable_bounds_checks=True,
                                             disable_semaphore_checks=True),
    )(x, mem0, wq, wk, wv, wo, w1, w2, w3, w4, c, wmod)


def pallas_adaLN_cond__memory_aug_recurrent_mem_tr__mixer_s_mlp__prompt_kernel(
    A_x, A_mem0, A_Wq, A_Wk, A_Wv, A_Wo, A_seg_len, B_x, B_w1, B_w2, B_w3, B_w4, c, w_mod,
):
    del B_x
    assert A_x.shape == (1, S, D) and A_mem0.shape == (1, MEM, D)
    assert not isinstance(A_seg_len, int) or A_seg_len == SEG
    out = _run(A_x.reshape(S, D), A_mem0.reshape(MEM, D), A_Wq, A_Wk, A_Wv,
               A_Wo.reshape(H * DH, D),
               B_w1.reshape(2, D // 2, D), B_w2.reshape(2, D // 2, D),
               B_w3, B_w4.reshape(4, F // 4, D), c, w_mod)
    return out.reshape(1, S, D)
```

```python
import jax
import jax.numpy as jnp
from jax import lax
import jax.experimental.pallas as pl
import jax.experimental.pallas.tpu as pltpu

bf16 = jnp.bfloat16
f32 = jnp.float32
u32 = jnp.uint32

S = 2048
D = 1024
H = 32
DH = 128
F = 3584
MEM = 8
SEG = 32
NSEG = S // SEG
L = MEM + SEG
RIDE = 24
NPRE = S - RIDE * NSEG
NR = NPRE + 2 * SEG
ROFF = (-(S - NPRE)) % NR
WP = 516
NGRP = 12
NSLOT = 6
NMOD = 6
EPS = 1e-5
MD = 128
MB = 512
GPAD = 8
NRING = 8
NWO = 3
X0 = NPRE + 2 * RIDE
W4T = 7 * 16

RLP, WLP, RSK = 27, 22, 2
SAT = {i: max(6 * (i // 2) + 11, 17) for i in range(32)}
PVAT = {i: min(6 * (i // 2) + 23, 107) for i in range(32)}
KSPLIT = 2
PIN = 6
SLOTS = [(0, n // 2, 3 * (n % 2)) for n in range(32)] + [(0, 96 + n, 0) for n in range(32)]
WPP, BG, BCH = 5, 2, 2
DF, DG, DL = 2, 10, 9
_ONLY = None


def _loop(name, lo, hi, body, init=0):
    if _ONLY is not None and name not in _ONLY:
        return init
    with _scope(name):
        return lax.fori_loop(lo, hi, body, init)


class _NoScope:
    def __init__(self, name):
        del name

    def __enter__(self):
        return self

    def __exit__(self, *a):
        return False


_scope = _NoScope


def _zero_after(*vs):
    bits = None
    for v in vs:
        if v is not None:
            b = pltpu.bitcast(v[0:8, 0:128], u32)
            bits = b if bits is None else bits | b
    return pltpu.bitcast((bits >> 31) >> 1, f32)


def _ln(x, anchor=None):
    if anchor is not None:
        z = jnp.concatenate([anchor] * (x.shape[0] // 8), axis=0)
        x = jnp.concatenate([x[:, 0:128] + z, x[:, 128:]], axis=1)
    mu = jnp.mean(x, axis=-1, keepdims=True)
    xc = x - mu
    var = jnp.mean(xc * xc, axis=-1, keepdims=True)
    return xc * lax.rsqrt(var + EPS)


def _gelu(x):
    inner = x * (0.7978845608028654 + (0.7978845608028654 * 0.044715) * (x * x))
    hx = 0.5 * x
    return hx + hx * jnp.tanh(inner)


def _split_rows(x):
    m, n = x.shape
    x3 = x.reshape(m // 16, 16, n)
    return x3[:, 0:8, :].reshape(m // 2, n), x3[:, 8:16, :].reshape(m // 2, n)


def _merge_rows(top, bot):
    m, n = top.shape
    return jnp.concatenate([top.reshape(m // 8, 8, n), bot.reshape(m // 8, 8, n)],
                           axis=1).reshape(2 * m, n)


def _a_operands(a11, a12, a21, a22):
    return [a11 + a22, a21 + a22, a11, a22, a11 + a12, a21 - a11, a12 - a22]


def _b_operands(b11, b12, b21, b22):
    return [b11 + b22, b11, b12 - b22, b21 - b11, b22, b11 + b12, b21 + b22]


_ATERMS = ((0, 3, 1), (2, 3, 1), (0, None, 0), (3, None, 0), (0, 1, 1), (2, 0, -1), (1, 3, -1))
_BTERMS = ((0, 3, 1), (0, None, 0), (1, 3, -1), (2, 0, -1), (3, None, 0), (0, 1, 1), (2, 3, 1))


def _strassen(a_of, b_of, hook=lambda v: None):
    def prod(k):
        return jnp.dot(a_of(k), b_of(k), preferred_element_type=f32)
    p5 = prod(4)
    hook(p5)
    p3 = prod(2)
    hook(p3)
    c12 = p3 + p5
    p4 = prod(3)
    hook(p4)
    c11 = p4 - p5
    p2 = prod(1)
    hook(p2)
    c21 = p2 + p4
    c22 = p3 - p2
    p1 = prod(0)
    hook(p1)
    c11 = prod(6) + (c11 + p1)
    hook(c11)
    c22 = prod(5) + (c22 + p1)
    hook(c22)
    return c11, c12, c21, c22


def _a_operands2(b):
    sub = [_a_operands(b[i][j], b[i][2 + j], b[2 + i][j], b[2 + i][2 + j])
           for i in range(2) for j in range(2)]
    return [_a_operands(*[t[k] for t in sub]) for k in range(7)]


def _strassen2(a_of, b_of, hook=lambda v: None):
    def prod(k1):
        return _strassen(lambda k: a_of(k1, k), lambda k: b_of(k1, k), hook)

    def add(x, y):
        return [p + q for p, q in zip(x, y)]

    def sub(x, y):
        return [p - q for p, q in zip(x, y)]
    p5 = prod(4)
    p3 = prod(2)
    c12 = add(p3, p5)
    p4 = prod(3)
    c11 = sub(p4, p5)
    p2 = prod(1)
    c21 = add(p2, p4)
    c22 = sub(p3, p2)
    p1 = prod(0)
    c11 = add(add(c11, p1), prod(6))
    c22 = add(add(c22, p1), prod(5))
    cq = (c11, c12, c21, c22)
    return [[cq[2 * (i // 2) + j // 2][2 * (i % 2) + j % 2] for j in range(4)] for i in range(4)]


def _pack8(v):
    return pltpu.bitcast(v.astype(bf16), u32)


def _unpack(w):
    return pltpu.bitcast(w, bf16)


def _kernel(x_hbm, mem0_hbm, wq_hbm, wk_hbm, wv_hbm, wo_hbm, w1_hbm, w2_hbm, w3_hbm, w4_hbm,
            c_hbm, wmod_hbm, out_hbm,
            xbuf, wqkv, rings, lhs_h, lhs_o, kvm, modv, scol, h2buf, n7, ws3, wsr, t7, a7, d49,
            nrms, c_ref, sems):
    w_hbms = (wq_hbm, wk_hbm, wv_hbm)
    SMOD, SSTG = 5, 9
    sem_x, sem_out, sem_w, sem_g, sem_r = (sems.at[k] for k in range(5))

    def rget(b, tile, n):
        return jnp.concatenate([rings[b % NRING][tile + e, b // NRING] for e in range(n)], axis=0)

    def rhalf(b, tile, half):
        return rings[b % NRING][tile, b // NRING, 4 * half:4 * half + 4, :]

    def rset(b, tile, half, val):
        rings[b % NRING][tile, b // NRING, 4 * half:4 * half + 4, :] = _pack8(val)

    x_copy = pltpu.make_async_copy(x_hbm.at[pl.ds(0, X0), :], xbuf.at[pl.ds(0, X0), :], sem_x)

    def stream_copies(c):
        al, lo = ((lambda v, m: v), min) if isinstance(c, int) else (pl.multiple_of, jnp.minimum)
        c3 = lo(c, 27)
        cps = [pltpu.make_async_copy(
            w3_hbm.at[pl.ds(al(i * 256 + (c3 % 4) * 64, 64), 64),
                      pl.ds(al(j * (F // 4) + (c3 // 4) * 128, 128), 128)],
            ws3.at[4 * i + j], sem_w) for i in range(4) for j in range(4)]
        dst = X0 + 2 * RIDE * c
        return [
            pltpu.make_async_copy(w4_hbm.at[:, pl.ds(al(c3 * 32, 32), 32), :],
                                  wsr.at[pl.ds(0, 4)], sem_g),
            pltpu.make_async_copy(w1_hbm.at[:, pl.ds(al(c * 16, 16), 16), :],
                                  wsr.at[pl.ds(4, 2), pl.ds(0, 16), :], sem_g),
            pltpu.make_async_copy(w2_hbm.at[:, pl.ds(al(c * 16, 16), 16), :],
                                  wsr.at[pl.ds(4, 2), pl.ds(16, 16), :], sem_g),
            pltpu.make_async_copy(wmod_hbm.at[pl.ds(al(c * 32, 32), 32), pl.ds(5 * D, D)],
                                  wsr.at[6], sem_g),
            pltpu.make_async_copy(x_hbm.at[pl.ds(al(lo(dst, S - 2 * RIDE), 16), 2 * RIDE), :],
                                  xbuf.at[pl.ds(al(dst, 16), 2 * RIDE), :], sem_r)] + cps

    def stream_wait(c):
        for dst, sem in ((ws3.at[pl.ds(0, 16)], sem_w), (wsr.at[pl.ds(0, 7)], sem_g),
                         (xbuf.at[pl.ds(X0 + 2 * RIDE * c, 2 * RIDE), :], sem_r)):
            pltpu.make_async_copy(dst, dst, sem).wait()

    def out_copy(row, n):
        return pltpu.make_async_copy(xbuf.at[pl.ds(row, n), :], out_hbm.at[pl.ds(row, n), :],
                                     sem_out)

    def mod_rows(acc, w, r):
        sc = jnp.concatenate([scol[pl.ds(r, 16), :]] * (w.shape[1] // 128), axis=1)
        p = w.astype(f32) * sc
        return acc + p[0:8] + p[8:16]

    def mod_finish(acc, j):
        is_scale = jnp.logical_or(j // 2 == 1, j // 2 == 4)
        tot = jnp.sum(acc, axis=0, keepdims=True) + jnp.where(is_scale, 1.0, 0.0)
        modv[j] = jnp.broadcast_to(tot, (8, 512))

    def modrows(k, n, lo=0, hi=D):
        m = jnp.concatenate([modv[2 * k], modv[2 * k + 1]], axis=1)[:, lo:hi]
        return jnp.concatenate([m] * (n // 8), axis=0)

    def adaln_a(xv, anchor=None):
        n = xv.shape[0]
        return _ln(xv, anchor) * modrows(1, n) + modrows(0, n)

    def adaln_b(xv, anchor=None):
        n = xv.shape[0]
        return _ln(xv, anchor) * modrows(4, n) + modrows(3, n)

    def row_operands(v):
        top, bot = _split_rows(v)
        k = v.shape[1] // 2
        return _a_operands(top[:, :k], top[:, k:], bot[:, :k], bot[:, k:])

    def stage_a16(r, anchor=None, dst=None):
        rr = pl.multiple_of(r, 16)
        xv = xbuf[pl.ds(rr, 16), :]
        if dst is not None:
            xv = (xv.astype(f32) + modrows(2, 16) * h2buf[pl.ds(rr, 16), :]).astype(bf16)
            xbuf[pl.ds(rr, 16), :] = xv
        h2 = adaln_b(xv.astype(f32), anchor)
        h2buf[pl.ds(rr, 16), :] = h2
        ref, ro = (n7, pl.multiple_of(rr // 2, 8)) if dst is None else dst
        ops = row_operands(_ln(h2))
        for t, op in enumerate(ops):
            ref[t, pl.ds(ro, 8), :] = op.astype(bf16)
        return ops[0]

    def prologue(stg, wos, wmodb, h7):
        def mod_copy(j):
            return pltpu.make_async_copy(wmod_hbm.at[:, pl.ds(j * 512, 512)], wmodb.at[j % NMOD],
                                         sems.at[SSTG + j + 4 if j >= 4 else SMOD + j])

        def piece_copy(g, dh):
            return pltpu.make_async_copy(
                w_hbms[g // 4].at[pl.ds(dh * 512, 512), pl.ds((g % 4) * 8, 8), :],
                stg.at[(2 * g + dh) % NSLOT], sems.at[SSTG + (g + 1 if g else dh)])

        def wo_copy(j):
            return pltpu.make_async_copy(wo_hbm.at[pl.ds(j * 512, 512), :], wos.at[j % NWO],
                                         sems.at[SSTG + j + 6])

        def group_start(g):
            for dh in range(2):
                piece_copy(g, dh).start()

        def stg_wait(slot, n, sem):
            dst = stg.at[pl.ds(slot, n)]
            pltpu.make_async_copy(dst, dst, sems.at[SSTG + sem]).wait()

        def relayout(g, slot, dh, lo_dp, n_dp):
            for u in range(n_dp):
                dp = lo_dp + u
                ev = pltpu.bitcast(stg[slot, 2 * dp].astype(f32), u32)
                od = pltpu.bitcast(stg[slot, 2 * dp + 1].astype(f32), u32)
                wqkv[g, pl.ds(dh * 256 + dp, 8, stride=WP), :] = (ev >> 16) | od

        def b_operand(g, q, k):
            def quad(i):
                r = (q + 4 * (i % 2)) * WP + (i // 2) * 256
                return _unpack(wqkv[g, r:r + 256, :])
            i, j, sign = _BTERMS[k]
            if j is None:
                return quad(i)
            u, v = quad(i).astype(f32), quad(j).astype(f32)
            return (u + v if sign > 0 else u - v).astype(bf16)

        c_copy = pltpu.make_async_copy(c_hbm, c_ref, sem_g)
        m_copy = pltpu.make_async_copy(mem0_hbm, lhs_h.at[pl.ds(0, MEM), :], sem_r)
        c_copy.start()
        m_copy.start()
        x_copy.start()
        for j in range(4):
            mod_copy(j).start()
        for g in range(3):
            group_start(g)
        h2buf[S - NPRE:S, :] = jnp.zeros((NPRE, D), f32)
        wos[2] = jnp.zeros((512, D), bf16)
        c_copy.wait()
        m_copy.wait()
        cv = c_ref[...].astype(f32)
        sv = jnp.broadcast_to(cv * (1.0 / (1.0 + jnp.exp(-cv))), (128, D))
        for k in range(8):
            scol[k * 128:(k + 1) * 128, :] = sv[:, k * 128:(k + 1) * 128].T
        x_copy.wait()

        def ln0_body(i, _):
            r = pl.multiple_of(i * 64, 64)
            h2buf[pl.ds(r, 64), :] = _ln(xbuf[pl.ds(r, 64), :].astype(f32))
            return 0
        lax.fori_loop(0, NPRE // 64, ln0_body, 0)

        def mod0_body(j, _):
            pltpu.make_async_copy(wmodb.at[j], wmodb.at[j], sems.at[SMOD + j]).wait()
            accs = [jnp.zeros((8, 512), f32)] * 2
            for k in range(64):
                accs[k % 2] = mod_rows(accs[k % 2], wmodb[j, k * 16:(k + 1) * 16, :], k * 16)
            mod_finish(accs[0] + accs[1], j)
            return 0
        _loop("mod0", 0, 4, mod0_body)

        def hpre_body(i, _):
            r = pl.multiple_of(i * 32, 32)
            hv = h2buf[pl.ds(r, 32), :] * modrows(1, 32) + modrows(0, 32)
            ro = pl.multiple_of(i * 8, 8)
            for t, op in enumerate(row_operands(hv)):
                h7[t, pl.ds(ro, 8), :] = pltpu.bitcast(op.astype(bf16), u32)
            return 0
        lax.fori_loop(0, NPRE // 32, hpre_body, 0)
        lhs_h[MEM:32, :] = adaln_a(xbuf[NPRE:NPRE + RIDE, :].astype(f32)).astype(bf16)

        def relayout_now(g, dh):
            def rl_body(t, _):
                relayout(g, 2 * g + dh, dh, t * 32, 32)
                return 0
            lax.fori_loop(0, 8, rl_body, 0)

        for dh in range(2):
            stg_wait(dh, 1, dh)
            relayout_now(0, dh)

        grp = lambda g: [piece_copy(g, 0), piece_copy(g, 1)]
        issue = {0: [wo_copy(0)], 1: grp(3) + grp(4), 2: grp(5) + [wo_copy(1), mod_copy(4)],
                 3: grp(6) + [mod_copy(5), mod_copy(6)], 4: grp(7) + [wo_copy(2)],
                 5: grp(8) + [wo_copy(3), mod_copy(7)], 6: grp(9) + [wo_copy(4)],
                 7: grp(10) + [wo_copy(5), mod_copy(8)], 8: grp(11) + [wo_copy(6)],
                 9: [wo_copy(7), mod_copy(9)], 10: stream_copies(0)}

        def pre_iter(g, m3):

            @pl.when(g == 1)
            def _():
                stg_wait(2, 2, 2)
                relayout_now(1, 0)
                relayout_now(1, 1)

            def slots():
                m3n = jnp.where(m3 == 2, 0, m3 + 1)
                cj = jnp.maximum(g - 2, 3)
                return (m3n, 2 * jnp.where(ends, m3, m3n),
                        jnp.where(jnp.logical_or(g < 4, m3 == 0), 2, m3 - 1),
                        cj, jnp.where(cj >= NMOD, cj - NMOD, cj))

            ends = jnp.logical_or(g == 0, g == NGRP - 1)

            @pl.when(jnp.logical_not(ends))
            def _():
                stg_wait(slots()[1], 2, g + 2)

            @pl.when(g >= 4)
            def _():
                buf = wos.at[slots()[2]]
                pltpu.make_async_copy(buf, buf, sems.at[SSTG + g + 2]).wait()

            @pl.when(g >= 6)
            def _():
                buf = wmodb.at[slots()[4]]
                pltpu.make_async_copy(buf, buf, sems.at[SSTG + g + 2]).wait()

            m3n, gslot, wslot, cj, cslot = slots()
            gn = jnp.where(ends, g, g + 1)
            wj = jnp.maximum(g - 4, 0)
            wgrp, wrow = NGRP + wj // 2, (wj % 2) * 256
            for k, cps in issue.items():
                @pl.when(g == k)
                def _():
                    for cp in cps:
                        cp.start()
            wtodo = [(r, c) for r in range(16) for c in range(8)]
            todo = [(dh, dp) for dh in range(2) for dp in range(256)]
            skip = [0] * RSK
            mtodo = list(range(0, D, 16))
            macc = [jnp.zeros((8, 512), f32)]

            def hook(v):
                if mtodo:
                    acc = macc[0] + jnp.concatenate([_zero_after(v)] * 4, axis=1)
                    for r in mtodo[:3]:
                        acc = mod_rows(acc, wmodb[cslot, r:r + 16, :], r)
                    del mtodo[:3]
                    macc[0] = acc

            for q in range(4):
                def b_of(k):
                    w = b_operand(g, q, k)
                    if skip:
                        skip.pop()
                        return w
                    nw = 0 if todo else WLP
                    for dh, dp in todo[:RLP]:
                        relayout(gn, gslot + dh, dh, dp, 1)
                    del todo[:RLP]
                    for r, c in wtodo[:nw]:
                        wqkv[wgrp, pl.ds(wrow + (c * 512 + r * 16), 16), :] = pltpu.bitcast(
                            wos[wslot, r * 32:(r + 1) * 32, c * 128:(c + 1) * 128], u32)
                    del wtodo[:nw]
                    return w
                c11, c12, c21, c22 = _strassen(lambda k: pltpu.bitcast(h7[k], bf16), b_of, hook)
                for blk, y in ((q + 4, _merge_rows(c12, c22)), (q, _merge_rows(c11, c21))):
                    for e in range(NPRE // 8):
                        tile, half = divmod(((8 * e + ROFF) % NR) // 8, 2)
                        rings[blk][tile, g, 4 * half:4 * half + 4, :] = _pack8(y[8 * e:8 * e + 8])
            assert not todo and not wtodo and not mtodo
            mod_finish(macc[0], cj)
            return m3n

        _loop("pre1", 0, NGRP, pre_iter)

    pl.run_scoped(prologue,
                  pltpu.VMEM((NSLOT, 512, 8, 128), bf16),
                  pltpu.VMEM((NWO, 512, D), bf16),
                  pltpu.VMEM((NMOD, D, 512), bf16),
                  pltpu.VMEM((7, NPRE // 4, 512), u32))

    def main(w7, w49):
        scale = DH ** -0.5
        ia = lax.broadcasted_iota(jnp.int32, (32, L), 0)
        ja = lax.broadcasted_iota(jnp.int32, (32, L), 1)
        mask_a = (((ia >= 16) & (ia < 24)) | (ja >= SEG)
                  | (jnp.where(ia < 16, ia + 16, ia - 16) >= ja))
        ib = lax.broadcasted_iota(jnp.int32, (48, 56), 0)
        jb = lax.broadcasted_iota(jnp.int32, (48, 56), 1)
        own = (ib < 40) == (jb < 40)
        mask_b = own & (((jb >= 32) & (jb < 48)) | (jnp.where(jb < 40, jb, jb - 8) <= ib))
        masked = -1e9 / scale
        j8 = lax.broadcasted_iota(jnp.int32, (8, 56), 1)
        fill_b = jnp.concatenate([jnp.where(j8 < 40, masked, -3e38).astype(f32)] * 5
                                 + [jnp.where(j8 < 40, -3e38, masked).astype(f32)], axis=0)

        def softmax(sc, mask, fill):
            sc = jnp.where(mask, sc, fill)
            mx = jnp.max(sc, axis=-1, keepdims=True)
            e = jnp.exp2((sc - mx) * (scale * 1.4426950408889634))
            den = jnp.sum(e, axis=-1, keepdims=True)
            return (e * pl.reciprocal(den, approx=True)).astype(bf16)

        def ride_tiles(it, is_b):
            first = (it == 0).astype(jnp.int32)
            if is_b:
                return 3 * it + 1 - first, 0, 3 * it + 2
            return 3 * it + 1 - first, 1, 3 * it + first

        def step(it, is_b, lhs_lo, lhs_hi, jobs, pins):
            NT, TOFF = NR // 16, ROFF // 16
            sega = (4 * it + TOFF) % NT
            seg = sega + 2 if is_b else sega
            wt = [(3 * it + (NPRE // 16 + TOFF + t + is_b)) % NT for t in range(2)]
            wr = [(wt[(t + is_b) // 2], (t + is_b) % 2) for t in range(3)]
            rt, rh, rf = ride_tiles(it, is_b)
            rt, rf = (rt + TOFF) % NT, (rf + TOFF) % NT
            lhs = jnp.concatenate([lhs_lo, lhs_hi], axis=1)
            QM, P, PART = {}, {}, {}
            mrow = 0 if is_b else 4

            def wblk(b, lo, n):
                r = (b % 8) * WP + lo
                return _unpack(wqkv[b // 8, r:r + n, :])

            def qkv_lo(i):
                for m in range(3):
                    PART[(m, i)] = jnp.dot(lhs_lo, wblk(m * H + i, 0, 256), preferred_element_type=f32)

            def qkv(i):
                for m in range(3):
                    b = m * H + i
                    if (m, i) in PART:
                        y = jnp.dot(lhs_hi, wblk(b, 256, 256),
                                    preferred_element_type=f32) + PART.pop((m, i))
                    else:
                        y = jnp.dot(lhs, wblk(b, 0, 512), preferred_element_type=f32)
                    if m < 2:
                        QM[b] = y[0:MEM] + pins[b] if b in pins else y[0:MEM]
                    if m == 2 or (m == 1 and not is_b):
                        kvm[b - H, mrow:mrow + 4, :] = _pack8(y[0:MEM])
                    for t in range(3):
                        rset(b, *wr[t], y[8 + 8 * t:16 + 8 * t])
                    for job in jobs.get(3 * i + m, []):
                        job(y)
                    side(3 * i + m)

            def keys(b):
                if is_b:
                    if b in QM:
                        mix = jnp.concatenate([_pack8(QM.pop(b)), kvm[b - H, 4:8, :]], axis=0)
                    else:
                        mix = kvm[b - H]
                    return _unpack(jnp.concatenate([rget(b, seg, 2), mix, rhalf(b, sega, 0)], axis=0))
                mk = _pack8(QM.pop(b)) if b in QM else kvm[b - H, 4:8, :]
                return _unpack(jnp.concatenate([rget(b, seg, 2), mk], axis=0))

            def scores(i):
                if is_b:
                    q = [rget(i, seg, 2), _pack8(QM.pop(i)), rhalf(i, sega, 0)]
                else:
                    q = [rget(i, seg + 1, 1), _pack8(QM.pop(i)), rhalf(i, seg, 1)]
                sc = lax.dot_general(_unpack(jnp.concatenate(q, axis=0)), keys(H + i),
                                     (((1,), (1,)), ((), ())), preferred_element_type=f32)
                P[i] = softmax(sc, mask_b, fill_b) if is_b else softmax(sc, mask_a, masked)

            def pv(i):
                o = jnp.dot(P.pop(i), keys(2 * H + i), preferred_element_type=f32)
                if is_b:
                    for e in range(4):
                        rset(i, seg + e // 2, e % 2, o[8 * e:8 * e + 8])
                    rset(i, sega, 0, o[40:48])
                    lhs_o[i, 0:4, :] = _pack8(o[SEG:L])
                else:
                    for e in range(2):
                        rset(i, seg + 1, e, o[8 * e:8 * e + 8])
                    rset(i, seg, 1, o[24:32])
                    lhs_o[i, 0:4, :] = _pack8(o[16:24])
                lhs_o[i, 4:8, :] = rhalf(i, rt, rh)
                lhs_o[i, 8:16, :] = rget(i, rf, 1)

            def wo_lhs(i0, i1):
                return _unpack(jnp.concatenate([lhs_o[i] for i in range(i0, i1)], axis=1))

            def wo_dot(lo, j, k):
                w = _unpack(wqkv[NGRP + k, j * 512:(j + 1) * 512, :])
                return jnp.dot(lo, w, preferred_element_type=f32)

            def side(d):
                for i in range(H):
                    if PVAT[i] == d:
                        pv(i)
                for i in range(H):
                    if SAT[i] == d:
                        scores(i)

            if is_b:
                for h in range(KSPLIT):
                    qkv_lo(h)
            for h in range(H):
                qkv(h)
            lo = [wo_lhs(8 * k, 8 * k + 8) for k in range(3)]
            acc = []
            for j in range(8):
                y = None
                for k in range(3):
                    z = wo_dot(lo[k], j, k)
                    y = z if y is None else z + y
                    for job in jobs.get(96 + 3 * j + k, []):
                        job(y)
                    side(96 + 3 * j + k)
                acc.append(y)
            lo = wo_lhs(24, H)
            for j in range(8):
                acc[j] = wo_dot(lo, j, 3) + acc[j]
                for job in jobs.get(120 + j, []):
                    job(acc[j])
            assert not (QM or P or PART)
            return jnp.concatenate(acc[0:4], axis=1), jnp.concatenate(acc[4:8], axis=1)

        def combine(c, n, y):
            mp, k1 = divmod(n, 8)
            m, p = divmod(mp, 4)
            c3 = jnp.minimum(c, 27)
            spare = pl.ds(pl.multiple_of(8 * (c // 64), 8), 8)
            if m == 0 and k1 < 7:
                ws3[16, spare, :] = y.astype(bf16)
            else:
                wsr[7, spare, 0:128] = y.astype(bf16)
            if k1 == 7:
                dst, base, r = w7, 0, (4 * m + p) * 32 + c
                blk = [wsr[4 + i, m * 16:(m + 1) * 16, j * 512 + p * 128:j * 512 + (p + 1) * 128]
                       .astype(f32) for i in range(2) for j in range(2)]
            else:
                dst, base = w49, 7 * k1
                if m == 0:
                    r = c3 * 4 + p
                    get = lambda i, j: ws3[4 * i + j, p * 16:(p + 1) * 16, :]
                else:
                    r = W4T + (p // 2) * 56 + c3 * 2 + p % 2
                    r0, c0 = (p % 2) * 16, (p // 2) * 128
                    get = lambda i, j: wsr[i, r0:r0 + 16, j * 256 + c0:j * 256 + c0 + 128]

                def quad(q):
                    return [get(2 * (q // 2) + i, 2 * (q % 2) + j).astype(f32)
                            for i in range(2) for j in range(2)]
                qi, qj, sign = _BTERMS[k1]
                blk = quad(qi)
                if qj is not None:
                    blk = [u + v if sign > 0 else u - v for u, v in zip(blk, quad(qj))]
            for k, op in enumerate(_b_operands(*blk)):
                for e in range(2):
                    dst[base + k, r, 4 * e:4 * e + 4, :] = _pack8(op[8 * e:8 * e + 8])

        def rec_body(it, gacc):
            stream_wait(it)
            lhs_lo = lhs_h[:, 0:512]
            lhs_hi = lhs_h[:, 512:1024]
            ra = jnp.maximum(it - 1, 0) * (2 * RIDE)
            for u in range(2):
                s = 2 * it + u
                jobs, pins = {}, {}
                for n, (su, d, g) in enumerate(SLOTS):
                    if su == u:
                        jobs.setdefault(d, []).append(
                            lambda y, n=n, g=g: combine(it, n, y[8 * g:8 * g + 8]))
                r1 = pl.multiple_of(jnp.minimum(NPRE + RIDE * (s + 1), S - RIDE), 8)
                xn = xbuf[pl.ds(r1, RIDE), :].astype(f32)
                if u == 0:
                    for k in range(2):
                        rm = pl.multiple_of(it * 32 + k * 16, 16)
                        gacc = mod_rows(gacc, wsr[6, k * 16:(k + 1) * 16, :], rm)
                    hn = adaln_a(xn, _zero_after(stage_a16(ra)))
                else:
                    def refill(y):
                        for cp in stream_copies(jnp.minimum(it + 1, NSEG // 2 - 1)):
                            cp.start()
                        spare = pl.ds(pl.multiple_of(8 * (it // 64), 8), 8)
                        pins[PIN] = _zero_after(ws3[16, spare, :].astype(f32))
                    jobs.setdefault(3 * (PIN - 4) + 2, []).append(refill)
                    hn = adaln_a(xn)
                    z = _zero_after(hn[0:8], hn[8:16], hn[16:24])
                    stage_a16(ra + 32, _zero_after(stage_a16(ra + 16, z)))
                a_lo, a_hi = step(it, u, lhs_lo, lhs_hi, jobs, pins)
                lhs_lo = jnp.concatenate([a_lo[0:MEM], hn[:, 0:512]], axis=0).astype(bf16)
                lhs_hi = jnp.concatenate([a_hi[0:MEM], hn[:, 512:1024]], axis=0).astype(bf16)
                a = jnp.concatenate([a_lo, a_hi], axis=1)
                rt, rh, rf = ride_tiles(it, u)
                rows = [pl.ds(pl.multiple_of(16 * rt + 8 * rh, 8), 8),
                        pl.ds(pl.multiple_of(16 * rf, 16), 16)]
                xs = [xbuf[r, :].astype(f32) for r in rows]
                xbuf[rows[0], :] = (xs[0] + modrows(2, 8) * a[8:16]).astype(bf16)
                xbuf[rows[1], :] = (xs[1] + modrows(2, 16) * a[16:32]).astype(bf16)
            lhs_h[:, 0:512] = lhs_lo
            lhs_h[:, 512:1024] = lhs_hi
            return gacc

        gacc = _loop("rec", 0, NSEG // 2, rec_body, jnp.zeros((8, D), f32))
        for c in range(2):
            mod_finish(gacc[:, c * 512:(c + 1) * 512], 10 + c)
        stream_wait(NSEG // 2 - 1)

        def wo_prep(i, half, k):
            o = jnp.concatenate([_unpack(rings[4 * half + h][k, i]).astype(f32)
                                 for h in range(4)], axis=1)
            for t, op in enumerate(row_operands(o)):
                a7[half, t, k * 8:(k + 1) * 8, :] = op.astype(bf16)

        def wo_chunk(i, half, inext, extra):
            todo = list(range(NPRE // 16))

            def hook(v):
                if todo:
                    for h in range(4):
                        rings[4 * (1 - half) + h][i // 64, 4] = pltpu.bitcast(v[0:8], u32)
                    n = 2 if len(todo) % WPP == 0 else 1
                    for k in todo[:n]:
                        wo_prep(inext, 1 - half, k)
                    del todo[:n]
                extra(v)

            for j in range(4):
                def b_of(k):
                    def quad(q):
                        r = (j + 4 * (q % 2)) * 512 + half * 256 + (q // 2) * 128
                        return _unpack(wqkv[NGRP + i, r:r + 128, :])
                    qi, qj, sign = _BTERMS[k]
                    if qj is None:
                        return quad(qi)
                    u, v = quad(qi).astype(f32), quad(qj).astype(f32)
                    return (u + v if sign > 0 else u - v).astype(bf16)
                c11, c12, c21, c22 = _strassen(lambda k: a7[half, k], b_of, hook)
                for c, y in ((j + 4, _merge_rows(c12, c22)), (j, _merge_rows(c11, c21))):
                    cs = slice(c * 128, (c + 1) * 128)
                    h2buf[S - NPRE:S, cs] = h2buf[S - NPRE:S, cs] + y

        for k in range(NPRE // 16):
            wo_prep(0, 0, k)

        def wo_tail(i, _):
            st = {"n": 0, "prev": None}

            def extra(v):
                n = st["n"]
                st["n"] += 1
                if n % 16 == 2 and n // 16 < 3:
                    st["prev"] = stage_a16(S - NPRE - 48 + 16 * (n // 16),
                                           _zero_after(v, st["prev"]))
            wo_chunk(i, 0, i, extra)
            wo_chunk(i, 1, jnp.minimum(i + 1, 3), extra)
            return 0
        _loop("wotail", 0, 4, wo_tail)

        def gget(c, row, n):
            return pltpu.bitcast(wqkv[c, pl.ds(row, n), :], f32)

        def gset(c, row, val):
            wqkv[c, pl.ds(row, val.shape[0]), :] = pltpu.bitcast(val, u32)

        def wop(j):
            return lambda k: _unpack(w7[k, j * 32:(j + 1) * 32].reshape(256, 128))

        zpad = jnp.zeros((GPAD, 128), f32)
        for cb in range(8):
            gset(cb, 0, zpad)
            gset(cb, GPAD + S, zpad)

        shifts = (-1, -1, 1, 1, -2, -2, 2, 2)
        HB = MB // 2

        def shift_piece(r, half, k):
            gs = jnp.concatenate([gget(c, r + (k * 16 + GPAD + shifts[c]), 16)
                                  for c in range(8)], axis=1)
            ro = half * (HB // 2) + k * 8
            for t, op in enumerate(row_operands(gs)):
                n7[t, ro:ro + 8, :] = op.astype(bf16)

        def gate(v, i):
            gset(0, GPAD + S + GPAD + 8 * (i // S), v[0:8])

        def b_body(i, _):
            rl = S - NPRE + i * 128
            st = {"n": 0, "prev": [None, None]}

            def hook(v):
                n = st["n"]
                st["n"] += 1
                if n % BG == 0 and n // BG < 8:
                    k = n // BG
                    st["prev"][k % BCH] = stage_a16(rl + 16 * k,
                                                    _zero_after(v, st["prev"][k % BCH]),
                                                    (t7, 8 * k))

            ro = pl.multiple_of(i * 192, 64)
            for lhs, row in ((lambda k: n7[k, pl.ds(ro, 192), :], i * 384), (lambda k: t7[k], rl)):
                rg = pl.multiple_of(GPAD + row, 8)
                for j in range(4):
                    c11, c12, c21, c22 = _strassen(lhs, wop(j), hook)
                    gset(j + 4, rg, _gelu(_merge_rows(c12, c22)))
                    gset(j, rg, _gelu(_merge_rows(c11, c21)))
            return 0
        _loop("b", 0, S // MB, b_body)
        for k in range(HB // 16):
            shift_piece(0, 0, k)

        def n2_norm(r, k, anchor):
            v = _ln(h2buf[pl.ds(pl.multiple_of(r + k * 16, 16), 16), :], anchor)
            nrms[k // 2][(k % 2) * 16:(k % 2) * 16 + 16, :] = v
            return v[0:8] + v[8:16]

        def n2_ops(k, k1, v, i):
            nrm = nrms[k]
            nrm[pl.ds(pl.multiple_of(32 + 8 * (i // S), 8), 8), 0:128] = v[0:8]

            def quad(q):
                r0, c0 = (q // 2) * 16, (q % 2) * 512
                return [nrm[r0 + 8 * a:r0 + 8 * a + 8, c0 + 256 * b:c0 + 256 * b + 256]
                        for a in range(2) for b in range(2)]
            qi, qj, sign = _ATERMS[k1]
            blk = quad(qi)
            if qj is not None:
                blk = [u + w if sign > 0 else u - w for u, w in zip(blk, quad(qj))]
            for k2, op in enumerate(_a_operands(*blk)):
                d49[7 * k1 + k2, k * 8:(k + 1) * 8, :] = op.astype(bf16)

        def n2_hook(r, i, first, gap, lag, st):
            def hook(v):
                n = st["n"] - first
                st["n"] += 1
                if n >= 0 and n % gap == 0 and n // gap < MD // 16:
                    st["prev"] = n2_norm(r, n // gap, _zero_after(v, st["prev"]))
                for _ in range(st["per"]):
                    k, k1 = divmod(st["ops"], 7)
                    if k < MD // 32 and n >= (2 * k + 1) * gap + lag:
                        n2_ops(k, k1, v, i)
                        st["ops"] += 1
            return hook

        def stage_c(i, r, half, rnext, extra):
            rr = pl.multiple_of(r, 8)
            ro = half * (HB // 2)
            cnt = [0]

            def hook(v):
                n = cnt[0]
                cnt[0] += 1
                if n < HB // 16:
                    gate(v, i)
                    shift_piece(rnext, 1 - half, n)
                extra(v)

            for j in range(4):
                c11, c12, c21, c22 = _strassen(lambda k: n7[k, ro:ro + HB // 2, :], wop(4 + j),
                                               hook)
                for c, y in ((j + 4, _merge_rows(c12, c22)), (j, _merge_rows(c11, c21))):
                    cs = slice(c * 128, (c + 1) * 128)
                    h2buf[pl.ds(rr, HB), cs] = h2buf[pl.ds(rr, HB), cs] + y

        def c_body(i, _):
            r = pl.multiple_of(i * MB, MB)
            st = {"n": 0, "prev": None, "ops": 0, "per": 1}
            extra = n2_hook(0, i, 0, 4, 4, st)
            stage_c(i, r, 0, r + HB, extra)
            stage_c(i, r + HB, 1, jnp.minimum(i + 1, S // MB - 1) * MB, extra)
            assert st["ops"] == 28
            return 0
        _loop("c", 0, S // MB, c_body)

        def wop2(lo, n):
            return lambda k1, k: _unpack(w49[7 * k1 + k, lo:lo + n].reshape(8 * n, 128))

        def d_body(i, _):
            r = pl.multiple_of(i * MD, MD)
            rn = jnp.minimum(r + MD, S - MD)
            lhs = [d49[k] for k in range(49)]
            uops = []
            for t in range(7):
                cb = _strassen2(lambda k1, k: lhs[7 * k1 + k], wop2(t * 16, 16))
                uops.append(_a_operands2([[_gelu(c) for c in row] for row in cb]))
            ul = [[jnp.concatenate([u[k1][k] for u in uops], axis=1).astype(bf16)
                   for k in range(7)] for k1 in range(7)]
            st = {"n": 0, "prev": None, "ops": 0, "per": 1}
            hook = n2_hook(rn, i, DF, DG, DL, st)
            for t in range(2):
                cb = _strassen2(lambda k1, k: ul[k1][k], wop2(W4T + t * 56, 56), hook)
                for j in range(4):
                    y = jnp.concatenate([cb[q][j].reshape(MD // 32, 8, 128) for q in range(4)],
                                        axis=1).reshape(MD, 128)
                    c = 2 * j + t
                    cs = slice(c * 128, (c + 1) * 128)
                    gb = modrows(5, MD, c * 128, (c + 1) * 128)
                    o = xbuf[pl.ds(r, MD), cs].astype(f32) + gb * (h2buf[pl.ds(r, MD), cs] + y)
                    xbuf[pl.ds(r, MD), cs] = o.astype(bf16)
            assert st["ops"] == 28
            out_copy(r, MD).start()
            return 0
        _loop("d", 0, S // MD, d_body)

    pl.run_scoped(main,
                  pltpu.VMEM((7, 8 * 32, 8, 128), u32),
                  pltpu.VMEM((49, 2 * W4T, 8, 128), u32))

    out_copy(0, S).wait()


def _run(x, mem0, wq, wk, wv, wo, w1, w2, w3, w4, c, wmod):
    any_spec = pl.BlockSpec(memory_space=pl.ANY)
    return pl.pallas_call(
        _kernel,
        out_shape=jax.ShapeDtypeStruct((S, D), bf16),
        in_specs=[any_spec] * 12,
        out_specs=any_spec,
        scratch_shapes=[
            pltpu.VMEM((S + 2 * RIDE, D), bf16),
            pltpu.VMEM((NGRP + 4, 8 * WP, 128), u32),
            [pltpu.VMEM((NR // 16, 96 // NRING, 8, 128), u32)] * NRING,
            pltpu.VMEM((32, D), bf16),
            pltpu.VMEM((H, 16, 128), u32),
            pltpu.VMEM((2 * H, 8, 128), u32),
            pltpu.VMEM((12, 8, 512), f32),
            pltpu.VMEM((D, 128), f32),
            pltpu.VMEM((S, D), f32),
            pltpu.VMEM((7, (S - NPRE) // 2, 512), bf16),
            pltpu.VMEM((17, 64, 128), bf16),
            pltpu.VMEM((8, 32, D), bf16),
            pltpu.VMEM((7, 64, 512), bf16),
            pltpu.VMEM((2, 7, NPRE // 2, 256), bf16),
            pltpu.VMEM((49, MD // 4, 256), bf16),
            [pltpu.VMEM((40, D), f32)] * (MD // 32),
            pltpu.VMEM((1, D), bf16),
            pltpu.SemaphoreType.DMA((9 + NGRP + 2,)),
        ],
        compiler_params=pltpu.CompilerParams(vmem_limit_bytes=124 * 1024 * 1024,
                                             disable_bounds_checks=True,
                                             disable_semaphore_checks=True),
    )(x, mem0, wq, wk, wv, wo, w1, w2, w3, w4, c, wmod)


def pallas_adaLN_cond__memory_aug_recurrent_mem_tr__mixer_s_mlp__prompt_kernel(
    A_x, A_mem0, A_Wq, A_Wk, A_Wv, A_Wo, A_seg_len, B_x, B_w1, B_w2, B_w3, B_w4, c, w_mod,
):
    del B_x
    assert A_x.shape == (1, S, D) and A_mem0.shape == (1, MEM, D)
    assert not isinstance(A_seg_len, int) or A_seg_len == SEG
    out = _run(A_x.reshape(S, D), A_mem0.reshape(MEM, D), A_Wq, A_Wk, A_Wv,
               A_Wo.reshape(H * DH, D),
               B_w1.reshape(2, D // 2, D), B_w2.reshape(2, D // 2, D),
               B_w3, B_w4.reshape(4, F // 4, D), c, w_mod)
    return out.reshape(1, S, D)
```

```python
import jax
import jax.numpy as jnp
from jax import lax
import jax.experimental.pallas as pl
import jax.experimental.pallas.tpu as pltpu

bf16 = jnp.bfloat16
f32 = jnp.float32
u32 = jnp.uint32

S = 2048
D = 1024
H = 32
DH = 128
F = 3584
MEM = 8
SEG = 32
NSEG = S // SEG
L = MEM + SEG
RIDE = 24
NPRE = S - RIDE * NSEG
NR = NPRE + 2 * SEG
ROFF = (-(S - NPRE)) % NR
WP = 516
NGRP = 12
NSLOT = 6
NMOD = 6
EPS = 1e-5
MD = 128
MB = 512
GPAD = 8
NRING = 8
NWO = 3
X0 = NPRE + 2 * RIDE
W4T = 7 * 16

RLP, WLP, RSK = 27, 22, 2
SAT = {i: max(6 * (i // 2) + 11, 17) for i in range(32)}
PVAT = {i: min(6 * (i // 2) + 23, 107) for i in range(32)}
KSPLIT = 2
PIN = 6
SLOTS = ([(0, -1, 0)] * 8 + [(0, n // 2, 3 * (n % 2)) for n in range(24)]
         + [(0, 96 + n, 0) for n in range(32)])
WPP, BG, BCH = 5, 2, 2
DF, DG, DL = 2, 10, 9
_ONLY = None


def _loop(name, lo, hi, body, init=0):
    if _ONLY is not None and name not in _ONLY:
        return init
    with _scope(name):
        return lax.fori_loop(lo, hi, body, init)


class _NoScope:
    def __init__(self, name):
        del name

    def __enter__(self):
        return self

    def __exit__(self, *a):
        return False


_scope = _NoScope


def _zero_after(*vs):
    bits = None
    for v in vs:
        if v is not None:
            b = pltpu.bitcast(v[0:8, 0:128], u32)
            bits = b if bits is None else bits | b
    return pltpu.bitcast((bits >> 31) >> 1, f32)


def _ln(x, anchor=None):
    if anchor is not None:
        z = jnp.concatenate([anchor] * (x.shape[0] // 8), axis=0)
        x = jnp.concatenate([x[:, 0:128] + z, x[:, 128:]], axis=1)
    mu = jnp.mean(x, axis=-1, keepdims=True)
    xc = x - mu
    var = jnp.mean(xc * xc, axis=-1, keepdims=True)
    return xc * lax.rsqrt(var + EPS)


def _gelu(x):
    inner = x * (0.7978845608028654 + (0.7978845608028654 * 0.044715) * (x * x))
    hx = 0.5 * x
    return hx + hx * jnp.tanh(inner)


def _split_rows(x):
    m, n = x.shape
    x3 = x.reshape(m // 16, 16, n)
    return x3[:, 0:8, :].reshape(m // 2, n), x3[:, 8:16, :].reshape(m // 2, n)


def _merge_rows(top, bot):
    m, n = top.shape
    return jnp.concatenate([top.reshape(m // 8, 8, n), bot.reshape(m // 8, 8, n)],
                           axis=1).reshape(2 * m, n)


def _a_operands(a11, a12, a21, a22):
    return [a11 + a22, a21 + a22, a11, a22, a11 + a12, a21 - a11, a12 - a22]


def _b_operands(b11, b12, b21, b22):
    return [b11 + b22, b11, b12 - b22, b21 - b11, b22, b11 + b12, b21 + b22]


_ATERMS = ((0, 3, 1), (2, 3, 1), (0, None, 0), (3, None, 0), (0, 1, 1), (2, 0, -1), (1, 3, -1))
_BTERMS = ((0, 3, 1), (0, None, 0), (1, 3, -1), (2, 0, -1), (3, None, 0), (0, 1, 1), (2, 3, 1))


def _strassen(a_of, b_of, hook=lambda v: None):
    def prod(k):
        return jnp.dot(a_of(k), b_of(k), preferred_element_type=f32)
    p5 = prod(4)
    hook(p5)
    p3 = prod(2)
    hook(p3)
    c12 = p3 + p5
    p4 = prod(3)
    hook(p4)
    c11 = p4 - p5
    p2 = prod(1)
    hook(p2)
    c21 = p2 + p4
    c22 = p3 - p2
    p1 = prod(0)
    hook(p1)
    c11 = prod(6) + (c11 + p1)
    hook(c11)
    c22 = prod(5) + (c22 + p1)
    hook(c22)
    return c11, c12, c21, c22


def _a_operands2(b):
    sub = [_a_operands(b[i][j], b[i][2 + j], b[2 + i][j], b[2 + i][2 + j])
           for i in range(2) for j in range(2)]
    return [_a_operands(*[t[k] for t in sub]) for k in range(7)]


def _strassen2(a_of, b_of, hook=lambda v: None):
    def prod(k1):
        return _strassen(lambda k: a_of(k1, k), lambda k: b_of(k1, k), hook)

    def add(x, y):
        return [p + q for p, q in zip(x, y)]

    def sub(x, y):
        return [p - q for p, q in zip(x, y)]
    p5 = prod(4)
    p3 = prod(2)
    c12 = add(p3, p5)
    p4 = prod(3)
    c11 = sub(p4, p5)
    p2 = prod(1)
    c21 = add(p2, p4)
    c22 = sub(p3, p2)
    p1 = prod(0)
    c11 = add(add(c11, p1), prod(6))
    c22 = add(add(c22, p1), prod(5))
    cq = (c11, c12, c21, c22)
    return [[cq[2 * (i // 2) + j // 2][2 * (i % 2) + j % 2] for j in range(4)] for i in range(4)]


def _pack8(v):
    return pltpu.bitcast(v.astype(bf16), u32)


def _unpack(w):
    return pltpu.bitcast(w, bf16)


def _kernel(x_hbm, mem0_hbm, wq_hbm, wk_hbm, wv_hbm, wo_hbm, w1_hbm, w2_hbm, w3_hbm, w4_hbm,
            c_hbm, wmod_hbm, out_hbm,
            xbuf, wqkv, rings, lhs_h, lhs_o, kvm, modv, scol, h2buf, n7, ws3, wsr, t7, a7, d49,
            nrms, c_ref, sems):
    w_hbms = (wq_hbm, wk_hbm, wv_hbm)
    SMOD, SSTG = 5, 9
    sem_x, sem_out, sem_w, sem_g, sem_r = (sems.at[k] for k in range(5))

    def rget(b, tile, n):
        return jnp.concatenate([rings[b % NRING][tile + e, b // NRING] for e in range(n)], axis=0)

    def rhalf(b, tile, half):
        return rings[b % NRING][tile, b // NRING, 4 * half:4 * half + 4, :]

    def rset(b, tile, half, val):
        rings[b % NRING][tile, b // NRING, 4 * half:4 * half + 4, :] = _pack8(val)

    x_copy = pltpu.make_async_copy(x_hbm.at[pl.ds(0, X0), :], xbuf.at[pl.ds(0, X0), :], sem_x)

    def stream_copies(c):
        al, lo = ((lambda v, m: v), min) if isinstance(c, int) else (pl.multiple_of, jnp.minimum)
        c3 = lo(c, 27)
        cps = [pltpu.make_async_copy(
            w3_hbm.at[pl.ds(al(i * 256 + (c3 % 4) * 64, 64), 64),
                      pl.ds(al(j * (F // 4) + (c3 // 4) * 128, 128), 128)],
            ws3.at[4 * i + j], sem_w) for i in range(4) for j in range(4)]
        dst = X0 + 2 * RIDE * c
        return [
            pltpu.make_async_copy(w4_hbm.at[:, pl.ds(al(c3 * 32, 32), 32), :],
                                  wsr.at[pl.ds(0, 4)], sem_g),
            pltpu.make_async_copy(w1_hbm.at[:, pl.ds(al(c * 16, 16), 16), :],
                                  wsr.at[pl.ds(4, 2), pl.ds(0, 16), :], sem_g),
            pltpu.make_async_copy(w2_hbm.at[:, pl.ds(al(c * 16, 16), 16), :],
                                  wsr.at[pl.ds(4, 2), pl.ds(16, 16), :], sem_g),
            pltpu.make_async_copy(wmod_hbm.at[pl.ds(al(c * 32, 32), 32), pl.ds(5 * D, D)],
                                  wsr.at[6], sem_g),
            pltpu.make_async_copy(x_hbm.at[pl.ds(al(lo(dst, S - 2 * RIDE), 16), 2 * RIDE), :],
                                  xbuf.at[pl.ds(al(dst, 16), 2 * RIDE), :], sem_r)] + cps

    def stream_wait(c):
        for dst, sem in ((ws3.at[pl.ds(0, 16)], sem_w), (wsr.at[pl.ds(0, 7)], sem_g),
                         (xbuf.at[pl.ds(X0 + 2 * RIDE * c, 2 * RIDE), :], sem_r)):
            pltpu.make_async_copy(dst, dst, sem).wait()

    def out_copy(row, n):
        return pltpu.make_async_copy(xbuf.at[pl.ds(row, n), :], out_hbm.at[pl.ds(row, n), :],
                                     sem_out)

    def mod_rows(acc, w, r):
        sc = jnp.concatenate([scol[pl.ds(r, 16), :]] * (w.shape[1] // 128), axis=1)
        p = w.astype(f32) * sc
        return acc + p[0:8] + p[8:16]

    def mod_finish(acc, j):
        is_scale = jnp.logical_or(j // 2 == 1, j // 2 == 4)
        tot = jnp.sum(acc, axis=0, keepdims=True) + jnp.where(is_scale, 1.0, 0.0)
        modv[j] = jnp.broadcast_to(tot, (8, 512))

    def modrows(k, n, lo=0, hi=D):
        m = jnp.concatenate([modv[2 * k], modv[2 * k + 1]], axis=1)[:, lo:hi]
        return jnp.concatenate([m] * (n // 8), axis=0)

    def adaln_a(xv, anchor=None):
        n = xv.shape[0]
        return _ln(xv, anchor) * modrows(1, n) + modrows(0, n)

    def adaln_b(xv, anchor=None):
        n = xv.shape[0]
        return _ln(xv, anchor) * modrows(4, n) + modrows(3, n)

    def set_lhs(mem, hn):
        v = jnp.concatenate([mem, hn], axis=0)
        for c in range(8):
            for e in range(4):
                lhs_h[c, 4 * e:4 * e + 4, :] = _pack8(v[8 * e:8 * e + 8, c * 128:(c + 1) * 128])

    def row_operands(v):
        top, bot = _split_rows(v)
        k = v.shape[1] // 2
        return _a_operands(top[:, :k], top[:, k:], bot[:, :k], bot[:, k:])

    def stage_a16(r, anchor=None, dst=None):
        rr = pl.multiple_of(r, 16)
        xv = xbuf[pl.ds(rr, 16), :]
        if dst is not None:
            xv = (xv.astype(f32) + modrows(2, 16) * h2buf[pl.ds(rr, 16), :]).astype(bf16)
            xbuf[pl.ds(rr, 16), :] = xv
        h2 = adaln_b(xv.astype(f32), anchor)
        h2buf[pl.ds(rr, 16), :] = h2
        ref, ro = (n7, pl.multiple_of(rr // 2, 8)) if dst is None else dst
        ops = row_operands(_ln(h2))
        for t, op in enumerate(ops):
            ref[t, pl.ds(ro, 8), :] = op.astype(bf16)
        return ops[0]

    def prologue(stg, wos, wmodb, h7):
        def mod_copy(j):
            return pltpu.make_async_copy(wmod_hbm.at[:, pl.ds(j * 512, 512)], wmodb.at[j % NMOD],
                                         sems.at[SSTG + j + 4 if j >= 4 else SMOD + j])

        def piece_copy(g, dh):
            return pltpu.make_async_copy(
                w_hbms[g // 4].at[pl.ds(dh * 512, 512), pl.ds((g % 4) * 8, 8), :],
                stg.at[(2 * g + dh) % NSLOT], sems.at[SSTG + (g + 1 if g else dh)])

        def wo_copy(j):
            return pltpu.make_async_copy(wo_hbm.at[pl.ds(j * 512, 512), :], wos.at[j % NWO],
                                         sems.at[SSTG + j + 6])

        def group_start(g):
            for dh in range(2):
                piece_copy(g, dh).start()

        def stg_wait(slot, n, sem):
            dst = stg.at[pl.ds(slot, n)]
            pltpu.make_async_copy(dst, dst, sems.at[SSTG + sem]).wait()

        def relayout(g, slot, dh, lo_dp, n_dp):
            for u in range(n_dp):
                dp = lo_dp + u
                ev = pltpu.bitcast(stg[slot, 2 * dp].astype(f32), u32)
                od = pltpu.bitcast(stg[slot, 2 * dp + 1].astype(f32), u32)
                wqkv[g, pl.ds(dh * 256 + dp, 8, stride=WP), :] = (ev >> 16) | od

        def b_operand(g, q, k):
            def quad(i):
                r = (q + 4 * (i % 2)) * WP + (i // 2) * 256
                return _unpack(wqkv[g, r:r + 256, :])
            i, j, sign = _BTERMS[k]
            if j is None:
                return quad(i)
            u, v = quad(i).astype(f32), quad(j).astype(f32)
            return (u + v if sign > 0 else u - v).astype(bf16)

        c_copy = pltpu.make_async_copy(c_hbm, c_ref, sem_g)
        m_copy = pltpu.make_async_copy(mem0_hbm, wsr.at[7, pl.ds(0, MEM), :], sem_r)
        c_copy.start()
        m_copy.start()
        x_copy.start()
        for j in range(4):
            mod_copy(j).start()
        for g in range(3):
            group_start(g)
        h2buf[S - NPRE:S, :] = jnp.zeros((NPRE, D), f32)
        wos[2] = jnp.zeros((512, D), bf16)
        c_copy.wait()
        m_copy.wait()
        cv = c_ref[...].astype(f32)
        sv = jnp.broadcast_to(cv * (1.0 / (1.0 + jnp.exp(-cv))), (128, D))
        for k in range(8):
            scol[k * 128:(k + 1) * 128, :] = sv[:, k * 128:(k + 1) * 128].T
        x_copy.wait()

        def ln0_body(i, _):
            r = pl.multiple_of(i * 64, 64)
            h2buf[pl.ds(r, 64), :] = _ln(xbuf[pl.ds(r, 64), :].astype(f32))
            return 0
        lax.fori_loop(0, NPRE // 64, ln0_body, 0)

        def mod0_body(j, _):
            pltpu.make_async_copy(wmodb.at[j], wmodb.at[j], sems.at[SMOD + j]).wait()
            accs = [jnp.zeros((8, 512), f32)] * 2
            for k in range(64):
                accs[k % 2] = mod_rows(accs[k % 2], wmodb[j, k * 16:(k + 1) * 16, :], k * 16)
            mod_finish(accs[0] + accs[1], j)
            return 0
        _loop("mod0", 0, 4, mod0_body)

        def hpre_body(i, _):
            r = pl.multiple_of(i * 32, 32)
            hv = h2buf[pl.ds(r, 32), :] * modrows(1, 32) + modrows(0, 32)
            ro = pl.multiple_of(i * 8, 8)
            for t, op in enumerate(row_operands(hv)):
                h7[t, pl.ds(ro, 8), :] = pltpu.bitcast(op.astype(bf16), u32)
            return 0
        lax.fori_loop(0, NPRE // 32, hpre_body, 0)
        set_lhs(wsr[7, 0:MEM, :].astype(f32), adaln_a(xbuf[NPRE:NPRE + RIDE, :].astype(f32)))

        def relayout_now(g, dh):
            def rl_body(t, _):
                relayout(g, 2 * g + dh, dh, t * 32, 32)
                return 0
            lax.fori_loop(0, 8, rl_body, 0)

        for dh in range(2):
            stg_wait(dh, 1, dh)
            relayout_now(0, dh)

        grp = lambda g: [piece_copy(g, 0), piece_copy(g, 1)]
        issue = {0: [wo_copy(0)], 1: grp(3) + grp(4), 2: grp(5) + [wo_copy(1), mod_copy(4)],
                 3: grp(6) + [mod_copy(5), mod_copy(6)], 4: grp(7) + [wo_copy(2)],
                 5: grp(8) + [wo_copy(3), mod_copy(7)], 6: grp(9) + [wo_copy(4)],
                 7: grp(10) + [wo_copy(5), mod_copy(8)], 8: grp(11) + [wo_copy(6)],
                 9: [wo_copy(7), mod_copy(9)], 10: stream_copies(0)}

        def pre_iter(g, m3):

            @pl.when(g == 1)
            def _():
                stg_wait(2, 2, 2)
                relayout_now(1, 0)
                relayout_now(1, 1)

            def slots():
                m3n = jnp.where(m3 == 2, 0, m3 + 1)
                cj = jnp.maximum(g - 2, 3)
                return (m3n, 2 * jnp.where(ends, m3, m3n),
                        jnp.where(jnp.logical_or(g < 4, m3 == 0), 2, m3 - 1),
                        cj, jnp.where(cj >= NMOD, cj - NMOD, cj))

            ends = jnp.logical_or(g == 0, g == NGRP - 1)

            @pl.when(jnp.logical_not(ends))
            def _():
                stg_wait(slots()[1], 2, g + 2)

            @pl.when(g >= 4)
            def _():
                buf = wos.at[slots()[2]]
                pltpu.make_async_copy(buf, buf, sems.at[SSTG + g + 2]).wait()

            @pl.when(g >= 6)
            def _():
                buf = wmodb.at[slots()[4]]
                pltpu.make_async_copy(buf, buf, sems.at[SSTG + g + 2]).wait()

            m3n, gslot, wslot, cj, cslot = slots()
            gn = jnp.where(ends, g, g + 1)
            wj = jnp.maximum(g - 4, 0)
            wgrp, wrow = NGRP + wj // 2, (wj % 2) * 256
            for k, cps in issue.items():
                @pl.when(g == k)
                def _():
                    for cp in cps:
                        cp.start()
            wtodo = [(r, c) for r in range(16) for c in range(8)]
            todo = [(dh, dp) for dh in range(2) for dp in range(256)]
            skip = [0] * RSK
            mtodo = list(range(0, D, 16))
            macc = [jnp.zeros((8, 512), f32)]

            def hook(v):
                if mtodo:
                    acc = macc[0] + jnp.concatenate([_zero_after(v)] * 4, axis=1)
                    for r in mtodo[:3]:
                        acc = mod_rows(acc, wmodb[cslot, r:r + 16, :], r)
                    del mtodo[:3]
                    macc[0] = acc

            for q in range(4):
                def b_of(k):
                    w = b_operand(g, q, k)
                    if skip:
                        skip.pop()
                        return w
                    nw = 0 if todo else WLP
                    for dh, dp in todo[:RLP]:
                        relayout(gn, gslot + dh, dh, dp, 1)
                    del todo[:RLP]
                    for r, c in wtodo[:nw]:
                        wqkv[wgrp, pl.ds(wrow + (c * 512 + r * 16), 16), :] = pltpu.bitcast(
                            wos[wslot, r * 32:(r + 1) * 32, c * 128:(c + 1) * 128], u32)
                    del wtodo[:nw]
                    return w
                c11, c12, c21, c22 = _strassen(lambda k: pltpu.bitcast(h7[k], bf16), b_of, hook)
                for blk, y in ((q + 4, _merge_rows(c12, c22)), (q, _merge_rows(c11, c21))):
                    for e in range(NPRE // 8):
                        tile, half = divmod(((8 * e + ROFF) % NR) // 8, 2)
                        rings[blk][tile, g, 4 * half:4 * half + 4, :] = _pack8(y[8 * e:8 * e + 8])
            assert not todo and not wtodo and not mtodo
            mod_finish(macc[0], cj)
            return m3n

        _loop("pre1", 0, NGRP, pre_iter)

    pl.run_scoped(prologue,
                  pltpu.VMEM((NSLOT, 512, 8, 128), bf16),
                  pltpu.VMEM((NWO, 512, D), bf16),
                  pltpu.VMEM((NMOD, D, 512), bf16),
                  pltpu.VMEM((7, NPRE // 4, 512), u32))

    def main(w7, w49):
        scale = DH ** -0.5
        ia = lax.broadcasted_iota(jnp.int32, (32, L), 0)
        ja = lax.broadcasted_iota(jnp.int32, (32, L), 1)
        mask_a = (((ia >= 16) & (ia < 24)) | (ja >= SEG)
                  | (jnp.where(ia < 16, ia + 16, ia - 16) >= ja))
        ib = lax.broadcasted_iota(jnp.int32, (48, 56), 0)
        jb = lax.broadcasted_iota(jnp.int32, (48, 56), 1)
        own = (ib < 40) == (jb < 40)
        mask_b = own & (((jb >= 32) & (jb < 48)) | (jnp.where(jb < 40, jb, jb - 8) <= ib))
        masked = -1e9 / scale
        j8 = lax.broadcasted_iota(jnp.int32, (8, 56), 1)
        fill_b = jnp.concatenate([jnp.where(j8 < 40, masked, -3e38).astype(f32)] * 5
                                 + [jnp.where(j8 < 40, -3e38, masked).astype(f32)], axis=0)

        def softmax(sc, mask, fill):
            sc = jnp.where(mask, sc, fill)
            mx = jnp.max(sc, axis=-1, keepdims=True)
            e = jnp.exp2((sc - mx) * (scale * 1.4426950408889634))
            den = jnp.sum(e, axis=-1, keepdims=True)
            return (e * pl.reciprocal(den, approx=True)).astype(bf16)

        def ride_tiles(it, is_b):
            first = (it == 0).astype(jnp.int32)
            if is_b:
                return 3 * it + 1 - first, 0, 3 * it + 2
            return 3 * it + 1 - first, 1, 3 * it + first

        def step(it, is_b, lhs_lo, lhs_hi, jobs, pins):
            NT, TOFF = NR // 16, ROFF // 16
            sega = (4 * it + TOFF) % NT
            seg = sega + 2 if is_b else sega
            wt = [(3 * it + (NPRE // 16 + TOFF + t + is_b)) % NT for t in range(2)]
            wr = [(wt[(t + is_b) // 2], (t + is_b) % 2) for t in range(3)]
            rt, rh, rf = ride_tiles(it, is_b)
            rt, rf = (rt + TOFF) % NT, (rf + TOFF) % NT
            lhs = jnp.concatenate([lhs_lo, lhs_hi], axis=1)
            QM, P, PART = {}, {}, {}
            mrow = 0 if is_b else 4

            def wblk(b, lo, n):
                r = (b % 8) * WP + lo
                return _unpack(wqkv[b // 8, r:r + n, :])

            def qkv_lo(i):
                for m in range(3):
                    PART[(m, i)] = jnp.dot(lhs_lo, wblk(m * H + i, 0, 256), preferred_element_type=f32)

            def qkv(i):
                for m in range(3):
                    b = m * H + i
                    if (m, i) in PART:
                        y = jnp.dot(lhs_hi, wblk(b, 256, 256),
                                    preferred_element_type=f32) + PART.pop((m, i))
                    else:
                        y = jnp.dot(lhs, wblk(b, 0, 512), preferred_element_type=f32)
                    if m < 2:
                        QM[b] = y[0:MEM] + pins[b] if b in pins else y[0:MEM]
                    if m == 2 or (m == 1 and not is_b):
                        kvm[b - H, mrow:mrow + 4, :] = _pack8(y[0:MEM])
                    for t in range(3):
                        rset(b, *wr[t], y[8 + 8 * t:16 + 8 * t])
                    for job in jobs.get(3 * i + m, []):
                        job(y)
                    side(3 * i + m)

            def keys(b):
                if is_b:
                    if b in QM:
                        mix = jnp.concatenate([_pack8(QM.pop(b)), kvm[b - H, 4:8, :]], axis=0)
                    else:
                        mix = kvm[b - H]
                    return _unpack(jnp.concatenate([rget(b, seg, 2), mix, rhalf(b, sega, 0)], axis=0))
                mk = _pack8(QM.pop(b)) if b in QM else kvm[b - H, 4:8, :]
                return _unpack(jnp.concatenate([rget(b, seg, 2), mk], axis=0))

            def scores(i):
                if is_b:
                    q = [rget(i, seg, 2), _pack8(QM.pop(i)), rhalf(i, sega, 0)]
                else:
                    q = [rget(i, seg + 1, 1), _pack8(QM.pop(i)), rhalf(i, seg, 1)]
                sc = lax.dot_general(_unpack(jnp.concatenate(q, axis=0)), keys(H + i),
                                     (((1,), (1,)), ((), ())), preferred_element_type=f32)
                P[i] = softmax(sc, mask_b, fill_b) if is_b else softmax(sc, mask_a, masked)

            def pv(i):
                o = jnp.dot(P.pop(i), keys(2 * H + i), preferred_element_type=f32)
                if is_b:
                    for e in range(4):
                        rset(i, seg + e // 2, e % 2, o[8 * e:8 * e + 8])
                    rset(i, sega, 0, o[40:48])
                    lhs_o[i, 0:4, :] = _pack8(o[SEG:L])
                else:
                    for e in range(2):
                        rset(i, seg + 1, e, o[8 * e:8 * e + 8])
                    rset(i, seg, 1, o[24:32])
                    lhs_o[i, 0:4, :] = _pack8(o[16:24])
                lhs_o[i, 4:8, :] = rhalf(i, rt, rh)
                lhs_o[i, 8:16, :] = rget(i, rf, 1)

            def wo_lhs(i0, i1):
                return _unpack(jnp.concatenate([lhs_o[i] for i in range(i0, i1)], axis=1))

            def wo_dot(lo, j, k):
                w = _unpack(wqkv[NGRP + k, j * 512:(j + 1) * 512, :])
                return jnp.dot(lo, w, preferred_element_type=f32)

            def side(d):
                for i in range(H):
                    if PVAT[i] == d:
                        pv(i)
                for i in range(H):
                    if SAT[i] == d:
                        scores(i)

            if is_b:
                for h in range(KSPLIT):
                    qkv_lo(h)
            for h in range(H):
                qkv(h)
            lo = [wo_lhs(8 * k, 8 * k + 8) for k in range(3)]
            acc = []
            for j in range(8):
                y = None
                for k in range(3):
                    z = wo_dot(lo[k], j, k)
                    y = z if y is None else z + y
                    for job in jobs.get(96 + 3 * j + k, []):
                        job(y)
                    side(96 + 3 * j + k)
                acc.append(y)
            lo = wo_lhs(24, H)
            for j in range(8):
                acc[j] = wo_dot(lo, j, 3) + acc[j]
                for job in jobs.get(120 + j, []):
                    job(acc[j])
            assert not (QM or P or PART)
            return jnp.concatenate(acc[0:4], axis=1), jnp.concatenate(acc[4:8], axis=1)

        def combine(c, n, y):
            mp, k1 = divmod(n, 8)
            m, p = divmod(mp, 4)
            c3 = jnp.minimum(c, 27)
            spare = pl.ds(pl.multiple_of(8 * (c // 64), 8), 8)
            if y is None:
                pass
            elif m == 0 and k1 < 7:
                ws3[16, spare, :] = y.astype(bf16)
            else:
                wsr[7, spare, 0:128] = y.astype(bf16)
            if k1 == 7:
                dst, base, r = w7, 0, (4 * m + p) * 32 + c
                blk = [wsr[4 + i, m * 16:(m + 1) * 16, j * 512 + p * 128:j * 512 + (p + 1) * 128]
                       .astype(f32) for i in range(2) for j in range(2)]
            else:
                dst, base = w49, 7 * k1
                if m == 0:
                    r = c3 * 4 + p
                    get = lambda i, j: ws3[4 * i + j, p * 16:(p + 1) * 16, :]
                else:
                    r = W4T + (p // 2) * 56 + c3 * 2 + p % 2
                    r0, c0 = (p % 2) * 16, (p // 2) * 128
                    get = lambda i, j: wsr[i, r0:r0 + 16, j * 256 + c0:j * 256 + c0 + 128]

                def quad(q):
                    return [get(2 * (q // 2) + i, 2 * (q % 2) + j).astype(f32)
                            for i in range(2) for j in range(2)]
                qi, qj, sign = _BTERMS[k1]
                blk = quad(qi)
                if qj is not None:
                    blk = [u + v if sign > 0 else u - v for u, v in zip(blk, quad(qj))]
            for k, op in enumerate(_b_operands(*blk)):
                for e in range(2):
                    dst[base + k, r, 4 * e:4 * e + 4, :] = _pack8(op[8 * e:8 * e + 8])

        def rec_body(it, gacc):
            stream_wait(it)
            lhs_lo = _unpack(jnp.concatenate([lhs_h[c] for c in range(4)], axis=1))
            lhs_hi = _unpack(jnp.concatenate([lhs_h[c] for c in range(4, 8)], axis=1))
            ra = jnp.maximum(it - 1, 0) * (2 * RIDE)
            for u in range(2):
                s = 2 * it + u
                jobs, pins = {}, {}
                for n, (su, d, g) in enumerate(SLOTS):
                    if su == u and d < 0:
                        combine(it, n, None)
                    elif su == u:
                        jobs.setdefault(d, []).append(
                            lambda y, n=n, g=g: combine(it, n, y[8 * g:8 * g + 8]))
                r1 = pl.multiple_of(jnp.minimum(NPRE + RIDE * (s + 1), S - RIDE), 8)
                xn = xbuf[pl.ds(r1, RIDE), :].astype(f32)
                if u == 0:
                    for k in range(2):
                        rm = pl.multiple_of(it * 32 + k * 16, 16)
                        gacc = mod_rows(gacc, wsr[6, k * 16:(k + 1) * 16, :], rm)
                    hn = adaln_a(xn, _zero_after(stage_a16(ra)))
                else:
                    def refill(y):
                        for cp in stream_copies(jnp.minimum(it + 1, NSEG // 2 - 1)):
                            cp.start()
                        spare = pl.ds(pl.multiple_of(8 * (it // 64), 8), 8)
                        pins[PIN] = _zero_after(ws3[16, spare, :].astype(f32))
                    jobs.setdefault(3 * (PIN - 4) + 2, []).append(refill)
                    hn = adaln_a(xn)
                    z = _zero_after(hn[0:8], hn[8:16], hn[16:24])
                    stage_a16(ra + 32, _zero_after(stage_a16(ra + 16, z)))
                a_lo, a_hi = step(it, u, lhs_lo, lhs_hi, jobs, pins)
                a = jnp.concatenate([a_lo, a_hi], axis=1)
                if u == 0:
                    lhs_lo = jnp.concatenate([a_lo[0:MEM], hn[:, 0:512]], axis=0).astype(bf16)
                    lhs_hi = jnp.concatenate([a_hi[0:MEM], hn[:, 512:1024]], axis=0).astype(bf16)
                else:
                    set_lhs(a[0:MEM], hn)
                rt, rh, rf = ride_tiles(it, u)
                rows = [pl.ds(pl.multiple_of(16 * rt + 8 * rh, 8), 8),
                        pl.ds(pl.multiple_of(16 * rf, 16), 16)]
                xs = [xbuf[r, :].astype(f32) for r in rows]
                xbuf[rows[0], :] = (xs[0] + modrows(2, 8) * a[8:16]).astype(bf16)
                xbuf[rows[1], :] = (xs[1] + modrows(2, 16) * a[16:32]).astype(bf16)
            return gacc

        gacc = _loop("rec", 0, NSEG // 2, rec_body, jnp.zeros((8, D), f32))
        for c in range(2):
            mod_finish(gacc[:, c * 512:(c + 1) * 512], 10 + c)
        stream_wait(NSEG // 2 - 1)

        def wo_prep(i, half, k):
            o = jnp.concatenate([_unpack(rings[4 * half + h][k, i]).astype(f32)
                                 for h in range(4)], axis=1)
            for t, op in enumerate(row_operands(o)):
                a7[half, t, k * 8:(k + 1) * 8, :] = op.astype(bf16)

        def wo_chunk(i, half, inext, extra):
            todo = list(range(NPRE // 16))

            def hook(v):
                if todo:
                    for h in range(4):
                        rings[4 * (1 - half) + h][i // 64, 4] = pltpu.bitcast(v[0:8], u32)
                    n = 2 if len(todo) % WPP == 0 else 1
                    for k in todo[:n]:
                        wo_prep(inext, 1 - half, k)
                    del todo[:n]
                extra(v)

            for j in range(4):
                def b_of(k):
                    def quad(q):
                        r = (j + 4 * (q % 2)) * 512 + half * 256 + (q // 2) * 128
                        return _unpack(wqkv[NGRP + i, r:r + 128, :])
                    qi, qj, sign = _BTERMS[k]
                    if qj is None:
                        return quad(qi)
                    u, v = quad(qi).astype(f32), quad(qj).astype(f32)
                    return (u + v if sign > 0 else u - v).astype(bf16)
                c11, c12, c21, c22 = _strassen(lambda k: a7[half, k], b_of, hook)
                for c, y in ((j + 4, _merge_rows(c12, c22)), (j, _merge_rows(c11, c21))):
                    cs = slice(c * 128, (c + 1) * 128)
                    h2buf[S - NPRE:S, cs] = h2buf[S - NPRE:S, cs] + y

        for k in range(NPRE // 16):
            wo_prep(0, 0, k)

        def wo_tail(i, _):
            st = {"n": 0, "prev": None}

            def extra(v):
                n = st["n"]
                st["n"] += 1
                if n % 16 == 2 and n // 16 < 3:
                    st["prev"] = stage_a16(S - NPRE - 48 + 16 * (n // 16),
                                           _zero_after(v, st["prev"]))
            wo_chunk(i, 0, i, extra)
            wo_chunk(i, 1, jnp.minimum(i + 1, 3), extra)
            return 0
        _loop("wotail", 0, 4, wo_tail)

        def gget(c, row, n):
            return pltpu.bitcast(wqkv[c, pl.ds(row, n), :], f32)

        def gset(c, row, val):
            wqkv[c, pl.ds(row, val.shape[0]), :] = pltpu.bitcast(val, u32)

        def wop(j):
            return lambda k: _unpack(w7[k, j * 32:(j + 1) * 32].reshape(256, 128))

        zpad = jnp.zeros((GPAD, 128), f32)
        for cb in range(8):
            gset(cb, 0, zpad)
            gset(cb, GPAD + S, zpad)

        shifts = (-1, -1, 1, 1, -2, -2, 2, 2)
        HB = MB // 2

        def shift_piece(r, half, k):
            gs = jnp.concatenate([gget(c, r + (k * 16 + GPAD + shifts[c]), 16)
                                  for c in range(8)], axis=1)
            ro = half * (HB // 2) + k * 8
            for t, op in enumerate(row_operands(gs)):
                n7[t, ro:ro + 8, :] = op.astype(bf16)

        def gate(v, i):
            gset(0, GPAD + S + GPAD + 8 * (i // S), v[0:8])

        def b_body(i, _):
            rl = S - NPRE + i * 128
            st = {"n": 0, "prev": [None, None]}

            def hook(v):
                n = st["n"]
                st["n"] += 1
                if n % BG == 0 and n // BG < 8:
                    k = n // BG
                    st["prev"][k % BCH] = stage_a16(rl + 16 * k,
                                                    _zero_after(v, st["prev"][k % BCH]),
                                                    (t7, 8 * k))

            ro = pl.multiple_of(i * 192, 64)
            for lhs, row in ((lambda k: n7[k, pl.ds(ro, 192), :], i * 384), (lambda k: t7[k], rl)):
                rg = pl.multiple_of(GPAD + row, 8)
                for j in range(4):
                    c11, c12, c21, c22 = _strassen(lhs, wop(j), hook)
                    gset(j + 4, rg, _gelu(_merge_rows(c12, c22)))
                    gset(j, rg, _gelu(_merge_rows(c11, c21)))
            return 0
        _loop("b", 0, S // MB, b_body)
        for k in range(HB // 16):
            shift_piece(0, 0, k)

        def n2_norm(r, k, anchor):
            v = _ln(h2buf[pl.ds(pl.multiple_of(r + k * 16, 16), 16), :], anchor)
            nrms[k // 2][(k % 2) * 16:(k % 2) * 16 + 16, :] = v
            return v[0:8] + v[8:16]

        def n2_ops(k, k1, v, i):
            nrm = nrms[k]
            nrm[pl.ds(pl.multiple_of(32 + 8 * (i // S), 8), 8), 0:128] = v[0:8]

            def quad(q):
                r0, c0 = (q // 2) * 16, (q % 2) * 512
                return [nrm[r0 + 8 * a:r0 + 8 * a + 8, c0 + 256 * b:c0 + 256 * b + 256]
                        for a in range(2) for b in range(2)]
            qi, qj, sign = _ATERMS[k1]
            blk = quad(qi)
            if qj is not None:
                blk = [u + w if sign > 0 else u - w for u, w in zip(blk, quad(qj))]
            for k2, op in enumerate(_a_operands(*blk)):
                d49[7 * k1 + k2, k * 8:(k + 1) * 8, :] = op.astype(bf16)

        def n2_hook(r, i, first, gap, lag, st):
            def hook(v):
                n = st["n"] - first
                st["n"] += 1
                if n >= 0 and n % gap == 0 and n // gap < MD // 16:
                    st["prev"] = n2_norm(r, n // gap, _zero_after(v, st["prev"]))
                for _ in range(st["per"]):
                    k, k1 = divmod(st["ops"], 7)
                    if k < MD // 32 and n >= (2 * k + 1) * gap + lag:
                        n2_ops(k, k1, v, i)
                        st["ops"] += 1
            return hook

        def stage_c(i, r, half, rnext, extra):
            rr = pl.multiple_of(r, 8)
            ro = half * (HB // 2)
            cnt = [0]

            def hook(v):
                n = cnt[0]
                cnt[0] += 1
                if n < HB // 16:
                    gate(v, i)
                    shift_piece(rnext, 1 - half, n)
                extra(v)

            for j in range(4):
                c11, c12, c21, c22 = _strassen(lambda k: n7[k, ro:ro + HB // 2, :], wop(4 + j),
                                               hook)
                for c, y in ((j + 4, _merge_rows(c12, c22)), (j, _merge_rows(c11, c21))):
                    cs = slice(c * 128, (c + 1) * 128)
                    h2buf[pl.ds(rr, HB), cs] = h2buf[pl.ds(rr, HB), cs] + y

        def c_body(i, _):
            r = pl.multiple_of(i * MB, MB)
            st = {"n": 0, "prev": None, "ops": 0, "per": 1}
            extra = n2_hook(0, i, 0, 4, 4, st)
            stage_c(i, r, 0, r + HB, extra)
            stage_c(i, r + HB, 1, jnp.minimum(i + 1, S // MB - 1) * MB, extra)
            assert st["ops"] == 28
            return 0
        _loop("c", 0, S // MB, c_body)

        def wop2(lo, n):
            return lambda k1, k: _unpack(w49[7 * k1 + k, lo:lo + n].reshape(8 * n, 128))

        def d_body(i, _):
            r = pl.multiple_of(i * MD, MD)
            rn = jnp.minimum(r + MD, S - MD)
            lhs = [d49[k] for k in range(49)]
            uops = []
            for t in range(7):
                cb = _strassen2(lambda k1, k: lhs[7 * k1 + k], wop2(t * 16, 16))
                uops.append(_a_operands2([[_gelu(c) for c in row] for row in cb]))
            ul = [[jnp.concatenate([u[k1][k] for u in uops], axis=1).astype(bf16)
                   for k in range(7)] for k1 in range(7)]
            st = {"n": 0, "prev": None, "ops": 0, "per": 1}
            hook = n2_hook(rn, i, DF, DG, DL, st)
            for t in range(2):
                cb = _strassen2(lambda k1, k: ul[k1][k], wop2(W4T + t * 56, 56), hook)
                for j in range(4):
                    y = jnp.concatenate([cb[q][j].reshape(MD // 32, 8, 128) for q in range(4)],
                                        axis=1).reshape(MD, 128)
                    c = 2 * j + t
                    cs = slice(c * 128, (c + 1) * 128)
                    gb = modrows(5, MD, c * 128, (c + 1) * 128)
                    o = xbuf[pl.ds(r, MD), cs].astype(f32) + gb * (h2buf[pl.ds(r, MD), cs] + y)
                    xbuf[pl.ds(r, MD), cs] = o.astype(bf16)
            assert st["ops"] == 28
            out_copy(r, MD).start()
            return 0
        _loop("d", 0, S // MD, d_body)

    pl.run_scoped(main,
                  pltpu.VMEM((7, 8 * 32, 8, 128), u32),
                  pltpu.VMEM((49, 2 * W4T, 8, 128), u32))

    out_copy(0, S).wait()


def _run(x, mem0, wq, wk, wv, wo, w1, w2, w3, w4, c, wmod):
    any_spec = pl.BlockSpec(memory_space=pl.ANY)
    return pl.pallas_call(
        _kernel,
        out_shape=jax.ShapeDtypeStruct((S, D), bf16),
        in_specs=[any_spec] * 12,
        out_specs=any_spec,
        scratch_shapes=[
            pltpu.VMEM((S + 2 * RIDE, D), bf16),
            pltpu.VMEM((NGRP + 4, 8 * WP, 128), u32),
            [pltpu.VMEM((NR // 16, 96 // NRING, 8, 128), u32)] * NRING,
            pltpu.VMEM((8, 16, 128), u32),
            pltpu.VMEM((H, 16, 128), u32),
            pltpu.VMEM((2 * H, 8, 128), u32),
            pltpu.VMEM((12, 8, 512), f32),
            pltpu.VMEM((D, 128), f32),
            pltpu.VMEM((S, D), f32),
            pltpu.VMEM((7, (S - NPRE) // 2, 512), bf16),
            pltpu.VMEM((17, 64, 128), bf16),
            pltpu.VMEM((8, 32, D), bf16),
            pltpu.VMEM((7, 64, 512), bf16),
            pltpu.VMEM((2, 7, NPRE // 2, 256), bf16),
            pltpu.VMEM((49, MD // 4, 256), bf16),
            [pltpu.VMEM((40, D), f32)] * (MD // 32),
            pltpu.VMEM((1, D), bf16),
            pltpu.SemaphoreType.DMA((9 + NGRP + 2,)),
        ],
        compiler_params=pltpu.CompilerParams(vmem_limit_bytes=124 * 1024 * 1024,
                                             disable_bounds_checks=True,
                                             disable_semaphore_checks=True),
    )(x, mem0, wq, wk, wv, wo, w1, w2, w3, w4, c, wmod)


def pallas_adaLN_cond__memory_aug_recurrent_mem_tr__mixer_s_mlp__prompt_kernel(
    A_x, A_mem0, A_Wq, A_Wk, A_Wv, A_Wo, A_seg_len, B_x, B_w1, B_w2, B_w3, B_w4, c, w_mod,
):
    del B_x
    assert A_x.shape == (1, S, D) and A_mem0.shape == (1, MEM, D)
    assert not isinstance(A_seg_len, int) or A_seg_len == SEG
    out = _run(A_x.reshape(S, D), A_mem0.reshape(MEM, D), A_Wq, A_Wk, A_Wv,
               A_Wo.reshape(H * DH, D),
               B_w1.reshape(2, D // 2, D), B_w2.reshape(2, D // 2, D),
               B_w3, B_w4.reshape(4, F // 4, D), c, w_mod)
    return out.reshape(1, S, D)
```

```python
import jax
import jax.numpy as jnp
from jax import lax
import jax.experimental.pallas as pl
import jax.experimental.pallas.tpu as pltpu

bf16 = jnp.bfloat16
f32 = jnp.float32
u32 = jnp.uint32

S = 2048
D = 1024
H = 32
DH = 128
F = 3584
MEM = 8
SEG = 32
NSEG = S // SEG
L = MEM + SEG
RIDE = 24
NPRE = S - RIDE * NSEG
NR = NPRE + 2 * SEG
ROFF = (-(S - NPRE)) % NR
WP = 516
NGRP = 12
NSLOT = 6
NMOD = 6
EPS = 1e-5
MD = 128
MB = 512
GPAD = 8
NRING = 8
NWO = 3
X0 = NPRE + 2 * RIDE
W4T = 7 * 16

RLP, WLP, RSK = 27, 22, 2
SAT = {i: max(6 * (i // 2) + 11, 17) for i in range(32)}
PVAT = {i: min(6 * (i // 2) + 23, 107) for i in range(32)}
KSPLIT = 2
PIN = 6
SLOTS = ([(0, -1, 0)] * 8 + [(0, n // 2, 3 * (n % 2)) for n in range(24)]
         + [(0, 96 + n, 0) for n in range(32)])
WPP, BG, BCH = 5, 2, 2
DF, DG, DL, DCH = 52, 3, 7, 2
_ONLY = None


def _loop(name, lo, hi, body, init=0):
    if _ONLY is not None and name not in _ONLY:
        return init
    with _scope(name):
        return lax.fori_loop(lo, hi, body, init)


class _NoScope:
    def __init__(self, name):
        del name

    def __enter__(self):
        return self

    def __exit__(self, *a):
        return False


_scope = _NoScope


def _zero_after(*vs):
    bits = None
    for v in vs:
        if v is not None:
            b = pltpu.bitcast(v[0:8, 0:128], u32)
            bits = b if bits is None else bits | b
    return pltpu.bitcast((bits >> 31) >> 1, f32)


def _ln(x, anchor=None):
    if anchor is not None:
        z = jnp.concatenate([anchor] * (x.shape[0] // 8), axis=0)
        x = jnp.concatenate([x[:, 0:128] + z, x[:, 128:]], axis=1)
    mu = jnp.mean(x, axis=-1, keepdims=True)
    xc = x - mu
    var = jnp.mean(xc * xc, axis=-1, keepdims=True)
    return xc * lax.rsqrt(var + EPS)


def _gelu(x):
    inner = x * (0.7978845608028654 + (0.7978845608028654 * 0.044715) * (x * x))
    hx = 0.5 * x
    return hx + hx * jnp.tanh(inner)


def _split_rows(x):
    m, n = x.shape
    x3 = x.reshape(m // 16, 16, n)
    return x3[:, 0:8, :].reshape(m // 2, n), x3[:, 8:16, :].reshape(m // 2, n)


def _merge_rows(top, bot):
    m, n = top.shape
    return jnp.concatenate([top.reshape(m // 8, 8, n), bot.reshape(m // 8, 8, n)],
                           axis=1).reshape(2 * m, n)


def _a_operands(a11, a12, a21, a22):
    return [a11 + a22, a21 + a22, a11, a22, a11 + a12, a21 - a11, a12 - a22]


def _b_operands(b11, b12, b21, b22):
    return [b11 + b22, b11, b12 - b22, b21 - b11, b22, b11 + b12, b21 + b22]


_ATERMS = ((0, 3, 1), (2, 3, 1), (0, None, 0), (3, None, 0), (0, 1, 1), (2, 0, -1), (1, 3, -1))
_BTERMS = ((0, 3, 1), (0, None, 0), (1, 3, -1), (2, 0, -1), (3, None, 0), (0, 1, 1), (2, 3, 1))


def _strassen(a_of, b_of, hook=lambda v: None):
    def prod(k):
        return jnp.dot(a_of(k), b_of(k), preferred_element_type=f32)
    p5 = prod(4)
    hook(p5)
    p3 = prod(2)
    hook(p3)
    c12 = p3 + p5
    p4 = prod(3)
    hook(p4)
    c11 = p4 - p5
    p2 = prod(1)
    hook(p2)
    c21 = p2 + p4
    c22 = p3 - p2
    p1 = prod(0)
    hook(p1)
    c11 = prod(6) + (c11 + p1)
    hook(c11)
    c22 = prod(5) + (c22 + p1)
    hook(c22)
    return c11, c12, c21, c22


def _a_operands2(b):
    sub = [_a_operands(b[i][j], b[i][2 + j], b[2 + i][j], b[2 + i][2 + j])
           for i in range(2) for j in range(2)]
    return [_a_operands(*[t[k] for t in sub]) for k in range(7)]


def _strassen2(a_of, b_of, hook=lambda v: None):
    def prod(k1):
        return _strassen(lambda k: a_of(k1, k), lambda k: b_of(k1, k), hook)

    def add(x, y):
        return [p + q for p, q in zip(x, y)]

    def sub(x, y):
        return [p - q for p, q in zip(x, y)]
    p5 = prod(4)
    p3 = prod(2)
    c12 = add(p3, p5)
    p4 = prod(3)
    c11 = sub(p4, p5)
    p2 = prod(1)
    c21 = add(p2, p4)
    c22 = sub(p3, p2)
    p1 = prod(0)
    c11 = add(add(c11, p1), prod(6))
    c22 = add(add(c22, p1), prod(5))
    cq = (c11, c12, c21, c22)
    return [[cq[2 * (i // 2) + j // 2][2 * (i % 2) + j % 2] for j in range(4)] for i in range(4)]


def _pack8(v):
    return pltpu.bitcast(v.astype(bf16), u32)


def _unpack(w):
    return pltpu.bitcast(w, bf16)


def _kernel(x_hbm, mem0_hbm, wq_hbm, wk_hbm, wv_hbm, wo_hbm, w1_hbm, w2_hbm, w3_hbm, w4_hbm,
            c_hbm, wmod_hbm, out_hbm,
            xbuf, wqkv, rings, lhs_h, lhs_o, kvm, modv, scol, h2buf, n7, ws3, wsr, t7, a7, d49,
            nrms, c_ref, sems):
    w_hbms = (wq_hbm, wk_hbm, wv_hbm)
    SMOD, SSTG = 5, 9
    sem_x, sem_out, sem_w, sem_g, sem_r = (sems.at[k] for k in range(5))

    def rget(b, tile, n):
        return jnp.concatenate([rings[b % NRING][tile + e, b // NRING] for e in range(n)], axis=0)

    def rhalf(b, tile, half):
        return rings[b % NRING][tile, b // NRING, 4 * half:4 * half + 4, :]

    def rset(b, tile, half, val):
        rings[b % NRING][tile, b // NRING, 4 * half:4 * half + 4, :] = _pack8(val)

    x_copy = pltpu.make_async_copy(x_hbm.at[pl.ds(0, X0), :], xbuf.at[pl.ds(0, X0), :], sem_x)

    def stream_copies(c):
        al, lo = ((lambda v, m: v), min) if isinstance(c, int) else (pl.multiple_of, jnp.minimum)
        c3 = lo(c, 27)
        cps = [pltpu.make_async_copy(
            w3_hbm.at[pl.ds(al(i * 256 + (c3 % 4) * 64, 64), 64),
                      pl.ds(al(j * (F // 4) + (c3 // 4) * 128, 128), 128)],
            ws3.at[4 * i + j], sem_w) for i in range(4) for j in range(4)]
        dst = X0 + 2 * RIDE * c
        return [
            pltpu.make_async_copy(w4_hbm.at[:, pl.ds(al(c3 * 32, 32), 32), :],
                                  wsr.at[pl.ds(0, 4)], sem_g),
            pltpu.make_async_copy(w1_hbm.at[:, pl.ds(al(c * 16, 16), 16), :],
                                  wsr.at[pl.ds(4, 2), pl.ds(0, 16), :], sem_g),
            pltpu.make_async_copy(w2_hbm.at[:, pl.ds(al(c * 16, 16), 16), :],
                                  wsr.at[pl.ds(4, 2), pl.ds(16, 16), :], sem_g),
            pltpu.make_async_copy(wmod_hbm.at[pl.ds(al(c * 32, 32), 32), pl.ds(5 * D, D)],
                                  wsr.at[6], sem_g),
            pltpu.make_async_copy(x_hbm.at[pl.ds(al(lo(dst, S - 2 * RIDE), 16), 2 * RIDE), :],
                                  xbuf.at[pl.ds(al(dst, 16), 2 * RIDE), :], sem_r)] + cps

    def stream_wait(c):
        for dst, sem in ((ws3.at[pl.ds(0, 16)], sem_w), (wsr.at[pl.ds(0, 7)], sem_g),
                         (xbuf.at[pl.ds(X0 + 2 * RIDE * c, 2 * RIDE), :], sem_r)):
            pltpu.make_async_copy(dst, dst, sem).wait()

    def out_copy(row, n):
        return pltpu.make_async_copy(xbuf.at[pl.ds(row, n), :], out_hbm.at[pl.ds(row, n), :],
                                     sem_out)

    def mod_rows(acc, w, r):
        sc = jnp.concatenate([scol[pl.ds(r, 16), :]] * (w.shape[1] // 128), axis=1)
        p = w.astype(f32) * sc
        return acc + p[0:8] + p[8:16]

    def mod_finish(acc, j):
        is_scale = jnp.logical_or(j // 2 == 1, j // 2 == 4)
        tot = jnp.sum(acc, axis=0, keepdims=True) + jnp.where(is_scale, 1.0, 0.0)
        modv[j] = jnp.broadcast_to(tot, (8, 512))

    def modrows(k, n, lo=0, hi=D):
        m = jnp.concatenate([modv[2 * k], modv[2 * k + 1]], axis=1)[:, lo:hi]
        return jnp.concatenate([m] * (n // 8), axis=0)

    def adaln_a(xv, anchor=None):
        n = xv.shape[0]
        return _ln(xv, anchor) * modrows(1, n) + modrows(0, n)

    def adaln_b(xv, anchor=None):
        n = xv.shape[0]
        return _ln(xv, anchor) * modrows(4, n) + modrows(3, n)

    def set_lhs(mem, hn):
        v = jnp.concatenate([mem, hn], axis=0)
        for c in range(8):
            for e in range(4):
                lhs_h[c, 4 * e:4 * e + 4, :] = _pack8(v[8 * e:8 * e + 8, c * 128:(c + 1) * 128])

    def row_operands(v):
        top, bot = _split_rows(v)
        k = v.shape[1] // 2
        return _a_operands(top[:, :k], top[:, k:], bot[:, :k], bot[:, k:])

    def stage_a16(r, anchor=None, dst=None):
        rr = pl.multiple_of(r, 16)
        xv = xbuf[pl.ds(rr, 16), :]
        if dst is not None:
            xv = (xv.astype(f32) + modrows(2, 16) * h2buf[pl.ds(rr, 16), :]).astype(bf16)
            xbuf[pl.ds(rr, 16), :] = xv
        h2 = adaln_b(xv.astype(f32), anchor)
        h2buf[pl.ds(rr, 16), :] = h2
        ref, ro = (n7, pl.multiple_of(rr // 2, 8)) if dst is None else dst
        ops = row_operands(_ln(h2))
        for t, op in enumerate(ops):
            ref[t, pl.ds(ro, 8), :] = op.astype(bf16)
        return ops[0]

    def prologue(stg, wos, wmodb, h7):
        def mod_copy(j):
            return pltpu.make_async_copy(wmod_hbm.at[:, pl.ds(j * 512, 512)], wmodb.at[j % NMOD],
                                         sems.at[SSTG + j + 4 if j >= 4 else SMOD + j])

        def piece_copy(g, dh):
            return pltpu.make_async_copy(
                w_hbms[g // 4].at[pl.ds(dh * 512, 512), pl.ds((g % 4) * 8, 8), :],
                stg.at[(2 * g + dh) % NSLOT], sems.at[SSTG + (g + 1 if g else dh)])

        def wo_copy(j):
            return pltpu.make_async_copy(wo_hbm.at[pl.ds(j * 512, 512), :], wos.at[j % NWO],
                                         sems.at[SSTG + j + 6])

        def group_start(g):
            for dh in range(2):
                piece_copy(g, dh).start()

        def stg_wait(slot, n, sem):
            dst = stg.at[pl.ds(slot, n)]
            pltpu.make_async_copy(dst, dst, sems.at[SSTG + sem]).wait()

        def relayout(g, slot, dh, lo_dp, n_dp):
            for u in range(n_dp):
                dp = lo_dp + u
                ev = pltpu.bitcast(stg[slot, 2 * dp].astype(f32), u32)
                od = pltpu.bitcast(stg[slot, 2 * dp + 1].astype(f32), u32)
                wqkv[g, pl.ds(dh * 256 + dp, 8, stride=WP), :] = (ev >> 16) | od

        def b_operand(g, q, k):
            def quad(i):
                r = (q + 4 * (i % 2)) * WP + (i // 2) * 256
                return _unpack(wqkv[g, r:r + 256, :])
            i, j, sign = _BTERMS[k]
            if j is None:
                return quad(i)
            u, v = quad(i).astype(f32), quad(j).astype(f32)
            return (u + v if sign > 0 else u - v).astype(bf16)

        c_copy = pltpu.make_async_copy(c_hbm, c_ref, sem_g)
        m_copy = pltpu.make_async_copy(mem0_hbm, wsr.at[7, pl.ds(0, MEM), :], sem_r)
        c_copy.start()
        m_copy.start()
        x_copy.start()
        for j in range(4):
            mod_copy(j).start()
        for g in range(3):
            group_start(g)
        h2buf[S - NPRE:S, :] = jnp.zeros((NPRE, D), f32)
        wos[2] = jnp.zeros((512, D), bf16)
        c_copy.wait()
        m_copy.wait()
        cv = c_ref[...].astype(f32)
        sv = jnp.broadcast_to(cv * (1.0 / (1.0 + jnp.exp(-cv))), (128, D))
        for k in range(8):
            scol[k * 128:(k + 1) * 128, :] = sv[:, k * 128:(k + 1) * 128].T
        x_copy.wait()

        def ln0_body(i, _):
            r = pl.multiple_of(i * 64, 64)
            h2buf[pl.ds(r, 64), :] = _ln(xbuf[pl.ds(r, 64), :].astype(f32))
            return 0
        lax.fori_loop(0, NPRE // 64, ln0_body, 0)

        def mod0_body(j, _):
            pltpu.make_async_copy(wmodb.at[j], wmodb.at[j], sems.at[SMOD + j]).wait()
            accs = [jnp.zeros((8, 512), f32)] * 2
            for k in range(64):
                accs[k % 2] = mod_rows(accs[k % 2], wmodb[j, k * 16:(k + 1) * 16, :], k * 16)
            mod_finish(accs[0] + accs[1], j)
            return 0
        _loop("mod0", 0, 4, mod0_body)

        def hpre_body(i, _):
            r = pl.multiple_of(i * 32, 32)
            hv = h2buf[pl.ds(r, 32), :] * modrows(1, 32) + modrows(0, 32)
            ro = pl.multiple_of(i * 8, 8)
            for t, op in enumerate(row_operands(hv)):
                h7[t, pl.ds(ro, 8), :] = pltpu.bitcast(op.astype(bf16), u32)
            return 0
        lax.fori_loop(0, NPRE // 32, hpre_body, 0)
        set_lhs(wsr[7, 0:MEM, :].astype(f32), adaln_a(xbuf[NPRE:NPRE + RIDE, :].astype(f32)))

        def relayout_now(g, dh):
            def rl_body(t, _):
                relayout(g, 2 * g + dh, dh, t * 32, 32)
                return 0
            lax.fori_loop(0, 8, rl_body, 0)

        for dh in range(2):
            stg_wait(dh, 1, dh)
            relayout_now(0, dh)

        grp = lambda g: [piece_copy(g, 0), piece_copy(g, 1)]
        issue = {0: [wo_copy(0)], 1: grp(3) + grp(4), 2: grp(5) + [wo_copy(1), mod_copy(4)],
                 3: grp(6) + [mod_copy(5), mod_copy(6)], 4: grp(7) + [wo_copy(2)],
                 5: grp(8) + [wo_copy(3), mod_copy(7)], 6: grp(9) + [wo_copy(4)],
                 7: grp(10) + [wo_copy(5), mod_copy(8)], 8: grp(11) + [wo_copy(6)],
                 9: [wo_copy(7), mod_copy(9)], 10: stream_copies(0)}

        def pre_iter(g, m3):

            @pl.when(g == 1)
            def _():
                stg_wait(2, 2, 2)
                relayout_now(1, 0)
                relayout_now(1, 1)

            def slots():
                m3n = jnp.where(m3 == 2, 0, m3 + 1)
                cj = jnp.maximum(g - 2, 3)
                return (m3n, 2 * jnp.where(ends, m3, m3n),
                        jnp.where(jnp.logical_or(g < 4, m3 == 0), 2, m3 - 1),
                        cj, jnp.where(cj >= NMOD, cj - NMOD, cj))

            ends = jnp.logical_or(g == 0, g == NGRP - 1)

            @pl.when(jnp.logical_not(ends))
            def _():
                stg_wait(slots()[1], 2, g + 2)

            @pl.when(g >= 4)
            def _():
                buf = wos.at[slots()[2]]
                pltpu.make_async_copy(buf, buf, sems.at[SSTG + g + 2]).wait()

            @pl.when(g >= 6)
            def _():
                buf = wmodb.at[slots()[4]]
                pltpu.make_async_copy(buf, buf, sems.at[SSTG + g + 2]).wait()

            m3n, gslot, wslot, cj, cslot = slots()
            gn = jnp.where(ends, g, g + 1)
            wj = jnp.maximum(g - 4, 0)
            wgrp, wrow = NGRP + wj // 2, (wj % 2) * 256
            for k, cps in issue.items():
                @pl.when(g == k)
                def _():
                    for cp in cps:
                        cp.start()
            wtodo = [(r, c) for r in range(16) for c in range(8)]
            todo = [(dh, dp) for dh in range(2) for dp in range(256)]
            skip = [0] * RSK
            mtodo = list(range(0, D, 16))
            macc = [jnp.zeros((8, 512), f32)]

            def hook(v):
                if mtodo:
                    acc = macc[0] + jnp.concatenate([_zero_after(v)] * 4, axis=1)
                    for r in mtodo[:3]:
                        acc = mod_rows(acc, wmodb[cslot, r:r + 16, :], r)
                    del mtodo[:3]
                    macc[0] = acc

            for q in range(4):
                def b_of(k):
                    w = b_operand(g, q, k)
                    if skip:
                        skip.pop()
                        return w
                    nw = 0 if todo else WLP
                    for dh, dp in todo[:RLP]:
                        relayout(gn, gslot + dh, dh, dp, 1)
                    del todo[:RLP]
                    for r, c in wtodo[:nw]:
                        wqkv[wgrp, pl.ds(wrow + (c * 512 + r * 16), 16), :] = pltpu.bitcast(
                            wos[wslot, r * 32:(r + 1) * 32, c * 128:(c + 1) * 128], u32)
                    del wtodo[:nw]
                    return w
                c11, c12, c21, c22 = _strassen(lambda k: pltpu.bitcast(h7[k], bf16), b_of, hook)
                for blk, y in ((q + 4, _merge_rows(c12, c22)), (q, _merge_rows(c11, c21))):
                    for e in range(NPRE // 8):
                        tile, half = divmod(((8 * e + ROFF) % NR) // 8, 2)
                        rings[blk][tile, g, 4 * half:4 * half + 4, :] = _pack8(y[8 * e:8 * e + 8])
            assert not todo and not wtodo and not mtodo
            mod_finish(macc[0], cj)
            return m3n

        _loop("pre1", 0, NGRP, pre_iter)

    pl.run_scoped(prologue,
                  pltpu.VMEM((NSLOT, 512, 8, 128), bf16),
                  pltpu.VMEM((NWO, 512, D), bf16),
                  pltpu.VMEM((NMOD, D, 512), bf16),
                  pltpu.VMEM((7, NPRE // 4, 512), u32))

    def main(w7, w49):
        scale = DH ** -0.5
        ia = lax.broadcasted_iota(jnp.int32, (32, L), 0)
        ja = lax.broadcasted_iota(jnp.int32, (32, L), 1)
        mask_a = (((ia >= 16) & (ia < 24)) | (ja >= SEG)
                  | (jnp.where(ia < 16, ia + 16, ia - 16) >= ja))
        ib = lax.broadcasted_iota(jnp.int32, (48, 56), 0)
        jb = lax.broadcasted_iota(jnp.int32, (48, 56), 1)
        own = (ib < 40) == (jb < 40)
        mask_b = own & (((jb >= 32) & (jb < 48)) | (jnp.where(jb < 40, jb, jb - 8) <= ib))
        masked = -1e9 / scale
        j8 = lax.broadcasted_iota(jnp.int32, (8, 56), 1)
        fill_b = jnp.concatenate([jnp.where(j8 < 40, masked, -3e38).astype(f32)] * 5
                                 + [jnp.where(j8 < 40, -3e38, masked).astype(f32)], axis=0)

        def softmax(sc, mask, fill):
            sc = jnp.where(mask, sc, fill)
            mx = jnp.max(sc, axis=-1, keepdims=True)
            e = jnp.exp2((sc - mx) * (scale * 1.4426950408889634))
            den = jnp.sum(e, axis=-1, keepdims=True)
            return (e * pl.reciprocal(den, approx=True)).astype(bf16)

        def ride_tiles(it, is_b):
            first = (it == 0).astype(jnp.int32)
            if is_b:
                return 3 * it + 1 - first, 0, 3 * it + 2
            return 3 * it + 1 - first, 1, 3 * it + first

        def step(it, is_b, lhs_lo, lhs_hi, jobs, pins):
            NT, TOFF = NR // 16, ROFF // 16
            sega = (4 * it + TOFF) % NT
            seg = sega + 2 if is_b else sega
            wt = [(3 * it + (NPRE // 16 + TOFF + t + is_b)) % NT for t in range(2)]
            wr = [(wt[(t + is_b) // 2], (t + is_b) % 2) for t in range(3)]
            rt, rh, rf = ride_tiles(it, is_b)
            rt, rf = (rt + TOFF) % NT, (rf + TOFF) % NT
            lhs = jnp.concatenate([lhs_lo, lhs_hi], axis=1)
            QM, P, PART = {}, {}, {}
            mrow = 0 if is_b else 4

            def wblk(b, lo, n):
                r = (b % 8) * WP + lo
                return _unpack(wqkv[b // 8, r:r + n, :])

            def qkv_lo(i):
                for m in range(3):
                    PART[(m, i)] = jnp.dot(lhs_lo, wblk(m * H + i, 0, 256), preferred_element_type=f32)

            def qkv(i):
                for m in range(3):
                    b = m * H + i
                    if (m, i) in PART:
                        y = jnp.dot(lhs_hi, wblk(b, 256, 256),
                                    preferred_element_type=f32) + PART.pop((m, i))
                    else:
                        y = jnp.dot(lhs, wblk(b, 0, 512), preferred_element_type=f32)
                    if m < 2:
                        QM[b] = y[0:MEM] + pins[b] if b in pins else y[0:MEM]
                    if m == 2 or (m == 1 and not is_b):
                        kvm[b - H, mrow:mrow + 4, :] = _pack8(y[0:MEM])
                    for t in range(3):
                        rset(b, *wr[t], y[8 + 8 * t:16 + 8 * t])
                    for job in jobs.get(3 * i + m, []):
                        job(y)
                    side(3 * i + m)

            def keys(b):
                if is_b:
                    if b in QM:
                        mix = jnp.concatenate([_pack8(QM.pop(b)), kvm[b - H, 4:8, :]], axis=0)
                    else:
                        mix = kvm[b - H]
                    return _unpack(jnp.concatenate([rget(b, seg, 2), mix, rhalf(b, sega, 0)], axis=0))
                mk = _pack8(QM.pop(b)) if b in QM else kvm[b - H, 4:8, :]
                return _unpack(jnp.concatenate([rget(b, seg, 2), mk], axis=0))

            def scores(i):
                if is_b:
                    q = [rget(i, seg, 2), _pack8(QM.pop(i)), rhalf(i, sega, 0)]
                else:
                    q = [rget(i, seg + 1, 1), _pack8(QM.pop(i)), rhalf(i, seg, 1)]
                sc = lax.dot_general(_unpack(jnp.concatenate(q, axis=0)), keys(H + i),
                                     (((1,), (1,)), ((), ())), preferred_element_type=f32)
                P[i] = softmax(sc, mask_b, fill_b) if is_b else softmax(sc, mask_a, masked)

            def pv(i):
                o = jnp.dot(P.pop(i), keys(2 * H + i), preferred_element_type=f32)
                if is_b:
                    for e in range(4):
                        rset(i, seg + e // 2, e % 2, o[8 * e:8 * e + 8])
                    rset(i, sega, 0, o[40:48])
                    lhs_o[i, 0:4, :] = _pack8(o[SEG:L])
                else:
                    for e in range(2):
                        rset(i, seg + 1, e, o[8 * e:8 * e + 8])
                    rset(i, seg, 1, o[24:32])
                    lhs_o[i, 0:4, :] = _pack8(o[16:24])
                lhs_o[i, 4:8, :] = rhalf(i, rt, rh)
                lhs_o[i, 8:16, :] = rget(i, rf, 1)

            def wo_lhs(i0, i1):
                return _unpack(jnp.concatenate([lhs_o[i] for i in range(i0, i1)], axis=1))

            def wo_dot(lo, j, k):
                w = _unpack(wqkv[NGRP + k, j * 512:(j + 1) * 512, :])
                return jnp.dot(lo, w, preferred_element_type=f32)

            def side(d):
                for i in range(H):
                    if PVAT[i] == d:
                        pv(i)
                for i in range(H):
                    if SAT[i] == d:
                        scores(i)

            if is_b:
                for h in range(KSPLIT):
                    qkv_lo(h)
            for h in range(H):
                qkv(h)
            lo = [wo_lhs(8 * k, 8 * k + 8) for k in range(3)]
            acc = []
            for j in range(8):
                y = None
                for k in range(3):
                    z = wo_dot(lo[k], j, k)
                    y = z if y is None else z + y
                    for job in jobs.get(96 + 3 * j + k, []):
                        job(y)
                    side(96 + 3 * j + k)
                acc.append(y)
            lo = wo_lhs(24, H)
            for j in range(8):
                acc[j] = wo_dot(lo, j, 3) + acc[j]
                for job in jobs.get(120 + j, []):
                    job(acc[j])
            assert not (QM or P or PART)
            return jnp.concatenate(acc[0:4], axis=1), jnp.concatenate(acc[4:8], axis=1)

        def combine(c, n, y):
            mp, k1 = divmod(n, 8)
            m, p = divmod(mp, 4)
            c3 = jnp.minimum(c, 27)
            spare = pl.ds(pl.multiple_of(8 * (c // 64), 8), 8)
            if y is None:
                pass
            elif m == 0 and k1 < 7:
                ws3[16, spare, :] = y.astype(bf16)
            else:
                wsr[7, spare, 0:128] = y.astype(bf16)
            if k1 == 7:
                dst, base, r = w7, 0, (4 * m + p) * 32 + c
                blk = [wsr[4 + i, m * 16:(m + 1) * 16, j * 512 + p * 128:j * 512 + (p + 1) * 128]
                       .astype(f32) for i in range(2) for j in range(2)]
            else:
                dst, base = w49, 7 * k1
                if m == 0:
                    r = c3 * 4 + p
                    get = lambda i, j: ws3[4 * i + j, p * 16:(p + 1) * 16, :]
                else:
                    r = W4T + (p // 2) * 56 + c3 * 2 + p % 2
                    r0, c0 = (p % 2) * 16, (p // 2) * 128
                    get = lambda i, j: wsr[i, r0:r0 + 16, j * 256 + c0:j * 256 + c0 + 128]

                def quad(q):
                    return [get(2 * (q // 2) + i, 2 * (q % 2) + j).astype(f32)
                            for i in range(2) for j in range(2)]
                qi, qj, sign = _BTERMS[k1]
                blk = quad(qi)
                if qj is not None:
                    blk = [u + v if sign > 0 else u - v for u, v in zip(blk, quad(qj))]
            for k, op in enumerate(_b_operands(*blk)):
                for e in range(2):
                    dst[base + k, r, 4 * e:4 * e + 4, :] = _pack8(op[8 * e:8 * e + 8])

        def rec_body(it, gacc):
            stream_wait(it)
            lhs_lo = _unpack(jnp.concatenate([lhs_h[c] for c in range(4)], axis=1))
            lhs_hi = _unpack(jnp.concatenate([lhs_h[c] for c in range(4, 8)], axis=1))
            ra = jnp.maximum(it - 1, 0) * (2 * RIDE)
            for u in range(2):
                s = 2 * it + u
                jobs, pins = {}, {}
                for n, (su, d, g) in enumerate(SLOTS):
                    if su == u and d < 0:
                        combine(it, n, None)
                    elif su == u:
                        jobs.setdefault(d, []).append(
                            lambda y, n=n, g=g: combine(it, n, y[8 * g:8 * g + 8]))
                r1 = pl.multiple_of(jnp.minimum(NPRE + RIDE * (s + 1), S - RIDE), 8)
                xn = xbuf[pl.ds(r1, RIDE), :].astype(f32)
                if u == 0:
                    for k in range(2):
                        rm = pl.multiple_of(it * 32 + k * 16, 16)
                        gacc = mod_rows(gacc, wsr[6, k * 16:(k + 1) * 16, :], rm)
                    hn = adaln_a(xn, _zero_after(stage_a16(ra)))
                else:
                    def refill(y):
                        for cp in stream_copies(jnp.minimum(it + 1, NSEG // 2 - 1)):
                            cp.start()
                        spare = pl.ds(pl.multiple_of(8 * (it // 64), 8), 8)
                        pins[PIN] = _zero_after(ws3[16, spare, :].astype(f32))
                    jobs.setdefault(3 * (PIN - 4) + 2, []).append(refill)
                    hn = adaln_a(xn)
                    z = _zero_after(hn[0:8], hn[8:16], hn[16:24])
                    stage_a16(ra + 32, _zero_after(stage_a16(ra + 16, z)))
                a_lo, a_hi = step(it, u, lhs_lo, lhs_hi, jobs, pins)
                a = jnp.concatenate([a_lo, a_hi], axis=1)
                if u == 0:
                    lhs_lo = jnp.concatenate([a_lo[0:MEM], hn[:, 0:512]], axis=0).astype(bf16)
                    lhs_hi = jnp.concatenate([a_hi[0:MEM], hn[:, 512:1024]], axis=0).astype(bf16)
                else:
                    set_lhs(a[0:MEM], hn)
                rt, rh, rf = ride_tiles(it, u)
                rows = [pl.ds(pl.multiple_of(16 * rt + 8 * rh, 8), 8),
                        pl.ds(pl.multiple_of(16 * rf, 16), 16)]
                xs = [xbuf[r, :].astype(f32) for r in rows]
                xbuf[rows[0], :] = (xs[0] + modrows(2, 8) * a[8:16]).astype(bf16)
                xbuf[rows[1], :] = (xs[1] + modrows(2, 16) * a[16:32]).astype(bf16)
            return gacc

        gacc = _loop("rec", 0, NSEG // 2, rec_body, jnp.zeros((8, D), f32))
        for c in range(2):
            mod_finish(gacc[:, c * 512:(c + 1) * 512], 10 + c)
        stream_wait(NSEG // 2 - 1)

        def wo_prep(i, half, k):
            o = jnp.concatenate([_unpack(rings[4 * half + h][k, i]).astype(f32)
                                 for h in range(4)], axis=1)
            for t, op in enumerate(row_operands(o)):
                a7[half, t, k * 8:(k + 1) * 8, :] = op.astype(bf16)

        def wo_chunk(i, half, inext, extra):
            todo = list(range(NPRE // 16))

            def hook(v):
                if todo:
                    for h in range(4):
                        rings[4 * (1 - half) + h][i // 64, 4] = pltpu.bitcast(v[0:8], u32)
                    n = 2 if len(todo) % WPP == 0 else 1
                    for k in todo[:n]:
                        wo_prep(inext, 1 - half, k)
                    del todo[:n]
                extra(v)

            for j in range(4):
                def b_of(k):
                    def quad(q):
                        r = (j + 4 * (q % 2)) * 512 + half * 256 + (q // 2) * 128
                        return _unpack(wqkv[NGRP + i, r:r + 128, :])
                    qi, qj, sign = _BTERMS[k]
                    if qj is None:
                        return quad(qi)
                    u, v = quad(qi).astype(f32), quad(qj).astype(f32)
                    return (u + v if sign > 0 else u - v).astype(bf16)
                c11, c12, c21, c22 = _strassen(lambda k: a7[half, k], b_of, hook)
                for c, y in ((j + 4, _merge_rows(c12, c22)), (j, _merge_rows(c11, c21))):
                    cs = slice(c * 128, (c + 1) * 128)
                    h2buf[S - NPRE:S, cs] = h2buf[S - NPRE:S, cs] + y

        for k in range(NPRE // 16):
            wo_prep(0, 0, k)

        def wo_tail(i, _):
            st = {"n": 0, "prev": None}

            def extra(v):
                n = st["n"]
                st["n"] += 1
                if n % 16 == 2 and n // 16 < 3:
                    st["prev"] = stage_a16(S - NPRE - 48 + 16 * (n // 16),
                                           _zero_after(v, st["prev"]))
            wo_chunk(i, 0, i, extra)
            wo_chunk(i, 1, jnp.minimum(i + 1, 3), extra)
            return 0
        _loop("wotail", 0, 4, wo_tail)

        def gget(c, row, n):
            return pltpu.bitcast(wqkv[c, pl.ds(row, n), :], f32)

        def gset(c, row, val):
            wqkv[c, pl.ds(row, val.shape[0]), :] = pltpu.bitcast(val, u32)

        def wop(j):
            return lambda k: _unpack(w7[k, j * 32:(j + 1) * 32].reshape(256, 128))

        zpad = jnp.zeros((GPAD, 128), f32)
        for cb in range(8):
            gset(cb, 0, zpad)
            gset(cb, GPAD + S, zpad)

        shifts = (-1, -1, 1, 1, -2, -2, 2, 2)
        HB = MB // 2

        def shift_piece(r, half, k):
            gs = jnp.concatenate([gget(c, r + (k * 16 + GPAD + shifts[c]), 16)
                                  for c in range(8)], axis=1)
            ro = half * (HB // 2) + k * 8
            for t, op in enumerate(row_operands(gs)):
                n7[t, ro:ro + 8, :] = op.astype(bf16)

        def gate(v, i):
            gset(0, GPAD + S + GPAD + 8 * (i // S), v[0:8])

        def b_body(i, _):
            rl = S - NPRE + i * 128
            st = {"n": 0, "prev": [None, None]}

            def hook(v):
                n = st["n"]
                st["n"] += 1
                if n % BG == 0 and n // BG < 8:
                    k = n // BG
                    st["prev"][k % BCH] = stage_a16(rl + 16 * k,
                                                    _zero_after(v, st["prev"][k % BCH]),
                                                    (t7, 8 * k))

            ro = pl.multiple_of(i * 192, 64)
            for lhs, row in ((lambda k: n7[k, pl.ds(ro, 192), :], i * 384), (lambda k: t7[k], rl)):
                rg = pl.multiple_of(GPAD + row, 8)
                for j in range(4):
                    c11, c12, c21, c22 = _strassen(lhs, wop(j), hook)
                    gset(j + 4, rg, _gelu(_merge_rows(c12, c22)))
                    gset(j, rg, _gelu(_merge_rows(c11, c21)))
            return 0
        _loop("b", 0, S // MB, b_body)
        for k in range(HB // 16):
            shift_piece(0, 0, k)

        def n2_norm(r, k, anchor):
            v = _ln(h2buf[pl.ds(pl.multiple_of(r + k * 16, 16), 16), :], anchor)
            nrms[k // 2][(k % 2) * 16:(k % 2) * 16 + 16, :] = v
            return v[0:8] + v[8:16]

        def n2_ops(k, k1, v, i):
            nrm = nrms[k]
            nrm[pl.ds(pl.multiple_of(32 + 8 * (i // S), 8), 8), 0:128] = v[0:8]

            def quad(q):
                r0, c0 = (q // 2) * 16, (q % 2) * 512
                return [nrm[r0 + 8 * a:r0 + 8 * a + 8, c0 + 256 * b:c0 + 256 * b + 256]
                        for a in range(2) for b in range(2)]
            qi, qj, sign = _ATERMS[k1]
            blk = quad(qi)
            if qj is not None:
                blk = [u + w if sign > 0 else u - w for u, w in zip(blk, quad(qj))]
            for k2, op in enumerate(_a_operands(*blk)):
                d49[7 * k1 + k2, k * 8:(k + 1) * 8, :] = op.astype(bf16)

        def n2_hook(r, i, first, gap, lag, st):
            def hook(v):
                n = st["n"] - first
                st["n"] += 1
                if n >= 0 and n % gap == 0 and n // gap < MD // 16:
                    ch = (n // gap) % st["ch"]
                    st[ch] = n2_norm(r, n // gap, _zero_after(v, st.get(ch)))
                for _ in range(st["per"]):
                    k, k1 = divmod(st["ops"], 7)
                    if k < MD // 32 and n >= (2 * k + 1) * gap + lag:
                        n2_ops(k, k1, v, i)
                        st["ops"] += 1
            return hook

        def stage_c(i, r, half, rnext, extra):
            rr = pl.multiple_of(r, 8)
            ro = half * (HB // 2)
            cnt = [0]

            def hook(v):
                n = cnt[0]
                cnt[0] += 1
                if n < HB // 16:
                    gate(v, i)
                    shift_piece(rnext, 1 - half, n)
                extra(v)

            for j in range(4):
                c11, c12, c21, c22 = _strassen(lambda k: n7[k, ro:ro + HB // 2, :], wop(4 + j),
                                               hook)
                for c, y in ((j + 4, _merge_rows(c12, c22)), (j, _merge_rows(c11, c21))):
                    cs = slice(c * 128, (c + 1) * 128)
                    h2buf[pl.ds(rr, HB), cs] = h2buf[pl.ds(rr, HB), cs] + y

        def c_body(i, _):
            r = pl.multiple_of(i * MB, MB)
            st = {"n": 0, "ops": 0, "per": 1, "ch": 1}
            extra = n2_hook(0, i, 0, 4, 4, st)
            stage_c(i, r, 0, r + HB, extra)
            stage_c(i, r + HB, 1, jnp.minimum(i + 1, S // MB - 1) * MB, extra)
            assert st["ops"] == 28
            return 0
        _loop("c", 0, S // MB, c_body)

        def wop2(lo, n):
            return lambda k1, k: _unpack(w49[7 * k1 + k, lo:lo + n].reshape(8 * n, 128))

        def d_body(i, _):
            r = pl.multiple_of(i * MD, MD)
            rn = jnp.minimum(r + MD, S - MD)
            lhs = [d49[k] for k in range(49)]
            uops = []
            for t in range(7):
                cb = _strassen2(lambda k1, k: lhs[7 * k1 + k], wop2(t * 16, 16))
                uops.append(_a_operands2([[_gelu(c) for c in row] for row in cb]))
            ul = [[jnp.concatenate([u[k1][k] for u in uops], axis=1).astype(bf16)
                   for k in range(7)] for k1 in range(7)]
            st = {"n": 0, "ops": 0, "per": 1, "ch": DCH}
            hook = n2_hook(rn, i, DF, DG, DL, st)
            for t in range(2):
                cb = _strassen2(lambda k1, k: ul[k1][k], wop2(W4T + t * 56, 56), hook)
                for j in range(4):
                    y = jnp.concatenate([cb[q][j].reshape(MD // 32, 8, 128) for q in range(4)],
                                        axis=1).reshape(MD, 128)
                    c = 2 * j + t
                    cs = slice(c * 128, (c + 1) * 128)
                    gb = modrows(5, MD, c * 128, (c + 1) * 128)
                    o = xbuf[pl.ds(r, MD), cs].astype(f32) + gb * (h2buf[pl.ds(r, MD), cs] + y)
                    xbuf[pl.ds(r, MD), cs] = o.astype(bf16)
            assert st["ops"] == 28
            out_copy(r, MD).start()
            return 0
        _loop("d", 0, S // MD, d_body)

    pl.run_scoped(main,
                  pltpu.VMEM((7, 8 * 32, 8, 128), u32),
                  pltpu.VMEM((49, 2 * W4T, 8, 128), u32))

    out_copy(0, S).wait()


def _run(x, mem0, wq, wk, wv, wo, w1, w2, w3, w4, c, wmod):
    any_spec = pl.BlockSpec(memory_space=pl.ANY)
    return pl.pallas_call(
        _kernel,
        out_shape=jax.ShapeDtypeStruct((S, D), bf16),
        in_specs=[any_spec] * 12,
        out_specs=any_spec,
        scratch_shapes=[
            pltpu.VMEM((S + 2 * RIDE, D), bf16),
            pltpu.VMEM((NGRP + 4, 8 * WP, 128), u32),
            [pltpu.VMEM((NR // 16, 96 // NRING, 8, 128), u32)] * NRING,
            pltpu.VMEM((8, 16, 128), u32),
            pltpu.VMEM((H, 16, 128), u32),
            pltpu.VMEM((2 * H, 8, 128), u32),
            pltpu.VMEM((12, 8, 512), f32),
            pltpu.VMEM((D, 128), f32),
            pltpu.VMEM((S, D), f32),
            pltpu.VMEM((7, (S - NPRE) // 2, 512), bf16),
            pltpu.VMEM((17, 64, 128), bf16),
            pltpu.VMEM((8, 32, D), bf16),
            pltpu.VMEM((7, 64, 512), bf16),
            pltpu.VMEM((2, 7, NPRE // 2, 256), bf16),
            pltpu.VMEM((49, MD // 4, 256), bf16),
            [pltpu.VMEM((40, D), f32)] * (MD // 32),
            pltpu.VMEM((1, D), bf16),
            pltpu.SemaphoreType.DMA((9 + NGRP + 2,)),
        ],
        compiler_params=pltpu.CompilerParams(vmem_limit_bytes=124 * 1024 * 1024,
                                             disable_bounds_checks=True,
                                             disable_semaphore_checks=True),
    )(x, mem0, wq, wk, wv, wo, w1, w2, w3, w4, c, wmod)


def pallas_adaLN_cond__memory_aug_recurrent_mem_tr__mixer_s_mlp__prompt_kernel(
    A_x, A_mem0, A_Wq, A_Wk, A_Wv, A_Wo, A_seg_len, B_x, B_w1, B_w2, B_w3, B_w4, c, w_mod,
):
    del B_x
    assert A_x.shape == (1, S, D) and A_mem0.shape == (1, MEM, D)
    assert not isinstance(A_seg_len, int) or A_seg_len == SEG
    out = _run(A_x.reshape(S, D), A_mem0.reshape(MEM, D), A_Wq, A_Wk, A_Wv,
               A_Wo.reshape(H * DH, D),
               B_w1.reshape(2, D // 2, D), B_w2.reshape(2, D // 2, D),
               B_w3, B_w4.reshape(4, F // 4, D), c, w_mod)
    return out.reshape(1, S, D)
```

```python
import jax
import jax.numpy as jnp
from jax import lax
import jax.experimental.pallas as pl
import jax.experimental.pallas.tpu as pltpu

bf16 = jnp.bfloat16
f32 = jnp.float32
u32 = jnp.uint32

S = 2048
D = 1024
H = 32
DH = 128
F = 3584
MEM = 8
SEG = 32
NSEG = S // SEG
L = MEM + SEG
RIDE = 24
NPRE = S - RIDE * NSEG
NR = NPRE + 2 * SEG
ROFF = (-(S - NPRE)) % NR
WP = 516
NGRP = 12
NSLOT = 6
NMOD = 6
EPS = 1e-5
MD = 128
MB = 512
GPAD = 8
NRING = 8
NWO = 3
X0 = NPRE + 2 * RIDE
W4T = 7 * 16

RLP, WLP, RSK = 27, 22, 2
SAT = {i: max(6 * (i // 2) + 11, 17) for i in range(32)}
PVAT = {i: min(6 * (i // 2) + 23, 107) for i in range(32)}
KSPLIT = 2
PIN = 6
SLOTS = ([(0, -1, 0)] * 8 + [(0, n // 2, 3 * (n % 2)) for n in range(24)]
         + [(0, 96 + n, 0) for n in range(32)])
WPP, BG, BCH = 5, 2, 2
DF, DG, DL, DCH = 52, 3, 7, 2
_ONLY = None


def _loop(name, lo, hi, body, init=0):
    if _ONLY is not None and name not in _ONLY:
        return init
    with _scope(name):
        return lax.fori_loop(lo, hi, body, init)


class _NoScope:
    def __init__(self, name):
        del name

    def __enter__(self):
        return self

    def __exit__(self, *a):
        return False


_scope = _NoScope


def _zero_after(*vs):
    bits = None
    for v in vs:
        if v is not None:
            b = pltpu.bitcast(v[0:8, 0:128], u32)
            bits = b if bits is None else bits | b
    return pltpu.bitcast((bits >> 31) >> 1, f32)


def _ln(x, anchor=None):
    if anchor is not None:
        z = jnp.concatenate([anchor] * (x.shape[0] // 8), axis=0)
        x = jnp.concatenate([x[:, 0:128] + z, x[:, 128:]], axis=1)
    mu = jnp.mean(x, axis=-1, keepdims=True)
    xc = x - mu
    var = jnp.mean(xc * xc, axis=-1, keepdims=True)
    return xc * lax.rsqrt(var + EPS)


def _gelu(x):
    inner = x * (0.7978845608028654 + (0.7978845608028654 * 0.044715) * (x * x))
    hx = 0.5 * x
    return hx + hx * jnp.tanh(inner)


def _split_rows(x):
    m, n = x.shape
    x3 = x.reshape(m // 16, 16, n)
    return x3[:, 0:8, :].reshape(m // 2, n), x3[:, 8:16, :].reshape(m // 2, n)


def _merge_rows(top, bot):
    m, n = top.shape
    return jnp.concatenate([top.reshape(m // 8, 8, n), bot.reshape(m // 8, 8, n)],
                           axis=1).reshape(2 * m, n)


def _a_operands(a11, a12, a21, a22):
    return [a11 + a22, a21 + a22, a11, a22, a11 + a12, a21 - a11, a12 - a22]


def _b_operands(b11, b12, b21, b22):
    return [b11 + b22, b11, b12 - b22, b21 - b11, b22, b11 + b12, b21 + b22]


_ATERMS = ((0, 3, 1), (2, 3, 1), (0, None, 0), (3, None, 0), (0, 1, 1), (2, 0, -1), (1, 3, -1))
_BTERMS = ((0, 3, 1), (0, None, 0), (1, 3, -1), (2, 0, -1), (3, None, 0), (0, 1, 1), (2, 3, 1))


def _strassen(a_of, b_of, hook=lambda v: None):
    def prod(k):
        return jnp.dot(a_of(k), b_of(k), preferred_element_type=f32)
    p5 = prod(4)
    hook(p5)
    p3 = prod(2)
    hook(p3)
    c12 = p3 + p5
    p4 = prod(3)
    hook(p4)
    c11 = p4 - p5
    p2 = prod(1)
    hook(p2)
    c21 = p2 + p4
    c22 = p3 - p2
    p1 = prod(0)
    hook(p1)
    c11 = prod(6) + (c11 + p1)
    hook(c11)
    c22 = prod(5) + (c22 + p1)
    hook(c22)
    return c11, c12, c21, c22


def _a_operands2(b):
    sub = [_a_operands(b[i][j], b[i][2 + j], b[2 + i][j], b[2 + i][2 + j])
           for i in range(2) for j in range(2)]
    return [_a_operands(*[t[k] for t in sub]) for k in range(7)]


def _strassen2(a_of, b_of, hook=lambda v: None):
    def prod(k1):
        return _strassen(lambda k: a_of(k1, k), lambda k: b_of(k1, k), hook)

    def add(x, y):
        return [p + q for p, q in zip(x, y)]

    def sub(x, y):
        return [p - q for p, q in zip(x, y)]
    p5 = prod(4)
    p3 = prod(2)
    c12 = add(p3, p5)
    p4 = prod(3)
    c11 = sub(p4, p5)
    p2 = prod(1)
    c21 = add(p2, p4)
    c22 = sub(p3, p2)
    p1 = prod(0)
    c11 = add(add(c11, p1), prod(6))
    c22 = add(add(c22, p1), prod(5))
    cq = (c11, c12, c21, c22)
    return [[cq[2 * (i // 2) + j // 2][2 * (i % 2) + j % 2] for j in range(4)] for i in range(4)]


def _pack8(v):
    return pltpu.bitcast(v.astype(bf16), u32)


def _unpack(w):
    return pltpu.bitcast(w, bf16)


def _kernel(x_hbm, mem0_hbm, wq_hbm, wk_hbm, wv_hbm, wo_hbm, w1_hbm, w2_hbm, w3_hbm, w4_hbm,
            c_hbm, wmod_hbm, out_hbm,
            xbuf, wqkv, rings, lhs_h, lhs_o, kvm, modv, scol, h2buf, n7, ws3, wsr, t7, a7, d49,
            nrms, c_ref, sems):
    w_hbms = (wq_hbm, wk_hbm, wv_hbm)
    SMOD, SSTG = 5, 9
    sem_x, sem_out, sem_w, sem_g, sem_r = (sems.at[k] for k in range(5))

    def rget(b, tile, n):
        return jnp.concatenate([rings[b % NRING][tile + e, b // NRING] for e in range(n)], axis=0)

    def rhalf(b, tile, half):
        return rings[b % NRING][tile, b // NRING, 4 * half:4 * half + 4, :]

    def rset(b, tile, half, val):
        rings[b % NRING][tile, b // NRING, 4 * half:4 * half + 4, :] = _pack8(val)

    x_copy = pltpu.make_async_copy(x_hbm.at[pl.ds(0, X0), :], xbuf.at[pl.ds(0, X0), :], sem_x)

    def stream_copies(c):
        al, lo = ((lambda v, m: v), min) if isinstance(c, int) else (pl.multiple_of, jnp.minimum)
        c3 = lo(c, 27)
        cps = [pltpu.make_async_copy(
            w3_hbm.at[pl.ds(al(i * 256 + (c3 % 4) * 64, 64), 64),
                      pl.ds(al(j * (F // 4) + (c3 // 4) * 128, 128), 128)],
            ws3.at[4 * i + j], sem_w) for i in range(4) for j in range(4)]
        dst = X0 + 2 * RIDE * c
        return [
            pltpu.make_async_copy(w4_hbm.at[:, pl.ds(al(c3 * 32, 32), 32), :],
                                  wsr.at[pl.ds(0, 4)], sem_g),
            pltpu.make_async_copy(w1_hbm.at[:, pl.ds(al(c * 16, 16), 16), :],
                                  wsr.at[pl.ds(4, 2), pl.ds(0, 16), :], sem_g),
            pltpu.make_async_copy(w2_hbm.at[:, pl.ds(al(c * 16, 16), 16), :],
                                  wsr.at[pl.ds(4, 2), pl.ds(16, 16), :], sem_g),
            pltpu.make_async_copy(wmod_hbm.at[pl.ds(al(c * 32, 32), 32), pl.ds(5 * D, D)],
                                  wsr.at[6], sem_g),
            pltpu.make_async_copy(x_hbm.at[pl.ds(al(lo(dst, S - 2 * RIDE), 16), 2 * RIDE), :],
                                  xbuf.at[pl.ds(al(dst, 16), 2 * RIDE), :], sem_r)] + cps

    def stream_wait(c):
        for dst, sem in ((ws3.at[pl.ds(0, 16)], sem_w), (wsr.at[pl.ds(0, 7)], sem_g),
                         (xbuf.at[pl.ds(X0 + 2 * RIDE * c, 2 * RIDE), :], sem_r)):
            pltpu.make_async_copy(dst, dst, sem).wait()

    def out_copy(row, n):
        return pltpu.make_async_copy(xbuf.at[pl.ds(row, n), :], out_hbm.at[pl.ds(row, n), :],
                                     sem_out)

    def mod_rows(acc, w, r):
        sc = jnp.concatenate([scol[pl.ds(r, 16), :]] * (w.shape[1] // 128), axis=1)
        p = w.astype(f32) * sc
        return acc + p[0:8] + p[8:16]

    def mod_finish(acc, j):
        is_scale = jnp.logical_or(j // 2 == 1, j // 2 == 4)
        tot = jnp.sum(acc, axis=0, keepdims=True) + jnp.where(is_scale, 1.0, 0.0)
        modv[j] = jnp.broadcast_to(tot, (8, 512))

    def modrows(k, n, lo=0, hi=D):
        m = jnp.concatenate([modv[2 * k], modv[2 * k + 1]], axis=1)[:, lo:hi]
        return jnp.concatenate([m] * (n // 8), axis=0)

    def adaln_a(xv, anchor=None):
        n = xv.shape[0]
        return _ln(xv, anchor) * modrows(1, n) + modrows(0, n)

    def adaln_b(xv, anchor=None):
        n = xv.shape[0]
        return _ln(xv, anchor) * modrows(4, n) + modrows(3, n)

    def set_lhs(mem, hn):
        v = jnp.concatenate([mem, hn], axis=0)
        for c in range(8):
            for e in range(4):
                lhs_h[c, 4 * e:4 * e + 4, :] = _pack8(v[8 * e:8 * e + 8, c * 128:(c + 1) * 128])

    def row_operands(v):
        top, bot = _split_rows(v)
        k = v.shape[1] // 2
        return _a_operands(top[:, :k], top[:, k:], bot[:, :k], bot[:, k:])

    def stage_a16(r, anchor=None, dst=None):
        rr = pl.multiple_of(r, 16)
        xv = xbuf[pl.ds(rr, 16), :]
        if dst is not None:
            xv = (xv.astype(f32) + modrows(2, 16) * h2buf[pl.ds(rr, 16), :]).astype(bf16)
            xbuf[pl.ds(rr, 16), :] = xv
        h2 = adaln_b(xv.astype(f32), anchor)
        h2buf[pl.ds(rr, 16), :] = h2
        ref, ro = (n7, pl.multiple_of(rr // 2, 8)) if dst is None else dst
        ops = row_operands(_ln(h2))
        for t, op in enumerate(ops):
            ref[t, pl.ds(ro, 8), :] = op.astype(bf16)
        return ops[0]

    def prologue(stg, wos, wmodb, h7):
        def mod_copy(j):
            return pltpu.make_async_copy(wmod_hbm.at[:, pl.ds(j * 512, 512)], wmodb.at[j % NMOD],
                                         sems.at[SSTG + j + 4 if j >= 4 else SMOD + j])

        def piece_copy(g, dh):
            return pltpu.make_async_copy(
                w_hbms[g // 4].at[pl.ds(dh * 512, 512), pl.ds((g % 4) * 8, 8), :],
                stg.at[(2 * g + dh) % NSLOT], sems.at[SSTG + (g + 1 if g else dh)])

        def wo_copy(j):
            return pltpu.make_async_copy(wo_hbm.at[pl.ds(j * 512, 512), :], wos.at[j % NWO],
                                         sems.at[SSTG + j + 6])

        def group_start(g):
            for dh in range(2):
                piece_copy(g, dh).start()

        def stg_wait(slot, n, sem):
            dst = stg.at[pl.ds(slot, n)]
            pltpu.make_async_copy(dst, dst, sems.at[SSTG + sem]).wait()

        def relayout(g, slot, dh, lo_dp, n_dp):
            for u in range(n_dp):
                dp = lo_dp + u
                ev = pltpu.bitcast(stg[slot, 2 * dp].astype(f32), u32)
                od = pltpu.bitcast(stg[slot, 2 * dp + 1].astype(f32), u32)
                wqkv[g, pl.ds(dh * 256 + dp, 8, stride=WP), :] = (ev >> 16) | od

        def b_operand(g, q, k):
            def quad(i):
                r = (q + 4 * (i % 2)) * WP + (i // 2) * 256
                return _unpack(wqkv[g, r:r + 256, :])
            i, j, sign = _BTERMS[k]
            if j is None:
                return quad(i)
            u, v = quad(i).astype(f32), quad(j).astype(f32)
            return (u + v if sign > 0 else u - v).astype(bf16)

        c_copy = pltpu.make_async_copy(c_hbm, c_ref, sem_g)
        m_copy = pltpu.make_async_copy(mem0_hbm, wsr.at[7, pl.ds(0, MEM), :], sem_r)
        c_copy.start()
        m_copy.start()
        x_copy.start()
        for j in range(4):
            mod_copy(j).start()
        for g in range(3):
            group_start(g)
        h2buf[S - NPRE:S, :] = jnp.zeros((NPRE, D), f32)
        wos[2] = jnp.zeros((512, D), bf16)
        c_copy.wait()
        m_copy.wait()
        cv = c_ref[...].astype(f32)
        sv = jnp.broadcast_to(cv * (1.0 / (1.0 + jnp.exp(-cv))), (128, D))
        for k in range(8):
            scol[k * 128:(k + 1) * 128, :] = sv[:, k * 128:(k + 1) * 128].T
        x_copy.wait()

        def ln0_body(i, _):
            r = pl.multiple_of(i * 64, 64)
            h2buf[pl.ds(r, 64), :] = _ln(xbuf[pl.ds(r, 64), :].astype(f32))
            return 0
        lax.fori_loop(0, NPRE // 64, ln0_body, 0)

        def mod0_body(j, _):
            pltpu.make_async_copy(wmodb.at[j], wmodb.at[j], sems.at[SMOD + j]).wait()
            accs = [jnp.zeros((8, 512), f32)] * 2
            for k in range(64):
                accs[k % 2] = mod_rows(accs[k % 2], wmodb[j, k * 16:(k + 1) * 16, :], k * 16)
            mod_finish(accs[0] + accs[1], j)
            return 0
        _loop("mod0", 0, 4, mod0_body)

        def hpre_body(i, _):
            r = pl.multiple_of(i * 32, 32)
            hv = h2buf[pl.ds(r, 32), :] * modrows(1, 32) + modrows(0, 32)
            ro = pl.multiple_of(i * 8, 8)
            for t, op in enumerate(row_operands(hv)):
                h7[t, pl.ds(ro, 8), :] = pltpu.bitcast(op.astype(bf16), u32)
            return 0
        lax.fori_loop(0, NPRE // 32, hpre_body, 0)
        set_lhs(wsr[7, 0:MEM, :].astype(f32), adaln_a(xbuf[NPRE:NPRE + RIDE, :].astype(f32)))

        def relayout_now(g, dh):
            def rl_body(t, _):
                relayout(g, 2 * g + dh, dh, t * 32, 32)
                return 0
            lax.fori_loop(0, 8, rl_body, 0)

        for dh in range(2):
            stg_wait(dh, 1, dh)
            relayout_now(0, dh)

        grp = lambda g: [piece_copy(g, 0), piece_copy(g, 1)]
        issue = {0: [wo_copy(0)], 1: grp(3) + grp(4), 2: grp(5) + [wo_copy(1), mod_copy(4)],
                 3: grp(6) + [mod_copy(5), mod_copy(6)], 4: grp(7) + [wo_copy(2)],
                 5: grp(8) + [wo_copy(3), mod_copy(7)], 6: grp(9) + [wo_copy(4)],
                 7: grp(10) + [wo_copy(5), mod_copy(8)], 8: grp(11) + [wo_copy(6)],
                 9: [wo_copy(7), mod_copy(9)], 10: stream_copies(0)}

        def pre_iter(g, m3):

            @pl.when(g == 1)
            def _():
                stg_wait(2, 2, 2)
                relayout_now(1, 0)
                relayout_now(1, 1)

            def slots():
                m3n = jnp.where(m3 == 2, 0, m3 + 1)
                cj = jnp.maximum(g - 2, 3)
                return (m3n, 2 * jnp.where(ends, m3, m3n),
                        jnp.where(jnp.logical_or(g < 4, m3 == 0), 2, m3 - 1),
                        cj, jnp.where(cj >= NMOD, cj - NMOD, cj))

            ends = jnp.logical_or(g == 0, g == NGRP - 1)

            @pl.when(jnp.logical_not(ends))
            def _():
                stg_wait(slots()[1], 2, g + 2)

            @pl.when(g >= 4)
            def _():
                buf = wos.at[slots()[2]]
                pltpu.make_async_copy(buf, buf, sems.at[SSTG + g + 2]).wait()

            @pl.when(g >= 6)
            def _():
                buf = wmodb.at[slots()[4]]
                pltpu.make_async_copy(buf, buf, sems.at[SSTG + g + 2]).wait()

            m3n, gslot, wslot, cj, cslot = slots()
            gn = jnp.where(ends, g, g + 1)
            wj = jnp.maximum(g - 4, 0)
            wgrp, wrow = NGRP + wj // 2, (wj % 2) * 256
            for k, cps in issue.items():
                @pl.when(g == k)
                def _():
                    for cp in cps:
                        cp.start()
            wtodo = [(r, c) for r in range(16) for c in range(8)]
            todo = [(dh, dp) for dh in range(2) for dp in range(256)]
            skip = [0] * RSK
            mtodo = list(range(0, D, 16))
            macc = [jnp.zeros((8, 512), f32)]

            def hook(v):
                if mtodo:
                    acc = macc[0] + jnp.concatenate([_zero_after(v)] * 4, axis=1)
                    for r in mtodo[:3]:
                        acc = mod_rows(acc, wmodb[cslot, r:r + 16, :], r)
                    del mtodo[:3]
                    macc[0] = acc

            for q in range(4):
                def b_of(k):
                    w = b_operand(g, q, k)
                    if skip:
                        skip.pop()
                        return w
                    nw = 0 if todo else WLP
                    for dh, dp in todo[:RLP]:
                        relayout(gn, gslot + dh, dh, dp, 1)
                    del todo[:RLP]
                    for r, c in wtodo[:nw]:
                        wqkv[wgrp, pl.ds(wrow + (c * 512 + r * 16), 16), :] = pltpu.bitcast(
                            wos[wslot, r * 32:(r + 1) * 32, c * 128:(c + 1) * 128], u32)
                    del wtodo[:nw]
                    return w
                c11, c12, c21, c22 = _strassen(lambda k: pltpu.bitcast(h7[k], bf16), b_of, hook)
                for blk, y in ((q + 4, _merge_rows(c12, c22)), (q, _merge_rows(c11, c21))):
                    for e in range(NPRE // 8):
                        tile, half = divmod(((8 * e + ROFF) % NR) // 8, 2)
                        rings[blk][tile, g, 4 * half:4 * half + 4, :] = _pack8(y[8 * e:8 * e + 8])
            assert not todo and not wtodo and not mtodo
            mod_finish(macc[0], cj)
            return m3n

        _loop("pre1", 0, NGRP, pre_iter)

    pl.run_scoped(prologue,
                  pltpu.VMEM((NSLOT, 512, 8, 128), bf16),
                  pltpu.VMEM((NWO, 512, D), bf16),
                  pltpu.VMEM((NMOD, D, 512), bf16),
                  pltpu.VMEM((7, NPRE // 4, 512), u32))

    def main(w7, w49):
        scale = DH ** -0.5
        ia = lax.broadcasted_iota(jnp.int32, (32, L), 0)
        ja = lax.broadcasted_iota(jnp.int32, (32, L), 1)
        mask_a = (((ia >= 16) & (ia < 24)) | (ja >= SEG)
                  | (jnp.where(ia < 16, ia + 16, ia - 16) >= ja))
        ib = lax.broadcasted_iota(jnp.int32, (48, 56), 0)
        jb = lax.broadcasted_iota(jnp.int32, (48, 56), 1)
        own = (ib < 40) == (jb < 40)
        mask_b = own & (((jb >= 32) & (jb < 48)) | (jnp.where(jb < 40, jb, jb - 8) <= ib))
        masked = -1e9 / scale
        j8 = lax.broadcasted_iota(jnp.int32, (8, 56), 1)
        fill_b = jnp.concatenate([jnp.where(j8 < 40, masked, -3e38).astype(f32)] * 5
                                 + [jnp.where(j8 < 40, -3e38, masked).astype(f32)], axis=0)

        def softmax(sc, mask, fill):
            sc = jnp.where(mask, sc, fill)
            mx = jnp.max(sc, axis=-1, keepdims=True)
            e = jnp.exp2((sc - mx) * (scale * 1.4426950408889634))
            den = jnp.sum(e, axis=-1, keepdims=True)
            return (e * pl.reciprocal(den, approx=True)).astype(bf16)

        def ride_tiles(it, is_b):
            first = (it == 0).astype(jnp.int32)
            if is_b:
                return 3 * it + 1 - first, 0, 3 * it + 2
            return 3 * it + 1 - first, 1, 3 * it + first

        def step(it, is_b, lhs_lo, lhs_hi, jobs, pins):
            NT, TOFF = NR // 16, ROFF // 16
            sega = (4 * it + TOFF) % NT
            seg = sega + 2 if is_b else sega
            wt = [(3 * it + (NPRE // 16 + TOFF + t + is_b)) % NT for t in range(2)]
            wr = [(wt[(t + is_b) // 2], (t + is_b) % 2) for t in range(3)]
            rt, rh, rf = ride_tiles(it, is_b)
            rt, rf = (rt + TOFF) % NT, (rf + TOFF) % NT
            lhs = jnp.concatenate([lhs_lo, lhs_hi], axis=1)
            QM, P, PART = {}, {}, {}
            mrow = 0 if is_b else 4

            def wblk(b, lo, n):
                r = (b % 8) * WP + lo
                return _unpack(wqkv[b // 8, r:r + n, :])

            def qkv_lo(i):
                for m in range(3):
                    PART[(m, i)] = jnp.dot(lhs_lo, wblk(m * H + i, 0, 256), preferred_element_type=f32)

            def qkv(i):
                for m in range(3):
                    b = m * H + i
                    if (m, i) in PART:
                        y = jnp.dot(lhs_hi, wblk(b, 256, 256),
                                    preferred_element_type=f32) + PART.pop((m, i))
                    else:
                        y = jnp.dot(lhs, wblk(b, 0, 512), preferred_element_type=f32)
                    if m < 2:
                        QM[b] = y[0:MEM] + pins[b] if b in pins else y[0:MEM]
                    if m == 2 or (m == 1 and not is_b):
                        kvm[b - H, mrow:mrow + 4, :] = _pack8(y[0:MEM])
                    for t in range(3):
                        rset(b, *wr[t], y[8 + 8 * t:16 + 8 * t])
                    for job in jobs.get(3 * i + m, []):
                        job(y)
                    side(3 * i + m)

            def keys(b):
                if is_b:
                    if b in QM:
                        mix = jnp.concatenate([_pack8(QM.pop(b)), kvm[b - H, 4:8, :]], axis=0)
                    else:
                        mix = kvm[b - H]
                    return _unpack(jnp.concatenate([rget(b, seg, 2), mix, rhalf(b, sega, 0)], axis=0))
                mk = _pack8(QM.pop(b)) if b in QM else kvm[b - H, 4:8, :]
                return _unpack(jnp.concatenate([rget(b, seg, 2), mk], axis=0))

            def scores(i):
                if is_b:
                    q = [rget(i, seg, 2), _pack8(QM.pop(i)), rhalf(i, sega, 0)]
                else:
                    q = [rget(i, seg + 1, 1), _pack8(QM.pop(i)), rhalf(i, seg, 1)]
                sc = lax.dot_general(_unpack(jnp.concatenate(q, axis=0)), keys(H + i),
                                     (((1,), (1,)), ((), ())), preferred_element_type=f32)
                P[i] = softmax(sc, mask_b, fill_b) if is_b else softmax(sc, mask_a, masked)

            def pv(i):
                o = jnp.dot(P.pop(i), keys(2 * H + i), preferred_element_type=f32)
                if is_b:
                    for e in range(4):
                        rset(i, seg + e // 2, e % 2, o[8 * e:8 * e + 8])
                    rset(i, sega, 0, o[40:48])
                    lhs_o[i, 0:4, :] = _pack8(o[SEG:L])
                else:
                    for e in range(2):
                        rset(i, seg + 1, e, o[8 * e:8 * e + 8])
                    rset(i, seg, 1, o[24:32])
                    lhs_o[i, 0:4, :] = _pack8(o[16:24])
                lhs_o[i, 4:8, :] = rhalf(i, rt, rh)
                lhs_o[i, 8:16, :] = rget(i, rf, 1)

            def wo_lhs(i0, i1):
                return _unpack(jnp.concatenate([lhs_o[i] for i in range(i0, i1)], axis=1))

            def wo_dot(lo, j, k):
                w = _unpack(wqkv[NGRP + k, j * 512:(j + 1) * 512, :])
                return jnp.dot(lo, w, preferred_element_type=f32)

            def side(d):
                for i in range(H):
                    if PVAT[i] == d:
                        pv(i)
                for i in range(H):
                    if SAT[i] == d:
                        scores(i)

            if is_b:
                for h in range(KSPLIT):
                    qkv_lo(h)
            for h in range(H):
                qkv(h)
            lo = [wo_lhs(8 * k, 8 * k + 8) for k in range(3)]
            acc = []
            for j in range(8):
                y = None
                for k in range(3):
                    z = wo_dot(lo[k], j, k)
                    y = z if y is None else z + y
                    for job in jobs.get(96 + 3 * j + k, []):
                        job(y)
                    side(96 + 3 * j + k)
                acc.append(y)
            lo = wo_lhs(24, H)
            for j in range(8):
                acc[j] = wo_dot(lo, j, 3) + acc[j]
                for job in jobs.get(120 + j, []):
                    job(acc[j])
            assert not (QM or P or PART)
            return jnp.concatenate(acc[0:4], axis=1), jnp.concatenate(acc[4:8], axis=1)

        def combine(c, n, y):
            mp, k1 = divmod(n, 8)
            m, p = divmod(mp, 4)
            c3 = jnp.minimum(c, 27)
            spare = pl.ds(pl.multiple_of(8 * (c // 64), 8), 8)
            if y is None:
                pass
            elif m == 0 and k1 < 7:
                ws3[16, spare, :] = y.astype(bf16)
            else:
                wsr[7, spare, 0:128] = y.astype(bf16)
            if k1 == 7:
                dst, base, r = w7, 0, (4 * m + p) * 32 + c
                blk = [wsr[4 + i, m * 16:(m + 1) * 16, j * 512 + p * 128:j * 512 + (p + 1) * 128]
                       .astype(f32) for i in range(2) for j in range(2)]
            else:
                dst, base = w49, 7 * k1
                if m == 0:
                    r = c3 * 4 + p
                    get = lambda i, j: ws3[4 * i + j, p * 16:(p + 1) * 16, :]
                else:
                    r = W4T + (p // 2) * 56 + c3 * 2 + p % 2
                    r0, c0 = (p % 2) * 16, (p // 2) * 128
                    get = lambda i, j: wsr[i, r0:r0 + 16, j * 256 + c0:j * 256 + c0 + 128]

                def quad(q):
                    return [get(2 * (q // 2) + i, 2 * (q % 2) + j).astype(f32)
                            for i in range(2) for j in range(2)]
                qi, qj, sign = _BTERMS[k1]
                blk = quad(qi)
                if qj is not None:
                    blk = [u + v if sign > 0 else u - v for u, v in zip(blk, quad(qj))]
            for k, op in enumerate(_b_operands(*blk)):
                for e in range(2):
                    dst[base + k, r, 4 * e:4 * e + 4, :] = _pack8(op[8 * e:8 * e + 8])

        def rec_body(it, gacc):
            stream_wait(it)
            lhs_lo = _unpack(jnp.concatenate([lhs_h[c] for c in range(4)], axis=1))
            lhs_hi = _unpack(jnp.concatenate([lhs_h[c] for c in range(4, 8)], axis=1))
            ra = jnp.maximum(it - 1, 0) * (2 * RIDE)
            for u in range(2):
                s = 2 * it + u
                jobs, pins = {}, {}
                for n, (su, d, g) in enumerate(SLOTS):
                    if su == u and d < 0:
                        combine(it, n, None)
                    elif su == u:
                        jobs.setdefault(d, []).append(
                            lambda y, n=n, g=g: combine(it, n, y[8 * g:8 * g + 8]))
                r1 = pl.multiple_of(jnp.minimum(NPRE + RIDE * (s + 1), S - RIDE), 8)
                xn = xbuf[pl.ds(r1, RIDE), :].astype(f32)
                if u == 0:
                    for k in range(2):
                        rm = pl.multiple_of(it * 32 + k * 16, 16)
                        gacc = mod_rows(gacc, wsr[6, k * 16:(k + 1) * 16, :], rm)
                    hn = adaln_a(xn, _zero_after(stage_a16(ra)))
                else:
                    def refill(y):
                        for cp in stream_copies(jnp.minimum(it + 1, NSEG // 2 - 1)):
                            cp.start()
                        spare = pl.ds(pl.multiple_of(8 * (it // 64), 8), 8)
                        pins[PIN] = _zero_after(ws3[16, spare, :].astype(f32))
                    jobs.setdefault(3 * (PIN - 4) + 2, []).append(refill)
                    hn = adaln_a(xn)
                    z = _zero_after(hn[0:8], hn[8:16], hn[16:24])
                    stage_a16(ra + 32, _zero_after(stage_a16(ra + 16, z)))
                a_lo, a_hi = step(it, u, lhs_lo, lhs_hi, jobs, pins)
                a = jnp.concatenate([a_lo, a_hi], axis=1)
                if u == 0:
                    lhs_lo = jnp.concatenate([a_lo[0:MEM], hn[:, 0:512]], axis=0).astype(bf16)
                    lhs_hi = jnp.concatenate([a_hi[0:MEM], hn[:, 512:1024]], axis=0).astype(bf16)
                else:
                    set_lhs(a[0:MEM], hn)
                rt, rh, rf = ride_tiles(it, u)
                rows = [pl.ds(pl.multiple_of(16 * rt + 8 * rh, 8), 8),
                        pl.ds(pl.multiple_of(16 * rf, 16), 16)]
                xs = [xbuf[r, :].astype(f32) for r in rows]
                xbuf[rows[0], :] = (xs[0] + modrows(2, 8) * a[8:16]).astype(bf16)
                xbuf[rows[1], :] = (xs[1] + modrows(2, 16) * a[16:32]).astype(bf16)
            return gacc

        gacc = _loop("rec", 0, NSEG // 2, rec_body, jnp.zeros((8, D), f32))
        for c in range(2):
            mod_finish(gacc[:, c * 512:(c + 1) * 512], 10 + c)
        stream_wait(NSEG // 2 - 1)

        def wo_prep(i, half, k):
            o = jnp.concatenate([_unpack(rings[4 * half + h][k, i]).astype(f32)
                                 for h in range(4)], axis=1)
            for t, op in enumerate(row_operands(o)):
                a7[half, t, k * 8:(k + 1) * 8, :] = op.astype(bf16)

        def wo_chunk(i, half, inext, extra):
            todo = list(range(NPRE // 16))

            def hook(v):
                if todo:
                    for h in range(4):
                        rings[4 * (1 - half) + h][i // 64, 4] = pltpu.bitcast(v[0:8], u32)
                    n = 2 if len(todo) % WPP == 0 else 1
                    for k in todo[:n]:
                        wo_prep(inext, 1 - half, k)
                    del todo[:n]
                extra(v)

            for j in range(4):
                def b_of(k):
                    def quad(q):
                        r = (j + 4 * (q % 2)) * 512 + half * 256 + (q // 2) * 128
                        return _unpack(wqkv[NGRP + i, r:r + 128, :])
                    qi, qj, sign = _BTERMS[k]
                    if qj is None:
                        return quad(qi)
                    u, v = quad(qi).astype(f32), quad(qj).astype(f32)
                    return (u + v if sign > 0 else u - v).astype(bf16)
                c11, c12, c21, c22 = _strassen(lambda k: a7[half, k], b_of, hook)
                for c, y in ((j + 4, _merge_rows(c12, c22)), (j, _merge_rows(c11, c21))):
                    cs = slice(c * 128, (c + 1) * 128)
                    h2buf[S - NPRE:S, cs] = h2buf[S - NPRE:S, cs] + y

        for k in range(NPRE // 16):
            wo_prep(0, 0, k)

        def wo_tail(i, _):
            st = {"n": 0, "prev": None}

            def extra(v):
                n = st["n"]
                st["n"] += 1
                if n % 16 == 2 and n // 16 < 3:
                    st["prev"] = stage_a16(S - NPRE - 48 + 16 * (n // 16),
                                           _zero_after(v, st["prev"]))
            wo_chunk(i, 0, i, extra)
            wo_chunk(i, 1, jnp.minimum(i + 1, 3), extra)
            return 0
        _loop("wotail", 0, 4, wo_tail)

        def gget(c, row, n):
            return pltpu.bitcast(wqkv[c, pl.ds(row, n), :], f32)

        def gset(c, row, val):
            wqkv[c, pl.ds(row, val.shape[0]), :] = pltpu.bitcast(val, u32)

        def wop(j):
            return lambda k: _unpack(w7[k, j * 32:(j + 1) * 32].reshape(256, 128))

        zpad = jnp.zeros((GPAD, 128), f32)
        for cb in range(8):
            gset(cb, 0, zpad)
            gset(cb, GPAD + S, zpad)

        shifts = (-1, -1, 1, 1, -2, -2, 2, 2)
        HB = MB // 2

        def shift_piece(r, half, k):
            gs = jnp.concatenate([gget(c, r + (k * 16 + GPAD + shifts[c]), 16)
                                  for c in range(8)], axis=1)
            ro = half * (HB // 2) + k * 8
            for t, op in enumerate(row_operands(gs)):
                n7[t, ro:ro + 8, :] = op.astype(bf16)

        def gate(v, i):
            gset(0, GPAD + S + GPAD + 8 * (i // S), v[0:8])

        def b_body(i, _):
            rl = S - NPRE + i * 128
            st = {"n": 0, "prev": [None, None]}

            def hook(v):
                n = st["n"]
                st["n"] += 1
                if n % BG == 0 and n // BG < 8:
                    k = n // BG
                    st["prev"][k % BCH] = stage_a16(rl + 16 * k,
                                                    _zero_after(v, st["prev"][k % BCH]),
                                                    (t7, 8 * k))

            ro = pl.multiple_of(i * 192, 64)
            for lhs, row in ((lambda k: n7[k, pl.ds(ro, 192), :], i * 384), (lambda k: t7[k], rl)):
                rg = pl.multiple_of(GPAD + row, 8)
                for j in range(4):
                    c11, c12, c21, c22 = _strassen(lhs, wop(j), hook)
                    gset(j + 4, rg, _gelu(_merge_rows(c12, c22)))
                    gset(j, rg, _gelu(_merge_rows(c11, c21)))
            return 0
        _loop("b", 0, S // MB, b_body)
        for k in range(HB // 16):
            shift_piece(0, 0, k)

        def n2_norm(r, k, anchor):
            v = _ln(h2buf[pl.ds(pl.multiple_of(r + k * 16, 16), 16), :], anchor)
            nrms[k // 2][(k % 2) * 16:(k % 2) * 16 + 16, :] = v
            return v[0:8] + v[8:16]

        def n2_ops(k, k1, v, i):
            nrm = nrms[k]
            nrm[pl.ds(pl.multiple_of(32 + 8 * (i // S), 8), 8), 0:128] = v[0:8]

            def quad(q):
                r0, c0 = (q // 2) * 16, (q % 2) * 512
                return [nrm[r0 + 8 * a:r0 + 8 * a + 8, c0 + 256 * b:c0 + 256 * b + 256]
                        for a in range(2) for b in range(2)]
            qi, qj, sign = _ATERMS[k1]
            blk = quad(qi)
            if qj is not None:
                blk = [u + w if sign > 0 else u - w for u, w in zip(blk, quad(qj))]
            for k2, op in enumerate(_a_operands(*blk)):
                d49[7 * k1 + k2, k * 8:(k + 1) * 8, :] = op.astype(bf16)

        def n2_hook(r, i, first, gap, lag, st):
            def hook(v):
                n = st["n"] - first
                st["n"] += 1
                if n >= 0 and n % gap == 0 and n // gap < MD // 16:
                    ch = (n // gap) % st["ch"]
                    st[ch] = n2_norm(r, n // gap, _zero_after(v, st.get(ch)))
                for _ in range(st["per"]):
                    k, k1 = divmod(st["ops"], 7)
                    if k < MD // 32 and n >= (2 * k + 1) * gap + lag:
                        n2_ops(k, k1, v, i)
                        st["ops"] += 1
            return hook

        def stage_c(i, r, half, rnext, extra):
            rr = pl.multiple_of(r, 8)
            ro = half * (HB // 2)
            cnt = [0]

            def hook(v):
                n = cnt[0]
                cnt[0] += 1
                if n < HB // 16:
                    gate(v, i)
                    shift_piece(rnext, 1 - half, n)
                extra(v)

            for j in range(4):
                c11, c12, c21, c22 = _strassen(lambda k: n7[k, ro:ro + HB // 2, :], wop(4 + j),
                                               hook)
                for c, y in ((j + 4, _merge_rows(c12, c22)), (j, _merge_rows(c11, c21))):
                    cs = slice(c * 128, (c + 1) * 128)
                    h2buf[pl.ds(rr, HB), cs] = h2buf[pl.ds(rr, HB), cs] + y

        def c_body(i, _):
            r = pl.multiple_of(i * MB, MB)
            st = {"n": 0, "ops": 0, "per": 1, "ch": 1}
            extra = n2_hook(0, i, 0, 4, 4, st)
            stage_c(i, r, 0, r + HB, extra)
            stage_c(i, r + HB, 1, jnp.minimum(i + 1, S // MB - 1) * MB, extra)
            assert st["ops"] == 28
            return 0
        _loop("c", 0, S // MB, c_body)

        def wop2(lo, n):
            return lambda k1, k: _unpack(w49[7 * k1 + k, lo:lo + n].reshape(8 * n, 128))

        def d_body(i, _):
            r = pl.multiple_of(i * MD, MD)
            rn = jnp.minimum(r + MD, S - MD)
            lhs = [d49[k] for k in range(49)]
            for t in range(7):
                cb = _strassen2(lambda k1, k: lhs[7 * k1 + k], wop2(t * 16, 16))
                ops = _a_operands2([[_gelu(c) for c in row] for row in cb])
                for n in range(49):
                    for e in range(4):
                        r0 = (n % 32) * 112 + t * 16 + 4 * e
                        wqkv[8 + n // 32, r0:r0 + 4, :] = _pack8(ops[n // 7][n % 7][8 * e:8 * e + 8])

            def ul(k1, k):
                n = 7 * k1 + k
                r0 = (n % 32) * 112
                return _unpack(jnp.concatenate(
                    [wqkv[8 + n // 32, r0 + 16 * t:r0 + 16 * t + 16, :] for t in range(7)], axis=1))
            st = {"n": 0, "ops": 0, "per": 1, "ch": DCH}
            hook = n2_hook(rn, i, DF, DG, DL, st)
            for t in range(2):
                cb = _strassen2(ul, wop2(W4T + t * 56, 56), hook)
                for j in range(4):
                    y = jnp.concatenate([cb[q][j].reshape(MD // 32, 8, 128) for q in range(4)],
                                        axis=1).reshape(MD, 128)
                    c = 2 * j + t
                    cs = slice(c * 128, (c + 1) * 128)
                    gb = modrows(5, MD, c * 128, (c + 1) * 128)
                    o = xbuf[pl.ds(r, MD), cs].astype(f32) + gb * (h2buf[pl.ds(r, MD), cs] + y)
                    xbuf[pl.ds(r, MD), cs] = o.astype(bf16)
            assert st["ops"] == 28
            out_copy(r, MD).start()
            return 0
        _loop("d", 0, S // MD, d_body)

    pl.run_scoped(main,
                  pltpu.VMEM((7, 8 * 32, 8, 128), u32),
                  pltpu.VMEM((49, 2 * W4T, 8, 128), u32))

    out_copy(0, S).wait()


def _run(x, mem0, wq, wk, wv, wo, w1, w2, w3, w4, c, wmod):
    any_spec = pl.BlockSpec(memory_space=pl.ANY)
    return pl.pallas_call(
        _kernel,
        out_shape=jax.ShapeDtypeStruct((S, D), bf16),
        in_specs=[any_spec] * 12,
        out_specs=any_spec,
        scratch_shapes=[
            pltpu.VMEM((S + 2 * RIDE, D), bf16),
            pltpu.VMEM((NGRP + 4, 8 * WP, 128), u32),
            [pltpu.VMEM((NR // 16, 96 // NRING, 8, 128), u32)] * NRING,
            pltpu.VMEM((8, 16, 128), u32),
            pltpu.VMEM((H, 16, 128), u32),
            pltpu.VMEM((2 * H, 8, 128), u32),
            pltpu.VMEM((12, 8, 512), f32),
            pltpu.VMEM((D, 128), f32),
            pltpu.VMEM((S, D), f32),
            pltpu.VMEM((7, (S - NPRE) // 2, 512), bf16),
            pltpu.VMEM((17, 64, 128), bf16),
            pltpu.VMEM((8, 32, D), bf16),
            pltpu.VMEM((7, 64, 512), bf16),
            pltpu.VMEM((2, 7, NPRE // 2, 256), bf16),
            pltpu.VMEM((49, MD // 4, 256), bf16),
            [pltpu.VMEM((40, D), f32)] * (MD // 32),
            pltpu.VMEM((1, D), bf16),
            pltpu.SemaphoreType.DMA((9 + NGRP + 2,)),
        ],
        compiler_params=pltpu.CompilerParams(vmem_limit_bytes=124 * 1024 * 1024,
                                             disable_bounds_checks=True,
                                             disable_semaphore_checks=True),
    )(x, mem0, wq, wk, wv, wo, w1, w2, w3, w4, c, wmod)


def pallas_adaLN_cond__memory_aug_recurrent_mem_tr__mixer_s_mlp__prompt_kernel(
    A_x, A_mem0, A_Wq, A_Wk, A_Wv, A_Wo, A_seg_len, B_x, B_w1, B_w2, B_w3, B_w4, c, w_mod,
):
    del B_x
    assert A_x.shape == (1, S, D) and A_mem0.shape == (1, MEM, D)
    assert not isinstance(A_seg_len, int) or A_seg_len == SEG
    out = _run(A_x.reshape(S, D), A_mem0.reshape(MEM, D), A_Wq, A_Wk, A_Wv,
               A_Wo.reshape(H * DH, D),
               B_w1.reshape(2, D // 2, D), B_w2.reshape(2, D // 2, D),
               B_w3, B_w4.reshape(4, F // 4, D), c, w_mod)
    return out.reshape(1, S, D)
```

```python
import jax
import jax.numpy as jnp
from jax import lax
import jax.experimental.pallas as pl
import jax.experimental.pallas.tpu as pltpu

bf16 = jnp.bfloat16
f32 = jnp.float32
u32 = jnp.uint32

S = 2048
D = 1024
H = 32
DH = 128
F = 3584
MEM = 8
SEG = 32
NSEG = S // SEG
L = MEM + SEG
RIDE = 24
NPRE = S - RIDE * NSEG
NR = NPRE + 2 * SEG
ROFF = (-(S - NPRE)) % NR
WP = 516
NGRP = 12
NSLOT = 6
NMOD = 6
EPS = 1e-5
MD = 256
HB = 128
GPAD = 8
NRING = 8
NWO = 3
X0 = NPRE + 2 * RIDE
W4T = 7 * 16

RLP, WLP, RSK = 27, 22, 2
SAT = {i: max(6 * (i // 2) + 11, 17) for i in range(32)}
PVAT = {i: min(6 * (i // 2) + 23, 107) for i in range(32)}
KSPLIT = 2
PIN = 6
SLOTS = ([(0, -1, 0)] * 8 + [(0, n // 2, 3 * (n % 2)) for n in range(24)]
         + [(0, 96 + n, 0) for n in range(32)])
WPP, BG, BCH = 5, 2, 2
CF, CG, CL = 0, 5, 6
DF, DG, DL = 8, 4, 4
_ONLY = None


def _loop(name, lo, hi, body, init=0):
    if _ONLY is not None and name not in _ONLY:
        return init
    with _scope(name):
        return lax.fori_loop(lo, hi, body, init)


class _NoScope:
    def __init__(self, name):
        del name

    def __enter__(self):
        return self

    def __exit__(self, *a):
        return False


_scope = _NoScope


def _zero_after(*vs):
    bits = None
    for v in vs:
        if v is not None:
            b = pltpu.bitcast(v[0:8, 0:128], u32)
            bits = b if bits is None else bits | b
    return pltpu.bitcast((bits >> 31) >> 1, f32)


def _ln(x, anchor=None):
    if anchor is not None:
        z = jnp.concatenate([anchor] * (x.shape[0] // 8), axis=0)
        x = jnp.concatenate([x[:, 0:128] + z, x[:, 128:]], axis=1)
    mu = jnp.mean(x, axis=-1, keepdims=True)
    xc = x - mu
    var = jnp.mean(xc * xc, axis=-1, keepdims=True)
    return xc * lax.rsqrt(var + EPS)


def _gelu(x):
    inner = x * (0.7978845608028654 + (0.7978845608028654 * 0.044715) * (x * x))
    hx = 0.5 * x
    return hx + hx * jnp.tanh(inner)


def _split_rows(x):
    m, n = x.shape
    x3 = x.reshape(m // 16, 16, n)
    return x3[:, 0:8, :].reshape(m // 2, n), x3[:, 8:16, :].reshape(m // 2, n)


def _merge_rows(top, bot):
    m, n = top.shape
    return jnp.concatenate([top.reshape(m // 8, 8, n), bot.reshape(m // 8, 8, n)],
                           axis=1).reshape(2 * m, n)


def _a_operands(a11, a12, a21, a22):
    return [a11 + a22, a21 + a22, a11, a22, a11 + a12, a21 - a11, a12 - a22]


def _b_operands(b11, b12, b21, b22):
    return [b11 + b22, b11, b12 - b22, b21 - b11, b22, b11 + b12, b21 + b22]


_ATERMS = ((0, 3, 1), (2, 3, 1), (0, None, 0), (3, None, 0), (0, 1, 1), (2, 0, -1), (1, 3, -1))
_BTERMS = ((0, 3, 1), (0, None, 0), (1, 3, -1), (2, 0, -1), (3, None, 0), (0, 1, 1), (2, 3, 1))


def _strassen(a_of, b_of, hook=lambda v: None):
    def prod(k):
        return jnp.dot(a_of(k), b_of(k), preferred_element_type=f32)
    p5 = prod(4)
    hook(p5)
    p3 = prod(2)
    hook(p3)
    c12 = p3 + p5
    p4 = prod(3)
    hook(p4)
    c11 = p4 - p5
    p2 = prod(1)
    hook(p2)
    c21 = p2 + p4
    c22 = p3 - p2
    p1 = prod(0)
    hook(p1)
    c11 = prod(6) + (c11 + p1)
    hook(c11)
    c22 = prod(5) + (c22 + p1)
    hook(c22)
    return c11, c12, c21, c22


def _a_operands2(b):
    sub = [_a_operands(b[i][j], b[i][2 + j], b[2 + i][j], b[2 + i][2 + j])
           for i in range(2) for j in range(2)]
    return [_a_operands(*[t[k] for t in sub]) for k in range(7)]


def _strassen2(a_of, b_of, hook=lambda v: None):
    def prod(k1):
        return _strassen(lambda k: a_of(k1, k), lambda k: b_of(k1, k), hook)

    def add(x, y):
        return [p + q for p, q in zip(x, y)]

    def sub(x, y):
        return [p - q for p, q in zip(x, y)]
    p5 = prod(4)
    p3 = prod(2)
    c12 = add(p3, p5)
    p4 = prod(3)
    c11 = sub(p4, p5)
    p2 = prod(1)
    c21 = add(p2, p4)
    c22 = sub(p3, p2)
    p1 = prod(0)
    c11 = add(add(c11, p1), prod(6))
    c22 = add(add(c22, p1), prod(5))
    cq = (c11, c12, c21, c22)
    return [[cq[2 * (i // 2) + j // 2][2 * (i % 2) + j % 2] for j in range(4)] for i in range(4)]


def _pack8(v):
    return pltpu.bitcast(v.astype(bf16), u32)


def _unpack(w):
    return pltpu.bitcast(w, bf16)


def _kernel(x_hbm, mem0_hbm, wq_hbm, wk_hbm, wv_hbm, wo_hbm, w1_hbm, w2_hbm, w3_hbm, w4_hbm,
            c_hbm, wmod_hbm, out_hbm,
            xbuf, wqkv, rings, lhs_h, lhs_o, kvm, modv, scol, h2buf, n7, ws3, wsr, t7, a7, d49,
            nrms, c_ref, sems):
    w_hbms = (wq_hbm, wk_hbm, wv_hbm)
    SMOD, SSTG = 5, 9
    sem_x, sem_out, sem_w, sem_g, sem_r = (sems.at[k] for k in range(5))

    def rget(b, tile, n):
        return jnp.concatenate([rings[b % NRING][tile + e, b // NRING] for e in range(n)], axis=0)

    def rhalf(b, tile, half):
        return rings[b % NRING][tile, b // NRING, 4 * half:4 * half + 4, :]

    def rset(b, tile, half, val):
        rings[b % NRING][tile, b // NRING, 4 * half:4 * half + 4, :] = _pack8(val)

    x_copy = pltpu.make_async_copy(x_hbm.at[pl.ds(0, X0), :], xbuf.at[pl.ds(0, X0), :], sem_x)

    def stream_copies(c):
        al, lo = ((lambda v, m: v), min) if isinstance(c, int) else (pl.multiple_of, jnp.minimum)
        c3 = lo(c, 27)
        cps = [pltpu.make_async_copy(
            w3_hbm.at[pl.ds(al(i * 256 + (c3 % 4) * 64, 64), 64),
                      pl.ds(al(j * (F // 4) + (c3 // 4) * 128, 128), 128)],
            ws3.at[4 * i + j], sem_w) for i in range(4) for j in range(4)]
        dst = X0 + 2 * RIDE * c
        return [
            pltpu.make_async_copy(w4_hbm.at[:, pl.ds(al(c3 * 32, 32), 32), :],
                                  wsr.at[pl.ds(0, 4)], sem_g),
            pltpu.make_async_copy(w1_hbm.at[:, pl.ds(al(c * 16, 16), 16), :],
                                  wsr.at[pl.ds(4, 2), pl.ds(0, 16), :], sem_g),
            pltpu.make_async_copy(w2_hbm.at[:, pl.ds(al(c * 16, 16), 16), :],
                                  wsr.at[pl.ds(4, 2), pl.ds(16, 16), :], sem_g),
            pltpu.make_async_copy(wmod_hbm.at[pl.ds(al(c * 32, 32), 32), pl.ds(5 * D, D)],
                                  wsr.at[6], sem_g),
            pltpu.make_async_copy(x_hbm.at[pl.ds(al(lo(dst, S - 2 * RIDE), 16), 2 * RIDE), :],
                                  xbuf.at[pl.ds(al(dst, 16), 2 * RIDE), :], sem_r)] + cps

    def stream_wait(c):
        for dst, sem in ((ws3.at[pl.ds(0, 16)], sem_w), (wsr.at[pl.ds(0, 7)], sem_g),
                         (xbuf.at[pl.ds(X0 + 2 * RIDE * c, 2 * RIDE), :], sem_r)):
            pltpu.make_async_copy(dst, dst, sem).wait()

    def out_copy(row, n, col, m):
        return pltpu.make_async_copy(xbuf.at[pl.ds(row, n), pl.ds(col, m)],
                                     out_hbm.at[pl.ds(row, n), pl.ds(col, m)], sem_out)

    def mod_rows(acc, w, r):
        sc = jnp.concatenate([scol[pl.ds(r, 16), :]] * (w.shape[1] // 128), axis=1)
        p = w.astype(f32) * sc
        return acc + p[0:8] + p[8:16]

    def mod_finish(acc, j):
        is_scale = jnp.logical_or(j // 2 == 1, j // 2 == 4)
        tot = jnp.sum(acc, axis=0, keepdims=True) + jnp.where(is_scale, 1.0, 0.0)
        modv[j] = jnp.broadcast_to(tot, (8, 512))

    def modrows(k, n, lo=0, hi=D):
        m = jnp.concatenate([modv[2 * k], modv[2 * k + 1]], axis=1)[:, lo:hi]
        return jnp.concatenate([m] * (n // 8), axis=0)

    def adaln_a(xv, anchor=None):
        n = xv.shape[0]
        return _ln(xv, anchor) * modrows(1, n) + modrows(0, n)

    def adaln_b(xv, anchor=None):
        n = xv.shape[0]
        return _ln(xv, anchor) * modrows(4, n) + modrows(3, n)

    def set_lhs(mem, hn):
        v = jnp.concatenate([mem, hn], axis=0)
        for c in range(8):
            for e in range(4):
                lhs_h[c, 4 * e:4 * e + 4, :] = _pack8(v[8 * e:8 * e + 8, c * 128:(c + 1) * 128])

    def row_operands(v):
        top, bot = _split_rows(v)
        k = v.shape[1] // 2
        return _a_operands(top[:, :k], top[:, k:], bot[:, :k], bot[:, k:])

    def stage_a16(r, anchor=None, dst=None):
        rr = pl.multiple_of(r, 16)
        xv = xbuf[pl.ds(rr, 16), :]
        if dst is not None:
            xv = (xv.astype(f32) + modrows(2, 16) * h2buf[pl.ds(rr, 16), :]).astype(bf16)
            xbuf[pl.ds(rr, 16), :] = xv
        h2 = adaln_b(xv.astype(f32), anchor)
        h2buf[pl.ds(rr, 16), :] = h2
        ref, ro = (n7, pl.multiple_of(rr // 2, 8)) if dst is None else dst
        ops = row_operands(_ln(h2))
        for t, op in enumerate(ops):
            ref[t, pl.ds(ro, 8), :] = op.astype(bf16)
        return ops[0]

    def prologue(stg, wos, wmodb, h7):
        def mod_copy(j):
            return pltpu.make_async_copy(wmod_hbm.at[:, pl.ds(j * 512, 512)], wmodb.at[j % NMOD],
                                         sems.at[SSTG + j + 4 if j >= 4 else SMOD + j])

        def piece_copy(g, dh):
            return pltpu.make_async_copy(
                w_hbms[g // 4].at[pl.ds(dh * 512, 512), pl.ds((g % 4) * 8, 8), :],
                stg.at[(2 * g + dh) % NSLOT], sems.at[SSTG + (g + 1 if g else dh)])

        def wo_copy(j):
            return pltpu.make_async_copy(wo_hbm.at[pl.ds(j * 512, 512), :], wos.at[j % NWO],
                                         sems.at[SSTG + j + 6])

        def group_start(g):
            for dh in range(2):
                piece_copy(g, dh).start()

        def stg_wait(slot, n, sem):
            dst = stg.at[pl.ds(slot, n)]
            pltpu.make_async_copy(dst, dst, sems.at[SSTG + sem]).wait()

        def relayout(g, slot, dh, lo_dp, n_dp):
            for u in range(n_dp):
                dp = lo_dp + u
                ev = pltpu.bitcast(stg[slot, 2 * dp].astype(f32), u32)
                od = pltpu.bitcast(stg[slot, 2 * dp + 1].astype(f32), u32)
                wqkv[g, pl.ds(dh * 256 + dp, 8, stride=WP), :] = (ev >> 16) | od

        def b_operand(g, q, k):
            def quad(i):
                r = (q + 4 * (i % 2)) * WP + (i // 2) * 256
                return _unpack(wqkv[g, r:r + 256, :])
            i, j, sign = _BTERMS[k]
            if j is None:
                return quad(i)
            u, v = quad(i).astype(f32), quad(j).astype(f32)
            return (u + v if sign > 0 else u - v).astype(bf16)

        c_copy = pltpu.make_async_copy(c_hbm, c_ref, sem_g)
        m_copy = pltpu.make_async_copy(mem0_hbm, wsr.at[7, pl.ds(0, MEM), :], sem_r)
        c_copy.start()
        m_copy.start()
        x_copy.start()
        for j in range(4):
            mod_copy(j).start()
        for g in range(3):
            group_start(g)
        def zero_body(i, _):
            r = pl.multiple_of(i * 32, 32)
            h2buf[pl.ds(S - NPRE + r, 32), :] = jnp.zeros((32, D), f32)
            wos[2, pl.ds(r, 32), :] = jnp.zeros((32, D), bf16)
            return 0
        lax.fori_loop(0, 16, zero_body, 0)
        c_copy.wait()
        m_copy.wait()
        cv = c_ref[...].astype(f32)
        sv = jnp.broadcast_to(cv * (1.0 / (1.0 + jnp.exp(-cv))), (128, D))
        for k in range(8):
            scol[k * 128:(k + 1) * 128, :] = sv[:, k * 128:(k + 1) * 128].T
        x_copy.wait()

        def ln0_body(i, _):
            r = pl.multiple_of(i * 64, 64)
            h2buf[pl.ds(r, 64), :] = _ln(xbuf[pl.ds(r, 64), :].astype(f32))
            return 0
        lax.fori_loop(0, NPRE // 64, ln0_body, 0)

        def mod0_body(j, _):
            pltpu.make_async_copy(wmodb.at[j], wmodb.at[j], sems.at[SMOD + j]).wait()

            def rows(t, accs):
                accs = list(accs)
                for k in range(16):
                    r = pl.multiple_of(t * 256 + k * 16, 16)
                    accs[k % 2] = mod_rows(accs[k % 2], wmodb[j, pl.ds(r, 16), :], r)
                return tuple(accs)
            accs = lax.fori_loop(0, 4, rows, (jnp.zeros((8, 512), f32),) * 2)
            mod_finish(accs[0] + accs[1], j)
            return 0
        _loop("mod0", 0, 4, mod0_body)

        def hpre_body(i, _):
            r = pl.multiple_of(i * 32, 32)
            hv = h2buf[pl.ds(r, 32), :] * modrows(1, 32) + modrows(0, 32)
            ro = pl.multiple_of(i * 8, 8)
            for t, op in enumerate(row_operands(hv)):
                h7[t, pl.ds(ro, 8), :] = pltpu.bitcast(op.astype(bf16), u32)
            return 0
        lax.fori_loop(0, NPRE // 32, hpre_body, 0)
        set_lhs(wsr[7, 0:MEM, :].astype(f32), adaln_a(xbuf[NPRE:NPRE + RIDE, :].astype(f32)))

        def relayout_now(g, dh):
            def rl_body(t, _):
                relayout(g, 2 * g + dh, dh, t * 32, 32)
                return 0
            lax.fori_loop(0, 8, rl_body, 0)

        for dh in range(2):
            stg_wait(dh, 1, dh)
            relayout_now(0, dh)

        grp = lambda g: [piece_copy(g, 0), piece_copy(g, 1)]
        issue = {0: [wo_copy(0)], 1: grp(3) + grp(4), 2: grp(5) + [wo_copy(1), mod_copy(4)],
                 3: grp(6) + [mod_copy(5), mod_copy(6)], 4: grp(7) + [wo_copy(2)],
                 5: grp(8) + [wo_copy(3), mod_copy(7)], 6: grp(9) + [wo_copy(4)],
                 7: grp(10) + [wo_copy(5), mod_copy(8)], 8: grp(11) + [wo_copy(6)],
                 9: [wo_copy(7), mod_copy(9)], 10: stream_copies(0)}

        def pre_iter(g, m3):

            @pl.when(g == 1)
            def _():
                stg_wait(2, 2, 2)
                relayout_now(1, 0)
                relayout_now(1, 1)

            def slots():
                m3n = jnp.where(m3 == 2, 0, m3 + 1)
                cj = jnp.maximum(g - 2, 3)
                return (m3n, 2 * jnp.where(ends, m3, m3n),
                        jnp.where(jnp.logical_or(g < 4, m3 == 0), 2, m3 - 1),
                        cj, jnp.where(cj >= NMOD, cj - NMOD, cj))

            ends = jnp.logical_or(g == 0, g == NGRP - 1)

            @pl.when(jnp.logical_not(ends))
            def _():
                stg_wait(slots()[1], 2, g + 2)

            @pl.when(g >= 4)
            def _():
                buf = wos.at[slots()[2]]
                pltpu.make_async_copy(buf, buf, sems.at[SSTG + g + 2]).wait()

            @pl.when(g >= 6)
            def _():
                buf = wmodb.at[slots()[4]]
                pltpu.make_async_copy(buf, buf, sems.at[SSTG + g + 2]).wait()

            m3n, gslot, wslot, cj, cslot = slots()
            gn = jnp.where(ends, g, g + 1)
            wj = jnp.maximum(g - 4, 0)
            wgrp, wrow = NGRP + wj // 2, (wj % 2) * 256
            for k, cps in issue.items():
                @pl.when(g == k)
                def _():
                    for cp in cps:
                        cp.start()
            wtodo = [(r, c) for r in range(16) for c in range(8)]
            todo = [(dh, dp) for dh in range(2) for dp in range(256)]
            skip = [0] * RSK
            mtodo = list(range(0, D, 16))
            macc = [jnp.zeros((8, 512), f32)]

            def hook(v):
                if mtodo:
                    acc = macc[0] + jnp.concatenate([_zero_after(v)] * 4, axis=1)
                    for r in mtodo[:3]:
                        acc = mod_rows(acc, wmodb[cslot, r:r + 16, :], r)
                    del mtodo[:3]
                    macc[0] = acc

            for q in range(4):
                def b_of(k):
                    w = b_operand(g, q, k)
                    if skip:
                        skip.pop()
                        return w
                    nw = 0 if todo else WLP
                    for dh, dp in todo[:RLP]:
                        relayout(gn, gslot + dh, dh, dp, 1)
                    del todo[:RLP]
                    for r, c in wtodo[:nw]:
                        wqkv[wgrp, pl.ds(wrow + (c * 512 + r * 16), 16), :] = pltpu.bitcast(
                            wos[wslot, r * 32:(r + 1) * 32, c * 128:(c + 1) * 128], u32)
                    del wtodo[:nw]
                    return w
                c11, c12, c21, c22 = _strassen(lambda k: pltpu.bitcast(h7[k], bf16), b_of, hook)
                for blk, y in ((q + 4, _merge_rows(c12, c22)), (q, _merge_rows(c11, c21))):
                    for e in range(NPRE // 8):
                        tile, half = divmod(((8 * e + ROFF) % NR) // 8, 2)
                        rings[blk][tile, g, 4 * half:4 * half + 4, :] = _pack8(y[8 * e:8 * e + 8])
            assert not todo and not wtodo and not mtodo
            mod_finish(macc[0], cj)
            return m3n

        _loop("pre1", 0, NGRP, pre_iter)

    pl.run_scoped(prologue,
                  pltpu.VMEM((NSLOT, 512, 8, 128), bf16),
                  pltpu.VMEM((NWO, 512, D), bf16),
                  pltpu.VMEM((NMOD, D, 512), bf16),
                  pltpu.VMEM((7, NPRE // 4, 512), u32))

    def main(w7, w49):
        scale = DH ** -0.5
        ia = lax.broadcasted_iota(jnp.int32, (32, L), 0)
        ja = lax.broadcasted_iota(jnp.int32, (32, L), 1)
        mask_a = (((ia >= 16) & (ia < 24)) | (ja >= SEG)
                  | (jnp.where(ia < 16, ia + 16, ia - 16) >= ja))
        ib = lax.broadcasted_iota(jnp.int32, (48, 56), 0)
        jb = lax.broadcasted_iota(jnp.int32, (48, 56), 1)
        own = (ib < 40) == (jb < 40)
        mask_b = own & (((jb >= 32) & (jb < 48)) | (jnp.where(jb < 40, jb, jb - 8) <= ib))
        masked = -1e9 / scale
        j8 = lax.broadcasted_iota(jnp.int32, (8, 56), 1)
        fill_b = jnp.concatenate([jnp.where(j8 < 40, masked, -3e38).astype(f32)] * 5
                                 + [jnp.where(j8 < 40, -3e38, masked).astype(f32)], axis=0)

        def softmax(sc, mask, fill):
            sc = jnp.where(mask, sc, fill)
            mx = jnp.max(sc, axis=-1, keepdims=True)
            e = jnp.exp2((sc - mx) * (scale * 1.4426950408889634))
            den = jnp.sum(e, axis=-1, keepdims=True)
            return (e * pl.reciprocal(den, approx=True)).astype(bf16)

        def ride_tiles(it, is_b):
            first = (it == 0).astype(jnp.int32)
            if is_b:
                return 3 * it + 1 - first, 0, 3 * it + 2
            return 3 * it + 1 - first, 1, 3 * it + first

        def step(it, is_b, lhs_lo, lhs_hi, jobs, pins):
            NT, TOFF = NR // 16, ROFF // 16
            sega = (4 * it + TOFF) % NT
            seg = sega + 2 if is_b else sega
            wt = [(3 * it + (NPRE // 16 + TOFF + t + is_b)) % NT for t in range(2)]
            wr = [(wt[(t + is_b) // 2], (t + is_b) % 2) for t in range(3)]
            rt, rh, rf = ride_tiles(it, is_b)
            rt, rf = (rt + TOFF) % NT, (rf + TOFF) % NT
            lhs = jnp.concatenate([lhs_lo, lhs_hi], axis=1)
            QM, P, PART = {}, {}, {}
            mrow = 0 if is_b else 4

            def wblk(b, lo, n):
                r = (b % 8) * WP + lo
                return _unpack(wqkv[b // 8, r:r + n, :])

            def qkv_lo(i):
                for m in range(3):
                    PART[(m, i)] = jnp.dot(lhs_lo, wblk(m * H + i, 0, 256), preferred_element_type=f32)

            def qkv(i):
                for m in range(3):
                    b = m * H + i
                    if (m, i) in PART:
                        y = jnp.dot(lhs_hi, wblk(b, 256, 256),
                                    preferred_element_type=f32) + PART.pop((m, i))
                    else:
                        y = jnp.dot(lhs, wblk(b, 0, 512), preferred_element_type=f32)
                    if m < 2:
                        QM[b] = y[0:MEM] + pins[b] if b in pins else y[0:MEM]
                    if m == 2 or (m == 1 and not is_b):
                        kvm[b - H, mrow:mrow + 4, :] = _pack8(y[0:MEM])
                    for t in range(3):
                        rset(b, *wr[t], y[8 + 8 * t:16 + 8 * t])
                    for job in jobs.get(3 * i + m, []):
                        job(y)
                    side(3 * i + m)

            def keys(b):
                if is_b:
                    if b in QM:
                        mix = jnp.concatenate([_pack8(QM.pop(b)), kvm[b - H, 4:8, :]], axis=0)
                    else:
                        mix = kvm[b - H]
                    return _unpack(jnp.concatenate([rget(b, seg, 2), mix, rhalf(b, sega, 0)], axis=0))
                mk = _pack8(QM.pop(b)) if b in QM else kvm[b - H, 4:8, :]
                return _unpack(jnp.concatenate([rget(b, seg, 2), mk], axis=0))

            def scores(i):
                if is_b:
                    q = [rget(i, seg, 2), _pack8(QM.pop(i)), rhalf(i, sega, 0)]
                else:
                    q = [rget(i, seg + 1, 1), _pack8(QM.pop(i)), rhalf(i, seg, 1)]
                sc = lax.dot_general(_unpack(jnp.concatenate(q, axis=0)), keys(H + i),
                                     (((1,), (1,)), ((), ())), preferred_element_type=f32)
                P[i] = softmax(sc, mask_b, fill_b) if is_b else softmax(sc, mask_a, masked)

            def pv(i):
                o = jnp.dot(P.pop(i), keys(2 * H + i), preferred_element_type=f32)
                if is_b:
                    for e in range(4):
                        rset(i, seg + e // 2, e % 2, o[8 * e:8 * e + 8])
                    rset(i, sega, 0, o[40:48])
                    lhs_o[i, 0:4, :] = _pack8(o[SEG:L])
                else:
                    for e in range(2):
                        rset(i, seg + 1, e, o[8 * e:8 * e + 8])
                    rset(i, seg, 1, o[24:32])
                    lhs_o[i, 0:4, :] = _pack8(o[16:24])
                lhs_o[i, 4:8, :] = rhalf(i, rt, rh)
                lhs_o[i, 8:16, :] = rget(i, rf, 1)

            def wo_lhs(i0, i1):
                return _unpack(jnp.concatenate([lhs_o[i] for i in range(i0, i1)], axis=1))

            def wo_dot(lo, j, k):
                w = _unpack(wqkv[NGRP + k, j * 512:(j + 1) * 512, :])
                return jnp.dot(lo, w, preferred_element_type=f32)

            def side(d):
                for i in range(H):
                    if PVAT[i] == d:
                        pv(i)
                for i in range(H):
                    if SAT[i] == d:
                        scores(i)

            if is_b:
                for h in range(KSPLIT):
                    qkv_lo(h)
            for h in range(H):
                qkv(h)
            lo = [wo_lhs(8 * k, 8 * k + 8) for k in range(3)]
            acc = []
            for j in range(8):
                y = None
                for k in range(3):
                    z = wo_dot(lo[k], j, k)
                    y = z if y is None else z + y
                    for job in jobs.get(96 + 3 * j + k, []):
                        job(y)
                    side(96 + 3 * j + k)
                acc.append(y)
            lo = wo_lhs(24, H)
            for j in range(8):
                acc[j] = wo_dot(lo, j, 3) + acc[j]
                for job in jobs.get(120 + j, []):
                    job(acc[j])
            assert not (QM or P or PART)
            return jnp.concatenate(acc[0:4], axis=1), jnp.concatenate(acc[4:8], axis=1)

        def combine(c, n, y):
            mp, k1 = divmod(n, 8)
            m, p = divmod(mp, 4)
            c3 = jnp.minimum(c, 27)
            spare = pl.ds(pl.multiple_of(8 * (c // 64), 8), 8)
            if y is None:
                pass
            elif m == 0 and k1 < 7:
                ws3[16, spare, :] = y.astype(bf16)
            else:
                wsr[7, spare, 0:128] = y.astype(bf16)
            if k1 == 7:
                dst, base, r = w7, 0, (4 * m + p) * 32 + c
                blk = [wsr[4 + i, m * 16:(m + 1) * 16, j * 512 + p * 128:j * 512 + (p + 1) * 128]
                       .astype(f32) for i in range(2) for j in range(2)]
            else:
                dst, base = w49, 7 * k1
                if m == 0:
                    r = c3 * 4 + p
                    get = lambda i, j: ws3[4 * i + j, p * 16:(p + 1) * 16, :]
                else:
                    r = W4T + (p // 2) * 56 + c3 * 2 + p % 2
                    r0, c0 = (p % 2) * 16, (p // 2) * 512
                    get = lambda i, j: wsr[(i + 2) % 4, r0:r0 + 16,
                                           j * 128 + c0:j * 128 + c0 + 128]

                def quad(q):
                    return [get(2 * (q // 2) + i, 2 * (q % 2) + j).astype(f32)
                            for i in range(2) for j in range(2)]
                qi, qj, sign = _BTERMS[k1]
                blk = quad(qi)
                if qj is not None:
                    blk = [u + v if sign > 0 else u - v for u, v in zip(blk, quad(qj))]
            for k, op in enumerate(_b_operands(*blk)):
                for e in range(2):
                    dst[base + k, r, 4 * e:4 * e + 4, :] = _pack8(op[8 * e:8 * e + 8])

        def rec_body(it, gacc):
            stream_wait(it)
            lhs_lo = _unpack(jnp.concatenate([lhs_h[c] for c in range(4)], axis=1))
            lhs_hi = _unpack(jnp.concatenate([lhs_h[c] for c in range(4, 8)], axis=1))
            ra = jnp.maximum(it - 1, 0) * (2 * RIDE)
            for u in range(2):
                s = 2 * it + u
                jobs, pins = {}, {}
                for n, (su, d, g) in enumerate(SLOTS):
                    if su == u and d < 0:
                        combine(it, n, None)
                    elif su == u:
                        jobs.setdefault(d, []).append(
                            lambda y, n=n, g=g: combine(it, n, y[8 * g:8 * g + 8]))
                r1 = pl.multiple_of(jnp.minimum(NPRE + RIDE * (s + 1), S - RIDE), 8)
                xn = xbuf[pl.ds(r1, RIDE), :].astype(f32)
                if u == 0:
                    for k in range(2):
                        rm = pl.multiple_of(it * 32 + k * 16, 16)
                        gacc = mod_rows(gacc, wsr[6, k * 16:(k + 1) * 16, :], rm)
                    hn = adaln_a(xn, _zero_after(stage_a16(ra)))
                else:
                    def refill(y):
                        for cp in stream_copies(jnp.minimum(it + 1, NSEG // 2 - 1)):
                            cp.start()
                        spare = pl.ds(pl.multiple_of(8 * (it // 64), 8), 8)
                        pins[PIN] = _zero_after(ws3[16, spare, :].astype(f32))
                    jobs.setdefault(3 * (PIN - 4) + 2, []).append(refill)
                    hn = adaln_a(xn)
                    z = _zero_after(hn[0:8], hn[8:16], hn[16:24])
                    stage_a16(ra + 32, _zero_after(stage_a16(ra + 16, z)))
                a_lo, a_hi = step(it, u, lhs_lo, lhs_hi, jobs, pins)
                a = jnp.concatenate([a_lo, a_hi], axis=1)
                if u == 0:
                    lhs_lo = jnp.concatenate([a_lo[0:MEM], hn[:, 0:512]], axis=0).astype(bf16)
                    lhs_hi = jnp.concatenate([a_hi[0:MEM], hn[:, 512:1024]], axis=0).astype(bf16)
                else:
                    set_lhs(a[0:MEM], hn)
                rt, rh, rf = ride_tiles(it, u)
                rows = [pl.ds(pl.multiple_of(16 * rt + 8 * rh, 8), 8),
                        pl.ds(pl.multiple_of(16 * rf, 16), 16)]
                xs = [xbuf[r, :].astype(f32) for r in rows]
                xbuf[rows[0], :] = (xs[0] + modrows(2, 8) * a[8:16]).astype(bf16)
                xbuf[rows[1], :] = (xs[1] + modrows(2, 16) * a[16:32]).astype(bf16)
            return gacc

        gacc = _loop("rec", 0, NSEG // 2, rec_body, jnp.zeros((8, D), f32))
        for c in range(2):
            mod_finish(gacc[:, c * 512:(c + 1) * 512], 10 + c)
        stream_wait(NSEG // 2 - 1)

        def wo_prep(i, half, k):
            o = jnp.concatenate([_unpack(rings[4 * half + h][k, i]).astype(f32)
                                 for h in range(4)], axis=1)
            for t, op in enumerate(row_operands(o)):
                a7[half, t, k * 8:(k + 1) * 8, :] = op.astype(bf16)

        def wo_chunk(i, half, inext, extra):
            todo = list(range(NPRE // 16))

            def hook(v):
                if todo:
                    for h in range(4):
                        rings[4 * (1 - half) + h][i // 64, 4] = pltpu.bitcast(v[0:8], u32)
                    n = 2 if len(todo) % WPP == 0 else 1
                    for k in todo[:n]:
                        wo_prep(inext, 1 - half, k)
                    del todo[:n]
                extra(v)

            for j in range(4):
                def b_of(k):
                    def quad(q):
                        r = (j + 4 * (q % 2)) * 512 + half * 256 + (q // 2) * 128
                        return _unpack(wqkv[NGRP + i, r:r + 128, :])
                    qi, qj, sign = _BTERMS[k]
                    if qj is None:
                        return quad(qi)
                    u, v = quad(qi).astype(f32), quad(qj).astype(f32)
                    return (u + v if sign > 0 else u - v).astype(bf16)
                c11, c12, c21, c22 = _strassen(lambda k: a7[half, k], b_of, hook)
                for c, y in ((j + 4, _merge_rows(c12, c22)), (j, _merge_rows(c11, c21))):
                    cs = slice(c * 128, (c + 1) * 128)
                    h2buf[S - NPRE:S, cs] = h2buf[S - NPRE:S, cs] + y

        for k in range(NPRE // 16):
            wo_prep(0, 0, k)

        def wo_tail(i, _):
            st = {"n": 0, "prev": None}

            def extra(v):
                n = st["n"]
                st["n"] += 1
                if n % 16 == 2 and n // 16 < 3:
                    st["prev"] = stage_a16(S - NPRE - 48 + 16 * (n // 16),
                                           _zero_after(v, st["prev"]))
            wo_chunk(i, 0, i, extra)
            wo_chunk(i, 1, jnp.minimum(i + 1, 3), extra)
            return 0
        _loop("wotail", 0, 4, wo_tail)

        def gget(c, row, n):
            return pltpu.bitcast(wqkv[c, pl.ds(row, n), :], f32)

        def gset(c, row, val):
            wqkv[c, pl.ds(row, val.shape[0]), :] = pltpu.bitcast(val, u32)

        def wop(j):
            return lambda k: _unpack(w7[k, j * 32:(j + 1) * 32].reshape(256, 128))

        zpad = jnp.zeros((GPAD, 128), f32)
        for cb in range(8):
            gset(cb, 0, zpad)
            gset(cb, GPAD + S, zpad)

        shifts = (-1, -1, 1, 1, -2, -2, 2, 2)

        def shift_piece(r, half, k):
            gs = jnp.concatenate([gget(c, r + (k * 16 + GPAD + shifts[c]), 16)
                                  for c in range(8)], axis=1)
            ro = half * (HB // 2) + k * 8
            for t, op in enumerate(row_operands(gs)):
                n7[t, ro:ro + 8, :] = op.astype(bf16)

        def gate(v, i):
            gset(0, GPAD + S + GPAD + 8 * (i // S), v[0:8])

        def b_body(i, _):
            rl = S - NPRE + i * 128
            st = {"n": 0, "prev": [None, None]}

            def hook(v):
                n = st["n"]
                st["n"] += 1
                if n % BG == 0 and n // BG < 8:
                    k = n // BG
                    st["prev"][k % BCH] = stage_a16(rl + 16 * k,
                                                    _zero_after(v, st["prev"][k % BCH]),
                                                    (t7, 8 * k))

            ro = pl.multiple_of(i * 192, 64)
            for lhs, row in ((lambda k: n7[k, pl.ds(ro, 192), :], i * 384), (lambda k: t7[k], rl)):
                rg = pl.multiple_of(GPAD + row, 8)
                for j in range(4):
                    c11, c12, c21, c22 = _strassen(lhs, wop(j), hook)
                    gset(j + 4, rg, _gelu(_merge_rows(c12, c22)))
                    gset(j, rg, _gelu(_merge_rows(c11, c21)))
            return 0
        _loop("b", 0, 4, b_body)
        for k in range(HB // 16):
            shift_piece(0, 0, k)

        def n2_norm(r, k, anchor):
            v = _ln(h2buf[pl.ds(pl.multiple_of(r + k * 16, 16), 16), :], anchor)
            nrms[k // 4][(k % 4) * 16:(k % 4) * 16 + 16, :] = v
            return v[0:8] + v[8:16]

        def n2_ops(kk, c, k1, tile, v, i):
            nrm = nrms[kk]
            nrm[pl.ds(pl.multiple_of(64 + 8 * (i // S), 8), 8), 0:128] = v[0:8]

            def quad(q):
                r0, c0 = (q // 2) * 16, (q % 2) * 512 + c * 128
                return [jnp.concatenate(
                    [nrm[32 * e + r0 + 8 * a:32 * e + r0 + 8 * a + 8, c0 + 256 * b:c0 + 256 * b + 128]
                     for e in range(2)], axis=0) for a in range(2) for b in range(2)]
            qi, qj, sign = _ATERMS[k1]
            blk = quad(qi)
            if qj is not None:
                blk = [u + w if sign > 0 else u - w for u, w in zip(blk, quad(qj))]
            for k2, op in enumerate(_a_operands(*blk)):
                for e in range(2):
                    d49[7 * k1 + k2, c, tile, 4 * e:4 * e + 4, :] = _pack8(op[8 * e:8 * e + 8])

        def n2_hook(r, tile0, nt, i, first, gap, lag, st):
            def hook(v):
                n = st["n"] - first
                st["n"] += 1
                if n >= 0 and n % gap == 0 and n // gap < 4 * nt:
                    st["prev"] = n2_norm(r, n // gap, _zero_after(v, st["prev"]))
                kk, rest = divmod(st["ops"], 14)
                if kk < nt and n >= (4 * kk + 3) * gap + lag:
                    n2_ops(kk, rest // 7, rest % 7, tile0 + kk, v, i)
                    st["ops"] += 1
            return hook

        def stage_c(i, r, half, rnext, extra):
            rr = pl.multiple_of(r, 8)
            ro = half * (HB // 2)
            cnt = [0]

            def hook(v):
                n = cnt[0]
                cnt[0] += 1
                if n % 2 == 0 and n // 2 < HB // 16:
                    gate(v, i)
                    shift_piece(rnext, 1 - half, n // 2)
                extra(v)

            for j in range(4):
                c11, c12, c21, c22 = _strassen(lambda k: n7[k, ro:ro + HB // 2, :], wop(4 + j),
                                               hook)
                for c, y in ((j + 4, _merge_rows(c12, c22)), (j, _merge_rows(c11, c21))):
                    cs = slice(c * 128, (c + 1) * 128)
                    h2buf[pl.ds(rr, HB), cs] = h2buf[pl.ds(rr, HB), cs] + y

        def c_body(i, _):
            r = pl.multiple_of(i * (2 * HB), 2 * HB)
            q = jnp.clip(i - 1, 0, MD // 64 - 1)
            st = {"n": 0, "ops": 0, "prev": None}
            extra = n2_hook(q * 64, q, 1, i, CF, CG, CL, st)
            stage_c(i, r, 0, r + HB, extra)
            stage_c(i, r + HB, 1, jnp.minimum(i + 1, S // (2 * HB) - 1) * (2 * HB), extra)
            assert st["ops"] == 14
            return 0
        _loop("c", 0, S // (2 * HB), c_body)

        def wop2(lo, n):
            return lambda k1, k: _unpack(w49[7 * k1 + k, lo:lo + n].reshape(8 * n, 128))

        def d_body(i, _):
            r = pl.multiple_of(i * MD, MD)
            rn = jnp.minimum(r + MD, S - MD)
            UW = MD // 8
            UN = 4096 // (7 * UW)

            def nl(k1, k):
                return _unpack(jnp.concatenate(
                    [d49[7 * k1 + k, c].reshape(UW, 128) for c in range(2)], axis=1))

            def ul(k1, k):
                n = 7 * k1 + k
                r0 = (n % UN) * 7 * UW
                return _unpack(jnp.concatenate(
                    [wqkv[8 + n // UN, r0 + UW * t:r0 + UW * (t + 1), :] for t in range(7)], axis=1))

            for t in range(7):
                cb = _strassen2(nl, wop2(t * 16, 16))
                ops = _a_operands2([[_gelu(row[(j + 2) % 4]) for j in range(4)] for row in cb])
                for n in [7 * k1 + k for k1 in (2, 3, 0, 4, 6, 1, 5) for k in range(7)]:
                    for e in range(MD // 32):
                        r0 = ((n % UN) * 7 + t) * UW + 4 * e
                        wqkv[8 + n // UN, r0:r0 + 4, :] = _pack8(ops[n // 7][n % 7][8 * e:8 * e + 8])
            st = {"n": 0, "ops": 0, "prev": None}
            hook = n2_hook(rn, 0, MD // 64, i, DF, DG, DL, st)
            for t in range(2):
                cb = _strassen2(ul, wop2(W4T + t * 56, 56), hook)
                for j in range(4):
                    y = jnp.concatenate([cb[q][j].reshape(MD // 32, 8, 128) for q in range(4)],
                                        axis=1).reshape(MD, 128)
                    c = j + 4 * t
                    cs = slice(c * 128, (c + 1) * 128)
                    gb = modrows(5, MD, c * 128, (c + 1) * 128)
                    o = xbuf[pl.ds(r, MD), cs].astype(f32) + gb * (h2buf[pl.ds(r, MD), cs] + y)
                    xbuf[pl.ds(r, MD), cs] = o.astype(bf16)
                    if c in (3, 5, 7):
                        out_copy(r, MD, *{3: (0, 512), 5: (512, 256), 7: (768, 256)}[c]).start()
            assert st["ops"] == 14 * (MD // 64)
            return 0
        _loop("d", 0, S // MD, d_body)

    pl.run_scoped(main,
                  pltpu.VMEM((7, 8 * 32, 8, 128), u32),
                  pltpu.VMEM((49, 2 * W4T, 8, 128), u32))

    out_copy(0, S, 0, D).wait()


def _run(x, mem0, wq, wk, wv, wo, w1, w2, w3, w4, c, wmod):
    any_spec = pl.BlockSpec(memory_space=pl.ANY)
    return pl.pallas_call(
        _kernel,
        out_shape=jax.ShapeDtypeStruct((S, D), bf16),
        in_specs=[any_spec] * 12,
        out_specs=any_spec,
        scratch_shapes=[
            pltpu.VMEM((S + 2 * RIDE, D), bf16),
            pltpu.VMEM((NGRP + 4, 8 * WP, 128), u32),
            [pltpu.VMEM((NR // 16, 96 // NRING, 8, 128), u32)] * NRING,
            pltpu.VMEM((8, 16, 128), u32),
            pltpu.VMEM((H, 16, 128), u32),
            pltpu.VMEM((2 * H, 8, 128), u32),
            pltpu.VMEM((12, 8, 512), f32),
            pltpu.VMEM((D, 128), f32),
            pltpu.VMEM((S, D), f32),
            pltpu.VMEM((7, (S - NPRE) // 2, 512), bf16),
            pltpu.VMEM((17, 64, 128), bf16),
            pltpu.VMEM((8, 32, D), bf16),
            pltpu.VMEM((7, 64, 512), bf16),
            pltpu.VMEM((2, 7, NPRE // 2, 256), bf16),
            pltpu.VMEM((49, 2, MD // 64, 8, 128), u32),
            [pltpu.VMEM((72, D), f32)] * (MD // 64),
            pltpu.VMEM((1, D), bf16),
            pltpu.SemaphoreType.DMA((9 + NGRP + 2,)),
        ],
        compiler_params=pltpu.CompilerParams(vmem_limit_bytes=126 * 1024 * 1024,
                                             disable_bounds_checks=True,
                                             disable_semaphore_checks=True),
    )(x, mem0, wq, wk, wv, wo, w1, w2, w3, w4, c, wmod)


def pallas_adaLN_cond__memory_aug_recurrent_mem_tr__mixer_s_mlp__prompt_kernel(
    A_x, A_mem0, A_Wq, A_Wk, A_Wv, A_Wo, A_seg_len, B_x, B_w1, B_w2, B_w3, B_w4, c, w_mod,
):
    del B_x
    assert A_x.shape == (1, S, D) and A_mem0.shape == (1, MEM, D)
    assert not isinstance(A_seg_len, int) or A_seg_len == SEG
    out = _run(A_x.reshape(S, D), A_mem0.reshape(MEM, D), A_Wq, A_Wk, A_Wv,
               A_Wo.reshape(H * DH, D),
               B_w1.reshape(2, D // 2, D), B_w2.reshape(2, D // 2, D),
               B_w3, B_w4.reshape(4, F // 4, D), c, w_mod)
    return out.reshape(1, S, D)
```
